```python
import jax
import jax.numpy as jnp

def _softmax(x, axis=-1):
    return jax.nn.softmax(x, axis=axis)
def _gelu(x):
    return jax.nn.gelu(x, approximate=True)
def _silu(x):
    return jax.nn.silu(x)
def _sigmoid(x):
    return jax.nn.sigmoid(x)
def _layernorm(x, axis=-1, eps=1e-5):
    m = jnp.mean(x, axis=axis, keepdims=True)
    v = jnp.var(x, axis=axis, keepdims=True)
    return (x - m) / jnp.sqrt(v + eps)
def _scatter_add(tgt, idx, src, axis=0):
    return tgt.at[idx].add(src)
def _segment_sum(src, seg, n):
    return jax.ops.segment_sum(src, seg, n)
class _Rng:
    def __init__(self, key):
        self._k = key
    def _next(self):
        self._k, sub = jax.random.split(self._k)
        return sub
    def normal(self, shape):
        return jax.random.normal(self._next(), shape, dtype=jnp.bfloat16)
    def randint(self, lo, hi, shape):
        return jax.random.randint(self._next(), shape, lo, hi, dtype=jnp.int32)
    def uniform(self, shape, lo=0.0, hi=1.0):
        return jax.random.uniform(self._next(), shape, jnp.bfloat16, lo, hi)
    def permutation(self, n):
        return jax.random.permutation(self._next(), n)


kernel_name = 'interleave_layers__spectral_gfnet__sliding_local_dilated__prompt'

def setup_inputs():
    _rng = _Rng(jax.random.key(int.from_bytes(__import__("os").urandom(4), "little")))
    _w = (lambda a: (lambda t: t.astype(jnp.bfloat16) if jnp.issubdtype(t.dtype, jnp.floating) else t)(jnp.asarray(a)))
    def _A_setup():
        B, S, D = 1, 2048, 1024
        Df = D // 2 + 1
        return {
            "x": _w((lambda *s: _rng.normal(s) * 0.05)(B, S, D)),
            "w_r": _w((lambda *s: _rng.normal(s) * 0.05)(S, Df) * 0.02),
            "w_i": _w((lambda *s: _rng.normal(s) * 0.05)(S, Df) * 0.02),
        }
    _A_in = _A_setup()

    def _B_setup():
        B, S, D = 1, 2048, 1024
        return {
            "x": _w((lambda *s: _rng.normal(s) * 0.05)(B, S, D)),
            "wqkv": _w((lambda *s: _rng.normal(s) * 0.05)(D, 3 * D)),
            "wo": _w((lambda *s: _rng.normal(s) * 0.05)(D, D)),
        }
    _B_in = _B_setup()

    return {
        "A_x": _A_in["x"],
        "A_w_r": _A_in["w_r"],
        "A_w_i": _A_in["w_i"],
        "B_x": _B_in["x"],
        "B_wqkv": _B_in["wqkv"],
        "B_wo": _B_in["wo"],
    }

def reference(A_x, A_w_r, A_w_i, B_x, B_wqkv, B_wo):
    def _A_ref(x, w_r, w_i):
        B, S, D = x.shape
        X = (lambda x, axes=(-2,-1): jnp.fft.rfft2(x.astype(jnp.float32), axes=axes))(x, axes=(-2, -1))
        W = w_r + 1j * w_i
        X = X * W
        y = (lambda x, s, axes=(-2,-1): jnp.fft.irfft2(x, s=s, axes=axes).astype(jnp.bfloat16))(X, (S, D), axes=(-2, -1))
        return y

    def _B_ref(x, wqkv, wo):
        B, S, D = x.shape
        H = 32; Dh = D // H
        W, dil = 8, 2
        qkv = (lambda x, *d: x.transpose(*d))((x @ wqkv).reshape(B, S, 3, H, Dh), 2, 0, 3, 1, 4)
        q, k, v = qkv[0], qkv[1], qkv[2]
        scale = Dh ** -0.5
        pos = jnp.arange(S)
        off = jnp.arange(W) * dil
        idx = pos[:, None] - off[None, :]
        mask = idx >= 0
        idx_c = jnp.where(mask, idx, 0).reshape(-1)
        kg = k[:, :, idx_c, :].reshape(B, H, S, W, Dh)
        vg = v[:, :, idx_c, :].reshape(B, H, S, W, Dh)
        logits = jnp.einsum("bhsd,bhswd->bhsw", q, kg) * scale
        logits = jnp.where(mask[None, None, :, :], logits, -1e9)
        attn = _softmax(logits, axis=-1)
        o = jnp.einsum("bhsw,bhswd->bhsd", attn, vg)
        return (lambda x, *d: x.transpose(*d))(o, 0, 2, 1, 3).reshape(B, S, D) @ wo

    x = A_x
    x = x + _A_ref(_layernorm(x, axis=-1), A_w_r, A_w_i)
    x = x + _B_ref(_layernorm(x, axis=-1), B_wqkv, B_wo)
    x = x + _A_ref(_layernorm(x, axis=-1), A_w_r, A_w_i)
    x = x + _B_ref(_layernorm(x, axis=-1), B_wqkv, B_wo)
    return x
```

```python
import functools

import jax
import jax.numpy as jnp
import numpy as np
from jax import lax
from jax.experimental import pallas as pl
from jax.experimental.pallas import tpu as pltpu

S, D = 2048, 1024
NT = D // 128
NC = 4
CR = S // NC
WIN = 8
HEAD_DIM = 32
EPS = 1e-5
F32, BF16, U32 = jnp.float32, jnp.bfloat16, jnp.uint32
PAIRS = ((0, 4), (1, 7), (2, 6), (3, 5))
RSQ2 = float(np.sqrt(0.5))


def _residues(r):
    return (0, 8) if r == 0 else (r, 16 - r)


def _d_matrices():
    n = np.arange(64)[:, None]
    a = np.arange(32)
    fwd = np.zeros((8, 128, 128))
    inv = np.zeros((8, 128, 128))
    for r in range(8):
        kd = np.concatenate([16 * a + p for p in _residues(r)])
        weight = np.full(64, 2.0)
        if r == 0:
            kd[0], weight[0] = D // 2, 1.0
            ph = np.exp(-2j * np.pi * n * kd[None, :] / D)
            sgn = np.where(kd % 16 == 0, 1.0, -1.0)[None, :]
            m = np.concatenate([ph, ph * sgn], axis=0)
            re, im = m.real.copy(), m.imag.copy()
            ire, iim = re.copy(), im.copy()
            im[:, 0] = 1.0
            iim[:, 0] = 1.0
        else:
            p = r if r < 4 else 16 - r
            ph = np.exp(-2j * np.pi * n * kd[None, :] / D)
            si = np.where(kd % 16 == p, 1.0, -1.0)[None, :]
            m = np.concatenate([ph, 1j * si * ph], axis=0)
            re, im = m.real, m.imag
            ire, iim = re, im
        swapped = r in (4, 7, 6, 5)
        cols = [im, re] if swapped else [re, im]
        icols = [iim * weight, ire * weight] if swapped else [ire * weight, iim * weight]
        fwd[r] = np.concatenate(cols, axis=1)
        inv[r] = np.concatenate(icols, axis=1).T / D
    return fwd, inv


def _s_matrices():
    k = np.arange(64)[:, None]
    l1 = np.arange(64)[None, :]
    idx = np.arange(128)
    order = ((idx // 8) % 2) * 64 + (idx // 16) * 8 + idx % 8
    fwd = np.zeros((32, 128, 128))
    for t in range(8):
        for e in range(4):
            g = np.exp(-2j * np.pi * (((4 * k + e) * (8 * l1 + t)) % S) / S)
            m = np.block([[g.real, -g.imag], [g.imag, g.real]])
            fwd[t * 4 + e] = m[order][:, order]
    return fwd, np.transpose(fwd, (0, 2, 1)) / S


def _side_matrices():
    l = np.arange(256)
    f = np.exp(-2j * np.pi * ((l[:, None] * l[None, :]) % 256) / 256)
    f256 = np.concatenate([f.real, f.imag], axis=1)
    t = np.arange(8)
    tw = np.exp(-2j * np.pi * t[:, None] * l[None, :] / S)
    tw = np.concatenate([tw.real, tw.imag], axis=0)
    g = np.exp(-2j * np.pi * t[:, None] * t[None, :] / 8)
    d8 = np.zeros((2, 16, 128))
    d8[0, :, :16] = np.block([[g.real, -g.imag], [g.imag, g.real]])
    d8[1, :, :16] = d8[0, :, :16].T / S
    return f256, tw, d8


def _perm_matrices():
    p = np.zeros((9, 128, 128))
    for i in range(8):
        for hh in range(4):
            for j in range(8):
                for dd in range(4):
                    p[i, hh * 32 + 4 * j + dd, dd * 32 + ((j + i) % 8) * 4 + hh] = 1.0
    for k in range(32):
        for e in range(4):
            p[8, e * 32 + k, 4 * k + e] = 1.0
    return p


@functools.lru_cache(maxsize=None)
def _constants():
    dfw, div = _d_matrices()
    sfw, siv = _s_matrices()
    f256, tw, d8 = _side_matrices()
    small = np.concatenate([dfw, div, _perm_matrices()], axis=0)
    b = lambda x: np.asarray(x, np.float32).astype(BF16)
    return dict(small=b(small), sfw=b(sfw), siv=b(siv), f256=b(f256),
                tw=np.asarray(tw, np.float32), d8=b(d8))


def _dot(a, b):
    return jnp.dot(a, b, preferred_element_type=F32)


def _dot_nt(a, b):
    return lax.dot_general(a, b, (((1,), (1,)), ((), ())), preferred_element_type=F32)


def _tree(op, xs):
    xs = list(xs)
    while len(xs) > 1:
        xs = [op(xs[i], xs[i + 1]) if i + 1 < len(xs) else xs[i] for i in range(0, len(xs), 2)]
    return xs[0]


def _chain(op, xs):
    return functools.reduce(op, xs)


def _lane(rows):
    return lax.broadcasted_iota(jnp.int32, (rows, 128), 1)


def _swap(x):
    return pltpu.roll(x, 64, 1)


def _unpack(w, i):
    return pltpu.unpack_elementwise(w, index=i, packed_dtype=BF16, unpacked_dtype=F32)


def _layernorm(xs):
    add = lambda a, b: a + b
    mean = jnp.sum(_tree(add, xs), axis=1, keepdims=True) * (1.0 / D)
    cs = [x - mean for x in xs]
    var = jnp.sum(_tree(add, [c * c for c in cs]), axis=1, keepdims=True) * (1.0 / D)
    inv = lax.rsqrt(var + EPS)
    return [c * inv for c in cs]


def _d_butterfly_fwd(a):
    lo = _lane(a[0].shape[0]) < 64
    s = [a[j] + a[j + 4] for j in range(4)]
    d = [a[j] - a[j + 4] for j in range(4)]
    e, o = s[0] + s[2], s[1] + s[3]
    p, q = (d[1] - d[3]) * RSQ2, (d[1] + d[3]) * RSQ2
    u = [None] * 8
    u[0], u[4] = e + o, e - o
    ts = {1: (d[0] + p, d[2] + q, -1.0), 2: (s[0] - s[2], s[1] - s[3], -1.0),
          3: (d[0] - p, d[2] - q, 1.0)}
    for r, (tr, ti, sg) in ts.items():
        if sg < 0:
            ti = -ti
        wr, wi = float(np.cos(np.pi * r / 8)), float(-np.sin(np.pi * r / 8))
        rr, ri = _swap(tr), _swap(ti)
        pp = jnp.where(lo, tr, ri)
        wq = jnp.where(lo, rr, ti) * wr + jnp.where(lo, ri, tr) * jnp.where(lo, -wi, wi)
        u[r], u[8 - r] = pp + wq, pp - wq
    return u


def _d_butterfly_inv(u):
    lo = _lane(u[0].shape[0]) < 64
    ts = {}
    for r in (1, 2, 3):
        wr, wi = float(np.cos(np.pi * r / 8)), float(-np.sin(np.pi * r / 8))
        pp, v = u[r] + u[8 - r], u[r] - u[8 - r]
        rp, rv = _swap(pp), _swap(v)
        ts[r] = (jnp.where(lo, pp, rv * wr + v * wi), jnp.where(lo, rp, v * wr - rv * wi))
    e, o = u[0] + u[4], u[0] - u[4]
    s = [e + ts[2][0], o - ts[2][1], e - ts[2][0], o + ts[2][1]]
    p = (ts[1][0] - ts[3][0]) * RSQ2
    q = (ts[1][1] + ts[3][1]) * RSQ2
    d = [ts[1][0] + ts[3][0], p - q, ts[3][1] - ts[1][1], -(p + q)]
    return [s[j] + d[j] for j in range(4)] + [s[j] - d[j] for j in range(4)]


def _cadd(a, b):
    return a[0] + b[0], a[1] + b[1]


def _csub(a, b):
    return a[0] - b[0], a[1] - b[1]


def _dft4(z, inverse):
    a, b = _cadd(z[0], z[2]), _csub(z[0], z[2])
    c, d = _cadd(z[1], z[3]), _csub(z[1], z[3])
    minus = (b[0] + d[1], b[1] - d[0])
    plus = (b[0] - d[1], b[1] + d[0])
    return [_cadd(a, c), plus if inverse else minus, _csub(a, c), minus if inverse else plus]


def _dft8(z, inverse):
    ev = _dft4(z[0::2], inverse)
    od = _dft4(z[1::2], inverse)
    out = [None] * 8
    out[0], out[4] = _cadd(ev[0], od[0]), _csub(ev[0], od[0])
    (er, ei), (x, y) = ev[2], od[2]
    minus, plus = (er + y, ei - x), (er - y, ei + x)
    out[2], out[6] = (plus, minus) if inverse else (minus, plus)
    for k in (1, 3):
        (er, ei), (x, y) = ev[k], od[k]
        sm, df = (x + y) * RSQ2, (x - y) * RSQ2
        if not inverse:
            if k == 1:
                out[1], out[5] = (er + sm, ei - df), (er - sm, ei + df)
            else:
                out[3], out[7] = (er - df, ei - sm), (er + df, ei + sm)
        else:
            if k == 1:
                out[1], out[5] = (er + df, ei + sm), (er - df, ei - sm)
            else:
                out[3], out[7] = (er - sm, ei + df), (er + sm, ei - df)
    return out


def _interleave(*tasks):
    state = [[g, n, 0] for g, n in tasks]
    while state:
        cur = min(state, key=lambda s: (s[2] + 0.5) / s[1])
        try:
            next(cur[0])
            cur[2] += 1
        except StopIteration:
            state.remove(cur)


def _run(*gens):
    for g in gens:
        for _ in g:
            pass


def _kernel(x_hbm, wr_hbm, wi_hbm, wr_edge, wi_edge, wqkv_hbm, wo_hbm,
            small_hbm, sfw_hbm, siv_hbm, f256_hbm, tw_ref, d8_ref,
            out_hbm,
            io, small, sfw, siv, f256, wraw, wf, wqkv_raw, wqkv, wo_raw, wo,
            xres, zin, zout, ubuf, abuf, obuf, qbuf, kbuf, vbuf, side,
            sem_x, sem_c, sem_w, sem_qkv, sem_wo, sem_out):

    def x_copies(c):
        return [pltpu.make_async_copy(x_hbm.at[:, c, :, pl.ds(j * 128, 128)], io.at[j, :, c],
                                      sem_x.at[c]) for j in range(NT)]

    def out_copies(c):
        return [pltpu.make_async_copy(io.at[j, :, c], out_hbm.at[:, c, :, pl.ds(j * 128, 128)],
                                      sem_out.at[c]) for j in range(NT)]

    const_copies = [pltpu.make_async_copy(s, d, sem_c.at[i]) for i, (s, d) in enumerate(
        ((small_hbm, small), (sfw_hbm, sfw), (siv_hbm, siv), (f256_hbm, f256)))]

    def w_copies(ri):
        src = (wr_hbm, wi_hbm)[ri]
        return [pltpu.make_async_copy(src.at[pl.ds(0, 512), pl.ds(m * 128, 128)], wraw.at[ri, m],
                                      sem_w.at[ri]) for m in range(16)]

    qkv_copies = [pltpu.make_async_copy(wqkv_hbm.at[:, pl.ds(g * D, D)], wqkv_raw.at[g],
                                        sem_qkv.at[g]) for g in range(3)]
    wo_copies = [pltpu.make_async_copy(wo_hbm.at[:, pl.ds(j * 128, 128)], wo_raw.at[j], sem_wo)
                 for j in range(NT)]

    def start(cs):
        for cp in cs:
            cp.start()

    def wait(cs):
        for cp in cs:
            cp.wait()

    io32 = io.bitcast(U32)
    wraw32 = wraw.bitcast(U32)
    wo32 = wo_raw.bitcast(U32)

    def rows(t, lb):
        return pl.ds((t * 4 + lb) * 16, 16)

    def tile(j):
        return pl.ds(j * 128, 128)

    def prep_filter():
        sub = lax.broadcasted_iota(jnp.int32, (8, 128), 0)
        for ri in range(2):
            wait(w_copies(ri))
            edge = (wr_edge, wi_edge)[ri]
            w0 = [jnp.zeros((8, 128), F32)] * 2
            for m in range(16):
                res = {}
                for i in range(8):
                    words = wraw32[ri, m, pl.ds(i, 32, stride=8), :]
                    res[2 * i], res[2 * i + 1] = _unpack(words, 0), _unpack(words, 1)
                first = res[0][0:8]
                w0[m % 2] = jnp.where(sub == m // 2, jnp.broadcast_to(first[0:1], (8, 128)), w0[m % 2])
                nyq = jnp.broadcast_to(edge[0:1, tile(m)].astype(F32), (8, 128))
                res[0] = jnp.concatenate([jnp.where(sub == 0, nyq, first), res[0][8:]], axis=0)
                for ct, (ra, rb) in enumerate(PAIRS):
                    blk = jnp.concatenate([res[p] for p in _residues(ra) + _residues(rb)], axis=0)
                    o = _dot_nt(small[24], blk.astype(BF16))
                    for e in range(4):
                        wf[ri, ct, e, m // 2, pl.ds((m % 2) * 32, 32), :] = o[e * 32:(e + 1) * 32]
                yield
            side[1, pl.ds(ri * 8, 8), :] = w0[0]
            side[1, pl.ds(16 + ri * 8, 8), :] = w0[1]

    def prep_wqkv():
        lane = _lane(8)
        pos = (lane >> 2) & 7
        for g in range(3):
            wait([qkv_copies[g]])
            for rb in range(4):
                rs = pl.ds(rb * 256, 256)
                sh = [pltpu.bitcast(_dot(wqkv_raw[g, rs, tile(i)], small[16 + i]).astype(BF16), U32)
                      for i in range(NT)]
                for b in range(16):
                    u = [sh[(-j) % 8][b * 8:(b + 1) * 8] for j in range(NT)]
                    for bit in range(3):
                        m = ((pos >> bit) & 1) == 1
                        u = [jnp.where(m, u[(j - (1 << bit)) % 8], u[j]) for j in range(NT)]
                    for j in range(NT):
                        v = u[j]
                        if j:
                            v = jnp.where(pos + j < 8, pltpu.roll(v, 128 - 4 * j, 1),
                                          pltpu.roll(v, 32 - 4 * j, 1))
                        wqkv[pl.ds(rb * 256 + b * 16, 16), tile(g * NT + j)] = pltpu.bitcast(v, BF16)
                yield

    def prep_wo():
        wait(wo_copies)
        for j in range(NT):
            for dp in range(16):
                words = wo32[j, pl.ds(dp, 32, stride=16), :]
                for i in range(2):
                    wo[pl.ds((2 * dp + i) * 32, 32), tile(j)] = _unpack(words, i).astype(BF16)
            yield

    def d_fwd_rows(t, lb, xs):
        u = _d_butterfly_fwd(_layernorm(xs))
        for r in range(8):
            ubuf[r, rows(t, lb), :] = u[r].astype(BF16)

    def d_fwd_block(c, t):
        lane = _lane(8)
        lo = lane < 64
        rs = pl.ds(t * 64, 64)
        for ct, (ra, rb) in enumerate(PAIRS):
            fa = _dot(ubuf[ra, rs, :], small[ra])
            fb = _dot(ubuf[rb, rs, :], small[rb])
            for h in range(2):
                z = []
                for lb in range(4):
                    sl = slice(lb * 16 + h * 8, lb * 16 + h * 8 + 8)
                    a, b = fa[sl], fb[sl]
                    if ct == 0:
                        ls = pl.ds(64 * lb + 16 * c + 8 * h, 8)
                        x0 = pltpu.roll(a, (t + 64) % 128, 1)
                        prev = jnp.zeros((8, 128), F32) if t == 0 else side[0, ls, :]
                        side[0, ls, :] = jnp.where(lane == t, x0, prev)
                        a = jnp.where(lane == 64, 0.0, a)
                    z.append((jnp.where(lo, a, b), _swap(jnp.where(lo, b, a))))
                for e, (re, im) in enumerate(_dft4(z, False)):
                    zin[ct, t * 4 + e, pl.ds((2 * c + h) * 16, 16), :] = (
                        jnp.concatenate([re, im], axis=0).astype(BF16))

    def load_chunk(c):
        wait(x_copies(c))
        for tp in range(4):
            for lb in range(4):
                words = [io32[j, lb, c, pl.ds(tp, 16, stride=4), :] for j in range(NT)]
                for i in range(2):
                    t = 2 * tp + i
                    xs = [_unpack(w, i) for w in words]
                    for j in range(NT):
                        xres[c, rows(t, lb), tile(j)] = xs[j]
                    d_fwd_rows(t, lb, xs)
                yield
            d_fwd_block(c, 2 * tp)
            d_fwd_block(c, 2 * tp + 1)

    def side_path():
        vt = side[0].T[0:8]
        zero8 = jnp.zeros((8, 256), F32)
        u = _dot(jnp.concatenate([vt, zero8], axis=0).astype(BF16), f256[...])[0:8]
        twr, twi = tw_ref[0:8, :], tw_ref[8:16, :]
        ur, ui = u[:, 0:256], u[:, 256:512]
        pad = jnp.zeros((112, 256), BF16)
        yield
        uu = jnp.concatenate([ur * twr - ui * twi, ur * twi + ui * twr], axis=0).astype(BF16)
        xk = _dot(d8_ref[0], jnp.concatenate([uu, pad], axis=0))
        wr = jnp.concatenate([side[1, 0:8, :], side[1, 16:24, :]], axis=1)
        wi = jnp.concatenate([side[1, 8:16, :], side[1, 24:32, :]], axis=1)
        xr, xi = xk[0:8], xk[8:16]
        yield
        yy = jnp.concatenate([xr * wr - xi * wi, xr * wi + xi * wr], axis=0).astype(BF16)
        p = _dot(d8_ref[1], jnp.concatenate([yy, pad], axis=0))
        pr, pi = p[0:8], p[8:16]
        yield
        g = jnp.concatenate([pr * twr + pi * twi, pi * twr - pr * twi], axis=1)
        g = jnp.concatenate([g, jnp.zeros((8, 512), F32)], axis=0).astype(BF16)
        y0 = _dot_nt(g, f256[...])
        side[2] = jnp.concatenate([y0, jnp.zeros((112, 256), F32)], axis=0).T
        yield

    def s_stage_fwd(ct, e):
        return [_dot(sfw[t * 4 + e], zin[ct, t * 4 + e]) for t in range(8)]

    def s_stage_filter(ct, e, y):
        parts = [[] for _ in range(8)]
        for g in range(8):
            z = [(y[t][g * 16:g * 16 + 8], y[t][g * 16 + 8:g * 16 + 16]) for t in range(8)]
            xk = _dft8(z, False)
            for k2 in range(8):
                wr = wf[0, ct, e, k2, pl.ds(g * 8, 8), :]
                wi = wf[1, ct, e, k2, pl.ds(g * 8, 8), :]
                re, im = xk[k2]
                xk[k2] = (re * wr - im * wi, re * wi + im * wr)
            for t, (re, im) in enumerate(_dft8(xk, True)):
                parts[t].append(jnp.concatenate([re, im], axis=0).astype(BF16))
        return [jnp.concatenate(p, axis=0) for p in parts]

    def s_stage():
        units = [(ct, e) for ct in range(4) for e in range(4)]
        y = s_stage_fwd(*units[0])
        for i, (ct, e) in enumerate(units):
            nxt = s_stage_fwd(*units[i + 1]) if i + 1 < len(units) else None
            f = s_stage_filter(ct, e, y)
            for t in range(8):
                zout[ct, t * 4 + e] = _dot(siv[t * 4 + e], f[t])
            y = nxt
            yield

    def d_inv_block(c, t, slot):
        lane = _lane(8)
        lo = lane < 64
        for ct, (ra, rb) in enumerate(PAIRS):
            half = [[None] * 4, [None] * 4]
            for h in range(2):
                r0 = (2 * c + h) * 16
                u = [(zout[ct, t * 4 + e, pl.ds(r0, 8), :], zout[ct, t * 4 + e, pl.ds(r0 + 8, 8), :])
                     for e in range(4)]
                for lb, (re, im) in enumerate(_dft4(u, True)):
                    sw = _swap(im)
                    a, b = jnp.where(lo, re, sw), jnp.where(lo, sw, re)
                    if ct == 0:
                        y0 = side[2, pl.ds(64 * lb + 16 * c + 8 * h, 8), :]
                        a = jnp.where(lane == 64, pltpu.roll(y0, 64 - t, 1), a)
                    half[h][lb] = (a, b)
            for lb in range(4):
                ubuf[ra, rows(t, lb), :] = jnp.concatenate(
                    [half[0][lb][0], half[1][lb][0]], axis=0).astype(BF16)
                ubuf[rb, rows(t, lb), :] = jnp.concatenate(
                    [half[0][lb][1], half[1][lb][1]], axis=0).astype(BF16)
        rs = pl.ds(t * 64, 64)
        us = [_dot(ubuf[r, rs, :], small[8 + r]) for r in range(8)]
        for lb in range(4):
            ys = _d_butterfly_inv([u[lb * 16:(lb + 1) * 16] for u in us])
            xs = [xres[c, rows(t, lb), tile(j)] + ys[j] for j in range(NT)]
            for j in range(NT):
                xres[c, rows(t, lb), tile(j)] = xs[j]
            for j, a in enumerate(_layernorm(xs)):
                abuf[slot, rows(t, lb), tile(j)] = a.astype(BF16)

    def d_inv(c, slot):
        for t in range(8):
            d_inv_block(c, t, slot)
            yield

    def qkv_proj(c, slot):
        for n in range(3 * NT):
            o = _dot(abuf[slot], wqkv[:, tile(n)])
            dst = (qbuf, kbuf, vbuf)[n // NT]
            for t in range(8):
                for lb in range(4):
                    r0 = (t * 4 + lb) * 16
                    dst[n % NT, t, pl.ds(8 + 64 * lb + 16 * c, 16), :] = o[r0:r0 + 16]
            if c == 0 and n >= NT:
                first = jnp.broadcast_to(o[0:1], (8, 128))
                for t in range(8):
                    dst[n % NT, t, pl.ds(0, 8), :] = first
            yield

    def attention(c, slot):
        scale = HEAD_DIM ** -0.5
        sub = lax.broadcasted_iota(jnp.int32, (8, 128), 0)
        add = lambda a, b: a + b
        for t in range(8):
            for lb in range(4):
                outs = []
                for h in range(2):
                    r0 = 8 + 64 * lb + 16 * c + 8 * h
                    src = [((t - 2 * w) % 8, -((t - 2 * w) // 8)) for w in range(WIN)]
                    q = [qbuf[j, t, pl.ds(r0, 8), :] for j in range(NT)]
                    logits = []
                    for ts, sh in src:
                        r = _chain(add, [q[j] * kbuf[j, ts, pl.ds(r0 - sh, 8), :] for j in range(NT)])
                        r = r + pltpu.roll(r, 64, 1)
                        r = r + pltpu.roll(r, 32, 1)
                        if c == 0 and lb == 0 and h == 0 and sh:
                            r = jnp.where(sub >= sh, r, -1e9 / scale)
                        logits.append(r)
                    m = _tree(jnp.maximum, logits)
                    ps = [jnp.exp2((r - m) * (scale * float(np.log2(np.e)))) for r in logits]
                    inv = 1.0 / _tree(add, ps)
                    outs.append([
                        _chain(add, [ps[w] * vbuf[j, ts, pl.ds(r0 - sh, 8), :]
                                     for w, (ts, sh) in enumerate(src)]) * inv
                        for j in range(NT)])
                for j in range(NT):
                    obuf[slot, rows(t, lb), tile(j)] = jnp.concatenate(
                        [outs[0][j], outs[1][j]], axis=0).astype(BF16)
                yield

    def out_proj(c, slot):
        for n in range(NT):
            xres[c, :, tile(n)] = xres[c, :, tile(n)] + _dot(obuf[slot], wo[:, tile(n)])
            yield

    def d_fwd(c):
        for t in range(8):
            for lb in range(4):
                d_fwd_rows(t, lb, [xres[c, rows(t, lb), tile(j)] for j in range(NT)])
            d_fwd_block(c, t)
            yield

    def store_chunk(c):
        for tp in range(4):
            for lb in range(4):
                for j in range(NT):
                    words = pltpu.pack_elementwise(
                        [xres[c, rows(2 * tp + i, lb), tile(j)] for i in range(2)], packed_dtype=BF16)
                    io32[j, lb, c, pl.ds(tp, 16, stride=4), :] = words.astype(U32)
            yield
            yield
        start(out_copies(c))

    def attention_block(last):
        tail = store_chunk if last else d_fwd
        _run(d_inv(0, 0))
        _interleave((qkv_proj(0, 0), 24), (d_inv(1, 1), 8))
        _interleave((qkv_proj(1, 1), 24), (d_inv(2, 0), 8))
        _interleave((qkv_proj(2, 0), 24), (d_inv(3, 1), 8), (attention(1, 0), 32))
        _interleave((qkv_proj(3, 1), 24), (attention(2, 1), 32))
        _interleave((out_proj(1, 0), 8), (attention(3, 2), 32))
        _interleave((out_proj(2, 1), 8), (attention(0, 0), 32), (tail(1), 8))
        _interleave((out_proj(3, 2), 8), (tail(2), 8))
        _interleave((out_proj(0, 0), 8), (tail(3), 8))
        _run(tail(0))

    start([const_copies[0]])
    for c in range(NC):
        start(x_copies(c))
    start(const_copies[1:2])
    start(w_copies(0))
    start(w_copies(1))
    start(const_copies[2:])
    start(qkv_copies)
    start(wo_copies)

    wait([const_copies[0]])
    for c in range(NC):
        _run(load_chunk(c))
    _run(prep_filter())
    wait(const_copies[1:])
    _interleave((s_stage(), 16), (side_path(), 4))
    _run(prep_wqkv(), prep_wo())
    attention_block(False)
    _interleave((s_stage(), 16), (side_path(), 4))
    attention_block(True)
    for c in range(NC):
        wait(out_copies(c))


@jax.jit
def pallas_interleave_layers__spectral_gfnet__sliding_local_dilated__prompt_kernel(
    A_x: jax.Array,
    A_w_r: jax.Array,
    A_w_i: jax.Array,
    B_x: jax.Array,
    B_wqkv: jax.Array,
    B_wo: jax.Array,
):
    del B_x
    assert A_x.shape == (1, S, D) and A_w_r.shape == (S, D // 2 + 1)
    cst = _constants()
    x = A_x.astype(BF16).reshape(4, NC, 128, D)
    wr, wi = A_w_r.astype(BF16).T, A_w_i.astype(BF16).T
    hbm = pl.BlockSpec(memory_space=pl.ANY)
    edge = pl.BlockSpec((16, S), lambda i: (D // 32, 0))
    vm = pltpu.VMEM
    out = pl.pallas_call(
        _kernel,
        grid=(1,),
        in_specs=[hbm, hbm, hbm, edge, edge, hbm, hbm, hbm, hbm, hbm, hbm,
                  pl.BlockSpec((16, 256), lambda i: (0, 0)),
                  pl.BlockSpec((2, 16, 128), lambda i: (0, 0, 0))],
        out_specs=hbm,
        out_shape=jax.ShapeDtypeStruct((4, NC, 128, D), BF16),
        scratch_shapes=[
            vm((NT, 4, NC, 128, 128), BF16),
            vm((25, 128, 128), BF16),
            vm((32, 128, 128), BF16),
            vm((32, 128, 128), BF16),
            vm((256, 512), BF16),
            vm((2, 16, 512, 128), BF16),
            vm((2, 4, 4, 8, 64, 128), F32),
            vm((3, D, D), BF16),
            vm((D, 3 * D), BF16),
            vm((NT, D, 128), BF16),
            vm((D, D), BF16),
            vm((NC, CR, D), F32),
            vm((4, 32, 128, 128), BF16),
            vm((4, 32, 128, 128), F32),
            vm((8, CR, 128), BF16),
            vm((2, CR, D), BF16),
            vm((3, CR, D), BF16),
            vm((NT, 8, 264, 128), F32),
            vm((NT, 8, 264, 128), F32),
            vm((NT, 8, 264, 128), F32),
            vm((3, 256, 128), F32),
            pltpu.SemaphoreType.DMA((NC,)),
            pltpu.SemaphoreType.DMA((4,)),
            pltpu.SemaphoreType.DMA((2,)),
            pltpu.SemaphoreType.DMA((3,)),
            pltpu.SemaphoreType.DMA(()),
            pltpu.SemaphoreType.DMA((NC,)),
        ],
        compiler_params=pltpu.CompilerParams(
            dimension_semantics=("arbitrary",), vmem_limit_bytes=120 * 2**20),
    )(x, wr, wi, wr, wi, B_wqkv.astype(BF16), B_wo.astype(BF16),
      cst["small"], cst["sfw"], cst["siv"], cst["f256"], cst["tw"], cst["d8"])
    return out.reshape(1, S, D)
```

```python
import functools

import jax
import jax.numpy as jnp
import numpy as np
from jax import lax
from jax.experimental import pallas as pl
from jax.experimental.pallas import tpu as pltpu

S, D = 2048, 1024
NT = D // 128
NC = 4
CR = S // NC
WIN = 8
HEAD_DIM = 32
EPS = 1e-5
F32, BF16, U32 = jnp.float32, jnp.bfloat16, jnp.uint32
PAIRS = ((0, 4), (1, 7), (2, 6), (3, 5))
RSQ2 = float(np.sqrt(0.5))
NB = 32
RING = 8
IGLAG = 4
KPACE = 1
PINS = 'bc'
NY = 4
SGLAG = 4
ATT0 = 0
GLAG = 6
XGAP = 3
AGAP = (3, 1, 1)
DGAP = 3
DLEAD = 4
STRASSEN = 1
S_LAG = 5


def _residues(r):
    return (0, 8) if r == 0 else (r, 16 - r)


def _d_matrices():
    n = np.arange(64)[:, None]
    a = np.arange(32)
    fwd = np.zeros((8, 128, 128))
    inv = np.zeros((8, 128, 128))
    for r in range(8):
        kd = np.concatenate([16 * a + p for p in _residues(r)])
        weight = np.full(64, 2.0)
        if r == 0:
            kd[0], weight[0] = D // 2, 1.0
            ph = np.exp(-2j * np.pi * n * kd[None, :] / D)
            sgn = np.where(kd % 16 == 0, 1.0, -1.0)[None, :]
            m = np.concatenate([ph, ph * sgn], axis=0)
            re, im = m.real.copy(), m.imag.copy()
            ire, iim = re.copy(), im.copy()
            im[:, 0] = 1.0
            iim[:, 0] = 1.0
        else:
            p = r if r < 4 else 16 - r
            ph = np.exp(-2j * np.pi * n * kd[None, :] / D)
            si = np.where(kd % 16 == p, 1.0, -1.0)[None, :]
            m = np.concatenate([ph, 1j * si * ph], axis=0)
            re, im = m.real, m.imag
            ire, iim = re, im
        swapped = r in (4, 7, 6, 5)
        cols = [im, re] if swapped else [re, im]
        icols = [iim * weight, ire * weight] if swapped else [ire * weight, iim * weight]
        fwd[r] = np.concatenate(cols, axis=1)
        inv[r] = np.concatenate(icols, axis=1).T / D
    return fwd, inv


def _d_wide_matrices():
    n = np.arange(128)[:, None]
    out = np.zeros((4, 2, 256, 128))
    for ct, (ra, rb) in enumerate(PAIRS):
        kd = np.concatenate([16 * np.arange(32) + p for p in _residues(ra) + _residues(rb)])
        if ct == 0:
            kd[0] = D // 2
        ph = np.exp(-2j * np.pi * n * kd[None, :] / D)
        if ct == 0:
            m = np.concatenate([ph * (kd % 8 == 0), ph * (kd % 8 == 4)], axis=0)
            m[:128, 0] += 1j
        else:
            m = np.concatenate([ph, 1j * np.where(kd % 8 == ra, 1.0, -1.0) * ph], axis=0)
        out[ct, 0], out[ct, 1] = m.real, m.imag
    return out.reshape(8, 256, 128)


def _s_matrices():
    k = np.arange(64)[:, None]
    l1 = np.arange(64)[None, :]
    idx = np.arange(128)
    grouped = ((idx // 8) % 2) * 64 + (idx // 16) * 8 + idx % 8
    packed = (idx % 2) * 64 + idx // 2
    fwd = np.zeros((32, 128, 128))
    inv = np.zeros((32, 128, 128))
    for t in range(8):
        for e in range(4):
            g = np.exp(-2j * np.pi * (((4 * k + e) * (8 * l1 + t)) % S) / S)
            m = np.block([[g.real, -g.imag], [g.imag, g.real]])
            fwd[t * 4 + e] = m[grouped][:, packed]
            inv[t * 4 + e] = m.T[:, packed] / S
    return fwd, inv


def _side_matrices():
    l = np.arange(256)
    f = np.exp(-2j * np.pi * ((l[:, None] * l[None, :]) % 256) / 256)
    f256 = np.concatenate([f.real, f.imag], axis=1)
    t = np.arange(8)
    tw = np.exp(-2j * np.pi * t[:, None] * l[None, :] / S)
    tw = np.concatenate([tw.real, tw.imag, np.zeros((8, 256))], axis=0)
    g = np.exp(-2j * np.pi * t[:, None] * t[None, :] / 8)
    d8 = np.zeros((2, 16, 128))
    d8[0, :, :16] = np.block([[g.real, -g.imag], [g.imag, g.real]])
    d8[1, :, :16] = d8[0, :, :16].T / S
    return f256, tw, d8


def _perm_matrices():
    p = np.zeros((9, 128, 128))
    for i in range(8):
        for hh in range(4):
            for j in range(8):
                for dd in range(4):
                    p[i, hh * 32 + 4 * j + dd, dd * 32 + ((j + i) % 8) * 4 + hh] = 1.0
    for k in range(32):
        for e in range(4):
            p[8, e * 32 + k, 4 * k + e] = 1.0
    return p


@functools.lru_cache(maxsize=None)
def _constants():
    dfw, div = _d_matrices()
    sfw, siv = _s_matrices()
    f256, tw, d8 = _side_matrices()
    small = np.concatenate([dfw, div, _perm_matrices()], axis=0)
    b = lambda x: np.asarray(x, np.float32).astype(BF16)
    return dict(wide=b(_d_wide_matrices()), small=b(small), sfw=b(sfw), siv=b(siv), f256=b(f256),
                tw=np.asarray(tw, np.float32), d8=b(d8))


def _dot(a, b):
    return jnp.dot(a, b, preferred_element_type=F32)


def _dot_nt(a, b):
    return lax.dot_general(a, b, (((1,), (1,)), ((), ())), preferred_element_type=F32)


def _tree(op, xs):
    xs = list(xs)
    while len(xs) > 1:
        xs = [op(xs[i], xs[i + 1]) if i + 1 < len(xs) else xs[i] for i in range(0, len(xs), 2)]
    return xs[0]


def _chain(op, xs):
    return functools.reduce(op, xs)


def _lane(rows):
    return lax.broadcasted_iota(jnp.int32, (rows, 128), 1)


def _swap(x):
    return pltpu.roll(x, 64, 1)


def _unpack(w, i):
    return pltpu.unpack_elementwise(w, index=i, packed_dtype=BF16, unpacked_dtype=F32)


def _latency():
    for _ in range(XGAP):
        yield


def _add(a, b):
    return a + b


def _row_mean(xs):
    return jnp.sum(_tree(_add, xs), axis=1, keepdims=True) * (1.0 / D)


def _twiddle16(r):
    return float(np.cos(np.pi * r / 8)), float(-np.sin(np.pi * r / 8))


def _d_butterfly_fwd(a, emit, pin, wide):
    lo = _lane(a[0].shape[0]) < 64
    s = [a[j] + a[j + 4] for j in range(4)]
    e, o = s[0] + s[2], s[1] + s[3]
    total, t4 = e + o, e - o
    emit(4, t4)
    d0, nd2 = a[0] - a[4], a[6] - a[2]
    d1, d3 = a[1] - a[5], a[3] - a[7]
    p, q = (d1 - d3) * RSQ2, (d1 + d3) * -RSQ2
    ts = {1: (d0 + p, q + nd2), 2: (s[0] - s[2], s[3] - s[1]), 3: (d0 - p, q - nd2)}
    mean8 = jnp.sum(total, axis=1, keepdims=True) * (1.0 / 128)
    if wide:
        for r, (tr, ti) in ts.items():
            emit(r, tr)
            emit(8 - r, ti)
    else:
        sw = {r: (_swap(tr), _swap(ti)) for r, (tr, ti) in ts.items()}
    dev = _tree(_add, [v * v for t in ts.values() for v in t]) * 2.0 + t4 * t4
    pin(dev)
    yield from _latency()
    t0 = total - mean8
    emit(0, t0)
    var = jnp.sum(dev + t0 * t0, axis=1, keepdims=True) * (1.0 / (NT * D))
    if not wide:
        for r, (tr, ti) in ts.items():
            wr, wi = _twiddle16(r)
            rr, ri = sw[r]
            pp = jnp.where(lo, tr, ri)
            wq = jnp.where(lo, rr, ti) * wr + jnp.where(lo, ri, tr) * jnp.where(lo, -wi, wi)
            emit(r, pp + wq)
            emit(8 - r, pp - wq)
    yield from _latency()
    return lax.rsqrt(var + EPS)


def _d_butterfly_inv(u, pin):
    lo = _lane(u[0].shape[0]) < 64
    pv = {r: (u[r] + u[8 - r], u[r] - u[8 - r]) for r in (1, 2, 3)}
    sw = {r: (_swap(p), _swap(v)) for r, (p, v) in pv.items()}
    e, o = u[0] + u[4], u[0] - u[4]
    yield from _latency()
    ts = {}
    for r, (pp, v) in pv.items():
        wr, wi = _twiddle16(r)
        rp, rv = sw[r]
        ts[r] = (jnp.where(lo, pp, rv * wr + v * wi), jnp.where(lo, rp, v * wr - rv * wi))
    s = [e + ts[2][0], o - ts[2][1], e - ts[2][0], o + ts[2][1]]
    p = (ts[1][0] - ts[3][0]) * RSQ2
    q = (ts[1][1] + ts[3][1]) * RSQ2
    d0, d1, d2, nd3 = ts[1][0] + ts[3][0], p - q, ts[3][1] - ts[1][1], p + q
    return [s[0] + d0, s[1] + d1, s[2] + d2, s[3] - nd3,
            s[0] - d0, s[1] - d1, s[2] - d2, s[3] + nd3]


def _strassen_lhs(a11, a12, a21, a22):
    return [a11 + a22, a21 + a22, a11, a22, a11 + a12, a21 - a11, a12 - a22]


def _strassen_rhs(b11, b12, b21, b22):
    return [-b11 - b22, b11, b22 - b12, b11 - b21, b22, b11 + b12, b21 + b22]


def _cadd(a, b):
    return a[0] + b[0], a[1] + b[1]


def _csub(a, b):
    return a[0] - b[0], a[1] - b[1]


def _dft4(z, inverse):
    a, b = _cadd(z[0], z[2]), _csub(z[0], z[2])
    c, d = _cadd(z[1], z[3]), _csub(z[1], z[3])
    minus = (b[0] + d[1], b[1] - d[0])
    plus = (b[0] - d[1], b[1] + d[0])
    return [_cadd(a, c), plus if inverse else minus, _csub(a, c), minus if inverse else plus]


def _dft8(z, inverse):
    ev = _dft4(z[0::2], inverse)
    od = _dft4(z[1::2], inverse)
    out = [None] * 8
    out[0], out[4] = _cadd(ev[0], od[0]), _csub(ev[0], od[0])
    (er, ei), (x, y) = ev[2], od[2]
    minus, plus = (er + y, ei - x), (er - y, ei + x)
    out[2], out[6] = (plus, minus) if inverse else (minus, plus)
    for k in (1, 3):
        (er, ei), (x, y) = ev[k], od[k]
        sm, df = (x + y) * RSQ2, (x - y) * RSQ2
        if not inverse:
            if k == 1:
                out[1], out[5] = (er + sm, ei - df), (er - sm, ei + df)
            else:
                out[3], out[7] = (er - df, ei - sm), (er + df, ei + sm)
        else:
            if k == 1:
                out[1], out[5] = (er + df, ei + sm), (er - df, ei - sm)
            else:
                out[3], out[7] = (er - sm, ei + df), (er + sm, ei - df)
    return out


class _Schedule:
    def __init__(self):
        self.pending = []

    def add(self, tick, gen):
        self.pending.append((int(tick), len(self.pending), gen))

    def run(self):
        pending = sorted(self.pending, key=lambda p: p[:2])
        active, tick, i = [], 0, 0
        while active or i < len(pending):
            while i < len(pending) and pending[i][0] <= tick:
                active.append(pending[i][2])
                i += 1
            for g in list(active):
                if next(g, 0) == 0:
                    active.remove(g)
            tick += 1
        self.pending = []


def _once(fn, *args):
    fn(*args)
    return
    yield


def _kernel(x_hbm, wr_hbm, wi_hbm, wr_edge, wi_edge, wqkv_hbm, wo_hbm,
            small_hbm, sfw_hbm, siv_hbm, f256_hbm, wide_hbm, tw_ref, d8_ref,
            out_hbm,
            io, small, sfw, siv, f256, wraw, wf, wqkv_raw, wtmp, wqkv, wo_raw, wo,
            xres, zin, zout, ybuf, fbuf, ubuf, uout, abuf, obuf, qbuf, kbuf, vbuf, side,
            wide, sem_x, sem_c, sem_w, sem_qkv, sem_wo, sem_out):

    def x_copies(c):
        return [pltpu.make_async_copy(x_hbm.at[:, c, :, pl.ds(j * 128, 128)], io.at[j, :, c],
                                      sem_x.at[c]) for j in range(NT)]

    def out_copies(c):
        return [pltpu.make_async_copy(io.at[j, :, c], out_hbm.at[:, c, :, pl.ds(j * 128, 128)],
                                      sem_out.at[c]) for j in range(NT)]

    const_copies = [pltpu.make_async_copy(s, d, sem_c.at[i]) for i, (s, d) in enumerate(
        ((wide_hbm, wide), (small_hbm.at[pl.ds(16, 9)], small.at[pl.ds(16, 9)]), (sfw_hbm, sfw),
         (f256_hbm, f256), (siv_hbm, siv), (small_hbm.at[pl.ds(0, 16)], small.at[pl.ds(0, 16)])))]
    wide_cp, perm_cp, sfw_cp, f256_cp, siv_cp, dmat_cp = ([cp] for cp in const_copies)

    def w_copies(ri):
        src = (wr_hbm, wi_hbm)[ri]
        return [pltpu.make_async_copy(src.at[pl.ds(0, 512), pl.ds(m * 128, 128)], wraw.at[ri, m],
                                      sem_w.at[ri]) for m in range(16)]

    def qkv_copies(g):
        return [pltpu.make_async_copy(wqkv_hbm.at[:, pl.ds(g * D + j * 128, 128)],
                                      wqkv_raw.at[g * NT + j], sem_qkv.at[g]) for j in range(NT)]

    wo_copies = [pltpu.make_async_copy(wo_hbm.at[:, pl.ds(j * 128, 128)], wo_raw.at[j], sem_wo)
                 for j in range(NT)]

    def start(cs):
        for cp in cs:
            cp.start()

    def wait(cs):
        for cp in cs:
            cp.wait()

    io32, wraw32, wo_raw32 = io.bitcast(U32), wraw.bitcast(U32), wo_raw.bitcast(U32)
    small32, sfw32, siv32, wide32 = (r.bitcast(U32) for r in (small, sfw, siv, wide))
    wqkv_raw32, wtmp32, wqkv32, wo32 = (r.bitcast(U32) for r in (wqkv_raw, wtmp, wqkv, wo))
    ubuf32, abuf32, obuf32 = ubuf.bitcast(U32), abuf.bitcast(U32), obuf.bitcast(U32)

    never = tw_ref[16:24, 0:128] != 0.0
    token = []

    def pin(*values):
        for v in values:
            for i in range(0, v.shape[0], 8):
                w = pltpu.bitcast(v[i:i + 8], U32)
                token[:] = [token[0] ^ w if token else w]

    clock, glag = [], [GLAG]

    def gate(v, lag=None):
        lag = lag or glag[0]
        if len(clock) < lag:
            return v
        head = jnp.where(never, pltpu.bitcast(clock[-lag], v.dtype), v[0:8])
        return head if v.shape[0] == 8 else jnp.concatenate([head, v[8:]], axis=0)

    def ticking(o):
        clock.append(o[0:8])
        del clock[:-16]
        return o

    def lhs(*tiles):
        if not token and len(tiles) == 4 and len(clock) >= 3:
            pin(clock[-3])
        if token:
            w = token.pop()
            tiles = [jnp.concatenate([jnp.where(never, w, t[0:8]), t[8:]], axis=0) for t in tiles]
        return jnp.concatenate([pltpu.bitcast(t, BF16) for t in tiles], axis=1)

    def bf(words):
        return pltpu.bitcast(words, BF16)

    def pack(a, b):
        return pltpu.bitcast(pltpu.pack_elementwise([a, b], packed_dtype=BF16), U32)

    def r16(i):
        return pl.ds(i * 16, 16)

    def put(ref, v):
        pltpu.store(ref, v, mask=jnp.ones(v.shape, jnp.bool_))

    def load_x(b, lb):
        return [xres[b, j, r16(lb), :] for j in range(NT)]

    def prep_filter(ri, m):
        sub = lax.broadcasted_iota(jnp.int32, (8, 128), 0)
        edge = (wr_edge, wi_edge)[ri]
        res = {}
        for i in range(8):
            words = wraw32[ri, m, pl.ds(i, 32, stride=8), :]
            res[2 * i], res[2 * i + 1] = _unpack(words, 0), _unpack(words, 1)
        first = res[0][0:8]
        dst = pl.ds((m % 2) * 16 + ri * 8, 8)
        prev = jnp.zeros((8, 128), F32) if m < 2 else side[1, dst, :]
        put(side.at[1, dst, :], jnp.where(sub == m // 2, jnp.broadcast_to(first[0:1], (8, 128)), prev))
        nyq = jnp.broadcast_to(edge[0:1, pl.ds(m * 128, 128)].astype(F32), (8, 128))
        res[0] = jnp.concatenate([jnp.where(sub == 0, nyq, first), res[0][8:]], axis=0)
        for ct, (ra, rb) in enumerate(PAIRS):
            blk = jnp.concatenate([res[p] for p in _residues(ra) + _residues(rb)], axis=0)
            o = _dot_nt(bf(small32[24]), blk.astype(BF16))
            for e in range(4):
                put(wf.at[ri, ct, e, m // 2, pl.ds((m % 2) * 32, 32), :], o[e * 32:(e + 1) * 32])

    def prep_wqkv_shuffle(g, rb):
        for i in range(NT):
            o = _dot(lhs(wqkv_raw32[g * NT + i, pl.ds(rb * 32, 32), :]), bf(small32[16 + i]))
            wtmp[i, pl.ds(rb * 64, 64), :] = o.astype(BF16)
            if i == 3:
                yield

    def prep_wqkv_rows(g, i8):
        pos = (_lane(8) >> 2) & 7
        halves = []
        for off in (0, 256):
            u = [wtmp32[(-j) % 8, pl.ds(off + i8 * 8, 8), :] for j in range(NT)]
            u[0], u[4] = gate(u[0]), gate(u[4])
            for bit in range(3):
                m = ((pos >> bit) & 1) == 1
                u = [jnp.where(m, u[(j - (1 << bit)) % 8], u[j]) for j in range(NT)]
            halves.append([u[0]] + [(pltpu.roll(u[j], 128 - 4 * j, 1), pltpu.roll(u[j], 32 - 4 * j, 1))
                                    for j in range(1, NT)])
            yield
        yield from _latency()
        top, bot = [[h[0]] + [jnp.where(pos + j < 8, *h[j]) for j in range(1, NT)] for h in halves]
        if STRASSEN:
            for p in range(NT // 2):
                ws = (top[2 * p], top[2 * p + 1], bot[2 * p], bot[2 * p + 1])
                ops = [_strassen_rhs(*[_unpack(w, i) for w in ws]) for i in range(2)]
                for k in range(7):
                    word = {1: ws[0], 4: ws[3]}.get(k)
                    if word is None:
                        word = pack(ops[0][k], ops[1][k])
                        pin(word)
                    put(wqkv32.at[g * 4 + p, k, pl.ds(i8 * 8, 8), :], word)
        else:
            for j in range(NT):
                pin(top[j], bot[j])
                wqkv32[g * NT + j, pl.ds(i8 * 8, 8), :] = top[j]
                wqkv32[g * NT + j, pl.ds(256 + i8 * 8, 8), :] = bot[j]

    def add_prep_wqkv(sched, tick, g, pace):
        for i in range(8):
            for half in range(2):
                sched.add(tick + (i + half / 2) * 4 * pace, prep_wqkv_shuffle(g, half * 8 + i))
        lead = 2 * pace + 5
        for i8 in range(32):
            sched.add(tick + lead + i8 * pace, prep_wqkv_rows(g, i8))
        return int(tick + lead + 31 * pace) + 3 + XGAP

    def prep_wo(p, dp):
        ws = [wo_raw32[2 * p + n, pl.ds(dp + off, 32, stride=16), :] for off in (0, 8) for n in (0, 1)]
        for i in range(2):
            b = [_unpack(w, i) for w in ws]
            r0 = (2 * dp + i) * 32
            if STRASSEN:
                for k, v in enumerate(_strassen_rhs(*b)):
                    if k not in (1, 4):
                        pin(v)
                    wo[p, k, pl.ds(r0, 32), :] = v.astype(BF16)
            else:
                for k, v in enumerate(b):
                    wo[2 * p + k % 2, pl.ds((k // 2) * 512 + r0, 32), :] = v.astype(BF16)

    def ln_stats(xs):
        lane_mean = _tree(_add, xs) * (1.0 / NT)
        lane_m2 = _tree(_add, [jnp.square(x - lane_mean) for x in xs])
        pin(lane_m2)
        mean = jnp.sum(lane_mean, axis=1, keepdims=True) * (1.0 / 128)
        yield from _latency()
        m2 = lane_m2 + jnp.square(gate(lane_mean) - mean) * float(NT)
        pin(m2)
        var = jnp.sum(m2, axis=1, keepdims=True) * (1.0 / D)
        yield from _latency()
        return mean, lax.rsqrt(gate(jnp.broadcast_to(var, (16, 128))) + EPS)

    def d_fwd_rows(b, lb, from_input=False):
        if from_input:
            c, t = divmod(b, 8)
            xs = [_unpack(io32[j, lb, c, pl.ds(t // 2, 16, stride=4), :], t % 2) for j in range(NT)]
            for j in range(NT):
                xres[b, j, r16(lb), :] = xs[j]
        else:
            xs = load_x(b, lb)

        def emit(r, v):
            pin(v)
            ubuf[b % RING, r, r16(lb), :] = v.astype(BF16)

        inv = yield from _d_butterfly_fwd([gate(x) if j < 4 else x for j, x in enumerate(xs)], emit, pin, from_input)
        inv = jnp.broadcast_to(inv, (16, 128))
        pin(inv)
        put(uout.at[b % RING, 8, r16(lb), :], inv)

    def d_dots(b, base, per_tick):
        for r in range(8):
            o = _dot(lhs(ubuf32[b % RING, r]), bf(small32[base + r]))
            put(uout.at[b % RING, r], o)
            if r % per_tick == per_tick - 1 and r < 7:
                yield

    def d_dots_wide(b):
        for ct, (ra, rb) in enumerate(PAIRS):
            u = lhs(ubuf32[b % RING, ra], ubuf32[b % RING, rb])
            for i, r in enumerate((ra, rb)):
                o = _dot(u, bf(wide32[2 * ct + i]))
                put(uout.at[b % RING, r], ticking(o) if i else o)
            if ct < 3:
                yield

    def d_fwd_cols(b, ct, is_wide):
        c, t = divmod(b, 8)
        ra, rb = PAIRS[ct]
        lane = _lane(16)
        lo = lane < 64
        z, x0 = [], []
        for lb in range(4):
            a, bb, inv = (uout[b % RING, r, r16(lb), :] for r in (ra, rb, 8))
            inv = gate(inv)
            a, bb = a * inv, bb * inv
            if is_wide:
                if ct == 0:
                    x0.append(pltpu.roll(bb, t, 1) if t else bb)
                    bb = jnp.where(lane == 0, 0.0, bb)
                z.append((a, bb))
                continue
            if ct == 0:
                x0.append(pltpu.roll(a, (t + 64) % 128, 1))
                a = jnp.where(lane == 64, 0.0, a)
            im = jnp.where(lo, bb, a)
            if 'd' in PINS:
                pin(im)
            z.append((jnp.where(lo, a, bb), _swap(im)))
        if not is_wide:
            yield from _latency()
        for e, (re, im) in enumerate(_dft4(z, False)):
            words = pack(re, im)
            pin(words)
            put(zin.at[ct, t * 4 + e, r16(c), :], words)
        if is_wide and ct == 0:
            yield from _latency()
        for lb, v in enumerate(x0):
            ls = pl.ds(64 * lb + 16 * c, 16)
            prev = jnp.zeros((16, 128), F32) if t == 0 else side[0, ls, :]
            v = jnp.where(lane == t, v, prev)
            pin(v)
            put(side.at[0, ls, :], v)

    def add_d_fwd(sched, tick, b, gap, per_tick=4, from_input=False):
        for lb in range(4):
            sched.add(tick + lb * gap, d_fwd_rows(b, lb, from_input))
        tick = int(tick + 3 * gap) + XGAP + 1
        sched.add(tick, d_dots_wide(b) if from_input else d_dots(b, 0, per_tick))
        for ct in range(4):
            sched.add(tick + 8 // per_tick + 3 + ct * gap, d_fwd_cols(b, ct, from_input))

    def side_path():
        vt = side[0].T[0:8]
        yield
        zero8 = jnp.zeros((8, 256), F32)
        u = _dot(jnp.concatenate([vt, zero8], axis=0).astype(BF16), f256[...])[0:8]
        twr, twi = tw_ref[0:8, :], tw_ref[8:16, :]
        ur, ui = u[:, 0:256], u[:, 256:512]
        pad = jnp.zeros((112, 256), BF16)
        for _ in range(4):
            yield
        uu = jnp.concatenate([ur * twr - ui * twi, ur * twi + ui * twr], axis=0).astype(BF16)
        xk = _dot(d8_ref[0], jnp.concatenate([uu, pad], axis=0))
        for _ in range(4):
            yield
        wr = jnp.concatenate([side[1, 0:8, :], side[1, 16:24, :]], axis=1)
        wi = jnp.concatenate([side[1, 8:16, :], side[1, 24:32, :]], axis=1)
        xr, xi = xk[0:8], xk[8:16]
        yy = jnp.concatenate([xr * wr - xi * wi, xr * wi + xi * wr], axis=0).astype(BF16)
        p = _dot(d8_ref[1], jnp.concatenate([yy, pad], axis=0))
        for _ in range(4):
            yield
        twr, twi = tw_ref[0:8, :], tw_ref[8:16, :]
        pr, pi = p[0:8], p[8:16]
        g = jnp.concatenate([pr * twr + pi * twi, pi * twr - pr * twi], axis=1)
        g = jnp.concatenate([g, jnp.zeros((8, 512), F32)], axis=0).astype(BF16)
        y0 = _dot_nt(g, f256[...])
        for _ in range(4):
            yield
        put(side.at[2], jnp.concatenate([y0, jnp.zeros((112, 256), F32)], axis=0).T)

    def s_fwd(u, t):
        ct, e = divmod(u, 4)
        put(ybuf.at[u % NY, t], ticking(_dot(lhs(sfw32[t * 4 + e]), bf(zin[ct, t * 4 + e]))))

    def s_filter(u, g):
        ct, e = divmod(u, 4)
        z = [tuple(ybuf[u % NY, t, pl.ds(g * 16 + i, 8), :] for i in (0, 8))
             for t in range(8)]
        z[0], z[1] = [tuple(gate(v, SGLAG) for v in zz) for zz in z[0:2]]
        xk = _dft8(z, False)
        for k2 in range(8):
            wr = wf[0, ct, e, k2, pl.ds(g * 8, 8), :]
            wi = wf[1, ct, e, k2, pl.ds(g * 8, 8), :]
            re, im = xk[k2]
            xk[k2] = (re * wr - im * wi, re * wi + im * wr)
        for t, (re, im) in enumerate(_dft8(xk, True)):
            words = pack(re, im)
            pin(words)
            put(fbuf.at[u % NY, t, pl.ds(g * 8, 8), :], words)

    def s_inv(u, t):
        ct, e = divmod(u, 4)
        put(zout.at[ct, t * 4 + e], _dot(lhs(siv32[t * 4 + e]), bf(fbuf[u % NY, t])))

    def add_s_stage(sched):
        lag = 8 + S_LAG
        for i in range(128):
            sched.add(i // 2 if i < 8 else i - 4, _once(s_fwd, *divmod(i, 8)))
            sched.add(i - 4 + lag, _once(s_filter, *divmod(i, 8)))
            sched.add((i if i < 120 else 120 + (i - 120) // 2) - 4 + lag + 9, _once(s_inv, *divmod(i, 8)))
        sched.add(4, side_path())

    def d_inv_cols(b, ct):
        c, t = divmod(b, 8)
        ra, rb = PAIRS[ct]
        lane = _lane(16)
        lo = lane < 64
        u = [(zout[ct, t * 4 + e, r16(c), :], zout[ct, t * 4 + e, r16(4 + c), :]) for e in range(4)]
        u[0], u[1] = tuple(map(gate, u[0])), tuple(map(gate, u[1]))
        z = _dft4(u, True)
        z = [(re, _swap(im)) for re, im in z]
        if ct == 0:
            y0 = [pltpu.roll(side[2, pl.ds(64 * lb + 16 * c, 16), :], 64 - t, 1) for lb in range(4)]
        yield from _latency()
        for lb, (re, sw) in enumerate(z):
            a, bb = jnp.where(lo, re, sw), jnp.where(lo, sw, re)
            if ct == 0:
                a = jnp.where(lane == 64, y0[lb], a)
            pin(a, bb)
            ubuf[b % RING, ra, r16(lb), :] = a.astype(BF16)
            ubuf[b % RING, rb, r16(lb), :] = bb.astype(BF16)

    def d_inv_rows(b, lb, stats):
        u = [uout[b % RING, r, r16(lb), :] for r in range(8)]
        ys = yield from _d_butterfly_inv([gate(v) if r < 4 else v for r, v in enumerate(u)], pin)
        xs = [x + y for x, y in zip(load_x(b, lb), ys)]
        for j in range(NT):
            put(xres.at[b, j, r16(lb), :], xs[j])
        stats[b, lb] = mean, inv = yield from ln_stats(xs)
        if not STRASSEN:
            for j, x in enumerate(load_x(b, lb)):
                v = (x - mean) * inv
                pin(v)
                abuf[b, j, r16(lb), :] = v.astype(BF16)
        elif b % 2:
            for j in range(4):
                a = [(xres[bb, j + o, r16(lb), :] - stats[bb, lb][0]) * stats[bb, lb][1]
                     for bb in (b - 1, b) for o in (0, 4)]
                for k, v in enumerate(_strassen_lhs(*a)):
                    if k not in (2, 3):
                        pin(v)
                    abuf[b // 2, k, j, r16(lb), :] = v.astype(BF16)
                if j < 3:
                    yield

    def add_d_inv(sched, tick, b, gap, stats, per_tick=4):
        for ct in range(4):
            sched.add(tick + ct * gap, d_inv_cols(b, ct))
        tick = int(tick + 3 * gap) + XGAP + 1
        sched.add(tick, d_dots(b, 8, per_tick))
        tick += 8 // per_tick + 3
        for lb in range(4):
            sched.add(tick + lb * gap, d_inv_rows(b, lb, stats))
        return int(tick + 3 * gap) + 3 * XGAP + 1 + 3 * STRASSEN

    def gemm(lhs32, rhs32, jobs, sink):
        for slot, b, n in jobs:
            if not STRASSEN:
                o = ticking(_dot(lhs(*[lhs32[slot, j] for j in range(4)]), bf(rhs32[n, pl.ds(0, 256), :])))
                yield
                sink(b, n, o + ticking(_dot(lhs(*[lhs32[slot, j] for j in range(4, 8)]),
                                            bf(rhs32[n, pl.ds(256, 256), :]))))
                yield
                continue
            m = {}
            for k in (6, 5, 0, 3, 1, 4, 2):
                m[k] = ticking(_dot(lhs(*[lhs32[slot, k, j] for j in range(4)]), bf(rhs32[n // 2, k])))
                if k == 0:
                    c11, c22 = m[6] - m[0], m[5] - m[0]
                elif k == 3:
                    c11 = c11 - m[3]
                elif k == 1:
                    sink(b + 1, n, m[1] - m[3])
                    c22 = c22 - m[1]
                elif k == 4:
                    sink(b, n, c11 - m[4])
                elif k == 2:
                    sink(b, n + 1, m[4] - m[2])
                    sink(b + 1, n + 1, c22 - m[2])
                yield

    def qkv_sink(b, n, o):
        c, t = divmod(b, 8)
        dst = (qbuf, kbuf, vbuf)[n // NT]
        for lb in range(4):
            put(dst.at[n % NT, t, pl.ds(8 + 64 * lb + 16 * c, 16), :], o[lb * 16:(lb + 1) * 16])
        if b == 0 and n >= NT:
            first = jnp.broadcast_to(o[0:1], (8, 128))
            for tt in range(8):
                dst[n % NT, tt, pl.ds(0, 8), :] = first

    def out_sink(b, n, o):
        put(xres.at[b, n], xres[b, n] + o)

    def attention(b, lb, h):
        c, t = divmod(b, 8)
        scale = HEAD_DIM ** -0.5
        r0 = 8 + 64 * lb + 16 * c + 8 * h
        src = [((t - 2 * w) % 8, -((t - 2 * w) // 8)) for w in range(WIN)]
        acc = [None] * WIN
        for j in range(NT):
            q = gate(qbuf[j, t, pl.ds(r0, 8), :])
            for w, (ts, sh) in enumerate(src):
                p = q * kbuf[j, ts, pl.ds(r0 - sh, 8), :]
                acc[w] = p if j == 0 else acc[w] + p
            if j == 3:
                pin(*acc)
                yield
        if 'e' in PINS:
            pin(*acc)
        part = [(r, pltpu.roll(r, 64, 1)) for r in acc]
        yield from _latency()
        part = [r + rr for r, rr in part]
        if 'f' in PINS:
            pin(*part)
        part = [(r, pltpu.roll(r, 32, 1)) for r in part]
        for _ in range(AGAP[0]):
            yield
        logits = [r + rr for r, rr in part]
        if r0 == 8:
            sub = lax.broadcasted_iota(jnp.int32, (8, 128), 0)
            logits = [jnp.where(sub >= sh, r, -1e9 / scale) if sh else r
                      for r, (_, sh) in zip(logits, src)]
        logits[0] = gate(logits[0])
        m = _tree(jnp.maximum, logits)
        ps = [jnp.exp2((r - m) * (scale * float(np.log2(np.e)))) for r in logits]
        total = _tree(_add, ps)
        pin(total)
        inv = pltpu.reciprocal(total, approx=True)
        inv = inv * (2.0 - total * inv)
        for j in range(NT):
            if j % 4 == 0:
                for _ in range(AGAP[1 + j // 4]):
                    yield
                ps[0] = gate(ps[0])
            o = _chain(_add, [ps[w] * vbuf[j, ts, pl.ds(r0 - sh, 8), :]
                              for w, (ts, sh) in enumerate(src)]) * inv
            pin(o)
            if STRASSEN:
                put(qbuf.at[j, t, pl.ds(r0, 8), :], o)
            else:
                obuf[b, j, pl.ds(lb * 16 + h * 8, 8), :] = o.astype(BF16)

    def out_operands(b, lb):
        c, t = divmod(b, 8)
        rs = pl.ds(8 + 64 * lb + 16 * c, 16)
        for j in range(4):
            a = [qbuf[j + o, tt, rs, :] for tt in (t, t + 1) for o in (0, 4)]
            a[0], a[3] = gate(a[0]), gate(a[3])
            for k, v in enumerate(_strassen_lhs(*a)):
                if k not in (2, 3):
                    pin(v)
                obuf[b // 2, k, j, r16(lb), :] = v.astype(BF16)
            if j == 1:
                yield

    def store_rows(b, lb):
        c, t = divmod(b, 8)
        for j in range(NT):
            words = pack(xres[b, j, r16(lb), :], xres[b + 1, j, r16(lb), :])
            pin(words)
            io32[j, lb, c, pl.ds(t // 2, 16, stride=4), :] = words

    step = 2 if STRASSEN else 1
    out_ticks = 28 if STRASSEN else 16

    def add_proj(sched, tick, c, lo, hi):
        jobs = [(b // step, b, n) for b in range(8 * c, 8 * c + 8, step) for n in range(lo, hi, step)]
        sched.add(tick, gemm(abuf32, wqkv32, jobs, qkv_sink))
        return tick + len(jobs) * out_ticks * step // NT

    def add_attention(sched, tick, interval, units):
        for i, (b, lb, h) in enumerate(units):
            sched.add(tick + i * interval, attention(b, lb, h))
            if STRASSEN and b % 2 and h:
                sched.add(int(tick + i * interval) + 2 + XGAP + sum(AGAP), out_operands(b - 1, lb))

    def add_out(sched, tick, blocks):
        sched.add(tick, gemm(obuf32, wo32, [(b // step, b, n) for b in blocks[::step]
                                            for n in range(0, NT, step)], out_sink))

    def add_tail(sched, tick, blocks, last, fast=False):
        for i, b in enumerate(blocks):
            t0 = tick + (0 if fast else i * out_ticks // step)
            if not last:
                add_d_fwd(sched, t0, b, 0 if fast else out_ticks / step / 4, 1 if fast else 4)
            elif b % 2:
                for lb in range(4):
                    sched.add(t0 + (0 if fast else 3 * lb), _once(store_rows, b - 1, lb))
                if b % 8 == 7:
                    sched.add(t0 + (1 if fast else 12), _once(start, out_copies(b // 8)))

    def units_of(blocks):
        return [(b, lb, h) for b in blocks for lb in range(4) for h in range(2)]

    q_ticks = 8 * out_ticks // step
    att_ticks = 3 + XGAP + sum(AGAP) + 3 * STRASSEN
    order = [(a + 8) % NB for a in range(NB)]

    def add_attention_block(sched, last):
        stats = {}
        t0 = max([add_d_inv(sched, 0, b, 0, stats, 1) for b in range(step)])
        if not last:
            sched.add(0, _once(wait, qkv_copies(1)))
            sched.add(0, _once(start, qkv_copies(0)))
            t0 = max(t0, add_prep_wqkv(sched, 0, 1, KPACE))
            sched.add(t0, _once(wait, qkv_copies(2)))
            sched.add(t0, _once(start, wo_copies))
            assert add_prep_wqkv(sched, t0, 2, (q_ticks - 12) / 34) <= t0 + q_ticks
            sched.add(t0 + q_ticks, _once(wait, qkv_copies(0)))
            assert add_prep_wqkv(sched, t0 + q_ticks, 0, 2 * q_ticks / 34) <= t0 + 4 * q_ticks
            sched.add(t0 + 8 * q_ticks, _once(wait, wo_copies))
            for i in range(32):
                sched.add(t0 + 8 * q_ticks + i * q_ticks / 16, _once(prep_wo, *divmod(i, 8)))
        tick, kv_start, q_start = t0, {}, {}
        for kind, c in ("k0", "k1", "q1", "k2", "q2", "k3", "q3", "q0"):
            if kind == "k":
                kv_start[int(c)] = tick
                if c == "0" and not last:
                    tick = add_proj(sched, add_proj(sched, tick, 0, NT, 2 * NT), 0, 2 * NT, 3 * NT)
                    continue
                tick = add_proj(sched, tick, int(c), NT, 3 * NT)
            else:
                q_start[int(c)] = tick
                tick = add_proj(sched, tick, int(c), 0, NT)
        pace = 2 * out_ticks / step
        for b in range(step, NB):
            due = kv_start[b // 8] + (b % 8 // step) * (2 if last or b >= 8 else 1) * out_ticks
            gap = min(1 + (b - step) * 1.0, pace / 4) if b < 18 else pace * 1.3 / 4
            at = t0 + ((b - step) * pace * 0.75 if b < 18 else
                       (18 - step) * pace * 0.75 + (b - 18) * pace * 1.3)
            if not last and b < 8:
                at, gap = max(0, t0 + (b // step - 1) * out_ticks - (step - b % step) * 8), 1
            end = add_d_inv(sched, at, b, gap, stats)
            assert end <= due, (b, end, due)
        begin = [q_start[c] + out_ticks + 3 for c in (1, 2, 3)] + [tick + ATT0]
        begin.append(tick + (NB // step - 1) * out_ticks - att_ticks)
        for i, c in enumerate((1, 2, 3, 0)):
            pace = (begin[i + 1] - begin[i]) / 64
            for t in range(8):
                first, done = begin[i] + 8 * t * pace, begin[i] + (8 * t + 7) * pace + att_ticks
                assert first >= q_start[c] + (t // step + 1) * out_ticks
                assert first >= max(kv_start[c], kv_start[(c - 1) % 4]) + 2 * q_ticks
                assert done <= tick + ((8 * i + t) // step) * out_ticks
            add_attention(sched, begin[i], pace, units_of(range(8 * c, 8 * c + 8)))
        add_out(sched, tick, order)
        add_tail(sched, tick + out_ticks + 3, order[:-step], last)
        add_tail(sched, tick + (NB // step) * out_ticks, order[-step:], last, True)

    def add_input(sched):
        glag[0] = IGLAG
        after = (x_copies(1) + x_copies(2), x_copies(3), perm_cp + w_copies(0), sfw_cp + w_copies(1))
        for c in range(NC):
            sched.add(c * 32, _once(wait, x_copies(c)))
            sched.add(c * 32, _once(start, after[c]))
            for t in range(8):
                add_d_fwd(sched, c * 32 + t * 4, c * 8 + t, 1, 2, True)

    def add_filter_prep(sched):
        after = (siv_cp + f256_cp, qkv_copies(1) + dmat_cp)
        for ri in range(2):
            sched.add(ri * 16, _once(wait, w_copies(ri) + (sfw_cp if ri else perm_cp)))
            sched.add(ri * 16, _once(start, after[ri]))
            for m in range(16):
                sched.add(ri * 16 + m, _once(prep_filter, ri, m))

    sched = _Schedule()

    def phase(fn, *args):
        fn(sched, *args)
        sched.run()
        token.clear()
        clock.clear()

    start(wide_cp + x_copies(0))
    wait(wide_cp)
    phase(add_input)
    glag[0] = GLAG
    phase(add_filter_prep)
    wait(siv_cp + f256_cp)
    start(qkv_copies(2))
    for layer in range(2):
        phase(add_s_stage)
        if layer == 0:
            wait(dmat_cp)
        phase(add_attention_block, layer == 1)
    for c in range(NC):
        wait(out_copies(c))


@jax.jit
def pallas_interleave_layers__spectral_gfnet__sliding_local_dilated__prompt_kernel(
    A_x: jax.Array,
    A_w_r: jax.Array,
    A_w_i: jax.Array,
    B_x: jax.Array,
    B_wqkv: jax.Array,
    B_wo: jax.Array,
):
    del B_x
    assert A_x.shape == (1, S, D) and A_w_r.shape == (S, D // 2 + 1)
    cst = _constants()
    x = A_x.astype(BF16).reshape(4, NC, 128, D)
    wr, wi = A_w_r.astype(BF16).T, A_w_i.astype(BF16).T
    hbm = pl.BlockSpec(memory_space=pl.ANY)
    edge = pl.BlockSpec((16, S), lambda i: (D // 32, 0))
    vm = pltpu.VMEM
    out = pl.pallas_call(
        _kernel,
        grid=(1,),
        in_specs=[hbm, hbm, hbm, edge, edge, hbm, hbm, hbm, hbm, hbm, hbm, hbm,
                  pl.BlockSpec((24, 256), lambda i: (0, 0)),
                  pl.BlockSpec((2, 16, 128), lambda i: (0, 0, 0))],
        out_specs=hbm,
        out_shape=jax.ShapeDtypeStruct((4, NC, 128, D), BF16),
        scratch_shapes=[
            vm((NT, 4, NC, 128, 128), BF16),
            vm((25, 128, 128), BF16),
            vm((32, 128, 128), BF16),
            vm((32, 128, 128), BF16),
            vm((256, 512), BF16),
            vm((2, 16, 512, 128), BF16),
            vm((2, 4, 4, 8, 64, 128), F32),
            vm((3 * NT, D, 128), BF16),
            vm((NT, D, 128), BF16),
            vm((12, 7, 512, 128) if STRASSEN else (3 * NT, D, 128), BF16),
            vm((NT, D, 128), BF16),
            vm((4, 7, 512, 128) if STRASSEN else (NT, D, 128), BF16),
            vm((NB, NT, 64, 128), F32),
            vm((4, 32, 64, 128), U32),
            vm((4, 32, 128, 128), F32),
            vm((NY, 8, 128, 128), F32),
            vm((NY, 8, 64, 128), U32),
            vm((RING, 8, 64, 128), BF16),
            vm((RING, 9, 64, 128), F32),
            vm((NB // 2, 7, 4, 64, 128) if STRASSEN else (NB, NT, 64, 128), BF16),
            vm((NB // 2, 7, 4, 64, 128) if STRASSEN else (NB, NT, 64, 128), BF16),
            vm((NT, 8, 264, 128), F32),
            vm((NT, 8, 264, 128), F32),
            vm((NT, 8, 264, 128), F32),
            vm((3, 256, 128), F32),
            vm((8, 256, 128), BF16),
            pltpu.SemaphoreType.DMA((NC,)),
            pltpu.SemaphoreType.DMA((6,)),
            pltpu.SemaphoreType.DMA((2,)),
            pltpu.SemaphoreType.DMA((3,)),
            pltpu.SemaphoreType.DMA(()),
            pltpu.SemaphoreType.DMA((NC,)),
        ],
        compiler_params=pltpu.CompilerParams(
            dimension_semantics=("arbitrary",), vmem_limit_bytes=120 * 2**20),
    )(x, wr, wi, wr, wi, B_wqkv.astype(BF16), B_wo.astype(BF16),
      cst["small"], cst["sfw"], cst["siv"], cst["f256"], cst["wide"], cst["tw"], cst["d8"])
    return out.reshape(1, S, D)
```

```python
import functools

import jax
import jax.numpy as jnp
import numpy as np
from jax import lax
from jax.experimental import pallas as pl
from jax.experimental.pallas import tpu as pltpu

S, D = 2048, 1024
NT = D // 128
NC = 4
CR = S // NC
WIN = 8
HEAD_DIM = 32
EPS = 1e-5
F32, BF16, U32 = jnp.float32, jnp.bfloat16, jnp.uint32
PAIRS = ((0, 4), (1, 7), (2, 6), (3, 5))
RSQ2 = float(np.sqrt(0.5))
NB = 32
RING = 8
IGLAG = 4
KPACE = 64
PINS = 'bcijklm'
QK = 2
PV = 2
QG = 1
PG = 4
KLEAD = 56
SGLAG2 = 3
WI0 = 112
NY = 4
SGLAG = 3
ATT0 = 0
GLAG = 4
XGAP = 3
AGAP = (3, 1, 1)
DGAP = 3.5
DPACE = 14.3
DPACE2 = 0
DB = 22
ATT1 = 90
STRASSEN = 1
S_LAG = 5


def _residues(r):
    return (0, 8) if r == 0 else (r, 16 - r)


def _d_matrices():
    n = np.arange(64)[:, None]
    a = np.arange(32)
    fwd = np.zeros((8, 128, 128))
    inv = np.zeros((8, 128, 128))
    for r in range(8):
        kd = np.concatenate([16 * a + p for p in _residues(r)])
        weight = np.full(64, 2.0)
        if r == 0:
            kd[0], weight[0] = D // 2, 1.0
            ph = np.exp(-2j * np.pi * n * kd[None, :] / D)
            sgn = np.where(kd % 16 == 0, 1.0, -1.0)[None, :]
            m = np.concatenate([ph, ph * sgn], axis=0)
            re, im = m.real.copy(), m.imag.copy()
            ire, iim = re.copy(), im.copy()
            im[:, 0] = 1.0
            iim[:, 0] = 1.0
        else:
            p = r if r < 4 else 16 - r
            ph = np.exp(-2j * np.pi * n * kd[None, :] / D)
            si = np.where(kd % 16 == p, 1.0, -1.0)[None, :]
            m = np.concatenate([ph, 1j * si * ph], axis=0)
            re, im = m.real, m.imag
            ire, iim = re, im
        swapped = r in (4, 7, 6, 5)
        cols = [im, re] if swapped else [re, im]
        icols = [iim * weight, ire * weight] if swapped else [ire * weight, iim * weight]
        fwd[r] = np.concatenate(cols, axis=1)
        inv[r] = np.concatenate(icols, axis=1).T / D
    return fwd, inv


def _d_wide_matrices():
    n = np.arange(128)[:, None]
    out = np.zeros((4, 2, 256, 128))
    for ct, (ra, rb) in enumerate(PAIRS):
        kd = np.concatenate([16 * np.arange(32) + p for p in _residues(ra) + _residues(rb)])
        if ct == 0:
            kd[0] = D // 2
        ph = np.exp(-2j * np.pi * n * kd[None, :] / D)
        if ct == 0:
            m = np.concatenate([ph * (kd % 8 == 0), ph * (kd % 8 == 4)], axis=0)
            m[:128, 0] += 1j
        else:
            m = np.concatenate([ph, 1j * np.where(kd % 8 == ra, 1.0, -1.0) * ph], axis=0)
        out[ct, 0], out[ct, 1] = m.real, m.imag
    return out.reshape(8, 256, 128)


def _s_matrices():
    k = np.arange(64)[:, None]
    l1 = np.arange(64)[None, :]
    idx = np.arange(128)
    grouped = ((idx // 8) % 2) * 64 + (idx // 16) * 8 + idx % 8
    packed = (idx % 2) * 64 + idx // 2
    fwd = np.zeros((32, 128, 128))
    inv = np.zeros((32, 128, 128))
    for t in range(8):
        for e in range(4):
            g = np.exp(-2j * np.pi * (((4 * k + e) * (8 * l1 + t)) % S) / S)
            m = np.block([[g.real, -g.imag], [g.imag, g.real]])
            fwd[t * 4 + e] = m[grouped][:, packed]
            inv[t * 4 + e] = m.T[:, packed] / S
    return fwd, inv


def _side_matrices():
    l = np.arange(256)
    f = np.exp(-2j * np.pi * ((l[:, None] * l[None, :]) % 256) / 256)
    f256 = np.concatenate([f.real, f.imag], axis=1)
    t = np.arange(8)
    tw = np.exp(-2j * np.pi * t[:, None] * l[None, :] / S)
    tw = np.concatenate([tw.real, tw.imag, np.zeros((8, 256))], axis=0)
    g = np.exp(-2j * np.pi * t[:, None] * t[None, :] / 8)
    d8 = np.zeros((2, 16, 128))
    d8[0, :, :16] = np.block([[g.real, -g.imag], [g.imag, g.real]])
    d8[1, :, :16] = d8[0, :, :16].T / S
    return f256, tw, d8


def _filter_rows():
    p = np.zeros((1, 128, 128))
    for k in range(32):
        for e in range(4):
            p[0, e * 32 + k, 4 * k + e] = 1.0
    return p


@functools.lru_cache(maxsize=None)
def _constants():
    dfw, div = _d_matrices()
    sfw, siv = _s_matrices()
    f256, tw, d8 = _side_matrices()
    small = np.concatenate([dfw, div, _filter_rows()], axis=0)
    b = lambda x: np.asarray(x, np.float32).astype(BF16)
    return dict(wide=b(_d_wide_matrices()), small=b(small), sfw=b(sfw), siv=b(siv), f256=b(f256),
                tw=np.asarray(tw, np.float32), d8=b(d8))


def _dot(a, b):
    return jnp.dot(a, b, preferred_element_type=F32)


def _dot_nt(a, b):
    return lax.dot_general(a, b, (((1,), (1,)), ((), ())), preferred_element_type=F32)


def _tree(op, xs):
    xs = list(xs)
    while len(xs) > 1:
        xs = [op(xs[i], xs[i + 1]) if i + 1 < len(xs) else xs[i] for i in range(0, len(xs), 2)]
    return xs[0]


def _chain(op, xs):
    return functools.reduce(op, xs)


def _lane(rows):
    return lax.broadcasted_iota(jnp.int32, (rows, 128), 1)


def _swap(x):
    return pltpu.roll(x, 64, 1)


def _unpack(w, i):
    return pltpu.unpack_elementwise(w, index=i, packed_dtype=BF16, unpacked_dtype=F32)


def _latency():
    for _ in range(XGAP):
        yield


def _add(a, b):
    return a + b


def _row_mean(xs):
    return jnp.sum(_tree(_add, xs), axis=1, keepdims=True) * (1.0 / D)


def _twiddle16(r):
    return float(np.cos(np.pi * r / 8)), float(-np.sin(np.pi * r / 8))


def _d_butterfly_fwd(a, emit, pin, gate, wide):
    lo = _lane(a[0].shape[0]) < 64
    s = [a[j] + a[j + 4] for j in range(4)]
    e, o = s[0] + s[2], s[1] + s[3]
    total, t4 = e + o, e - o
    emit(4, t4)
    d0, nd2 = a[0] - a[4], a[6] - a[2]
    d1, d3 = a[1] - a[5], a[3] - a[7]
    p, q = (d1 - d3) * RSQ2, (d1 + d3) * -RSQ2
    ts = {1: (d0 + p, q + nd2), 2: (s[0] - s[2], s[3] - s[1]), 3: (d0 - p, q - nd2)}
    mean8 = jnp.sum(total, axis=1, keepdims=True) * (1.0 / 128)
    if wide:
        for r, (tr, ti) in ts.items():
            emit(r, tr)
            emit(8 - r, ti)
    else:
        sw = {r: (_swap(tr), _swap(ti)) for r, (tr, ti) in ts.items()}
    dev = _tree(_add, [v * v for t in ts.values() for v in t]) * 2.0 + t4 * t4
    pin(dev)
    yield from _latency()
    t0 = total - mean8
    emit(0, t0)
    var = jnp.sum(dev + t0 * t0, axis=1, keepdims=True) * (1.0 / (NT * D))
    if not wide:
        for r, (tr, ti) in ts.items():
            wr, wi = _twiddle16(r)
            rr, ri = sw[r]
            if 'g' in PINS:
                ri = gate(ri)
            pp = jnp.where(lo, tr, ri)
            wq = jnp.where(lo, rr, ti) * wr + jnp.where(lo, ri, tr) * jnp.where(lo, -wi, wi)
            emit(r, pp + wq)
            emit(8 - r, pp - wq)
            if 'g' in PINS:
                yield
    if wide or 'g' not in PINS:
        yield from _latency()
    return lax.rsqrt(var + EPS)


def _d_butterfly_inv(u, pin, gate):
    lo = _lane(u[0].shape[0]) < 64
    pv = {r: (u[r] + u[8 - r], u[r] - u[8 - r]) for r in (1, 2, 3)}
    sw = {r: (_swap(p), _swap(v)) for r, (p, v) in pv.items()}
    e, o = u[0] + u[4], u[0] - u[4]
    yield from _latency()
    ts = {}
    for r, (pp, v) in pv.items():
        wr, wi = _twiddle16(r)
        rp, rv = sw[r]
        if 'k' in PINS:
            rv = gate(rv)
        ts[r] = (jnp.where(lo, pp, rv * wr + v * wi), jnp.where(lo, rp, v * wr - rv * wi))
    if 'i' in PINS:
        pin(*[v for t in ts.values() for v in t])
        yield
    s = [e + ts[2][0], o - ts[2][1], e - ts[2][0], o + ts[2][1]]
    p = (ts[1][0] - ts[3][0]) * RSQ2
    q = (ts[1][1] + ts[3][1]) * RSQ2
    d0, d1, d2, nd3 = ts[1][0] + ts[3][0], p - q, ts[3][1] - ts[1][1], p + q
    return [s[0] + d0, s[1] + d1, s[2] + d2, s[3] - nd3,
            s[0] - d0, s[1] - d1, s[2] - d2, s[3] + nd3]


def _strassen_lhs(a11, a12, a21, a22):
    return [a11 + a22, a21 + a22, a11, a22, a11 + a12, a21 - a11, a12 - a22]


def _strassen_rhs(b11, b12, b21, b22):
    return [-b11 - b22, b11, b22 - b12, b11 - b21, b22, b11 + b12, b21 + b22]


def _cadd(a, b):
    return a[0] + b[0], a[1] + b[1]


def _csub(a, b):
    return a[0] - b[0], a[1] - b[1]


def _dft4(z, inverse):
    a, b = _cadd(z[0], z[2]), _csub(z[0], z[2])
    c, d = _cadd(z[1], z[3]), _csub(z[1], z[3])
    minus = (b[0] + d[1], b[1] - d[0])
    plus = (b[0] - d[1], b[1] + d[0])
    return [_cadd(a, c), plus if inverse else minus, _csub(a, c), minus if inverse else plus]


def _dft8(z, inverse):
    ev = _dft4(z[0::2], inverse)
    od = _dft4(z[1::2], inverse)
    out = [None] * 8
    out[0], out[4] = _cadd(ev[0], od[0]), _csub(ev[0], od[0])
    (er, ei), (x, y) = ev[2], od[2]
    minus, plus = (er + y, ei - x), (er - y, ei + x)
    out[2], out[6] = (plus, minus) if inverse else (minus, plus)
    for k in (1, 3):
        (er, ei), (x, y) = ev[k], od[k]
        sm, df = (x + y) * RSQ2, (x - y) * RSQ2
        if not inverse:
            if k == 1:
                out[1], out[5] = (er + sm, ei - df), (er - sm, ei + df)
            else:
                out[3], out[7] = (er - df, ei - sm), (er + df, ei + sm)
        else:
            if k == 1:
                out[1], out[5] = (er + df, ei + sm), (er - df, ei - sm)
            else:
                out[3], out[7] = (er - sm, ei + df), (er + sm, ei - df)
    return out


class _Schedule:
    def __init__(self):
        self.pending = []

    def add(self, tick, gen):
        self.pending.append((int(tick), len(self.pending), gen))

    def run(self):
        pending = sorted(self.pending, key=lambda p: p[:2])
        active, tick, i = [], 0, 0
        while active or i < len(pending):
            while i < len(pending) and pending[i][0] <= tick:
                active.append(pending[i][2])
                i += 1
            for g in list(active):
                if next(g, 0) == 0:
                    active.remove(g)
            tick += 1
        self.pending = []


def _once(fn, *args):
    fn(*args)
    return
    yield


def _kernel(x_hbm, wr_hbm, wi_hbm, wr_edge, wi_edge, wqkv_hbm, wo_hbm,
            small_hbm, sfw_hbm, siv_hbm, f256_hbm, wide_hbm, tw_ref, d8_ref,
            out_hbm,
            io, small, sfw, siv, f256, wraw, wf, wqkv_raw, wtmp, wqkv, wo_raw, wo,
            xres, zin, zout, ybuf, fbuf, ubuf, uout, abuf, obuf, qbuf, kbuf, vbuf, side,
            wide, sem_x, sem_c, sem_w, sem_qkv, sem_wo, sem_out):

    def x_copies(c):
        return [pltpu.make_async_copy(x_hbm.at[:, c, :, pl.ds(j * 128, 128)], io.at[j, :, c],
                                      sem_x.at[c]) for j in range(NT)]

    def out_copies(c):
        return [pltpu.make_async_copy(io.at[j, :, c], out_hbm.at[:, c, :, pl.ds(j * 128, 128)],
                                      sem_out.at[c]) for j in range(NT)]

    const_copies = [pltpu.make_async_copy(s, d, sem_c.at[i]) for i, (s, d) in enumerate(
        ((wide_hbm, wide), (small_hbm.at[pl.ds(16, 1)], small.at[pl.ds(16, 1)]), (sfw_hbm, sfw),
         (f256_hbm, f256), (siv_hbm, siv), (small_hbm.at[pl.ds(0, 16)], small.at[pl.ds(0, 16)])))]
    wide_cp, perm_cp, sfw_cp, f256_cp, siv_cp, dmat_cp = ([cp] for cp in const_copies)

    def w_copies(g):
        src = (wr_hbm, wi_hbm)[g // 4]
        return [pltpu.make_async_copy(src.at[pl.ds(0, 512), pl.ds(m * 128, 128)], wraw.at[g // 4, m],
                                      sem_w.at[g]) for m in range(g % 4 * 4, g % 4 * 4 + 4)]

    def qkv_copies(g):
        return [pltpu.make_async_copy(wqkv_hbm.at[:, pl.ds(g * D + j * 128, 128)],
                                      wqkv_raw.at[g * NT + j], sem_qkv.at[g]) for j in range(NT)]

    wo_copies = [pltpu.make_async_copy(wo_hbm.at[:, pl.ds(j * 128, 128)], wo_raw.at[j], sem_wo)
                 for j in range(NT)]

    def start(cs):
        for cp in cs:
            cp.start()

    def wait(cs):
        for cp in cs:
            cp.wait()

    io32, wraw32, wo_raw32 = io.bitcast(U32), wraw.bitcast(U32), wo_raw.bitcast(U32)
    small32, sfw32, siv32, wide32 = (r.bitcast(U32) for r in (small, sfw, siv, wide))
    wqkv_raw32, wqkv32, wo32 = (r.bitcast(U32) for r in (wqkv_raw, wqkv, wo))
    ubuf32, abuf32, obuf32 = ubuf.bitcast(U32), abuf.bitcast(U32), obuf.bitcast(U32)

    never = tw_ref[16:24, 0:128] != 0.0
    token = []

    def pin(*values):
        for v in values:
            for i in range(0, v.shape[0], 8):
                w = pltpu.bitcast(v[i:i + 8], U32)
                token[:] = [token[0] ^ w if token else w]

    clock, glag = [], [GLAG]

    def gate(v, lag=None):
        lag = lag or glag[0]
        if len(clock) < lag:
            return v
        head = jnp.where(never, pltpu.bitcast(clock[-lag], v.dtype), v[0:8])
        return head if v.shape[0] == 8 else jnp.concatenate([head, v[8:]], axis=0)

    def ticking(o):
        clock.append(o[0:8])
        del clock[:-16]
        return o

    def lhs(*tiles):
        if not token and len(tiles) == 4 and len(clock) >= 3:
            pin(clock[-3])
        if token:
            w = token.pop()
            tiles = [jnp.concatenate([jnp.where(never, w, t[0:8]), t[8:]], axis=0) for t in tiles]
        return jnp.concatenate([pltpu.bitcast(t, BF16) for t in tiles], axis=1)

    def bf(words):
        return pltpu.bitcast(words, BF16)

    def pack(a, b):
        return pltpu.bitcast(pltpu.pack_elementwise([a, b], packed_dtype=BF16), U32)

    def r16(i):
        return pl.ds(i * 16, 16)

    def put(ref, v):
        pltpu.store(ref, v, mask=jnp.ones(v.shape, jnp.bool_))

    def load_x(b, lb):
        return [xres[b, j, r16(lb), :] for j in range(NT)]

    def prep_filter(ri, m):
        sub = lax.broadcasted_iota(jnp.int32, (8, 128), 0)
        edge = (wr_edge, wi_edge)[ri]
        res = {}
        for i in range(8):
            words = wraw32[ri, m, pl.ds(i, 32, stride=8), :]
            res[2 * i], res[2 * i + 1] = _unpack(words, 0), _unpack(words, 1)
        first = res[0][0:8]
        dst = pl.ds((m % 2) * 16 + ri * 8, 8)
        prev = jnp.zeros((8, 128), F32) if m < 2 else side[1, dst, :]
        put(side.at[1, dst, :], jnp.where(sub == m // 2, jnp.broadcast_to(first[0:1], (8, 128)), prev))
        nyq = jnp.broadcast_to(edge[0:1, pl.ds(m * 128, 128)].astype(F32), (8, 128))
        res[0] = jnp.concatenate([jnp.where(sub == 0, nyq, first), res[0][8:]], axis=0)
        for ct, (ra, rb) in enumerate(PAIRS):
            blk = jnp.concatenate([res[p] for p in _residues(ra) + _residues(rb)], axis=0)
            o = _dot_nt(bf(small32[16]), blk.astype(BF16))
            for e in range(4):
                put(wf.at[ri, ct, e, m // 2, pl.ds((m % 2) * 32, 32), :], o[e * 32:(e + 1) * 32])

    def shuffle(words, index):
        return jnp.take_along_axis(words, index, axis=1)

    def prep_wqkv_tile(g, i, part):
        lane = _lane(8)
        index = (lane & 3) * 32 + (((lane >> 2) - i) & 7) * 4 + (lane >> 5)
        rows = [pl.ds((part * 16 + r) * 8, 8) for r in range(16)]
        ws = [shuffle(gate(wqkv_raw32[g * NT + i, rs, :]), index) for rs in rows]
        yield from _latency()
        for rs, w in zip(rows, ws):
            pin(w)
            put(wtmp.at[i, rs, :], w)

    def prep_wqkv_cross(g, r):
        pos = (_lane(8) >> 2) & 7
        u = [wtmp[(-j) % 8, pl.ds(r * 8, 8), :] for j in range(NT)]
        u[0], u[4] = gate(u[0]), gate(u[4])
        for bit in range(3):
            m = ((pos >> bit) & 1) == 1
            u = [jnp.where(m, u[(j - (1 << bit)) % 8], u[j]) for j in range(NT)]
        for j in range(NT):
            pin(u[j])
            put(wqkv_raw32.at[g * NT + j, pl.ds(r * 8, 8), :], u[j])

    def prep_wqkv_pair(g, p, part):
        lane = _lane(8)
        ws = {}
        for n in range(2):
            index = (lane & 96) | ((lane + 4 * (2 * p + n)) & 31)
            for half in range(2):
                for r in range(part * 2, part * 2 + 2):
                    w = gate(wqkv_raw32[g * NT + 2 * p + n, pl.ds(half * 256 + r * 8, 8), :])
                    ws[r, half, n] = shuffle(w, index) if p + n else w
        yield from _latency()
        for r in range(part * 2, part * 2 + 2):
            quad = [ws[r, half, n] for half in range(2) for n in range(2)]
            if STRASSEN:
                ops = [_strassen_rhs(*[_unpack(w, i) for w in quad]) for i in range(2)]
                for k in range(7):
                    word = {1: quad[0], 4: quad[3]}.get(k)
                    if word is None:
                        word = pack(ops[0][k], ops[1][k])
                        pin(word)
                    put(wqkv32.at[g * 4 + p, k, pl.ds(r * 8, 8), :], word)
            else:
                for k, w in enumerate(quad):
                    pin(w)
                    put(wqkv32.at[g * NT + 2 * p + k % 2, pl.ds((k // 2) * 256 + r * 8, 8), :], w)

    def add_prep_wqkv(sched, tick, g, ticks):
        for i in range(32):
            sched.add(tick + i * ticks / 128, prep_wqkv_tile(g, *divmod(i, 4)))
        tick = int(tick + ticks / 4) + XGAP + 1
        for r in range(64):
            sched.add(tick + r * ticks / 256, _once(prep_wqkv_cross, g, r))
        tick = int(tick + ticks / 4) + 1
        for i in range(64):
            sched.add(tick + i * ticks / 128, prep_wqkv_pair(g, *divmod(i, 16)))
        return int(tick + ticks / 2) + XGAP + 1

    def prep_wo(p, dp):
        ws = [wo_raw32[2 * p + n, pl.ds(dp + off, 32, stride=16), :] for off in (0, 8) for n in (0, 1)]
        for i in range(2):
            b = [_unpack(w, i) for w in ws]
            r0 = (2 * dp + i) * 32
            if STRASSEN:
                for k, v in enumerate(_strassen_rhs(*b)):
                    if k not in (1, 4):
                        pin(v)
                    wo[p, k, pl.ds(r0, 32), :] = v.astype(BF16)
            else:
                for k, v in enumerate(b):
                    wo[2 * p + k % 2, pl.ds((k // 2) * 512 + r0, 32), :] = v.astype(BF16)

    def ln_stats(xs):
        lane_mean = _tree(_add, xs) * (1.0 / NT)
        lane_m2 = _tree(_add, [jnp.square(x - lane_mean) for x in xs])
        pin(lane_m2)
        mean = jnp.sum(lane_mean, axis=1, keepdims=True) * (1.0 / 128)
        yield from _latency()
        m2 = lane_m2 + jnp.square(gate(lane_mean) - mean) * float(NT)
        pin(m2)
        var = jnp.sum(m2, axis=1, keepdims=True) * (1.0 / D)
        yield from _latency()
        return mean, lax.rsqrt(gate(jnp.broadcast_to(var, (16, 128))) + EPS)

    def d_fwd_rows(b, lb, from_input=False):
        if from_input:
            c, t = divmod(b, 8)
            xs = [_unpack(io32[j, lb, c, pl.ds(t // 2, 16, stride=4), :], t % 2) for j in range(NT)]
            for j in range(NT):
                xres[b, j, r16(lb), :] = xs[j]
        else:
            xs = load_x(b, lb)

        def emit(r, v):
            pin(v)
            ubuf[b % RING, r, r16(lb), :] = v.astype(BF16)

        inv = yield from _d_butterfly_fwd([gate(x) if j < 4 else x for j, x in enumerate(xs)], emit, pin, gate, from_input)
        inv = jnp.broadcast_to(inv, (16, 128))
        pin(inv)
        put(uout.at[b % RING, 8, r16(lb), :], inv)

    def d_dots(b, base, per_tick):
        for r in range(8):
            o = _dot(lhs(ubuf32[b % RING, r]), bf(small32[base + r]))
            put(uout.at[b % RING, r], o)
            if r % per_tick == per_tick - 1 and r < 7:
                yield

    def d_dots_wide(b):
        for ct, (ra, rb) in enumerate(PAIRS):
            u = lhs(ubuf32[b % RING, ra], ubuf32[b % RING, rb])
            for i, r in enumerate((ra, rb)):
                o = _dot(u, bf(wide32[2 * ct + i]))
                put(uout.at[b % RING, r], ticking(o) if i else o)
            if ct < 3:
                yield

    def d_fwd_cols(b, ct, is_wide):
        c, t = divmod(b, 8)
        ra, rb = PAIRS[ct]
        lane = _lane(16)
        lo = lane < 64
        z, x0 = [], []
        for lb in range(4):
            a, bb, inv = (uout[b % RING, r, r16(lb), :] for r in (ra, rb, 8))
            inv = gate(inv)
            a, bb = a * inv, bb * inv
            if is_wide:
                if ct == 0:
                    x0.append(pltpu.roll(bb, t, 1) if t else bb)
                    bb = jnp.where(lane == 0, 0.0, bb)
                z.append((a, bb))
                continue
            if ct == 0:
                x0.append(pltpu.roll(a, (t + 64) % 128, 1))
                a = jnp.where(lane == 64, 0.0, a)
            im = jnp.where(lo, bb, a)
            if 'd' in PINS:
                pin(im)
            z.append((jnp.where(lo, a, bb), _swap(im)))
        if not is_wide:
            yield from _latency()
            if 'n' in PINS:
                z[0], z[1] = [(gate(re), gate(im)) for re, im in z[0:2]]
        for e, (re, im) in enumerate(_dft4(z, False)):
            words = pack(re, im)
            pin(words)
            put(zin.at[ct, t * 4 + e, r16(c), :], words)
        if is_wide and ct == 0:
            yield from _latency()
        for lb, v in enumerate(x0):
            ls = pl.ds(64 * lb + 16 * c, 16)
            prev = jnp.zeros((16, 128), F32) if t == 0 else side[0, ls, :]
            v = jnp.where(lane == t, v, prev)
            pin(v)
            put(side.at[0, ls, :], v)

    def add_d_fwd(sched, tick, b, gap, per_tick=4, from_input=False):
        for lb in range(4):
            sched.add(tick + lb * gap, d_fwd_rows(b, lb, from_input))
        tick = int(tick + 3 * gap) + XGAP + 1
        sched.add(tick, d_dots_wide(b) if from_input else d_dots(b, 0, per_tick))
        for ct in range(4):
            sched.add(tick + 8 // per_tick + 3 + ct * gap, d_fwd_cols(b, ct, from_input))
        return int(tick + 8 // per_tick + 3 + 3 * gap) + XGAP + 1

    def side_path():
        vt = side[0].T[0:8]
        yield
        zero8 = jnp.zeros((8, 256), F32)
        u = _dot(jnp.concatenate([vt, zero8], axis=0).astype(BF16), f256[...])[0:8]
        twr, twi = tw_ref[0:8, :], tw_ref[8:16, :]
        ur, ui = u[:, 0:256], u[:, 256:512]
        pad = jnp.zeros((112, 256), BF16)
        for _ in range(4):
            yield
        uu = jnp.concatenate([ur * twr - ui * twi, ur * twi + ui * twr], axis=0).astype(BF16)
        xk = _dot(d8_ref[0], jnp.concatenate([uu, pad], axis=0))
        for _ in range(4):
            yield
        wr = jnp.concatenate([side[1, 0:8, :], side[1, 16:24, :]], axis=1)
        wi = jnp.concatenate([side[1, 8:16, :], side[1, 24:32, :]], axis=1)
        xr, xi = xk[0:8], xk[8:16]
        yy = jnp.concatenate([xr * wr - xi * wi, xr * wi + xi * wr], axis=0).astype(BF16)
        p = _dot(d8_ref[1], jnp.concatenate([yy, pad], axis=0))
        for _ in range(4):
            yield
        twr, twi = tw_ref[0:8, :], tw_ref[8:16, :]
        pr, pi = p[0:8], p[8:16]
        g = jnp.concatenate([pr * twr + pi * twi, pi * twr - pr * twi], axis=1)
        g = jnp.concatenate([g, jnp.zeros((8, 512), F32)], axis=0).astype(BF16)
        y0 = _dot_nt(g, f256[...])
        for _ in range(4):
            yield
        put(side.at[2], jnp.concatenate([y0, jnp.zeros((112, 256), F32)], axis=0).T)

    def s_fwd(u, t):
        ct, e = divmod(u, 4)
        put(ybuf.at[u % NY, t], ticking(_dot(lhs(sfw32[t * 4 + e]), bf(zin[ct, t * 4 + e]))))

    def s_filter(u, g):
        ct, e = divmod(u, 4)
        z = [tuple(ybuf[u % NY, t, pl.ds(g * 16 + i, 8), :] for i in (0, 8))
             for t in range(8)]
        z[0], z[1] = [tuple(gate(v, SGLAG if u <= 16 - NY else SGLAG2) for v in zz) for zz in z[0:2]]
        xk = _dft8(z, False)
        for k2 in range(8):
            wr = wf[0, ct, e, k2, pl.ds(g * 8, 8), :]
            wi = wf[1, ct, e, k2, pl.ds(g * 8, 8), :]
            re, im = xk[k2]
            xk[k2] = (re * wr - im * wi, re * wi + im * wr)
        for t, (re, im) in enumerate(_dft8(xk, True)):
            words = pack(re, im)
            pin(words)
            put(fbuf.at[u % NY, t, pl.ds(g * 8, 8), :], words)

    def s_inv(u, t):
        ct, e = divmod(u, 4)
        o = _dot(lhs(siv32[t * 4 + e]), bf(fbuf[u % NY, t]))
        put(zout.at[ct, t * 4 + e], ticking(o) if u > 16 - NY - 1 else o)

    def add_s_stage(sched, early, ready, t1):
        ahead = NY - 1
        tick = early
        for t in sorted(range(8), key=lambda t: ready[t]):
            for u in range(ahead):
                tick = max(tick + 0.5, ready[t])
                sched.add(tick, _once(s_fwd, u, t))
        t1 = max(t1, int(tick) + S_LAG)
        sched.add(max(max(ready), t1), side_path())
        for i in range(128):
            if i + 8 * ahead < 128:
                sched.add(t1 + i, _once(s_fwd, *divmod(i + 8 * ahead, 8)))
            sched.add(t1 + i, _once(s_filter, *divmod(i, 8)))
            sched.add(t1 + 9 + (i if i < 120 else 120 + (i - 120) // 4), _once(s_inv, *divmod(i, 8)))
        return [t1 + 32 * ct + 40 for ct in range(3)] + [t1 + 131]

    def d_inv_cols(b, ct):
        c, t = divmod(b, 8)
        ra, rb = PAIRS[ct]
        lane = _lane(16)
        lo = lane < 64
        u = [(zout[ct, t * 4 + e, r16(c), :], zout[ct, t * 4 + e, r16(4 + c), :]) for e in range(4)]
        u[0], u[1] = tuple(map(gate, u[0])), tuple(map(gate, u[1]))
        z = _dft4(u, True)
        z = [(re, _swap(im)) for re, im in z]
        if ct == 0:
            y0 = [pltpu.roll(side[2, pl.ds(64 * lb + 16 * c, 16), :], 64 - t, 1) for lb in range(4)]
        yield from _latency()
        for lb, (re, sw) in enumerate(z):
            if 'l' in PINS:
                sw = gate(sw)
            a, bb = jnp.where(lo, re, sw), jnp.where(lo, sw, re)
            if ct == 0:
                a = jnp.where(lane == 64, y0[lb], a)
            pin(a, bb)
            ubuf[b % RING, ra, r16(lb), :] = a.astype(BF16)
            ubuf[b % RING, rb, r16(lb), :] = bb.astype(BF16)

    def d_inv_rows(b, lb, stats):
        u = [uout[b % RING, r, r16(lb), :] for r in range(8)]
        ys = yield from _d_butterfly_inv([gate(v) if r < 4 else v for r, v in enumerate(u)], pin, gate)
        xs = [x + y for x, y in zip(load_x(b, lb), ys)]
        for j in range(NT):
            put(xres.at[b, j, r16(lb), :], xs[j])
        if 'h' in PINS:
            pin(*xs)
            yield
            xs = [gate(x) if j % 4 == 0 else x for j, x in enumerate(load_x(b, lb))]
        stats[b, lb] = mean, inv = yield from ln_stats(xs)
        if not STRASSEN:
            for j, x in enumerate(load_x(b, lb)):
                v = (x - mean) * inv
                pin(v)
                abuf[b, j, r16(lb), :] = v.astype(BF16)
        elif b % 2:
            for j in range(4):
                a = [(xres[bb, j + o, r16(lb), :] - stats[bb, lb][0]) * stats[bb, lb][1]
                     for bb in (b - 1, b) for o in (0, 4)]
                if 'm' in PINS:
                    a[0], a[3] = gate(a[0]), gate(a[3])
                for k, v in enumerate(_strassen_lhs(*a)):
                    if k not in (2, 3):
                        pin(v)
                    abuf[b // 2, k, j, r16(lb), :] = v.astype(BF16)
                if j < 3:
                    yield

    def add_d_inv(sched, tick, b, gap, stats, per_tick=4, cols=None):
        cols = cols or [tick + ct * gap for ct in range(4)]
        for ct in range(4):
            sched.add(cols[ct], d_inv_cols(b, ct))
        tick = int(cols[3]) + XGAP + 1
        sched.add(tick, d_dots(b, 8, per_tick))
        tick += 8 // per_tick + 3
        for lb in range(4):
            sched.add(tick + lb * gap, d_inv_rows(b, lb, stats))
        return int(tick + 3 * gap) + 3 * XGAP + 1 + 3 * STRASSEN + ('h' in PINS) + ('i' in PINS)

    def gemm(lhs32, rhs32, jobs, sink):
        for slot, b, n in jobs:
            if not STRASSEN:
                o = ticking(_dot(lhs(*[lhs32[slot, j] for j in range(4)]), bf(rhs32[n, pl.ds(0, 256), :])))
                yield
                sink(b, n, o + ticking(_dot(lhs(*[lhs32[slot, j] for j in range(4, 8)]),
                                            bf(rhs32[n, pl.ds(256, 256), :]))))
                yield
                continue
            m = {}
            for k in (6, 5, 0, 3, 1, 4, 2):
                m[k] = ticking(_dot(lhs(*[lhs32[slot, k, j] for j in range(4)]), bf(rhs32[n // 2, k])))
                if k == 0:
                    c11, c22 = m[6] - m[0], m[5] - m[0]
                elif k == 3:
                    c11 = c11 - m[3]
                elif k == 1:
                    sink(b + 1, n, m[1] - m[3])
                    c22 = c22 - m[1]
                elif k == 4:
                    sink(b, n, c11 - m[4])
                elif k == 2:
                    sink(b, n + 1, m[4] - m[2])
                    sink(b + 1, n + 1, c22 - m[2])
                yield

    def qkv_sink(b, n, o):
        c, t = divmod(b, 8)
        dst = (qbuf, kbuf, vbuf)[n // NT]
        for lb in range(4):
            put(dst.at[n % NT, t, pl.ds(8 + 64 * lb + 16 * c, 16), :], o[lb * 16:(lb + 1) * 16])
        if b == 0 and n >= NT:
            first = jnp.broadcast_to(o[0:1], (8, 128))
            for tt in range(8):
                dst[n % NT, tt, pl.ds(0, 8), :] = first

    def out_sink(b, n, o):
        put(xres.at[b, n], xres[b, n] + o)

    def attention(b, lb, h):
        c, t = divmod(b, 8)
        scale = HEAD_DIM ** -0.5
        r0 = 8 + 64 * lb + 16 * c + 8 * h
        src = [((t - 2 * w) % 8, -((t - 2 * w) // 8)) for w in range(WIN)]
        acc = [None] * WIN
        for j in range(NT):
            q = qbuf[j, t, pl.ds(r0, 8), :]
            if j % QG == 0:
                q = gate(q)
            for w, (ts, sh) in enumerate(src):
                p = q * kbuf[j, ts, pl.ds(r0 - sh, 8), :]
                acc[w] = p if j == 0 else acc[w] + p
            if j % QK == QK - 1 and j < NT - 1:
                pin(*acc)
                yield
        if 'e' in PINS:
            pin(*acc)
        part = [(r, pltpu.roll(r, 64, 1)) for r in acc]
        yield from _latency()
        part = [r + rr for r, rr in part]
        if 'f' in PINS:
            pin(*part)
        part = [(r, pltpu.roll(r, 32, 1)) for r in part]
        for _ in range(AGAP[0]):
            yield
        logits = [r + rr for r, rr in part]
        if r0 == 8:
            sub = lax.broadcasted_iota(jnp.int32, (8, 128), 0)
            logits = [jnp.where(sub >= sh, r, -1e9 / scale) if sh else r
                      for r, (_, sh) in zip(logits, src)]
        logits[0] = gate(logits[0])
        m = _tree(jnp.maximum, logits)
        ps = [jnp.exp2((r - m) * (scale * float(np.log2(np.e)))) for r in logits]
        total = _tree(_add, ps)
        pin(total)
        inv = pltpu.reciprocal(total, approx=True)
        inv = inv * (2.0 - total * inv)
        for j in range(NT):
            if j % PV == 0:
                yield
                for w in range(0, WIN, PG):
                    ps[w] = gate(ps[w])
            o = _chain(_add, [ps[w] * vbuf[j, ts, pl.ds(r0 - sh, 8), :]
                              for w, (ts, sh) in enumerate(src)]) * inv
            pin(o)
            if STRASSEN:
                put(qbuf.at[j, t, pl.ds(r0, 8), :], o)
            else:
                obuf[b, j, pl.ds(lb * 16 + h * 8, 8), :] = o.astype(BF16)

    def out_operands(b, lb):
        c, t = divmod(b, 8)
        rs = pl.ds(8 + 64 * lb + 16 * c, 16)
        for j in range(4):
            a = [qbuf[j + o, tt, rs, :] for tt in (t, t + 1) for o in (0, 4)]
            a[0], a[3] = gate(a[0]), gate(a[3])
            for k, v in enumerate(_strassen_lhs(*a)):
                if k not in (2, 3):
                    pin(v)
                obuf[b // 2, k, j, r16(lb), :] = v.astype(BF16)
            if j == 1 or ('j' in PINS and j < 3):
                yield

    def store_rows(b, lb):
        c, t = divmod(b, 8)
        for j in range(NT):
            words = pack(xres[b, j, r16(lb), :], xres[b + 1, j, r16(lb), :])
            pin(words)
            io32[j, lb, c, pl.ds(t // 2, 16, stride=4), :] = words

    unit_ticks = NT // QK + XGAP + AGAP[0] + NT // PV
    step = 2 if STRASSEN else 1
    out_ticks = 28 if STRASSEN else 16

    def add_proj(sched, tick, c, lo, hi):
        jobs = [(b // step, b, n) for b in range(8 * c, 8 * c + 8, step) for n in range(lo, hi, step)]
        sched.add(tick, gemm(abuf32, wqkv32, jobs, qkv_sink))
        return tick + len(jobs) * out_ticks * step // NT

    def add_attention(sched, tick, interval, units):
        for i, (b, lb, h) in enumerate(units):
            sched.add(tick + i * interval, attention(b, lb, h))
            if STRASSEN and b % 2 and h:
                sched.add(int(tick + i * interval) + unit_ticks, out_operands(b - 1, lb))

    def add_out(sched, tick, blocks):
        sched.add(tick, gemm(obuf32, wo32, [(b // step, b, n) for b in blocks[::step]
                                            for n in range(0, NT, step)], out_sink))

    def add_tail(sched, tick, blocks, last):
        ready = {}
        for i, b in enumerate(blocks):
            t0 = tick + (i // step + 1) * out_ticks
            fast = i >= len(blocks) - 2 * step
            if not fast:
                t0 += 3 + i % step * out_ticks // step
            if not last:
                ready[b % 8] = add_d_fwd(sched, t0, b, i % step if fast else out_ticks / step / 4)
            elif b % 2:
                for lb in range(4):
                    sched.add(t0 + (0 if fast else 3 * lb), _once(store_rows, b - 1, lb))
                if b % 8 == 7:
                    sched.add(t0 + (1 if fast else 12), _once(start, out_copies(b // 8)))
        return ready

    def units_of(blocks):
        return [(b, lb, h) for b in blocks for lb in range(4) for h in range(2)]

    q_ticks = 8 * out_ticks // step
    att_ticks = unit_ticks + 1 + 2 * STRASSEN
    order = [(a + 8) % NB for a in range(NB)]

    def add_attention_block(sched, cols, last):
        stats = {}
        t0 = max([add_d_inv(sched, 0, b, 0, stats, 4, cols) for b in range(step)])
        if not last:
            sched.add(cols[3] - KLEAD, _once(wait, qkv_copies(1) + dmat_cp))
            sched.add(cols[3] - KLEAD, _once(start, qkv_copies(2)))
            t0 = max(t0, add_prep_wqkv(sched, cols[3] - KLEAD, 1, KPACE))
            sched.add(t0, _once(wait, qkv_copies(2)))
            sched.add(t0, _once(start, qkv_copies(0)))
            assert add_prep_wqkv(sched, t0, 2, q_ticks - 10) <= t0 + q_ticks
            sched.add(t0 + q_ticks, _once(wait, qkv_copies(0)))
            sched.add(t0 + q_ticks, _once(start, wo_copies))
            assert add_prep_wqkv(sched, t0 + q_ticks, 0, 3 * q_ticks - 10) <= t0 + 4 * q_ticks
            sched.add(t0 + 8 * q_ticks, _once(wait, wo_copies))
            for i in range(32):
                sched.add(t0 + 8 * q_ticks + i * q_ticks / 16, _once(prep_wo, *divmod(i, 8)))
        tick, kv_start, q_start = t0, {}, {}
        for kind, c in ("k0", "k1", "q1", "k2", "q2", "k3", "q3", "q0"):
            if kind == "k":
                kv_start[int(c)] = tick
                if c == "0" and not last:
                    tick = add_proj(sched, add_proj(sched, tick, 0, NT, 2 * NT), 0, 2 * NT, 3 * NT)
                    continue
                tick = add_proj(sched, tick, int(c), NT, 3 * NT)
            else:
                q_start[int(c)] = tick
                tick = add_proj(sched, tick, int(c), 0, NT)
        pace = 2 * out_ticks / step
        for b in range(step, NB):
            due = kv_start[b // 8] + (b % 8 // step) * (2 if last or b >= 8 else 1) * out_ticks
            gap = min(1 + (b - step) * 0.5, DGAP)
            at = t0 + (b - step) * DPACE + max(0, b - DB) * DPACE2
            if not last and b < 8:
                at, gap = max(cols[3], t0 + (b // step - 1) * out_ticks - (step - b % step) * 8), 1
            end = add_d_inv(sched, at, b, gap, stats)
            assert end <= due, (b, end, due)
        begin = [q_start[c] + out_ticks + 3 for c in (1, 2, 3)] + [tick + (ATT1 if last else ATT0)]
        begin.append(tick + (NB // step - 1) * out_ticks - att_ticks)
        for i, c in enumerate((1, 2, 3, 0)):
            pace = (begin[i + 1] - begin[i]) / 64
            for t in range(8):
                first, done = begin[i] + 8 * t * pace, begin[i] + (8 * t + 7) * pace + att_ticks
                assert first >= q_start[c] + (t // step + 1) * out_ticks
                assert first >= max(kv_start[c], kv_start[(c - 1) % 4]) + 2 * q_ticks
                assert done <= tick + ((8 * i + t) // step) * out_ticks
            add_attention(sched, begin[i], pace, units_of(range(8 * c, 8 * c + 8)))
        add_out(sched, tick, order)
        return tick + (NB // step) * out_ticks, add_tail(sched, tick, order, last)

    def add_input(sched):
        ready = {}
        after = (x_copies(1) + x_copies(2), x_copies(3) + w_copies(0) + w_copies(1),
                 perm_cp + w_copies(2) + w_copies(3), sfw_cp + w_copies(4))
        for c in range(NC):
            sched.add(c * 32, _once(wait, x_copies(c)))
            sched.add(c * 32, _once(start, after[c]))
            for t in range(8):
                ready[t] = add_d_fwd(sched, c * 32 + t * 4, c * 8 + t, 1, 2, True)
        return 128 + 9, ready

    def add_filter_prep(sched, tick):
        after = {0: w_copies(5), 2: w_copies(6), 4: w_copies(7), 5: siv_cp + f256_cp,
                 7: dmat_cp + qkv_copies(1)}
        for g in range(8):
            sched.add(tick + g * 4, _once(wait, w_copies(g) + {0: perm_cp, 2: sfw_cp}.get(g, [])))
            sched.add(tick + g * 4, _once(start, after.get(g, [])))
            for m in range(4):
                sched.add(tick + g * 4 + m, _once(prep_filter, g // 4, g % 4 * 4 + m))
        sched.add(tick + 40, _once(wait, siv_cp + f256_cp))
        return tick + 34

    sched = _Schedule()

    def phase(fn, *args):
        fn(sched, *args)
        sched.run()
        token.clear()
        clock.clear()

    start(wide_cp + x_copies(0))
    wait(wide_cp)
    tick, ready = add_input(sched)
    cols = add_s_stage(sched, tick + 8, ready, add_filter_prep(sched, tick))
    tick, ready = add_attention_block(sched, cols, False)
    cols = add_s_stage(sched, tick, ready, tick)
    add_attention_block(sched, cols, True)
    sched.run()
    for c in range(NC):
        wait(out_copies(c))


@jax.jit
def pallas_interleave_layers__spectral_gfnet__sliding_local_dilated__prompt_kernel(
    A_x: jax.Array,
    A_w_r: jax.Array,
    A_w_i: jax.Array,
    B_x: jax.Array,
    B_wqkv: jax.Array,
    B_wo: jax.Array,
):
    del B_x
    assert A_x.shape == (1, S, D) and A_w_r.shape == (S, D // 2 + 1)
    cst = _constants()
    x = A_x.astype(BF16).reshape(4, NC, 128, D)
    wr, wi = A_w_r.astype(BF16).T, A_w_i.astype(BF16).T
    hbm = pl.BlockSpec(memory_space=pl.ANY)
    edge = pl.BlockSpec((16, S), lambda i: (D // 32, 0))
    vm = pltpu.VMEM
    out = pl.pallas_call(
        _kernel,
        grid=(1,),
        in_specs=[hbm, hbm, hbm, edge, edge, hbm, hbm, hbm, hbm, hbm, hbm, hbm,
                  pl.BlockSpec((24, 256), lambda i: (0, 0)),
                  pl.BlockSpec((2, 16, 128), lambda i: (0, 0, 0))],
        out_specs=hbm,
        out_shape=jax.ShapeDtypeStruct((4, NC, 128, D), BF16),
        scratch_shapes=[
            vm((NT, 4, NC, 128, 128), BF16),
            vm((17, 128, 128), BF16),
            vm((32, 128, 128), BF16),
            vm((32, 128, 128), BF16),
            vm((256, 512), BF16),
            vm((2, 16, 512, 128), BF16),
            vm((2, 4, 4, 8, 64, 128), F32),
            vm((3 * NT, D, 128), BF16),
            vm((NT, D // 2, 128), U32),
            vm((12, 7, 512, 128) if STRASSEN else (3 * NT, D, 128), BF16),
            vm((NT, D, 128), BF16),
            vm((4, 7, 512, 128) if STRASSEN else (NT, D, 128), BF16),
            vm((NB, NT, 64, 128), F32),
            vm((4, 32, 64, 128), U32),
            vm((4, 32, 128, 128), F32),
            vm((NY, 8, 128, 128), F32),
            vm((NY, 8, 64, 128), U32),
            vm((RING, 8, 64, 128), BF16),
            vm((RING, 9, 64, 128), F32),
            vm((NB // 2, 7, 4, 64, 128) if STRASSEN else (NB, NT, 64, 128), BF16),
            vm((NB // 2, 7, 4, 64, 128) if STRASSEN else (NB, NT, 64, 128), BF16),
            vm((NT, 8, 264, 128), F32),
            vm((NT, 8, 264, 128), F32),
            vm((NT, 8, 264, 128), F32),
            vm((3, 256, 128), F32),
            vm((8, 256, 128), BF16),
            pltpu.SemaphoreType.DMA((NC,)),
            pltpu.SemaphoreType.DMA((6,)),
            pltpu.SemaphoreType.DMA((8,)),
            pltpu.SemaphoreType.DMA((3,)),
            pltpu.SemaphoreType.DMA(()),
            pltpu.SemaphoreType.DMA((NC,)),
        ],
        compiler_params=pltpu.CompilerParams(
            dimension_semantics=("arbitrary",), vmem_limit_bytes=120 * 2**20),
    )(x, wr, wi, wr, wi, B_wqkv.astype(BF16), B_wo.astype(BF16),
      cst["small"], cst["sfw"], cst["siv"], cst["f256"], cst["wide"], cst["tw"], cst["d8"])
    return out.reshape(1, S, D)
```

```python
import functools

import jax
import jax.numpy as jnp
import numpy as np
from jax import lax
from jax.experimental import pallas as pl
from jax.experimental.pallas import tpu as pltpu

S, D = 2048, 1024
NT = D // 128
NC = 4
CR = S // NC
WIN = 8
HEAD_DIM = 32
EPS = 1e-5
F32, BF16, U32 = jnp.float32, jnp.bfloat16, jnp.uint32
PAIRS = ((0, 4), (1, 7), (2, 6), (3, 5))
RSQ2 = float(np.sqrt(0.5))
NB = 32
RING = 8
IGLAG = 4
KPACE = 32
PINS = 'bcijklm'
QK = 2
PV = 2
QG = 1
PG = 4
KLEAD = 24
SGLAG2 = 4
WI0 = 112
NY = 4
SGLAG = 3
ATT0 = 0
GLAG = 4
XGAP = 3
AGAP = (3, 1, 1)
DGAP = 3.5
DPACE = 14.3
DPACE2 = 0
DB = 22
ATT1 = 90
S_LAG = 4


def _residues(r):
    return (0, 8) if r == 0 else (r, 16 - r)


def _d_matrices():
    n = np.arange(64)[:, None]
    a = np.arange(32)
    fwd = np.zeros((8, 128, 128))
    inv = np.zeros((8, 128, 128))
    for r in range(8):
        kd = np.concatenate([16 * a + p for p in _residues(r)])
        weight = np.full(64, 2.0)
        if r == 0:
            kd[0], weight[0] = D // 2, 1.0
            ph = np.exp(-2j * np.pi * n * kd[None, :] / D)
            sgn = np.where(kd % 16 == 0, 1.0, -1.0)[None, :]
            m = np.concatenate([ph, ph * sgn], axis=0)
            re, im = m.real.copy(), m.imag.copy()
            ire, iim = re.copy(), im.copy()
            im[:, 0] = 1.0
            iim[:, 0] = 1.0
        else:
            p = r if r < 4 else 16 - r
            ph = np.exp(-2j * np.pi * n * kd[None, :] / D)
            si = np.where(kd % 16 == p, 1.0, -1.0)[None, :]
            m = np.concatenate([ph, 1j * si * ph], axis=0)
            re, im = m.real, m.imag
            ire, iim = re, im
        swapped = r in (4, 7, 6, 5)
        cols = [im, re] if swapped else [re, im]
        icols = [iim * weight, ire * weight] if swapped else [ire * weight, iim * weight]
        fwd[r] = np.concatenate(cols, axis=1)
        inv[r] = np.concatenate(icols, axis=1).T / D
    return fwd, inv


def _side_matrices():
    l = np.arange(256)
    f = np.exp(-2j * np.pi * ((l[:, None] * l[None, :]) % 256) / 256)
    f256 = np.concatenate([f.real, f.imag], axis=1)
    t = np.arange(8)
    tw = np.exp(-2j * np.pi * t[:, None] * l[None, :] / S)
    tw = np.concatenate([tw.real, tw.imag, np.zeros((8, 256))], axis=0)
    g = np.exp(-2j * np.pi * t[:, None] * t[None, :] / 8)
    d8 = np.zeros((2, 16, 128))
    d8[0, :, :16] = np.block([[g.real, -g.imag], [g.imag, g.real]])
    d8[1, :, :16] = d8[0, :, :16].T / S
    return f256, tw, d8


def _filter_rows():
    p = np.zeros((1, 128, 128))
    for k in range(32):
        for e in range(4):
            p[0, e * 32 + k, 4 * k + e] = 1.0
    return p


@functools.lru_cache(maxsize=None)
def _constants():
    dfw, div = _d_matrices()
    f256, tw, d8 = _side_matrices()
    small = np.concatenate([dfw, div, _filter_rows()], axis=0)
    b = lambda x: np.asarray(x, np.float32).astype(BF16)
    return dict(small=b(small), f256=b(f256),
                tw=np.asarray(tw, np.float32), d8=b(d8))


def _dot(a, b):
    return jnp.dot(a, b, preferred_element_type=F32)


def _dot_nt(a, b):
    return lax.dot_general(a, b, (((1,), (1,)), ((), ())), preferred_element_type=F32)


def _tree(op, xs):
    xs = list(xs)
    while len(xs) > 1:
        xs = [op(xs[i], xs[i + 1]) if i + 1 < len(xs) else xs[i] for i in range(0, len(xs), 2)]
    return xs[0]


def _chain(op, xs):
    return functools.reduce(op, xs)


def _lane(rows):
    return lax.broadcasted_iota(jnp.int32, (rows, 128), 1)


def _swap(x):
    return pltpu.roll(x, 64, 1)


def _unpack(w, i):
    return pltpu.unpack_elementwise(w, index=i, packed_dtype=BF16, unpacked_dtype=F32)


def _latency():
    for _ in range(XGAP):
        yield


def _add(a, b):
    return a + b


def _row_mean(xs):
    return jnp.sum(_tree(_add, xs), axis=1, keepdims=True) * (1.0 / D)


def _twiddle16(r):
    return float(np.cos(np.pi * r / 8)), float(-np.sin(np.pi * r / 8))


def _d_butterfly_fwd(a, emit, pin, gate, wide):
    lo = _lane(a[0].shape[0]) < 64
    s = [a[j] + a[j + 4] for j in range(4)]
    e, o = s[0] + s[2], s[1] + s[3]
    total, t4 = e + o, e - o
    emit(4, t4)
    d0, nd2 = a[0] - a[4], a[6] - a[2]
    d1, d3 = a[1] - a[5], a[3] - a[7]
    p, q = (d1 - d3) * RSQ2, (d1 + d3) * -RSQ2
    ts = {1: (d0 + p, q + nd2), 2: (s[0] - s[2], s[3] - s[1]), 3: (d0 - p, q - nd2)}
    mean8 = jnp.sum(total, axis=1, keepdims=True) * (1.0 / 128)
    if wide:
        for r, (tr, ti) in ts.items():
            emit(r, tr)
            emit(8 - r, ti)
    else:
        sw = {r: (_swap(tr), _swap(ti)) for r, (tr, ti) in ts.items()}
    dev = _tree(_add, [v * v for t in ts.values() for v in t]) * 2.0 + t4 * t4
    pin(dev)
    yield from _latency()
    t0 = total - mean8
    emit(0, t0)
    var = jnp.sum(dev + t0 * t0, axis=1, keepdims=True) * (1.0 / (NT * D))
    if not wide:
        for r, (tr, ti) in ts.items():
            wr, wi = _twiddle16(r)
            rr, ri = sw[r]
            if 'g' in PINS:
                ri = gate(ri)
            pp = jnp.where(lo, tr, ri)
            wq = jnp.where(lo, rr, ti) * wr + jnp.where(lo, ri, tr) * jnp.where(lo, -wi, wi)
            emit(r, pp + wq)
            emit(8 - r, pp - wq)
            if 'g' in PINS:
                yield
    if wide or 'g' not in PINS:
        yield from _latency()
    return lax.rsqrt(var + EPS)


def _d_butterfly_inv(u, pin, gate):
    lo = _lane(u[0].shape[0]) < 64
    pv = {r: (u[r] + u[8 - r], u[r] - u[8 - r]) for r in (1, 2, 3)}
    sw = {r: (_swap(p), _swap(v)) for r, (p, v) in pv.items()}
    e, o = u[0] + u[4], u[0] - u[4]
    yield from _latency()
    ts = {}
    for r, (pp, v) in pv.items():
        wr, wi = _twiddle16(r)
        rp, rv = sw[r]
        if 'k' in PINS:
            rv = gate(rv)
        ts[r] = (jnp.where(lo, pp, rv * wr + v * wi), jnp.where(lo, rp, v * wr - rv * wi))
    if 'i' in PINS:
        pin(*[v for t in ts.values() for v in t])
        yield
    s = [e + ts[2][0], o - ts[2][1], e - ts[2][0], o + ts[2][1]]
    p = (ts[1][0] - ts[3][0]) * RSQ2
    q = (ts[1][1] + ts[3][1]) * RSQ2
    d0, d1, d2, nd3 = ts[1][0] + ts[3][0], p - q, ts[3][1] - ts[1][1], p + q
    return [s[0] + d0, s[1] + d1, s[2] + d2, s[3] - nd3,
            s[0] - d0, s[1] - d1, s[2] - d2, s[3] + nd3]


def _strassen_lhs(a11, a12, a21, a22):
    return [a11 + a22, a21 + a22, a11, a22, a11 + a12, a21 - a11, a12 - a22]


def _strassen_rhs(b11, b12, b21, b22):
    return [-b11 - b22, b11, b22 - b12, b11 - b21, b22, b11 + b12, b21 + b22]


def _cadd(a, b):
    return a[0] + b[0], a[1] + b[1]


def _csub(a, b):
    return a[0] - b[0], a[1] - b[1]


def _dft4(z, inverse):
    a, b = _cadd(z[0], z[2]), _csub(z[0], z[2])
    c, d = _cadd(z[1], z[3]), _csub(z[1], z[3])
    minus = (b[0] + d[1], b[1] - d[0])
    plus = (b[0] - d[1], b[1] + d[0])
    return [_cadd(a, c), plus if inverse else minus, _csub(a, c), minus if inverse else plus]


def _dft8(z, inverse):
    ev = _dft4(z[0::2], inverse)
    od = _dft4(z[1::2], inverse)
    out = [None] * 8
    out[0], out[4] = _cadd(ev[0], od[0]), _csub(ev[0], od[0])
    (er, ei), (x, y) = ev[2], od[2]
    minus, plus = (er + y, ei - x), (er - y, ei + x)
    out[2], out[6] = (plus, minus) if inverse else (minus, plus)
    for k in (1, 3):
        (er, ei), (x, y) = ev[k], od[k]
        sm, df = (x + y) * RSQ2, (x - y) * RSQ2
        if not inverse:
            if k == 1:
                out[1], out[5] = (er + sm, ei - df), (er - sm, ei + df)
            else:
                out[3], out[7] = (er - df, ei - sm), (er + df, ei + sm)
        else:
            if k == 1:
                out[1], out[5] = (er + df, ei + sm), (er - df, ei - sm)
            else:
                out[3], out[7] = (er - sm, ei + df), (er + sm, ei - df)
    return out


class _Schedule:
    def __init__(self):
        self.pending = []

    def add(self, tick, gen):
        self.pending.append((int(tick), len(self.pending), gen))

    def run(self):
        pending = sorted(self.pending, key=lambda p: p[:2])
        active, tick, i = [], 0, 0
        while active or i < len(pending):
            while i < len(pending) and pending[i][0] <= tick:
                active.append(pending[i][2])
                i += 1
            for g in list(active):
                if next(g, 0) == 0:
                    active.remove(g)
            tick += 1
        self.pending = []


def _once(fn, *args):
    fn(*args)
    return
    yield


def _kernel(x_hbm, wr_hbm, wi_hbm, wr_edge, wi_edge, wqkv_hbm, wo_hbm,
            small_hbm, f256_hbm, tw_ref, d8_ref,
            out_hbm,
            io, small, sfw, siv, f256, wraw, wf, wqkv_raw, wtmp, wqkv, wo_raw, wo,
            xres, zin, zout, ybuf, fbuf, ubuf, uout, abuf, obuf, qbuf, kbuf, vbuf, side,
            wide, sem_x, sem_c, sem_w, sem_qkv, sem_wo, sem_out):

    def x_copies(c):
        return [pltpu.make_async_copy(x_hbm.at[:, c, :, pl.ds(j * 128, 128)], io.at[j, :, c],
                                      sem_x.at[c]) for j in range(NT)]

    def out_copies(c, lb):
        return [pltpu.make_async_copy(io.at[j, lb, c], out_hbm.at[lb, c, :, pl.ds(j * 128, 128)],
                                      sem_out) for j in range(NT)]

    perm_cp, dmat_cp, f256_cp = ([pltpu.make_async_copy(s, d, sem_c.at[i])] for i, (s, d) in enumerate((
        (small_hbm.at[pl.ds(16, 1)], small.at[pl.ds(16, 1)]),
        (small_hbm.at[pl.ds(0, 16)], small.at[pl.ds(0, 16)]), (f256_hbm, f256))))

    def w_copies(g):
        src = (wr_hbm, wi_hbm)[g // 4]
        return [pltpu.make_async_copy(src.at[pl.ds(0, 512), pl.ds(m * 128, 128)], wraw.at[g // 4, m],
                                      sem_w.at[g]) for m in range(g % 4 * 4, g % 4 * 4 + 4)]

    def qkv_copies(g):
        return [pltpu.make_async_copy(wqkv_hbm.at[:, pl.ds(g * D + j * 128, 128)],
                                      wqkv_raw.at[g * NT + j], sem_qkv.at[g]) for j in range(NT)]

    wo_copies = [pltpu.make_async_copy(wo_hbm.at[:, pl.ds(j * 128, 128)], wo_raw.at[j], sem_wo)
                 for j in range(NT)]

    def start(cs):
        for cp in cs:
            cp.start()

    def wait(cs):
        for cp in cs:
            cp.wait()

    io32, wraw32, wo_raw32 = io.bitcast(U32), wraw.bitcast(U32), wo_raw.bitcast(U32)
    small32, sfw32, siv32, wide32 = (r.bitcast(U32) for r in (small, sfw, siv, wide))
    wqkv_raw32, wqkv32, wo32 = (r.bitcast(U32) for r in (wqkv_raw, wqkv, wo))
    ubuf32, abuf32, obuf32 = ubuf.bitcast(U32), abuf.bitcast(U32), obuf.bitcast(U32)

    never = tw_ref[16:24, 0:128] != 0.0
    token = []

    def pin(*values):
        for v in values:
            for i in range(0, v.shape[0], 8):
                w = pltpu.bitcast(v[i:i + 8], U32)
                token[:] = [token[0] ^ w if token else w]

    clock, glag = [], [GLAG]

    def gate(v, lag=None):
        lag = lag or glag[0]
        if len(clock) < lag:
            return v
        head = jnp.where(never, pltpu.bitcast(clock[-lag], v.dtype), v[0:8])
        return head if v.shape[0] == 8 else jnp.concatenate([head, v[8:]], axis=0)

    def ticking(o):
        clock.append(o[0:8])
        del clock[:-16]
        return o

    def lhs(*tiles):
        if not token and len(tiles) == 4 and len(clock) >= 3:
            pin(clock[-3])
        if token:
            w = token.pop()
            tiles = [jnp.concatenate([jnp.where(never, w, t[0:8]), t[8:]], axis=0) for t in tiles]
        return jnp.concatenate([pltpu.bitcast(t, BF16) for t in tiles], axis=1)

    def bf(words):
        return pltpu.bitcast(words, BF16)

    def pack(a, b):
        return pltpu.bitcast(pltpu.pack_elementwise([a, b], packed_dtype=BF16), U32)

    def r16(i):
        return pl.ds(i * 16, 16)

    def put(ref, v):
        pltpu.store(ref, v, mask=jnp.ones(v.shape, jnp.bool_))

    def load_x(b, lb):
        return [xres[b, j, r16(lb), :] for j in range(NT)]

    def make_matrices():
        row, lane = lax.broadcasted_iota(jnp.int32, (8, 128), 0), _lane(8)

        def unit(p):
            angle = (((p + S // 2) & (S - 1)) - S // 2).astype(F32) * (2 * np.pi / S)
            return jnp.cos(angle), jnp.sin(angle)

        def times_row(a, b, i):
            br, bi = (jnp.broadcast_to(v[i:i + 1], (8, 128)) for v in b)
            return a[0] * br - a[1] * bi, a[0] * bi + a[1] * br

        for ct, (ra, rb) in enumerate(PAIRS):
            res = _residues(ra) + _residues(rb)
            kd = (lane & 31) * 16 + _chain(_add, [jnp.where(lane >> 5 == g, p, 0) for g, p in enumerate(res)])
            if ct == 0:
                kd = jnp.where(lane == 0, D // 2, kd)
            fine, coarse = unit(-2 * row * kd), [unit(-16 * (row + 8 * h) * kd) for h in range(2)]
            for a in range(16):
                re, im = times_row(fine, coarse[a // 8], a % 8)
                if ct == 0:
                    even = kd & 7 == 0
                    top = jnp.where(even, re, 0.0), jnp.where(lane == 0, 1.0, jnp.where(even, im, 0.0))
                    bottom = jnp.where(even, 0.0, re), jnp.where(even, 0.0, im)
                else:
                    sign = jnp.where(kd & 7 == ra, 1.0, -1.0)
                    top, bottom = (re, im), (-sign * im, sign * re)
                for i in range(2):
                    wide[2 * ct + i, pl.ds(8 * a, 8), :] = top[i].astype(BF16)
                    wide[2 * ct + i, pl.ds(128 + 8 * a, 8), :] = bottom[i].astype(BF16)
        start(x_copies(1))
        half, turn = lane >> 1, (lane & 1) * (S // 4)
        for t in range(8):
            pos = 8 * half + t
            fine, shift, coarse = unit(turn - 4 * row * pos), unit(-row * pos), unit(-32 * row * pos)
            for e in range(4):
                base = times_row(fine, shift, e)
                for g in range(8):
                    for i, v in enumerate(times_row(base, coarse, g)):
                        sfw[t * 4 + e, pl.ds(16 * g + 8 * i, 8), :] = v.astype(BF16)
        for e in range(4):
            freq = 4 * half + e
            fine, shift, coarse = unit(turn + 8 * row * freq), unit(row * freq), unit(64 * row * freq)
            fine = fine[0] * (1.0 / S), fine[1] * (1.0 / S)
            for t in range(8):
                base = times_row(fine, shift, t)
                for g in range(8):
                    for i, v in enumerate(times_row(base, coarse, g)):
                        siv[t * 4 + e, pl.ds(64 * i + 8 * g, 8), :] = v.astype(BF16)

    def prep_filter(ri, m):
        sub = lax.broadcasted_iota(jnp.int32, (8, 128), 0)
        edge = (wr_edge, wi_edge)[ri]
        res = {}
        for i in range(8):
            words = wraw32[ri, m, pl.ds(i, 32, stride=8), :]
            res[2 * i], res[2 * i + 1] = _unpack(words, 0), _unpack(words, 1)
        first = res[0][0:8]
        dst = pl.ds((m % 2) * 16 + ri * 8, 8)
        prev = jnp.zeros((8, 128), F32) if m < 2 else side[1, dst, :]
        put(side.at[1, dst, :], jnp.where(sub == m // 2, jnp.broadcast_to(first[0:1], (8, 128)), prev))
        nyq = jnp.broadcast_to(edge[0:1, pl.ds(m * 128, 128)].astype(F32), (8, 128))
        res[0] = jnp.concatenate([jnp.where(sub == 0, nyq, first), res[0][8:]], axis=0)
        for ct, (ra, rb) in enumerate(PAIRS):
            blk = jnp.concatenate([res[p] for p in _residues(ra) + _residues(rb)], axis=0)
            o = _dot_nt(bf(small32[16]), blk.astype(BF16))
            for e in range(4):
                put(wf.at[ri, ct, e, m // 2, pl.ds((m % 2) * 32, 32), :], o[e * 32:(e + 1) * 32])

    def shuffle(words, index):
        return jnp.take_along_axis(words, index, axis=1)

    def prep_wqkv_tile(g, i, part):
        lane = _lane(8)
        index = (lane & 3) * 32 + (((lane >> 2) - i) & 7) * 4 + (lane >> 5)
        rows = [pl.ds((part * 16 + r) * 8, 8) for r in range(16)]
        ws = [shuffle(gate(wqkv_raw32[g * NT + i, rs, :]), index) for rs in rows]
        yield from _latency()
        for rs, w in zip(rows, ws):
            pin(w)
            put(wtmp.at[i, rs, :], w)

    def prep_wqkv_cross(g, r):
        pos = (_lane(8) >> 2) & 7
        u = [wtmp[(-j) % 8, pl.ds(r * 8, 8), :] for j in range(NT)]
        u[0], u[4] = gate(u[0]), gate(u[4])
        for bit in range(3):
            m = ((pos >> bit) & 1) == 1
            u = [jnp.where(m, u[(j - (1 << bit)) % 8], u[j]) for j in range(NT)]
        for j in range(NT):
            pin(u[j])
            put(wqkv_raw32.at[g * NT + j, pl.ds(r * 8, 8), :], u[j])

    def prep_wqkv_pair(g, p, part):
        lane = _lane(8)
        ws = {}
        for n in range(2):
            index = (lane & 96) | ((lane + 4 * (2 * p + n)) & 31)
            for half in range(2):
                for r in range(part * 2, part * 2 + 2):
                    w = gate(wqkv_raw32[g * NT + 2 * p + n, pl.ds(half * 256 + r * 8, 8), :])
                    ws[r, half, n] = shuffle(w, index) if p + n else w
        yield from _latency()
        for r in range(part * 2, part * 2 + 2):
            quad = [ws[r, half, n] for half in range(2) for n in range(2)]
            ops = [_strassen_rhs(*[_unpack(w, i) for w in quad]) for i in range(2)]
            for k in range(7):
                word = {1: quad[0], 4: quad[3]}.get(k)
                if word is None:
                    word = pack(ops[0][k], ops[1][k])
                    pin(word)
                put(wqkv32.at[g * 4 + p, k, pl.ds(r * 8, 8), :], word)

    def add_prep_wqkv(sched, tick, g, ticks, pair_ticks):
        for i in range(32):
            sched.add(tick + i * ticks / 64, prep_wqkv_tile(g, *divmod(i, 4)))
        tick = int(tick + ticks / 2) + XGAP + 1
        for r in range(64):
            sched.add(tick + r * ticks / 128, _once(prep_wqkv_cross, g, r))
        tick = int(tick + ticks / 2) + 1
        done = []
        for p, n in enumerate(pair_ticks):
            for i in range(16):
                sched.add(tick + i * n / 16, prep_wqkv_pair(g, p, i))
            tick += n
            done.append(int(tick) + XGAP + 1)
        return done

    def prep_wo(p, dp):
        ws = [wo_raw32[2 * p + n, pl.ds(dp + off, 32, stride=16), :] for off in (0, 8) for n in (0, 1)]
        for i in range(2):
            b = [_unpack(w, i) for w in ws]
            r0 = (2 * dp + i) * 32
            for k, v in enumerate(_strassen_rhs(*b)):
                if k not in (1, 4):
                    pin(v)
                wo[p, k, pl.ds(r0, 32), :] = v.astype(BF16)

    def ln_stats(xs):
        lane_mean = _tree(_add, xs) * (1.0 / NT)
        lane_m2 = _tree(_add, [jnp.square(x - lane_mean) for x in xs])
        pin(lane_m2)
        mean = jnp.sum(lane_mean, axis=1, keepdims=True) * (1.0 / 128)
        yield from _latency()
        m2 = lane_m2 + jnp.square(gate(lane_mean) - mean) * float(NT)
        pin(m2)
        var = jnp.sum(m2, axis=1, keepdims=True) * (1.0 / D)
        yield from _latency()
        return mean, lax.rsqrt(gate(jnp.broadcast_to(var, (16, 128))) + EPS)

    def d_fwd_rows(b, lb, from_input=False):
        if from_input:
            c, t = divmod(b, 8)
            xs = [_unpack(io32[j, lb, c, pl.ds(t // 2, 16, stride=4), :], t % 2) for j in range(NT)]
            for j in range(NT):
                xres[b, j, r16(lb), :] = xs[j]
        else:
            xs = load_x(b, lb)

        def emit(r, v):
            pin(v)
            ubuf[b % RING, r, r16(lb), :] = v.astype(BF16)

        inv = yield from _d_butterfly_fwd([gate(x) if j < 4 else x for j, x in enumerate(xs)], emit, pin, gate, from_input)
        inv = jnp.broadcast_to(inv, (16, 128))
        pin(inv)
        put(uout.at[b % RING, 8, r16(lb), :], inv)

    def d_dots(b, base, per_tick):
        for r in range(8):
            o = _dot(lhs(ubuf32[b % RING, r]), bf(small32[base + r]))
            put(uout.at[b % RING, r], o)
            if r % per_tick == per_tick - 1 and r < 7:
                yield

    def d_dots_wide(b):
        for ct, (ra, rb) in enumerate(PAIRS):
            u = lhs(ubuf32[b % RING, ra], ubuf32[b % RING, rb])
            for i, r in enumerate((ra, rb)):
                o = _dot(u, bf(wide32[2 * ct + i]))
                put(uout.at[b % RING, r], ticking(o) if i else o)
            if ct < 3:
                yield

    def d_fwd_cols(b, ct, is_wide):
        c, t = divmod(b, 8)
        ra, rb = PAIRS[ct]
        lane = _lane(16)
        lo = lane < 64
        z, x0 = [], []
        for lb in range(4):
            a, bb, inv = (uout[b % RING, r, r16(lb), :] for r in (ra, rb, 8))
            inv = gate(inv)
            a, bb = a * inv, bb * inv
            if is_wide:
                if ct == 0:
                    x0.append(pltpu.roll(bb, t, 1) if t else bb)
                    bb = jnp.where(lane == 0, 0.0, bb)
                z.append((a, bb))
                continue
            if ct == 0:
                x0.append(pltpu.roll(a, (t + 64) % 128, 1))
                a = jnp.where(lane == 64, 0.0, a)
            im = jnp.where(lo, bb, a)
            if 'd' in PINS:
                pin(im)
            z.append((jnp.where(lo, a, bb), _swap(im)))
        if not is_wide:
            yield from _latency()
            if 'n' in PINS:
                z[0], z[1] = [(gate(re), gate(im)) for re, im in z[0:2]]
        for e, (re, im) in enumerate(_dft4(z, False)):
            words = pack(re, im)
            pin(words)
            put(zin.at[ct, t * 4 + e, r16(c), :], words)
        if is_wide and ct == 0:
            yield from _latency()
        for lb, v in enumerate(x0):
            ls = pl.ds(64 * lb + 16 * c, 16)
            prev = jnp.zeros((16, 128), F32) if t == 0 else side[0, ls, :]
            v = jnp.where(lane == t, v, prev)
            pin(v)
            put(side.at[0, ls, :], v)

    def add_d_fwd(sched, tick, b, gap, per_tick=4, from_input=False):
        for lb in range(4):
            sched.add(tick + lb * gap, d_fwd_rows(b, lb, from_input))
        tick = int(tick + 3 * gap) + XGAP + 1
        sched.add(tick, d_dots_wide(b) if from_input else d_dots(b, 0, per_tick))
        for ct in range(4):
            sched.add(tick + 8 // per_tick + 3 + ct * gap, d_fwd_cols(b, ct, from_input))
        return int(tick + 8 // per_tick + 3 + 3 * gap) + XGAP + 1

    def side_path():
        vt = side[0].T[0:8]
        yield
        zero8 = jnp.zeros((8, 256), F32)
        u = _dot(jnp.concatenate([vt, zero8], axis=0).astype(BF16), f256[...])[0:8]
        twr, twi = tw_ref[0:8, :], tw_ref[8:16, :]
        ur, ui = u[:, 0:256], u[:, 256:512]
        pad = jnp.zeros((112, 256), BF16)
        for _ in range(4):
            yield
        uu = jnp.concatenate([ur * twr - ui * twi, ur * twi + ui * twr], axis=0).astype(BF16)
        xk = _dot(d8_ref[0], jnp.concatenate([uu, pad], axis=0))
        for _ in range(4):
            yield
        wr = jnp.concatenate([side[1, 0:8, :], side[1, 16:24, :]], axis=1)
        wi = jnp.concatenate([side[1, 8:16, :], side[1, 24:32, :]], axis=1)
        xr, xi = xk[0:8], xk[8:16]
        yy = jnp.concatenate([xr * wr - xi * wi, xr * wi + xi * wr], axis=0).astype(BF16)
        p = _dot(d8_ref[1], jnp.concatenate([yy, pad], axis=0))
        for _ in range(4):
            yield
        twr, twi = tw_ref[0:8, :], tw_ref[8:16, :]
        pr, pi = p[0:8], p[8:16]
        g = jnp.concatenate([pr * twr + pi * twi, pi * twr - pr * twi], axis=1)
        g = jnp.concatenate([g, jnp.zeros((8, 512), F32)], axis=0).astype(BF16)
        y0 = _dot_nt(g, f256[...])
        for _ in range(4):
            yield
        put(side.at[2], jnp.concatenate([y0, jnp.zeros((112, 256), F32)], axis=0).T)

    def s_fwd(u, t):
        ct, e = divmod(u, 4)
        put(ybuf.at[u % NY, t], ticking(_dot(lhs(sfw32[t * 4 + e]), bf(zin[ct, t * 4 + e]))))

    def s_filter(u, g):
        ct, e = divmod(u, 4)
        z = [tuple(ybuf[u % NY, t, pl.ds(g * 16 + i, 8), :] for i in (0, 8))
             for t in range(8)]
        z[0], z[1] = [tuple(gate(v, SGLAG if u * 8 + g < 122 - S_LAG else SGLAG2) for v in zz) for zz in z[0:2]]
        xk = _dft8(z, False)
        for k2 in range(8):
            wr = wf[0, ct, e, k2, pl.ds(g * 8, 8), :]
            wi = wf[1, ct, e, k2, pl.ds(g * 8, 8), :]
            re, im = xk[k2]
            xk[k2] = (re * wr - im * wi, re * wi + im * wr)
        for t, (re, im) in enumerate(_dft8(xk, True)):
            words = pack(re, im)
            pin(words)
            put(fbuf.at[u % NY, t, pl.ds(g * 8, 8), :], words)

    def s_inv(u, t):
        ct, e = divmod(u, 4)
        o = _dot(lhs(siv32[t * 4 + e]), bf(fbuf[u % NY, t]))
        put(zout.at[ct, t * 4 + e], ticking(o) if u * 8 + t >= 110 - S_LAG else o)

    def add_s_stage(sched, early, ready, t1):
        ahead = 8 + S_LAG
        tick = early
        for t in sorted(range(8), key=lambda t: ready[t]):
            for i in range(t, ahead, 8):
                tick = max(tick + 0.5, ready[t])
                sched.add(tick, _once(s_fwd, i // 8, t))
        t1 = max(t1, int(tick) + 1)
        sched.add(max(max(ready), t1), side_path())
        for i in range(128):
            if i + ahead < 128:
                sched.add(t1 + i, _once(s_fwd, *divmod(i + ahead, 8)))
            sched.add(t1 + i, _once(s_filter, *divmod(i, 8)))
            sched.add(t1 + 9 + (i if i < 120 else 120 + (i - 120) // 4), _once(s_inv, *divmod(i, 8)))
        return [t1 + 32 * ct + 40 for ct in range(3)] + [t1 + 131]

    def d_inv_cols(b, ct):
        c, t = divmod(b, 8)
        ra, rb = PAIRS[ct]
        lane = _lane(16)
        lo = lane < 64
        u = [(zout[ct, t * 4 + e, r16(c), :], zout[ct, t * 4 + e, r16(4 + c), :]) for e in range(4)]
        u[0], u[1] = tuple(map(gate, u[0])), tuple(map(gate, u[1]))
        z = _dft4(u, True)
        z = [(re, _swap(im)) for re, im in z]
        if ct == 0:
            y0 = [pltpu.roll(side[2, pl.ds(64 * lb + 16 * c, 16), :], 64 - t, 1) for lb in range(4)]
        yield from _latency()
        for lb, (re, sw) in enumerate(z):
            if 'l' in PINS:
                sw = gate(sw)
            a, bb = jnp.where(lo, re, sw), jnp.where(lo, sw, re)
            if ct == 0:
                a = jnp.where(lane == 64, y0[lb], a)
            pin(a, bb)
            ubuf[b % RING, ra, r16(lb), :] = a.astype(BF16)
            ubuf[b % RING, rb, r16(lb), :] = bb.astype(BF16)

    def d_inv_rows(b, lb, stats):
        u = [uout[b % RING, r, r16(lb), :] for r in range(8)]
        ys = yield from _d_butterfly_inv([gate(v) if r < 4 else v for r, v in enumerate(u)], pin, gate)
        xs = [x + y for x, y in zip(load_x(b, lb), ys)]
        for j in range(NT):
            put(xres.at[b, j, r16(lb), :], xs[j])
        if 'h' in PINS:
            pin(*xs)
            yield
            xs = [gate(x) if j % 4 == 0 else x for j, x in enumerate(load_x(b, lb))]
        stats[b, lb] = yield from ln_stats(xs)
        if b % 2:
            for j in range(4):
                a = [(xres[bb, j + o, r16(lb), :] - stats[bb, lb][0]) * stats[bb, lb][1]
                     for bb in (b - 1, b) for o in (0, 4)]
                if 'm' in PINS:
                    a[0], a[3] = gate(a[0]), gate(a[3])
                for k, v in enumerate(_strassen_lhs(*a)):
                    if k not in (2, 3):
                        pin(v)
                    abuf[b // 2, k, j, r16(lb), :] = v.astype(BF16)
                if j < 3:
                    yield

    def add_d_inv(sched, tick, b, gap, stats, per_tick=4, cols=None):
        cols = cols or [tick + ct * gap for ct in range(4)]
        for ct in range(4):
            sched.add(cols[ct], d_inv_cols(b, ct))
        tick = int(cols[3]) + XGAP + 1
        sched.add(tick, d_dots(b, 8, per_tick))
        tick += 8 // per_tick + 3
        for lb in range(4):
            sched.add(tick + lb * gap, d_inv_rows(b, lb, stats))
        return int(tick + 3 * gap) + 3 * XGAP + 1 + 3 + ('h' in PINS) + ('i' in PINS)

    def gemm(lhs32, rhs32, jobs, sink):
        for slot, b, n in jobs:
            m = {}
            for k in (6, 5, 0, 3, 1, 4, 2):
                m[k] = ticking(_dot(lhs(*[lhs32[slot, k, j] for j in range(4)]), bf(rhs32[n // 2, k])))
                if k == 0:
                    c11, c22 = m[6] - m[0], m[5] - m[0]
                elif k == 3:
                    c11 = c11 - m[3]
                elif k == 1:
                    sink(b + 1, n, m[1] - m[3])
                    c22 = c22 - m[1]
                elif k == 4:
                    sink(b, n, c11 - m[4])
                elif k == 2:
                    sink(b, n + 1, m[4] - m[2])
                    sink(b + 1, n + 1, c22 - m[2])
                yield

    def qkv_sink(b, n, o):
        c, t = divmod(b, 8)
        dst = (qbuf, kbuf, vbuf)[n // NT]
        for lb in range(4):
            put(dst.at[n % NT, t, pl.ds(8 + 64 * lb + 16 * c, 16), :], o[lb * 16:(lb + 1) * 16])
        if b == 0 and n >= NT:
            first = jnp.broadcast_to(o[0:1], (8, 128))
            for tt in range(8):
                dst[n % NT, tt, pl.ds(0, 8), :] = first

    def out_rows(r, i, last):
        c, t = divmod(r, 8)
        return (c * 8 + t % 2 * 4 + i, t // 2) if last and c == 0 else (r, i)

    def out_sink(last, r, n, o):
        for i in range(4):
            b, lb = out_rows(r, i, last)
            put(xres.at[b, n, r16(lb), :], xres[b, n, r16(lb), :] + o[i * 16:(i + 1) * 16])

    def attention(b, lb, h):
        c, t = divmod(b, 8)
        scale = HEAD_DIM ** -0.5
        r0 = 8 + 64 * lb + 16 * c + 8 * h
        src = [((t - 2 * w) % 8, -((t - 2 * w) // 8)) for w in range(WIN)]
        acc = [None] * WIN
        for j in range(NT):
            q = qbuf[j, t, pl.ds(r0, 8), :]
            if j % QG == 0:
                q = gate(q)
            for w, (ts, sh) in enumerate(src):
                p = q * kbuf[j, ts, pl.ds(r0 - sh, 8), :]
                acc[w] = p if j == 0 else acc[w] + p
            if j % QK == QK - 1 and j < NT - 1:
                pin(*acc)
                yield
        if 'e' in PINS:
            pin(*acc)
        part = [(r, pltpu.roll(r, 64, 1)) for r in acc]
        yield from _latency()
        part = [r + rr for r, rr in part]
        if 'f' in PINS:
            pin(*part)
        part = [(r, pltpu.roll(r, 32, 1)) for r in part]
        for _ in range(AGAP[0]):
            yield
        logits = [r + rr for r, rr in part]
        if r0 == 8:
            sub = lax.broadcasted_iota(jnp.int32, (8, 128), 0)
            logits = [jnp.where(sub >= sh, r, -1e9 / scale) if sh else r
                      for r, (_, sh) in zip(logits, src)]
        logits[0] = gate(logits[0])
        m = _tree(jnp.maximum, logits)
        ps = [jnp.exp2((r - m) * (scale * float(np.log2(np.e)))) for r in logits]
        total = _tree(_add, ps)
        pin(total)
        inv = pltpu.reciprocal(total, approx=True)
        inv = inv * (2.0 - total * inv)
        for j in range(NT):
            if j % PV == 0:
                yield
                for w in range(0, WIN, PG):
                    ps[w] = gate(ps[w])
            o = _chain(_add, [ps[w] * vbuf[j, ts, pl.ds(r0 - sh, 8), :]
                              for w, (ts, sh) in enumerate(src)]) * inv
            pin(o)
            put(qbuf.at[j, t, pl.ds(r0, 8), :], o)

    def out_operands(r, i, last):
        for j in range(4):
            a = [qbuf[j + o, b % 8, pl.ds(8 + 64 * lb + 16 * (b // 8), 16), :]
                 for b, lb in (out_rows(r, i, last), out_rows(r + 1, i, last)) for o in (0, 4)]
            a[0], a[3] = gate(a[0]), gate(a[3])
            for k, v in enumerate(_strassen_lhs(*a)):
                if k not in (2, 3):
                    pin(v)
                obuf[r // 2, k, j, r16(i), :] = v.astype(BF16)
            if j < 3:
                yield

    def store_rows(b, lb):
        c, t = divmod(b, 8)
        for j in range(NT):
            words = pack(xres[b, j, r16(lb), :], xres[b + 1, j, r16(lb), :])
            pin(words)
            io32[j, lb, c, pl.ds(t // 2, 16, stride=4), :] = words

    unit_ticks = NT // QK + XGAP + AGAP[0] + NT // PV
    step = 2
    out_ticks = 28

    def add_proj(sched, tick, c, lo, hi):
        jobs = [(b // step, b, n) for b in range(8 * c, 8 * c + 8, step) for n in range(lo, hi, step)]
        sched.add(tick, gemm(abuf32, wqkv32, jobs, qkv_sink))
        return tick + len(jobs) * out_ticks * step // NT

    def add_attention(sched, tick, pace, rows, last):
        units = [(r, i, half, h) for r in rows[::2] for i in range(4) for half in range(2) for h in range(2)]
        for n, (r, i, half, h) in enumerate(units):
            sched.add(tick + n * pace, attention(*out_rows(r + half, i, last), h))
            if half and h:
                sched.add(int(tick + n * pace) + unit_ticks, out_operands(r, i, last))

    def add_out(sched, tick, rows, last):
        jobs = [(r // 2, r, n) for r in rows[::2] for n in range(0, NT, 2)]
        sched.add(tick, gemm(obuf32, wo32, jobs, functools.partial(out_sink, last)))

    def add_tail(sched, tick, rows, last):
        ready = {}
        for i, r in enumerate(rows):
            t0 = tick + (i // 2 + 1) * out_ticks
            fast = i >= len(rows) - (2 if last else 4)
            if not last:
                t0 += 0 if fast else 3 + i % 2 * out_ticks // 2
                ready[r % 8] = add_d_fwd(sched, t0, r, i % 2 if fast else out_ticks / 8)
            elif r % 2:
                c, p = r // 8, r % 8 // 2
                gap = 0 if fast else 3
                for j in range(4):
                    sched.add(t0 + (j + 1) * gap, _once(store_rows, *((r - 1, j) if c else (2 * j, p))))
                for lb in ([p] if c == 0 else range(4) if p == 3 else []):
                    sched.add(t0 + 5 * gap + 1, _once(start, out_copies(c, lb)))
        return ready

    q_ticks = 8 * out_ticks // step
    att_ticks = unit_ticks + 1 + 2
    order = [(a + 8) % NB for a in range(NB)]

    def add_attention_block(sched, cols, last):
        stats = {}
        t0 = max([add_d_inv(sched, 0, b, 0, stats, 4, cols) for b in range(step)])
        if not last:
            sched.add(cols[3] - KLEAD, _once(wait, qkv_copies(1) + dmat_cp))
            done = add_prep_wqkv(sched, cols[3] - KLEAD, 1, KPACE, [7] * 4)
            t0 = max(t0, done[0])
            assert all(d <= t0 + p * out_ticks / 4 for p, d in enumerate(done))
            sched.add(t0 + out_ticks, _once(wait, qkv_copies(2)))
            sched.add(t0 + out_ticks, _once(start, qkv_copies(0)))
            done = add_prep_wqkv(sched, t0 + out_ticks, 2, 2 * out_ticks - 6, [out_ticks - 4] * 4)
            assert all(d <= t0 + q_ticks + p * out_ticks for p, d in enumerate(done))
            sched.add(t0 + 2 * q_ticks, _once(wait, qkv_copies(0)))
            sched.add(t0 + 2 * q_ticks, _once(start, wo_copies))
            done = add_prep_wqkv(sched, t0 + 2 * q_ticks, 0, q_ticks - 10, [q_ticks / 4] * 4)
            assert done[-1] <= t0 + 4 * q_ticks
            sched.add(t0 + 8 * q_ticks, _once(wait, wo_copies))
            for i in range(32):
                sched.add(t0 + 8 * q_ticks + i * q_ticks / 16, _once(prep_wo, *divmod(i, 8)))
        tick, kv_start, q_start = t0, {}, {}
        for kind, c in ("k0", "k1", "q1", "k2", "q2", "k3", "q3", "q0"):
            if kind == "k":
                kv_start[int(c)] = tick
                if c == "0" and not last:
                    tick = add_proj(sched, tick, 0, NT, 2 * NT)
                    jobs = [(b // step, b, n) for n in range(2 * NT, 3 * NT, step) for b in range(0, 8, step)]
                    sched.add(tick, gemm(abuf32, wqkv32, jobs, qkv_sink))
                    tick += q_ticks
                    continue
                tick = add_proj(sched, tick, int(c), NT, 3 * NT)
            else:
                q_start[int(c)] = tick
                tick = add_proj(sched, tick, int(c), 0, NT)
        pace = 2 * out_ticks / step
        for b in range(step, NB):
            due = kv_start[b // 8] + (b % 8 // step) * (2 if last or b >= 8 else 1) * out_ticks
            gap = min(1 + (b - step) * 0.5, DGAP)
            at = t0 + (b - step) * DPACE + max(0, b - DB) * DPACE2
            if not last and b < 8:
                at, gap = max(cols[3], t0 + (b // step - 1) * out_ticks - (step - b % step) * 8), 1
            end = add_d_inv(sched, at, b, gap, stats)
            assert end <= due, (b, end, due)
        begin = [q_start[c] + out_ticks + 3 for c in (1, 2, 3)] + [tick + (ATT1 if last else ATT0)]
        begin.append(tick + (NB // step - 1) * out_ticks - att_ticks)
        for i, c in enumerate((1, 2, 3, 0)):
            pace = (begin[i + 1] - begin[i]) / 64
            assert begin[i] >= max(kv_start[c], kv_start[(c - 1) % 4]) + 2 * q_ticks
            for p in range(4):
                assert begin[i] + 16 * p * pace >= q_start[c] + (4 if last and c == 0 else p + 1) * out_ticks
                assert begin[i] + (16 * p + 15) * pace + att_ticks <= tick + (4 * i + p) * out_ticks + 1e-6
            add_attention(sched, begin[i], pace, range(8 * c, 8 * c + 8), last)
        add_out(sched, tick, order, last)
        return tick + (NB // step) * out_ticks, add_tail(sched, tick, order, last)

    def add_input(sched):
        ready = {}
        after = (x_copies(2), x_copies(3) + perm_cp + w_copies(0) + w_copies(1),
                 w_copies(2) + w_copies(3) + w_copies(4), w_copies(5) + w_copies(6))
        for c in range(NC):
            sched.add(c * 32, _once(wait, x_copies(c)))
            sched.add(c * 32, _once(start, after[c]))
            for t in range(8):
                ready[t] = add_d_fwd(sched, c * 32 + t * 4, c * 8 + t, 1, 2, True)
        return 128 + 9, ready

    def add_filter_prep(sched, tick):
        after = {0: w_copies(7) + f256_cp + dmat_cp, 3: qkv_copies(1), 7: qkv_copies(2)}
        for g in range(8):
            sched.add(tick + g * 4, _once(wait, w_copies(g) + ([] if g else perm_cp)))
            sched.add(tick + g * 4, _once(start, after.get(g, [])))
            for m in range(4):
                sched.add(tick + g * 4 + m, _once(prep_filter, g // 4, g % 4 * 4 + m))
        sched.add(tick + 33, _once(wait, f256_cp))
        return tick + 34

    sched = _Schedule()

    def phase(fn, *args):
        fn(sched, *args)
        sched.run()
        token.clear()
        clock.clear()

    start(x_copies(0))
    make_matrices()
    tick, ready = add_input(sched)
    cols = add_s_stage(sched, tick + 8, ready, add_filter_prep(sched, tick))
    tick, ready = add_attention_block(sched, cols, False)
    cols = add_s_stage(sched, tick, ready, tick)
    add_attention_block(sched, cols, True)
    sched.run()
    for c in range(NC):
        for lb in range(4):
            wait(out_copies(c, lb))


@jax.jit
def pallas_interleave_layers__spectral_gfnet__sliding_local_dilated__prompt_kernel(
    A_x: jax.Array,
    A_w_r: jax.Array,
    A_w_i: jax.Array,
    B_x: jax.Array,
    B_wqkv: jax.Array,
    B_wo: jax.Array,
):
    del B_x
    assert A_x.shape == (1, S, D) and A_w_r.shape == (S, D // 2 + 1)
    cst = _constants()
    x = A_x.astype(BF16).reshape(4, NC, 128, D)
    wr, wi = A_w_r.astype(BF16).T, A_w_i.astype(BF16).T
    hbm = pl.BlockSpec(memory_space=pl.ANY)
    edge = pl.BlockSpec((16, S), lambda i: (D // 32, 0))
    vm = pltpu.VMEM
    out = pl.pallas_call(
        _kernel,
        grid=(1,),
        in_specs=[hbm, hbm, hbm, edge, edge, hbm, hbm, hbm, hbm,
                  pl.BlockSpec((24, 256), lambda i: (0, 0)),
                  pl.BlockSpec((2, 16, 128), lambda i: (0, 0, 0))],
        out_specs=hbm,
        out_shape=jax.ShapeDtypeStruct((4, NC, 128, D), BF16),
        scratch_shapes=[
            vm((NT, 4, NC, 128, 128), BF16),
            vm((17, 128, 128), BF16),
            vm((32, 128, 128), BF16),
            vm((32, 128, 128), BF16),
            vm((256, 512), BF16),
            vm((2, 16, 512, 128), BF16),
            vm((2, 4, 4, 8, 64, 128), F32),
            vm((3 * NT, D, 128), BF16),
            vm((NT, D // 2, 128), U32),
            vm((12, 7, 512, 128), BF16),
            vm((NT, D, 128), BF16),
            vm((4, 7, 512, 128), BF16),
            vm((NB, NT, 64, 128), F32),
            vm((4, 32, 64, 128), U32),
            vm((4, 32, 128, 128), F32),
            vm((NY, 8, 128, 128), F32),
            vm((NY, 8, 64, 128), U32),
            vm((RING, 8, 64, 128), BF16),
            vm((RING, 9, 64, 128), F32),
            vm((NB // 2, 7, 4, 64, 128), BF16),
            vm((NB // 2, 7, 4, 64, 128), BF16),
            vm((NT, 8, 264, 128), F32),
            vm((NT, 8, 264, 128), F32),
            vm((NT, 8, 264, 128), F32),
            vm((3, 256, 128), F32),
            vm((8, 256, 128), BF16),
            pltpu.SemaphoreType.DMA((NC,)),
            pltpu.SemaphoreType.DMA((3,)),
            pltpu.SemaphoreType.DMA((8,)),
            pltpu.SemaphoreType.DMA((3,)),
            pltpu.SemaphoreType.DMA(()),
            pltpu.SemaphoreType.DMA(()),
        ],
        compiler_params=pltpu.CompilerParams(
            dimension_semantics=("arbitrary",), vmem_limit_bytes=120 * 2**20),
    )(x, wr, wi, wr, wi, B_wqkv.astype(BF16), B_wo.astype(BF16),
      cst["small"], cst["f256"], cst["tw"], cst["d8"])
    return out.reshape(1, S, D)
```

```python
import functools

import jax
import jax.numpy as jnp
import numpy as np
from jax import lax
from jax.experimental import pallas as pl
from jax.experimental.pallas import tpu as pltpu

S, D = 2048, 1024
NT = D // 128
NC = 4
WIN = 8
HEAD_DIM = 32
EPS = 1e-5
F32, BF16, U32 = jnp.float32, jnp.bfloat16, jnp.uint32
PAIRS = ((0, 4), (1, 7), (2, 6), (3, 5))
RSQ2 = float(np.sqrt(0.5))
NB = S // 64

RING = 8
NY = 4
XGAP = 3
GLAG = 4
SGLAG = 3
SGLAG2 = 4
S_LAG = 4
F0 = 104
KLEAD = 44
KPACE = 52
DGAP0 = 4.75
DGAP1 = 4.2
DPACE0 = 21
DPACE1 = 15.5
DSLOW = 0.6
SYNC = 3
ATT0 = 25
ATT1 = 80


def _residues(r):
    return (0, 8) if r == 0 else (r, 16 - r)


def _d_matrices():
    n = np.arange(64)[:, None]
    a = np.arange(32)
    fwd = np.zeros((8, 128, 128))
    inv = np.zeros((8, 128, 128))
    for r in range(8):
        kd = np.concatenate([16 * a + p for p in _residues(r)])
        weight = np.full(64, 2.0)
        if r == 0:
            kd[0], weight[0] = D // 2, 1.0
            ph = np.exp(-2j * np.pi * n * kd[None, :] / D)
            sgn = np.where(kd % 16 == 0, 1.0, -1.0)[None, :]
            m = np.concatenate([ph, ph * sgn], axis=0)
            re, im = m.real.copy(), m.imag.copy()
            ire, iim = re.copy(), im.copy()
            im[:, 0] = 1.0
            iim[:, 0] = 1.0
        else:
            p = 12 if r == 4 else r
            ph = np.exp(-2j * np.pi * n * kd[None, :] / D)
            si = np.where(kd % 16 == p, 1.0, -1.0)[None, :]
            m = np.concatenate([ph, 1j * si * ph], axis=0)
            re, im = m.real, m.imag
            ire, iim = re, im
        swapped = r in (4, 7, 6, 5)
        cols = [im, re] if swapped else [re, im]
        icols = [iim * weight, ire * weight] if swapped else [ire * weight, iim * weight]
        fwd[r] = np.concatenate(cols, axis=1)
        inv[r] = np.concatenate(icols, axis=1).T / D
    return fwd, inv


def _side_matrices():
    l = np.arange(256)
    f = np.exp(-2j * np.pi * ((l[:, None] * l[None, :]) % 256) / 256)
    f256 = np.concatenate([f.real, f.imag], axis=1)
    t = np.arange(8)
    tw = np.exp(-2j * np.pi * t[:, None] * l[None, :] / S)
    tw = np.concatenate([tw.real, tw.imag, np.zeros((8, 256))], axis=0)
    g = np.exp(-2j * np.pi * t[:, None] * t[None, :] / 8)
    d8 = np.zeros((2, 16, 128))
    d8[0, :, :16] = np.block([[g.real, -g.imag], [g.imag, g.real]])
    d8[1, :, :16] = d8[0, :, :16].T / S
    return f256, tw, d8


def _filter_rows():
    p = np.zeros((1, 128, 128))
    for k in range(32):
        for e in range(4):
            p[0, e * 32 + k, 4 * k + e] = 1.0
    return p


@functools.lru_cache(maxsize=None)
def _constants():
    dfw, div = _d_matrices()
    f256, tw, d8 = _side_matrices()
    small = np.concatenate([dfw, div, _filter_rows()], axis=0)
    b = lambda x: np.asarray(x, np.float32).astype(BF16)
    return dict(small=b(small), f256=b(f256),
                tw=np.asarray(tw, np.float32), d8=b(d8))


def _dot(a, b):
    return jnp.dot(a, b, preferred_element_type=F32)


def _dot_nt(a, b):
    return lax.dot_general(a, b, (((1,), (1,)), ((), ())), preferred_element_type=F32)


def _tree(op, xs):
    xs = list(xs)
    while len(xs) > 1:
        xs = [op(xs[i], xs[i + 1]) if i + 1 < len(xs) else xs[i] for i in range(0, len(xs), 2)]
    return xs[0]


def _chain(op, xs):
    return functools.reduce(op, xs)


def _lane(rows):
    return lax.broadcasted_iota(jnp.int32, (rows, 128), 1)


def _swap(x):
    return pltpu.roll(x, 64, 1)


def _unpack(w, i):
    return pltpu.unpack_elementwise(w, index=i, packed_dtype=BF16, unpacked_dtype=F32)


def _latency():
    for _ in range(XGAP):
        yield


def _add(a, b):
    return a + b


def _row_mean(xs):
    return jnp.sum(_tree(_add, xs), axis=1, keepdims=True) * (1.0 / D)


def _twiddle16(r, x, y):
    lo = _lane(x.shape[0]) < 64
    wr, wi = float(np.cos(np.pi * r / 8)), float(-np.sin(np.pi * r / 8))
    cross = jnp.where(lo, 0.0, wr)
    return x * jnp.where(lo, 1.0, wi) + y * cross, y * jnp.where(lo, 1.0, -wi) + x * cross


def _d_butterfly_fwd(a, emit, pin, gate, wide):
    s = [a[j] + a[j + 4] for j in range(4)]
    e, o = s[0] + s[2], s[1] + s[3]
    total, t4 = e + o, e - o
    emit(4, t4)
    d0, nd2 = a[0] - a[4], a[6] - a[2]
    d1, d3 = a[1] - a[5], a[3] - a[7]
    p, q = (d1 - d3) * RSQ2, (d1 + d3) * -RSQ2
    ts = {1: (d0 + p, q + nd2), 2: (s[0] - s[2], s[3] - s[1]), 3: (d0 - p, q - nd2)}
    mean8 = jnp.sum(total, axis=1, keepdims=True) * (1.0 / 128)
    if wide:
        for r, (tr, ti) in ts.items():
            emit(r, tr)
            emit(8 - r, ti)
    else:
        ab = {r: _twiddle16(r, *t) for r, t in ts.items()}
        ab = {r: (a, _swap(b)) for r, (a, b) in ab.items()}
    dev = _tree(_add, [v * v for t in ts.values() for v in t]) * 2.0 + t4 * t4
    pin(dev)
    yield from _latency()
    t0 = total - mean8
    emit(0, t0)
    var = jnp.sum(dev + t0 * t0, axis=1, keepdims=True) * (1.0 / (NT * D))
    if not wide:
        for r, (x, y) in ab.items():
            emit(r, x + y)
            emit(8 - r, x - y)
    yield from _latency()
    return lax.rsqrt(var + EPS)


def _d_butterfly_inv(u, pin, gate):
    ab = {r: (u[r] + u[8 - r], _swap(u[r] - u[8 - r])) for r in (1, 2, 3)}
    e, o = u[0] + u[4], u[0] - u[4]
    yield from _latency()
    ts = {r: _twiddle16(r, x, gate(y)) for r, (x, y) in ab.items()}
    pin(*[v for t in ts.values() for v in t])
    yield
    s = [e + ts[2][0], o - ts[2][1], e - ts[2][0], o + ts[2][1]]
    p = (ts[1][0] - ts[3][0]) * RSQ2
    q = (ts[1][1] + ts[3][1]) * RSQ2
    d0, d1, d2, nd3 = ts[1][0] + ts[3][0], p - q, ts[3][1] - ts[1][1], p + q
    return [s[0] + d0, s[1] + d1, s[2] + d2, s[3] - nd3,
            s[0] - d0, s[1] - d1, s[2] - d2, s[3] + nd3]


def _strassen_lhs(a11, a12, a21, a22):
    return [a11 + a22, a21 + a22, a11, a22, a11 + a12, a21 - a11, a12 - a22]


def _strassen_rhs(b11, b12, b21, b22):
    return [-b11 - b22, b11, b22 - b12, b11 - b21, b22, b11 + b12, b21 + b22]


def _cadd(a, b):
    return a[0] + b[0], a[1] + b[1]


def _csub(a, b):
    return a[0] - b[0], a[1] - b[1]


def _dft4(z, inverse):
    a, b = _cadd(z[0], z[2]), _csub(z[0], z[2])
    c, d = _cadd(z[1], z[3]), _csub(z[1], z[3])
    minus = (b[0] + d[1], b[1] - d[0])
    plus = (b[0] - d[1], b[1] + d[0])
    return [_cadd(a, c), plus if inverse else minus, _csub(a, c), minus if inverse else plus]


def _dft8(z, inverse):
    ev = _dft4(z[0::2], inverse)
    od = _dft4(z[1::2], inverse)
    out = [None] * 8
    out[0], out[4] = _cadd(ev[0], od[0]), _csub(ev[0], od[0])
    (er, ei), (x, y) = ev[2], od[2]
    minus, plus = (er + y, ei - x), (er - y, ei + x)
    out[2], out[6] = (plus, minus) if inverse else (minus, plus)
    for k in (1, 3):
        (er, ei), (x, y) = ev[k], od[k]
        sm, df = (x + y) * RSQ2, (x - y) * RSQ2
        if not inverse:
            if k == 1:
                out[1], out[5] = (er + sm, ei - df), (er - sm, ei + df)
            else:
                out[3], out[7] = (er - df, ei - sm), (er + df, ei + sm)
        else:
            if k == 1:
                out[1], out[5] = (er + df, ei + sm), (er - df, ei - sm)
            else:
                out[3], out[7] = (er - sm, ei + df), (er + sm, ei - df)
    return out


class _Schedule:
    def __init__(self):
        self.pending = []

    def add(self, tick, gen):
        self.pending.append((int(tick), len(self.pending), gen))

    def run(self):
        pending = sorted(self.pending, key=lambda p: p[:2])
        active, tick, i = [], 0, 0
        while active or i < len(pending):
            while i < len(pending) and pending[i][0] <= tick:
                active.append(pending[i][2])
                i += 1
            for g in list(active):
                if next(g, 0) == 0:
                    active.remove(g)
            tick += 1
        self.pending = []


def _once(fn, *args):
    fn(*args)
    return
    yield


def _kernel(x_hbm, wr_hbm, wi_hbm, wr_edge, wi_edge, wqkv_hbm, wo_hbm,
            small_hbm, f256_hbm, tw_ref, d8_ref,
            out_hbm,
            io, small, sfw, siv, f256, wraw, wf, wqkv_raw, wtmp, wqkv, wo_raw, wo,
            xres, zin, zout, ybuf, fbuf, ubuf, uout, abuf, obuf, qbuf, kbuf, vbuf, side,
            wide, sem_x, sem_c, sem_w, sem_qkv, sem_wo, sem_out):

    def x_copies(c):
        return [pltpu.make_async_copy(x_hbm.at[:, c, :, pl.ds(j * 128, 128)], io.at[j, :, c],
                                      sem_x.at[c]) for j in range(NT)]

    def out_copies(c, lb):
        return [pltpu.make_async_copy(io.at[j, lb, c], out_hbm.at[lb, c, :, pl.ds(j * 128, 128)],
                                      sem_out) for j in range(NT)]

    perm_cp, dmat_cp, f256_cp = ([pltpu.make_async_copy(s, d, sem_c.at[i])] for i, (s, d) in enumerate((
        (small_hbm.at[pl.ds(16, 1)], small.at[pl.ds(16, 1)]),
        (small_hbm.at[pl.ds(0, 16)], small.at[pl.ds(0, 16)]), (f256_hbm, f256))))

    def w_copies(g):
        src = (wr_hbm, wi_hbm)[g // 4]
        return [pltpu.make_async_copy(src.at[pl.ds(0, 512), pl.ds(m * 128, 128)], wraw.at[g // 4, m],
                                      sem_w.at[g]) for m in range(g % 4 * 4, g % 4 * 4 + 4)]

    def qkv_copies(g):
        return [pltpu.make_async_copy(wqkv_hbm.at[:, pl.ds(g * D + j * 128, 128)],
                                      wqkv_raw.at[g * NT + j], sem_qkv.at[g]) for j in range(NT)]

    wo_copies = [pltpu.make_async_copy(wo_hbm.at[:, pl.ds(j * 128, 128)], wo_raw.at[j], sem_wo)
                 for j in range(NT)]

    def start(cs):
        for cp in cs:
            cp.start()

    def wait(cs):
        for cp in cs:
            cp.wait()

    io32, wraw32, wo_raw32 = io.bitcast(U32), wraw.bitcast(U32), wo_raw.bitcast(U32)
    small32, sfw32, siv32, wide32 = (r.bitcast(U32) for r in (small, sfw, siv, wide))
    wqkv_raw32, wqkv32, wo32 = (r.bitcast(U32) for r in (wqkv_raw, wqkv, wo))
    ubuf32, abuf32, obuf32 = ubuf.bitcast(U32), abuf.bitcast(U32), obuf.bitcast(U32)

    never = tw_ref[16:24, 0:128] != 0.0
    token = []

    def pin(*values):
        for v in values:
            for i in range(0, v.shape[0], 8):
                w = pltpu.bitcast(v[i:i + 8], U32)
                token[:] = [token[0] ^ w if token else w]

    clock = []

    def gate(v, lag=GLAG):
        if len(clock) < lag:
            return v
        head = jnp.where(never, pltpu.bitcast(clock[-lag], v.dtype), v[0:8])
        return head if v.shape[0] == 8 else jnp.concatenate([head, v[8:]], axis=0)

    def ticking(o):
        clock.append(o[0:8])
        del clock[:-16]
        return o

    def lhs(*tiles):
        if not token and len(tiles) == 4 and len(clock) >= SYNC:
            pin(clock[-SYNC])
        if token:
            w = token.pop()
            tiles = [jnp.concatenate([jnp.where(never, w, t[0:8]), t[8:]], axis=0) for t in tiles]
        return jnp.concatenate([pltpu.bitcast(t, BF16) for t in tiles], axis=1)

    def bf(words):
        return pltpu.bitcast(words, BF16)

    def pack(a, b):
        return pltpu.bitcast(pltpu.pack_elementwise([a, b], packed_dtype=BF16), U32)

    def r16(i):
        return pl.ds(i * 16, 16)

    def put(ref, v):
        pltpu.store(ref, v, mask=jnp.ones(v.shape, jnp.bool_))

    def load_x(b, lb):
        return [xres[b, j, r16(lb), :] for j in range(NT)]

    def unit(p):
        angle = (((p + S // 2) & (S - 1)) - S // 2).astype(F32) * (2 * np.pi / S)
        return jnp.cos(angle), jnp.sin(angle)

    def times_row(a, b, i):
        br, bi = (jnp.broadcast_to(v[i:i + 1], (8, 128)) for v in b)
        return a[0] * br - a[1] * bi, a[0] * bi + a[1] * br

    def make_wide():
        row, lane = lax.broadcasted_iota(jnp.int32, (8, 128), 0), _lane(8)
        for ct, (ra, rb) in enumerate(PAIRS):
            res = _residues(ra) + _residues(rb)
            kd = (lane & 31) * 16 + _chain(
                _add, [jnp.where(lane >> 5 == g, p, 0) for g, p in enumerate(res)])
            if ct == 0:
                kd = jnp.where(lane == 0, D // 2, kd)
            fine, coarse = unit(-2 * row * kd), [unit(-16 * (row + 8 * h) * kd) for h in range(2)]
            for a in range(16):
                re, im = times_row(fine, coarse[a // 8], a % 8)
                if ct == 0:
                    even = kd & 7 == 0
                    top = jnp.where(even, re, 0.0), jnp.where(lane == 0, 1.0, jnp.where(even, im, 0.0))
                    bottom = jnp.where(even, 0.0, re), jnp.where(even, 0.0, im)
                else:
                    sign = jnp.where(kd & 7 == ra, 1.0, -1.0)
                    top, bottom = (re, im), (-sign * im, sign * re)
                for i in range(2):
                    wide[2 * ct + i, pl.ds(8 * a, 8), :] = top[i].astype(BF16)
                    wide[2 * ct + i, pl.ds(128 + 8 * a, 8), :] = bottom[i].astype(BF16)

    def make_s_fwd(t):
        row, lane = lax.broadcasted_iota(jnp.int32, (8, 128), 0), _lane(8)
        pos = 8 * (lane >> 1) + t
        fine = unit((lane & 1) * (S // 4) - 4 * row * pos)
        shift, coarse = unit(-row * pos), unit(-32 * row * pos)
        for e in range(4):
            base = times_row(fine, shift, e)
            for g in range(8):
                for i, v in enumerate(times_row(base, coarse, g)):
                    sfw[t * 4 + e, pl.ds(16 * g + 8 * i, 8), :] = v.astype(BF16)

    def make_s_inv(e):
        row, lane = lax.broadcasted_iota(jnp.int32, (8, 128), 0), _lane(8)
        freq = 4 * (lane >> 1) + e
        fine = [v * (1.0 / S) for v in unit((lane & 1) * (S // 4) + 8 * row * freq)]
        shift, coarse = unit(row * freq), unit(64 * row * freq)
        for t in range(8):
            base = times_row(fine, shift, t)
            for g in range(8):
                for i, v in enumerate(times_row(base, coarse, g)):
                    siv[t * 4 + e, pl.ds(64 * i + 8 * g, 8), :] = v.astype(BF16)

    def prep_filter(ri, m):
        sub = lax.broadcasted_iota(jnp.int32, (8, 128), 0)
        edge = (wr_edge, wi_edge)[ri]
        res = {}
        for i in range(8):
            words = wraw32[ri, m, pl.ds(i, 32, stride=8), :]
            res[2 * i], res[2 * i + 1] = _unpack(words, 0), _unpack(words, 1)
        first = res[0][0:8]
        dst = pl.ds((m % 2) * 16 + ri * 8, 8)
        prev = jnp.zeros((8, 128), F32) if m < 2 else side[1, dst, :]
        put(side.at[1, dst, :], jnp.where(sub == m // 2, jnp.broadcast_to(first[0:1], (8, 128)), prev))
        nyq = jnp.broadcast_to(edge[0:1, pl.ds(m * 128, 128)].astype(F32), (8, 128))
        res[0] = jnp.concatenate([jnp.where(sub == 0, nyq, first), res[0][8:]], axis=0)
        for ct, (ra, rb) in enumerate(PAIRS):
            blk = jnp.concatenate([res[p] for p in _residues(ra) + _residues(rb)], axis=0)
            o = _dot_nt(lhs(small32[16]), blk.astype(BF16))
            for e in range(4):
                put(wf.at[ri, ct, e, m // 2, pl.ds((m % 2) * 32, 32), :], o[e * 32:(e + 1) * 32])

    def shuffle(words, index):
        return jnp.take_along_axis(words, index, axis=1)

    def prep_wqkv_tile(g, i, part):
        lane = _lane(8)
        index = (lane & 3) * 32 + (((lane >> 2) - i) & 7) * 4 + (lane >> 5)
        rows = [pl.ds((part * 16 + r) * 8, 8) for r in range(16)]
        ws = [shuffle(gate(wqkv_raw32[g * NT + i, rs, :]), index) for rs in rows]
        yield from _latency()
        for rs, w in zip(rows, ws):
            pin(w)
            put(wtmp.at[i, rs, :], w)

    def prep_wqkv_cross(g, r):
        pos = (_lane(8) >> 2) & 7
        u = [wtmp[(-j) % 8, pl.ds(r * 8, 8), :] for j in range(NT)]
        u[0], u[4] = gate(u[0]), gate(u[4])
        for bit in range(3):
            m = ((pos >> bit) & 1) == 1
            u = [jnp.where(m, u[(j - (1 << bit)) % 8], u[j]) for j in range(NT)]
        for j in range(NT):
            pin(u[j])
            put(wqkv_raw32.at[g * NT + j, pl.ds(r * 8, 8), :], u[j])

    def prep_wqkv_pair(g, p, part):
        lane = _lane(8)
        ws = {}
        for n in range(2):
            index = (lane & 96) | ((lane + 4 * (2 * p + n)) & 31)
            for half in range(2):
                for r in range(part * 2, part * 2 + 2):
                    w = gate(wqkv_raw32[g * NT + 2 * p + n, pl.ds(half * 256 + r * 8, 8), :])
                    ws[r, half, n] = shuffle(w, index) if p + n else w
        yield from _latency()
        for r in range(part * 2, part * 2 + 2):
            quad = [ws[r, half, n] for half in range(2) for n in range(2)]
            ops = [_strassen_rhs(*[_unpack(w, i) for w in quad]) for i in range(2)]
            for k in range(7):
                word = {1: quad[0], 4: quad[3]}.get(k)
                if word is None:
                    word = pack(ops[0][k], ops[1][k])
                    pin(word)
                put(wqkv32.at[g * 4 + p, k, pl.ds(r * 8, 8), :], word)

    def add_prep_wqkv(sched, tick, g, ticks, pair_ticks):
        for i in range(32):
            sched.add(tick + i * ticks / 64, prep_wqkv_tile(g, *divmod(i, 4)))
        tick = int(tick + ticks / 2) + XGAP + 1
        for r in range(64):
            sched.add(tick + r * ticks / 128, _once(prep_wqkv_cross, g, r))
        tick = int(tick + ticks / 2) + 1
        done = []
        for p, n in enumerate(pair_ticks):
            for i in range(16):
                sched.add(tick + i * n / 16, prep_wqkv_pair(g, p, i))
            tick += n
            done.append(int(tick) + XGAP + 1)
        return done

    def prep_wo(p, dp):
        ws = [wo_raw32[2 * p + n, pl.ds(dp + off, 32, stride=16), :] for off in (0, 8) for n in (0, 1)]
        for i in range(2):
            b = [_unpack(w, i) for w in ws]
            r0 = (2 * dp + i) * 32
            for k, v in enumerate(_strassen_rhs(*b)):
                if k not in (1, 4):
                    pin(v)
                wo[p, k, pl.ds(r0, 32), :] = v.astype(BF16)

    def ln_stats(xs):
        lane_mean = _tree(_add, xs) * (1.0 / NT)
        lane_m2 = _tree(_add, [jnp.square(x - lane_mean) for x in xs])
        pin(lane_m2)
        mean = jnp.sum(lane_mean, axis=1, keepdims=True) * (1.0 / 128)
        yield from _latency()
        m2 = lane_m2 + jnp.square(gate(lane_mean) - mean) * float(NT)
        pin(m2)
        var = jnp.sum(m2, axis=1, keepdims=True) * (1.0 / D)
        yield from _latency()
        return mean, lax.rsqrt(gate(jnp.broadcast_to(var, (16, 128))) + EPS)

    def d_fwd_rows(b, lb, from_input=False):
        if from_input:
            c, t = divmod(b, 8)
            xs = [_unpack(io32[j, lb, c, pl.ds(t // 2, 16, stride=4), :], t % 2) for j in range(NT)]
            for j in range(NT):
                xres[b, j, r16(lb), :] = xs[j]
        else:
            xs = load_x(b, lb)

        def emit(r, v):
            pin(v)
            ubuf[b % RING, r, r16(lb), :] = v.astype(BF16)

        inv = yield from _d_butterfly_fwd([gate(x) if j < 4 else x for j, x in enumerate(xs)], emit, pin, gate, from_input)
        inv = jnp.broadcast_to(inv, (16, 128))
        pin(inv)
        put(uout.at[b % RING, 8, r16(lb), :], inv)

    def d_dots(b, base, per_tick):
        for r in range(8):
            o = _dot(lhs(ubuf32[b % RING, r]), bf(small32[base + r]))
            put(uout.at[b % RING, r], o)
            if r % per_tick == per_tick - 1 and r < 7:
                yield

    def d_dots_wide(b):
        for ct, (ra, rb) in enumerate(PAIRS):
            u = lhs(ubuf32[b % RING, ra], ubuf32[b % RING, rb])
            for i, r in enumerate((ra, rb)):
                o = _dot(u, bf(wide32[2 * ct + i]))
                put(uout.at[b % RING, r], ticking(o) if i else o)
            if ct < 3:
                yield

    def d_fwd_cols(b, ct, is_wide):
        c, t = divmod(b, 8)
        ra, rb = PAIRS[ct]
        lane = _lane(16)
        lo = lane < 64
        z, x0 = [], []
        for lb in range(4):
            a, bb, inv = (uout[b % RING, r, r16(lb), :] for r in (ra, rb, 8))
            inv = gate(inv)
            a, bb = a * inv, bb * inv
            if is_wide:
                if ct == 0:
                    x0.append(pltpu.roll(bb, t, 1) if t else bb)
                    bb = jnp.where(lane == 0, 0.0, bb)
                z.append((a, bb))
                continue
            if ct == 0:
                x0.append(pltpu.roll(a, (t + 64) % 128, 1))
                a = jnp.where(lane == 64, 0.0, a)
            im = jnp.where(lo, bb, a)
            z.append((jnp.where(lo, a, bb), _swap(im)))
        if not is_wide:
            yield from _latency()
        for e, (re, im) in enumerate(_dft4(z, False)):
            words = pack(re, im)
            pin(words)
            put(zin.at[ct, t * 4 + e, r16(c), :], words)
        if is_wide and ct == 0:
            yield from _latency()
        for lb, v in enumerate(x0):
            ls = pl.ds(64 * lb + 16 * c, 16)
            prev = jnp.zeros((16, 128), F32) if t == 0 else side[0, ls, :]
            v = jnp.where(lane == t, v, prev)
            pin(v)
            put(side.at[0, ls, :], v)

    def add_d_fwd(sched, tick, b, gap, per_tick=4, from_input=False):
        for lb in range(4):
            sched.add(tick + lb * gap, d_fwd_rows(b, lb, from_input))
        tick = int(tick + 3 * gap) + XGAP + 1
        sched.add(tick, d_dots_wide(b) if from_input else d_dots(b, 0, per_tick))
        for ct in range(4):
            sched.add(tick + 8 // per_tick + 3 + ct * gap, d_fwd_cols(b, ct, from_input))
        return int(tick + 8 // per_tick + 3 + 3 * gap) + XGAP + 1

    def side_path():
        vt = side[0].T[0:8]
        yield
        zero8 = jnp.zeros((8, 256), F32)
        u = _dot(jnp.concatenate([vt, zero8], axis=0).astype(BF16), f256[...])[0:8]
        twr, twi = tw_ref[0:8, :], tw_ref[8:16, :]
        ur, ui = u[:, 0:256], u[:, 256:512]
        pad = jnp.zeros((112, 256), BF16)
        for _ in range(4):
            yield
        uu = jnp.concatenate([ur * twr - ui * twi, ur * twi + ui * twr], axis=0).astype(BF16)
        xk = _dot(d8_ref[0], jnp.concatenate([uu, pad], axis=0))
        for _ in range(4):
            yield
        wr = jnp.concatenate([side[1, 0:8, :], side[1, 16:24, :]], axis=1)
        wi = jnp.concatenate([side[1, 8:16, :], side[1, 24:32, :]], axis=1)
        xr, xi = xk[0:8], xk[8:16]
        yy = jnp.concatenate([xr * wr - xi * wi, xr * wi + xi * wr], axis=0).astype(BF16)
        p = _dot(d8_ref[1], jnp.concatenate([yy, pad], axis=0))
        for _ in range(4):
            yield
        twr, twi = tw_ref[0:8, :], tw_ref[8:16, :]
        pr, pi = p[0:8], p[8:16]
        g = jnp.concatenate([pr * twr + pi * twi, pi * twr - pr * twi], axis=1)
        g = jnp.concatenate([g, jnp.zeros((8, 512), F32)], axis=0).astype(BF16)
        y0 = _dot_nt(g, f256[...])
        for _ in range(4):
            yield
        put(side.at[2], jnp.concatenate([y0, jnp.zeros((112, 256), F32)], axis=0).T)

    def s_fwd(u, t):
        ct, e = divmod(u, 4)
        put(ybuf.at[u % NY, t], ticking(_dot(lhs(sfw32[t * 4 + e]), bf(zin[ct, t * 4 + e]))))

    def s_filter(u, g):
        ct, e = divmod(u, 4)
        z = [tuple(ybuf[u % NY, t, pl.ds(g * 16 + i, 8), :] for i in (0, 8))
             for t in range(8)]
        z[0], z[1] = [tuple(gate(v, SGLAG if u * 8 + g < 122 - S_LAG else SGLAG2) for v in zz) for zz in z[0:2]]
        xk = _dft8(z, False)
        for k2 in range(8):
            wr = wf[0, ct, e, k2, pl.ds(g * 8, 8), :]
            wi = wf[1, ct, e, k2, pl.ds(g * 8, 8), :]
            re, im = xk[k2]
            xk[k2] = (re * wr - im * wi, re * wi + im * wr)
        for t, (re, im) in enumerate(_dft8(xk, True)):
            words = pack(re, im)
            pin(words)
            put(fbuf.at[u % NY, t, pl.ds(g * 8, 8), :], words)

    def s_inv(u, t):
        ct, e = divmod(u, 4)
        o = _dot(lhs(siv32[t * 4 + e]), bf(fbuf[u % NY, t]))
        put(zout.at[ct, t * 4 + e], ticking(o) if u * 8 + t >= 110 - S_LAG else o)

    def add_s_stage(sched, early, ready, t1):
        ahead = 8 + S_LAG
        tick = early
        for t in sorted(range(8), key=lambda t: ready[t]):
            for i in range(t, ahead, 8):
                tick = max(tick + 0.5, ready[t])
                sched.add(tick, _once(s_fwd, i // 8, t))
        t1 = max(t1, int(tick) + 1)
        sched.add(max(max(ready), t1), side_path())
        for i in range(128):
            if i + ahead < 128:
                sched.add(t1 + i, _once(s_fwd, *divmod(i + ahead, 8)))
            sched.add(t1 + i, _once(s_filter, *divmod(i, 8)))
            sched.add(t1 + 9 + (i if i < 120 else 120 + (i - 120) // 4), _once(s_inv, *divmod(i, 8)))
        return [t1 + 32 * ct + 40 for ct in range(3)] + [t1 + 131]

    def d_inv_cols(b, ct):
        c, t = divmod(b, 8)
        ra, rb = PAIRS[ct]
        lane = _lane(16)
        lo = lane < 64
        u = [(zout[ct, t * 4 + e, r16(c), :], zout[ct, t * 4 + e, r16(4 + c), :]) for e in range(4)]
        u[0], u[1] = tuple(map(gate, u[0])), tuple(map(gate, u[1]))
        z = _dft4(u, True)
        z = [(re, _swap(im)) for re, im in z]
        if ct == 0:
            y0 = [pltpu.roll(side[2, pl.ds(64 * lb + 16 * c, 16), :], 64 - t, 1) for lb in range(4)]
        yield from _latency()
        for lb, (re, sw) in enumerate(z):
            sw = gate(sw)
            a, bb = jnp.where(lo, re, sw), jnp.where(lo, sw, re)
            if ct == 0:
                a = jnp.where(lane == 64, y0[lb], a)
            pin(a, bb)
            ubuf[b % RING, ra, r16(lb), :] = a.astype(BF16)
            ubuf[b % RING, rb, r16(lb), :] = bb.astype(BF16)

    def d_inv_rows(b, lb, stats):
        u = [uout[b % RING, r, r16(lb), :] for r in range(8)]
        ys = yield from _d_butterfly_inv([gate(v) if r < 4 else v for r, v in enumerate(u)], pin, gate)
        xs = [x + y for x, y in zip(load_x(b, lb), ys)]
        for j in range(NT):
            put(xres.at[b, j, r16(lb), :], xs[j])
        stats[b, lb] = yield from ln_stats(xs)
        if b % 2:
            for j in range(4):
                a = [(xres[bb, j + o, r16(lb), :] - stats[bb, lb][0]) * stats[bb, lb][1]
                     for bb in (b - 1, b) for o in (0, 4)]
                a[0], a[3] = gate(a[0]), gate(a[3])
                for k, v in enumerate(_strassen_lhs(*a)):
                    if k not in (2, 3):
                        pin(v)
                    abuf[b // 2, k, j, r16(lb), :] = v.astype(BF16)
                if j < 3:
                    yield

    def add_d_inv(sched, tick, b, gap, stats, per_tick=4, cols=None):
        cols = cols or [tick + ct * gap for ct in range(4)]
        for ct in range(4):
            sched.add(cols[ct], d_inv_cols(b, ct))
        tick = int(cols[3]) + XGAP + 1
        sched.add(tick, d_dots(b, 8, per_tick))
        tick += 8 // per_tick + 3
        for lb in range(4):
            sched.add(tick + lb * gap, d_inv_rows(b, lb, stats))
        return int(tick + 3 * gap) + 3 * XGAP + 1 + 4

    def gemm(lhs32, rhs32, jobs, sink):
        for slot, b, n in jobs:
            m = {}
            for k in (6, 5, 0, 3, 1, 4, 2):
                m[k] = ticking(_dot(lhs(*[lhs32[slot, k, j] for j in range(4)]), bf(rhs32[n // 2, k])))
                if k == 0:
                    c11, c22 = m[6] - m[0], m[5] - m[0]
                elif k == 3:
                    c11 = c11 - m[3]
                elif k == 1:
                    sink(b + 1, n, m[1] - m[3])
                    c22 = c22 - m[1]
                elif k == 4:
                    sink(b, n, c11 - m[4])
                elif k == 2:
                    sink(b, n + 1, m[4] - m[2])
                    sink(b + 1, n + 1, c22 - m[2])
                yield

    def qkv_sink(b, n, o):
        c, t = divmod(b, 8)
        dst = (qbuf, kbuf, vbuf)[n // NT]
        for lb in range(4):
            put(dst.at[n % NT, t, pl.ds(8 + 64 * lb + 16 * c, 16), :], o[lb * 16:(lb + 1) * 16])
        if b == 0 and n >= NT:
            first = jnp.broadcast_to(o[0:1], (8, 128))
            for tt in range(8):
                dst[n % NT, tt, pl.ds(0, 8), :] = first

    def out_rows(r, i, last):
        c, t = divmod(r, 8)
        return (c * 8 + t % 2 * 4 + i, t // 2) if last and c == 0 else (r, i)

    def out_sink(last, r, n, o):
        for i in range(4):
            b, lb = out_rows(r, i, last)
            put(xres.at[b, n, r16(lb), :], xres[b, n, r16(lb), :] + o[i * 16:(i + 1) * 16])

    def attention(b, lb, h):
        c, t = divmod(b, 8)
        scale = HEAD_DIM ** -0.5
        r0 = 8 + 64 * lb + 16 * c + 8 * h
        src = [((t - 2 * w) % 8, -((t - 2 * w) // 8)) for w in range(WIN)]
        acc = [None] * WIN
        for j in range(NT):
            q = gate(qbuf[j, t, pl.ds(r0, 8), :])
            for w, (ts, sh) in enumerate(src):
                p = q * kbuf[j, ts, pl.ds(r0 - sh, 8), :]
                acc[w] = p if j == 0 else acc[w] + p
            if j % 2 and j < NT - 1:
                pin(*acc)
                yield
        part = [(r, pltpu.roll(r, 64, 1)) for r in acc]
        yield from _latency()
        part = [r + rr for r, rr in part]
        part = [(r, pltpu.roll(r, 32, 1)) for r in part]
        yield from _latency()
        logits = [r + rr for r, rr in part]
        if r0 == 8:
            sub = lax.broadcasted_iota(jnp.int32, (8, 128), 0)
            logits = [jnp.where(sub >= sh, r, -1e9 / scale) if sh else r
                      for r, (_, sh) in zip(logits, src)]
        logits[0] = gate(logits[0])
        m = _tree(jnp.maximum, logits)
        ps = [jnp.exp2((r - m) * (scale * float(np.log2(np.e)))) for r in logits]
        total = _tree(_add, ps)
        pin(total)
        inv = pltpu.reciprocal(total, approx=True)
        inv = inv * (2.0 - total * inv)
        for j in range(NT):
            if j % 2 == 0:
                yield
                ps[0], ps[4] = gate(ps[0]), gate(ps[4])
            o = _chain(_add, [ps[w] * vbuf[j, ts, pl.ds(r0 - sh, 8), :]
                              for w, (ts, sh) in enumerate(src)]) * inv
            pin(o)
            put(qbuf.at[j, t, pl.ds(r0, 8), :], o)

    def out_operands(r, i, last):
        for j in range(4):
            a = [qbuf[j + o, b % 8, pl.ds(8 + 64 * lb + 16 * (b // 8), 16), :]
                 for b, lb in (out_rows(r, i, last), out_rows(r + 1, i, last)) for o in (0, 4)]
            a[0], a[3] = gate(a[0]), gate(a[3])
            for k, v in enumerate(_strassen_lhs(*a)):
                if k not in (2, 3):
                    pin(v)
                obuf[r // 2, k, j, r16(i), :] = v.astype(BF16)
            if j < 3:
                yield

    def store_rows(b, lb):
        c, t = divmod(b, 8)
        for j in range(NT):
            words = pack(xres[b, j, r16(lb), :], xres[b + 1, j, r16(lb), :])
            pin(words)
            io32[j, lb, c, pl.ds(t // 2, 16, stride=4), :] = words

    unit_ticks = NT + 2 * XGAP
    step = 2
    out_ticks = 28

    def add_proj(sched, tick, c, lo, hi):
        jobs = [(b // step, b, n) for b in range(8 * c, 8 * c + 8, step) for n in range(lo, hi, step)]
        sched.add(tick, gemm(abuf32, wqkv32, jobs, qkv_sink))
        return tick + len(jobs) * out_ticks * step // NT

    def add_attention(sched, tick, pace, rows, last):
        units = [(r, i, half, h) for r in rows[::2] for i in range(4) for half in range(2) for h in range(2)]
        for n, (r, i, half, h) in enumerate(units):
            sched.add(tick + n * pace, attention(*out_rows(r + half, i, last), h))
            if half and h:
                sched.add(int(tick + n * pace) + unit_ticks, out_operands(r, i, last))

    def add_out(sched, tick, rows, last):
        jobs = [(r // 2, r, n) for r in rows[::2] for n in range(0, NT, 2)]
        sched.add(tick, gemm(obuf32, wo32, jobs, functools.partial(out_sink, last)))

    def add_tail(sched, tick, rows, last):
        ready = {}
        for i, r in enumerate(rows):
            t0 = tick + (i // 2 + 1) * out_ticks
            fast = i >= len(rows) - (2 if last else 4)
            if not last:
                t0 += 0 if fast else 3 + i % 2 * out_ticks // 2
                ready[r % 8] = add_d_fwd(sched, t0, r, i % 2 if fast else out_ticks / 8)
            elif r % 2:
                c, p = r // 8, r % 8 // 2
                gap = 0 if fast else 3
                for j in range(4):
                    sched.add(t0 + (j + 1) * gap, _once(store_rows, *((r - 1, j) if c else (2 * j, p))))
                for lb in ([p] if c == 0 else range(4) if p == 3 else []):
                    sched.add(t0 + 5 * gap + 1, _once(start, out_copies(c, lb)))
        return ready

    q_ticks = 8 * out_ticks // step
    att_ticks = unit_ticks + 1 + 2
    order = [(a + 8) % NB for a in range(NB)]

    def add_attention_block(sched, cols, last):
        stats = {}
        t0 = max([add_d_inv(sched, 0, b, 0, stats, 4, cols) for b in range(step)])
        if not last:
            sched.add(cols[3] - KLEAD, _once(wait, qkv_copies(1) + dmat_cp))
            done = add_prep_wqkv(sched, cols[3] - KLEAD, 1, KPACE, [7] * 4)
            t0 = max(t0, done[0])
            assert all(d <= t0 + p * out_ticks / 4 for p, d in enumerate(done))
            sched.add(t0 + out_ticks, _once(wait, qkv_copies(2)))
            sched.add(t0 + out_ticks, _once(start, qkv_copies(0)))
            done = add_prep_wqkv(sched, t0 + out_ticks, 2, 2 * out_ticks - 6, [out_ticks - 4] * 4)
            assert all(d <= t0 + q_ticks + p * out_ticks for p, d in enumerate(done))
            sched.add(t0 + 2 * q_ticks, _once(wait, qkv_copies(0)))
            sched.add(t0 + 2 * q_ticks, _once(start, wo_copies))
            done = add_prep_wqkv(sched, t0 + 2 * q_ticks, 0, q_ticks - 10, [q_ticks / 4] * 4)
            assert done[-1] <= t0 + 4 * q_ticks
            sched.add(t0 + 8 * q_ticks, _once(wait, wo_copies))
            for i in range(32):
                sched.add(t0 + 8 * q_ticks + i * q_ticks / 16, _once(prep_wo, *divmod(i, 8)))
        tick, kv_start, q_start = t0, {}, {}
        for kind, c in ("k0", "k1", "q1", "k2", "q2", "k3", "q3", "q0"):
            if kind == "k":
                kv_start[int(c)] = tick
                if c == "0" and not last:
                    tick = add_proj(sched, tick, 0, NT, 2 * NT)
                    jobs = [(b // step, b, n) for n in range(2 * NT, 3 * NT, step) for b in range(0, 8, step)]
                    sched.add(tick, gemm(abuf32, wqkv32, jobs, qkv_sink))
                    tick += q_ticks
                    continue
                tick = add_proj(sched, tick, int(c), NT, 3 * NT)
            else:
                q_start[int(c)] = tick
                tick = add_proj(sched, tick, int(c), 0, NT)
        pace = 2 * out_ticks / step
        for b in range(step, NB):
            due = kv_start[b // 8] + (b % 8 // step) * (2 if last or b >= 8 else 1) * out_ticks
            gap = min(1 + (b - step) * 0.5, DGAP1 if last else DGAP0)
            pace = DPACE1 if last else DPACE0
            at = (b - step) * pace
            at = t0 + at + max(0, at - 4 * q_ticks - out_ticks) * DSLOW
            if not last and b < 8:
                at, gap = max(cols[3], t0 + (b // step - 1) * out_ticks - (step - b % step) * 8), 1
            end = add_d_inv(sched, at, b, gap, stats)
            assert end <= due, (b, end, due)
        begin = [q_start[c] + out_ticks + 3 for c in (1, 2, 3)] + [tick + (ATT1 if last else ATT0)]
        begin.append(tick + (NB // step - 1) * out_ticks - att_ticks)
        for i, c in enumerate((1, 2, 3, 0)):
            pace = (begin[i + 1] - begin[i]) / 64
            assert begin[i] >= max(kv_start[c], kv_start[(c - 1) % 4]) + 2 * q_ticks
            for p in range(4):
                assert begin[i] + 16 * p * pace >= q_start[c] + (4 if last and c == 0 else p + 1) * out_ticks
                assert begin[i] + (16 * p + 15) * pace + att_ticks <= tick + (4 * i + p) * out_ticks + 1e-6
            add_attention(sched, begin[i], pace, range(8 * c, 8 * c + 8), last)
        add_out(sched, tick, order, last)
        return tick + (NB // step) * out_ticks, add_tail(sched, tick, order, last)

    def add_input(sched):
        ready = {}
        after = (x_copies(2), x_copies(3) + perm_cp + w_copies(0) + w_copies(1),
                 w_copies(2) + w_copies(3), w_copies(4))
        for c in range(NC):
            sched.add(c * 32, _once(wait, x_copies(c)))
            sched.add(c * 32, _once(start, after[c]))
            for t in range(8):
                ready[t] = add_d_fwd(sched, c * 32 + t * 4, c * 8 + t, 1, 2, True)
        return 128 + 9, ready

    def add_filter_prep(sched, tick):
        after = {0: w_copies(5), 1: w_copies(6), 2: w_copies(7), 3: f256_cp + dmat_cp,
                 5: qkv_copies(1), 7: qkv_copies(2)}
        begin = [F0 + g * (tick - F0) / 4 for g in range(4)] + [tick + 4 * g for g in range(5)]
        for g in range(8):
            sched.add(begin[g], _once(wait, w_copies(g) + ([] if g else perm_cp)))
            sched.add(begin[g], _once(start, after.get(g, [])))
            for m in range(4):
                sched.add(begin[g] + m * (begin[g + 1] - begin[g]) / 4,
                          _once(prep_filter, g // 4, g % 4 * 4 + m))
        sched.add(begin[8] + 1, _once(wait, f256_cp))
        return begin[8] + 2

    sched = _Schedule()

    def phase(fn, *args):
        fn(sched, *args)
        sched.run()
        token.clear()
        clock.clear()

    start(x_copies(0))
    for ref in (abuf32, obuf32, ubuf32, wo32, sfw32, siv32, wide32):
        put(ref.at[(0,) * (len(ref.shape) - 2) + (pl.ds(0, 8),)], jnp.zeros((8, 128), U32))
    make_wide()
    start(x_copies(1))
    for t in range(8):
        make_s_fwd(t)
    for e in range(4):
        make_s_inv(e)
    tick, ready = add_input(sched)
    cols = add_s_stage(sched, tick, ready, add_filter_prep(sched, tick))
    tick, ready = add_attention_block(sched, cols, False)
    cols = add_s_stage(sched, tick, ready, tick)
    add_attention_block(sched, cols, True)
    sched.run()
    for c in range(NC):
        for lb in range(4):
            wait(out_copies(c, lb))


@jax.jit
def pallas_interleave_layers__spectral_gfnet__sliding_local_dilated__prompt_kernel(
    A_x: jax.Array,
    A_w_r: jax.Array,
    A_w_i: jax.Array,
    B_x: jax.Array,
    B_wqkv: jax.Array,
    B_wo: jax.Array,
):
    del B_x
    assert A_x.shape == (1, S, D) and A_w_r.shape == (S, D // 2 + 1)
    cst = _constants()
    x = A_x.astype(BF16).reshape(4, NC, 128, D)
    wr, wi = A_w_r.astype(BF16).T, A_w_i.astype(BF16).T
    hbm = pl.BlockSpec(memory_space=pl.ANY)
    edge = pl.BlockSpec((16, S), lambda i: (D // 32, 0))
    vm = pltpu.VMEM
    out = pl.pallas_call(
        _kernel,
        grid=(1,),
        in_specs=[hbm, hbm, hbm, edge, edge, hbm, hbm, hbm, hbm,
                  pl.BlockSpec((24, 256), lambda i: (0, 0)),
                  pl.BlockSpec((2, 16, 128), lambda i: (0, 0, 0))],
        out_specs=hbm,
        out_shape=jax.ShapeDtypeStruct((4, NC, 128, D), BF16),
        scratch_shapes=[
            vm((NT, 4, NC, 128, 128), BF16),
            vm((17, 128, 128), BF16),
            vm((32, 128, 128), BF16),
            vm((32, 128, 128), BF16),
            vm((256, 512), BF16),
            vm((2, 16, 512, 128), BF16),
            vm((2, 4, 4, 8, 64, 128), F32),
            vm((3 * NT, D, 128), BF16),
            vm((NT, D // 2, 128), U32),
            vm((12, 7, 512, 128), BF16),
            vm((NT, D, 128), BF16),
            vm((4, 7, 512, 128), BF16),
            vm((NB, NT, 64, 128), F32),
            vm((4, 32, 64, 128), U32),
            vm((4, 32, 128, 128), F32),
            vm((NY, 8, 128, 128), F32),
            vm((NY, 8, 64, 128), U32),
            vm((RING, 8, 64, 128), BF16),
            vm((RING, 9, 64, 128), F32),
            vm((NB // 2, 7, 4, 64, 128), BF16),
            vm((NB // 2, 7, 4, 64, 128), BF16),
            vm((NT, 8, 264, 128), F32),
            vm((NT, 8, 264, 128), F32),
            vm((NT, 8, 264, 128), F32),
            vm((3, 256, 128), F32),
            vm((8, 256, 128), BF16),
            pltpu.SemaphoreType.DMA((NC,)),
            pltpu.SemaphoreType.DMA((3,)),
            pltpu.SemaphoreType.DMA((8,)),
            pltpu.SemaphoreType.DMA((3,)),
            pltpu.SemaphoreType.DMA(()),
            pltpu.SemaphoreType.DMA(()),
        ],
        compiler_params=pltpu.CompilerParams(
            dimension_semantics=("arbitrary",), vmem_limit_bytes=120 * 2**20),
    )(x, wr, wi, wr, wi, B_wqkv.astype(BF16), B_wo.astype(BF16),
      cst["small"], cst["f256"], cst["tw"], cst["d8"])
    return out.reshape(1, S, D)
```

```python
import functools

import jax
import jax.numpy as jnp
import numpy as np
from jax import lax
from jax.experimental import pallas as pl
from jax.experimental.pallas import tpu as pltpu

S, D = 2048, 1024
NT = D // 128
NC = 4
WIN = 8
HEAD_DIM = 32
EPS = 1e-5
F32, BF16, U32 = jnp.float32, jnp.bfloat16, jnp.uint32
PAIRS = ((0, 4), (1, 7), (2, 6), (3, 5))
RSQ2 = float(np.sqrt(0.5))
NB = S // 64

RING = 8
NY = 4
XGAP = 3
GLAG = 4
ALAG = 5
SGLAG = 3
SGLAG2 = 4
S_LAG = 4
F0 = 104
KLEAD = 44
KPACE = 52
DGAP0 = 4.75
DGAP1 = 4.2
DPACE0 = 21
DPACE1 = 15.5
DSLOW = 0.6
SYNC = 3
ATT0 = 25
ATT1 = 80


def _residues(r):
    return (0, 8) if r == 0 else (r, 16 - r)


def _d_matrices():
    n = np.arange(64)[:, None]
    a = np.arange(32)
    fwd = np.zeros((8, 128, 128))
    inv = np.zeros((8, 128, 128))
    for r in range(8):
        kd = np.concatenate([16 * a + p for p in _residues(r)])
        weight = np.full(64, 2.0)
        if r == 0:
            kd[0], weight[0] = D // 2, 1.0
            ph = np.exp(-2j * np.pi * n * kd[None, :] / D)
            sgn = np.where(kd % 16 == 0, 1.0, -1.0)[None, :]
            m = np.concatenate([ph, ph * sgn], axis=0)
            re, im = m.real.copy(), m.imag.copy()
            ire, iim = re.copy(), im.copy()
            im[:, 0] = 1.0
            iim[:, 0] = 1.0
        else:
            p = 12 if r == 4 else r
            ph = np.exp(-2j * np.pi * n * kd[None, :] / D)
            si = np.where(kd % 16 == p, 1.0, -1.0)[None, :]
            m = np.concatenate([ph, 1j * si * ph], axis=0)
            re, im = m.real, m.imag
            ire, iim = re, im
        swapped = r in (4, 7, 6, 5)
        cols = [im, re] if swapped else [re, im]
        icols = [iim * weight, ire * weight] if swapped else [ire * weight, iim * weight]
        fwd[r] = np.concatenate(cols, axis=1)
        inv[r] = np.concatenate(icols, axis=1).T / D
    return fwd, inv


def _side_matrices():
    l = np.arange(256)
    f = np.exp(-2j * np.pi * ((l[:, None] * l[None, :]) % 256) / 256)
    f256 = np.concatenate([f.real, f.imag], axis=1)
    t = np.arange(8)
    tw = np.exp(-2j * np.pi * t[:, None] * l[None, :] / S)
    tw = np.concatenate([tw.real, tw.imag, np.zeros((8, 256))], axis=0)
    g = np.exp(-2j * np.pi * t[:, None] * t[None, :] / 8)
    d8 = np.zeros((2, 16, 128))
    d8[0, :, :16] = np.block([[g.real, -g.imag], [g.imag, g.real]])
    d8[1, :, :16] = d8[0, :, :16].T / S
    return f256, tw, d8


def _filter_rows():
    p = np.zeros((1, 128, 128))
    for k in range(32):
        for e in range(4):
            p[0, e * 32 + k, 4 * k + e] = 1.0
    return p


@functools.lru_cache(maxsize=None)
def _constants():
    dfw, div = _d_matrices()
    f256, tw, d8 = _side_matrices()
    small = np.concatenate([dfw, div, _filter_rows()], axis=0)
    b = lambda x: np.asarray(x, np.float32).astype(BF16)
    return dict(small=b(small), f256=b(f256),
                tw=np.asarray(tw, np.float32), d8=b(d8))


def _dot(a, b):
    return jnp.dot(a, b, preferred_element_type=F32)


def _dot_nt(a, b):
    return lax.dot_general(a, b, (((1,), (1,)), ((), ())), preferred_element_type=F32)


def _tree(op, xs):
    xs = list(xs)
    while len(xs) > 1:
        xs = [op(xs[i], xs[i + 1]) if i + 1 < len(xs) else xs[i] for i in range(0, len(xs), 2)]
    return xs[0]


def _chain(op, xs):
    return functools.reduce(op, xs)


def _lane(rows):
    return lax.broadcasted_iota(jnp.int32, (rows, 128), 1)


def _swap(x):
    return pltpu.roll(x, 64, 1)


def _unpack(w, i):
    return pltpu.unpack_elementwise(w, index=i, packed_dtype=BF16, unpacked_dtype=F32)


def _latency():
    for _ in range(XGAP):
        yield


def _add(a, b):
    return a + b


def _row_mean(xs):
    return jnp.sum(_tree(_add, xs), axis=1, keepdims=True) * (1.0 / D)


def _twiddle16(r, x, y):
    lo = _lane(x.shape[0]) < 64
    wr, wi = float(np.cos(np.pi * r / 8)), float(-np.sin(np.pi * r / 8))
    cross = jnp.where(lo, 0.0, wr)
    return x * jnp.where(lo, 1.0, wi) + y * cross, y * jnp.where(lo, 1.0, -wi) + x * cross


def _d_butterfly_fwd(a, emit, pin, gate, wide):
    s = [a[j] + a[j + 4] for j in range(4)]
    e, o = s[0] + s[2], s[1] + s[3]
    total, t4 = e + o, e - o
    emit(4, t4)
    d0, nd2 = a[0] - a[4], a[6] - a[2]
    d1, d3 = a[1] - a[5], a[3] - a[7]
    p, q = (d1 - d3) * RSQ2, (d1 + d3) * -RSQ2
    ts = {1: (d0 + p, q + nd2), 2: (s[0] - s[2], s[3] - s[1]), 3: (d0 - p, q - nd2)}
    mean8 = jnp.sum(total, axis=1, keepdims=True) * (1.0 / 128)
    if wide:
        for r, (tr, ti) in ts.items():
            emit(r, tr)
            emit(8 - r, ti)
    else:
        ab = {r: _twiddle16(r, *t) for r, t in ts.items()}
        ab = {r: (a, _swap(b)) for r, (a, b) in ab.items()}
    dev = _tree(_add, [v * v for t in ts.values() for v in t]) * 2.0 + t4 * t4
    pin(dev)
    yield from _latency()
    t0 = total - mean8
    emit(0, t0)
    var = jnp.sum(dev + t0 * t0, axis=1, keepdims=True) * (1.0 / (NT * D))
    if not wide:
        for r, (x, y) in ab.items():
            emit(r, x + y)
            emit(8 - r, x - y)
    yield from _latency()
    return lax.rsqrt(var + EPS)


def _d_butterfly_inv(u, pin, gate):
    ab = {r: (u[r] + u[8 - r], _swap(u[r] - u[8 - r])) for r in (1, 2, 3)}
    e, o = u[0] + u[4], u[0] - u[4]
    yield from _latency()
    ts = {r: _twiddle16(r, x, gate(y)) for r, (x, y) in ab.items()}
    pin(*[v for t in ts.values() for v in t])
    yield
    s = [e + ts[2][0], o - ts[2][1], e - ts[2][0], o + ts[2][1]]
    p = (ts[1][0] - ts[3][0]) * RSQ2
    q = (ts[1][1] + ts[3][1]) * RSQ2
    d0, d1, d2, nd3 = ts[1][0] + ts[3][0], p - q, ts[3][1] - ts[1][1], p + q
    return [s[0] + d0, s[1] + d1, s[2] + d2, s[3] - nd3,
            s[0] - d0, s[1] - d1, s[2] - d2, s[3] + nd3]


def _strassen_lhs(a11, a12, a21, a22):
    return [a11 + a22, a21 + a22, a11, a22, a11 + a12, a21 - a11, a12 - a22]


def _strassen_rhs(b11, b12, b21, b22):
    return [b11 + b22, b11, b22 - b12, b11 - b21, b22, b11 + b12, b21 + b22]


def _cadd(a, b):
    return a[0] + b[0], a[1] + b[1]


def _csub(a, b):
    return a[0] - b[0], a[1] - b[1]


def _dft4(z, inverse):
    a, b = _cadd(z[0], z[2]), _csub(z[0], z[2])
    c, d = _cadd(z[1], z[3]), _csub(z[1], z[3])
    minus = (b[0] + d[1], b[1] - d[0])
    plus = (b[0] - d[1], b[1] + d[0])
    return [_cadd(a, c), plus if inverse else minus, _csub(a, c), minus if inverse else plus]


def _dft8(z, inverse):
    ev = _dft4(z[0::2], inverse)
    od = _dft4(z[1::2], inverse)
    out = [None] * 8
    out[0], out[4] = _cadd(ev[0], od[0]), _csub(ev[0], od[0])
    (er, ei), (x, y) = ev[2], od[2]
    minus, plus = (er + y, ei - x), (er - y, ei + x)
    out[2], out[6] = (plus, minus) if inverse else (minus, plus)
    for k in (1, 3):
        (er, ei), (x, y) = ev[k], od[k]
        sm, df = (x + y) * RSQ2, (x - y) * RSQ2
        if not inverse:
            if k == 1:
                out[1], out[5] = (er + sm, ei - df), (er - sm, ei + df)
            else:
                out[3], out[7] = (er - df, ei - sm), (er + df, ei + sm)
        else:
            if k == 1:
                out[1], out[5] = (er + df, ei + sm), (er - df, ei - sm)
            else:
                out[3], out[7] = (er - sm, ei + df), (er + sm, ei - df)
    return out


class _Schedule:
    def __init__(self):
        self.pending = []

    def add(self, tick, gen):
        self.pending.append((int(tick), len(self.pending), gen))

    def run(self):
        pending = sorted(self.pending, key=lambda p: p[:2])
        active, tick, i = [], 0, 0
        while active or i < len(pending):
            while i < len(pending) and pending[i][0] <= tick:
                active.append(pending[i][2])
                i += 1
            for g in list(active):
                if next(g, 0) == 0:
                    active.remove(g)
            tick += 1
        self.pending = []


def _once(fn, *args):
    fn(*args)
    return
    yield


def _kernel(x_hbm, wr_hbm, wi_hbm, wr_edge, wi_edge, wqkv_hbm, wo_hbm,
            small_hbm, f256_hbm, tw_ref, d8_ref,
            out_hbm,
            io, small, sfw, siv, f256, wraw, wf, wqkv_raw, wtmp, wqkv, wo_raw, wo,
            xres, zin, zout, ybuf, fbuf, ubuf, uout, abuf, obuf, qbuf, kbuf, vbuf, side,
            wide, sem_x, sem_c, sem_w, sem_qkv, sem_wo, sem_out):

    def x_copies(c):
        return [pltpu.make_async_copy(x_hbm.at[:, c, :, pl.ds(j * 128, 128)], io.at[j, :, c],
                                      sem_x.at[c]) for j in range(NT)]

    def out_copies(c, lb):
        return [pltpu.make_async_copy(io.at[j, lb, c], out_hbm.at[lb, c, :, pl.ds(j * 128, 128)],
                                      sem_out) for j in range(NT)]

    perm_cp, dmat_cp, f256_cp = ([pltpu.make_async_copy(s, d, sem_c.at[i])] for i, (s, d) in enumerate((
        (small_hbm.at[pl.ds(16, 1)], small.at[pl.ds(16, 1)]),
        (small_hbm.at[pl.ds(0, 16)], small.at[pl.ds(0, 16)]), (f256_hbm, f256))))

    def w_copies(g):
        src = (wr_hbm, wi_hbm)[g // 4]
        return [pltpu.make_async_copy(src.at[pl.ds(0, 512), pl.ds(m * 128, 128)], wraw.at[g // 4, m],
                                      sem_w.at[g]) for m in range(g % 4 * 4, g % 4 * 4 + 4)]

    def qkv_copies(g):
        return [pltpu.make_async_copy(wqkv_hbm.at[:, pl.ds(g * D + j * 128, 128)],
                                      wqkv_raw.at[g * NT + j], sem_qkv.at[g]) for j in range(NT)]

    wo_copies = [pltpu.make_async_copy(wo_hbm.at[:, pl.ds(j * 128, 128)], wo_raw.at[j], sem_wo)
                 for j in range(NT)]

    def start(cs):
        for cp in cs:
            cp.start()

    def wait(cs):
        for cp in cs:
            cp.wait()

    io32, wraw32, wo_raw32 = io.bitcast(U32), wraw.bitcast(U32), wo_raw.bitcast(U32)
    small32, sfw32, siv32, wide32 = (r.bitcast(U32) for r in (small, sfw, siv, wide))
    wqkv_raw32, wqkv32, wo32 = (r.bitcast(U32) for r in (wqkv_raw, wqkv, wo))
    ubuf32, abuf32, obuf32 = ubuf.bitcast(U32), abuf.bitcast(U32), obuf.bitcast(U32)

    never = tw_ref[16:24, 0:128] != 0.0
    token = []

    def pin(*values):
        for v in values:
            for i in range(0, v.shape[0], 8):
                w = pltpu.bitcast(v[i:i + 8], U32)
                token[:] = [token[0] ^ w if token else w]

    clock = []

    def gate(v, lag=GLAG):
        if len(clock) < lag:
            return v
        head = jnp.where(never, pltpu.bitcast(clock[-lag], v.dtype), v[0:8])
        return head if v.shape[0] == 8 else jnp.concatenate([head, v[8:]], axis=0)

    def ticking(o):
        clock.append(o[0:8])
        del clock[:-16]
        return o

    def lhs(*tiles):
        if not token and len(tiles) == 4 and len(clock) >= SYNC:
            pin(clock[-SYNC])
        if token:
            w = token.pop()
            tiles = [jnp.concatenate([jnp.where(never, w, t[0:8]), t[8:]], axis=0) for t in tiles]
        return jnp.concatenate([pltpu.bitcast(t, BF16) for t in tiles], axis=1)

    def bf(words):
        return pltpu.bitcast(words, BF16)

    def pack(a, b):
        return pltpu.bitcast(pltpu.pack_elementwise([a, b], packed_dtype=BF16), U32)

    def r16(i):
        return pl.ds(i * 16, 16)

    def put(ref, v):
        pltpu.store(ref, v, mask=jnp.ones(v.shape, jnp.bool_))

    def load_x(b, lb):
        return [xres[b, j, r16(lb), :] for j in range(NT)]

    def unit(p):
        angle = (((p + S // 2) & (S - 1)) - S // 2).astype(F32) * (2 * np.pi / S)
        return jnp.cos(angle), jnp.sin(angle)

    def times_row(a, b, i):
        br, bi = (jnp.broadcast_to(v[i:i + 1], (8, 128)) for v in b)
        return a[0] * br - a[1] * bi, a[0] * bi + a[1] * br

    def make_wide():
        row, lane = lax.broadcasted_iota(jnp.int32, (8, 128), 0), _lane(8)
        for ct, (ra, rb) in enumerate(PAIRS):
            res = _residues(ra) + _residues(rb)
            kd = (lane & 31) * 16 + _chain(
                _add, [jnp.where(lane >> 5 == g, p, 0) for g, p in enumerate(res)])
            if ct == 0:
                kd = jnp.where(lane == 0, D // 2, kd)
            fine, coarse = unit(-2 * row * kd), [unit(-16 * (row + 8 * h) * kd) for h in range(2)]
            for a in range(16):
                re, im = times_row(fine, coarse[a // 8], a % 8)
                if ct == 0:
                    even = kd & 7 == 0
                    top = jnp.where(even, re, 0.0), jnp.where(lane == 0, 1.0, jnp.where(even, im, 0.0))
                    bottom = jnp.where(even, 0.0, re), jnp.where(even, 0.0, im)
                else:
                    sign = jnp.where(kd & 7 == ra, 1.0, -1.0)
                    top, bottom = (re, im), (-sign * im, sign * re)
                for i in range(2):
                    wide[2 * ct + i, pl.ds(8 * a, 8), :] = top[i].astype(BF16)
                    wide[2 * ct + i, pl.ds(128 + 8 * a, 8), :] = bottom[i].astype(BF16)

    def make_s_fwd(t):
        row, lane = lax.broadcasted_iota(jnp.int32, (8, 128), 0), _lane(8)
        pos = 8 * (lane >> 1) + t
        fine = unit((lane & 1) * (S // 4) - 4 * row * pos)
        shift, coarse = unit(-row * pos), unit(-32 * row * pos)
        for e in range(4):
            base = times_row(fine, shift, e)
            for g in range(8):
                for i, v in enumerate(times_row(base, coarse, g)):
                    sfw[t * 4 + e, pl.ds(16 * g + 8 * i, 8), :] = v.astype(BF16)

    def make_s_inv(e):
        row, lane = lax.broadcasted_iota(jnp.int32, (8, 128), 0), _lane(8)
        freq = 4 * (lane >> 1) + e
        fine = [v * (1.0 / S) for v in unit((lane & 1) * (S // 4) + 8 * row * freq)]
        shift, coarse = unit(row * freq), unit(64 * row * freq)
        for t in range(8):
            base = times_row(fine, shift, t)
            for g in range(8):
                for i, v in enumerate(times_row(base, coarse, g)):
                    siv[t * 4 + e, pl.ds(64 * i + 8 * g, 8), :] = v.astype(BF16)

    def prep_filter(ri, m):
        sub = lax.broadcasted_iota(jnp.int32, (8, 128), 0)
        edge = (wr_edge, wi_edge)[ri]
        res = {}
        for i in range(8):
            words = wraw32[ri, m, pl.ds(i, 32, stride=8), :]
            res[2 * i], res[2 * i + 1] = _unpack(words, 0), _unpack(words, 1)
        first = res[0][0:8]
        dst = pl.ds((m % 2) * 16 + ri * 8, 8)
        prev = jnp.zeros((8, 128), F32) if m < 2 else side[1, dst, :]
        put(side.at[1, dst, :], jnp.where(sub == m // 2, jnp.broadcast_to(first[0:1], (8, 128)), prev))
        nyq = jnp.broadcast_to(edge[0:1, pl.ds(m * 128, 128)].astype(F32), (8, 128))
        res[0] = jnp.concatenate([jnp.where(sub == 0, nyq, first), res[0][8:]], axis=0)
        for ct, (ra, rb) in enumerate(PAIRS):
            blk = jnp.concatenate([res[p] for p in _residues(ra) + _residues(rb)], axis=0)
            o = _dot_nt(lhs(small32[16]), blk.astype(BF16))
            for e in range(4):
                put(wf.at[ri, ct, e, m // 2, pl.ds((m % 2) * 32, 32), :], o[e * 32:(e + 1) * 32])

    def shuffle(words, index):
        return jnp.take_along_axis(words, index, axis=1)

    def prep_wqkv_tile(g, i, part):
        lane = _lane(8)
        index = (lane & 3) * 32 + (((lane >> 2) - i) & 7) * 4 + (lane >> 5)
        rows = [pl.ds((part * 16 + r) * 8, 8) for r in range(16)]
        ws = [shuffle(gate(wqkv_raw32[g * NT + i, rs, :]), index) for rs in rows]
        yield from _latency()
        for rs, w in zip(rows, ws):
            pin(w)
            put(wtmp.at[i, rs, :], w)

    def prep_wqkv_cross(g, r):
        pos = (_lane(8) >> 2) & 7
        u = [wtmp[(-j) % 8, pl.ds(r * 8, 8), :] for j in range(NT)]
        u[0], u[4] = gate(u[0]), gate(u[4])
        for bit in range(3):
            m = ((pos >> bit) & 1) == 1
            u = [jnp.where(m, u[(j - (1 << bit)) % 8], u[j]) for j in range(NT)]
        for j in range(NT):
            pin(u[j])
            put(wqkv_raw32.at[g * NT + j, pl.ds(r * 8, 8), :], u[j])

    def prep_wqkv_pair(g, p, part):
        lane = _lane(8)
        ws = {}
        for n in range(2):
            index = (lane & 96) | ((lane + 4 * (2 * p + n)) & 31)
            for half in range(2):
                for r in range(part * 2, part * 2 + 2):
                    w = gate(wqkv_raw32[g * NT + 2 * p + n, pl.ds(half * 256 + r * 8, 8), :])
                    ws[r, half, n] = shuffle(w, index) if p + n else w
        yield from _latency()
        for r in range(part * 2, part * 2 + 2):
            quad = [ws[r, half, n] for half in range(2) for n in range(2)]
            ops = [_strassen_rhs(*[_unpack(w, i) for w in quad]) for i in range(2)]
            for k in range(7):
                word = {1: quad[0], 4: quad[3]}.get(k)
                if word is None:
                    word = pack(ops[0][k], ops[1][k])
                    pin(word)
                put(wqkv32.at[g * 4 + p, k, pl.ds(r * 8, 8), :], word)

    def add_prep_wqkv(sched, tick, g, ticks, pair_ticks):
        for i in range(32):
            sched.add(tick + i * ticks / 64, prep_wqkv_tile(g, *divmod(i, 4)))
        tick = int(tick + ticks / 2) + XGAP + 1
        for r in range(64):
            sched.add(tick + r * ticks / 128, _once(prep_wqkv_cross, g, r))
        tick = int(tick + ticks / 2) + 1
        done = []
        for p, n in enumerate(pair_ticks):
            for i in range(16):
                sched.add(tick + i * n / 16, prep_wqkv_pair(g, p, i))
            tick += n
            done.append(int(tick) + XGAP + 1)
        return done

    def prep_wo(p, dp):
        ws = [wo_raw32[2 * p + n, pl.ds(dp + off, 32, stride=16), :] for off in (0, 8) for n in (0, 1)]
        for i in range(2):
            b = [_unpack(w, i) for w in ws]
            r0 = (2 * dp + i) * 32
            for k, v in enumerate(_strassen_rhs(*b)):
                if k not in (1, 4):
                    pin(v)
                wo[p, k, pl.ds(r0, 32), :] = v.astype(BF16)

    def ln_stats(xs):
        lane_mean = _tree(_add, xs) * (1.0 / NT)
        lane_m2 = _tree(_add, [jnp.square(x - lane_mean) for x in xs])
        pin(lane_m2)
        mean = jnp.sum(lane_mean, axis=1, keepdims=True) * (1.0 / 128)
        yield from _latency()
        m2 = lane_m2 + jnp.square(gate(lane_mean) - mean) * float(NT)
        pin(m2)
        var = jnp.sum(m2, axis=1, keepdims=True) * (1.0 / D)
        yield from _latency()
        return mean, lax.rsqrt(gate(jnp.broadcast_to(var, (16, 128))) + EPS)

    def d_fwd_rows(b, lb, from_input=False):
        if from_input:
            c, t = divmod(b, 8)
            xs = [_unpack(io32[j, lb, c, pl.ds(t // 2, 16, stride=4), :], t % 2) for j in range(NT)]
            for j in range(NT):
                xres[b, j, r16(lb), :] = xs[j]
        else:
            xs = load_x(b, lb)

        def emit(r, v):
            pin(v)
            ubuf[b % RING, r, r16(lb), :] = v.astype(BF16)

        inv = yield from _d_butterfly_fwd([gate(x) if j < 4 else x for j, x in enumerate(xs)], emit, pin, gate, from_input)
        inv = jnp.broadcast_to(inv, (16, 128))
        pin(inv)
        put(uout.at[b % RING, 8, r16(lb), :], inv)

    def d_dots(b, base, per_tick):
        for r in range(8):
            o = _dot(lhs(ubuf32[b % RING, r]), bf(small32[base + r]))
            put(uout.at[b % RING, r], o)
            if r % per_tick == per_tick - 1 and r < 7:
                yield

    def d_dots_wide(b):
        for ct, (ra, rb) in enumerate(PAIRS):
            u = lhs(ubuf32[b % RING, ra], ubuf32[b % RING, rb])
            for i, r in enumerate((ra, rb)):
                o = _dot(u, bf(wide32[2 * ct + i]))
                put(uout.at[b % RING, r], ticking(o) if i else o)
            if ct < 3:
                yield

    def d_fwd_cols(b, ct, is_wide):
        c, t = divmod(b, 8)
        ra, rb = PAIRS[ct]
        lane = _lane(16)
        lo = lane < 64
        z, x0 = [], []
        for lb in range(4):
            a, bb, inv = (uout[b % RING, r, r16(lb), :] for r in (ra, rb, 8))
            inv = gate(inv)
            a, bb = a * inv, bb * inv
            if is_wide:
                if ct == 0:
                    x0.append(pltpu.roll(bb, t, 1) if t else bb)
                    bb = jnp.where(lane == 0, 0.0, bb)
                z.append((a, bb))
                continue
            if ct == 0:
                x0.append(pltpu.roll(a, (t + 64) % 128, 1))
                a = jnp.where(lane == 64, 0.0, a)
            im = jnp.where(lo, bb, a)
            z.append((jnp.where(lo, a, bb), _swap(im)))
        if not is_wide:
            yield from _latency()
        for e, (re, im) in enumerate(_dft4(z, False)):
            words = pack(re, im)
            pin(words)
            put(zin.at[ct, t * 4 + e, r16(c), :], words)
        if is_wide and ct == 0:
            yield from _latency()
        for lb, v in enumerate(x0):
            ls = pl.ds(64 * lb + 16 * c, 16)
            prev = jnp.zeros((16, 128), F32) if t == 0 else side[0, ls, :]
            v = jnp.where(lane == t, v, prev)
            pin(v)
            put(side.at[0, ls, :], v)

    def add_d_fwd(sched, tick, b, gap, per_tick=4, from_input=False):
        for lb in range(4):
            sched.add(tick + lb * gap, d_fwd_rows(b, lb, from_input))
        tick = int(tick + 3 * gap) + XGAP + 1
        sched.add(tick, d_dots_wide(b) if from_input else d_dots(b, 0, per_tick))
        for ct in range(4):
            sched.add(tick + 8 // per_tick + 3 + ct * gap, d_fwd_cols(b, ct, from_input))
        return int(tick + 8 // per_tick + 3 + 3 * gap) + XGAP + 1

    def side_path():
        vt = side[0].T[0:8]
        yield
        zero8 = jnp.zeros((8, 256), F32)
        u = _dot(jnp.concatenate([vt, zero8], axis=0).astype(BF16), f256[...])[0:8]
        twr, twi = tw_ref[0:8, :], tw_ref[8:16, :]
        ur, ui = u[:, 0:256], u[:, 256:512]
        pad = jnp.zeros((112, 256), BF16)
        for _ in range(4):
            yield
        uu = jnp.concatenate([ur * twr - ui * twi, ur * twi + ui * twr], axis=0).astype(BF16)
        xk = _dot(d8_ref[0], jnp.concatenate([uu, pad], axis=0))
        for _ in range(4):
            yield
        wr = jnp.concatenate([side[1, 0:8, :], side[1, 16:24, :]], axis=1)
        wi = jnp.concatenate([side[1, 8:16, :], side[1, 24:32, :]], axis=1)
        xr, xi = xk[0:8], xk[8:16]
        yy = jnp.concatenate([xr * wr - xi * wi, xr * wi + xi * wr], axis=0).astype(BF16)
        p = _dot(d8_ref[1], jnp.concatenate([yy, pad], axis=0))
        for _ in range(4):
            yield
        twr, twi = tw_ref[0:8, :], tw_ref[8:16, :]
        pr, pi = p[0:8], p[8:16]
        g = jnp.concatenate([pr * twr + pi * twi, pi * twr - pr * twi], axis=1)
        g = jnp.concatenate([g, jnp.zeros((8, 512), F32)], axis=0).astype(BF16)
        y0 = _dot_nt(g, f256[...])
        for _ in range(4):
            yield
        put(side.at[2], jnp.concatenate([y0, jnp.zeros((112, 256), F32)], axis=0).T)

    def s_fwd(u, t):
        ct, e = divmod(u, 4)
        put(ybuf.at[u % NY, t], ticking(_dot(lhs(sfw32[t * 4 + e]), bf(zin[ct, t * 4 + e]))))

    def s_filter(u, g):
        ct, e = divmod(u, 4)
        z = [tuple(ybuf[u % NY, t, pl.ds(g * 16 + i, 8), :] for i in (0, 8))
             for t in range(8)]
        z[0], z[1] = [tuple(gate(v, SGLAG if u * 8 + g < 122 - S_LAG else SGLAG2) for v in zz) for zz in z[0:2]]
        xk = _dft8(z, False)
        for k2 in range(8):
            wr = wf[0, ct, e, k2, pl.ds(g * 8, 8), :]
            wi = wf[1, ct, e, k2, pl.ds(g * 8, 8), :]
            re, im = xk[k2]
            xk[k2] = (re * wr - im * wi, re * wi + im * wr)
        for t, (re, im) in enumerate(_dft8(xk, True)):
            words = pack(re, im)
            pin(words)
            put(fbuf.at[u % NY, t, pl.ds(g * 8, 8), :], words)

    def s_inv(u, t):
        ct, e = divmod(u, 4)
        o = _dot(lhs(siv32[t * 4 + e]), bf(fbuf[u % NY, t]))
        put(zout.at[ct, t * 4 + e], ticking(o) if u * 8 + t >= 110 - S_LAG else o)

    def add_s_stage(sched, early, ready, t1):
        ahead = 8 + S_LAG
        tick = early
        for t in sorted(range(8), key=lambda t: ready[t]):
            for i in range(t, ahead, 8):
                tick = max(tick + 0.5, ready[t])
                sched.add(tick, _once(s_fwd, i // 8, t))
        t1 = max(t1, int(tick) + 1)
        sched.add(max(max(ready), t1), side_path())
        for i in range(128):
            if i + ahead < 128:
                sched.add(t1 + i, _once(s_fwd, *divmod(i + ahead, 8)))
            sched.add(t1 + i, _once(s_filter, *divmod(i, 8)))
            sched.add(t1 + 9 + (i if i < 120 else 120 + (i - 120) // 4), _once(s_inv, *divmod(i, 8)))
        return [t1 + 32 * ct + 40 for ct in range(3)] + [t1 + 131]

    def d_inv_cols(b, ct):
        c, t = divmod(b, 8)
        ra, rb = PAIRS[ct]
        lane = _lane(16)
        lo = lane < 64
        u = [(zout[ct, t * 4 + e, r16(c), :], zout[ct, t * 4 + e, r16(4 + c), :]) for e in range(4)]
        u[0], u[1] = tuple(map(gate, u[0])), tuple(map(gate, u[1]))
        z = _dft4(u, True)
        z = [(re, _swap(im)) for re, im in z]
        if ct == 0:
            y0 = [pltpu.roll(side[2, pl.ds(64 * lb + 16 * c, 16), :], 64 - t, 1) for lb in range(4)]
        yield from _latency()
        for lb, (re, sw) in enumerate(z):
            sw = gate(sw)
            a, bb = jnp.where(lo, re, sw), jnp.where(lo, sw, re)
            if ct == 0:
                a = jnp.where(lane == 64, y0[lb], a)
            pin(a, bb)
            ubuf[b % RING, ra, r16(lb), :] = a.astype(BF16)
            ubuf[b % RING, rb, r16(lb), :] = bb.astype(BF16)

    def d_inv_rows(b, lb, stats):
        u = [uout[b % RING, r, r16(lb), :] for r in range(8)]
        ys = yield from _d_butterfly_inv([gate(v) if r < 4 else v for r, v in enumerate(u)], pin, gate)
        xs = [x + y for x, y in zip(load_x(b, lb), ys)]
        for j in range(NT):
            put(xres.at[b, j, r16(lb), :], xs[j])
        stats[b, lb] = yield from ln_stats(xs)
        if b % 2:
            for j in range(4):
                a = [(xres[bb, j + o, r16(lb), :] - stats[bb, lb][0]) * stats[bb, lb][1]
                     for bb in (b - 1, b) for o in (0, 4)]
                a[0], a[3] = gate(a[0]), gate(a[3])
                for k, v in enumerate(_strassen_lhs(*a)):
                    if k not in (2, 3):
                        pin(v)
                    abuf[b // 2, k, j, r16(lb), :] = v.astype(BF16)
                if j < 3:
                    yield

    def add_d_inv(sched, tick, b, gap, stats, per_tick=4, cols=None):
        cols = cols or [tick + ct * gap for ct in range(4)]
        for ct in range(4):
            sched.add(cols[ct], d_inv_cols(b, ct))
        tick = int(cols[3]) + XGAP + 1
        sched.add(tick, d_dots(b, 8, per_tick))
        tick += 8 // per_tick + 3
        for lb in range(4):
            sched.add(tick + lb * gap, d_inv_rows(b, lb, stats))
        return int(tick + 3 * gap) + 3 * XGAP + 1 + 4

    def gemm(lhs32, rhs32, jobs, sink):
        for slot, b, n in jobs:
            m = {}
            for k in (3, 1, 0, 6, 5, 4, 2):
                m[k] = ticking(_dot(lhs(*[lhs32[slot, k, j] for j in range(4)]), bf(rhs32[n // 2, k])))
                if k == 1:
                    sink(b + 1, n, m[1] - m[3])
                elif k == 0:
                    c11, c22 = m[3] - m[0], m[1] - m[0]
                elif k == 6:
                    c11 = m[6] - c11
                elif k == 5:
                    c22 = m[5] - c22
                elif k == 4:
                    sink(b, n, c11 - m[4])
                elif k == 2:
                    sink(b, n + 1, m[4] - m[2])
                    sink(b + 1, n + 1, c22 - m[2])
                yield

    def qkv_sink(b, n, o):
        c, t = divmod(b, 8)
        dst = (qbuf, kbuf, vbuf)[n // NT]
        for lb in range(4):
            put(dst.at[n % NT, t, pl.ds(8 + 64 * lb + 16 * c, 16), :], o[lb * 16:(lb + 1) * 16])
        if b == 0 and n >= NT:
            first = jnp.broadcast_to(o[0:1], (8, 128))
            for tt in range(8):
                dst[n % NT, tt, pl.ds(0, 8), :] = first

    def out_rows(r, i, last):
        c, t = divmod(r, 8)
        return (c * 8 + t % 2 * 4 + i, t // 2) if last and c == 0 else (r, i)

    def out_sink(last, r, n, o):
        for i in range(4):
            b, lb = out_rows(r, i, last)
            put(xres.at[b, n, r16(lb), :], xres[b, n, r16(lb), :] + o[i * 16:(i + 1) * 16])

    def attention(b, lb, h):
        c, t = divmod(b, 8)
        scale = HEAD_DIM ** -0.5
        r0 = 8 + 64 * lb + 16 * c + 8 * h
        src = [((t - 2 * w) % 8, -((t - 2 * w) // 8)) for w in range(WIN)]
        acc = [None] * WIN
        for j in range(NT):
            q = gate(qbuf[j, t, pl.ds(r0, 8), :], ALAG)
            for w, (ts, sh) in enumerate(src):
                p = q * kbuf[j, ts, pl.ds(r0 - sh, 8), :]
                acc[w] = p if j == 0 else acc[w] + p
            if j % 2 and j < NT - 1:
                pin(*acc)
                yield
        part = [(r, pltpu.roll(r, 64, 1)) for r in acc]
        yield from _latency()
        part = [r + rr for r, rr in part]
        part = [(r, pltpu.roll(r, 32, 1)) for r in part]
        yield from _latency()
        logits = [r + rr for r, rr in part]
        if r0 == 8:
            sub = lax.broadcasted_iota(jnp.int32, (8, 128), 0)
            logits = [jnp.where(sub >= sh, r, -1e9 / scale) if sh else r
                      for r, (_, sh) in zip(logits, src)]
        logits[0] = gate(logits[0], ALAG)
        m = _tree(jnp.maximum, logits)
        ps = [jnp.exp2((r - m) * (scale * float(np.log2(np.e)))) for r in logits]
        total = _tree(_add, ps)
        pin(total)
        inv = pltpu.reciprocal(total, approx=True)
        inv = inv * (2.0 - total * inv)
        for j in range(NT):
            if j % 2 == 0:
                yield
                ps[0], ps[4] = gate(ps[0], ALAG), gate(ps[4], ALAG)
            o = _chain(_add, [ps[w] * vbuf[j, ts, pl.ds(r0 - sh, 8), :]
                              for w, (ts, sh) in enumerate(src)]) * inv
            pin(o)
            put(qbuf.at[j, t, pl.ds(r0, 8), :], o)

    def out_operands(r, i, last):
        for j in range(4):
            a = [qbuf[j + o, b % 8, pl.ds(8 + 64 * lb + 16 * (b // 8), 16), :]
                 for b, lb in (out_rows(r, i, last), out_rows(r + 1, i, last)) for o in (0, 4)]
            a[0], a[3] = gate(a[0]), gate(a[3])
            for k, v in enumerate(_strassen_lhs(*a)):
                if k not in (2, 3):
                    pin(v)
                obuf[r // 2, k, j, r16(i), :] = v.astype(BF16)
            if j < 3:
                yield

    def store_rows(b, lb):
        c, t = divmod(b, 8)
        for j in range(NT):
            words = pack(xres[b, j, r16(lb), :], xres[b + 1, j, r16(lb), :])
            pin(words)
            io32[j, lb, c, pl.ds(t // 2, 16, stride=4), :] = words

    unit_ticks = NT + 2 * XGAP
    step = 2
    out_ticks = 28

    def add_proj(sched, tick, c, lo, hi):
        jobs = [(b // step, b, n) for b in range(8 * c, 8 * c + 8, step) for n in range(lo, hi, step)]
        sched.add(tick, gemm(abuf32, wqkv32, jobs, qkv_sink))
        return tick + len(jobs) * out_ticks * step // NT

    def add_attention(sched, tick, pace, rows, last):
        units = [(r, i, half, h) for r in rows[::2] for i in range(4) for half in range(2) for h in range(2)]
        for n, (r, i, half, h) in enumerate(units):
            sched.add(tick + n * pace, attention(*out_rows(r + half, i, last), h))
            if half and h:
                sched.add(int(tick + n * pace) + unit_ticks, out_operands(r, i, last))

    def add_out(sched, tick, rows, last):
        jobs = [(r // 2, r, n) for r in rows[::2] for n in range(0, NT, 2)]
        sched.add(tick, gemm(obuf32, wo32, jobs, functools.partial(out_sink, last)))

    def add_tail(sched, tick, rows, last):
        ready = {}
        for i, r in enumerate(rows):
            t0 = tick + (i // 2 + 1) * out_ticks
            fast = i >= len(rows) - (2 if last else 4)
            if not last:
                t0 += 0 if fast else 3 + i % 2 * out_ticks // 2
                ready[r % 8] = add_d_fwd(sched, t0, r, i % 2 if fast else out_ticks / 8)
            elif r % 2:
                c, p = r // 8, r % 8 // 2
                gap = 0 if fast else 3
                for j in range(4):
                    sched.add(t0 + (j + 1) * gap, _once(store_rows, *((r - 1, j) if c else (2 * j, p))))
                for lb in ([p] if c == 0 else range(4) if p == 3 else []):
                    sched.add(t0 + 5 * gap + 1, _once(start, out_copies(c, lb)))
        return ready

    q_ticks = 8 * out_ticks // step
    att_ticks = unit_ticks + 1 + 2
    order = [(a + 8) % NB for a in range(NB)]

    def add_attention_block(sched, cols, last):
        stats = {}
        t0 = max([add_d_inv(sched, 0, b, 0, stats, 4, cols) for b in range(step)])
        if not last:
            sched.add(cols[3] - KLEAD, _once(wait, qkv_copies(1) + dmat_cp))
            done = add_prep_wqkv(sched, cols[3] - KLEAD, 1, KPACE, [7] * 4)
            t0 = max(t0, done[0])
            assert all(d <= t0 + p * out_ticks / 4 for p, d in enumerate(done))
            sched.add(t0 + out_ticks, _once(wait, qkv_copies(2)))
            sched.add(t0 + out_ticks, _once(start, qkv_copies(0)))
            done = add_prep_wqkv(sched, t0 + out_ticks, 2, 2 * out_ticks - 6, [out_ticks - 4] * 4)
            assert all(d <= t0 + q_ticks + p * out_ticks for p, d in enumerate(done))
            sched.add(t0 + 2 * q_ticks, _once(wait, qkv_copies(0)))
            sched.add(t0 + 2 * q_ticks, _once(start, wo_copies))
            done = add_prep_wqkv(sched, t0 + 2 * q_ticks, 0, q_ticks - 10, [q_ticks / 4] * 4)
            assert done[-1] <= t0 + 4 * q_ticks
            sched.add(t0 + 8 * q_ticks, _once(wait, wo_copies))
            for i in range(32):
                sched.add(t0 + 8 * q_ticks + i * q_ticks / 16, _once(prep_wo, *divmod(i, 8)))
        tick, kv_start, q_start = t0, {}, {}
        for kind, c in ("k0", "k1", "q1", "k2", "q2", "k3", "q3", "q0"):
            if kind == "k":
                kv_start[int(c)] = tick
                if c == "0" and not last:
                    tick = add_proj(sched, tick, 0, NT, 2 * NT)
                    jobs = [(b // step, b, n) for n in range(2 * NT, 3 * NT, step) for b in range(0, 8, step)]
                    sched.add(tick, gemm(abuf32, wqkv32, jobs, qkv_sink))
                    tick += q_ticks
                    continue
                tick = add_proj(sched, tick, int(c), NT, 3 * NT)
            else:
                q_start[int(c)] = tick
                tick = add_proj(sched, tick, int(c), 0, NT)
        pace = 2 * out_ticks / step
        for b in range(step, NB):
            due = kv_start[b // 8] + (b % 8 // step) * (2 if last or b >= 8 else 1) * out_ticks
            gap = min(1 + (b - step) * 0.5, DGAP1 if last else DGAP0)
            pace = DPACE1 if last else DPACE0
            at = (b - step) * pace
            at = t0 + at + max(0, at - 4 * q_ticks - out_ticks) * DSLOW
            if not last and b < 8:
                at, gap = max(cols[3], t0 + (b // step - 1) * out_ticks - (step - b % step) * 8), 1
            end = add_d_inv(sched, at, b, gap, stats)
            assert end <= due, (b, end, due)
        begin = [q_start[c] + out_ticks + 3 for c in (1, 2, 3)] + [tick + (ATT1 if last else ATT0)]
        begin.append(tick + (NB // step - 1) * out_ticks - att_ticks)
        for i, c in enumerate((1, 2, 3, 0)):
            pace = (begin[i + 1] - begin[i]) / 64
            assert begin[i] >= max(kv_start[c], kv_start[(c - 1) % 4]) + 2 * q_ticks
            for p in range(4):
                assert begin[i] + 16 * p * pace >= q_start[c] + (4 if last and c == 0 else p + 1) * out_ticks
                assert begin[i] + (16 * p + 15) * pace + att_ticks <= tick + (4 * i + p) * out_ticks + 1e-6
            add_attention(sched, begin[i], pace, range(8 * c, 8 * c + 8), last)
        add_out(sched, tick, order, last)
        return tick + (NB // step) * out_ticks, add_tail(sched, tick, order, last)

    def add_input(sched):
        ready = {}
        after = (x_copies(2), x_copies(3) + perm_cp + w_copies(0) + w_copies(1),
                 w_copies(2) + w_copies(3), w_copies(4))
        for c in range(NC):
            sched.add(c * 32, _once(wait, x_copies(c)))
            sched.add(c * 32, _once(start, after[c]))
            for t in range(8):
                ready[t] = add_d_fwd(sched, c * 32 + t * 4, c * 8 + t, 1, 2, True)
        return 128 + 9, ready

    def add_filter_prep(sched, tick):
        after = {0: w_copies(5), 1: w_copies(6), 2: w_copies(7), 3: f256_cp + dmat_cp,
                 5: qkv_copies(1), 7: qkv_copies(2)}
        begin = [F0 + g * (tick - F0) / 4 for g in range(4)] + [tick + 4 * g for g in range(5)]
        for g in range(8):
            sched.add(begin[g], _once(wait, w_copies(g) + ([] if g else perm_cp)))
            sched.add(begin[g], _once(start, after.get(g, [])))
            for m in range(4):
                sched.add(begin[g] + m * (begin[g + 1] - begin[g]) / 4,
                          _once(prep_filter, g // 4, g % 4 * 4 + m))
        sched.add(begin[8] + 1, _once(wait, f256_cp))
        return begin[8] + 2

    sched = _Schedule()

    def phase(fn, *args):
        fn(sched, *args)
        sched.run()
        token.clear()
        clock.clear()

    start(x_copies(0))
    for ref in (abuf32, obuf32, ubuf32, wo32, sfw32, siv32, wide32):
        put(ref.at[(0,) * (len(ref.shape) - 2) + (pl.ds(0, 8),)], jnp.zeros((8, 128), U32))
    make_wide()
    start(x_copies(1))
    for t in range(8):
        make_s_fwd(t)
    for e in range(4):
        make_s_inv(e)
    tick, ready = add_input(sched)
    cols = add_s_stage(sched, tick, ready, add_filter_prep(sched, tick))
    tick, ready = add_attention_block(sched, cols, False)
    cols = add_s_stage(sched, tick, ready, tick)
    add_attention_block(sched, cols, True)
    sched.run()
    for c in range(NC):
        for lb in range(4):
            wait(out_copies(c, lb))


@jax.jit
def pallas_interleave_layers__spectral_gfnet__sliding_local_dilated__prompt_kernel(
    A_x: jax.Array,
    A_w_r: jax.Array,
    A_w_i: jax.Array,
    B_x: jax.Array,
    B_wqkv: jax.Array,
    B_wo: jax.Array,
):
    del B_x
    assert A_x.shape == (1, S, D) and A_w_r.shape == (S, D // 2 + 1)
    cst = _constants()
    x = A_x.astype(BF16).reshape(4, NC, 128, D)
    wr, wi = A_w_r.astype(BF16).T, A_w_i.astype(BF16).T
    hbm = pl.BlockSpec(memory_space=pl.ANY)
    edge = pl.BlockSpec((16, S), lambda i: (D // 32, 0))
    vm = pltpu.VMEM
    out = pl.pallas_call(
        _kernel,
        grid=(1,),
        in_specs=[hbm, hbm, hbm, edge, edge, hbm, hbm, hbm, hbm,
                  pl.BlockSpec((24, 256), lambda i: (0, 0)),
                  pl.BlockSpec((2, 16, 128), lambda i: (0, 0, 0))],
        out_specs=hbm,
        out_shape=jax.ShapeDtypeStruct((4, NC, 128, D), BF16),
        scratch_shapes=[
            vm((NT, 4, NC, 128, 128), BF16),
            vm((17, 128, 128), BF16),
            vm((32, 128, 128), BF16),
            vm((32, 128, 128), BF16),
            vm((256, 512), BF16),
            vm((2, 16, 512, 128), BF16),
            vm((2, 4, 4, 8, 64, 128), F32),
            vm((3 * NT, D, 128), BF16),
            vm((NT, D // 2, 128), U32),
            vm((12, 7, 512, 128), BF16),
            vm((NT, D, 128), BF16),
            vm((4, 7, 512, 128), BF16),
            vm((NB, NT, 64, 128), F32),
            vm((4, 32, 64, 128), U32),
            vm((4, 32, 128, 128), F32),
            vm((NY, 8, 128, 128), F32),
            vm((NY, 8, 64, 128), U32),
            vm((RING, 8, 64, 128), BF16),
            vm((RING, 9, 64, 128), F32),
            vm((NB // 2, 7, 4, 64, 128), BF16),
            vm((NB // 2, 7, 4, 64, 128), BF16),
            vm((NT, 8, 264, 128), F32),
            vm((NT, 8, 264, 128), F32),
            vm((NT, 8, 264, 128), F32),
            vm((3, 256, 128), F32),
            vm((8, 256, 128), BF16),
            pltpu.SemaphoreType.DMA((NC,)),
            pltpu.SemaphoreType.DMA((3,)),
            pltpu.SemaphoreType.DMA((8,)),
            pltpu.SemaphoreType.DMA((3,)),
            pltpu.SemaphoreType.DMA(()),
            pltpu.SemaphoreType.DMA(()),
        ],
        compiler_params=pltpu.CompilerParams(
            dimension_semantics=("arbitrary",), vmem_limit_bytes=120 * 2**20),
    )(x, wr, wi, wr, wi, B_wqkv.astype(BF16), B_wo.astype(BF16),
      cst["small"], cst["f256"], cst["tw"], cst["d8"])
    return out.reshape(1, S, D)
```

```python
import functools

import jax
import jax.numpy as jnp
import numpy as np
from jax import lax
from jax.experimental import pallas as pl
from jax.experimental.pallas import tpu as pltpu

S, D = 2048, 1024
NT = D // 128
NC = 4
WIN = 8
HEAD_DIM = 32
EPS = 1e-5
F32, BF16, U32 = jnp.float32, jnp.bfloat16, jnp.uint32
PAIRS = ((0, 4), (1, 7), (2, 6), (3, 5))
RSQ2 = float(np.sqrt(0.5))
NB = S // 64

RING = 8
NY = 4
XGAP = 3
GLAG = 4
ALAG = 4
SGLAG = 3
SGLAG2 = 5
S_LAG = 3
F0 = 112
KLEAD = 52
KPACE = 48
DGAP0 = 4.75
DGAP1 = 4.2
DPACE0 = 21
DPACE1 = 15.5
DSLOW = 0.6
SYNC = 3
ILAG = 3
FG = 4
ATT0 = 10
ATT1 = 95


def _residues(r):
    return (0, 8) if r == 0 else (r, 16 - r)


def _d_matrices():
    n = np.arange(64)[:, None]
    a = np.arange(32)
    fwd = np.zeros((8, 128, 128))
    inv = np.zeros((8, 128, 128))
    for r in range(8):
        kd = np.concatenate([16 * a + p for p in _residues(r)])
        weight = np.full(64, 2.0)
        if r == 0:
            kd[0], weight[0] = D // 2, 1.0
            ph = np.exp(-2j * np.pi * n * kd[None, :] / D)
            sgn = np.where(kd % 16 == 0, 1.0, -1.0)[None, :]
            m = np.concatenate([ph, ph * sgn], axis=0)
            re, im = m.real.copy(), m.imag.copy()
            ire, iim = re.copy(), im.copy()
            im[:, 0] = 1.0
            iim[:, 0] = 1.0
        else:
            p = 12 if r == 4 else r
            ph = np.exp(-2j * np.pi * n * kd[None, :] / D)
            si = np.where(kd % 16 == p, 1.0, -1.0)[None, :]
            m = np.concatenate([ph, 1j * si * ph], axis=0)
            re, im = m.real, m.imag
            ire, iim = re, im
        swapped = r in (4, 7, 6, 5)
        cols = [im, re] if swapped else [re, im]
        icols = [iim * weight, ire * weight] if swapped else [ire * weight, iim * weight]
        fwd[r] = np.concatenate(cols, axis=1)
        inv[r] = np.concatenate(icols, axis=1).T / D
    return fwd, inv


def _side_matrices():
    l = np.arange(256)
    f = np.exp(-2j * np.pi * ((l[:, None] * l[None, :]) % 256) / 256)
    f256 = np.concatenate([f.real, f.imag], axis=1)
    t = np.arange(8)
    tw = np.exp(-2j * np.pi * t[:, None] * l[None, :] / S)
    tw = np.concatenate([tw.real, tw.imag, np.zeros((8, 256))], axis=0)
    g = np.exp(-2j * np.pi * t[:, None] * t[None, :] / 8)
    d8 = np.zeros((2, 16, 128))
    d8[0, :, :16] = np.block([[g.real, -g.imag], [g.imag, g.real]])
    d8[1, :, :16] = d8[0, :, :16].T / S
    return f256, tw, d8


def _filter_rows():
    p = np.zeros((1, 128, 128))
    for k in range(32):
        for e in range(4):
            p[0, e * 32 + k, 4 * k + e] = 1.0
    return p


@functools.lru_cache(maxsize=None)
def _constants():
    dfw, div = _d_matrices()
    f256, tw, d8 = _side_matrices()
    small = np.concatenate([dfw, div, _filter_rows()], axis=0)
    b = lambda x: np.asarray(x, np.float32).astype(BF16)
    return dict(small=b(small), f256=b(f256),
                tw=np.asarray(tw, np.float32), d8=b(d8))


def _dot(a, b):
    return jnp.dot(a, b, preferred_element_type=F32)


def _dot_nt(a, b):
    return lax.dot_general(a, b, (((1,), (1,)), ((), ())), preferred_element_type=F32)


def _tree(op, xs):
    xs = list(xs)
    while len(xs) > 1:
        xs = [op(xs[i], xs[i + 1]) if i + 1 < len(xs) else xs[i] for i in range(0, len(xs), 2)]
    return xs[0]


def _chain(op, xs):
    return functools.reduce(op, xs)


def _lane(rows):
    return lax.broadcasted_iota(jnp.int32, (rows, 128), 1)


def _swap(x):
    return pltpu.roll(x, 64, 1)


def _unpack(w, i):
    return pltpu.unpack_elementwise(w, index=i, packed_dtype=BF16, unpacked_dtype=F32)


def _latency():
    for _ in range(XGAP):
        yield


def _add(a, b):
    return a + b


def _row_mean(xs):
    return jnp.sum(_tree(_add, xs), axis=1, keepdims=True) * (1.0 / D)


def _twiddle16(r, x, y):
    lo = _lane(x.shape[0]) < 64
    wr, wi = float(np.cos(np.pi * r / 8)), float(-np.sin(np.pi * r / 8))
    cross = jnp.where(lo, 0.0, wr)
    return x * jnp.where(lo, 1.0, wi) + y * cross, y * jnp.where(lo, 1.0, -wi) + x * cross


def _d_butterfly_fwd(a, emit, pin, gate, wide):
    s = [a[j] + a[j + 4] for j in range(4)]
    e, o = s[0] + s[2], s[1] + s[3]
    total, t4 = e + o, e - o
    emit(4, t4)
    d0, nd2 = a[0] - a[4], a[6] - a[2]
    d1, d3 = a[1] - a[5], a[3] - a[7]
    p, q = (d1 - d3) * RSQ2, (d1 + d3) * -RSQ2
    ts = {1: (d0 + p, q + nd2), 2: (s[0] - s[2], s[3] - s[1]), 3: (d0 - p, q - nd2)}
    mean8 = jnp.sum(total, axis=1, keepdims=True) * (1.0 / 128)
    if wide:
        for r, (tr, ti) in ts.items():
            emit(r, tr)
            emit(8 - r, ti)
    else:
        ab = {r: _twiddle16(r, *t) for r, t in ts.items()}
        ab = {r: (a, _swap(b)) for r, (a, b) in ab.items()}
    dev = _tree(_add, [v * v for t in ts.values() for v in t]) * 2.0 + t4 * t4
    pin(dev)
    yield from _latency()
    t0 = total - mean8
    emit(0, t0)
    var = jnp.sum(dev + t0 * t0, axis=1, keepdims=True) * (1.0 / (NT * D))
    if not wide:
        for r, (x, y) in ab.items():
            emit(r, x + y)
            emit(8 - r, x - y)
    yield from _latency()
    return lax.rsqrt(var + EPS)


def _d_butterfly_inv(u, pin, gate):
    ab = {r: (u[r] + u[8 - r], _swap(u[r] - u[8 - r])) for r in (1, 2, 3)}
    e, o = u[0] + u[4], u[0] - u[4]
    yield from _latency()
    ts = {r: _twiddle16(r, x, gate(y)) for r, (x, y) in ab.items()}
    pin(*[v for t in ts.values() for v in t])
    yield
    s = [e + ts[2][0], o - ts[2][1], e - ts[2][0], o + ts[2][1]]
    p = (ts[1][0] - ts[3][0]) * RSQ2
    q = (ts[1][1] + ts[3][1]) * RSQ2
    d0, d1, d2, nd3 = ts[1][0] + ts[3][0], p - q, ts[3][1] - ts[1][1], p + q
    return [s[0] + d0, s[1] + d1, s[2] + d2, s[3] - nd3,
            s[0] - d0, s[1] - d1, s[2] - d2, s[3] + nd3]


def _strassen_lhs(a11, a12, a21, a22):
    return [a11 + a22, a21 + a22, a11, a22, a11 + a12, a21 - a11, a12 - a22]


def _strassen_rhs(b11, b12, b21, b22):
    return [b11 + b22, b11, b22 - b12, b11 - b21, b22, b11 + b12, b21 + b22]


def _cadd(a, b):
    return a[0] + b[0], a[1] + b[1]


def _csub(a, b):
    return a[0] - b[0], a[1] - b[1]


def _dft4(z, inverse):
    a, b = _cadd(z[0], z[2]), _csub(z[0], z[2])
    c, d = _cadd(z[1], z[3]), _csub(z[1], z[3])
    minus = (b[0] + d[1], b[1] - d[0])
    plus = (b[0] - d[1], b[1] + d[0])
    return [_cadd(a, c), plus if inverse else minus, _csub(a, c), minus if inverse else plus]


def _dft8(z, inverse):
    ev = _dft4(z[0::2], inverse)
    od = _dft4(z[1::2], inverse)
    out = [None] * 8
    out[0], out[4] = _cadd(ev[0], od[0]), _csub(ev[0], od[0])
    (er, ei), (x, y) = ev[2], od[2]
    minus, plus = (er + y, ei - x), (er - y, ei + x)
    out[2], out[6] = (plus, minus) if inverse else (minus, plus)
    for k in (1, 3):
        (er, ei), (x, y) = ev[k], od[k]
        sm, df = (x + y) * RSQ2, (x - y) * RSQ2
        if not inverse:
            if k == 1:
                out[1], out[5] = (er + sm, ei - df), (er - sm, ei + df)
            else:
                out[3], out[7] = (er - df, ei - sm), (er + df, ei + sm)
        else:
            if k == 1:
                out[1], out[5] = (er + df, ei + sm), (er - df, ei - sm)
            else:
                out[3], out[7] = (er - sm, ei + df), (er + sm, ei - df)
    return out


class _Schedule:
    def __init__(self):
        self.pending = []

    def add(self, tick, gen):
        self.pending.append((int(tick), len(self.pending), gen))

    def run(self):
        pending = sorted(self.pending, key=lambda p: p[:2])
        active, tick, i = [], 0, 0
        while active or i < len(pending):
            while i < len(pending) and pending[i][0] <= tick:
                active.append(pending[i][2])
                i += 1
            for g in list(active):
                if next(g, 0) == 0:
                    active.remove(g)
            tick += 1
        self.pending = []


def _once(fn, *args):
    fn(*args)
    return
    yield


def _kernel(x_hbm, wr_hbm, wi_hbm, wr_edge, wi_edge, wqkv_hbm, wo_hbm,
            small_hbm, f256_hbm, tw_ref, d8_ref,
            out_hbm,
            io, small, sfw, siv, f256, wraw, wf, wqkv_raw, wtmp, wqkv, wo_raw, wo,
            xres, zin, zout, ybuf, fbuf, ubuf, uout, abuf, obuf, qbuf, kbuf, vbuf, side,
            wide, sem_x, sem_c, sem_w, sem_qkv, sem_wo, sem_out):

    def x_copies(c):
        return [pltpu.make_async_copy(x_hbm.at[:, c, :, pl.ds(j * 128, 128)], io.at[j, :, c],
                                      sem_x.at[c]) for j in range(NT)]

    def out_copies(c, lb):
        return [pltpu.make_async_copy(io.at[j, lb, c], out_hbm.at[lb, c, :, pl.ds(j * 128, 128)],
                                      sem_out) for j in range(NT)]

    perm_cp, dmat_cp, f256_cp = ([pltpu.make_async_copy(s, d, sem_c.at[i])] for i, (s, d) in enumerate((
        (small_hbm.at[pl.ds(16, 1)], small.at[pl.ds(16, 1)]),
        (small_hbm.at[pl.ds(0, 16)], small.at[pl.ds(0, 16)]), (f256_hbm, f256))))

    def w_copies(g):
        src = (wr_hbm, wi_hbm)[g // 4]
        return [pltpu.make_async_copy(src.at[pl.ds(0, 512), pl.ds(m * 128, 128)], wraw.at[g // 4, m],
                                      sem_w.at[g]) for m in range(g % 4 * 4, g % 4 * 4 + 4)]

    def qkv_copies(g):
        return [pltpu.make_async_copy(wqkv_hbm.at[:, pl.ds(g * D + j * 128, 128)],
                                      wqkv_raw.at[g * NT + j], sem_qkv.at[g]) for j in range(NT)]

    wo_copies = [pltpu.make_async_copy(wo_hbm.at[:, pl.ds(j * 128, 128)], wo_raw.at[j], sem_wo)
                 for j in range(NT)]

    def start(cs):
        for cp in cs:
            cp.start()

    def wait(cs):
        for cp in cs:
            cp.wait()

    io32, wraw32, wo_raw32 = io.bitcast(U32), wraw.bitcast(U32), wo_raw.bitcast(U32)
    small32, sfw32, siv32, wide32 = (r.bitcast(U32) for r in (small, sfw, siv, wide))
    wqkv_raw32, wqkv32, wo32 = (r.bitcast(U32) for r in (wqkv_raw, wqkv, wo))
    ubuf32, abuf32, obuf32 = ubuf.bitcast(U32), abuf.bitcast(U32), obuf.bitcast(U32)

    never = tw_ref[16:24, 0:128] != 0.0
    never_wide = {n: jnp.concatenate([tw_ref[16:24, 0:128]] * n, axis=1) != 0.0 for n in (1, 2, 4)}
    token = {}

    def pin(*values):
        for v in values:
            key = v.shape[0], v.dtype == F32
            token[key] = (lax.max if key[1] else lax.bitwise_xor)(token[key], v) if key in token else v

    clock = []

    def gate(v, lag=GLAG):
        if len(clock) < lag:
            return v
        old = clock[-lag] if v.dtype == F32 else pltpu.bitcast(clock[-lag], v.dtype)
        if v.shape[0] == 8:
            return lax.select(never, old, v)
        return lax.concatenate([lax.select(never, old, v[0:8]), v[8:]], 0)

    def ticking(o):
        clock.append(o[0:8])
        del clock[:-16]
        return o

    def lhs(*tiles):
        if not token and len(tiles) == 4 and len(clock) >= SYNC:
            pin(clock[-SYNC])
        words = lax.concatenate(tiles, 1) if len(tiles) > 1 else tiles[0]
        if token:
            parts = [pltpu.bitcast(v, U32) if is_float else v for (_, is_float), v in token.items()]
            token.clear()
            w = _chain(lax.bitwise_xor, [v[i:i + 8] if v.shape[0] > 8 else v
                                         for v in parts for i in range(0, v.shape[0], 8)])
            w = lax.concatenate([w] * len(tiles), 1) if len(tiles) > 1 else w
            words = lax.concatenate([lax.select(never_wide[len(tiles)], w, words[0:8]), words[8:]], 0)
        return pltpu.bitcast(words, BF16)

    def bf(words):
        return pltpu.bitcast(words, BF16)

    def pack(a, b):
        return pltpu.bitcast(pltpu.pack_elementwise([a, b], packed_dtype=BF16), U32)

    def r16(i):
        return pl.ds(i * 16, 16)

    always = {}

    def put(ref, v):
        if v.shape not in always:
            always[v.shape] = jnp.ones(v.shape, jnp.bool_)
        pltpu.store(ref, v, mask=always[v.shape])

    def load_x(b, lb, from_input):
        if from_input:
            c, t = divmod(b, 8)
            return [_unpack(io32[j, lb, c, pl.ds(t // 2, 16, stride=4), :], t % 2) for j in range(NT)]
        return [xres[b, j, r16(lb), :] for j in range(NT)]

    def unit(p):
        angle = (((p + S // 2) & (S - 1)) - S // 2).astype(F32) * (2 * np.pi / S)
        return jnp.cos(angle), jnp.sin(angle)

    def times_row(a, b, i):
        br, bi = (jnp.broadcast_to(v[i:i + 1], (8, 128)) for v in b)
        return a[0] * br - a[1] * bi, a[0] * bi + a[1] * br

    def make_wide():
        row, lane = lax.broadcasted_iota(jnp.int32, (8, 128), 0), _lane(8)
        for ct, (ra, rb) in enumerate(PAIRS):
            res = _residues(ra) + _residues(rb)
            kd = (lane & 31) * 16 + _chain(
                _add, [jnp.where(lane >> 5 == g, p, 0) for g, p in enumerate(res)])
            if ct == 0:
                kd = jnp.where(lane == 0, D // 2, kd)
            fine, coarse = unit(-2 * row * kd), [unit(-16 * (row + 8 * h) * kd) for h in range(2)]
            for a in range(16):
                re, im = times_row(fine, coarse[a // 8], a % 8)
                if ct == 0:
                    even = kd & 7 == 0
                    top = jnp.where(even, re, 0.0), jnp.where(lane == 0, 1.0, jnp.where(even, im, 0.0))
                    bottom = jnp.where(even, 0.0, re), jnp.where(even, 0.0, im)
                else:
                    sign = jnp.where(kd & 7 == ra, 1.0, -1.0)
                    top, bottom = (re, im), (-sign * im, sign * re)
                for i in range(2):
                    wide[2 * ct + i, pl.ds(8 * a, 8), :] = top[i].astype(BF16)
                    wide[2 * ct + i, pl.ds(128 + 8 * a, 8), :] = bottom[i].astype(BF16)

    def make_s_fwd(t):
        row, lane = lax.broadcasted_iota(jnp.int32, (8, 128), 0), _lane(8)
        pos = 8 * (lane >> 1) + t
        fine = unit((lane & 1) * (S // 4) - 4 * row * pos)
        shift, coarse = unit(-row * pos), unit(-32 * row * pos)
        for e in range(4):
            base = times_row(fine, shift, e)
            for g in range(8):
                for i, v in enumerate(times_row(base, coarse, g)):
                    sfw[t * 4 + e, pl.ds(16 * g + 8 * i, 8), :] = v.astype(BF16)

    def make_s_inv(e):
        row, lane = lax.broadcasted_iota(jnp.int32, (8, 128), 0), _lane(8)
        freq = 4 * (lane >> 1) + e
        fine = [v * (1.0 / S) for v in unit((lane & 1) * (S // 4) + 8 * row * freq)]
        shift, coarse = unit(row * freq), unit(64 * row * freq)
        for t in range(8):
            base = times_row(fine, shift, t)
            for g in range(8):
                for i, v in enumerate(times_row(base, coarse, g)):
                    siv[t * 4 + e, pl.ds(64 * i + 8 * g, 8), :] = v.astype(BF16)

    def prep_filter(ri, m):
        sub = lax.broadcasted_iota(jnp.int32, (8, 128), 0)
        edge = (wr_edge, wi_edge)[ri]
        res = {}
        for i in range(8):
            words = wraw32[ri, m, pl.ds(i, 32, stride=8), :]
            res[2 * i], res[2 * i + 1] = _unpack(words, 0), _unpack(words, 1)
        first = res[0][0:8]
        dst = pl.ds((m % 2) * 16 + ri * 8, 8)
        prev = jnp.zeros((8, 128), F32) if m < 2 else side[1, dst, :]
        put(side.at[1, dst, :], jnp.where(sub == m // 2, jnp.broadcast_to(first[0:1], (8, 128)), prev))
        nyq = jnp.broadcast_to(edge[0:1, pl.ds(m * 128, 128)].astype(F32), (8, 128))
        res[0] = jnp.concatenate([jnp.where(sub == 0, nyq, first), res[0][8:]], axis=0)
        for ct, (ra, rb) in enumerate(PAIRS):
            blk = jnp.concatenate([res[p] for p in _residues(ra) + _residues(rb)], axis=0)
            o = _dot_nt(lhs(small32[16]), blk.astype(BF16))
            for e in range(4):
                put(wf.at[ri, ct, e, m // 2, pl.ds((m % 2) * 32, 32), :], o[e * 32:(e + 1) * 32])

    def shuffle(words, index):
        return jnp.take_along_axis(words, index, axis=1)

    def prep_wqkv_tile(g, i, part):
        lane = _lane(8)
        index = (lane & 3) * 32 + (((lane >> 2) - i) & 7) * 4 + (lane >> 5)
        rows = [pl.ds((part * 16 + r) * 8, 8) for r in range(16)]
        ws = [shuffle(gate(wqkv_raw32[g * NT + i, rs, :]), index) for rs in rows]
        yield from _latency()
        for rs, w in zip(rows, ws):
            pin(w)
            put(wtmp.at[i, rs, :], w)

    def prep_wqkv_cross(g, r):
        pos = (_lane(8) >> 2) & 7
        u = [wtmp[(-j) % 8, pl.ds(r * 8, 8), :] for j in range(NT)]
        u[0], u[4] = gate(u[0]), gate(u[4])
        for bit in range(3):
            m = ((pos >> bit) & 1) == 1
            u = [lax.select(m, u[(j - (1 << bit)) % 8], u[j]) for j in range(NT)]
        for j in range(NT):
            pin(u[j])
            put(wqkv_raw32.at[g * NT + j, pl.ds(r * 8, 8), :], u[j])

    def prep_wqkv_pair(g, p, part):
        lane = _lane(8)
        ws = {}
        for n in range(2):
            index = (lane & 96) | ((lane + 4 * (2 * p + n)) & 31)
            for half in range(2):
                for r in range(part * 2, part * 2 + 2):
                    w = gate(wqkv_raw32[g * NT + 2 * p + n, pl.ds(half * 256 + r * 8, 8), :])
                    ws[r, half, n] = shuffle(w, index) if p + n else w
        yield from _latency()
        for r in range(part * 2, part * 2 + 2):
            quad = [ws[r, half, n] for half in range(2) for n in range(2)]
            ops = [_strassen_rhs(*[_unpack(w, i) for w in quad]) for i in range(2)]
            for k in range(7):
                word = {1: quad[0], 4: quad[3]}.get(k)
                if word is None:
                    word = pack(ops[0][k], ops[1][k])
                    pin(word)
                put(wqkv32.at[g * 4 + p, k, pl.ds(r * 8, 8), :], word)

    def add_prep_wqkv(sched, tick, g, ticks, pair_ticks):
        for i in range(32):
            sched.add(tick + i * ticks / 64, prep_wqkv_tile(g, *divmod(i, 4)))
        tick = int(tick + ticks / 2) + XGAP + 1
        for r in range(64):
            sched.add(tick + r * ticks / 128, _once(prep_wqkv_cross, g, r))
        tick = int(tick + ticks / 2) + 1
        done = []
        for p, n in enumerate(pair_ticks):
            for i in range(16):
                sched.add(tick + i * n / 16, prep_wqkv_pair(g, p, i))
            tick += n
            done.append(int(tick) + XGAP + 1)
        return done

    def prep_wo(p, dp):
        ws = [wo_raw32[2 * p + n, pl.ds(dp + off, 32, stride=16), :] for off in (0, 8) for n in (0, 1)]
        for i in range(2):
            b = [_unpack(w, i) for w in ws]
            r0 = (2 * dp + i) * 32
            for k, v in enumerate(_strassen_rhs(*b)):
                if k not in (1, 4):
                    pin(v)
                wo[p, k, pl.ds(r0, 32), :] = v.astype(BF16)

    def ln_stats(xs):
        lane_mean = _tree(_add, xs) * (1.0 / NT)
        lane_m2 = _tree(_add, [jnp.square(x - lane_mean) for x in xs])
        pin(lane_m2)
        mean = jnp.sum(lane_mean, axis=1, keepdims=True) * (1.0 / 128)
        yield from _latency()
        m2 = lane_m2 + jnp.square(gate(lane_mean) - mean) * float(NT)
        pin(m2)
        var = jnp.sum(m2, axis=1, keepdims=True) * (1.0 / D)
        yield from _latency()
        return mean, lax.rsqrt(gate(jnp.broadcast_to(var, (16, 128))) + EPS)

    def d_fwd_rows(b, lb, from_input=False):
        xs = load_x(b, lb, from_input)

        def emit(r, v):
            if not from_input or r % 4 == 0:
                pin(v)
            ubuf[b % RING, r, r16(lb), :] = v.astype(BF16)

        inv = yield from _d_butterfly_fwd([gate(x, ILAG if from_input else GLAG) if j < 4 else x for j, x in enumerate(xs)], emit, pin, gate, from_input)
        inv = jnp.broadcast_to(inv, (16, 128))
        pin(inv)
        put(uout.at[b % RING, 8, r16(lb), :], inv)

    def d_dots(b, base, per_tick):
        for r in range(8):
            o = _dot(lhs(ubuf32[b % RING, r]), bf(small32[base + r]))
            put(uout.at[b % RING, r], o)
            if r % per_tick == per_tick - 1 and r < 7:
                yield

    def d_dots_wide(b):
        for ct, (ra, rb) in enumerate(PAIRS):
            u = lhs(ubuf32[b % RING, ra], ubuf32[b % RING, rb])
            for i, r in enumerate((ra, rb)):
                o = _dot(u, bf(wide32[2 * ct + i]))
                put(uout.at[b % RING, r], ticking(o) if i else o)
            if ct < 3:
                yield

    def d_fwd_cols(b, ct, is_wide):
        c, t = divmod(b, 8)
        ra, rb = PAIRS[ct]
        lane = _lane(16)
        lo = lane < 64
        z, x0 = [], []
        for lb in range(4):
            a, bb, inv = (uout[b % RING, r, r16(lb), :] for r in (ra, rb, 8))
            inv = gate(inv, ILAG if is_wide else GLAG)
            a, bb = a * inv, bb * inv
            if is_wide:
                if ct == 0:
                    x0.append(pltpu.roll(bb, t, 1) if t else bb)
                    bb = jnp.where(lane == 0, 0.0, bb)
                z.append((a, bb))
                continue
            if ct == 0:
                x0.append(pltpu.roll(a, (t + 64) % 128, 1))
                a = jnp.where(lane == 64, 0.0, a)
            im = lax.select(lo, bb, a)
            z.append((lax.select(lo, a, bb), _swap(im)))
        if not is_wide:
            yield from _latency()
        for e, (re, im) in enumerate(_dft4(z, False)):
            words = pack(re, im)
            pin(words)
            put(zin.at[ct, t * 4 + e, r16(c), :], words)
        if is_wide and ct == 0:
            yield from _latency()
        for lb, v in enumerate(x0):
            ls = pl.ds(64 * lb + 16 * c, 16)
            prev = jnp.zeros((16, 128), F32) if t == 0 else side[0, ls, :]
            v = jnp.where(lane == t, v, prev)
            pin(v)
            put(side.at[0, ls, :], v)

    def add_d_fwd(sched, tick, b, gap, per_tick=4, from_input=False):
        for lb in range(4):
            sched.add(tick + lb * gap, d_fwd_rows(b, lb, from_input))
        tick = int(tick + 3 * gap) + XGAP + 1
        sched.add(tick, d_dots_wide(b) if from_input else d_dots(b, 0, per_tick))
        for ct in range(4):
            sched.add(tick + 8 // per_tick + 3 + ct * gap, d_fwd_cols(b, ct, from_input))
        return int(tick + 8 // per_tick + 3 + 3 * gap) + XGAP + 1

    def side_path():
        vt = side[0].T[0:8]
        yield
        zero8 = jnp.zeros((8, 256), F32)
        u = _dot(jnp.concatenate([vt, zero8], axis=0).astype(BF16), f256[...])[0:8]
        twr, twi = tw_ref[0:8, :], tw_ref[8:16, :]
        ur, ui = u[:, 0:256], u[:, 256:512]
        pad = jnp.zeros((112, 256), BF16)
        for _ in range(4):
            yield
        uu = jnp.concatenate([ur * twr - ui * twi, ur * twi + ui * twr], axis=0).astype(BF16)
        xk = _dot(d8_ref[0], jnp.concatenate([uu, pad], axis=0))
        for _ in range(4):
            yield
        wr = jnp.concatenate([side[1, 0:8, :], side[1, 16:24, :]], axis=1)
        wi = jnp.concatenate([side[1, 8:16, :], side[1, 24:32, :]], axis=1)
        xr, xi = xk[0:8], xk[8:16]
        yy = jnp.concatenate([xr * wr - xi * wi, xr * wi + xi * wr], axis=0).astype(BF16)
        p = _dot(d8_ref[1], jnp.concatenate([yy, pad], axis=0))
        for _ in range(4):
            yield
        twr, twi = tw_ref[0:8, :], tw_ref[8:16, :]
        pr, pi = p[0:8], p[8:16]
        g = jnp.concatenate([pr * twr + pi * twi, pi * twr - pr * twi], axis=1)
        g = jnp.concatenate([g, jnp.zeros((8, 512), F32)], axis=0).astype(BF16)
        y0 = _dot_nt(g, f256[...])
        for _ in range(4):
            yield
        put(side.at[2], jnp.concatenate([y0, jnp.zeros((112, 256), F32)], axis=0).T)

    def s_fwd(u, t):
        ct, e = divmod(u, 4)
        put(ybuf.at[u % NY, t], ticking(_dot(lhs(sfw32[t * 4 + e]), bf(zin[ct, t * 4 + e]))))

    def s_filter(u, g):
        ct, e = divmod(u, 4)
        z = [tuple(ybuf[u % NY, t, pl.ds(g * 16 + i, 8), :] for i in (0, 8))
             for t in range(8)]
        z[0], z[1] = [tuple(gate(v, SGLAG if u * 8 + g < 122 - S_LAG else SGLAG2) for v in zz) for zz in z[0:2]]
        xk = _dft8(z, False)
        for k2 in range(8):
            wr = wf[0, ct, e, k2, pl.ds(g * 8, 8), :]
            wi = wf[1, ct, e, k2, pl.ds(g * 8, 8), :]
            re, im = xk[k2]
            xk[k2] = (re * wr - im * wi, re * wi + im * wr)
        for t, (re, im) in enumerate(_dft8(xk, True)):
            words = pack(re, im)
            pin(words)
            put(fbuf.at[u % NY, t, pl.ds(g * 8, 8), :], words)

    def s_inv(u, t):
        ct, e = divmod(u, 4)
        o = _dot(lhs(siv32[t * 4 + e]), bf(fbuf[u % NY, t]))
        put(zout.at[ct, t * 4 + e], ticking(o) if u * 8 + t >= 110 - S_LAG else o)

    def add_s_stage(sched, early, ready, t1):
        ahead = 8 + S_LAG
        tick = early
        for t in sorted(range(8), key=lambda t: ready[t]):
            for i in range(t, ahead, 8):
                tick = max(tick + 0.5, ready[t])
                sched.add(tick, _once(s_fwd, i // 8, t))
        t1 = max(t1, int(tick) + 1)
        sched.add(max(max(ready), t1), side_path())
        for i in range(128):
            if i + ahead < 128:
                sched.add(t1 + i, _once(s_fwd, *divmod(i + ahead, 8)))
            sched.add(t1 + i, _once(s_filter, *divmod(i, 8)))
            sched.add(t1 + 9 + (i if i < 120 else 120 + (i - 120) // 4), _once(s_inv, *divmod(i, 8)))
        return [t1 + 32 * ct + 40 for ct in range(3)] + [t1 + 131]

    def d_inv_cols(b, ct):
        c, t = divmod(b, 8)
        ra, rb = PAIRS[ct]
        lane = _lane(16)
        lo = lane < 64
        u = [(zout[ct, t * 4 + e, r16(c), :], zout[ct, t * 4 + e, r16(4 + c), :]) for e in range(4)]
        u[0], u[1] = tuple(map(gate, u[0])), tuple(map(gate, u[1]))
        z = _dft4(u, True)
        z = [(re, _swap(im)) for re, im in z]
        if ct == 0:
            y0 = [pltpu.roll(side[2, pl.ds(64 * lb + 16 * c, 16), :], 64 - t, 1) for lb in range(4)]
        yield from _latency()
        for lb, (re, sw) in enumerate(z):
            sw = gate(sw)
            a, bb = lax.select(lo, re, sw), lax.select(lo, sw, re)
            if ct == 0:
                a = jnp.where(lane == 64, y0[lb], a)
            pin(a, bb)
            ubuf[b % RING, ra, r16(lb), :] = a.astype(BF16)
            ubuf[b % RING, rb, r16(lb), :] = bb.astype(BF16)

    def d_inv_rows(b, lb, stats, first):
        u = [uout[b % RING, r, r16(lb), :] for r in range(8)]
        ys = yield from _d_butterfly_inv([gate(v) if r < 4 else v for r, v in enumerate(u)], pin, gate)
        xs = [x + y for x, y in zip(load_x(b, lb, first), ys)]
        for j in range(NT):
            put(xres.at[b, j, r16(lb), :], xs[j])
        stats[b, lb] = yield from ln_stats(xs)
        if b % 2:
            for j in range(4):
                a = [(xres[bb, j + o, r16(lb), :] - stats[bb, lb][0]) * stats[bb, lb][1]
                     for bb in (b - 1, b) for o in (0, 4)]
                a[0], a[3] = gate(a[0]), gate(a[3])
                for k, v in enumerate(_strassen_lhs(*a)):
                    if k not in (2, 3):
                        pin(v)
                    abuf[b // 2, k, j, r16(lb), :] = v.astype(BF16)
                if j < 3:
                    yield

    def add_d_inv(sched, tick, b, gap, stats, first, cols=None):
        per_tick = 4
        cols = cols or [tick + ct * gap for ct in range(4)]
        for ct in range(4):
            sched.add(cols[ct], d_inv_cols(b, ct))
        tick = int(cols[3]) + XGAP + 1
        sched.add(tick, d_dots(b, 8, per_tick))
        tick += 8 // per_tick + 3
        for lb in range(4):
            sched.add(tick + lb * gap, d_inv_rows(b, lb, stats, first))
        return int(tick + 3 * gap) + 3 * XGAP + 1 + 4

    def gemm(lhs32, rhs32, jobs, sink):
        for slot, b, n in jobs:
            m = {}
            for k in (3, 1, 0, 6, 5, 4, 2):
                m[k] = ticking(_dot(lhs(*[lhs32[slot, k, j] for j in range(4)]), bf(rhs32[n // 2, k])))
                if k == 1:
                    sink(b + 1, n, m[1] - m[3])
                elif k == 0:
                    c11, c22 = m[3] - m[0], m[1] - m[0]
                elif k == 6:
                    c11 = m[6] - c11
                elif k == 5:
                    c22 = m[5] - c22
                elif k == 4:
                    sink(b, n, c11 - m[4])
                elif k == 2:
                    sink(b, n + 1, m[4] - m[2])
                    sink(b + 1, n + 1, c22 - m[2])
                yield

    def qkv_sink(b, n, o):
        c, t = divmod(b, 8)
        dst = (qbuf, kbuf, vbuf)[n // NT]
        for lb in range(4):
            put(dst.at[n % NT, t, pl.ds(8 + 64 * lb + 16 * c, 16), :], o[lb * 16:(lb + 1) * 16])
        if b == 0 and n >= NT:
            first = jnp.broadcast_to(o[0:1], (8, 128))
            for tt in range(8):
                dst[n % NT, tt, pl.ds(0, 8), :] = first

    def out_rows(r, i, last):
        c, t = divmod(r, 8)
        return (c * 8 + t % 2 * 4 + i, t // 2) if last and c == 0 else (r, i)

    def out_sink(last, r, n, o):
        for i in range(4):
            b, lb = out_rows(r, i, last)
            put(xres.at[b, n, r16(lb), :], xres[b, n, r16(lb), :] + o[i * 16:(i + 1) * 16])

    def attention(b, lb, h):
        c, t = divmod(b, 8)
        scale = HEAD_DIM ** -0.5
        r0 = 8 + 64 * lb + 16 * c + 8 * h
        src = [((t - 2 * w) % 8, -((t - 2 * w) // 8)) for w in range(WIN)]
        acc = [None] * WIN
        for j in range(NT):
            q = gate(qbuf[j, t, pl.ds(r0, 8), :], ALAG)
            for w, (ts, sh) in enumerate(src):
                p = q * kbuf[j, ts, pl.ds(r0 - sh, 8), :]
                acc[w] = p if j == 0 else acc[w] + p
            if j % 2 and j < NT - 1:
                pin(*acc)
                yield
        part = [(r, pltpu.roll(r, 64, 1)) for r in acc]
        yield from _latency()
        part = [r + rr for r, rr in part]
        part = [(r, pltpu.roll(r, 32, 1)) for r in part]
        yield from _latency()
        logits = [r + rr for r, rr in part]
        if r0 == 8:
            sub = lax.broadcasted_iota(jnp.int32, (8, 128), 0)
            logits = [jnp.where(sub >= sh, r, -1e9 / scale) if sh else r
                      for r, (_, sh) in zip(logits, src)]
        logits[0] = gate(logits[0], ALAG)
        m = _tree(jnp.maximum, logits)
        ps = [jnp.exp2((r - m) * (scale * float(np.log2(np.e)))) for r in logits]
        total = _tree(_add, ps)
        pin(total)
        inv = pltpu.reciprocal(total, approx=True)
        inv = inv * (2.0 - total * inv)
        for j in range(NT):
            if j % 2 == 0:
                yield
                ps[0], ps[4] = gate(ps[0], ALAG), gate(ps[4], ALAG)
            o = _chain(_add, [ps[w] * vbuf[j, ts, pl.ds(r0 - sh, 8), :]
                              for w, (ts, sh) in enumerate(src)]) * inv
            pin(o)
            put(qbuf.at[j, t, pl.ds(r0, 8), :], o)

    def out_operands(r, i, last):
        for j in range(4):
            a = [qbuf[j + o, b % 8, pl.ds(8 + 64 * lb + 16 * (b // 8), 16), :]
                 for b, lb in (out_rows(r, i, last), out_rows(r + 1, i, last)) for o in (0, 4)]
            a[0], a[3] = gate(a[0]), gate(a[3])
            for k, v in enumerate(_strassen_lhs(*a)):
                if k not in (2, 3):
                    pin(v)
                obuf[r // 2, k, j, r16(i), :] = v.astype(BF16)
            if j < 3:
                yield

    def store_rows(b, lb):
        c, t = divmod(b, 8)
        for j in range(NT):
            words = pack(xres[b, j, r16(lb), :], xres[b + 1, j, r16(lb), :])
            pin(words)
            io32[j, lb, c, pl.ds(t // 2, 16, stride=4), :] = words

    unit_ticks = NT + 2 * XGAP
    step = 2
    out_ticks = 28

    def add_proj(sched, tick, c, lo, hi):
        jobs = [(b // step, b, n) for b in range(8 * c, 8 * c + 8, step) for n in range(lo, hi, step)]
        sched.add(tick, gemm(abuf32, wqkv32, jobs, qkv_sink))
        return tick + len(jobs) * out_ticks * step // NT

    def add_attention(sched, tick, pace, rows, last):
        units = [(r, i, half, h) for r in rows[::2] for i in range(4) for half in range(2) for h in range(2)]
        for n, (r, i, half, h) in enumerate(units):
            sched.add(tick + n * pace, attention(*out_rows(r + half, i, last), h))
            if half and h:
                sched.add(int(tick + n * pace) + unit_ticks, out_operands(r, i, last))

    def add_out(sched, tick, rows, last):
        jobs = [(r // 2, r, n) for r in rows[::2] for n in range(0, NT, 2)]
        sched.add(tick, gemm(obuf32, wo32, jobs, functools.partial(out_sink, last)))

    def add_tail(sched, tick, rows, last):
        ready = {}
        for i, r in enumerate(rows):
            t0 = tick + (i // 2 + 1) * out_ticks
            fast = i >= len(rows) - (2 if last else 4)
            if not last:
                t0 += 0 if fast else 3 + i % 2 * out_ticks // 2
                ready[r % 8] = add_d_fwd(sched, t0, r, i % 2 if fast else out_ticks / 8)
            elif r % 2:
                c, p = r // 8, r % 8 // 2
                gap = 0 if fast else 3
                for j in range(4):
                    sched.add(t0 + (j + 1) * gap, _once(store_rows, *((r - 1, j) if c else (2 * j, p))))
                for lb in ([p] if c == 0 else range(4) if p == 3 else []):
                    sched.add(t0 + 5 * gap + 1, _once(start, out_copies(c, lb)))
        return ready

    q_ticks = 8 * out_ticks // step
    att_ticks = unit_ticks + 1 + 2
    order = [(a + 8) % NB for a in range(NB)]

    def add_attention_block(sched, cols, last):
        stats = {}
        t0 = max([add_d_inv(sched, 0, b, 0, stats, not last, cols) for b in range(step)])
        if not last:
            sched.add(cols[3] - KLEAD, _once(wait, qkv_copies(1) + dmat_cp))
            done = add_prep_wqkv(sched, cols[3] - KLEAD, 1, KPACE, [7] * 4)
            t0 = max(t0, done[0])
            assert all(d <= t0 + p * out_ticks / 4 for p, d in enumerate(done))
            sched.add(t0 + out_ticks, _once(wait, qkv_copies(2)))
            sched.add(t0 + out_ticks, _once(start, qkv_copies(0)))
            done = add_prep_wqkv(sched, t0 + out_ticks, 2, 2 * out_ticks - 6, [out_ticks - 4] * 4)
            assert all(d <= t0 + q_ticks + p * out_ticks for p, d in enumerate(done))
            sched.add(t0 + 2 * q_ticks, _once(wait, qkv_copies(0)))
            sched.add(t0 + 2 * q_ticks, _once(start, wo_copies))
            done = add_prep_wqkv(sched, t0 + 2 * q_ticks, 0, q_ticks - 10, [q_ticks / 4] * 4)
            assert done[-1] <= t0 + 4 * q_ticks
            sched.add(t0 + 8 * q_ticks, _once(wait, wo_copies))
            for i in range(32):
                sched.add(t0 + 8 * q_ticks + i * q_ticks / 16, _once(prep_wo, *divmod(i, 8)))
        tick, kv_start, q_start = t0, {}, {}
        for kind, c in ("k0", "k1", "q1", "k2", "q2", "k3", "q3", "q0"):
            if kind == "k":
                kv_start[int(c)] = tick
                if c == "0" and not last:
                    tick = add_proj(sched, tick, 0, NT, 2 * NT)
                    jobs = [(b // step, b, n) for n in range(2 * NT, 3 * NT, step) for b in range(0, 8, step)]
                    sched.add(tick, gemm(abuf32, wqkv32, jobs, qkv_sink))
                    tick += q_ticks
                    continue
                tick = add_proj(sched, tick, int(c), NT, 3 * NT)
            else:
                q_start[int(c)] = tick
                tick = add_proj(sched, tick, int(c), 0, NT)
        pace = 2 * out_ticks / step
        for b in range(step, NB):
            due = kv_start[b // 8] + (b % 8 // step) * (2 if last or b >= 8 else 1) * out_ticks
            gap = min(1 + (b - step) * 0.5, DGAP1 if last else DGAP0)
            pace = DPACE1 if last else DPACE0
            at = (b - step) * pace
            at = t0 + at + max(0, at - 4 * q_ticks - out_ticks) * DSLOW
            if not last and b < 8:
                at, gap = max(cols[3], t0 + (b // step - 1) * out_ticks - (step - b % step) * 8), 1
            end = add_d_inv(sched, at, b, gap, stats, not last)
            assert end <= due, (b, end, due)
        begin = [q_start[c] + out_ticks + 3 for c in (1, 2, 3)] + [tick + (ATT1 if last else ATT0)]
        begin.append(tick + (NB // step - 1) * out_ticks - att_ticks)
        for i, c in enumerate((1, 2, 3, 0)):
            pace = (begin[i + 1] - begin[i]) / 64
            assert begin[i] >= max(kv_start[c], kv_start[(c - 1) % 4]) + 2 * q_ticks
            for p in range(4):
                assert begin[i] + 16 * p * pace >= q_start[c] + (4 if last and c == 0 else p + 1) * out_ticks
                assert begin[i] + (16 * p + 15) * pace + att_ticks <= tick + (4 * i + p) * out_ticks + 1e-6
            add_attention(sched, begin[i], pace, range(8 * c, 8 * c + 8), last)
        add_out(sched, tick, order, last)
        return tick + (NB // step) * out_ticks, add_tail(sched, tick, order, last)

    def add_input(sched):
        ready = {}
        after = (x_copies(2), x_copies(3) + perm_cp + w_copies(0) + w_copies(1),
                 w_copies(2) + w_copies(3), w_copies(4))
        for c in range(NC):
            sched.add(c * 32, _once(wait, x_copies(c)))
            sched.add(c * 32, _once(start, after[c]))
            for t in range(8):
                ready[t] = add_d_fwd(sched, c * 32 + t * 4, c * 8 + t, 1, 2, True)
        return 128 + 9, ready

    def add_filter_prep(sched, tick):
        after = {0: w_copies(5), 1: w_copies(6), 2: w_copies(7), 3: f256_cp + dmat_cp,
                 5: qkv_copies(1), 7: qkv_copies(2)}
        begin = [F0 + g * (tick - F0) / 4 for g in range(4)] + [tick + FG * g for g in range(5)]
        for g in range(8):
            sched.add(begin[g], _once(wait, w_copies(g) + ([] if g else perm_cp)))
            sched.add(begin[g], _once(start, after.get(g, [])))
            for m in range(4):
                sched.add(begin[g] + m * (begin[g + 1] - begin[g]) / 4,
                          _once(prep_filter, g // 4, g % 4 * 4 + m))
        sched.add(begin[8] + 1, _once(wait, f256_cp))
        return begin[8] + 2

    sched = _Schedule()

    def phase(fn, *args):
        fn(sched, *args)
        sched.run()
        token.clear()
        clock.clear()

    start(x_copies(0))
    for ref in (abuf32, obuf32, ubuf32, wo32, sfw32, siv32, wide32):
        put(ref.at[(0,) * (len(ref.shape) - 2) + (pl.ds(0, 8),)], jnp.zeros((8, 128), U32))
    make_wide()
    start(x_copies(1))
    for t in range(8):
        make_s_fwd(t)
    for e in range(4):
        make_s_inv(e)
    tick, ready = add_input(sched)
    cols = add_s_stage(sched, tick, ready, add_filter_prep(sched, tick))
    tick, ready = add_attention_block(sched, cols, False)
    cols = add_s_stage(sched, tick, ready, tick)
    add_attention_block(sched, cols, True)
    sched.run()
    for c in range(NC):
        for lb in range(4):
            wait(out_copies(c, lb))


@jax.jit
def pallas_interleave_layers__spectral_gfnet__sliding_local_dilated__prompt_kernel(
    A_x: jax.Array,
    A_w_r: jax.Array,
    A_w_i: jax.Array,
    B_x: jax.Array,
    B_wqkv: jax.Array,
    B_wo: jax.Array,
):
    del B_x
    assert A_x.shape == (1, S, D) and A_w_r.shape == (S, D // 2 + 1)
    cst = _constants()
    x = A_x.astype(BF16).reshape(4, NC, 128, D)
    wr, wi = A_w_r.astype(BF16).T, A_w_i.astype(BF16).T
    hbm = pl.BlockSpec(memory_space=pl.ANY)
    edge = pl.BlockSpec((16, S), lambda i: (D // 32, 0))
    vm = pltpu.VMEM
    out = pl.pallas_call(
        _kernel,
        grid=(1,),
        in_specs=[hbm, hbm, hbm, edge, edge, hbm, hbm, hbm, hbm,
                  pl.BlockSpec((24, 256), lambda i: (0, 0)),
                  pl.BlockSpec((2, 16, 128), lambda i: (0, 0, 0))],
        out_specs=hbm,
        out_shape=jax.ShapeDtypeStruct((4, NC, 128, D), BF16),
        scratch_shapes=[
            vm((NT, 4, NC, 128, 128), BF16),
            vm((17, 128, 128), BF16),
            vm((32, 128, 128), BF16),
            vm((32, 128, 128), BF16),
            vm((256, 512), BF16),
            vm((2, 16, 512, 128), BF16),
            vm((2, 4, 4, 8, 64, 128), F32),
            vm((3 * NT, D, 128), BF16),
            vm((NT, D // 2, 128), U32),
            vm((12, 7, 512, 128), BF16),
            vm((NT, D, 128), BF16),
            vm((4, 7, 512, 128), BF16),
            vm((NB, NT, 64, 128), F32),
            vm((4, 32, 64, 128), U32),
            vm((4, 32, 128, 128), F32),
            vm((NY, 8, 128, 128), F32),
            vm((NY, 8, 64, 128), U32),
            vm((RING, 8, 64, 128), BF16),
            vm((RING, 9, 64, 128), F32),
            vm((NB // 2, 7, 4, 64, 128), BF16),
            vm((NB // 2, 7, 4, 64, 128), BF16),
            vm((NT, 8, 264, 128), F32),
            vm((NT, 8, 264, 128), F32),
            vm((NT, 8, 264, 128), F32),
            vm((3, 256, 128), F32),
            vm((8, 256, 128), BF16),
            pltpu.SemaphoreType.DMA((NC,)),
            pltpu.SemaphoreType.DMA((3,)),
            pltpu.SemaphoreType.DMA((8,)),
            pltpu.SemaphoreType.DMA((3,)),
            pltpu.SemaphoreType.DMA(()),
            pltpu.SemaphoreType.DMA(()),
        ],
        compiler_params=pltpu.CompilerParams(
            dimension_semantics=("arbitrary",), vmem_limit_bytes=120 * 2**20),
    )(x, wr, wi, wr, wi, B_wqkv.astype(BF16), B_wo.astype(BF16),
      cst["small"], cst["f256"], cst["tw"], cst["d8"])
    return out.reshape(1, S, D)
```

```python
import functools

import jax
import jax.numpy as jnp
import numpy as np
from jax import lax
from jax.experimental import pallas as pl
from jax.experimental.pallas import tpu as pltpu

S, D = 2048, 1024
NT = D // 128
NC = 4
WIN = 8
HEAD_DIM = 32
EPS = 1e-5
F32, BF16, U32 = jnp.float32, jnp.bfloat16, jnp.uint32
PAIRS = ((0, 4), (1, 7), (2, 6), (3, 5))
RSQ2 = float(np.sqrt(0.5))
NB = S // 64

RING = 8
NY = 4
XGAP = 3
GLAG = 4
ALAG = 4
SGLAG = 3
SGLAG2 = 5
S_LAG = 3
F0 = 112
KLEAD = 52
KPACE = 48
DGAP0 = 4.75
DGAP1 = 4.2
DPACE0 = 21
DPACE1 = 15.5
DSLOW = 0.6
SYNC = 3
ILAG = 3
FG = 4
TOFF = 3
ATT0 = 10
ATT1 = 95


def _residues(r):
    return (0, 8) if r == 0 else (r, 16 - r)


def _d_matrices():
    n = np.arange(64)[:, None]
    a = np.arange(32)
    fwd = np.zeros((8, 128, 128))
    inv = np.zeros((8, 128, 128))
    for r in range(8):
        kd = np.concatenate([16 * a + p for p in _residues(r)])
        weight = np.full(64, 2.0)
        if r == 0:
            kd[0], weight[0] = D // 2, 1.0
            ph = np.exp(-2j * np.pi * n * kd[None, :] / D)
            sgn = np.where(kd % 16 == 0, 1.0, -1.0)[None, :]
            m = np.concatenate([ph, ph * sgn], axis=0)
            re, im = m.real.copy(), m.imag.copy()
            ire, iim = re.copy(), im.copy()
            im[:, 0] = 1.0
            iim[:, 0] = 1.0
        else:
            p = 12 if r == 4 else r
            ph = np.exp(-2j * np.pi * n * kd[None, :] / D)
            si = np.where(kd % 16 == p, 1.0, -1.0)[None, :]
            m = np.concatenate([ph, 1j * si * ph], axis=0)
            re, im = m.real, m.imag
            ire, iim = re, im
        swapped = r in (4, 7, 6, 5)
        cols = [im, re] if swapped else [re, im]
        icols = [iim * weight, ire * weight] if swapped else [ire * weight, iim * weight]
        fwd[r] = np.concatenate(cols, axis=1)
        inv[r] = np.concatenate(icols, axis=1).T / D
    return fwd, inv


def _side_matrices():
    l = np.arange(256)
    f = np.exp(-2j * np.pi * ((l[:, None] * l[None, :]) % 256) / 256)
    f256 = np.concatenate([f.real, f.imag], axis=1)
    t = np.arange(8)
    tw = np.exp(-2j * np.pi * t[:, None] * l[None, :] / S)
    tw = np.concatenate([tw.real, tw.imag, np.zeros((8, 256))], axis=0)
    g = np.exp(-2j * np.pi * t[:, None] * t[None, :] / 8)
    d8 = np.zeros((2, 16, 128))
    d8[0, :, :16] = np.block([[g.real, -g.imag], [g.imag, g.real]])
    d8[1, :, :16] = d8[0, :, :16].T / S
    return f256, tw, d8


def _filter_rows():
    p = np.zeros((1, 128, 128))
    for k in range(32):
        for e in range(4):
            p[0, e * 32 + k, 4 * k + e] = 1.0
    return p


@functools.lru_cache(maxsize=None)
def _constants():
    dfw, div = _d_matrices()
    f256, tw, d8 = _side_matrices()
    small = np.concatenate([dfw, div, _filter_rows()], axis=0)
    b = lambda x: np.asarray(x, np.float32).astype(BF16)
    return dict(small=b(small), f256=b(f256),
                tw=np.asarray(tw, np.float32), d8=b(d8))


def _dot(a, b):
    return jnp.dot(a, b, preferred_element_type=F32)


def _dot_nt(a, b):
    return lax.dot_general(a, b, (((1,), (1,)), ((), ())), preferred_element_type=F32)


def _tree(op, xs):
    xs = list(xs)
    while len(xs) > 1:
        xs = [op(xs[i], xs[i + 1]) if i + 1 < len(xs) else xs[i] for i in range(0, len(xs), 2)]
    return xs[0]


def _chain(op, xs):
    return functools.reduce(op, xs)


def _lane(rows):
    return lax.broadcasted_iota(jnp.int32, (rows, 128), 1)


def _swap(x):
    return pltpu.roll(x, 64, 1)


def _unpack(w, i):
    return pltpu.unpack_elementwise(w, index=i, packed_dtype=BF16, unpacked_dtype=F32)


def _latency():
    for _ in range(XGAP):
        yield


def _add(a, b):
    return a + b


def _row_mean(xs):
    return jnp.sum(_tree(_add, xs), axis=1, keepdims=True) * (1.0 / D)


def _twiddle16(r, x, y):
    lo = _lane(x.shape[0]) < 64
    wr, wi = float(np.cos(np.pi * r / 8)), float(-np.sin(np.pi * r / 8))
    cross = jnp.where(lo, 0.0, wr)
    return x * jnp.where(lo, 1.0, wi) + y * cross, y * jnp.where(lo, 1.0, -wi) + x * cross


def _d_butterfly_fwd(a, emit, pin, wide):
    s = [a[j] + a[j + 4] for j in range(4)]
    e, o = s[0] + s[2], s[1] + s[3]
    total, t4 = e + o, e - o
    emit(4, t4)
    d0, nd2 = a[0] - a[4], a[6] - a[2]
    d1, d3 = a[1] - a[5], a[3] - a[7]
    p, q = (d1 - d3) * RSQ2, (d1 + d3) * -RSQ2
    ts = {1: (d0 + p, q + nd2), 2: (s[0] - s[2], s[3] - s[1]), 3: (d0 - p, q - nd2)}
    mean8 = jnp.sum(total, axis=1, keepdims=True) * (1.0 / 128)
    if wide:
        for r, (tr, ti) in ts.items():
            emit(r, tr)
            emit(8 - r, ti)
    else:
        ab = {r: _twiddle16(r, *t) for r, t in ts.items()}
        ab = {r: (a, _swap(b)) for r, (a, b) in ab.items()}
    dev = _tree(_add, [v * v for t in ts.values() for v in t]) * 2.0 + t4 * t4
    pin(dev)
    yield from _latency()
    t0 = total - mean8
    emit(0, t0)
    var = jnp.sum(dev + t0 * t0, axis=1, keepdims=True) * (1.0 / (NT * D))
    if not wide:
        for r, (x, y) in ab.items():
            emit(r, x + y)
            emit(8 - r, x - y)
    yield from _latency()
    return lax.rsqrt(var + EPS)


def _d_butterfly_inv(u, pin, gate):
    ab = {r: (u[r] + u[8 - r], _swap(u[r] - u[8 - r])) for r in (1, 2, 3)}
    e, o = u[0] + u[4], u[0] - u[4]
    yield from _latency()
    ts = {r: _twiddle16(r, x, gate(y)) for r, (x, y) in ab.items()}
    pin(*[v for t in ts.values() for v in t])
    yield
    s = [e + ts[2][0], o - ts[2][1], e - ts[2][0], o + ts[2][1]]
    p = (ts[1][0] - ts[3][0]) * RSQ2
    q = (ts[1][1] + ts[3][1]) * RSQ2
    d0, d1, d2, nd3 = ts[1][0] + ts[3][0], p - q, ts[3][1] - ts[1][1], p + q
    return [s[0] + d0, s[1] + d1, s[2] + d2, s[3] - nd3,
            s[0] - d0, s[1] - d1, s[2] - d2, s[3] + nd3]


def _strassen_lhs(a11, a12, a21, a22):
    return [a11 + a22, a21 + a22, a11, a22, a11 + a12, a21 - a11, a12 - a22]


def _strassen_rhs(b11, b12, b21, b22):
    return [b11 + b22, b11, b22 - b12, b11 - b21, b22, b11 + b12, b21 + b22]


def _cadd(a, b):
    return a[0] + b[0], a[1] + b[1]


def _csub(a, b):
    return a[0] - b[0], a[1] - b[1]


def _dft4(z, inverse):
    a, b = _cadd(z[0], z[2]), _csub(z[0], z[2])
    c, d = _cadd(z[1], z[3]), _csub(z[1], z[3])
    minus = (b[0] + d[1], b[1] - d[0])
    plus = (b[0] - d[1], b[1] + d[0])
    return [_cadd(a, c), plus if inverse else minus, _csub(a, c), minus if inverse else plus]


def _dft8(z, inverse):
    ev = _dft4(z[0::2], inverse)
    od = _dft4(z[1::2], inverse)
    out = [None] * 8
    out[0], out[4] = _cadd(ev[0], od[0]), _csub(ev[0], od[0])
    (er, ei), (x, y) = ev[2], od[2]
    minus, plus = (er + y, ei - x), (er - y, ei + x)
    out[2], out[6] = (plus, minus) if inverse else (minus, plus)
    for k in (1, 3):
        (er, ei), (x, y) = ev[k], od[k]
        sm, df = (x + y) * RSQ2, (x - y) * RSQ2
        if not inverse:
            if k == 1:
                out[1], out[5] = (er + sm, ei - df), (er - sm, ei + df)
            else:
                out[3], out[7] = (er - df, ei - sm), (er + df, ei + sm)
        else:
            if k == 1:
                out[1], out[5] = (er + df, ei + sm), (er - df, ei - sm)
            else:
                out[3], out[7] = (er - sm, ei + df), (er + sm, ei - df)
    return out


class _Schedule:
    def __init__(self):
        self.pending = []

    def add(self, tick, gen):
        self.pending.append((int(tick), len(self.pending), gen))

    def run(self):
        pending = sorted(self.pending, key=lambda p: p[:2])
        active, tick, i = [], 0, 0
        while active or i < len(pending):
            while i < len(pending) and pending[i][0] <= tick:
                active.append(pending[i][2])
                i += 1
            for g in list(active):
                if next(g, 0) == 0:
                    active.remove(g)
            tick += 1
        self.pending = []


def _once(fn, *args):
    fn(*args)
    return
    yield


def _kernel(x_hbm, wr_hbm, wi_hbm, wr_edge, wi_edge, wqkv_hbm, wo_hbm,
            small_hbm, f256_hbm, tw_ref, d8_ref,
            out_hbm,
            io, small, sfw, siv, f256, wraw, wf, wqkv_raw, wtmp, wqkv, wo_raw, wo,
            xres, zin, zout, ybuf, fbuf, ubuf, uout, abuf, obuf, qbuf, kbuf, vbuf, side,
            wide, sem_x, sem_c, sem_w, sem_qkv, sem_wo, sem_out):

    def x_copies(c):
        return [pltpu.make_async_copy(x_hbm.at[:, c, :, pl.ds(j * 128, 128)], io.at[j, :, c],
                                      sem_x.at[c]) for j in range(NT)]

    def out_copies(c, lb):
        return [pltpu.make_async_copy(io.at[j, lb, c], out_hbm.at[lb, c, :, pl.ds(j * 128, 128)],
                                      sem_out) for j in range(NT)]

    perm_cp, dmat_cp, f256_cp = ([pltpu.make_async_copy(s, d, sem_c.at[i])] for i, (s, d) in enumerate((
        (small_hbm.at[pl.ds(16, 1)], small.at[pl.ds(16, 1)]),
        (small_hbm.at[pl.ds(0, 16)], small.at[pl.ds(0, 16)]), (f256_hbm, f256))))

    def w_copies(g):
        src = (wr_hbm, wi_hbm)[g // 4]
        return [pltpu.make_async_copy(src.at[pl.ds(0, 512), pl.ds(m * 128, 128)], wraw.at[g // 4, m],
                                      sem_w.at[g]) for m in range(g % 4 * 4, g % 4 * 4 + 4)]

    def qkv_copies(g):
        return [pltpu.make_async_copy(wqkv_hbm.at[:, pl.ds(g * D + j * 128, 128)],
                                      wqkv_raw.at[g * NT + j], sem_qkv.at[g]) for j in range(NT)]

    wo_copies = [pltpu.make_async_copy(wo_hbm.at[:, pl.ds(j * 128, 128)], wo_raw.at[j], sem_wo)
                 for j in range(NT)]

    def start(cs):
        for cp in cs:
            cp.start()

    def wait(cs):
        for cp in cs:
            cp.wait()

    io32, wraw32, wo_raw32 = io.bitcast(U32), wraw.bitcast(U32), wo_raw.bitcast(U32)
    small32, sfw32, siv32, wide32 = (r.bitcast(U32) for r in (small, sfw, siv, wide))
    wqkv_raw32, wqkv32, wo32 = (r.bitcast(U32) for r in (wqkv_raw, wqkv, wo))
    ubuf32, abuf32, obuf32 = ubuf.bitcast(U32), abuf.bitcast(U32), obuf.bitcast(U32)

    never = tw_ref[16:24, 0:128] != 0.0
    never_wide = {n: jnp.concatenate([tw_ref[16:24, 0:128]] * n, axis=1) != 0.0 for n in (1, 2, 4)}
    token = {}

    def pin(*values):
        for v in values:
            key = v.shape[0], v.dtype == F32
            token[key] = (lax.max if key[1] else lax.bitwise_xor)(token[key], v) if key in token else v

    clock = []

    def gate(v, lag=GLAG):
        if len(clock) < lag:
            return v
        old = clock[-lag] if v.dtype == F32 else pltpu.bitcast(clock[-lag], v.dtype)
        if v.shape[0] == 8:
            return lax.select(never, old, v)
        return lax.concatenate([lax.select(never, old, v[0:8]), v[8:]], 0)

    def ticking(o):
        clock.append(o[0:8])
        del clock[:-16]
        return o

    def lhs(*tiles):
        if not token and len(tiles) == 4 and len(clock) >= SYNC:
            pin(clock[-SYNC])
        words = lax.concatenate(tiles, 1) if len(tiles) > 1 else tiles[0]
        if token:
            parts = [pltpu.bitcast(v, U32) if is_float else v for (_, is_float), v in token.items()]
            token.clear()
            w = _chain(lax.bitwise_xor, [v[i:i + 8] if v.shape[0] > 8 else v
                                         for v in parts for i in range(0, v.shape[0], 8)])
            w = lax.concatenate([w] * len(tiles), 1) if len(tiles) > 1 else w
            words = lax.concatenate([lax.select(never_wide[len(tiles)], w, words[0:8]), words[8:]], 0)
        return pltpu.bitcast(words, BF16)

    def bf(words):
        return pltpu.bitcast(words, BF16)

    def pack(a, b):
        return pltpu.bitcast(pltpu.pack_elementwise([a, b], packed_dtype=BF16), U32)

    def r16(i):
        return pl.ds(i * 16, 16)

    always = {}

    def put(ref, v):
        if v.shape not in always:
            always[v.shape] = jnp.ones(v.shape, jnp.bool_)
        pltpu.store(ref, v, mask=always[v.shape])

    def load_x(b, lb, from_input):
        if from_input:
            c, t = divmod(b, 8)
            return [_unpack(io32[j, lb, c, pl.ds(t // 2, 16, stride=4), :], t % 2) for j in range(NT)]
        return [xres[b, j, r16(lb), :] for j in range(NT)]

    def unit(p):
        angle = (((p + S // 2) & (S - 1)) - S // 2).astype(F32) * (2 * np.pi / S)
        return jnp.cos(angle), jnp.sin(angle)

    def times_row(a, b, i):
        br, bi = (jnp.broadcast_to(v[i:i + 1], (8, 128)) for v in b)
        return a[0] * br - a[1] * bi, a[0] * bi + a[1] * br

    def make_wide():
        row, lane = lax.broadcasted_iota(jnp.int32, (8, 128), 0), _lane(8)
        for ct, (ra, rb) in enumerate(PAIRS):
            res = _residues(ra) + _residues(rb)
            kd = (lane & 31) * 16 + _chain(
                _add, [jnp.where(lane >> 5 == g, p, 0) for g, p in enumerate(res)])
            if ct == 0:
                kd = jnp.where(lane == 0, D // 2, kd)
            fine, coarse = unit(-2 * row * kd), [unit(-16 * (row + 8 * h) * kd) for h in range(2)]
            for a in range(16):
                re, im = times_row(fine, coarse[a // 8], a % 8)
                if ct == 0:
                    even = kd & 7 == 0
                    top = jnp.where(even, re, 0.0), jnp.where(lane == 0, 1.0, jnp.where(even, im, 0.0))
                    bottom = jnp.where(even, 0.0, re), jnp.where(even, 0.0, im)
                else:
                    sign = jnp.where(kd & 7 == ra, 1.0, -1.0)
                    top, bottom = (re, im), (-sign * im, sign * re)
                for i in range(2):
                    wide[2 * ct + i, pl.ds(8 * a, 8), :] = top[i].astype(BF16)
                    wide[2 * ct + i, pl.ds(128 + 8 * a, 8), :] = bottom[i].astype(BF16)

    def make_s_fwd(t):
        row, lane = lax.broadcasted_iota(jnp.int32, (8, 128), 0), _lane(8)
        pos = 8 * (lane >> 1) + t
        fine = unit((lane & 1) * (S // 4) - 4 * row * pos)
        shift, coarse = unit(-row * pos), unit(-32 * row * pos)
        for e in range(4):
            base = times_row(fine, shift, e)
            for g in range(8):
                for i, v in enumerate(times_row(base, coarse, g)):
                    sfw[t * 4 + e, pl.ds(16 * g + 8 * i, 8), :] = v.astype(BF16)

    def make_s_inv(e):
        row, lane = lax.broadcasted_iota(jnp.int32, (8, 128), 0), _lane(8)
        freq = 4 * (lane >> 1) + e
        fine = [v * (1.0 / S) for v in unit((lane & 1) * (S // 4) + 8 * row * freq)]
        shift, coarse = unit(row * freq), unit(64 * row * freq)
        for t in range(8):
            base = times_row(fine, shift, t)
            for g in range(8):
                for i, v in enumerate(times_row(base, coarse, g)):
                    siv[t * 4 + e, pl.ds(64 * i + 8 * g, 8), :] = v.astype(BF16)

    def prep_filter(ri, m):
        sub = lax.broadcasted_iota(jnp.int32, (8, 128), 0)
        edge = (wr_edge, wi_edge)[ri]
        res = {}
        for i in range(8):
            words = wraw32[ri, m, pl.ds(i, 32, stride=8), :]
            res[2 * i], res[2 * i + 1] = _unpack(words, 0), _unpack(words, 1)
        first = res[0][0:8]
        dst = pl.ds((m % 2) * 16 + ri * 8, 8)
        prev = jnp.zeros((8, 128), F32) if m < 2 else side[1, dst, :]
        put(side.at[1, dst, :], jnp.where(sub == m // 2, jnp.broadcast_to(first[0:1], (8, 128)), prev))
        nyq = jnp.broadcast_to(edge[0:1, pl.ds(m * 128, 128)].astype(F32), (8, 128))
        res[0] = jnp.concatenate([jnp.where(sub == 0, nyq, first), res[0][8:]], axis=0)
        for ct, (ra, rb) in enumerate(PAIRS):
            blk = jnp.concatenate([res[p] for p in _residues(ra) + _residues(rb)], axis=0)
            o = _dot_nt(lhs(small32[16]), blk.astype(BF16))
            for e in range(4):
                put(wf.at[ri, ct, e, m // 2, pl.ds((m % 2) * 32, 32), :], o[e * 32:(e + 1) * 32])

    def shuffle(words, index):
        return jnp.take_along_axis(words, index, axis=1)

    def prep_wqkv_tile(g, i, part):
        lane = _lane(8)
        index = (lane & 3) * 32 + (((lane >> 2) - i) & 7) * 4 + (lane >> 5)
        rows = [pl.ds((part * 16 + r) * 8, 8) for r in range(16)]
        ws = [shuffle(gate(wqkv_raw32[g * NT + i, rs, :]), index) for rs in rows]
        yield from _latency()
        for rs, w in zip(rows, ws):
            pin(w)
            put(wtmp.at[i, rs, :], w)

    def prep_wqkv_cross(g, r):
        pos = (_lane(8) >> 2) & 7
        u = [wtmp[(-j) % 8, pl.ds(r * 8, 8), :] for j in range(NT)]
        u[0], u[4] = gate(u[0]), gate(u[4])
        for bit in range(3):
            m = ((pos >> bit) & 1) == 1
            u = [lax.select(m, u[(j - (1 << bit)) % 8], u[j]) for j in range(NT)]
        for j in range(NT):
            pin(u[j])
            put(wqkv_raw32.at[g * NT + j, pl.ds(r * 8, 8), :], u[j])

    def prep_wqkv_pair(g, p, part):
        lane = _lane(8)
        ws = {}
        for n in range(2):
            index = (lane & 96) | ((lane + 4 * (2 * p + n)) & 31)
            for half in range(2):
                for r in range(part * 2, part * 2 + 2):
                    w = gate(wqkv_raw32[g * NT + 2 * p + n, pl.ds(half * 256 + r * 8, 8), :])
                    ws[r, half, n] = shuffle(w, index) if p + n else w
        yield from _latency()
        for r in range(part * 2, part * 2 + 2):
            quad = [ws[r, half, n] for half in range(2) for n in range(2)]
            ops = [_strassen_rhs(*[_unpack(w, i) for w in quad]) for i in range(2)]
            for k in range(7):
                word = {1: quad[0], 4: quad[3]}.get(k)
                if word is None:
                    word = pack(ops[0][k], ops[1][k])
                    pin(word)
                put(wqkv32.at[g * 4 + p, k, pl.ds(r * 8, 8), :], word)

    def add_prep_wqkv(sched, tick, g, ticks, pair_ticks):
        for i in range(32):
            sched.add(tick + i * ticks / 64, prep_wqkv_tile(g, *divmod(i, 4)))
        tick = int(tick + ticks / 2) + XGAP + 1
        for r in range(64):
            sched.add(tick + r * ticks / 128, _once(prep_wqkv_cross, g, r))
        tick = int(tick + ticks / 2) + 1
        done = []
        for p, n in enumerate(pair_ticks):
            for i in range(16):
                sched.add(tick + i * n / 16, prep_wqkv_pair(g, p, i))
            tick += n
            done.append(int(tick) + XGAP + 1)
        return done

    def prep_wo(p, dp):
        ws = [wo_raw32[2 * p + n, pl.ds(dp + off, 32, stride=16), :] for off in (0, 8) for n in (0, 1)]
        for i in range(2):
            b = [_unpack(w, i) for w in ws]
            r0 = (2 * dp + i) * 32
            for k, v in enumerate(_strassen_rhs(*b)):
                if k not in (1, 4):
                    pin(v)
                wo[p, k, pl.ds(r0, 32), :] = v.astype(BF16)

    def ln_stats(xs):
        lane_mean = _tree(_add, xs) * (1.0 / NT)
        lane_m2 = _tree(_add, [jnp.square(x - lane_mean) for x in xs])
        pin(lane_m2)
        mean = jnp.sum(lane_mean, axis=1, keepdims=True) * (1.0 / 128)
        yield from _latency()
        m2 = lane_m2 + jnp.square(gate(lane_mean) - mean) * float(NT)
        pin(m2)
        var = jnp.sum(m2, axis=1, keepdims=True) * (1.0 / D)
        yield from _latency()
        return mean, lax.rsqrt(gate(jnp.broadcast_to(var, (16, 128))) + EPS)

    def d_fwd_rows(b, lb, from_input=False):
        xs = load_x(b, lb, from_input)

        def emit(r, v):
            if not from_input or r % 4 == 0:
                pin(v)
            ubuf[b % RING, r, r16(lb), :] = v.astype(BF16)

        xs[:4] = [gate(x, ILAG if from_input else GLAG) for x in xs[:4]]
        inv = yield from _d_butterfly_fwd(xs, emit, pin, from_input)
        inv = jnp.broadcast_to(inv, (16, 128))
        pin(inv)
        put(uout.at[b % RING, 8, r16(lb), :], inv)

    def d_dots(b, base, per_tick):
        for r in range(8):
            o = _dot(lhs(ubuf32[b % RING, r]), bf(small32[base + r]))
            put(uout.at[b % RING, r], o)
            if r % per_tick == per_tick - 1 and r < 7:
                yield

    def d_dots_wide(b):
        for ct, (ra, rb) in enumerate(PAIRS):
            u = lhs(ubuf32[b % RING, ra], ubuf32[b % RING, rb])
            for i, r in enumerate((ra, rb)):
                o = _dot(u, bf(wide32[2 * ct + i]))
                put(uout.at[b % RING, r], ticking(o) if i else o)
            if ct < 3:
                yield

    def d_fwd_cols(b, ct, is_wide):
        c, t = divmod(b, 8)
        ra, rb = PAIRS[ct]
        lane = _lane(16)
        lo = lane < 64
        z, x0 = [], []
        for lb in range(4):
            a, bb, inv = (uout[b % RING, r, r16(lb), :] for r in (ra, rb, 8))
            inv = gate(inv, ILAG if is_wide else GLAG)
            a, bb = a * inv, bb * inv
            if is_wide:
                if ct == 0:
                    x0.append(pltpu.roll(bb, t, 1) if t else bb)
                    bb = jnp.where(lane == 0, 0.0, bb)
                z.append((a, bb))
                continue
            if ct == 0:
                x0.append(pltpu.roll(a, (t + 64) % 128, 1))
                a = jnp.where(lane == 64, 0.0, a)
            im = lax.select(lo, bb, a)
            z.append((lax.select(lo, a, bb), _swap(im)))
        if not is_wide:
            yield from _latency()
        for e, (re, im) in enumerate(_dft4(z, False)):
            words = pack(re, im)
            pin(words)
            put(zin.at[ct, t * 4 + e, r16(c), :], words)
        if is_wide and ct == 0:
            yield from _latency()
        for lb, v in enumerate(x0):
            ls = pl.ds(64 * lb + 16 * c, 16)
            prev = jnp.zeros((16, 128), F32) if t == 0 else side[0, ls, :]
            v = jnp.where(lane == t, v, prev)
            pin(v)
            put(side.at[0, ls, :], v)

    def add_d_fwd(sched, tick, b, gap, per_tick=4, from_input=False):
        for lb in range(4):
            sched.add(tick + lb * gap, d_fwd_rows(b, lb, from_input))
        tick = int(tick + 3 * gap) + XGAP + 1
        sched.add(tick, d_dots_wide(b) if from_input else d_dots(b, 0, per_tick))
        for ct in range(4):
            sched.add(tick + 8 // per_tick + 3 + ct * gap, d_fwd_cols(b, ct, from_input))
        return int(tick + 8 // per_tick + 3 + 3 * gap) + XGAP + 1

    def side_path():
        vt = side[0].T[0:8]
        yield
        zero8 = jnp.zeros((8, 256), F32)
        u = _dot(jnp.concatenate([vt, zero8], axis=0).astype(BF16), f256[...])[0:8]
        twr, twi = tw_ref[0:8, :], tw_ref[8:16, :]
        ur, ui = u[:, 0:256], u[:, 256:512]
        pad = jnp.zeros((112, 256), BF16)
        for _ in range(4):
            yield
        uu = jnp.concatenate([ur * twr - ui * twi, ur * twi + ui * twr], axis=0).astype(BF16)
        xk = _dot(d8_ref[0], jnp.concatenate([uu, pad], axis=0))
        for _ in range(4):
            yield
        wr = jnp.concatenate([side[1, 0:8, :], side[1, 16:24, :]], axis=1)
        wi = jnp.concatenate([side[1, 8:16, :], side[1, 24:32, :]], axis=1)
        xr, xi = xk[0:8], xk[8:16]
        yy = jnp.concatenate([xr * wr - xi * wi, xr * wi + xi * wr], axis=0).astype(BF16)
        p = _dot(d8_ref[1], jnp.concatenate([yy, pad], axis=0))
        for _ in range(4):
            yield
        twr, twi = tw_ref[0:8, :], tw_ref[8:16, :]
        pr, pi = p[0:8], p[8:16]
        g = jnp.concatenate([pr * twr + pi * twi, pi * twr - pr * twi], axis=1)
        g = jnp.concatenate([g, jnp.zeros((8, 512), F32)], axis=0).astype(BF16)
        y0 = _dot_nt(g, f256[...])
        for _ in range(4):
            yield
        put(side.at[2], jnp.concatenate([y0, jnp.zeros((112, 256), F32)], axis=0).T)

    def s_fwd(u, t):
        ct, e = divmod(u, 4)
        put(ybuf.at[u % NY, t], ticking(_dot(lhs(sfw32[t * 4 + e]), bf(zin[ct, t * 4 + e]))))

    def s_filter(u, g):
        ct, e = divmod(u, 4)
        z = [tuple(ybuf[u % NY, t, pl.ds(g * 16 + i, 8), :] for i in (0, 8))
             for t in range(8)]
        lag = SGLAG if u * 8 + g < 122 - S_LAG else SGLAG2
        z[0], z[1] = [tuple(gate(v, lag) for v in zz) for zz in z[0:2]]
        xk = _dft8(z, False)
        for k2 in range(8):
            wr = wf[0, ct, e, k2, pl.ds(g * 8, 8), :]
            wi = wf[1, ct, e, k2, pl.ds(g * 8, 8), :]
            re, im = xk[k2]
            xk[k2] = (re * wr - im * wi, re * wi + im * wr)
        for t, (re, im) in enumerate(_dft8(xk, True)):
            words = pack(re, im)
            pin(words)
            put(fbuf.at[u % NY, t, pl.ds(g * 8, 8), :], words)

    def s_inv(u, t):
        ct, e = divmod(u, 4)
        o = _dot(lhs(siv32[t * 4 + e]), bf(fbuf[u % NY, t]))
        put(zout.at[ct, t * 4 + e], ticking(o) if u * 8 + t >= 110 - S_LAG else o)

    def add_s_stage(sched, early, ready, t1):
        ahead = 8 + S_LAG
        tick = early
        for t in sorted(range(8), key=lambda t: ready[t]):
            for i in range(t, ahead, 8):
                tick = max(tick + 0.5, ready[t])
                sched.add(tick, _once(s_fwd, i // 8, t))
        t1 = max(t1, int(tick) + 1)
        sched.add(max(max(ready), t1), side_path())
        for i in range(128):
            if i + ahead < 128:
                sched.add(t1 + i, _once(s_fwd, *divmod(i + ahead, 8)))
            sched.add(t1 + i, _once(s_filter, *divmod(i, 8)))
            sched.add(t1 + 9 + (i if i < 120 else 120 + (i - 120) // 4), _once(s_inv, *divmod(i, 8)))
        return [t1 + 32 * ct + 40 for ct in range(3)] + [t1 + 131]

    def d_inv_cols(b, ct):
        c, t = divmod(b, 8)
        ra, rb = PAIRS[ct]
        lane = _lane(16)
        lo = lane < 64
        u = [(zout[ct, t * 4 + e, r16(c), :], zout[ct, t * 4 + e, r16(4 + c), :]) for e in range(4)]
        u[0], u[1] = tuple(map(gate, u[0])), tuple(map(gate, u[1]))
        z = _dft4(u, True)
        z = [(re, _swap(im)) for re, im in z]
        if ct == 0:
            y0 = [pltpu.roll(side[2, pl.ds(64 * lb + 16 * c, 16), :], 64 - t, 1) for lb in range(4)]
        yield from _latency()
        for lb, (re, sw) in enumerate(z):
            sw = gate(sw)
            a, bb = lax.select(lo, re, sw), lax.select(lo, sw, re)
            if ct == 0:
                a = jnp.where(lane == 64, y0[lb], a)
            pin(a, bb)
            ubuf[b % RING, ra, r16(lb), :] = a.astype(BF16)
            ubuf[b % RING, rb, r16(lb), :] = bb.astype(BF16)

    def d_inv_rows(b, lb, stats, first):
        u = [uout[b % RING, r, r16(lb), :] for r in range(8)]
        ys = yield from _d_butterfly_inv([gate(v) if r < 4 else v for r, v in enumerate(u)], pin, gate)
        xs = [x + y for x, y in zip(load_x(b, lb, first), ys)]
        for j in range(NT):
            put(xres.at[b, j, r16(lb), :], xs[j])
        stats[b, lb] = yield from ln_stats(xs)
        if b % 2:
            for j in range(4):
                a = [(xres[bb, j + o, r16(lb), :] - stats[bb, lb][0]) * stats[bb, lb][1]
                     for bb in (b - 1, b) for o in (0, 4)]
                a[0], a[3] = gate(a[0]), gate(a[3])
                for k, v in enumerate(_strassen_lhs(*a)):
                    if k not in (2, 3):
                        pin(v)
                    abuf[b // 2, k, j, r16(lb), :] = v.astype(BF16)
                if j < 3:
                    yield

    def add_d_inv(sched, tick, b, gap, stats, first, cols=None):
        per_tick = 4
        cols = cols or [tick + ct * gap for ct in range(4)]
        for ct in range(4):
            sched.add(cols[ct], d_inv_cols(b, ct))
        tick = int(cols[3]) + XGAP + 1
        sched.add(tick, d_dots(b, 8, per_tick))
        tick += 8 // per_tick + 3
        for lb in range(4):
            sched.add(tick + lb * gap, d_inv_rows(b, lb, stats, first))
        return int(tick + 3 * gap) + 3 * XGAP + 1 + 4

    def gemm(lhs32, rhs32, jobs, sink):
        for slot, b, n in jobs:
            m = {}
            for k in (3, 1, 0, 6, 5, 4, 2):
                m[k] = ticking(_dot(lhs(*[lhs32[slot, k, j] for j in range(4)]), bf(rhs32[n // 2, k])))
                if k == 1:
                    sink(b + 1, n, m[1] - m[3])
                elif k == 0:
                    c11, c22 = m[3] - m[0], m[1] - m[0]
                elif k == 6:
                    c11 = m[6] - c11
                elif k == 5:
                    c22 = m[5] - c22
                elif k == 4:
                    sink(b, n, c11 - m[4])
                elif k == 2:
                    sink(b, n + 1, m[4] - m[2])
                    sink(b + 1, n + 1, c22 - m[2])
                yield

    def qkv_sink(b, n, o):
        c, t = divmod(b, 8)
        dst = (qbuf, kbuf, vbuf)[n // NT]
        for lb in range(4):
            put(dst.at[n % NT, t, pl.ds(8 + 64 * lb + 16 * c, 16), :], o[lb * 16:(lb + 1) * 16])
        if b == 0 and n >= NT:
            first = jnp.broadcast_to(o[0:1], (8, 128))
            for tt in range(8):
                dst[n % NT, tt, pl.ds(0, 8), :] = first

    def out_rows(r, i, last):
        c, t = divmod(r, 8)
        return (c * 8 + t % 2 * 4 + i, t // 2) if last and c == 0 else (r, i)

    def out_sink(last, r, n, o):
        for i in range(4):
            b, lb = out_rows(r, i, last)
            put(xres.at[b, n, r16(lb), :], xres[b, n, r16(lb), :] + o[i * 16:(i + 1) * 16])

    def attention(b, lb, h):
        c, t = divmod(b, 8)
        scale = HEAD_DIM ** -0.5
        r0 = 8 + 64 * lb + 16 * c + 8 * h
        src = [((t - 2 * w) % 8, -((t - 2 * w) // 8)) for w in range(WIN)]
        acc = [None] * WIN
        for j in range(NT):
            q = gate(qbuf[j, t, pl.ds(r0, 8), :], ALAG)
            for w, (ts, sh) in enumerate(src):
                p = q * kbuf[j, ts, pl.ds(r0 - sh, 8), :]
                acc[w] = p if j == 0 else acc[w] + p
            if j % 2 and j < NT - 1:
                pin(*acc)
                yield
        part = [(r, pltpu.roll(r, 64, 1)) for r in acc]
        yield from _latency()
        part = [r + rr for r, rr in part]
        part = [(r, pltpu.roll(r, 32, 1)) for r in part]
        yield from _latency()
        logits = [r + rr for r, rr in part]
        if r0 == 8:
            sub = lax.broadcasted_iota(jnp.int32, (8, 128), 0)
            logits = [jnp.where(sub >= sh, r, -1e9 / scale) if sh else r
                      for r, (_, sh) in zip(logits, src)]
        logits[0] = gate(logits[0], ALAG)
        m = _tree(jnp.maximum, logits)
        ps = [jnp.exp2((r - m) * (scale * float(np.log2(np.e)))) for r in logits]
        total = _tree(_add, ps)
        pin(total)
        inv = pltpu.reciprocal(total, approx=True)
        inv = inv * (2.0 - total * inv)
        for j in range(NT):
            if j % 2 == 0:
                yield
                ps[0], ps[4] = gate(ps[0], ALAG), gate(ps[4], ALAG)
            o = _chain(_add, [ps[w] * vbuf[j, ts, pl.ds(r0 - sh, 8), :]
                              for w, (ts, sh) in enumerate(src)]) * inv
            pin(o)
            put(qbuf.at[j, t, pl.ds(r0, 8), :], o)

    def out_operands(r, i, last):
        for j in range(4):
            a = [qbuf[j + o, b % 8, pl.ds(8 + 64 * lb + 16 * (b // 8), 16), :]
                 for b, lb in (out_rows(r, i, last), out_rows(r + 1, i, last)) for o in (0, 4)]
            a[0], a[3] = gate(a[0]), gate(a[3])
            for k, v in enumerate(_strassen_lhs(*a)):
                if k not in (2, 3):
                    pin(v)
                obuf[r // 2, k, j, r16(i), :] = v.astype(BF16)
            if j < 3:
                yield

    def store_rows(b, lb):
        c, t = divmod(b, 8)
        for j in range(NT):
            words = pack(xres[b, j, r16(lb), :], xres[b + 1, j, r16(lb), :])
            pin(words)
            io32[j, lb, c, pl.ds(t // 2, 16, stride=4), :] = words

    unit_ticks = NT + 2 * XGAP
    step = 2
    out_ticks = 28

    def add_proj(sched, tick, c, lo, hi):
        jobs = [(b // step, b, n) for b in range(8 * c, 8 * c + 8, step) for n in range(lo, hi, step)]
        sched.add(tick, gemm(abuf32, wqkv32, jobs, qkv_sink))
        return tick + len(jobs) * out_ticks * step // NT

    def add_attention(sched, tick, pace, rows, last):
        units = [(r, i, half, h) for r in rows[::2] for i in range(4) for half in range(2) for h in range(2)]
        for n, (r, i, half, h) in enumerate(units):
            sched.add(tick + n * pace, attention(*out_rows(r + half, i, last), h))
            if half and h:
                sched.add(int(tick + n * pace) + unit_ticks, out_operands(r, i, last))

    def add_out(sched, tick, rows, last):
        jobs = [(r // 2, r, n) for r in rows[::2] for n in range(0, NT, 2)]
        sched.add(tick, gemm(obuf32, wo32, jobs, functools.partial(out_sink, last)))

    def add_tail(sched, tick, rows, last):
        ready = {}
        for i, r in enumerate(rows):
            t0 = tick + (i // 2 + 1) * out_ticks
            fast = i >= len(rows) - (2 if last else 4)
            if not last:
                t0 += 0 if fast else TOFF + i % 2 * out_ticks // 2
                ready[r % 8] = add_d_fwd(sched, t0, r, i % 2 if fast else out_ticks / 8)
            elif r % 2:
                c, p = r // 8, r % 8 // 2
                gap = 0 if fast else 3
                for j in range(4):
                    sched.add(t0 + (j + 1) * gap, _once(store_rows, *((r - 1, j) if c else (2 * j, p))))
                for lb in ([p] if c == 0 else range(4) if p == 3 else []):
                    sched.add(t0 + 5 * gap + 1, _once(start, out_copies(c, lb)))
        return ready

    q_ticks = 8 * out_ticks // step
    att_ticks = unit_ticks + 1 + 2
    order = [(a + 8) % NB for a in range(NB)]

    def add_attention_block(sched, cols, last):
        stats = {}
        t0 = max([add_d_inv(sched, 0, b, 0, stats, not last, cols) for b in range(step)])
        if not last:
            sched.add(cols[3] - KLEAD, _once(wait, qkv_copies(1) + dmat_cp))
            done = add_prep_wqkv(sched, cols[3] - KLEAD, 1, KPACE, [7] * 4)
            t0 = max(t0, done[0])
            assert all(d <= t0 + p * out_ticks / 4 for p, d in enumerate(done))
            sched.add(t0 + out_ticks, _once(wait, qkv_copies(2)))
            sched.add(t0 + out_ticks, _once(start, qkv_copies(0)))
            done = add_prep_wqkv(sched, t0 + out_ticks, 2, 2 * out_ticks - 6, [out_ticks - 4] * 4)
            assert all(d <= t0 + q_ticks + p * out_ticks for p, d in enumerate(done))
            sched.add(t0 + 2 * q_ticks, _once(wait, qkv_copies(0)))
            sched.add(t0 + 2 * q_ticks, _once(start, wo_copies))
            done = add_prep_wqkv(sched, t0 + 2 * q_ticks, 0, q_ticks - 10, [q_ticks / 4] * 4)
            assert done[-1] <= t0 + 4 * q_ticks
            sched.add(t0 + 8 * q_ticks, _once(wait, wo_copies))
            for i in range(32):
                sched.add(t0 + 8 * q_ticks + i * q_ticks / 16, _once(prep_wo, *divmod(i, 8)))
        tick, kv_start, q_start = t0, {}, {}
        for kind, c in ("k0", "k1", "q1", "k2", "q2", "k3", "q3", "q0"):
            if kind == "k":
                kv_start[int(c)] = tick
                if c == "0" and not last:
                    tick = add_proj(sched, tick, 0, NT, 2 * NT)
                    jobs = [(b // step, b, n) for n in range(2 * NT, 3 * NT, step) for b in range(0, 8, step)]
                    sched.add(tick, gemm(abuf32, wqkv32, jobs, qkv_sink))
                    tick += q_ticks
                    continue
                tick = add_proj(sched, tick, int(c), NT, 3 * NT)
            else:
                q_start[int(c)] = tick
                tick = add_proj(sched, tick, int(c), 0, NT)
        pace = 2 * out_ticks / step
        for b in range(step, NB):
            due = kv_start[b // 8] + (b % 8 // step) * (2 if last or b >= 8 else 1) * out_ticks
            gap = min(1 + (b - step) * 0.5, DGAP1 if last else DGAP0)
            pace = DPACE1 if last else DPACE0
            at = (b - step) * pace
            at = t0 + at + max(0, at - 4 * q_ticks - out_ticks) * DSLOW
            if not last and b < 8:
                at, gap = max(cols[3], t0 + (b // step - 1) * out_ticks - (step - b % step) * 8), 1
            end = add_d_inv(sched, at, b, gap, stats, not last)
            assert end <= due, (b, end, due)
        begin = [q_start[c] + out_ticks + 3 for c in (1, 2, 3)] + [tick + (ATT1 if last else ATT0)]
        begin.append(tick + (NB // step - 1) * out_ticks - att_ticks)
        for i, c in enumerate((1, 2, 3, 0)):
            pace = (begin[i + 1] - begin[i]) / 64
            assert begin[i] >= max(kv_start[c], kv_start[(c - 1) % 4]) + 2 * q_ticks
            for p in range(4):
                assert begin[i] + 16 * p * pace >= q_start[c] + (4 if last and c == 0 else p + 1) * out_ticks
                assert begin[i] + (16 * p + 15) * pace + att_ticks <= tick + (4 * i + p) * out_ticks + 1e-6
            add_attention(sched, begin[i], pace, range(8 * c, 8 * c + 8), last)
        add_out(sched, tick, order, last)
        return tick + (NB // step) * out_ticks, add_tail(sched, tick, order, last)

    def add_input(sched):
        ready = {}
        after = (x_copies(2), x_copies(3) + perm_cp + w_copies(0) + w_copies(1),
                 w_copies(2) + w_copies(3), w_copies(4))
        for c in range(NC):
            sched.add(c * 32, _once(wait, x_copies(c)))
            sched.add(c * 32, _once(start, after[c]))
            for t in range(8):
                ready[t] = add_d_fwd(sched, c * 32 + t * 4, c * 8 + t, 1, 2, True)
        return 128 + 9, ready

    def add_filter_prep(sched, tick):
        after = (w_copies(5) + w_copies(6), w_copies(7) + f256_cp + dmat_cp, qkv_copies(1), qkv_copies(2))
        begin = [F0 + g * (tick - F0) / 4 for g in range(4)] + [tick + FG * g for g in range(5)]
        for g in range(8):
            if g % 2 == 0:
                sched.add(begin[g], _once(wait, w_copies(g) + w_copies(g + 1) + ([] if g else perm_cp)))
                sched.add(begin[g], _once(start, after[g // 2]))
            for m in range(4):
                sched.add(begin[g] + m * (begin[g + 1] - begin[g]) / 4,
                          _once(prep_filter, g // 4, g % 4 * 4 + m))
        sched.add(begin[8] + 1, _once(wait, f256_cp))
        return begin[8] + 2

    sched = _Schedule()

    start(x_copies(0))
    for ref in (abuf32, obuf32, ubuf32, wo32, sfw32, siv32, wide32):
        put(ref.at[(0,) * (len(ref.shape) - 2) + (pl.ds(0, 8),)], jnp.zeros((8, 128), U32))
    make_wide()
    start(x_copies(1))
    for t in range(8):
        make_s_fwd(t)
    for e in range(4):
        make_s_inv(e)
    tick, ready = add_input(sched)
    cols = add_s_stage(sched, tick, ready, add_filter_prep(sched, tick))
    tick, ready = add_attention_block(sched, cols, False)
    cols = add_s_stage(sched, tick, ready, tick)
    add_attention_block(sched, cols, True)
    sched.run()
    for c in range(NC):
        for lb in range(4):
            wait(out_copies(c, lb))


@jax.jit
def pallas_interleave_layers__spectral_gfnet__sliding_local_dilated__prompt_kernel(
    A_x: jax.Array,
    A_w_r: jax.Array,
    A_w_i: jax.Array,
    B_x: jax.Array,
    B_wqkv: jax.Array,
    B_wo: jax.Array,
):
    del B_x
    assert A_x.shape == (1, S, D) and A_w_r.shape == (S, D // 2 + 1)
    cst = _constants()
    x = A_x.astype(BF16).reshape(4, NC, 128, D)
    wr, wi = A_w_r.astype(BF16).T, A_w_i.astype(BF16).T
    hbm = pl.BlockSpec(memory_space=pl.ANY)
    edge = pl.BlockSpec((16, S), lambda i: (D // 32, 0))
    vm = pltpu.VMEM
    out = pl.pallas_call(
        _kernel,
        grid=(1,),
        in_specs=[hbm, hbm, hbm, edge, edge, hbm, hbm, hbm, hbm,
                  pl.BlockSpec((24, 256), lambda i: (0, 0)),
                  pl.BlockSpec((2, 16, 128), lambda i: (0, 0, 0))],
        out_specs=hbm,
        out_shape=jax.ShapeDtypeStruct((4, NC, 128, D), BF16),
        scratch_shapes=[
            vm((NT, 4, NC, 128, 128), BF16),
            vm((17, 128, 128), BF16),
            vm((32, 128, 128), BF16),
            vm((32, 128, 128), BF16),
            vm((256, 512), BF16),
            vm((2, 16, 512, 128), BF16),
            vm((2, 4, 4, 8, 64, 128), F32),
            vm((3 * NT, D, 128), BF16),
            vm((NT, D // 2, 128), U32),
            vm((12, 7, 512, 128), BF16),
            vm((NT, D, 128), BF16),
            vm((4, 7, 512, 128), BF16),
            vm((NB, NT, 64, 128), F32),
            vm((4, 32, 64, 128), U32),
            vm((4, 32, 128, 128), F32),
            vm((NY, 8, 128, 128), F32),
            vm((NY, 8, 64, 128), U32),
            vm((RING, 8, 64, 128), BF16),
            vm((RING, 9, 64, 128), F32),
            vm((NB // 2, 7, 4, 64, 128), BF16),
            vm((NB // 2, 7, 4, 64, 128), BF16),
            vm((NT, 8, 264, 128), F32),
            vm((NT, 8, 264, 128), F32),
            vm((NT, 8, 264, 128), F32),
            vm((3, 256, 128), F32),
            vm((8, 256, 128), BF16),
            pltpu.SemaphoreType.DMA((NC,)),
            pltpu.SemaphoreType.DMA((3,)),
            pltpu.SemaphoreType.DMA((8,)),
            pltpu.SemaphoreType.DMA((3,)),
            pltpu.SemaphoreType.DMA(()),
            pltpu.SemaphoreType.DMA(()),
        ],
        compiler_params=pltpu.CompilerParams(
            dimension_semantics=("arbitrary",), vmem_limit_bytes=120 * 2**20),
    )(x, wr, wi, wr, wi, B_wqkv.astype(BF16), B_wo.astype(BF16),
      cst["small"], cst["f256"], cst["tw"], cst["d8"])
    return out.reshape(1, S, D)
```

```python
import functools

import jax
import jax.numpy as jnp
import numpy as np
from jax import lax
from jax.experimental import pallas as pl
from jax.experimental.pallas import tpu as pltpu

S, D = 2048, 1024
NT = D // 128
NC = 4
WIN = 8
HEAD_DIM = 32
EPS = 1e-5
F32, BF16, U32 = jnp.float32, jnp.bfloat16, jnp.uint32
PAIRS = ((0, 4), (1, 7), (2, 6), (3, 5))
RSQ2 = float(np.sqrt(0.5))
NB = S // 64

RING = 8
NY = 4
XGAP = 3
GLAG = 4
ALAG = 4
SGLAG = 3
SGLAG2 = 5
S_LAG = 3
F0 = 112
KLEAD = 52
KPACE = 48
DGAP0 = 4.75
DGAP1 = 4.2
DPACE0 = 21
DPACE1 = 15.5
DSLOW = 0.6
SYNC = 3
ILAG = 3
FG = 4
TOFF = 3
ATT0 = 10
ATT1 = 95


def _residues(r):
    return (0, 8) if r == 0 else (r, 16 - r)


def _d_matrices():
    n = np.arange(64)[:, None]
    a = np.arange(32)
    fwd = np.zeros((8, 128, 128))
    inv = np.zeros((8, 128, 128))
    for r in range(8):
        kd = np.concatenate([16 * a + p for p in _residues(r)])
        weight = np.full(64, 2.0)
        if r == 0:
            kd[0], weight[0] = D // 2, 1.0
            ph = np.exp(-2j * np.pi * n * kd[None, :] / D)
            sgn = np.where(kd % 16 == 0, 1.0, -1.0)[None, :]
            m = np.concatenate([ph, ph * sgn], axis=0)
            re, im = m.real.copy(), m.imag.copy()
            ire, iim = re.copy(), im.copy()
            im[:, 0] = 1.0
            iim[:, 0] = 1.0
        else:
            p = 12 if r == 4 else r
            ph = np.exp(-2j * np.pi * n * kd[None, :] / D)
            si = np.where(kd % 16 == p, 1.0, -1.0)[None, :]
            m = np.concatenate([ph, 1j * si * ph], axis=0)
            re, im = m.real, m.imag
            ire, iim = re, im
        swapped = r in (4, 7, 6, 5)
        cols = [im, re] if swapped else [re, im]
        icols = [iim * weight, ire * weight] if swapped else [ire * weight, iim * weight]
        fwd[r] = np.concatenate(cols, axis=1)
        inv[r] = np.concatenate(icols, axis=1).T / D
    return fwd, inv


def _side_matrices():
    l = np.arange(256)
    f = np.exp(-2j * np.pi * ((l[:, None] * l[None, :]) % 256) / 256)
    f256 = np.concatenate([f.real, f.imag], axis=1)
    t = np.arange(8)
    tw = np.exp(-2j * np.pi * t[:, None] * l[None, :] / S)
    tw = np.concatenate([tw.real, tw.imag, np.zeros((8, 256))], axis=0)
    g = np.exp(-2j * np.pi * t[:, None] * t[None, :] / 8)
    d8 = np.zeros((2, 16, 128))
    d8[0, :, :16] = np.block([[g.real, -g.imag], [g.imag, g.real]])
    d8[1, :, :16] = d8[0, :, :16].T / S
    return f256, tw, d8


def _filter_rows():
    p = np.zeros((1, 128, 128))
    for k in range(32):
        for e in range(4):
            p[0, e * 32 + k, 4 * k + e] = 1.0
    return p


@functools.lru_cache(maxsize=None)
def _constants():
    dfw, div = _d_matrices()
    f256, tw, d8 = _side_matrices()
    small = np.concatenate([dfw, div, _filter_rows()], axis=0)
    b = lambda x: np.asarray(x, np.float32).astype(BF16)
    return dict(small=b(small), f256=b(f256),
                tw=np.asarray(tw, np.float32), d8=b(d8))


def _dot(a, b):
    return jnp.dot(a, b, preferred_element_type=F32)


def _dot_nt(a, b):
    return lax.dot_general(a, b, (((1,), (1,)), ((), ())), preferred_element_type=F32)


def _tree(op, xs):
    xs = list(xs)
    while len(xs) > 1:
        xs = [op(xs[i], xs[i + 1]) if i + 1 < len(xs) else xs[i] for i in range(0, len(xs), 2)]
    return xs[0]


def _chain(op, xs):
    return functools.reduce(op, xs)


def _lane(rows):
    return lax.broadcasted_iota(jnp.int32, (rows, 128), 1)


def _swap(x):
    return pltpu.roll(x, 64, 1)


def _unpack(w, i):
    return pltpu.unpack_elementwise(w, index=i, packed_dtype=BF16, unpacked_dtype=F32)


def _latency():
    for _ in range(XGAP):
        yield


def _add(a, b):
    return a + b


def _row_mean(xs):
    return jnp.sum(_tree(_add, xs), axis=1, keepdims=True) * (1.0 / D)


def _twiddle16(r, x, y):
    lo = _lane(x.shape[0]) < 64
    wr, wi = float(np.cos(np.pi * r / 8)), float(-np.sin(np.pi * r / 8))
    cross = jnp.where(lo, 0.0, wr)
    return x * jnp.where(lo, 1.0, wi) + y * cross, y * jnp.where(lo, 1.0, -wi) + x * cross


def _d_butterfly_fwd(a, emit, pin, wide):
    s = [a[j] + a[j + 4] for j in range(4)]
    e, o = s[0] + s[2], s[1] + s[3]
    total, t4 = e + o, e - o
    emit(4, t4)
    d0, nd2 = a[0] - a[4], a[6] - a[2]
    d1, d3 = a[1] - a[5], a[3] - a[7]
    p, q = (d1 - d3) * RSQ2, (d1 + d3) * -RSQ2
    ts = {1: (d0 + p, q + nd2), 2: (s[0] - s[2], s[3] - s[1]), 3: (d0 - p, q - nd2)}
    mean8 = jnp.sum(total, axis=1, keepdims=True) * (1.0 / 128)
    if wide:
        for r, (tr, ti) in ts.items():
            emit(r, tr)
            emit(8 - r, ti)
    else:
        ab = {r: _twiddle16(r, *t) for r, t in ts.items()}
        ab = {r: (a, _swap(b)) for r, (a, b) in ab.items()}
    dev = _tree(_add, [v * v for t in ts.values() for v in t]) * 2.0 + t4 * t4
    pin(dev)
    yield from _latency()
    t0 = total - mean8
    emit(0, t0)
    var = jnp.sum(dev + t0 * t0, axis=1, keepdims=True) * (1.0 / (NT * D))
    if not wide:
        for r, (x, y) in ab.items():
            emit(r, x + y)
            emit(8 - r, x - y)
    yield from _latency()
    return lax.rsqrt(var + EPS)


def _d_butterfly_inv(u, pin, gate):
    ab = {r: (u[r] + u[8 - r], _swap(u[r] - u[8 - r])) for r in (1, 2, 3)}
    e, o = u[0] + u[4], u[0] - u[4]
    yield from _latency()
    ts = {r: _twiddle16(r, x, gate(y)) for r, (x, y) in ab.items()}
    pin(*[t[0] for t in ts.values()])
    yield
    s = [e + ts[2][0], o - ts[2][1], e - ts[2][0], o + ts[2][1]]
    p = (ts[1][0] - ts[3][0]) * RSQ2
    q = (ts[1][1] + ts[3][1]) * RSQ2
    d0, d1, d2, nd3 = ts[1][0] + ts[3][0], p - q, ts[3][1] - ts[1][1], p + q
    return [s[0] + d0, s[1] + d1, s[2] + d2, s[3] - nd3,
            s[0] - d0, s[1] - d1, s[2] - d2, s[3] + nd3]


def _strassen_lhs(a11, a12, a21, a22):
    return [a11 + a22, a21 + a22, a11, a22, a11 + a12, a21 - a11, a12 - a22]


def _strassen_rhs(b11, b12, b21, b22):
    return [b11 + b22, b11, b22 - b12, b11 - b21, b22, b11 + b12, b21 + b22]


def _cadd(a, b):
    return a[0] + b[0], a[1] + b[1]


def _csub(a, b):
    return a[0] - b[0], a[1] - b[1]


def _dft4(z, inverse):
    a, b = _cadd(z[0], z[2]), _csub(z[0], z[2])
    c, d = _cadd(z[1], z[3]), _csub(z[1], z[3])
    minus = (b[0] + d[1], b[1] - d[0])
    plus = (b[0] - d[1], b[1] + d[0])
    return [_cadd(a, c), plus if inverse else minus, _csub(a, c), minus if inverse else plus]


def _dft8(z, inverse):
    ev = _dft4(z[0::2], inverse)
    od = _dft4(z[1::2], inverse)
    out = [None] * 8
    out[0], out[4] = _cadd(ev[0], od[0]), _csub(ev[0], od[0])
    (er, ei), (x, y) = ev[2], od[2]
    minus, plus = (er + y, ei - x), (er - y, ei + x)
    out[2], out[6] = (plus, minus) if inverse else (minus, plus)
    for k in (1, 3):
        (er, ei), (x, y) = ev[k], od[k]
        sm, df = (x + y) * RSQ2, (x - y) * RSQ2
        if not inverse:
            if k == 1:
                out[1], out[5] = (er + sm, ei - df), (er - sm, ei + df)
            else:
                out[3], out[7] = (er - df, ei - sm), (er + df, ei + sm)
        else:
            if k == 1:
                out[1], out[5] = (er + df, ei + sm), (er - df, ei - sm)
            else:
                out[3], out[7] = (er - sm, ei + df), (er + sm, ei - df)
    return out


class _Schedule:
    def __init__(self):
        self.pending = []

    def add(self, tick, gen):
        self.pending.append((int(tick), len(self.pending), gen))

    def run(self):
        pending = sorted(self.pending, key=lambda p: p[:2])
        active, tick, i = [], 0, 0
        while active or i < len(pending):
            while i < len(pending) and pending[i][0] <= tick:
                active.append(pending[i][2])
                i += 1
            for g in list(active):
                if next(g, 0) == 0:
                    active.remove(g)
            tick += 1
        self.pending = []


def _once(fn, *args):
    fn(*args)
    return
    yield


def _kernel(x_hbm, wr_hbm, wi_hbm, wr_edge, wi_edge, wqkv_hbm, wo_hbm,
            small_hbm, f256_hbm, tw_ref, d8_ref,
            out_hbm,
            io, small, sfw, siv, f256, wraw, wf, wqkv_raw, wtmp, wqkv, wo_raw, wo,
            xres, zin, zout, ybuf, fbuf, ubuf, uout, abuf, obuf, qbuf, kbuf, vbuf, side,
            wide, sem_x, sem_c, sem_w, sem_qkv, sem_wo, sem_out):

    def x_copies(c):
        return [pltpu.make_async_copy(x_hbm.at[:, c, :, pl.ds(j * 128, 128)], io.at[j, :, c],
                                      sem_x.at[c]) for j in range(NT)]

    def out_copies(c, lb):
        return [pltpu.make_async_copy(io.at[j, lb, c], out_hbm.at[lb, c, :, pl.ds(j * 128, 128)],
                                      sem_out) for j in range(NT)]

    perm_cp, dmat_cp, f256_cp = ([pltpu.make_async_copy(s, d, sem_c.at[i])] for i, (s, d) in enumerate((
        (small_hbm.at[pl.ds(16, 1)], small.at[pl.ds(16, 1)]),
        (small_hbm.at[pl.ds(0, 16)], small.at[pl.ds(0, 16)]), (f256_hbm, f256))))

    def w_copies(g):
        src = (wr_hbm, wi_hbm)[g // 4]
        return [pltpu.make_async_copy(src.at[pl.ds(0, 512), pl.ds(m * 128, 128)], wraw.at[g // 4, m],
                                      sem_w.at[g]) for m in range(g % 4 * 4, g % 4 * 4 + 4)]

    def qkv_copies(g):
        return [pltpu.make_async_copy(wqkv_hbm.at[:, pl.ds(g * D + j * 128, 128)],
                                      wqkv_raw.at[g * NT + j], sem_qkv.at[g]) for j in range(NT)]

    wo_copies = [pltpu.make_async_copy(wo_hbm.at[:, pl.ds(j * 128, 128)], wo_raw.at[j], sem_wo)
                 for j in range(NT)]

    def start(cs):
        for cp in cs:
            cp.start()

    def wait(cs):
        for cp in cs:
            cp.wait()

    io32, wraw32, wo_raw32 = io.bitcast(U32), wraw.bitcast(U32), wo_raw.bitcast(U32)
    small32, sfw32, siv32, wide32 = (r.bitcast(U32) for r in (small, sfw, siv, wide))
    wqkv_raw32, wqkv32, wo32 = (r.bitcast(U32) for r in (wqkv_raw, wqkv, wo))
    ubuf32, abuf32, obuf32 = ubuf.bitcast(U32), abuf.bitcast(U32), obuf.bitcast(U32)

    never = tw_ref[16:24, 0:128] != 0.0
    never_wide = {n: jnp.concatenate([tw_ref[16:24, 0:128]] * n, axis=1) != 0.0 for n in (1, 2, 4)}
    token = {}

    def pin(*values):
        for v in values:
            key = v.shape[0], v.dtype == F32
            token[key] = (lax.max if key[1] else lax.bitwise_xor)(token[key], v) if key in token else v

    clock = []

    def gate(v, lag=GLAG):
        if len(clock) < lag:
            return v
        old = clock[-lag] if v.dtype == F32 else pltpu.bitcast(clock[-lag], v.dtype)
        if v.shape[0] == 8:
            return lax.select(never, old, v)
        return lax.concatenate([lax.select(never, old, v[0:8]), v[8:]], 0)

    def ticking(o):
        clock.append(o[0:8])
        del clock[:-16]
        return o

    def lhs(*tiles):
        if not token and len(tiles) == 4 and len(clock) >= SYNC:
            pin(clock[-SYNC])
        words = lax.concatenate(tiles, 1) if len(tiles) > 1 else tiles[0]
        if token:
            parts = [pltpu.bitcast(v, U32) if is_float else v for (_, is_float), v in token.items()]
            token.clear()
            w = _chain(lax.bitwise_xor, [v[i:i + 8] if v.shape[0] > 8 else v
                                         for v in parts for i in range(0, v.shape[0], 8)])
            w = lax.concatenate([w] * len(tiles), 1) if len(tiles) > 1 else w
            words = lax.concatenate([lax.select(never_wide[len(tiles)], w, words[0:8]), words[8:]], 0)
        return pltpu.bitcast(words, BF16)

    def bf(words):
        return pltpu.bitcast(words, BF16)

    def pack(a, b):
        return pltpu.bitcast(pltpu.pack_elementwise([a, b], packed_dtype=BF16), U32)

    def r16(i):
        return pl.ds(i * 16, 16)

    always = {}

    def put(ref, v):
        if v.shape not in always:
            always[v.shape] = jnp.ones(v.shape, jnp.bool_)
        pltpu.store(ref, v, mask=always[v.shape])

    def load_x(b, lb, from_input):
        if from_input:
            c, t = divmod(b, 8)
            return [_unpack(io32[j, lb, c, pl.ds(t // 2, 16, stride=4), :], t % 2) for j in range(NT)]
        return [xres[b, j, r16(lb), :] for j in range(NT)]

    def unit(p):
        angle = (((p + S // 2) & (S - 1)) - S // 2).astype(F32) * (2 * np.pi / S)
        return jnp.cos(angle), jnp.sin(angle)

    def times_row(a, b, i):
        br, bi = (jnp.broadcast_to(v[i:i + 1], (8, 128)) for v in b)
        return a[0] * br - a[1] * bi, a[0] * bi + a[1] * br

    def make_wide():
        row, lane = lax.broadcasted_iota(jnp.int32, (8, 128), 0), _lane(8)
        for ct, (ra, rb) in enumerate(PAIRS):
            res = _residues(ra) + _residues(rb)
            kd = (lane & 31) * 16 + _chain(
                _add, [jnp.where(lane >> 5 == g, p, 0) for g, p in enumerate(res)])
            if ct == 0:
                kd = jnp.where(lane == 0, D // 2, kd)
            fine, coarse = unit(-2 * row * kd), [unit(-16 * (row + 8 * h) * kd) for h in range(2)]
            for a in range(16):
                re, im = times_row(fine, coarse[a // 8], a % 8)
                if ct == 0:
                    even = kd & 7 == 0
                    top = jnp.where(even, re, 0.0), jnp.where(lane == 0, 1.0, jnp.where(even, im, 0.0))
                    bottom = jnp.where(even, 0.0, re), jnp.where(even, 0.0, im)
                else:
                    sign = jnp.where(kd & 7 == ra, 1.0, -1.0)
                    top, bottom = (re, im), (-sign * im, sign * re)
                for i in range(2):
                    wide[2 * ct + i, pl.ds(8 * a, 8), :] = top[i].astype(BF16)
                    wide[2 * ct + i, pl.ds(128 + 8 * a, 8), :] = bottom[i].astype(BF16)

    def make_s_fwd(t):
        row, lane = lax.broadcasted_iota(jnp.int32, (8, 128), 0), _lane(8)
        pos = 8 * (lane >> 1) + t
        fine = unit((lane & 1) * (S // 4) - 4 * row * pos)
        shift, coarse = unit(-row * pos), unit(-32 * row * pos)
        for e in range(4):
            base = times_row(fine, shift, e)
            for g in range(8):
                for i, v in enumerate(times_row(base, coarse, g)):
                    sfw[t * 4 + e, pl.ds(16 * g + 8 * i, 8), :] = v.astype(BF16)

    def make_s_inv(e):
        row, lane = lax.broadcasted_iota(jnp.int32, (8, 128), 0), _lane(8)
        freq = 4 * (lane >> 1) + e
        fine = [v * (1.0 / S) for v in unit((lane & 1) * (S // 4) + 8 * row * freq)]
        shift, coarse = unit(row * freq), unit(64 * row * freq)
        for t in range(8):
            base = times_row(fine, shift, t)
            for g in range(8):
                for i, v in enumerate(times_row(base, coarse, g)):
                    siv[t * 4 + e, pl.ds(64 * i + 8 * g, 8), :] = v.astype(BF16)

    def prep_filter(ri, m):
        sub = lax.broadcasted_iota(jnp.int32, (8, 128), 0)
        edge = (wr_edge, wi_edge)[ri]
        res = {}
        for i in range(8):
            words = wraw32[ri, m, pl.ds(i, 32, stride=8), :]
            res[2 * i], res[2 * i + 1] = _unpack(words, 0), _unpack(words, 1)
        first = res[0][0:8]
        dst = pl.ds((m % 2) * 16 + ri * 8, 8)
        prev = jnp.zeros((8, 128), F32) if m < 2 else side[1, dst, :]
        put(side.at[1, dst, :], jnp.where(sub == m // 2, jnp.broadcast_to(first[0:1], (8, 128)), prev))
        nyq = jnp.broadcast_to(edge[0:1, pl.ds(m * 128, 128)].astype(F32), (8, 128))
        res[0] = jnp.concatenate([jnp.where(sub == 0, nyq, first), res[0][8:]], axis=0)
        for ct, (ra, rb) in enumerate(PAIRS):
            blk = jnp.concatenate([res[p] for p in _residues(ra) + _residues(rb)], axis=0)
            o = _dot_nt(lhs(small32[16]), blk.astype(BF16))
            for e in range(4):
                put(wf.at[ri, ct, e, m // 2, pl.ds((m % 2) * 32, 32), :], o[e * 32:(e + 1) * 32])

    def shuffle(words, index):
        return jnp.take_along_axis(words, index, axis=1)

    def prep_wqkv_tile(g, i, part):
        lane = _lane(8)
        index = (lane & 3) * 32 + (((lane >> 2) - i) & 7) * 4 + (lane >> 5)
        rows = [pl.ds((part * 16 + r) * 8, 8) for r in range(16)]
        ws = [shuffle(gate(wqkv_raw32[g * NT + i, rs, :]), index) for rs in rows]
        yield from _latency()
        for rs, w in zip(rows, ws):
            pin(w)
            put(wtmp.at[i, rs, :], w)

    def prep_wqkv_cross(g, r):
        pos = (_lane(8) >> 2) & 7
        u = [wtmp[(-j) % 8, pl.ds(r * 8, 8), :] for j in range(NT)]
        u[0], u[4] = gate(u[0]), gate(u[4])
        for bit in range(3):
            m = ((pos >> bit) & 1) == 1
            u = [lax.select(m, u[(j - (1 << bit)) % 8], u[j]) for j in range(NT)]
        for j in range(NT):
            pin(u[j])
            put(wqkv_raw32.at[g * NT + j, pl.ds(r * 8, 8), :], u[j])

    def prep_wqkv_pair(g, p, part):
        lane = _lane(8)
        ws = {}
        for n in range(2):
            index = (lane & 96) | ((lane + 4 * (2 * p + n)) & 31)
            for half in range(2):
                for r in range(part * 2, part * 2 + 2):
                    w = gate(wqkv_raw32[g * NT + 2 * p + n, pl.ds(half * 256 + r * 8, 8), :])
                    ws[r, half, n] = shuffle(w, index) if p + n else w
        yield from _latency()
        for r in range(part * 2, part * 2 + 2):
            quad = [ws[r, half, n] for half in range(2) for n in range(2)]
            ops = [_strassen_rhs(*[_unpack(w, i) for w in quad]) for i in range(2)]
            for k in range(7):
                word = {1: quad[0], 4: quad[3]}.get(k)
                if word is None:
                    word = pack(ops[0][k], ops[1][k])
                    pin(word)
                put(wqkv32.at[g * 4 + p, k, pl.ds(r * 8, 8), :], word)

    def add_prep_wqkv(sched, tick, g, ticks, pair_ticks):
        for i in range(32):
            sched.add(tick + i * ticks / 64, prep_wqkv_tile(g, *divmod(i, 4)))
        tick = int(tick + ticks / 2) + XGAP + 1
        for r in range(64):
            sched.add(tick + r * ticks / 128, _once(prep_wqkv_cross, g, r))
        tick = int(tick + ticks / 2) + 1
        done = []
        for p, n in enumerate(pair_ticks):
            for i in range(16):
                sched.add(tick + i * n / 16, prep_wqkv_pair(g, p, i))
            tick += n
            done.append(int(tick) + XGAP + 1)
        return done

    def prep_wo(p, dp):
        ws = [wo_raw32[2 * p + n, pl.ds(dp + off, 32, stride=16), :] for off in (0, 8) for n in (0, 1)]
        for i in range(2):
            b = [_unpack(w, i) for w in ws]
            r0 = (2 * dp + i) * 32
            for k, v in enumerate(_strassen_rhs(*b)):
                if k not in (1, 4):
                    pin(v)
                wo[p, k, pl.ds(r0, 32), :] = v.astype(BF16)

    def ln_stats(xs):
        lane_mean = _tree(_add, xs) * (1.0 / NT)
        lane_m2 = _tree(_add, [jnp.square(x - lane_mean) for x in xs])
        pin(lane_m2)
        mean = jnp.sum(lane_mean, axis=1, keepdims=True) * (1.0 / 128)
        yield from _latency()
        m2 = lane_m2 + jnp.square(gate(lane_mean) - mean) * float(NT)
        pin(m2)
        var = jnp.sum(m2, axis=1, keepdims=True) * (1.0 / D)
        yield from _latency()
        return mean, lax.rsqrt(gate(jnp.broadcast_to(var, (16, 128))) + EPS)

    def d_fwd_rows(b, lb, from_input=False):
        xs = load_x(b, lb, from_input)

        def emit(r, v):
            if r % 4 == 0 or (r < 4 and not from_input):
                pin(v)
            ubuf[b % RING, r, r16(lb), :] = v.astype(BF16)

        xs[:4] = [gate(x, ILAG if from_input else GLAG) for x in xs[:4]]
        inv = yield from _d_butterfly_fwd(xs, emit, pin, from_input)
        inv = jnp.broadcast_to(inv, (16, 128))
        pin(inv)
        put(uout.at[b % RING, 8, r16(lb), :], inv)

    def d_dots(b, base, per_tick):
        for r in range(8):
            o = _dot(lhs(ubuf32[b % RING, r]), bf(small32[base + r]))
            put(uout.at[b % RING, r], o)
            if r % per_tick == per_tick - 1 and r < 7:
                yield

    def d_dots_wide(b):
        for ct, (ra, rb) in enumerate(PAIRS):
            u = lhs(ubuf32[b % RING, ra], ubuf32[b % RING, rb])
            for i, r in enumerate((ra, rb)):
                o = _dot(u, bf(wide32[2 * ct + i]))
                put(uout.at[b % RING, r], ticking(o) if i else o)
            if ct < 3:
                yield

    def d_fwd_cols(b, ct, is_wide):
        c, t = divmod(b, 8)
        ra, rb = PAIRS[ct]
        lane = _lane(16)
        lo = lane < 64
        z, x0 = [], []
        for lb in range(4):
            a, bb, inv = (uout[b % RING, r, r16(lb), :] for r in (ra, rb, 8))
            inv = gate(inv, ILAG if is_wide else GLAG)
            a, bb = a * inv, bb * inv
            if is_wide:
                if ct == 0:
                    x0.append(pltpu.roll(bb, t, 1) if t else bb)
                    bb = jnp.where(lane == 0, 0.0, bb)
                z.append((a, bb))
                continue
            if ct == 0:
                x0.append(pltpu.roll(a, (t + 64) % 128, 1))
                a = jnp.where(lane == 64, 0.0, a)
            im = lax.select(lo, bb, a)
            z.append((lax.select(lo, a, bb), _swap(im)))
        if not is_wide:
            yield from _latency()
        for e, (re, im) in enumerate(_dft4(z, False)):
            words = pack(re, im)
            if e < 2:
                pin(words)
            put(zin.at[ct, t * 4 + e, r16(c), :], words)
        if is_wide and ct == 0:
            yield from _latency()
        for lb, v in enumerate(x0):
            ls = pl.ds(64 * lb + 16 * c, 16)
            prev = jnp.zeros((16, 128), F32) if t == 0 else side[0, ls, :]
            v = jnp.where(lane == t, v, prev)
            pin(v)
            put(side.at[0, ls, :], v)

    def add_d_fwd(sched, tick, b, gap, per_tick=4, from_input=False):
        for lb in range(4):
            sched.add(tick + lb * gap, d_fwd_rows(b, lb, from_input))
        tick = int(tick + 3 * gap) + XGAP + 1
        sched.add(tick, d_dots_wide(b) if from_input else d_dots(b, 0, per_tick))
        for ct in range(4):
            sched.add(tick + 8 // per_tick + 3 + ct * gap, d_fwd_cols(b, ct, from_input))
        return int(tick + 8 // per_tick + 3 + 3 * gap) + XGAP + 1

    def side_path():
        vt = side[0].T[0:8]
        yield
        zero8 = jnp.zeros((8, 256), F32)
        u = _dot(jnp.concatenate([vt, zero8], axis=0).astype(BF16), f256[...])[0:8]
        twr, twi = tw_ref[0:8, :], tw_ref[8:16, :]
        ur, ui = u[:, 0:256], u[:, 256:512]
        pad = jnp.zeros((112, 256), BF16)
        for _ in range(4):
            yield
        uu = jnp.concatenate([ur * twr - ui * twi, ur * twi + ui * twr], axis=0).astype(BF16)
        xk = _dot(d8_ref[0], jnp.concatenate([uu, pad], axis=0))
        for _ in range(4):
            yield
        wr = jnp.concatenate([side[1, 0:8, :], side[1, 16:24, :]], axis=1)
        wi = jnp.concatenate([side[1, 8:16, :], side[1, 24:32, :]], axis=1)
        xr, xi = xk[0:8], xk[8:16]
        yy = jnp.concatenate([xr * wr - xi * wi, xr * wi + xi * wr], axis=0).astype(BF16)
        p = _dot(d8_ref[1], jnp.concatenate([yy, pad], axis=0))
        for _ in range(4):
            yield
        twr, twi = tw_ref[0:8, :], tw_ref[8:16, :]
        pr, pi = p[0:8], p[8:16]
        g = jnp.concatenate([pr * twr + pi * twi, pi * twr - pr * twi], axis=1)
        g = jnp.concatenate([g, jnp.zeros((8, 512), F32)], axis=0).astype(BF16)
        y0 = _dot_nt(g, f256[...])
        for _ in range(4):
            yield
        put(side.at[2], jnp.concatenate([y0, jnp.zeros((112, 256), F32)], axis=0).T)

    def s_fwd(u, t):
        ct, e = divmod(u, 4)
        put(ybuf.at[u % NY, t], ticking(_dot(lhs(sfw32[t * 4 + e]), bf(zin[ct, t * 4 + e]))))

    def s_filter(u, g):
        ct, e = divmod(u, 4)
        z = [tuple(ybuf[u % NY, t, pl.ds(g * 16 + i, 8), :] for i in (0, 8))
             for t in range(8)]
        lag = SGLAG if u * 8 + g < 122 - S_LAG else SGLAG2
        z[0], z[1] = [tuple(gate(v, lag) for v in zz) for zz in z[0:2]]
        xk = _dft8(z, False)
        for k2 in range(8):
            wr = wf[0, ct, e, k2, pl.ds(g * 8, 8), :]
            wi = wf[1, ct, e, k2, pl.ds(g * 8, 8), :]
            re, im = xk[k2]
            xk[k2] = (re * wr - im * wi, re * wi + im * wr)
        for t, (re, im) in enumerate(_dft8(xk, True)):
            words = pack(re, im)
            pin(words)
            put(fbuf.at[u % NY, t, pl.ds(g * 8, 8), :], words)

    def s_inv(u, t):
        ct, e = divmod(u, 4)
        o = _dot(lhs(siv32[t * 4 + e]), bf(fbuf[u % NY, t]))
        put(zout.at[ct, t * 4 + e], ticking(o) if u * 8 + t >= 110 - S_LAG else o)

    def add_s_stage(sched, early, ready, t1):
        ahead = 8 + S_LAG
        tick = early
        for t in sorted(range(8), key=lambda t: ready[t]):
            for i in range(t, ahead, 8):
                tick = max(tick + 0.5, ready[t])
                sched.add(tick, _once(s_fwd, i // 8, t))
        t1 = max(t1, int(tick) + 1)
        sched.add(max(max(ready), t1), side_path())
        for i in range(128):
            if i + ahead < 128:
                sched.add(t1 + i, _once(s_fwd, *divmod(i + ahead, 8)))
            sched.add(t1 + i, _once(s_filter, *divmod(i, 8)))
            sched.add(t1 + 9 + (i if i < 120 else 120 + (i - 120) // 4), _once(s_inv, *divmod(i, 8)))
        return [t1 + 32 * ct + 40 for ct in range(3)] + [t1 + 131]

    def d_inv_cols(b, ct):
        c, t = divmod(b, 8)
        ra, rb = PAIRS[ct]
        lane = _lane(16)
        lo = lane < 64
        u = [(zout[ct, t * 4 + e, r16(c), :], zout[ct, t * 4 + e, r16(4 + c), :]) for e in range(4)]
        u[0], u[1] = tuple(map(gate, u[0])), tuple(map(gate, u[1]))
        z = _dft4(u, True)
        z = [(re, _swap(im)) for re, im in z]
        if ct == 0:
            y0 = [pltpu.roll(side[2, pl.ds(64 * lb + 16 * c, 16), :], 64 - t, 1) for lb in range(4)]
        yield from _latency()
        for lb, (re, sw) in enumerate(z):
            sw = gate(sw)
            a, bb = lax.select(lo, re, sw), lax.select(lo, sw, re)
            if ct == 0:
                a = jnp.where(lane == 64, y0[lb], a)
            pin(a)
            ubuf[b % RING, ra, r16(lb), :] = a.astype(BF16)
            ubuf[b % RING, rb, r16(lb), :] = bb.astype(BF16)

    def d_inv_rows(b, lb, stats, first):
        u = [uout[b % RING, r, r16(lb), :] for r in range(8)]
        ys = yield from _d_butterfly_inv([gate(v) if r < 4 else v for r, v in enumerate(u)], pin, gate)
        xs = [x + y for x, y in zip(load_x(b, lb, first), ys)]
        for j in range(NT):
            put(xres.at[b, j, r16(lb), :], xs[j])
        stats[b, lb] = yield from ln_stats(xs)
        if b % 2:
            for j in range(4):
                a = [(xres[bb, j + o, r16(lb), :] - stats[bb, lb][0]) * stats[bb, lb][1]
                     for bb in (b - 1, b) for o in (0, 4)]
                a[0], a[3] = gate(a[0]), gate(a[3])
                for k, v in enumerate(_strassen_lhs(*a)):
                    if k in (1, 4):
                        pin(v)
                    abuf[b // 2, k, j, r16(lb), :] = v.astype(BF16)
                if j < 3:
                    yield

    def add_d_inv(sched, tick, b, gap, stats, first, cols=None):
        per_tick = 4
        cols = cols or [tick + ct * gap for ct in range(4)]
        for ct in range(4):
            sched.add(cols[ct], d_inv_cols(b, ct))
        tick = int(cols[3]) + XGAP + 1
        sched.add(tick, d_dots(b, 8, per_tick))
        tick += 8 // per_tick + 3
        for lb in range(4):
            sched.add(tick + lb * gap, d_inv_rows(b, lb, stats, first))
        return int(tick + 3 * gap) + 3 * XGAP + 1 + 4

    def gemm(lhs32, rhs32, jobs, sink):
        for slot, b, n in jobs:
            m = {}
            for k in (3, 1, 0, 6, 5, 4, 2):
                m[k] = ticking(_dot(lhs(*[lhs32[slot, k, j] for j in range(4)]), bf(rhs32[n // 2, k])))
                if k == 1:
                    sink(b + 1, n, m[1] - m[3])
                elif k == 0:
                    c11, c22 = m[3] - m[0], m[1] - m[0]
                elif k == 6:
                    c11 = m[6] - c11
                elif k == 5:
                    c22 = m[5] - c22
                elif k == 4:
                    sink(b, n, c11 - m[4])
                elif k == 2:
                    sink(b, n + 1, m[4] - m[2])
                    sink(b + 1, n + 1, c22 - m[2])
                yield

    def qkv_sink(b, n, o):
        c, t = divmod(b, 8)
        dst = (qbuf, kbuf, vbuf)[n // NT]
        for lb in range(4):
            put(dst.at[n % NT, t, pl.ds(8 + 64 * lb + 16 * c, 16), :], o[lb * 16:(lb + 1) * 16])
        if b == 0 and n >= NT:
            first = jnp.broadcast_to(o[0:1], (8, 128))
            for tt in range(8):
                dst[n % NT, tt, pl.ds(0, 8), :] = first

    def out_rows(r, i, last):
        c, t = divmod(r, 8)
        return (c * 8 + t % 2 * 4 + i, t // 2) if last and c == 0 else (r, i)

    def out_sink(last, r, n, o):
        for i in range(4):
            b, lb = out_rows(r, i, last)
            put(xres.at[b, n, r16(lb), :], xres[b, n, r16(lb), :] + o[i * 16:(i + 1) * 16])

    def attention(b, lb, h):
        c, t = divmod(b, 8)
        scale = HEAD_DIM ** -0.5
        r0 = 8 + 64 * lb + 16 * c + 8 * h
        src = [((t - 2 * w) % 8, -((t - 2 * w) // 8)) for w in range(WIN)]
        acc = [None] * WIN
        for j in range(NT):
            q = gate(qbuf[j, t, pl.ds(r0, 8), :], ALAG)
            for w, (ts, sh) in enumerate(src):
                p = q * kbuf[j, ts, pl.ds(r0 - sh, 8), :]
                acc[w] = p if j == 0 else acc[w] + p
            if j % 2 and j < NT - 1:
                pin(*acc)
                yield
        part = [(r, pltpu.roll(r, 64, 1)) for r in acc]
        yield from _latency()
        part = [r + rr for r, rr in part]
        part = [(r, pltpu.roll(r, 32, 1)) for r in part]
        yield from _latency()
        logits = [r + rr for r, rr in part]
        if r0 == 8:
            sub = lax.broadcasted_iota(jnp.int32, (8, 128), 0)
            logits = [jnp.where(sub >= sh, r, -1e9 / scale) if sh else r
                      for r, (_, sh) in zip(logits, src)]
        logits[0] = gate(logits[0], ALAG)
        m = _tree(jnp.maximum, logits)
        ps = [jnp.exp2((r - m) * (scale * float(np.log2(np.e)))) for r in logits]
        total = _tree(_add, ps)
        pin(total)
        inv = pltpu.reciprocal(total, approx=True)
        inv = inv * (2.0 - total * inv)
        for j in range(NT):
            if j % 2 == 0:
                yield
                ps[0], ps[4] = gate(ps[0], ALAG), gate(ps[4], ALAG)
            o = _chain(_add, [ps[w] * vbuf[j, ts, pl.ds(r0 - sh, 8), :]
                              for w, (ts, sh) in enumerate(src)]) * inv
            pin(o)
            put(qbuf.at[j, t, pl.ds(r0, 8), :], o)

    def out_operands(r, i, last):
        for j in range(4):
            a = [qbuf[j + o, b % 8, pl.ds(8 + 64 * lb + 16 * (b // 8), 16), :]
                 for b, lb in (out_rows(r, i, last), out_rows(r + 1, i, last)) for o in (0, 4)]
            a[0], a[3] = gate(a[0]), gate(a[3])
            for k, v in enumerate(_strassen_lhs(*a)):
                if k in (1, 4):
                    pin(v)
                obuf[r // 2, k, j, r16(i), :] = v.astype(BF16)
            if j < 3:
                yield

    def store_rows(b, lb):
        c, t = divmod(b, 8)
        for j in range(NT):
            words = pack(xres[b, j, r16(lb), :], xres[b + 1, j, r16(lb), :])
            pin(words)
            io32[j, lb, c, pl.ds(t // 2, 16, stride=4), :] = words

    unit_ticks = NT + 2 * XGAP
    step = 2
    out_ticks = 28

    def add_proj(sched, tick, c, lo, hi):
        jobs = [(b // step, b, n) for b in range(8 * c, 8 * c + 8, step) for n in range(lo, hi, step)]
        sched.add(tick, gemm(abuf32, wqkv32, jobs, qkv_sink))
        return tick + len(jobs) * out_ticks * step // NT

    def add_attention(sched, tick, pace, rows, last):
        units = [(r, i, half, h) for r in rows[::2] for i in range(4) for half in range(2) for h in range(2)]
        for n, (r, i, half, h) in enumerate(units):
            sched.add(tick + n * pace, attention(*out_rows(r + half, i, last), h))
            if half and h:
                sched.add(int(tick + n * pace) + unit_ticks, out_operands(r, i, last))

    def add_out(sched, tick, rows, last):
        jobs = [(r // 2, r, n) for r in rows[::2] for n in range(0, NT, 2)]
        sched.add(tick, gemm(obuf32, wo32, jobs, functools.partial(out_sink, last)))

    def add_tail(sched, tick, rows, last):
        ready = {}
        for i, r in enumerate(rows):
            t0 = tick + (i // 2 + 1) * out_ticks
            fast = i >= len(rows) - (2 if last else 4)
            if not last:
                t0 += 0 if fast else TOFF + i % 2 * out_ticks // 2
                ready[r % 8] = add_d_fwd(sched, t0, r, i % 2 if fast else out_ticks / 8)
            elif r % 2:
                c, p = r // 8, r % 8 // 2
                gap = 0 if fast else 3
                for j in range(4):
                    sched.add(t0 + (j + 1) * gap, _once(store_rows, *((r - 1, j) if c else (2 * j, p))))
                for lb in ([p] if c == 0 else range(4) if p == 3 else []):
                    sched.add(t0 + 5 * gap + 1, _once(start, out_copies(c, lb)))
        return ready

    q_ticks = 8 * out_ticks // step
    att_ticks = unit_ticks + 1 + 2
    order = [(a + 8) % NB for a in range(NB)]

    def add_attention_block(sched, cols, last):
        stats = {}
        t0 = max([add_d_inv(sched, 0, b, 0, stats, not last, cols) for b in range(step)])
        if not last:
            sched.add(cols[3] - KLEAD, _once(wait, qkv_copies(1) + dmat_cp))
            done = add_prep_wqkv(sched, cols[3] - KLEAD, 1, KPACE, [7] * 4)
            t0 = max(t0, done[0])
            assert all(d <= t0 + p * out_ticks / 4 for p, d in enumerate(done))
            sched.add(t0 + out_ticks, _once(wait, qkv_copies(2)))
            sched.add(t0 + out_ticks, _once(start, qkv_copies(0)))
            done = add_prep_wqkv(sched, t0 + out_ticks, 2, 2 * out_ticks - 6, [out_ticks - 4] * 4)
            assert all(d <= t0 + q_ticks + p * out_ticks for p, d in enumerate(done))
            sched.add(t0 + 2 * q_ticks, _once(wait, qkv_copies(0)))
            sched.add(t0 + 2 * q_ticks, _once(start, wo_copies))
            done = add_prep_wqkv(sched, t0 + 2 * q_ticks, 0, q_ticks - 10, [q_ticks / 4] * 4)
            assert done[-1] <= t0 + 4 * q_ticks
            sched.add(t0 + 8 * q_ticks, _once(wait, wo_copies))
            for i in range(32):
                sched.add(t0 + 8 * q_ticks + i * q_ticks / 16, _once(prep_wo, *divmod(i, 8)))
        tick, kv_start, q_start = t0, {}, {}
        for kind, c in ("k0", "k1", "q1", "k2", "q2", "k3", "q3", "q0"):
            if kind == "k":
                kv_start[int(c)] = tick
                if c == "0" and not last:
                    tick = add_proj(sched, tick, 0, NT, 2 * NT)
                    jobs = [(b // step, b, n) for n in range(2 * NT, 3 * NT, step) for b in range(0, 8, step)]
                    sched.add(tick, gemm(abuf32, wqkv32, jobs, qkv_sink))
                    tick += q_ticks
                    continue
                tick = add_proj(sched, tick, int(c), NT, 3 * NT)
            else:
                q_start[int(c)] = tick
                tick = add_proj(sched, tick, int(c), 0, NT)
        pace = 2 * out_ticks / step
        for b in range(step, NB):
            due = kv_start[b // 8] + (b % 8 // step) * (2 if last or b >= 8 else 1) * out_ticks
            gap = min(1 + (b - step) * 0.5, DGAP1 if last else DGAP0)
            pace = DPACE1 if last else DPACE0
            at = (b - step) * pace
            at = t0 + at + max(0, at - 4 * q_ticks - out_ticks) * DSLOW
            if not last and b < 8:
                at, gap = max(cols[3], t0 + (b // step - 1) * out_ticks - (step - b % step) * 8), 1
            end = add_d_inv(sched, at, b, gap, stats, not last)
            assert end <= due, (b, end, due)
        begin = [q_start[c] + out_ticks + 3 for c in (1, 2, 3)] + [tick + (ATT1 if last else ATT0)]
        begin.append(tick + (NB // step - 1) * out_ticks - att_ticks)
        for i, c in enumerate((1, 2, 3, 0)):
            pace = (begin[i + 1] - begin[i]) / 64
            assert begin[i] >= max(kv_start[c], kv_start[(c - 1) % 4]) + 2 * q_ticks
            for p in range(4):
                assert begin[i] + 16 * p * pace >= q_start[c] + (4 if last and c == 0 else p + 1) * out_ticks
                assert begin[i] + (16 * p + 15) * pace + att_ticks <= tick + (4 * i + p) * out_ticks + 1e-6
            add_attention(sched, begin[i], pace, range(8 * c, 8 * c + 8), last)
        add_out(sched, tick, order, last)
        return tick + (NB // step) * out_ticks, add_tail(sched, tick, order, last)

    def add_input(sched):
        ready = {}
        after = (x_copies(2), x_copies(3) + perm_cp + w_copies(0) + w_copies(1),
                 w_copies(2) + w_copies(3), w_copies(4))
        for c in range(NC):
            sched.add(c * 32, _once(wait, x_copies(c)))
            sched.add(c * 32, _once(start, after[c]))
            for t in range(8):
                ready[t] = add_d_fwd(sched, c * 32 + t * 4, c * 8 + t, 1, 2, True)
        return 128 + 9, ready

    def add_filter_prep(sched, tick):
        after = (w_copies(5) + w_copies(6), w_copies(7) + f256_cp + dmat_cp, qkv_copies(1), qkv_copies(2))
        begin = [F0 + g * (tick - F0) / 4 for g in range(4)] + [tick + FG * g for g in range(5)]
        for g in range(8):
            if g % 2 == 0:
                sched.add(begin[g], _once(wait, w_copies(g) + w_copies(g + 1) + ([] if g else perm_cp)))
                sched.add(begin[g], _once(start, after[g // 2]))
            for m in range(4):
                sched.add(begin[g] + m * (begin[g + 1] - begin[g]) / 4,
                          _once(prep_filter, g // 4, g % 4 * 4 + m))
        sched.add(begin[8] + 1, _once(wait, f256_cp))
        return begin[8] + 2

    sched = _Schedule()

    start(x_copies(0))
    for ref in (abuf32, obuf32, ubuf32, wo32, sfw32, siv32, wide32):
        put(ref.at[(0,) * (len(ref.shape) - 2) + (pl.ds(0, 8),)], jnp.zeros((8, 128), U32))
    make_wide()
    start(x_copies(1))
    for t in range(8):
        make_s_fwd(t)
    for e in range(4):
        make_s_inv(e)
    tick, ready = add_input(sched)
    cols = add_s_stage(sched, tick, ready, add_filter_prep(sched, tick))
    tick, ready = add_attention_block(sched, cols, False)
    cols = add_s_stage(sched, tick, ready, tick)
    add_attention_block(sched, cols, True)
    sched.run()
    for c in range(NC):
        for lb in range(4):
            wait(out_copies(c, lb))


@jax.jit
def pallas_interleave_layers__spectral_gfnet__sliding_local_dilated__prompt_kernel(
    A_x: jax.Array,
    A_w_r: jax.Array,
    A_w_i: jax.Array,
    B_x: jax.Array,
    B_wqkv: jax.Array,
    B_wo: jax.Array,
):
    del B_x
    assert A_x.shape == (1, S, D) and A_w_r.shape == (S, D // 2 + 1)
    cst = _constants()
    x = A_x.astype(BF16).reshape(4, NC, 128, D)
    wr, wi = A_w_r.astype(BF16).T, A_w_i.astype(BF16).T
    hbm = pl.BlockSpec(memory_space=pl.ANY)
    edge = pl.BlockSpec((16, S), lambda i: (D // 32, 0))
    vm = pltpu.VMEM
    out = pl.pallas_call(
        _kernel,
        grid=(1,),
        in_specs=[hbm, hbm, hbm, edge, edge, hbm, hbm, hbm, hbm,
                  pl.BlockSpec((24, 256), lambda i: (0, 0)),
                  pl.BlockSpec((2, 16, 128), lambda i: (0, 0, 0))],
        out_specs=hbm,
        out_shape=jax.ShapeDtypeStruct((4, NC, 128, D), BF16),
        scratch_shapes=[
            vm((NT, 4, NC, 128, 128), BF16),
            vm((17, 128, 128), BF16),
            vm((32, 128, 128), BF16),
            vm((32, 128, 128), BF16),
            vm((256, 512), BF16),
            vm((2, 16, 512, 128), BF16),
            vm((2, 4, 4, 8, 64, 128), F32),
            vm((3 * NT, D, 128), BF16),
            vm((NT, D // 2, 128), U32),
            vm((12, 7, 512, 128), BF16),
            vm((NT, D, 128), BF16),
            vm((4, 7, 512, 128), BF16),
            vm((NB, NT, 64, 128), F32),
            vm((4, 32, 64, 128), U32),
            vm((4, 32, 128, 128), F32),
            vm((NY, 8, 128, 128), F32),
            vm((NY, 8, 64, 128), U32),
            vm((RING, 8, 64, 128), BF16),
            vm((RING, 9, 64, 128), F32),
            vm((NB // 2, 7, 4, 64, 128), BF16),
            vm((NB // 2, 7, 4, 64, 128), BF16),
            vm((NT, 8, 264, 128), F32),
            vm((NT, 8, 264, 128), F32),
            vm((NT, 8, 264, 128), F32),
            vm((3, 256, 128), F32),
            vm((8, 256, 128), BF16),
            pltpu.SemaphoreType.DMA((NC,)),
            pltpu.SemaphoreType.DMA((3,)),
            pltpu.SemaphoreType.DMA((8,)),
            pltpu.SemaphoreType.DMA((3,)),
            pltpu.SemaphoreType.DMA(()),
            pltpu.SemaphoreType.DMA(()),
        ],
        compiler_params=pltpu.CompilerParams(
            dimension_semantics=("arbitrary",), vmem_limit_bytes=120 * 2**20),
    )(x, wr, wi, wr, wi, B_wqkv.astype(BF16), B_wo.astype(BF16),
      cst["small"], cst["f256"], cst["tw"], cst["d8"])
    return out.reshape(1, S, D)
```

```python
import functools

import jax
import jax.numpy as jnp
import numpy as np
from jax import lax
from jax.experimental import pallas as pl
from jax.experimental.pallas import tpu as pltpu

S, D = 2048, 1024
NT = D // 128
NC = 4
WIN = 8
HEAD_DIM = 32
EPS = 1e-5
F32, BF16, U32 = jnp.float32, jnp.bfloat16, jnp.uint32
PAIRS = ((0, 4), (1, 7), (2, 6), (3, 5))
RSQ2 = float(np.sqrt(0.5))
NB = S // 64

RING = 8
NY = 4
XGAP = 3
GLAG = 4
ALAG = 4
SGLAG = 3
SGLAG2 = 5
S_LAG = 3
F0 = 112
KLEAD = 52
KPACE = 48
DGAP0 = 4.75
DGAP1 = 4.2
DPACE0 = 21
DPACE1 = 15.5
DSLOW = 0.6
SYNC = 3
ILAG = 3
FG = 4
TOFF = 3
ATT0 = 10
ATT1 = 95


def _residues(r):
    return (0, 8) if r == 0 else (r, 16 - r)


def _d_matrices():
    n = np.arange(64)[:, None]
    a = np.arange(32)
    fwd = np.zeros((8, 128, 128))
    inv = np.zeros((8, 128, 128))
    for r in range(8):
        kd = np.concatenate([16 * a + p for p in _residues(r)])
        weight = np.full(64, 2.0)
        if r == 0:
            kd[0], weight[0] = D // 2, 1.0
            ph = np.exp(-2j * np.pi * n * kd[None, :] / D)
            sgn = np.where(kd % 16 == 0, 1.0, -1.0)[None, :]
            m = np.concatenate([ph, ph * sgn], axis=0)
            re, im = m.real.copy(), m.imag.copy()
            ire, iim = re.copy(), im.copy()
            im[:, 0] = 1.0
            iim[:, 0] = 1.0
        else:
            p = 12 if r == 4 else r
            ph = np.exp(-2j * np.pi * n * kd[None, :] / D)
            si = np.where(kd % 16 == p, 1.0, -1.0)[None, :]
            m = np.concatenate([ph, 1j * si * ph], axis=0)
            re, im = m.real, m.imag
            ire, iim = re, im
        swapped = r in (4, 7, 6, 5)
        cols = [im, re] if swapped else [re, im]
        icols = [iim * weight, ire * weight] if swapped else [ire * weight, iim * weight]
        fwd[r] = np.concatenate(cols, axis=1)
        inv[r] = np.concatenate(icols, axis=1).T / D
    return fwd, inv


def _side_matrices():
    l = np.arange(256)
    f = np.exp(-2j * np.pi * ((l[:, None] * l[None, :]) % 256) / 256)
    f256 = np.concatenate([f.real, f.imag], axis=1)
    t = np.arange(8)
    tw = np.exp(-2j * np.pi * t[:, None] * l[None, :] / S)
    tw = np.concatenate([tw.real, tw.imag, np.zeros((8, 256))], axis=0)
    g = np.exp(-2j * np.pi * t[:, None] * t[None, :] / 8)
    d8 = np.zeros((2, 16, 128))
    d8[0, :, :16] = np.block([[g.real, -g.imag], [g.imag, g.real]])
    d8[1, :, :16] = d8[0, :, :16].T / S
    return f256, tw, d8


def _filter_rows():
    p = np.zeros((1, 128, 128))
    for k in range(32):
        for e in range(4):
            p[0, e * 32 + k, 4 * k + e] = 1.0
    return p


@functools.lru_cache(maxsize=None)
def _constants():
    dfw, div = _d_matrices()
    f256, tw, d8 = _side_matrices()
    small = np.concatenate([dfw, div, _filter_rows()], axis=0)
    b = lambda x: np.asarray(x, np.float32).astype(BF16)
    return dict(small=b(small), f256=b(f256),
                tw=np.asarray(tw, np.float32), d8=b(d8))


def _dot(a, b):
    return jnp.dot(a, b, preferred_element_type=F32)


def _dot_nt(a, b):
    return lax.dot_general(a, b, (((1,), (1,)), ((), ())), preferred_element_type=F32)


def _tree(op, xs):
    xs = list(xs)
    while len(xs) > 1:
        xs = [op(xs[i], xs[i + 1]) if i + 1 < len(xs) else xs[i] for i in range(0, len(xs), 2)]
    return xs[0]


def _chain(op, xs):
    return functools.reduce(op, xs)


def _lane(rows):
    return lax.broadcasted_iota(jnp.int32, (rows, 128), 1)


def _swap(x):
    return pltpu.roll(x, 64, 1)


def _unpack(w, i):
    return pltpu.unpack_elementwise(w, index=i, packed_dtype=BF16, unpacked_dtype=F32)


def _latency():
    for _ in range(XGAP):
        yield


def _add(a, b):
    return a + b


def _row_mean(xs):
    return jnp.sum(_tree(_add, xs), axis=1, keepdims=True) * (1.0 / D)


def _twiddle16(r, x, y):
    lo = _lane(x.shape[0]) < 64
    wr, wi = float(np.cos(np.pi * r / 8)), float(-np.sin(np.pi * r / 8))
    cross = jnp.where(lo, 0.0, wr)
    return x * jnp.where(lo, 1.0, wi) + y * cross, y * jnp.where(lo, 1.0, -wi) + x * cross


def _d_butterfly_fwd(a, emit, pin, wide):
    s = [a[j] + a[j + 4] for j in range(4)]
    e, o = s[0] + s[2], s[1] + s[3]
    total, t4 = e + o, e - o
    emit(4, t4)
    d0, nd2 = a[0] - a[4], a[6] - a[2]
    d1, d3 = a[1] - a[5], a[3] - a[7]
    p, q = (d1 - d3) * RSQ2, (d1 + d3) * -RSQ2
    ts = {1: (d0 + p, q + nd2), 2: (s[0] - s[2], s[3] - s[1]), 3: (d0 - p, q - nd2)}
    mean8 = jnp.sum(total, axis=1, keepdims=True) * (1.0 / 128)
    if wide:
        for r, (tr, ti) in ts.items():
            emit(r, tr)
            emit(8 - r, ti)
    else:
        ab = {r: _twiddle16(r, *t) for r, t in ts.items()}
        ab = {r: (a, _swap(b)) for r, (a, b) in ab.items()}
    dev = _tree(_add, [v * v for t in ts.values() for v in t]) * 2.0 + t4 * t4
    pin(dev)
    yield from _latency()
    t0 = total - mean8
    emit(0, t0)
    var = jnp.sum(dev + t0 * t0, axis=1, keepdims=True) * (1.0 / (NT * D))
    if not wide:
        for r, (x, y) in ab.items():
            emit(r, x + y)
            emit(8 - r, x - y)
    yield from _latency()
    return lax.rsqrt(var + EPS)


def _d_butterfly_inv(u, pin, gate):
    ab = {r: (u[r] + u[8 - r], _swap(u[r] - u[8 - r])) for r in (1, 2, 3)}
    e, o = u[0] + u[4], u[0] - u[4]
    yield from _latency()
    ts = {r: _twiddle16(r, x, gate(y)) for r, (x, y) in ab.items()}
    pin(*[t[0] for t in ts.values()])
    yield
    s = [e + ts[2][0], o - ts[2][1], e - ts[2][0], o + ts[2][1]]
    p = (ts[1][0] - ts[3][0]) * RSQ2
    q = (ts[1][1] + ts[3][1]) * RSQ2
    d0, d1, d2, nd3 = ts[1][0] + ts[3][0], p - q, ts[3][1] - ts[1][1], p + q
    return [s[0] + d0, s[1] + d1, s[2] + d2, s[3] - nd3,
            s[0] - d0, s[1] - d1, s[2] - d2, s[3] + nd3]


def _strassen_lhs(a11, a12, a21, a22):
    return [a11 + a22, a21 + a22, a11, a22, a11 + a12, a21 - a11, a12 - a22]


def _strassen_rhs(b11, b12, b21, b22):
    return [b11 + b22, b11, b22 - b12, b11 - b21, b22, b11 + b12, b21 + b22]


def _cadd(a, b):
    return a[0] + b[0], a[1] + b[1]


def _csub(a, b):
    return a[0] - b[0], a[1] - b[1]


def _dft4(z, inverse):
    a, b = _cadd(z[0], z[2]), _csub(z[0], z[2])
    c, d = _cadd(z[1], z[3]), _csub(z[1], z[3])
    minus = (b[0] + d[1], b[1] - d[0])
    plus = (b[0] - d[1], b[1] + d[0])
    return [_cadd(a, c), plus if inverse else minus, _csub(a, c), minus if inverse else plus]


def _dft8(z, inverse):
    ev = _dft4(z[0::2], inverse)
    od = _dft4(z[1::2], inverse)
    out = [None] * 8
    out[0], out[4] = _cadd(ev[0], od[0]), _csub(ev[0], od[0])
    (er, ei), (x, y) = ev[2], od[2]
    minus, plus = (er + y, ei - x), (er - y, ei + x)
    out[2], out[6] = (plus, minus) if inverse else (minus, plus)
    for k in (1, 3):
        (er, ei), (x, y) = ev[k], od[k]
        sm, df = (x + y) * RSQ2, (x - y) * RSQ2
        if not inverse:
            if k == 1:
                out[1], out[5] = (er + sm, ei - df), (er - sm, ei + df)
            else:
                out[3], out[7] = (er - df, ei - sm), (er + df, ei + sm)
        else:
            if k == 1:
                out[1], out[5] = (er + df, ei + sm), (er - df, ei - sm)
            else:
                out[3], out[7] = (er - sm, ei + df), (er + sm, ei - df)
    return out


class _Schedule:
    def __init__(self):
        self.pending = []

    def add(self, tick, gen):
        self.pending.append((int(tick), len(self.pending), gen))

    def run(self):
        pending = sorted(self.pending, key=lambda p: p[:2])
        active, tick, i = [], 0, 0
        while active or i < len(pending):
            while i < len(pending) and pending[i][0] <= tick:
                active.append(pending[i][2])
                i += 1
            for g in list(active):
                if next(g, 0) == 0:
                    active.remove(g)
            tick += 1
        self.pending = []


def _once(fn, *args):
    fn(*args)
    return
    yield


def _kernel(x_hbm, wr_hbm, wi_hbm, wr_edge, wi_edge, wqkv_hbm, wo_hbm,
            small_hbm, f256_hbm, tw_ref, d8_ref,
            out_hbm,
            io, small, sfw, siv, f256, wraw, wf, wqkv_raw, wtmp, wqkv, wo_raw, wo,
            xres, zin, zout, ybuf, fbuf, ubuf, uout, abuf, obuf, qbuf, kbuf, vbuf, side,
            wide, sem_x, sem_c, sem_w, sem_qkv, sem_wo, sem_out):

    def x_copies(c):
        return [pltpu.make_async_copy(x_hbm.at[:, c, :, pl.ds(j * 128, 128)], io.at[j, :, c],
                                      sem_x.at[c]) for j in range(NT)]

    def out_copies(c, lb):
        return [pltpu.make_async_copy(io.at[j, lb, c], out_hbm.at[lb, c, :, pl.ds(j * 128, 128)],
                                      sem_out) for j in range(NT)]

    perm_cp, dmat_cp, f256_cp = ([pltpu.make_async_copy(s, d, sem_c.at[i])] for i, (s, d) in enumerate((
        (small_hbm.at[pl.ds(16, 1)], small.at[pl.ds(16, 1)]),
        (small_hbm.at[pl.ds(0, 16)], small.at[pl.ds(0, 16)]), (f256_hbm, f256))))

    def w_copies(g):
        src = (wr_hbm, wi_hbm)[g // 4]
        return [pltpu.make_async_copy(src.at[pl.ds(0, 512), pl.ds(m * 128, 128)], wraw.at[g // 4, m],
                                      sem_w.at[g]) for m in range(g % 4 * 4, g % 4 * 4 + 4)]

    def qkv_copies(g):
        return [pltpu.make_async_copy(wqkv_hbm.at[:, pl.ds(g * D + j * 128, 128)],
                                      wqkv_raw.at[g * NT + j], sem_qkv.at[g]) for j in range(NT)]

    wo_copies = [pltpu.make_async_copy(wo_hbm.at[:, pl.ds(j * 128, 128)], wo_raw.at[j], sem_wo)
                 for j in range(NT)]

    def start(cs):
        for cp in cs:
            cp.start()

    def wait(cs):
        for cp in cs:
            cp.wait()

    io32, wraw32, wo_raw32 = io.bitcast(U32), wraw.bitcast(U32), wo_raw.bitcast(U32)
    small32, sfw32, siv32, wide32 = (r.bitcast(U32) for r in (small, sfw, siv, wide))
    wqkv_raw32, wqkv32, wo32 = (r.bitcast(U32) for r in (wqkv_raw, wqkv, wo))
    ubuf32, abuf32, obuf32 = ubuf.bitcast(U32), abuf.bitcast(U32), obuf.bitcast(U32)

    never = tw_ref[16:24, 0:128] != 0.0
    never_wide = {n: jnp.concatenate([tw_ref[16:24, 0:128]] * n, axis=1) != 0.0 for n in (1, 2, 4)}
    token = {}

    def pin(*values):
        for v in values:
            key = v.shape[0], v.dtype == F32
            token[key] = (lax.max if key[1] else lax.bitwise_xor)(token[key], v) if key in token else v

    clock = []

    def gate(v, lag=GLAG):
        if len(clock) < lag:
            return v
        old = clock[-lag] if v.dtype == F32 else pltpu.bitcast(clock[-lag], v.dtype)
        if v.shape[0] == 8:
            return lax.select(never, old, v)
        return lax.concatenate([lax.select(never, old, v[0:8]), v[8:]], 0)

    def ticking(o):
        clock.append(o[0:8])
        del clock[:-16]
        return o

    def lhs(*tiles):
        if not token and len(tiles) == 4 and len(clock) >= SYNC:
            pin(clock[-SYNC])
        words = lax.concatenate(tiles, 1) if len(tiles) > 1 else tiles[0]
        if token:
            parts = [pltpu.bitcast(v, U32) if is_float else v for (_, is_float), v in token.items()]
            token.clear()
            w = _chain(lax.bitwise_xor, [v[i:i + 8] if v.shape[0] > 8 else v
                                         for v in parts for i in range(0, v.shape[0], 8)])
            w = lax.concatenate([w] * len(tiles), 1) if len(tiles) > 1 else w
            words = lax.concatenate([lax.select(never_wide[len(tiles)], w, words[0:8]), words[8:]], 0)
        return pltpu.bitcast(words, BF16)

    def bf(words):
        return pltpu.bitcast(words, BF16)

    def pack(a, b):
        return pltpu.bitcast(pltpu.pack_elementwise([a, b], packed_dtype=BF16), U32)

    def r16(i):
        return pl.ds(i * 16, 16)

    always = {}

    def put(ref, v):
        if v.shape not in always:
            always[v.shape] = jnp.ones(v.shape, jnp.bool_)
        pltpu.store(ref, v, mask=always[v.shape])

    def load_x(b, lb, from_input):
        if from_input:
            c, t = divmod(b, 8)
            return [_unpack(io32[j, lb, c, pl.ds(t // 2, 16, stride=4), :], t % 2) for j in range(NT)]
        return [xres[b, j, r16(lb), :] for j in range(NT)]

    def unit(p):
        angle = (((p + S // 2) & (S - 1)) - S // 2).astype(F32) * (2 * np.pi / S)
        return jnp.cos(angle), jnp.sin(angle)

    def times_row(a, b, i):
        br, bi = (jnp.broadcast_to(v[i:i + 1], (8, 128)) for v in b)
        return a[0] * br - a[1] * bi, a[0] * bi + a[1] * br

    def make_wide():
        row, lane = lax.broadcasted_iota(jnp.int32, (8, 128), 0), _lane(8)
        for ct, (ra, rb) in enumerate(PAIRS):
            res = _residues(ra) + _residues(rb)
            kd = (lane & 31) * 16 + _chain(
                _add, [jnp.where(lane >> 5 == g, p, 0) for g, p in enumerate(res)])
            if ct == 0:
                kd = jnp.where(lane == 0, D // 2, kd)
            fine, coarse = unit(-2 * row * kd), [unit(-16 * (row + 8 * h) * kd) for h in range(2)]
            for a in range(16):
                re, im = times_row(fine, coarse[a // 8], a % 8)
                if ct == 0:
                    even = kd & 7 == 0
                    top = jnp.where(even, re, 0.0), jnp.where(lane == 0, 1.0, jnp.where(even, im, 0.0))
                    bottom = jnp.where(even, 0.0, re), jnp.where(even, 0.0, im)
                else:
                    sign = jnp.where(kd & 7 == ra, 1.0, -1.0)
                    top, bottom = (re, im), (-sign * im, sign * re)
                for i in range(2):
                    wide[2 * ct + i, pl.ds(8 * a, 8), :] = top[i].astype(BF16)
                    wide[2 * ct + i, pl.ds(128 + 8 * a, 8), :] = bottom[i].astype(BF16)

    def make_s_fwd(t):
        row, lane = lax.broadcasted_iota(jnp.int32, (8, 128), 0), _lane(8)
        pos = 8 * (lane >> 1) + t
        fine = unit((lane & 1) * (S // 4) - 4 * row * pos)
        shift, coarse = unit(-row * pos), unit(-32 * row * pos)
        for e in range(4):
            base = times_row(fine, shift, e)
            for g in range(8):
                for i, v in enumerate(times_row(base, coarse, g)):
                    sfw[t * 4 + e, pl.ds(16 * g + 8 * i, 8), :] = v.astype(BF16)

    def make_s_inv(e):
        row, lane = lax.broadcasted_iota(jnp.int32, (8, 128), 0), _lane(8)
        freq = 4 * (lane >> 1) + e
        fine = [v * (1.0 / S) for v in unit((lane & 1) * (S // 4) + 8 * row * freq)]
        shift, coarse = unit(row * freq), unit(64 * row * freq)
        for t in range(8):
            base = times_row(fine, shift, t)
            for g in range(8):
                for i, v in enumerate(times_row(base, coarse, g)):
                    siv[t * 4 + e, pl.ds(64 * i + 8 * g, 8), :] = v.astype(BF16)

    def prep_filter(ri, m):
        sub = lax.broadcasted_iota(jnp.int32, (8, 128), 0)
        edge = (wr_edge, wi_edge)[ri]
        res = {}
        for i in range(8):
            words = wraw32[ri, m, pl.ds(i, 32, stride=8), :]
            res[2 * i], res[2 * i + 1] = _unpack(words, 0), _unpack(words, 1)
        first = res[0][0:8]
        dst = pl.ds((m % 2) * 16 + ri * 8, 8)
        prev = jnp.zeros((8, 128), F32) if m < 2 else side[1, dst, :]
        put(side.at[1, dst, :], jnp.where(sub == m // 2, jnp.broadcast_to(first[0:1], (8, 128)), prev))
        nyq = jnp.broadcast_to(edge[0:1, pl.ds(m * 128, 128)].astype(F32), (8, 128))
        res[0] = jnp.concatenate([jnp.where(sub == 0, nyq, first), res[0][8:]], axis=0)
        for ct, (ra, rb) in enumerate(PAIRS):
            blk = jnp.concatenate([res[p] for p in _residues(ra) + _residues(rb)], axis=0)
            o = _dot_nt(lhs(small32[16]), blk.astype(BF16))
            for e in range(4):
                put(wf.at[ri, ct, e, m // 2, pl.ds((m % 2) * 32, 32), :], o[e * 32:(e + 1) * 32])

    def shuffle(words, index):
        return jnp.take_along_axis(words, index, axis=1)

    def prep_wqkv_tile(g, i, part):
        lane = _lane(8)
        index = (lane & 3) * 32 + (((lane >> 2) - i) & 7) * 4 + (lane >> 5)
        rows = [pl.ds((part * 16 + r) * 8, 8) for r in range(16)]
        ws = [shuffle(gate(wqkv_raw32[g * NT + i, rs, :]), index) for rs in rows]
        yield from _latency()
        for rs, w in zip(rows, ws):
            pin(w)
            put(wtmp.at[i, rs, :], w)

    def prep_wqkv_cross(g, r):
        pos = (_lane(8) >> 2) & 7
        u = [wtmp[(-j) % 8, pl.ds(r * 8, 8), :] for j in range(NT)]
        u[0], u[4] = gate(u[0]), gate(u[4])
        for bit in range(3):
            m = ((pos >> bit) & 1) == 1
            u = [lax.select(m, u[(j - (1 << bit)) % 8], u[j]) for j in range(NT)]
        for j in range(NT):
            if j < 4:
                pin(u[j])
            put(wqkv_raw32.at[g * NT + j, pl.ds(r * 8, 8), :], u[j])

    def prep_wqkv_pair(g, p, part):
        lane = _lane(8)
        ws = {}
        for n in range(2):
            index = (lane & 96) | ((lane + 4 * (2 * p + n)) & 31)
            for half in range(2):
                for r in range(part * 2, part * 2 + 2):
                    w = gate(wqkv_raw32[g * NT + 2 * p + n, pl.ds(half * 256 + r * 8, 8), :])
                    ws[r, half, n] = shuffle(w, index) if p + n else w
        yield from _latency()
        for r in range(part * 2, part * 2 + 2):
            quad = [ws[r, half, n] for half in range(2) for n in range(2)]
            ops = [_strassen_rhs(*[_unpack(w, i) for w in quad]) for i in range(2)]
            for k in range(7):
                word = {1: quad[0], 4: quad[3]}.get(k)
                if word is None:
                    word = pack(ops[0][k], ops[1][k])
                if k in (2, 3):
                    pin(word)
                put(wqkv32.at[g * 4 + p, k, pl.ds(r * 8, 8), :], word)

    def add_prep_wqkv(sched, tick, g, ticks, pair_ticks):
        for i in range(32):
            sched.add(tick + i * ticks / 64, prep_wqkv_tile(g, *divmod(i, 4)))
        tick = int(tick + ticks / 2) + XGAP + 1
        for r in range(64):
            sched.add(tick + r * ticks / 128, _once(prep_wqkv_cross, g, r))
        tick = int(tick + ticks / 2) + 1
        done = []
        for p, n in enumerate(pair_ticks):
            for i in range(16):
                sched.add(tick + i * n / 16, prep_wqkv_pair(g, p, i))
            tick += n
            done.append(int(tick) + XGAP + 1)
        return done

    def prep_wo(p, dp):
        ws = [wo_raw32[2 * p + n, pl.ds(dp + off, 32, stride=16), :] for off in (0, 8) for n in (0, 1)]
        for i in range(2):
            b = [_unpack(w, i) for w in ws]
            r0 = (2 * dp + i) * 32
            for k, v in enumerate(_strassen_rhs(*b)):
                if k in (2, 3):
                    pin(v)
                wo[p, k, pl.ds(r0, 32), :] = v.astype(BF16)

    def ln_stats(xs):
        lane_mean = _tree(_add, xs) * (1.0 / NT)
        lane_m2 = _tree(_add, [jnp.square(x - lane_mean) for x in xs])
        pin(lane_m2)
        mean = jnp.sum(lane_mean, axis=1, keepdims=True) * (1.0 / 128)
        yield from _latency()
        m2 = lane_m2 + jnp.square(gate(lane_mean) - mean) * float(NT)
        pin(m2)
        var = jnp.sum(m2, axis=1, keepdims=True) * (1.0 / D)
        yield from _latency()
        return mean, lax.rsqrt(gate(jnp.broadcast_to(var, (16, 128))) + EPS)

    def d_fwd_rows(b, lb, from_input=False):
        xs = load_x(b, lb, from_input)

        def emit(r, v):
            if r % 4 == 0 or (r < 4 and not from_input):
                pin(v)
            ubuf[b % RING, r, r16(lb), :] = v.astype(BF16)

        xs[:4] = [gate(x, ILAG if from_input else GLAG) for x in xs[:4]]
        inv = yield from _d_butterfly_fwd(xs, emit, pin, from_input)
        inv = jnp.broadcast_to(inv, (16, 128))
        pin(inv)
        put(uout.at[b % RING, 8, r16(lb), :], inv)

    def d_dots(b, base, per_tick):
        for r in range(8):
            o = _dot(lhs(ubuf32[b % RING, r]), bf(small32[base + r]))
            put(uout.at[b % RING, r], o)
            if r % per_tick == per_tick - 1 and r < 7:
                yield

    def d_dots_wide(b):
        for ct, (ra, rb) in enumerate(PAIRS):
            u = lhs(ubuf32[b % RING, ra], ubuf32[b % RING, rb])
            for i, r in enumerate((ra, rb)):
                o = _dot(u, bf(wide32[2 * ct + i]))
                put(uout.at[b % RING, r], ticking(o) if i else o)
            if ct < 3:
                yield

    def d_fwd_cols(b, ct, is_wide):
        c, t = divmod(b, 8)
        ra, rb = PAIRS[ct]
        lane = _lane(16)
        lo = lane < 64
        z, x0 = [], []
        for lb in range(4):
            a, bb, inv = (uout[b % RING, r, r16(lb), :] for r in (ra, rb, 8))
            inv = gate(inv, ILAG if is_wide else GLAG)
            a, bb = a * inv, bb * inv
            if is_wide:
                if ct == 0:
                    x0.append(pltpu.roll(bb, t, 1) if t else bb)
                    bb = jnp.where(lane == 0, 0.0, bb)
                z.append((a, bb))
                continue
            if ct == 0:
                x0.append(pltpu.roll(a, (t + 64) % 128, 1))
                a = jnp.where(lane == 64, 0.0, a)
            im = lax.select(lo, bb, a)
            z.append((lax.select(lo, a, bb), _swap(im)))
        if not is_wide:
            yield from _latency()
        for e, (re, im) in enumerate(_dft4(z, False)):
            words = pack(re, im)
            if e < 2:
                pin(words)
            put(zin.at[ct, t * 4 + e, r16(c), :], words)
        if is_wide and ct == 0:
            yield from _latency()
        for lb, v in enumerate(x0):
            ls = pl.ds(64 * lb + 16 * c, 16)
            prev = jnp.zeros((16, 128), F32) if t == 0 else side[0, ls, :]
            v = jnp.where(lane == t, v, prev)
            pin(v)
            put(side.at[0, ls, :], v)

    def add_d_fwd(sched, tick, b, gap, per_tick=4, from_input=False):
        for lb in range(4):
            sched.add(tick + lb * gap, d_fwd_rows(b, lb, from_input))
        tick = int(tick + 3 * gap) + XGAP + 1
        sched.add(tick, d_dots_wide(b) if from_input else d_dots(b, 0, per_tick))
        for ct in range(4):
            sched.add(tick + 8 // per_tick + 3 + ct * gap, d_fwd_cols(b, ct, from_input))
        return int(tick + 8 // per_tick + 3 + 3 * gap) + XGAP + 1

    def side_path():
        vt = side[0].T[0:8]
        yield
        zero8 = jnp.zeros((8, 256), F32)
        u = _dot(jnp.concatenate([vt, zero8], axis=0).astype(BF16), f256[...])[0:8]
        twr, twi = tw_ref[0:8, :], tw_ref[8:16, :]
        ur, ui = u[:, 0:256], u[:, 256:512]
        pad = jnp.zeros((112, 256), BF16)
        for _ in range(4):
            yield
        uu = jnp.concatenate([ur * twr - ui * twi, ur * twi + ui * twr], axis=0).astype(BF16)
        xk = _dot(d8_ref[0], jnp.concatenate([uu, pad], axis=0))
        for _ in range(4):
            yield
        wr = jnp.concatenate([side[1, 0:8, :], side[1, 16:24, :]], axis=1)
        wi = jnp.concatenate([side[1, 8:16, :], side[1, 24:32, :]], axis=1)
        xr, xi = xk[0:8], xk[8:16]
        yy = jnp.concatenate([xr * wr - xi * wi, xr * wi + xi * wr], axis=0).astype(BF16)
        p = _dot(d8_ref[1], jnp.concatenate([yy, pad], axis=0))
        for _ in range(4):
            yield
        twr, twi = tw_ref[0:8, :], tw_ref[8:16, :]
        pr, pi = p[0:8], p[8:16]
        g = jnp.concatenate([pr * twr + pi * twi, pi * twr - pr * twi], axis=1)
        g = jnp.concatenate([g, jnp.zeros((8, 512), F32)], axis=0).astype(BF16)
        y0 = _dot_nt(g, f256[...])
        for _ in range(4):
            yield
        put(side.at[2], jnp.concatenate([y0, jnp.zeros((112, 256), F32)], axis=0).T)

    def s_fwd(u, t):
        ct, e = divmod(u, 4)
        put(ybuf.at[u % NY, t], ticking(_dot(lhs(sfw32[t * 4 + e]), bf(zin[ct, t * 4 + e]))))

    def s_filter(u, g):
        ct, e = divmod(u, 4)
        z = [tuple(ybuf[u % NY, t, pl.ds(g * 16 + i, 8), :] for i in (0, 8))
             for t in range(8)]
        lag = SGLAG if u * 8 + g < 122 - S_LAG else SGLAG2
        z[0], z[1] = [tuple(gate(v, lag) for v in zz) for zz in z[0:2]]
        xk = _dft8(z, False)
        for k2 in range(8):
            wr = wf[0, ct, e, k2, pl.ds(g * 8, 8), :]
            wi = wf[1, ct, e, k2, pl.ds(g * 8, 8), :]
            re, im = xk[k2]
            xk[k2] = (re * wr - im * wi, re * wi + im * wr)
        for t, (re, im) in enumerate(_dft8(xk, True)):
            words = pack(re, im)
            if t < 4:
                pin(words)
            put(fbuf.at[u % NY, t, pl.ds(g * 8, 8), :], words)

    def s_inv(u, t):
        ct, e = divmod(u, 4)
        o = _dot(lhs(siv32[t * 4 + e]), bf(fbuf[u % NY, t]))
        put(zout.at[ct, t * 4 + e], ticking(o) if u * 8 + t >= 110 - S_LAG else o)

    def add_s_stage(sched, early, ready, t1):
        ahead = 8 + S_LAG
        tick = early
        for t in sorted(range(8), key=lambda t: ready[t]):
            for i in range(t, ahead, 8):
                tick = max(tick + 0.5, ready[t])
                sched.add(tick, _once(s_fwd, i // 8, t))
        t1 = max(t1, int(tick) + 1)
        sched.add(max(max(ready), t1), side_path())
        for i in range(128):
            if i + ahead < 128:
                sched.add(t1 + i, _once(s_fwd, *divmod(i + ahead, 8)))
            sched.add(t1 + i, _once(s_filter, *divmod(i, 8)))
            sched.add(t1 + 9 + (i if i < 120 else 120 + (i - 120) // 4), _once(s_inv, *divmod(i, 8)))
        return [t1 + 32 * ct + 40 for ct in range(3)] + [t1 + 131]

    def d_inv_cols(b, ct):
        c, t = divmod(b, 8)
        ra, rb = PAIRS[ct]
        lane = _lane(16)
        lo = lane < 64
        u = [(zout[ct, t * 4 + e, r16(c), :], zout[ct, t * 4 + e, r16(4 + c), :]) for e in range(4)]
        u[0], u[1] = tuple(map(gate, u[0])), tuple(map(gate, u[1]))
        z = _dft4(u, True)
        z = [(re, _swap(im)) for re, im in z]
        if ct == 0:
            y0 = [pltpu.roll(side[2, pl.ds(64 * lb + 16 * c, 16), :], 64 - t, 1) for lb in range(4)]
        yield from _latency()
        for lb, (re, sw) in enumerate(z):
            sw = gate(sw)
            a, bb = lax.select(lo, re, sw), lax.select(lo, sw, re)
            if ct == 0:
                a = jnp.where(lane == 64, y0[lb], a)
            pin(a)
            ubuf[b % RING, ra, r16(lb), :] = a.astype(BF16)
            ubuf[b % RING, rb, r16(lb), :] = bb.astype(BF16)

    def d_inv_rows(b, lb, stats, first):
        u = [uout[b % RING, r, r16(lb), :] for r in range(8)]
        ys = yield from _d_butterfly_inv([gate(v) if r < 4 else v for r, v in enumerate(u)], pin, gate)
        xs = [x + y for x, y in zip(load_x(b, lb, first), ys)]
        for j in range(NT):
            put(xres.at[b, j, r16(lb), :], xs[j])
        stats[b, lb] = yield from ln_stats(xs)
        if b % 2:
            for j in range(4):
                a = [(xres[bb, j + o, r16(lb), :] - stats[bb, lb][0]) * stats[bb, lb][1]
                     for bb in (b - 1, b) for o in (0, 4)]
                a[0], a[3] = gate(a[0]), gate(a[3])
                for k, v in enumerate(_strassen_lhs(*a)):
                    if k in (1, 4):
                        pin(v)
                    abuf[b // 2, k, j, r16(lb), :] = v.astype(BF16)
                if j < 3:
                    yield

    def add_d_inv(sched, tick, b, gap, stats, first, cols=None):
        per_tick = 4
        cols = cols or [tick + ct * gap for ct in range(4)]
        for ct in range(4):
            sched.add(cols[ct], d_inv_cols(b, ct))
        tick = int(cols[3]) + XGAP + 1
        sched.add(tick, d_dots(b, 8, per_tick))
        tick += 8 // per_tick + 3
        for lb in range(4):
            sched.add(tick + lb * gap, d_inv_rows(b, lb, stats, first))
        return int(tick + 3 * gap) + 3 * XGAP + 1 + 4

    def gemm(lhs32, rhs32, jobs, sink):
        for slot, b, n in jobs:
            m = {}
            for k in (3, 1, 0, 6, 5, 4, 2):
                m[k] = ticking(_dot(lhs(*[lhs32[slot, k, j] for j in range(4)]), bf(rhs32[n // 2, k])))
                if k == 1:
                    sink(b + 1, n, m[1] - m[3])
                elif k == 0:
                    c11, c22 = m[3] - m[0], m[1] - m[0]
                elif k == 6:
                    c11 = m[6] - c11
                elif k == 5:
                    c22 = m[5] - c22
                elif k == 4:
                    sink(b, n, c11 - m[4])
                elif k == 2:
                    sink(b, n + 1, m[4] - m[2])
                    sink(b + 1, n + 1, c22 - m[2])
                yield

    def qkv_sink(b, n, o):
        c, t = divmod(b, 8)
        dst = (qbuf, kbuf, vbuf)[n // NT]
        for lb in range(4):
            put(dst.at[n % NT, t, pl.ds(8 + 64 * lb + 16 * c, 16), :], o[lb * 16:(lb + 1) * 16])
        if b == 0 and n >= NT:
            first = jnp.broadcast_to(o[0:1], (8, 128))
            for tt in range(8):
                dst[n % NT, tt, pl.ds(0, 8), :] = first

    def out_rows(r, i, last):
        c, t = divmod(r, 8)
        return (c * 8 + t % 2 * 4 + i, t // 2) if last and c == 0 else (r, i)

    def out_sink(last, r, n, o):
        for i in range(4):
            b, lb = out_rows(r, i, last)
            put(xres.at[b, n, r16(lb), :], xres[b, n, r16(lb), :] + o[i * 16:(i + 1) * 16])

    def attention(b, lb, h):
        c, t = divmod(b, 8)
        log2e = float(np.log2(np.e))
        scale = HEAD_DIM ** -0.5 * log2e
        r0 = 8 + 64 * lb + 16 * c + 8 * h
        src = [((t - 2 * w) % 8, -((t - 2 * w) // 8)) for w in range(WIN)]
        acc = [None] * WIN
        for j in range(NT):
            if j % 2 == 0:
                factor = gate(jnp.full((8, 128), scale, F32), ALAG)
            q = qbuf[j, t, pl.ds(r0, 8), :] * factor
            for w, (ts, sh) in enumerate(src):
                p = q * kbuf[j, ts, pl.ds(r0 - sh, 8), :]
                acc[w] = p if j == 0 else acc[w] + p
            if j % 2 and j < NT - 1:
                pin(*acc)
                yield
        part = [(r, pltpu.roll(r, 64, 1)) for r in acc]
        yield from _latency()
        part = [r + rr for r, rr in part]
        part = [(r, pltpu.roll(r, 32, 1)) for r in part]
        yield from _latency()
        logits = [r + rr for r, rr in part]
        if r0 == 8:
            sub = lax.broadcasted_iota(jnp.int32, (8, 128), 0)
            logits = [jnp.where(sub >= sh, r, -1e9 * log2e) if sh else r
                      for r, (_, sh) in zip(logits, src)]
        logits[0] = gate(logits[0], ALAG)
        m = _tree(jnp.maximum, logits)
        ps = [jnp.exp2(r - m) for r in logits]
        total = _tree(_add, ps)
        pin(total)
        inv = pltpu.reciprocal(total, approx=True)
        inv = inv * (2.0 - total * inv)
        for j in range(NT):
            if j % 2 == 0:
                yield
                ps[0], ps[4] = gate(ps[0], ALAG), gate(ps[4], ALAG)
            o = _chain(_add, [ps[w] * vbuf[j, ts, pl.ds(r0 - sh, 8), :]
                              for w, (ts, sh) in enumerate(src)]) * inv
            pin(o)
            put(qbuf.at[j, t, pl.ds(r0, 8), :], o)

    def out_operands(r, i, last):
        for j in range(4):
            a = [qbuf[j + o, b % 8, pl.ds(8 + 64 * lb + 16 * (b // 8), 16), :]
                 for b, lb in (out_rows(r, i, last), out_rows(r + 1, i, last)) for o in (0, 4)]
            a[0], a[3] = gate(a[0]), gate(a[3])
            for k, v in enumerate(_strassen_lhs(*a)):
                if k in (1, 4):
                    pin(v)
                obuf[r // 2, k, j, r16(i), :] = v.astype(BF16)
            if j < 3:
                yield

    def store_rows(b, lb):
        c, t = divmod(b, 8)
        for j in range(NT):
            words = pack(xres[b, j, r16(lb), :], xres[b + 1, j, r16(lb), :])
            pin(words)
            io32[j, lb, c, pl.ds(t // 2, 16, stride=4), :] = words

    unit_ticks = NT + 2 * XGAP
    step = 2
    out_ticks = 28

    def add_proj(sched, tick, c, lo, hi):
        jobs = [(b // step, b, n) for b in range(8 * c, 8 * c + 8, step) for n in range(lo, hi, step)]
        sched.add(tick, gemm(abuf32, wqkv32, jobs, qkv_sink))
        return tick + len(jobs) * out_ticks * step // NT

    def add_attention(sched, tick, pace, rows, last):
        units = [(r, i, half, h) for r in rows[::2] for i in range(4) for half in range(2) for h in range(2)]
        for n, (r, i, half, h) in enumerate(units):
            sched.add(tick + n * pace, attention(*out_rows(r + half, i, last), h))
            if half and h:
                sched.add(int(tick + n * pace) + unit_ticks, out_operands(r, i, last))

    def add_out(sched, tick, rows, last):
        jobs = [(r // 2, r, n) for r in rows[::2] for n in range(0, NT, 2)]
        sched.add(tick, gemm(obuf32, wo32, jobs, functools.partial(out_sink, last)))

    def add_tail(sched, tick, rows, last):
        ready = {}
        for i, r in enumerate(rows):
            t0 = tick + (i // 2 + 1) * out_ticks
            fast = i >= len(rows) - (2 if last else 4)
            if not last:
                t0 += 0 if fast else TOFF + i % 2 * out_ticks // 2
                ready[r % 8] = add_d_fwd(sched, t0, r, i % 2 if fast else out_ticks / 8)
            elif r % 2:
                c, p = r // 8, r % 8 // 2
                gap = 0 if fast else 3
                for j in range(4):
                    sched.add(t0 + (j + 1) * gap, _once(store_rows, *((r - 1, j) if c else (2 * j, p))))
                for lb in ([p] if c == 0 else range(4) if p == 3 else []):
                    sched.add(t0 + 5 * gap + 1, _once(start, out_copies(c, lb)))
        return ready

    q_ticks = 8 * out_ticks // step
    att_ticks = unit_ticks + 1 + 2
    order = [(a + 8) % NB for a in range(NB)]

    def add_attention_block(sched, cols, last):
        stats = {}
        t0 = max([add_d_inv(sched, 0, b, 0, stats, not last, cols) for b in range(step)])
        if not last:
            sched.add(cols[3] - KLEAD, _once(wait, qkv_copies(1) + dmat_cp))
            done = add_prep_wqkv(sched, cols[3] - KLEAD, 1, KPACE, [7] * 4)
            t0 = max(t0, done[0])
            assert all(d <= t0 + p * out_ticks / 4 for p, d in enumerate(done))
            sched.add(t0 + out_ticks, _once(wait, qkv_copies(2)))
            sched.add(t0 + out_ticks, _once(start, qkv_copies(0)))
            done = add_prep_wqkv(sched, t0 + out_ticks, 2, 2 * out_ticks - 6, [out_ticks - 4] * 4)
            assert all(d <= t0 + q_ticks + p * out_ticks for p, d in enumerate(done))
            sched.add(t0 + 2 * q_ticks, _once(wait, qkv_copies(0)))
            sched.add(t0 + 2 * q_ticks, _once(start, wo_copies))
            done = add_prep_wqkv(sched, t0 + 2 * q_ticks, 0, q_ticks - 10, [q_ticks / 4] * 4)
            assert done[-1] <= t0 + 4 * q_ticks
            sched.add(t0 + 8 * q_ticks, _once(wait, wo_copies))
            for i in range(32):
                sched.add(t0 + 8 * q_ticks + i * q_ticks / 16, _once(prep_wo, *divmod(i, 8)))
        tick, kv_start, q_start = t0, {}, {}
        for kind, c in ("k0", "k1", "q1", "k2", "q2", "k3", "q3", "q0"):
            if kind == "k":
                kv_start[int(c)] = tick
                if c == "0" and not last:
                    tick = add_proj(sched, tick, 0, NT, 2 * NT)
                    jobs = [(b // step, b, n) for n in range(2 * NT, 3 * NT, step) for b in range(0, 8, step)]
                    sched.add(tick, gemm(abuf32, wqkv32, jobs, qkv_sink))
                    tick += q_ticks
                    continue
                tick = add_proj(sched, tick, int(c), NT, 3 * NT)
            else:
                q_start[int(c)] = tick
                tick = add_proj(sched, tick, int(c), 0, NT)
        pace = 2 * out_ticks / step
        for b in range(step, NB):
            due = kv_start[b // 8] + (b % 8 // step) * (2 if last or b >= 8 else 1) * out_ticks
            gap = min(1 + (b - step) * 0.5, DGAP1 if last else DGAP0)
            pace = DPACE1 if last else DPACE0
            at = (b - step) * pace
            at = t0 + at + max(0, at - 4 * q_ticks - out_ticks) * DSLOW
            if not last and b < 8:
                at, gap = max(cols[3], t0 + (b // step - 1) * out_ticks - (step - b % step) * 8), 1
            end = add_d_inv(sched, at, b, gap, stats, not last)
            assert end <= due, (b, end, due)
        begin = [q_start[c] + out_ticks + 3 for c in (1, 2, 3)] + [tick + (ATT1 if last else ATT0)]
        begin.append(tick + (NB // step - 1) * out_ticks - att_ticks)
        for i, c in enumerate((1, 2, 3, 0)):
            pace = (begin[i + 1] - begin[i]) / 64
            assert begin[i] >= max(kv_start[c], kv_start[(c - 1) % 4]) + 2 * q_ticks
            for p in range(4):
                assert begin[i] + 16 * p * pace >= q_start[c] + (4 if last and c == 0 else p + 1) * out_ticks
                assert begin[i] + (16 * p + 15) * pace + att_ticks <= tick + (4 * i + p) * out_ticks + 1e-6
            add_attention(sched, begin[i], pace, range(8 * c, 8 * c + 8), last)
        add_out(sched, tick, order, last)
        return tick + (NB // step) * out_ticks, add_tail(sched, tick, order, last)

    def add_input(sched):
        ready = {}
        after = (x_copies(2), x_copies(3) + perm_cp + w_copies(0) + w_copies(1),
                 w_copies(2) + w_copies(3), w_copies(4))
        for c in range(NC):
            sched.add(c * 32, _once(wait, x_copies(c)))
            sched.add(c * 32, _once(start, after[c]))
            for t in range(8):
                ready[t] = add_d_fwd(sched, c * 32 + t * 4, c * 8 + t, 1, 2, True)
        return 128 + 9, ready

    def add_filter_prep(sched, tick):
        after = (w_copies(5) + w_copies(6), w_copies(7) + f256_cp + dmat_cp, qkv_copies(1), qkv_copies(2))
        begin = [F0 + g * (tick - F0) / 4 for g in range(4)] + [tick + FG * g for g in range(5)]
        for g in range(8):
            if g % 2 == 0:
                sched.add(begin[g], _once(wait, w_copies(g) + w_copies(g + 1) + ([] if g else perm_cp)))
                sched.add(begin[g], _once(start, after[g // 2]))
            for m in range(4):
                sched.add(begin[g] + m * (begin[g + 1] - begin[g]) / 4,
                          _once(prep_filter, g // 4, g % 4 * 4 + m))
        sched.add(begin[8] + 1, _once(wait, f256_cp))
        return begin[8] + 2

    sched = _Schedule()

    start(x_copies(0))
    for ref in (abuf32, obuf32, ubuf32, wo32, sfw32, siv32, wide32):
        put(ref.at[(0,) * (len(ref.shape) - 2) + (pl.ds(0, 8),)], jnp.zeros((8, 128), U32))
    make_wide()
    start(x_copies(1))
    for t in range(8):
        make_s_fwd(t)
    for e in range(4):
        make_s_inv(e)
    tick, ready = add_input(sched)
    cols = add_s_stage(sched, tick, ready, add_filter_prep(sched, tick))
    tick, ready = add_attention_block(sched, cols, False)
    cols = add_s_stage(sched, tick, ready, tick)
    add_attention_block(sched, cols, True)
    sched.run()
    for c in range(NC):
        for lb in range(4):
            wait(out_copies(c, lb))


@jax.jit
def pallas_interleave_layers__spectral_gfnet__sliding_local_dilated__prompt_kernel(
    A_x: jax.Array,
    A_w_r: jax.Array,
    A_w_i: jax.Array,
    B_x: jax.Array,
    B_wqkv: jax.Array,
    B_wo: jax.Array,
):
    del B_x
    assert A_x.shape == (1, S, D) and A_w_r.shape == (S, D // 2 + 1)
    cst = _constants()
    x = A_x.astype(BF16).reshape(4, NC, 128, D)
    wr, wi = A_w_r.astype(BF16).T, A_w_i.astype(BF16).T
    hbm = pl.BlockSpec(memory_space=pl.ANY)
    edge = pl.BlockSpec((16, S), lambda i: (D // 32, 0))
    vm = pltpu.VMEM
    out = pl.pallas_call(
        _kernel,
        grid=(1,),
        in_specs=[hbm, hbm, hbm, edge, edge, hbm, hbm, hbm, hbm,
                  pl.BlockSpec((24, 256), lambda i: (0, 0)),
                  pl.BlockSpec((2, 16, 128), lambda i: (0, 0, 0))],
        out_specs=hbm,
        out_shape=jax.ShapeDtypeStruct((4, NC, 128, D), BF16),
        scratch_shapes=[
            vm((NT, 4, NC, 128, 128), BF16),
            vm((17, 128, 128), BF16),
            vm((32, 128, 128), BF16),
            vm((32, 128, 128), BF16),
            vm((256, 512), BF16),
            vm((2, 16, 512, 128), BF16),
            vm((2, 4, 4, 8, 64, 128), F32),
            vm((3 * NT, D, 128), BF16),
            vm((NT, D // 2, 128), U32),
            vm((12, 7, 512, 128), BF16),
            vm((NT, D, 128), BF16),
            vm((4, 7, 512, 128), BF16),
            vm((NB, NT, 64, 128), F32),
            vm((4, 32, 64, 128), U32),
            vm((4, 32, 128, 128), F32),
            vm((NY, 8, 128, 128), F32),
            vm((NY, 8, 64, 128), U32),
            vm((RING, 8, 64, 128), BF16),
            vm((RING, 9, 64, 128), F32),
            vm((NB // 2, 7, 4, 64, 128), BF16),
            vm((NB // 2, 7, 4, 64, 128), BF16),
            vm((NT, 8, 264, 128), F32),
            vm((NT, 8, 264, 128), F32),
            vm((NT, 8, 264, 128), F32),
            vm((3, 256, 128), F32),
            vm((8, 256, 128), BF16),
            pltpu.SemaphoreType.DMA((NC,)),
            pltpu.SemaphoreType.DMA((3,)),
            pltpu.SemaphoreType.DMA((8,)),
            pltpu.SemaphoreType.DMA((3,)),
            pltpu.SemaphoreType.DMA(()),
            pltpu.SemaphoreType.DMA(()),
        ],
        compiler_params=pltpu.CompilerParams(
            dimension_semantics=("arbitrary",), vmem_limit_bytes=120 * 2**20),
    )(x, wr, wi, wr, wi, B_wqkv.astype(BF16), B_wo.astype(BF16),
      cst["small"], cst["f256"], cst["tw"], cst["d8"])
    return out.reshape(1, S, D)
```

```python
import functools

import jax
import jax.numpy as jnp
import numpy as np
from jax import lax
from jax.experimental import pallas as pl
from jax.experimental.pallas import tpu as pltpu

S, D = 2048, 1024
NT = D // 128
NC = 4
WIN = 8
HEAD_DIM = 32
EPS = 1e-5
F32, BF16, U32 = jnp.float32, jnp.bfloat16, jnp.uint32
PAIRS = ((0, 4), (1, 7), (2, 6), (3, 5))
RSQ2 = float(np.sqrt(0.5))
NB = S // 64

RING = 8
NY = 4
XGAP = 3
GLAG = 4
ALAG = 4
SGLAG = 3
SGLAG2 = 5
S_LAG = 3
F0 = 112
KLEAD = 52
KPACE = 48
DGAP0 = 4.75
DGAP1 = 4.2
DPACE0 = 20
DPACE1 = 15.5
DSLOW = 0.6
SYNC = 3
ILAG = 3
FG = 4
TOFF = 3
ATT0 = 25
ATT1 = 95


def _residues(r):
    return (0, 8) if r == 0 else (r, 16 - r)


def _d_matrices():
    n = np.arange(64)[:, None]
    a = np.arange(32)
    fwd = np.zeros((8, 128, 128))
    inv = np.zeros((8, 128, 128))
    for r in range(8):
        kd = np.concatenate([16 * a + p for p in _residues(r)])
        weight = np.full(64, 2.0)
        if r == 0:
            kd[0], weight[0] = D // 2, 1.0
            ph = np.exp(-2j * np.pi * n * kd[None, :] / D)
            sgn = np.where(kd % 16 == 0, 1.0, -1.0)[None, :]
            m = np.concatenate([ph, ph * sgn], axis=0)
            re, im = m.real.copy(), m.imag.copy()
            ire, iim = re.copy(), im.copy()
            im[:, 0] = 1.0
            iim[:, 0] = 1.0
        else:
            p = 12 if r == 4 else r
            ph = np.exp(-2j * np.pi * n * kd[None, :] / D)
            si = np.where(kd % 16 == p, 1.0, -1.0)[None, :]
            m = np.concatenate([ph, 1j * si * ph], axis=0)
            re, im = m.real, m.imag
            ire, iim = re, im
        swapped = r in (4, 7, 6, 5)
        cols = [im, re] if swapped else [re, im]
        icols = [iim * weight, ire * weight] if swapped else [ire * weight, iim * weight]
        fwd[r] = np.concatenate(cols, axis=1)
        inv[r] = np.concatenate(icols, axis=1).T / D
    return fwd, inv


def _side_matrices():
    l = np.arange(256)
    f = np.exp(-2j * np.pi * ((l[:, None] * l[None, :]) % 256) / 256)
    f256 = np.concatenate([f.real, f.imag], axis=1)
    t = np.arange(8)
    tw = np.exp(-2j * np.pi * t[:, None] * l[None, :] / S)
    tw = np.concatenate([tw.real, tw.imag, np.zeros((8, 256))], axis=0)
    g = np.exp(-2j * np.pi * t[:, None] * t[None, :] / 8)
    d8 = np.zeros((2, 16, 128))
    d8[0, :, :16] = np.block([[g.real, -g.imag], [g.imag, g.real]])
    d8[1, :, :16] = d8[0, :, :16].T / S
    return f256, tw, d8


def _filter_rows():
    p = np.zeros((1, 128, 128))
    for k in range(32):
        for e in range(4):
            p[0, e * 32 + k, 4 * k + e] = 1.0
    return p


@functools.lru_cache(maxsize=None)
def _constants():
    dfw, div = _d_matrices()
    f256, tw, d8 = _side_matrices()
    small = np.concatenate([dfw, div, _filter_rows()], axis=0)
    b = lambda x: np.asarray(x, np.float32).astype(BF16)
    return dict(small=b(small), f256=b(f256),
                tw=np.asarray(tw, np.float32), d8=b(d8))


def _dot(a, b):
    return jnp.dot(a, b, preferred_element_type=F32)


def _dot_nt(a, b):
    return lax.dot_general(a, b, (((1,), (1,)), ((), ())), preferred_element_type=F32)


def _tree(op, xs):
    xs = list(xs)
    while len(xs) > 1:
        xs = [op(xs[i], xs[i + 1]) if i + 1 < len(xs) else xs[i] for i in range(0, len(xs), 2)]
    return xs[0]


def _chain(op, xs):
    return functools.reduce(op, xs)


def _lane(rows):
    return lax.broadcasted_iota(jnp.int32, (rows, 128), 1)


def _swap(x):
    return pltpu.roll(x, 64, 1)


def _unpack(w, i):
    return pltpu.unpack_elementwise(w, index=i, packed_dtype=BF16, unpacked_dtype=F32)


def _latency():
    for _ in range(XGAP):
        yield


def _add(a, b):
    return a + b


def _row_mean(xs):
    return jnp.sum(_tree(_add, xs), axis=1, keepdims=True) * (1.0 / D)


def _twiddle16(r, x, y):
    lo = _lane(x.shape[0]) < 64
    wr, wi = float(np.cos(np.pi * r / 8)), float(-np.sin(np.pi * r / 8))
    cross = jnp.where(lo, 0.0, wr)
    return x * jnp.where(lo, 1.0, wi) + y * cross, y * jnp.where(lo, 1.0, -wi) + x * cross


def _d_butterfly_fwd(a, emit, pin, wide):
    s = [a[j] + a[j + 4] for j in range(4)]
    e, o = s[0] + s[2], s[1] + s[3]
    total, t4 = e + o, e - o
    emit(4, t4)
    d0, nd2 = a[0] - a[4], a[6] - a[2]
    d1, d3 = a[1] - a[5], a[3] - a[7]
    p, q = (d1 - d3) * RSQ2, (d1 + d3) * -RSQ2
    ts = {1: (d0 + p, q + nd2), 2: (s[0] - s[2], s[3] - s[1]), 3: (d0 - p, q - nd2)}
    mean8 = jnp.sum(total, axis=1, keepdims=True) * (1.0 / 128)
    if wide:
        for r, (tr, ti) in ts.items():
            emit(r, tr)
            emit(8 - r, ti)
    else:
        ab = {r: _twiddle16(r, *t) for r, t in ts.items()}
        ab = {r: (a, _swap(b)) for r, (a, b) in ab.items()}
    dev = _tree(_add, [v * v for t in ts.values() for v in t]) * 2.0 + t4 * t4
    pin(dev)
    yield from _latency()
    t0 = total - mean8
    emit(0, t0)
    var = jnp.sum(dev + t0 * t0, axis=1, keepdims=True) * (1.0 / (NT * D))
    if not wide:
        for r, (x, y) in ab.items():
            emit(r, x + y)
            emit(8 - r, x - y)
    yield from _latency()
    return lax.rsqrt(var + EPS)


def _d_butterfly_inv(u, pin, gate):
    ab = {r: (u[r] + u[8 - r], _swap(u[r] - u[8 - r])) for r in (1, 2, 3)}
    e, o = u[0] + u[4], u[0] - u[4]
    yield from _latency()
    ts = {r: _twiddle16(r, x, gate(y)) for r, (x, y) in ab.items()}
    pin(*[t[0] for t in ts.values()])
    yield
    s = [e + ts[2][0], o - ts[2][1], e - ts[2][0], o + ts[2][1]]
    p = (ts[1][0] - ts[3][0]) * RSQ2
    q = (ts[1][1] + ts[3][1]) * RSQ2
    d0, d1, d2, nd3 = ts[1][0] + ts[3][0], p - q, ts[3][1] - ts[1][1], p + q
    return [s[0] + d0, s[1] + d1, s[2] + d2, s[3] - nd3,
            s[0] - d0, s[1] - d1, s[2] - d2, s[3] + nd3]


def _strassen_lhs(a11, a12, a21, a22):
    return [a11 + a22, a21 + a22, a11, a22, a11 + a12, a21 - a11, a12 - a22]


def _strassen_rhs(b11, b12, b21, b22):
    return [b11 + b22, b11, b22 - b12, b11 - b21, b22, b11 + b12, b21 + b22]


def _cadd(a, b):
    return a[0] + b[0], a[1] + b[1]


def _csub(a, b):
    return a[0] - b[0], a[1] - b[1]


def _dft4(z, inverse):
    a, b = _cadd(z[0], z[2]), _csub(z[0], z[2])
    c, d = _cadd(z[1], z[3]), _csub(z[1], z[3])
    minus = (b[0] + d[1], b[1] - d[0])
    plus = (b[0] - d[1], b[1] + d[0])
    return [_cadd(a, c), plus if inverse else minus, _csub(a, c), minus if inverse else plus]


def _dft8(z, inverse):
    ev = _dft4(z[0::2], inverse)
    od = _dft4(z[1::2], inverse)
    out = [None] * 8
    out[0], out[4] = _cadd(ev[0], od[0]), _csub(ev[0], od[0])
    (er, ei), (x, y) = ev[2], od[2]
    minus, plus = (er + y, ei - x), (er - y, ei + x)
    out[2], out[6] = (plus, minus) if inverse else (minus, plus)
    for k in (1, 3):
        (er, ei), (x, y) = ev[k], od[k]
        sm, df = (x + y) * RSQ2, (x - y) * RSQ2
        if not inverse:
            if k == 1:
                out[1], out[5] = (er + sm, ei - df), (er - sm, ei + df)
            else:
                out[3], out[7] = (er - df, ei - sm), (er + df, ei + sm)
        else:
            if k == 1:
                out[1], out[5] = (er + df, ei + sm), (er - df, ei - sm)
            else:
                out[3], out[7] = (er - sm, ei + df), (er + sm, ei - df)
    return out


class _Schedule:
    def __init__(self):
        self.pending = []

    def add(self, tick, gen):
        self.pending.append((int(tick), len(self.pending), gen))

    def run(self):
        pending = sorted(self.pending, key=lambda p: p[:2])
        active, tick, i = [], 0, 0
        while active or i < len(pending):
            while i < len(pending) and pending[i][0] <= tick:
                active.append(pending[i][2])
                i += 1
            for g in list(active):
                if next(g, 0) == 0:
                    active.remove(g)
            tick += 1
        self.pending = []


def _once(fn, *args):
    fn(*args)
    return
    yield


def _kernel(x_hbm, wr_hbm, wi_hbm, wr_edge, wi_edge, wqkv_hbm, wo_hbm,
            small_hbm, f256_hbm, tw_ref, d8_ref,
            out_hbm,
            io, small, sfw, siv, f256, wraw, wf, wqkv_raw, wtmp, wqkv, wo_raw, wo,
            xres, zin, zout, ybuf, fbuf, ubuf, uout, abuf, obuf, qbuf, kbuf, vbuf, side,
            wide, sem_x, sem_c, sem_w, sem_qkv, sem_wo, sem_out):

    def x_copies(c):
        return [pltpu.make_async_copy(x_hbm.at[:, c, :, pl.ds(j * 128, 128)], io.at[j, :, c],
                                      sem_x.at[c]) for j in range(NT)]

    def out_copies(c, lb):
        return [pltpu.make_async_copy(io.at[j, lb, c], out_hbm.at[lb, c, :, pl.ds(j * 128, 128)],
                                      sem_out) for j in range(NT)]

    perm_cp, dmat_cp, f256_cp = ([pltpu.make_async_copy(s, d, sem_c.at[i])] for i, (s, d) in enumerate((
        (small_hbm.at[pl.ds(16, 1)], small.at[pl.ds(16, 1)]),
        (small_hbm.at[pl.ds(0, 16)], small.at[pl.ds(0, 16)]), (f256_hbm, f256))))

    def w_copies(g):
        src = (wr_hbm, wi_hbm)[g // 4]
        return [pltpu.make_async_copy(src.at[pl.ds(0, 512), pl.ds(m * 128, 128)], wraw.at[g // 4, m],
                                      sem_w.at[g]) for m in range(g % 4 * 4, g % 4 * 4 + 4)]

    def qkv_copies(g):
        return [pltpu.make_async_copy(wqkv_hbm.at[:, pl.ds(g * D + j * 128, 128)],
                                      wqkv_raw.at[g * NT + j], sem_qkv.at[g]) for j in range(NT)]

    wo_copies = [pltpu.make_async_copy(wo_hbm.at[:, pl.ds(j * 128, 128)], wo_raw.at[j], sem_wo)
                 for j in range(NT)]

    def start(cs):
        for cp in cs:
            cp.start()

    def wait(cs):
        for cp in cs:
            cp.wait()

    io32, wraw32, wo_raw32 = io.bitcast(U32), wraw.bitcast(U32), wo_raw.bitcast(U32)
    small32, sfw32, siv32, wide32 = (r.bitcast(U32) for r in (small, sfw, siv, wide))
    wqkv_raw32, wqkv32, wo32 = (r.bitcast(U32) for r in (wqkv_raw, wqkv, wo))
    ubuf32, abuf32, obuf32 = ubuf.bitcast(U32), abuf.bitcast(U32), obuf.bitcast(U32)

    never = tw_ref[16:24, 0:128] != 0.0
    never_wide = {n: jnp.concatenate([tw_ref[16:24, 0:128]] * n, axis=1) != 0.0 for n in (1, 2, 4)}
    token = {}

    def pin(*values):
        for v in values:
            key = v.shape[0], v.dtype == F32
            token[key] = (lax.max if key[1] else lax.bitwise_xor)(token[key], v) if key in token else v

    clock = []

    def gate(v, lag=GLAG):
        if len(clock) < lag:
            return v
        old = clock[-lag] if v.dtype == F32 else pltpu.bitcast(clock[-lag], v.dtype)
        if v.shape[0] == 8:
            return lax.select(never, old, v)
        return lax.concatenate([lax.select(never, old, v[0:8]), v[8:]], 0)

    def ticking(o):
        clock.append(o[0:8])
        del clock[:-16]
        return o

    def lhs(*tiles):
        if not token and len(tiles) == 4 and len(clock) >= SYNC:
            pin(clock[-SYNC])
        words = lax.concatenate(tiles, 1) if len(tiles) > 1 else tiles[0]
        if token:
            parts = [pltpu.bitcast(v, U32) if is_float else v for (_, is_float), v in token.items()]
            token.clear()
            w = _chain(lax.bitwise_xor, [v[i:i + 8] if v.shape[0] > 8 else v
                                         for v in parts for i in range(0, v.shape[0], 8)])
            w = lax.concatenate([w] * len(tiles), 1) if len(tiles) > 1 else w
            words = lax.concatenate([lax.select(never_wide[len(tiles)], w, words[0:8]), words[8:]], 0)
        return pltpu.bitcast(words, BF16)

    def bf(words):
        return pltpu.bitcast(words, BF16)

    def pack(a, b):
        return pltpu.bitcast(pltpu.pack_elementwise([a, b], packed_dtype=BF16), U32)

    def r16(i):
        return pl.ds(i * 16, 16)

    always = {}

    def put(ref, v):
        if v.shape not in always:
            always[v.shape] = jnp.ones(v.shape, jnp.bool_)
        pltpu.store(ref, v, mask=always[v.shape])

    def load_x(b, lb, from_input):
        if from_input:
            c, t = divmod(b, 8)
            return [_unpack(io32[j, lb, c, pl.ds(t // 2, 16, stride=4), :], t % 2) for j in range(NT)]
        return [xres[b, j, r16(lb), :] for j in range(NT)]

    def unit(p):
        angle = (((p + S // 2) & (S - 1)) - S // 2).astype(F32) * (2 * np.pi / S)
        return jnp.cos(angle), jnp.sin(angle)

    def times_row(a, b, i):
        br, bi = (jnp.broadcast_to(v[i:i + 1], (8, 128)) for v in b)
        return a[0] * br - a[1] * bi, a[0] * bi + a[1] * br

    def make_wide():
        row, lane = lax.broadcasted_iota(jnp.int32, (8, 128), 0), _lane(8)
        for ct, (ra, rb) in enumerate(PAIRS):
            res = _residues(ra) + _residues(rb)
            kd = (lane & 31) * 16 + _chain(
                _add, [jnp.where(lane >> 5 == g, p, 0) for g, p in enumerate(res)])
            if ct == 0:
                kd = jnp.where(lane == 0, D // 2, kd)
            fine, coarse = unit(-2 * row * kd), [unit(-16 * (row + 8 * h) * kd) for h in range(2)]
            for a in range(16):
                re, im = times_row(fine, coarse[a // 8], a % 8)
                if ct == 0:
                    even = kd & 7 == 0
                    top = jnp.where(even, re, 0.0), jnp.where(lane == 0, 1.0, jnp.where(even, im, 0.0))
                    bottom = jnp.where(even, 0.0, re), jnp.where(even, 0.0, im)
                else:
                    sign = jnp.where(kd & 7 == ra, 1.0, -1.0)
                    top, bottom = (re, im), (-sign * im, sign * re)
                for i in range(2):
                    wide[2 * ct + i, pl.ds(8 * a, 8), :] = top[i].astype(BF16)
                    wide[2 * ct + i, pl.ds(128 + 8 * a, 8), :] = bottom[i].astype(BF16)

    def make_s_fwd(t):
        row, lane = lax.broadcasted_iota(jnp.int32, (8, 128), 0), _lane(8)
        pos = 8 * (lane >> 1) + t
        fine = unit((lane & 1) * (S // 4) - 4 * row * pos)
        shift, coarse = unit(-row * pos), unit(-32 * row * pos)
        for e in range(4):
            base = times_row(fine, shift, e)
            for g in range(8):
                for i, v in enumerate(times_row(base, coarse, g)):
                    sfw[t * 4 + e, pl.ds(16 * g + 8 * i, 8), :] = v.astype(BF16)

    def make_s_inv(e):
        row, lane = lax.broadcasted_iota(jnp.int32, (8, 128), 0), _lane(8)
        freq = 4 * (lane >> 1) + e
        fine = [v * (1.0 / S) for v in unit((lane & 1) * (S // 4) + 8 * row * freq)]
        shift, coarse = unit(row * freq), unit(64 * row * freq)
        for t in range(8):
            base = times_row(fine, shift, t)
            for g in range(8):
                for i, v in enumerate(times_row(base, coarse, g)):
                    siv[t * 4 + e, pl.ds(64 * i + 8 * g, 8), :] = v.astype(BF16)

    def prep_filter(ri, m):
        sub = lax.broadcasted_iota(jnp.int32, (8, 128), 0)
        edge = (wr_edge, wi_edge)[ri]
        res = {}
        for i in range(8):
            words = wraw32[ri, m, pl.ds(i, 32, stride=8), :]
            res[2 * i], res[2 * i + 1] = _unpack(words, 0), _unpack(words, 1)
        first = res[0][0:8]
        dst = pl.ds((m % 2) * 16 + ri * 8, 8)
        prev = jnp.zeros((8, 128), F32) if m < 2 else side[1, dst, :]
        put(side.at[1, dst, :], jnp.where(sub == m // 2, jnp.broadcast_to(first[0:1], (8, 128)), prev))
        nyq = jnp.broadcast_to(edge[0:1, pl.ds(m * 128, 128)].astype(F32), (8, 128))
        res[0] = jnp.concatenate([jnp.where(sub == 0, nyq, first), res[0][8:]], axis=0)
        for ct, (ra, rb) in enumerate(PAIRS):
            blk = jnp.concatenate([res[p] for p in _residues(ra) + _residues(rb)], axis=0)
            o = _dot_nt(lhs(small32[16]), blk.astype(BF16))
            for e in range(4):
                put(wf.at[ri, ct, e, m // 2, pl.ds((m % 2) * 32, 32), :], o[e * 32:(e + 1) * 32])

    def shuffle(words, index):
        return jnp.take_along_axis(words, index, axis=1)

    def prep_wqkv_tile(g, i, part):
        lane = _lane(8)
        index = (lane & 3) * 32 + (((lane >> 2) - i) & 7) * 4 + (lane >> 5)
        rows = [pl.ds((part * 16 + r) * 8, 8) for r in range(16)]
        ws = [shuffle(gate(wqkv_raw32[g * NT + i, rs, :]), index) for rs in rows]
        yield from _latency()
        for rs, w in zip(rows, ws):
            pin(w)
            put(wtmp.at[i, rs, :], w)

    def prep_wqkv_cross(g, r):
        pos = (_lane(8) >> 2) & 7
        u = [wtmp[(-j) % 8, pl.ds(r * 8, 8), :] for j in range(NT)]
        u[0], u[4] = gate(u[0]), gate(u[4])
        for bit in range(3):
            m = ((pos >> bit) & 1) == 1
            u = [lax.select(m, u[(j - (1 << bit)) % 8], u[j]) for j in range(NT)]
        for j in range(NT):
            if j < 4:
                pin(u[j])
            put(wqkv_raw32.at[g * NT + j, pl.ds(r * 8, 8), :], u[j])

    def prep_wqkv_pair(g, p, part):
        lane = _lane(8)
        ws = {}
        for n in range(2):
            index = (lane & 96) | ((lane + 4 * (2 * p + n)) & 31)
            for half in range(2):
                for r in range(part * 2, part * 2 + 2):
                    w = gate(wqkv_raw32[g * NT + 2 * p + n, pl.ds(half * 256 + r * 8, 8), :])
                    ws[r, half, n] = shuffle(w, index) if p + n else w
        yield from _latency()
        for r in range(part * 2, part * 2 + 2):
            quad = [ws[r, half, n] for half in range(2) for n in range(2)]
            ops = [_strassen_rhs(*[_unpack(w, i) for w in quad]) for i in range(2)]
            for k in range(7):
                word = {1: quad[0], 4: quad[3]}.get(k)
                if word is None:
                    word = pack(ops[0][k], ops[1][k])
                if k in (2, 3):
                    pin(word)
                put(wqkv32.at[g * 4 + p, k, pl.ds(r * 8, 8), :], word)

    def add_prep_wqkv(sched, tick, g, ticks, pair_ticks):
        for i in range(32):
            sched.add(tick + i * ticks / 64, prep_wqkv_tile(g, *divmod(i, 4)))
        tick = int(tick + ticks / 2) + XGAP + 1
        for r in range(64):
            sched.add(tick + r * ticks / 128, _once(prep_wqkv_cross, g, r))
        tick = int(tick + ticks / 2) + 1
        done = []
        for p, n in enumerate(pair_ticks):
            for i in range(16):
                sched.add(tick + i * n / 16, prep_wqkv_pair(g, p, i))
            tick += n
            done.append(int(tick) + XGAP + 1)
        return done

    def prep_wo(p, dp):
        ws = [wo_raw32[2 * p + n, pl.ds(dp + off, 32, stride=16), :] for off in (0, 8) for n in (0, 1)]
        for i in range(2):
            b = [_unpack(w, i) for w in ws]
            r0 = (2 * dp + i) * 32
            for k, v in enumerate(_strassen_rhs(*b)):
                if k in (2, 3):
                    pin(v)
                wo[p, k, pl.ds(r0, 32), :] = v.astype(BF16)

    def ln_stats(xs):
        lane_mean = _tree(_add, xs) * (1.0 / NT)
        lane_m2 = _tree(_add, [jnp.square(x - lane_mean) for x in xs])
        pin(lane_m2)
        mean = jnp.sum(lane_mean, axis=1, keepdims=True) * (1.0 / 128)
        yield from _latency()
        m2 = lane_m2 + jnp.square(gate(lane_mean) - mean) * float(NT)
        pin(m2)
        var = jnp.sum(m2, axis=1, keepdims=True) * (1.0 / D)
        yield from _latency()
        return mean, lax.rsqrt(gate(jnp.broadcast_to(var, (16, 128))) + EPS)

    def d_fwd_rows(b, lb, from_input=False):
        xs = load_x(b, lb, from_input)

        def emit(r, v):
            if r % 4 == 0 or (r < 4 and not from_input):
                pin(v)
            ubuf[b % RING, r, r16(lb), :] = v.astype(BF16)

        xs[:4] = [gate(x, ILAG if from_input else GLAG) for x in xs[:4]]
        inv = yield from _d_butterfly_fwd(xs, emit, pin, from_input)
        inv = jnp.broadcast_to(inv, (16, 128))
        pin(inv)
        put(uout.at[b % RING, 8, r16(lb), :], inv)

    def d_dots(b, base, per_tick):
        for r in range(8):
            o = _dot(lhs(ubuf32[b % RING, r]), bf(small32[base + r]))
            put(uout.at[b % RING, r], o)
            if r % per_tick == per_tick - 1 and r < 7:
                yield

    def d_dots_wide(b):
        for ct, (ra, rb) in enumerate(PAIRS):
            u = lhs(ubuf32[b % RING, ra], ubuf32[b % RING, rb])
            for i, r in enumerate((ra, rb)):
                o = _dot(u, bf(wide32[2 * ct + i]))
                put(uout.at[b % RING, r], ticking(o) if i else o)
            if ct < 3:
                yield

    def d_fwd_cols(b, ct, is_wide):
        c, t = divmod(b, 8)
        ra, rb = PAIRS[ct]
        lane = _lane(16)
        lo = lane < 64
        z, x0 = [], []
        for lb in range(4):
            a, bb, inv = (uout[b % RING, r, r16(lb), :] for r in (ra, rb, 8))
            inv = gate(inv, ILAG if is_wide else GLAG)
            a, bb = a * inv, bb * inv
            if is_wide:
                if ct == 0:
                    x0.append(pltpu.roll(bb, t, 1) if t else bb)
                    bb = jnp.where(lane == 0, 0.0, bb)
                z.append((a, bb))
                continue
            if ct == 0:
                x0.append(pltpu.roll(a, (t + 64) % 128, 1))
                a = jnp.where(lane == 64, 0.0, a)
            im = lax.select(lo, bb, a)
            z.append((lax.select(lo, a, bb), _swap(im)))
        if not is_wide:
            yield from _latency()
        for e, (re, im) in enumerate(_dft4(z, False)):
            words = pack(re, im)
            if e < 2:
                pin(words)
            put(zin.at[ct, t * 4 + e, r16(c), :], words)
        if is_wide and ct == 0:
            yield from _latency()
        for lb, v in enumerate(x0):
            ls = pl.ds(64 * lb + 16 * c, 16)
            prev = jnp.zeros((16, 128), F32) if t == 0 else side[0, ls, :]
            v = jnp.where(lane == t, v, prev)
            pin(v)
            put(side.at[0, ls, :], v)

    def add_d_fwd(sched, tick, b, gap, per_tick=4, from_input=False):
        for lb in range(4):
            sched.add(tick + lb * gap, d_fwd_rows(b, lb, from_input))
        tick = int(tick + 3 * gap) + XGAP + 1
        sched.add(tick, d_dots_wide(b) if from_input else d_dots(b, 0, per_tick))
        for ct in range(4):
            sched.add(tick + 8 // per_tick + 3 + ct * gap, d_fwd_cols(b, ct, from_input))
        return int(tick + 8 // per_tick + 3 + 3 * gap) + XGAP + 1

    def side_path():
        vt = side[0].T[0:8]
        yield
        zero8 = jnp.zeros((8, 256), F32)
        u = _dot(jnp.concatenate([vt, zero8], axis=0).astype(BF16), f256[...])[0:8]
        twr, twi = tw_ref[0:8, :], tw_ref[8:16, :]
        ur, ui = u[:, 0:256], u[:, 256:512]
        pad = jnp.zeros((112, 256), BF16)
        for _ in range(4):
            yield
        uu = jnp.concatenate([ur * twr - ui * twi, ur * twi + ui * twr], axis=0).astype(BF16)
        xk = _dot(d8_ref[0], jnp.concatenate([uu, pad], axis=0))
        for _ in range(4):
            yield
        wr = jnp.concatenate([side[1, 0:8, :], side[1, 16:24, :]], axis=1)
        wi = jnp.concatenate([side[1, 8:16, :], side[1, 24:32, :]], axis=1)
        xr, xi = xk[0:8], xk[8:16]
        yy = jnp.concatenate([xr * wr - xi * wi, xr * wi + xi * wr], axis=0).astype(BF16)
        p = _dot(d8_ref[1], jnp.concatenate([yy, pad], axis=0))
        for _ in range(4):
            yield
        twr, twi = tw_ref[0:8, :], tw_ref[8:16, :]
        pr, pi = p[0:8], p[8:16]
        g = jnp.concatenate([pr * twr + pi * twi, pi * twr - pr * twi], axis=1)
        g = jnp.concatenate([g, jnp.zeros((8, 512), F32)], axis=0).astype(BF16)
        y0 = _dot_nt(g, f256[...])
        for _ in range(4):
            yield
        put(side.at[2], jnp.concatenate([y0, jnp.zeros((112, 256), F32)], axis=0).T)

    def s_fwd(u, t):
        ct, e = divmod(u, 4)
        put(ybuf.at[u % NY, t], ticking(_dot(lhs(sfw32[t * 4 + e]), bf(zin[ct, t * 4 + e]))))

    def s_filter(u, g):
        ct, e = divmod(u, 4)
        z = [tuple(ybuf[u % NY, t, pl.ds(g * 16 + i, 8), :] for i in (0, 8))
             for t in range(8)]
        lag = SGLAG if u * 8 + g < 122 - S_LAG else SGLAG2
        z[0], z[1] = [tuple(gate(v, lag) for v in zz) for zz in z[0:2]]
        xk = _dft8(z, False)
        for k2 in range(8):
            wr = wf[0, ct, e, k2, pl.ds(g * 8, 8), :]
            wi = wf[1, ct, e, k2, pl.ds(g * 8, 8), :]
            re, im = xk[k2]
            xk[k2] = (re * wr - im * wi, re * wi + im * wr)
        for t, (re, im) in enumerate(_dft8(xk, True)):
            words = pack(re, im)
            if t < 4:
                pin(words)
            put(fbuf.at[u % NY, t, pl.ds(g * 8, 8), :], words)

    def s_inv(u, t):
        ct, e = divmod(u, 4)
        o = _dot(lhs(siv32[t * 4 + e]), bf(fbuf[u % NY, t]))
        put(zout.at[ct, t * 4 + e], ticking(o) if u * 8 + t >= 110 - S_LAG else o)

    def add_s_stage(sched, early, ready, t1):
        ahead = 8 + S_LAG
        tick = early
        for t in sorted(range(8), key=lambda t: ready[t]):
            for i in range(t, ahead, 8):
                tick = max(tick + 0.5, ready[t])
                sched.add(tick, _once(s_fwd, i // 8, t))
        t1 = max(t1, int(tick) + 1)
        sched.add(max(max(ready), t1), side_path())
        for i in range(128):
            if i + ahead < 128:
                sched.add(t1 + i, _once(s_fwd, *divmod(i + ahead, 8)))
            sched.add(t1 + i, _once(s_filter, *divmod(i, 8)))
            sched.add(t1 + 9 + (i if i < 120 else 120 + (i - 120) // 4), _once(s_inv, *divmod(i, 8)))
        return [t1 + 32 * ct + 40 for ct in range(3)] + [t1 + 131]

    def d_inv_cols(b, ct):
        c, t = divmod(b, 8)
        ra, rb = PAIRS[ct]
        lane = _lane(16)
        lo = lane < 64
        u = [(zout[ct, t * 4 + e, r16(c), :], zout[ct, t * 4 + e, r16(4 + c), :]) for e in range(4)]
        u[0], u[1] = tuple(map(gate, u[0])), tuple(map(gate, u[1]))
        z = _dft4(u, True)
        z = [(re, _swap(im)) for re, im in z]
        if ct == 0:
            y0 = [pltpu.roll(side[2, pl.ds(64 * lb + 16 * c, 16), :], 64 - t, 1) for lb in range(4)]
        yield from _latency()
        for lb, (re, sw) in enumerate(z):
            sw = gate(sw)
            a, bb = lax.select(lo, re, sw), lax.select(lo, sw, re)
            if ct == 0:
                a = jnp.where(lane == 64, y0[lb], a)
            pin(a)
            ubuf[b % RING, ra, r16(lb), :] = a.astype(BF16)
            ubuf[b % RING, rb, r16(lb), :] = bb.astype(BF16)

    def d_inv_rows(b, lb, stats, first):
        u = [uout[b % RING, r, r16(lb), :] for r in range(8)]
        ys = yield from _d_butterfly_inv([gate(v) if r < 4 else v for r, v in enumerate(u)], pin, gate)
        xs = [x + y for x, y in zip(load_x(b, lb, first), ys)]
        for j in range(NT):
            put(xres.at[b, j, r16(lb), :], xs[j])
        stats[b, lb] = yield from ln_stats(xs)
        if b % 2:
            for j in range(4):
                a = [(xres[bb, j + o, r16(lb), :] - stats[bb, lb][0]) * stats[bb, lb][1]
                     for bb in (b - 1, b) for o in (0, 4)]
                a[0], a[3] = gate(a[0]), gate(a[3])
                for k, v in enumerate(_strassen_lhs(*a)):
                    if k in (1, 4):
                        pin(v)
                    abuf[b // 2, k, j, r16(lb), :] = v.astype(BF16)
                if j < 3:
                    yield

    def add_d_inv(sched, tick, b, gap, stats, first, cols=None):
        per_tick = 4
        cols = cols or [tick + ct * gap for ct in range(4)]
        for ct in range(4):
            sched.add(cols[ct], d_inv_cols(b, ct))
        tick = int(cols[3]) + XGAP + 1
        sched.add(tick, d_dots(b, 8, per_tick))
        tick += 8 // per_tick + 3
        for lb in range(4):
            sched.add(tick + lb * gap, d_inv_rows(b, lb, stats, first))
        return int(tick + 3 * gap) + 3 * XGAP + 1 + 4

    def gemm(lhs32, rhs32, jobs, sink):
        for slot, b, n in jobs:
            m = {}
            for k in (3, 1, 0, 6, 5, 4, 2):
                m[k] = ticking(_dot(lhs(*[lhs32[slot, k, j] for j in range(4)]), bf(rhs32[n // 2, k])))
                if k == 1:
                    sink(b + 1, n, m[1] - m[3])
                elif k == 0:
                    c11, c22 = m[3] - m[0], m[1] - m[0]
                elif k == 6:
                    c11 = m[6] - c11
                elif k == 5:
                    c22 = m[5] - c22
                elif k == 4:
                    sink(b, n, c11 - m[4])
                elif k == 2:
                    sink(b, n + 1, m[4] - m[2])
                    sink(b + 1, n + 1, c22 - m[2])
                yield

    def qkv_sink(b, n, o):
        c, t = divmod(b, 8)
        dst = (qbuf, kbuf, vbuf)[n // NT]
        for lb in range(4):
            put(dst.at[n % NT, t, pl.ds(8 + 64 * lb + 16 * c, 16), :], o[lb * 16:(lb + 1) * 16])
        if b == 0 and n >= NT:
            first = jnp.broadcast_to(o[0:1], (8, 128))
            for tt in range(8):
                dst[n % NT, tt, pl.ds(0, 8), :] = first

    def out_rows(r, i, last):
        c, t = divmod(r, 8)
        return (c * 8 + t % 2 * 4 + i, t // 2) if last and c == 0 else (r, i)

    def out_sink(last, r, n, o):
        for i in range(4):
            b, lb = out_rows(r, i, last)
            put(xres.at[b, n, r16(lb), :], xres[b, n, r16(lb), :] + o[i * 16:(i + 1) * 16])

    def attention(b, lb, h):
        c, t = divmod(b, 8)
        log2e = float(np.log2(np.e))
        scale = HEAD_DIM ** -0.5 * log2e
        r0 = 8 + 64 * lb + 16 * c + 8 * h
        src = [((t - 2 * w) % 8, -((t - 2 * w) // 8)) for w in range(WIN)]
        acc = [None] * WIN
        for j in range(NT):
            if j % 2 == 0:
                factor = gate(jnp.full((8, 128), scale, F32), ALAG)
            q = qbuf[j, t, pl.ds(r0, 8), :] * factor
            for w, (ts, sh) in enumerate(src):
                p = q * kbuf[j, ts, pl.ds(r0 - sh, 8), :]
                acc[w] = p if j == 0 else acc[w] + p
            if j % 2 and j < NT - 1:
                pin(*acc[j // 2 % 2::2])
                yield
        part = [(r, pltpu.roll(r, 64, 1)) for r in acc]
        yield from _latency()
        part = [r + rr for r, rr in part]
        part = [(r, pltpu.roll(r, 32, 1)) for r in part]
        yield from _latency()
        logits = [r + rr for r, rr in part]
        if r0 == 8:
            sub = lax.broadcasted_iota(jnp.int32, (8, 128), 0)
            logits = [jnp.where(sub >= sh, r, -1e9 * log2e) if sh else r
                      for r, (_, sh) in zip(logits, src)]
        logits[0] = gate(logits[0], ALAG)
        m = _tree(jnp.maximum, logits)
        ps = [jnp.exp2(r - m) for r in logits]
        total = _tree(_add, ps)
        pin(total)
        inv = pltpu.reciprocal(total, approx=True)
        inv = inv * (2.0 - total * inv)
        for j in range(NT):
            if j % 2 == 0:
                yield
                ps[0], ps[4] = gate(ps[0], ALAG), gate(ps[4], ALAG)
            o = _chain(_add, [ps[w] * vbuf[j, ts, pl.ds(r0 - sh, 8), :]
                              for w, (ts, sh) in enumerate(src)]) * inv
            if j % 2:
                pin(o)
            put(qbuf.at[j, t, pl.ds(r0, 8), :], o)

    def out_operands(r, i, last):
        for j in range(4):
            a = [qbuf[j + o, b % 8, pl.ds(8 + 64 * lb + 16 * (b // 8), 16), :]
                 for b, lb in (out_rows(r, i, last), out_rows(r + 1, i, last)) for o in (0, 4)]
            a[0], a[3] = gate(a[0]), gate(a[3])
            for k, v in enumerate(_strassen_lhs(*a)):
                if k in (1, 4):
                    pin(v)
                obuf[r // 2, k, j, r16(i), :] = v.astype(BF16)
            if j < 3:
                yield

    def store_rows(b, lb):
        c, t = divmod(b, 8)
        for j in range(NT):
            words = pack(xres[b, j, r16(lb), :], xres[b + 1, j, r16(lb), :])
            pin(words)
            io32[j, lb, c, pl.ds(t // 2, 16, stride=4), :] = words

    unit_ticks = NT + 2 * XGAP
    step = 2
    out_ticks = 28

    def add_proj(sched, tick, c, lo, hi):
        jobs = [(b // step, b, n) for b in range(8 * c, 8 * c + 8, step) for n in range(lo, hi, step)]
        sched.add(tick, gemm(abuf32, wqkv32, jobs, qkv_sink))
        return tick + len(jobs) * out_ticks * step // NT

    def add_attention(sched, tick, pace, rows, last):
        units = [(r, i, half, h) for r in rows[::2] for i in range(4) for half in range(2) for h in range(2)]
        for n, (r, i, half, h) in enumerate(units):
            sched.add(tick + n * pace, attention(*out_rows(r + half, i, last), h))
            if half and h:
                sched.add(int(tick + n * pace) + unit_ticks, out_operands(r, i, last))

    def add_out(sched, tick, rows, last):
        jobs = [(r // 2, r, n) for r in rows[::2] for n in range(0, NT, 2)]
        sched.add(tick, gemm(obuf32, wo32, jobs, functools.partial(out_sink, last)))

    def add_tail(sched, tick, rows, last):
        ready = {}
        for i, r in enumerate(rows):
            t0 = tick + (i // 2 + 1) * out_ticks
            fast = i >= len(rows) - (2 if last else 4)
            if not last:
                t0 += 0 if fast else TOFF + i % 2 * out_ticks // 2
                ready[r % 8] = add_d_fwd(sched, t0, r, i % 2 if fast else out_ticks / 8)
            elif r % 2:
                c, p = r // 8, r % 8 // 2
                gap = 0 if fast else 3
                for j in range(4):
                    sched.add(t0 + (j + 1) * gap, _once(store_rows, *((r - 1, j) if c else (2 * j, p))))
                for lb in ([p] if c == 0 else range(4) if p == 3 else []):
                    sched.add(t0 + 5 * gap + 1, _once(start, out_copies(c, lb)))
        return ready

    q_ticks = 8 * out_ticks // step
    att_ticks = unit_ticks + 1 + 2
    order = [(a + 8) % NB for a in range(NB)]

    def add_attention_block(sched, cols, last):
        stats = {}
        t0 = max([add_d_inv(sched, 0, b, 0, stats, not last, cols) for b in range(step)])
        if not last:
            sched.add(cols[3] - KLEAD, _once(wait, qkv_copies(1) + dmat_cp))
            done = add_prep_wqkv(sched, cols[3] - KLEAD, 1, KPACE, [7] * 4)
            t0 = max(t0, done[0])
            assert all(d <= t0 + p * out_ticks / 4 for p, d in enumerate(done))
            sched.add(t0 + out_ticks, _once(wait, qkv_copies(2)))
            sched.add(t0 + out_ticks, _once(start, qkv_copies(0)))
            done = add_prep_wqkv(sched, t0 + out_ticks, 2, 2 * out_ticks - 6, [out_ticks - 4] * 4)
            assert all(d <= t0 + q_ticks + p * out_ticks for p, d in enumerate(done))
            sched.add(t0 + 2 * q_ticks, _once(wait, qkv_copies(0)))
            sched.add(t0 + 2 * q_ticks, _once(start, wo_copies))
            done = add_prep_wqkv(sched, t0 + 2 * q_ticks, 0, q_ticks - 10, [q_ticks / 4] * 4)
            assert done[-1] <= t0 + 4 * q_ticks
            sched.add(t0 + 8 * q_ticks, _once(wait, wo_copies))
            for i in range(32):
                sched.add(t0 + 8 * q_ticks + i * q_ticks / 16, _once(prep_wo, *divmod(i, 8)))
        tick, kv_start, q_start = t0, {}, {}
        for kind, c in ("k0", "k1", "q1", "k2", "q2", "k3", "q3", "q0"):
            if kind == "k":
                kv_start[int(c)] = tick
                if c == "0" and not last:
                    tick = add_proj(sched, tick, 0, NT, 2 * NT)
                    jobs = [(b // step, b, n) for n in range(2 * NT, 3 * NT, step) for b in range(0, 8, step)]
                    sched.add(tick, gemm(abuf32, wqkv32, jobs, qkv_sink))
                    tick += q_ticks
                    continue
                tick = add_proj(sched, tick, int(c), NT, 3 * NT)
            else:
                q_start[int(c)] = tick
                tick = add_proj(sched, tick, int(c), 0, NT)
        pace = 2 * out_ticks / step
        for b in range(step, NB):
            due = kv_start[b // 8] + (b % 8 // step) * (2 if last or b >= 8 else 1) * out_ticks
            gap = min(1 + (b - step) * 0.5, DGAP1 if last else DGAP0)
            pace = DPACE1 if last else DPACE0
            at = (b - step) * pace
            at = t0 + at + max(0, at - 4 * q_ticks - out_ticks) * DSLOW
            if not last and b < 8:
                at, gap = max(cols[3], t0 + (b // step - 1) * out_ticks - (step - b % step) * 8), 1
            end = add_d_inv(sched, at, b, gap, stats, not last)
            assert end <= due, (b, end, due)
        begin = [q_start[c] + out_ticks + 3 for c in (1, 2, 3)] + [tick + (ATT1 if last else ATT0)]
        begin.append(tick + (NB // step - 1) * out_ticks - att_ticks)
        for i, c in enumerate((1, 2, 3, 0)):
            pace = (begin[i + 1] - begin[i]) / 64
            assert begin[i] >= max(kv_start[c], kv_start[(c - 1) % 4]) + 2 * q_ticks
            for p in range(4):
                assert begin[i] + 16 * p * pace >= q_start[c] + (4 if last and c == 0 else p + 1) * out_ticks
                assert begin[i] + (16 * p + 15) * pace + att_ticks <= tick + (4 * i + p) * out_ticks + 1e-6
            add_attention(sched, begin[i], pace, range(8 * c, 8 * c + 8), last)
        add_out(sched, tick, order, last)
        return tick + (NB // step) * out_ticks, add_tail(sched, tick, order, last)

    def add_input(sched):
        ready = {}
        after = (x_copies(2), x_copies(3) + perm_cp + w_copies(0) + w_copies(1),
                 w_copies(2) + w_copies(3), w_copies(4))
        for c in range(NC):
            sched.add(c * 32, _once(wait, x_copies(c)))
            sched.add(c * 32, _once(start, after[c]))
            for t in range(8):
                ready[t] = add_d_fwd(sched, c * 32 + t * 4, c * 8 + t, 1, 2, True)
        return 128 + 9, ready

    def add_filter_prep(sched, tick):
        after = (w_copies(5) + w_copies(6), w_copies(7) + f256_cp + dmat_cp, qkv_copies(1), qkv_copies(2))
        begin = [F0 + g * (tick - F0) / 4 for g in range(4)] + [tick + FG * g for g in range(5)]
        for g in range(8):
            if g % 2 == 0:
                sched.add(begin[g], _once(wait, w_copies(g) + w_copies(g + 1) + ([] if g else perm_cp)))
                sched.add(begin[g], _once(start, after[g // 2]))
            for m in range(4):
                sched.add(begin[g] + m * (begin[g + 1] - begin[g]) / 4,
                          _once(prep_filter, g // 4, g % 4 * 4 + m))
        sched.add(begin[8] + 1, _once(wait, f256_cp))
        return begin[8] + 2

    sched = _Schedule()

    start(x_copies(0))
    for ref in (abuf32, obuf32, ubuf32, wo32, sfw32, siv32, wide32):
        put(ref.at[(0,) * (len(ref.shape) - 2) + (pl.ds(0, 8),)], jnp.zeros((8, 128), U32))
    make_wide()
    start(x_copies(1))
    for t in range(8):
        make_s_fwd(t)
    for e in range(4):
        make_s_inv(e)
    tick, ready = add_input(sched)
    cols = add_s_stage(sched, tick, ready, add_filter_prep(sched, tick))
    tick, ready = add_attention_block(sched, cols, False)
    cols = add_s_stage(sched, tick, ready, tick)
    add_attention_block(sched, cols, True)
    sched.run()
    for c in range(NC):
        for lb in range(4):
            wait(out_copies(c, lb))


@jax.jit
def pallas_interleave_layers__spectral_gfnet__sliding_local_dilated__prompt_kernel(
    A_x: jax.Array,
    A_w_r: jax.Array,
    A_w_i: jax.Array,
    B_x: jax.Array,
    B_wqkv: jax.Array,
    B_wo: jax.Array,
):
    del B_x
    assert A_x.shape == (1, S, D) and A_w_r.shape == (S, D // 2 + 1)
    cst = _constants()
    x = A_x.astype(BF16).reshape(4, NC, 128, D)
    wr, wi = A_w_r.astype(BF16).T, A_w_i.astype(BF16).T
    hbm = pl.BlockSpec(memory_space=pl.ANY)
    edge = pl.BlockSpec((16, S), lambda i: (D // 32, 0))
    vm = pltpu.VMEM
    out = pl.pallas_call(
        _kernel,
        grid=(1,),
        in_specs=[hbm, hbm, hbm, edge, edge, hbm, hbm, hbm, hbm,
                  pl.BlockSpec((24, 256), lambda i: (0, 0)),
                  pl.BlockSpec((2, 16, 128), lambda i: (0, 0, 0))],
        out_specs=hbm,
        out_shape=jax.ShapeDtypeStruct((4, NC, 128, D), BF16),
        scratch_shapes=[
            vm((NT, 4, NC, 128, 128), BF16),
            vm((17, 128, 128), BF16),
            vm((32, 128, 128), BF16),
            vm((32, 128, 128), BF16),
            vm((256, 512), BF16),
            vm((2, 16, 512, 128), BF16),
            vm((2, 4, 4, 8, 64, 128), F32),
            vm((3 * NT, D, 128), BF16),
            vm((NT, D // 2, 128), U32),
            vm((12, 7, 512, 128), BF16),
            vm((NT, D, 128), BF16),
            vm((4, 7, 512, 128), BF16),
            vm((NB, NT, 64, 128), F32),
            vm((4, 32, 64, 128), U32),
            vm((4, 32, 128, 128), F32),
            vm((NY, 8, 128, 128), F32),
            vm((NY, 8, 64, 128), U32),
            vm((RING, 8, 64, 128), BF16),
            vm((RING, 9, 64, 128), F32),
            vm((NB // 2, 7, 4, 64, 128), BF16),
            vm((NB // 2, 7, 4, 64, 128), BF16),
            vm((NT, 8, 264, 128), F32),
            vm((NT, 8, 264, 128), F32),
            vm((NT, 8, 264, 128), F32),
            vm((3, 256, 128), F32),
            vm((8, 256, 128), BF16),
            pltpu.SemaphoreType.DMA((NC,)),
            pltpu.SemaphoreType.DMA((3,)),
            pltpu.SemaphoreType.DMA((8,)),
            pltpu.SemaphoreType.DMA((3,)),
            pltpu.SemaphoreType.DMA(()),
            pltpu.SemaphoreType.DMA(()),
        ],
        compiler_params=pltpu.CompilerParams(
            dimension_semantics=("arbitrary",), vmem_limit_bytes=120 * 2**20),
    )(x, wr, wi, wr, wi, B_wqkv.astype(BF16), B_wo.astype(BF16),
      cst["small"], cst["f256"], cst["tw"], cst["d8"])
    return out.reshape(1, S, D)
```

```python
import functools

import jax
import jax.numpy as jnp
import numpy as np
from jax import lax
from jax.experimental import pallas as pl
from jax.experimental.pallas import tpu as pltpu

S, D = 2048, 1024
NT = D // 128
NC = 4
WIN = 8
HEAD_DIM = 32
EPS = 1e-5
F32, BF16, U32 = jnp.float32, jnp.bfloat16, jnp.uint32
PAIRS = ((0, 4), (1, 7), (2, 6), (3, 5))
RSQ2 = float(np.sqrt(0.5))
NB = S // 64

RING = 8
NY = 4
XGAP = 3
GLAG = 4
ALAG = 4
SGLAG = 3
SGLAG2 = 5
S_LAG = 3
F0 = 112
KLEAD = 56
KPACE = 36
DGAP0 = 4.75
DGAP1 = 4.2
DPACE0 = 20
DPACE1 = 15.5
DSLOW = 0.6
SYNC = 3
ILAG = 3
FG = 4
TOFF = 3
ATT0 = 25
ATT1 = 95


def _residues(r):
    return (0, 8) if r == 0 else (r, 16 - r)


def _d_matrices():
    n = np.arange(64)[:, None]
    a = np.arange(32)
    fwd = np.zeros((8, 128, 128))
    inv = np.zeros((8, 128, 128))
    for r in range(8):
        kd = np.concatenate([16 * a + p for p in _residues(r)])
        weight = np.full(64, 2.0)
        if r == 0:
            kd[0], weight[0] = D // 2, 1.0
            ph = np.exp(-2j * np.pi * n * kd[None, :] / D)
            sgn = np.where(kd % 16 == 0, 1.0, -1.0)[None, :]
            m = np.concatenate([ph, ph * sgn], axis=0)
            re, im = m.real.copy(), m.imag.copy()
            ire, iim = re.copy(), im.copy()
            im[:, 0] = 1.0
            iim[:, 0] = 1.0
        else:
            p = 12 if r == 4 else r
            ph = np.exp(-2j * np.pi * n * kd[None, :] / D)
            si = np.where(kd % 16 == p, 1.0, -1.0)[None, :]
            m = np.concatenate([ph, 1j * si * ph], axis=0)
            re, im = m.real, m.imag
            ire, iim = re, im
        swapped = r in (4, 7, 6, 5)
        cols = [im, re] if swapped else [re, im]
        icols = [iim * weight, ire * weight] if swapped else [ire * weight, iim * weight]
        fwd[r] = np.concatenate(cols, axis=1)
        inv[r] = np.concatenate(icols, axis=1).T / D
    return fwd, inv


def _side_matrices():
    l = np.arange(256)
    f = np.exp(-2j * np.pi * ((l[:, None] * l[None, :]) % 256) / 256)
    f256 = np.concatenate([f.real, f.imag], axis=1)
    t = np.arange(8)
    tw = np.exp(-2j * np.pi * t[:, None] * l[None, :] / S)
    tw = np.concatenate([tw.real, tw.imag, np.zeros((8, 256))], axis=0)
    g = np.exp(-2j * np.pi * t[:, None] * t[None, :] / 8)
    d8 = np.zeros((2, 16, 128))
    d8[0, :, :16] = np.block([[g.real, -g.imag], [g.imag, g.real]])
    d8[1, :, :16] = d8[0, :, :16].T / S
    return f256, tw, d8


def _filter_rows():
    p = np.zeros((1, 128, 128))
    for k in range(32):
        for e in range(4):
            p[0, e * 32 + k, 4 * k + e] = 1.0
    return p


@functools.lru_cache(maxsize=None)
def _constants():
    dfw, div = _d_matrices()
    f256, tw, d8 = _side_matrices()
    small = np.concatenate([dfw, div, _filter_rows()], axis=0)
    b = lambda x: np.asarray(x, np.float32).astype(BF16)
    return dict(small=b(small), f256=b(f256),
                tw=np.asarray(tw, np.float32), d8=b(d8))


def _dot(a, b):
    return jnp.dot(a, b, preferred_element_type=F32)


def _dot_nt(a, b):
    return lax.dot_general(a, b, (((1,), (1,)), ((), ())), preferred_element_type=F32)


def _tree(op, xs):
    xs = list(xs)
    while len(xs) > 1:
        xs = [op(xs[i], xs[i + 1]) if i + 1 < len(xs) else xs[i] for i in range(0, len(xs), 2)]
    return xs[0]


def _chain(op, xs):
    return functools.reduce(op, xs)


def _lane(rows):
    return lax.broadcasted_iota(jnp.int32, (rows, 128), 1)


def _swap(x):
    return pltpu.roll(x, 64, 1)


def _unpack(w, i):
    return pltpu.unpack_elementwise(w, index=i, packed_dtype=BF16, unpacked_dtype=F32)


def _latency():
    for _ in range(XGAP):
        yield


def _add(a, b):
    return a + b


def _row_mean(xs):
    return jnp.sum(_tree(_add, xs), axis=1, keepdims=True) * (1.0 / D)


def _twiddle16(r, x, y):
    lo = _lane(x.shape[0]) < 64
    wr, wi = float(np.cos(np.pi * r / 8)), float(-np.sin(np.pi * r / 8))
    cross = jnp.where(lo, 0.0, wr)
    return x * jnp.where(lo, 1.0, wi) + y * cross, y * jnp.where(lo, 1.0, -wi) + x * cross


def _d_butterfly_fwd(a, emit, pin, wide):
    s = [a[j] + a[j + 4] for j in range(4)]
    e, o = s[0] + s[2], s[1] + s[3]
    total, t4 = e + o, e - o
    emit(4, t4)
    d0, nd2 = a[0] - a[4], a[6] - a[2]
    d1, d3 = a[1] - a[5], a[3] - a[7]
    p, q = (d1 - d3) * RSQ2, (d1 + d3) * -RSQ2
    ts = {1: (d0 + p, q + nd2), 2: (s[0] - s[2], s[3] - s[1]), 3: (d0 - p, q - nd2)}
    mean8 = jnp.sum(total, axis=1, keepdims=True) * (1.0 / 128)
    if wide:
        for r, (tr, ti) in ts.items():
            emit(r, tr)
            emit(8 - r, ti)
    else:
        ab = {r: _twiddle16(r, *t) for r, t in ts.items()}
        ab = {r: (a, _swap(b)) for r, (a, b) in ab.items()}
    dev = _tree(_add, [v * v for t in ts.values() for v in t]) * 2.0 + t4 * t4
    pin(dev)
    yield from _latency()
    t0 = total - mean8
    emit(0, t0)
    var = jnp.sum(dev + t0 * t0, axis=1, keepdims=True) * (1.0 / (NT * D))
    if not wide:
        for r, (x, y) in ab.items():
            emit(r, x + y)
            emit(8 - r, x - y)
    yield from _latency()
    return lax.rsqrt(var + EPS)


def _d_butterfly_inv(u, pin, gate):
    ab = {r: (u[r] + u[8 - r], _swap(u[r] - u[8 - r])) for r in (1, 2, 3)}
    e, o = u[0] + u[4], u[0] - u[4]
    yield from _latency()
    ts = {r: _twiddle16(r, x, gate(y)) for r, (x, y) in ab.items()}
    pin(*[t[0] for t in ts.values()])
    yield
    s = [e + ts[2][0], o - ts[2][1], e - ts[2][0], o + ts[2][1]]
    p = (ts[1][0] - ts[3][0]) * RSQ2
    q = (ts[1][1] + ts[3][1]) * RSQ2
    d0, d1, d2, nd3 = ts[1][0] + ts[3][0], p - q, ts[3][1] - ts[1][1], p + q
    return [s[0] + d0, s[1] + d1, s[2] + d2, s[3] - nd3,
            s[0] - d0, s[1] - d1, s[2] - d2, s[3] + nd3]


def _strassen_lhs(a11, a12, a21, a22):
    return [a11 + a22, a21 + a22, a11, a22, a11 + a12, a21 - a11, a12 - a22]


def _strassen_rhs(b11, b12, b21, b22):
    return [b11 + b22, b11, b22 - b12, b11 - b21, b22, b11 + b12, b21 + b22]


def _cadd(a, b):
    return a[0] + b[0], a[1] + b[1]


def _csub(a, b):
    return a[0] - b[0], a[1] - b[1]


def _dft4(z, inverse):
    a, b = _cadd(z[0], z[2]), _csub(z[0], z[2])
    c, d = _cadd(z[1], z[3]), _csub(z[1], z[3])
    minus = (b[0] + d[1], b[1] - d[0])
    plus = (b[0] - d[1], b[1] + d[0])
    return [_cadd(a, c), plus if inverse else minus, _csub(a, c), minus if inverse else plus]


def _dft8(z, inverse):
    ev = _dft4(z[0::2], inverse)
    od = _dft4(z[1::2], inverse)
    out = [None] * 8
    out[0], out[4] = _cadd(ev[0], od[0]), _csub(ev[0], od[0])
    (er, ei), (x, y) = ev[2], od[2]
    minus, plus = (er + y, ei - x), (er - y, ei + x)
    out[2], out[6] = (plus, minus) if inverse else (minus, plus)
    for k in (1, 3):
        (er, ei), (x, y) = ev[k], od[k]
        sm, df = (x + y) * RSQ2, (x - y) * RSQ2
        if not inverse:
            if k == 1:
                out[1], out[5] = (er + sm, ei - df), (er - sm, ei + df)
            else:
                out[3], out[7] = (er - df, ei - sm), (er + df, ei + sm)
        else:
            if k == 1:
                out[1], out[5] = (er + df, ei + sm), (er - df, ei - sm)
            else:
                out[3], out[7] = (er - sm, ei + df), (er + sm, ei - df)
    return out


class _Schedule:
    def __init__(self):
        self.pending = []

    def add(self, tick, gen):
        self.pending.append((int(tick), len(self.pending), gen))

    def run(self):
        pending = sorted(self.pending, key=lambda p: p[:2])
        active, tick, i = [], 0, 0
        while active or i < len(pending):
            while i < len(pending) and pending[i][0] <= tick:
                active.append(pending[i][2])
                i += 1
            for g in list(active):
                if next(g, 0) == 0:
                    active.remove(g)
            tick += 1
        self.pending = []


def _once(fn, *args):
    fn(*args)
    return
    yield


def _kernel(x_hbm, wr_hbm, wi_hbm, wr_edge, wi_edge, wqkv_hbm, wo_hbm,
            small_hbm, f256_hbm, tw_ref, d8_ref,
            out_hbm,
            io, small, sfw, siv, f256, wraw, wf, wqkv_raw, wtmp, wqkv, wo_raw, wo,
            xres, zin, zout, ybuf, fbuf, ubuf, uout, abuf, obuf, qbuf, kbuf, vbuf, side,
            wide, sem_x, sem_c, sem_w, sem_qkv, sem_wo, sem_out):

    def x_copies(c):
        return [pltpu.make_async_copy(x_hbm.at[:, c, :, pl.ds(j * 128, 128)], io.at[j, :, c],
                                      sem_x.at[c]) for j in range(NT)]

    def out_copies(c, lb):
        return [pltpu.make_async_copy(io.at[j, lb, c], out_hbm.at[lb, c, :, pl.ds(j * 128, 128)],
                                      sem_out) for j in range(NT)]

    perm_cp, dmat_cp, f256_cp = ([pltpu.make_async_copy(s, d, sem_c.at[i])] for i, (s, d) in enumerate((
        (small_hbm.at[pl.ds(16, 1)], small.at[pl.ds(16, 1)]),
        (small_hbm.at[pl.ds(0, 16)], small.at[pl.ds(0, 16)]), (f256_hbm, f256))))

    def w_copies(g):
        src = (wr_hbm, wi_hbm)[g // 4]
        return [pltpu.make_async_copy(src.at[pl.ds(0, 512), pl.ds(m * 128, 128)], wraw.at[g // 4, m],
                                      sem_w.at[g]) for m in range(g % 4 * 4, g % 4 * 4 + 4)]

    def qkv_copies(g):
        return [pltpu.make_async_copy(wqkv_hbm.at[:, pl.ds(g * D + j * 128, 128)],
                                      wqkv_raw.at[g * NT + j], sem_qkv.at[g]) for j in range(NT)]

    wo_copies = [pltpu.make_async_copy(wo_hbm.at[:, pl.ds(j * 128, 128)], wo_raw.at[j], sem_wo)
                 for j in range(NT)]

    def start(cs):
        for cp in cs:
            cp.start()

    def wait(cs):
        for cp in cs:
            cp.wait()

    io32, wraw32, wo_raw32 = io.bitcast(U32), wraw.bitcast(U32), wo_raw.bitcast(U32)
    small32, sfw32, siv32, wide32 = (r.bitcast(U32) for r in (small, sfw, siv, wide))
    wqkv_raw32, wqkv32, wo32 = (r.bitcast(U32) for r in (wqkv_raw, wqkv, wo))
    ubuf32, abuf32, obuf32 = ubuf.bitcast(U32), abuf.bitcast(U32), obuf.bitcast(U32)

    never = tw_ref[16:24, 0:128] != 0.0
    never_wide = {n: jnp.concatenate([tw_ref[16:24, 0:128]] * n, axis=1) != 0.0 for n in (1, 2, 4)}
    token = {}

    def pin(*values):
        for v in values:
            key = v.shape[0], v.dtype == F32
            token[key] = (lax.max if key[1] else lax.bitwise_xor)(token[key], v) if key in token else v

    clock = []

    def gate(v, lag=GLAG):
        if len(clock) < lag:
            return v
        old = clock[-lag] if v.dtype == F32 else pltpu.bitcast(clock[-lag], v.dtype)
        if v.shape[0] == 8:
            return lax.select(never, old, v)
        return lax.concatenate([lax.select(never, old, v[0:8]), v[8:]], 0)

    def ticking(o):
        clock.append(o[0:8])
        del clock[:-16]
        return o

    def lhs(*tiles):
        if not token and len(tiles) == 4 and len(clock) >= SYNC:
            pin(clock[-SYNC])
        words = lax.concatenate(tiles, 1) if len(tiles) > 1 else tiles[0]
        if token:
            parts = [pltpu.bitcast(v, U32) if is_float else v for (_, is_float), v in token.items()]
            token.clear()
            w = _chain(lax.bitwise_xor, [v[i:i + 8] if v.shape[0] > 8 else v
                                         for v in parts for i in range(0, v.shape[0], 8)])
            w = lax.concatenate([w] * len(tiles), 1) if len(tiles) > 1 else w
            words = lax.concatenate([lax.select(never_wide[len(tiles)], w, words[0:8]), words[8:]], 0)
        return pltpu.bitcast(words, BF16)

    def bf(words):
        return pltpu.bitcast(words, BF16)

    def pack(a, b):
        return pltpu.bitcast(pltpu.pack_elementwise([a, b], packed_dtype=BF16), U32)

    def r16(i):
        return pl.ds(i * 16, 16)

    always = {}

    def put(ref, v):
        if v.shape not in always:
            always[v.shape] = jnp.ones(v.shape, jnp.bool_)
        pltpu.store(ref, v, mask=always[v.shape])

    def load_x(b, lb, from_input):
        if from_input:
            c, t = divmod(b, 8)
            return [_unpack(io32[j, lb, c, pl.ds(t // 2, 16, stride=4), :], t % 2) for j in range(NT)]
        return [xres[b, j, r16(lb), :] for j in range(NT)]

    def unit(p):
        angle = (((p + S // 2) & (S - 1)) - S // 2).astype(F32) * (2 * np.pi / S)
        return jnp.cos(angle), jnp.sin(angle)

    def times_row(a, b, i):
        br, bi = (jnp.broadcast_to(v[i:i + 1], (8, 128)) for v in b)
        return a[0] * br - a[1] * bi, a[0] * bi + a[1] * br

    def make_wide():
        row, lane = lax.broadcasted_iota(jnp.int32, (8, 128), 0), _lane(8)
        for ct, (ra, rb) in enumerate(PAIRS):
            res = _residues(ra) + _residues(rb)
            kd = (lane & 31) * 16 + _chain(
                _add, [jnp.where(lane >> 5 == g, p, 0) for g, p in enumerate(res)])
            if ct == 0:
                kd = jnp.where(lane == 0, D // 2, kd)
            fine, coarse = unit(-2 * row * kd), [unit(-16 * (row + 8 * h) * kd) for h in range(2)]
            for a in range(16):
                re, im = times_row(fine, coarse[a // 8], a % 8)
                if ct == 0:
                    even = kd & 7 == 0
                    top = jnp.where(even, re, 0.0), jnp.where(lane == 0, 1.0, jnp.where(even, im, 0.0))
                    bottom = jnp.where(even, 0.0, re), jnp.where(even, 0.0, im)
                else:
                    sign = jnp.where(kd & 7 == ra, 1.0, -1.0)
                    top, bottom = (re, im), (-sign * im, sign * re)
                for i in range(2):
                    wide[2 * ct + i, pl.ds(8 * a, 8), :] = top[i].astype(BF16)
                    wide[2 * ct + i, pl.ds(128 + 8 * a, 8), :] = bottom[i].astype(BF16)

    def make_s_fwd(t):
        row, lane = lax.broadcasted_iota(jnp.int32, (8, 128), 0), _lane(8)
        pos = 8 * (lane >> 1) + t
        fine = unit((lane & 1) * (S // 4) - 4 * row * pos)
        shift, coarse = unit(-row * pos), unit(-32 * row * pos)
        for e in range(4):
            base = times_row(fine, shift, e)
            for g in range(8):
                for i, v in enumerate(times_row(base, coarse, g)):
                    sfw[t * 4 + e, pl.ds(16 * g + 8 * i, 8), :] = v.astype(BF16)

    def make_s_inv(e):
        row, lane = lax.broadcasted_iota(jnp.int32, (8, 128), 0), _lane(8)
        freq = 4 * (lane >> 1) + e
        fine = [v * (1.0 / S) for v in unit((lane & 1) * (S // 4) + 8 * row * freq)]
        shift, coarse = unit(row * freq), unit(64 * row * freq)
        for t in range(8):
            base = times_row(fine, shift, t)
            for g in range(8):
                for i, v in enumerate(times_row(base, coarse, g)):
                    siv[t * 4 + e, pl.ds(64 * i + 8 * g, 8), :] = v.astype(BF16)

    def prep_filter(ri, m):
        sub = lax.broadcasted_iota(jnp.int32, (8, 128), 0)
        edge = (wr_edge, wi_edge)[ri]
        res = {}
        for i in range(8):
            words = wraw32[ri, m, pl.ds(i, 32, stride=8), :]
            res[2 * i], res[2 * i + 1] = _unpack(words, 0), _unpack(words, 1)
        first = res[0][0:8]
        dst = pl.ds((m % 2) * 16 + ri * 8, 8)
        prev = jnp.zeros((8, 128), F32) if m < 2 else side[1, dst, :]
        put(side.at[1, dst, :], jnp.where(sub == m // 2, jnp.broadcast_to(first[0:1], (8, 128)), prev))
        nyq = jnp.broadcast_to(edge[0:1, pl.ds(m * 128, 128)].astype(F32), (8, 128))
        res[0] = jnp.concatenate([jnp.where(sub == 0, nyq, first), res[0][8:]], axis=0)
        for ct, (ra, rb) in enumerate(PAIRS):
            blk = jnp.concatenate([res[p] for p in _residues(ra) + _residues(rb)], axis=0)
            o = _dot_nt(lhs(small32[16]), blk.astype(BF16))
            for e in range(4):
                put(wf.at[ri, ct, e, m // 2, pl.ds((m % 2) * 32, 32), :], o[e * 32:(e + 1) * 32])

    def prep_wqkv_cross(g, r):
        pos = (_lane(8) >> 2) & 7
        u = [wqkv_raw32[g * NT + (-j) % 8, pl.ds(r * 8, 8), :] for j in range(NT)]
        u[0], u[4] = gate(u[0]), gate(u[4])
        for bit in range(3):
            m = ((pos >> bit) & 1) == 1
            u = [lax.select(m, u[(j - (1 << bit)) % 8], u[j]) for j in range(NT)]
        for j in range(NT):
            if j < 4:
                pin(u[j])
            put(wtmp.at[j, pl.ds(r * 8, 8), :], u[j])

    def prep_wqkv_pair(g, p, part):
        lane = _lane(8)
        ws = {}
        for n in range(2):
            index = (lane & 3) * 32 + (((lane >> 2) + 2 * p + n) & 7) * 4 + (lane >> 5)
            for half in range(2):
                for r in range(part * 2, part * 2 + 2):
                    w = gate(wtmp[2 * p + n, pl.ds(half * 256 + r * 8, 8), :])
                    ws[r, half, n] = jnp.take_along_axis(w, index, axis=1)
        yield from _latency()
        for r in range(part * 2, part * 2 + 2):
            quad = [ws[r, half, n] for half in range(2) for n in range(2)]
            ops = [_strassen_rhs(*[_unpack(w, i) for w in quad]) for i in range(2)]
            for k in range(7):
                word = {1: quad[0], 4: quad[3]}.get(k)
                if word is None:
                    word = pack(ops[0][k], ops[1][k])
                if k in (2, 3):
                    pin(word)
                put(wqkv32.at[g * 4 + p, k, pl.ds(r * 8, 8), :], word)

    def add_prep_wqkv(sched, tick, g, ticks, pair_ticks):
        for r in range(64):
            sched.add(tick + r * ticks / 64, _once(prep_wqkv_cross, g, r))
        tick = int(tick + ticks) + 1
        done = []
        for p, n in enumerate(pair_ticks):
            for i in range(16):
                sched.add(tick + i * n / 16, prep_wqkv_pair(g, p, i))
            tick += n
            done.append(int(tick) + XGAP + 1)
        return done

    def prep_wo(p, part):
        v, pair = divmod(part, 2)
        upper = lax.broadcasted_iota(jnp.int32, (8, 128), 0) >= 4
        ws = [[wo_raw32[2 * p + n, pl.ds(128 * v + 2 * f + pair, 8, stride=16), :] for f in range(8)]
              for n in range(2)]
        for o in range(4):
            quad = [lax.select(upper, w[(2 * v + 1 + j) % 8], w[(2 * v + j) % 8])
                    for j in (o, o + 4) for w in ws]
            quad[0] = gate(quad[0])
            for i in range(2):
                for k, x in enumerate(_strassen_rhs(*[_unpack(w, i) for w in quad])):
                    if k in (2, 3):
                        pin(x)
                    wo[p, k, pl.ds(o * 128 + (2 * pair + i) * 32 + 8 * v, 8), :] = x.astype(BF16)
            if o < 3:
                yield

    def ln_stats(xs):
        lane_mean = _tree(_add, xs) * (1.0 / NT)
        lane_m2 = _tree(_add, [jnp.square(x - lane_mean) for x in xs])
        pin(lane_m2)
        mean = jnp.sum(lane_mean, axis=1, keepdims=True) * (1.0 / 128)
        yield from _latency()
        m2 = lane_m2 + jnp.square(gate(lane_mean) - mean) * float(NT)
        pin(m2)
        var = jnp.sum(m2, axis=1, keepdims=True) * (1.0 / D)
        yield from _latency()
        return mean, lax.rsqrt(gate(jnp.broadcast_to(var, (16, 128))) + EPS)

    def d_fwd_rows(b, lb, from_input=False):
        xs = load_x(b, lb, from_input)

        def emit(r, v):
            if r % 4 == 0 or (r < 4 and not from_input):
                pin(v)
            ubuf[b % RING, r, r16(lb), :] = v.astype(BF16)

        xs[:4] = [gate(x, ILAG if from_input else GLAG) for x in xs[:4]]
        inv = yield from _d_butterfly_fwd(xs, emit, pin, from_input)
        inv = jnp.broadcast_to(inv, (16, 128))
        pin(inv)
        put(uout.at[b % RING, 8, r16(lb), :], inv)

    def d_dots(b, base, per_tick):
        for r in range(8):
            o = _dot(lhs(ubuf32[b % RING, r]), bf(small32[base + r]))
            put(uout.at[b % RING, r], o)
            if r % per_tick == per_tick - 1 and r < 7:
                yield

    def d_dots_wide(b):
        for ct, (ra, rb) in enumerate(PAIRS):
            u = lhs(ubuf32[b % RING, ra], ubuf32[b % RING, rb])
            for i, r in enumerate((ra, rb)):
                o = _dot(u, bf(wide32[2 * ct + i]))
                put(uout.at[b % RING, r], ticking(o) if i else o)
            if ct < 3:
                yield

    def d_fwd_cols(b, ct, is_wide):
        c, t = divmod(b, 8)
        ra, rb = PAIRS[ct]
        lane = _lane(16)
        lo = lane < 64
        z, x0 = [], []
        for lb in range(4):
            a, bb, inv = (uout[b % RING, r, r16(lb), :] for r in (ra, rb, 8))
            inv = gate(inv, ILAG if is_wide else GLAG)
            a, bb = a * inv, bb * inv
            if is_wide:
                if ct == 0:
                    x0.append(pltpu.roll(bb, t, 1) if t else bb)
                    bb = jnp.where(lane == 0, 0.0, bb)
                z.append((a, bb))
                continue
            if ct == 0:
                x0.append(pltpu.roll(a, (t + 64) % 128, 1))
                a = jnp.where(lane == 64, 0.0, a)
            im = lax.select(lo, bb, a)
            z.append((lax.select(lo, a, bb), _swap(im)))
        if not is_wide:
            yield from _latency()
        for e, (re, im) in enumerate(_dft4(z, False)):
            words = pack(re, im)
            if e < 2:
                pin(words)
            put(zin.at[ct, t * 4 + e, r16(c), :], words)
        if is_wide and ct == 0:
            yield from _latency()
        for lb, v in enumerate(x0):
            ls = pl.ds(64 * lb + 16 * c, 16)
            prev = jnp.zeros((16, 128), F32) if t == 0 else side[0, ls, :]
            v = jnp.where(lane == t, v, prev)
            pin(v)
            put(side.at[0, ls, :], v)

    def add_d_fwd(sched, tick, b, gap, per_tick=4, from_input=False):
        for lb in range(4):
            sched.add(tick + lb * gap, d_fwd_rows(b, lb, from_input))
        tick = int(tick + 3 * gap) + XGAP + 1
        sched.add(tick, d_dots_wide(b) if from_input else d_dots(b, 0, per_tick))
        for ct in range(4):
            sched.add(tick + 8 // per_tick + 3 + ct * gap, d_fwd_cols(b, ct, from_input))
        return int(tick + 8 // per_tick + 3 + 3 * gap) + XGAP + 1

    def side_path():
        vt = side[0].T[0:8]
        yield
        zero8 = jnp.zeros((8, 256), F32)
        u = _dot(jnp.concatenate([vt, zero8], axis=0).astype(BF16), f256[...])[0:8]
        twr, twi = tw_ref[0:8, :], tw_ref[8:16, :]
        ur, ui = u[:, 0:256], u[:, 256:512]
        pad = jnp.zeros((112, 256), BF16)
        for _ in range(4):
            yield
        uu = jnp.concatenate([ur * twr - ui * twi, ur * twi + ui * twr], axis=0).astype(BF16)
        xk = _dot(d8_ref[0], jnp.concatenate([uu, pad], axis=0))
        for _ in range(4):
            yield
        wr = jnp.concatenate([side[1, 0:8, :], side[1, 16:24, :]], axis=1)
        wi = jnp.concatenate([side[1, 8:16, :], side[1, 24:32, :]], axis=1)
        xr, xi = xk[0:8], xk[8:16]
        yy = jnp.concatenate([xr * wr - xi * wi, xr * wi + xi * wr], axis=0).astype(BF16)
        p = _dot(d8_ref[1], jnp.concatenate([yy, pad], axis=0))
        for _ in range(4):
            yield
        twr, twi = tw_ref[0:8, :], tw_ref[8:16, :]
        pr, pi = p[0:8], p[8:16]
        g = jnp.concatenate([pr * twr + pi * twi, pi * twr - pr * twi], axis=1)
        g = jnp.concatenate([g, jnp.zeros((8, 512), F32)], axis=0).astype(BF16)
        y0 = _dot_nt(g, f256[...])
        for _ in range(4):
            yield
        put(side.at[2], jnp.concatenate([y0, jnp.zeros((112, 256), F32)], axis=0).T)

    def s_fwd(u, t):
        ct, e = divmod(u, 4)
        put(ybuf.at[u % NY, t], ticking(_dot(lhs(sfw32[t * 4 + e]), bf(zin[ct, t * 4 + e]))))

    def s_filter(u, g):
        ct, e = divmod(u, 4)
        z = [tuple(ybuf[u % NY, t, pl.ds(g * 16 + i, 8), :] for i in (0, 8))
             for t in range(8)]
        lag = SGLAG if u * 8 + g < 122 - S_LAG else SGLAG2
        z[0], z[1] = [tuple(gate(v, lag) for v in zz) for zz in z[0:2]]
        xk = _dft8(z, False)
        for k2 in range(8):
            wr = wf[0, ct, e, k2, pl.ds(g * 8, 8), :]
            wi = wf[1, ct, e, k2, pl.ds(g * 8, 8), :]
            re, im = xk[k2]
            xk[k2] = (re * wr - im * wi, re * wi + im * wr)
        for t, (re, im) in enumerate(_dft8(xk, True)):
            words = pack(re, im)
            if t < 4:
                pin(words)
            put(fbuf.at[u % NY, t, pl.ds(g * 8, 8), :], words)

    def s_inv(u, t):
        ct, e = divmod(u, 4)
        o = _dot(lhs(siv32[t * 4 + e]), bf(fbuf[u % NY, t]))
        put(zout.at[ct, t * 4 + e], ticking(o) if u * 8 + t >= 110 - S_LAG else o)

    def add_s_stage(sched, early, ready, t1):
        ahead = 8 + S_LAG
        tick = early
        for t in sorted(range(8), key=lambda t: ready[t]):
            for i in range(t, ahead, 8):
                tick = max(tick + 0.5, ready[t])
                sched.add(tick, _once(s_fwd, i // 8, t))
        t1 = max(t1, int(tick) + 1)
        sched.add(max(max(ready), t1), side_path())
        for i in range(128):
            if i + ahead < 128:
                sched.add(t1 + i, _once(s_fwd, *divmod(i + ahead, 8)))
            sched.add(t1 + i, _once(s_filter, *divmod(i, 8)))
            sched.add(t1 + 9 + (i if i < 120 else 120 + (i - 120) // 4), _once(s_inv, *divmod(i, 8)))
        return [t1 + 32 * ct + 40 for ct in range(3)] + [t1 + 131]

    def d_inv_cols(b, ct):
        c, t = divmod(b, 8)
        ra, rb = PAIRS[ct]
        lane = _lane(16)
        lo = lane < 64
        u = [(zout[ct, t * 4 + e, r16(c), :], zout[ct, t * 4 + e, r16(4 + c), :]) for e in range(4)]
        u[0], u[1] = tuple(map(gate, u[0])), tuple(map(gate, u[1]))
        z = _dft4(u, True)
        z = [(re, _swap(im)) for re, im in z]
        if ct == 0:
            y0 = [pltpu.roll(side[2, pl.ds(64 * lb + 16 * c, 16), :], 64 - t, 1) for lb in range(4)]
        yield from _latency()
        for lb, (re, sw) in enumerate(z):
            sw = gate(sw)
            a, bb = lax.select(lo, re, sw), lax.select(lo, sw, re)
            if ct == 0:
                a = jnp.where(lane == 64, y0[lb], a)
            pin(a)
            ubuf[b % RING, ra, r16(lb), :] = a.astype(BF16)
            ubuf[b % RING, rb, r16(lb), :] = bb.astype(BF16)

    def d_inv_rows(b, lb, stats, first):
        u = [uout[b % RING, r, r16(lb), :] for r in range(8)]
        ys = yield from _d_butterfly_inv([gate(v) if r < 4 else v for r, v in enumerate(u)], pin, gate)
        xs = [x + y for x, y in zip(load_x(b, lb, first), ys)]
        for j in range(NT):
            put(xres.at[b, j, r16(lb), :], xs[j])
        stats[b, lb] = yield from ln_stats(xs)
        if b % 2:
            for j in range(4):
                a = [(xres[bb, j + o, r16(lb), :] - stats[bb, lb][0]) * stats[bb, lb][1]
                     for bb in (b - 1, b) for o in (0, 4)]
                a[0], a[3] = gate(a[0]), gate(a[3])
                for k, v in enumerate(_strassen_lhs(*a)):
                    if k in (1, 4):
                        pin(v)
                    abuf[b // 2, k, j, r16(lb), :] = v.astype(BF16)
                if j < 3:
                    yield

    def add_d_inv(sched, tick, b, gap, stats, first, cols=None):
        per_tick = 4
        cols = cols or [tick + ct * gap for ct in range(4)]
        for ct in range(4):
            sched.add(cols[ct], d_inv_cols(b, ct))
        tick = int(cols[3]) + XGAP + 1
        sched.add(tick, d_dots(b, 8, per_tick))
        tick += 8 // per_tick + 3
        for lb in range(4):
            sched.add(tick + lb * gap, d_inv_rows(b, lb, stats, first))
        return int(tick + 3 * gap) + 3 * XGAP + 1 + 4

    def gemm(lhs32, rhs32, jobs, sink):
        for slot, b, n in jobs:
            m = {}
            for k in (3, 1, 0, 6, 5, 4, 2):
                m[k] = ticking(_dot(lhs(*[lhs32[slot, k, j] for j in range(4)]), bf(rhs32[n // 2, k])))
                if k == 1:
                    sink(b + 1, n, m[1] - m[3])
                elif k == 0:
                    c11, c22 = m[3] - m[0], m[1] - m[0]
                elif k == 6:
                    c11 = m[6] - c11
                elif k == 5:
                    c22 = m[5] - c22
                elif k == 4:
                    sink(b, n, c11 - m[4])
                elif k == 2:
                    sink(b, n + 1, m[4] - m[2])
                    sink(b + 1, n + 1, c22 - m[2])
                yield

    def qkv_sink(b, n, o):
        c, t = divmod(b, 8)
        dst = (qbuf, kbuf, vbuf)[n // NT]
        for lb in range(4):
            put(dst.at[n % NT, t, pl.ds(8 + 64 * lb + 16 * c, 16), :], o[lb * 16:(lb + 1) * 16])
        if b == 0 and n >= NT:
            first = jnp.broadcast_to(o[0:1], (8, 128))
            for tt in range(8):
                dst[n % NT, tt, pl.ds(0, 8), :] = first

    def out_rows(r, i, last):
        c, t = divmod(r, 8)
        return (c * 8 + t % 2 * 4 + i, t // 2) if last and c == 0 else (r, i)

    def out_sink(last, r, n, o):
        for i in range(4):
            b, lb = out_rows(r, i, last)
            put(xres.at[b, n, r16(lb), :], xres[b, n, r16(lb), :] + o[i * 16:(i + 1) * 16])

    def attention(b, lb, h):
        c, t = divmod(b, 8)
        log2e = float(np.log2(np.e))
        scale = HEAD_DIM ** -0.5 * log2e
        r0 = 8 + 64 * lb + 16 * c + 8 * h
        src = [((t - 2 * w) % 8, -((t - 2 * w) // 8)) for w in range(WIN)]
        acc = [None] * WIN
        for j in range(NT):
            if j % 2 == 0:
                factor = gate(jnp.full((8, 128), scale, F32), ALAG)
            q = qbuf[j, t, pl.ds(r0, 8), :] * factor
            for w, (ts, sh) in enumerate(src):
                p = q * kbuf[j, ts, pl.ds(r0 - sh, 8), :]
                acc[w] = p if j == 0 else acc[w] + p
            if j % 2 and j < NT - 1:
                pin(*acc[j // 2 % 2::2])
                yield
        part = [(r, pltpu.roll(r, 64, 1)) for r in acc]
        yield from _latency()
        part = [r + rr for r, rr in part]
        part = [(r, pltpu.roll(r, 32, 1)) for r in part]
        yield from _latency()
        logits = [r + rr for r, rr in part]
        if r0 == 8:
            sub = lax.broadcasted_iota(jnp.int32, (8, 128), 0)
            logits = [jnp.where(sub >= sh, r, -1e9 * log2e) if sh else r
                      for r, (_, sh) in zip(logits, src)]
        logits[0] = gate(logits[0], ALAG)
        m = _tree(jnp.maximum, logits)
        ps = [jnp.exp2(r - m) for r in logits]
        total = _tree(_add, ps)
        pin(total)
        inv = pltpu.reciprocal(total, approx=True)
        inv = inv * (2.0 - total * inv)
        for j in range(NT):
            if j % 2 == 0:
                yield
                ps[0], ps[4] = gate(ps[0], ALAG), gate(ps[4], ALAG)
            o = _chain(_add, [ps[w] * vbuf[j, ts, pl.ds(r0 - sh, 8), :]
                              for w, (ts, sh) in enumerate(src)]) * inv
            if j % 2:
                pin(o)
            put(qbuf.at[j, t, pl.ds(r0, 8), :], o)

    def out_operands(r, i, last):
        for j in range(4):
            a = [qbuf[j + o, b % 8, pl.ds(8 + 64 * lb + 16 * (b // 8), 16), :]
                 for b, lb in (out_rows(r, i, last), out_rows(r + 1, i, last)) for o in (0, 4)]
            a[0], a[3] = gate(a[0]), gate(a[3])
            for k, v in enumerate(_strassen_lhs(*a)):
                if k in (1, 4):
                    pin(v)
                obuf[r // 2, k, j, r16(i), :] = v.astype(BF16)
            if j < 3:
                yield

    def store_rows(b, lb):
        c, t = divmod(b, 8)
        for j in range(NT):
            words = pack(xres[b, j, r16(lb), :], xres[b + 1, j, r16(lb), :])
            pin(words)
            io32[j, lb, c, pl.ds(t // 2, 16, stride=4), :] = words

    unit_ticks = NT + 2 * XGAP
    step = 2
    out_ticks = 28

    def add_proj(sched, tick, c, lo, hi):
        jobs = [(b // step, b, n) for b in range(8 * c, 8 * c + 8, step) for n in range(lo, hi, step)]
        sched.add(tick, gemm(abuf32, wqkv32, jobs, qkv_sink))
        return tick + len(jobs) * out_ticks * step // NT

    def add_attention(sched, tick, pace, rows, last):
        units = [(r, i, half, h) for r in rows[::2] for i in range(4) for half in range(2) for h in range(2)]
        for n, (r, i, half, h) in enumerate(units):
            sched.add(tick + n * pace, attention(*out_rows(r + half, i, last), h))
            if half and h:
                sched.add(int(tick + n * pace) + unit_ticks, out_operands(r, i, last))

    def add_out(sched, tick, rows, last):
        jobs = [(r // 2, r, n) for r in rows[::2] for n in range(0, NT, 2)]
        sched.add(tick, gemm(obuf32, wo32, jobs, functools.partial(out_sink, last)))

    def add_tail(sched, tick, rows, last):
        ready = {}
        for i, r in enumerate(rows):
            t0 = tick + (i // 2 + 1) * out_ticks
            fast = i >= len(rows) - (2 if last else 4)
            if not last:
                t0 += 0 if fast else TOFF + i % 2 * out_ticks // 2
                ready[r % 8] = add_d_fwd(sched, t0, r, i % 2 if fast else out_ticks / 8)
            elif r % 2:
                c, p = r // 8, r % 8 // 2
                gap = 0 if fast else 3
                for j in range(4):
                    sched.add(t0 + (j + 1) * gap, _once(store_rows, *((r - 1, j) if c else (2 * j, p))))
                for lb in ([p] if c == 0 else range(4) if p == 3 else []):
                    sched.add(t0 + 5 * gap + 1, _once(start, out_copies(c, lb)))
        return ready

    q_ticks = 8 * out_ticks // step
    att_ticks = unit_ticks + 1 + 2
    order = [(a + 8) % NB for a in range(NB)]

    def add_attention_block(sched, cols, last):
        stats = {}
        t0 = max([add_d_inv(sched, 0, b, 0, stats, not last, cols) for b in range(step)])
        if not last:
            sched.add(cols[3] - KLEAD, _once(wait, qkv_copies(1) + dmat_cp))
            done = add_prep_wqkv(sched, cols[3] - KLEAD, 1, KPACE, [7] * 4)
            t0 = max(t0, done[0])
            assert all(d <= t0 + p * out_ticks / 4 for p, d in enumerate(done))
            sched.add(t0 + out_ticks, _once(wait, qkv_copies(2)))
            sched.add(t0 + out_ticks, _once(start, qkv_copies(0)))
            done = add_prep_wqkv(sched, t0 + out_ticks, 2, 2 * out_ticks - 4, [out_ticks - 4] * 4)
            assert all(d <= t0 + q_ticks + p * out_ticks for p, d in enumerate(done))
            sched.add(t0 + 2 * q_ticks, _once(wait, qkv_copies(0)))
            sched.add(t0 + 2 * q_ticks, _once(start, wo_copies))
            done = add_prep_wqkv(sched, t0 + 2 * q_ticks, 0, q_ticks - 10, [q_ticks / 4] * 4)
            assert done[-1] <= t0 + 4 * q_ticks
            sched.add(t0 + 8 * q_ticks, _once(wait, wo_copies))
            for i in range(32):
                sched.add(t0 + 8 * q_ticks + i * q_ticks / 16, prep_wo(*divmod(i, 8)))
        tick, kv_start, q_start = t0, {}, {}
        for kind, c in ("k0", "k1", "q1", "k2", "q2", "k3", "q3", "q0"):
            if kind == "k":
                kv_start[int(c)] = tick
                if c == "0" and not last:
                    tick = add_proj(sched, tick, 0, NT, 2 * NT)
                    jobs = [(b // step, b, n) for n in range(2 * NT, 3 * NT, step) for b in range(0, 8, step)]
                    sched.add(tick, gemm(abuf32, wqkv32, jobs, qkv_sink))
                    tick += q_ticks
                    continue
                tick = add_proj(sched, tick, int(c), NT, 3 * NT)
            else:
                q_start[int(c)] = tick
                tick = add_proj(sched, tick, int(c), 0, NT)
        pace = 2 * out_ticks / step
        for b in range(step, NB):
            due = kv_start[b // 8] + (b % 8 // step) * (2 if last or b >= 8 else 1) * out_ticks
            gap = min(1 + (b - step) * 0.5, DGAP1 if last else DGAP0)
            pace = DPACE1 if last else DPACE0
            at = (b - step) * pace
            at = t0 + at + max(0, at - 4 * q_ticks - out_ticks) * DSLOW
            if not last and b < 8:
                at, gap = max(cols[3], t0 + (b // step - 1) * out_ticks - (step - b % step) * 8), 1
            end = add_d_inv(sched, at, b, gap, stats, not last)
            assert end <= due, (b, end, due)
        begin = [q_start[c] + out_ticks + 3 for c in (1, 2, 3)] + [tick + (ATT1 if last else ATT0)]
        begin.append(tick + (NB // step - 1) * out_ticks - att_ticks)
        for i, c in enumerate((1, 2, 3, 0)):
            pace = (begin[i + 1] - begin[i]) / 64
            assert begin[i] >= max(kv_start[c], kv_start[(c - 1) % 4]) + 2 * q_ticks
            for p in range(4):
                assert begin[i] + 16 * p * pace >= q_start[c] + (4 if last and c == 0 else p + 1) * out_ticks
                assert begin[i] + (16 * p + 15) * pace + att_ticks <= tick + (4 * i + p) * out_ticks + 1e-6
            add_attention(sched, begin[i], pace, range(8 * c, 8 * c + 8), last)
        add_out(sched, tick, order, last)
        return tick + (NB // step) * out_ticks, add_tail(sched, tick, order, last)

    def add_input(sched):
        ready = {}
        after = (x_copies(2), x_copies(3) + perm_cp + w_copies(0) + w_copies(1),
                 w_copies(2) + w_copies(3), w_copies(4))
        for c in range(NC):
            sched.add(c * 32, _once(wait, x_copies(c)))
            sched.add(c * 32, _once(start, after[c]))
            for t in range(8):
                ready[t] = add_d_fwd(sched, c * 32 + t * 4, c * 8 + t, 1, 2, True)
        return 128 + 9, ready

    def add_filter_prep(sched, tick):
        after = (w_copies(5) + w_copies(6), w_copies(7) + f256_cp + dmat_cp, qkv_copies(1), qkv_copies(2))
        begin = [F0 + g * (tick - F0) / 4 for g in range(4)] + [tick + FG * g for g in range(5)]
        for g in range(8):
            if g % 2 == 0:
                sched.add(begin[g], _once(wait, w_copies(g) + w_copies(g + 1) + ([] if g else perm_cp)))
                sched.add(begin[g], _once(start, after[g // 2]))
            for m in range(4):
                sched.add(begin[g] + m * (begin[g + 1] - begin[g]) / 4,
                          _once(prep_filter, g // 4, g % 4 * 4 + m))
        sched.add(begin[8] + 1, _once(wait, f256_cp))
        return begin[8] + 2

    sched = _Schedule()

    start(x_copies(0))
    for ref in (abuf32, obuf32, ubuf32, wo32, sfw32, siv32, wide32):
        put(ref.at[(0,) * (len(ref.shape) - 2) + (pl.ds(0, 8),)], jnp.zeros((8, 128), U32))
    make_wide()
    start(x_copies(1))
    for t in range(8):
        make_s_fwd(t)
    for e in range(4):
        make_s_inv(e)
    tick, ready = add_input(sched)
    cols = add_s_stage(sched, tick, ready, add_filter_prep(sched, tick))
    tick, ready = add_attention_block(sched, cols, False)
    cols = add_s_stage(sched, tick, ready, tick)
    add_attention_block(sched, cols, True)
    sched.run()
    for c in range(NC):
        for lb in range(4):
            wait(out_copies(c, lb))


@jax.jit
def pallas_interleave_layers__spectral_gfnet__sliding_local_dilated__prompt_kernel(
    A_x: jax.Array,
    A_w_r: jax.Array,
    A_w_i: jax.Array,
    B_x: jax.Array,
    B_wqkv: jax.Array,
    B_wo: jax.Array,
):
    del B_x
    assert A_x.shape == (1, S, D) and A_w_r.shape == (S, D // 2 + 1)
    cst = _constants()
    x = A_x.astype(BF16).reshape(4, NC, 128, D)
    wr, wi = A_w_r.astype(BF16).T, A_w_i.astype(BF16).T
    hbm = pl.BlockSpec(memory_space=pl.ANY)
    edge = pl.BlockSpec((16, S), lambda i: (D // 32, 0))
    vm = pltpu.VMEM
    out = pl.pallas_call(
        _kernel,
        grid=(1,),
        in_specs=[hbm, hbm, hbm, edge, edge, hbm, hbm, hbm, hbm,
                  pl.BlockSpec((24, 256), lambda i: (0, 0)),
                  pl.BlockSpec((2, 16, 128), lambda i: (0, 0, 0))],
        out_specs=hbm,
        out_shape=jax.ShapeDtypeStruct((4, NC, 128, D), BF16),
        scratch_shapes=[
            vm((NT, 4, NC, 128, 128), BF16),
            vm((17, 128, 128), BF16),
            vm((32, 128, 128), BF16),
            vm((32, 128, 128), BF16),
            vm((256, 512), BF16),
            vm((2, 16, 512, 128), BF16),
            vm((2, 4, 4, 8, 64, 128), F32),
            vm((3 * NT, D, 128), BF16),
            vm((NT, D // 2, 128), U32),
            vm((12, 7, 512, 128), BF16),
            vm((NT, D, 128), BF16),
            vm((4, 7, 512, 128), BF16),
            vm((NB, NT, 64, 128), F32),
            vm((4, 32, 64, 128), U32),
            vm((4, 32, 128, 128), F32),
            vm((NY, 8, 128, 128), F32),
            vm((NY, 8, 64, 128), U32),
            vm((RING, 8, 64, 128), BF16),
            vm((RING, 9, 64, 128), F32),
            vm((NB // 2, 7, 4, 64, 128), BF16),
            vm((NB // 2, 7, 4, 64, 128), BF16),
            vm((NT, 8, 264, 128), F32),
            vm((NT, 8, 264, 128), F32),
            vm((NT, 8, 264, 128), F32),
            vm((3, 256, 128), F32),
            vm((8, 256, 128), BF16),
            pltpu.SemaphoreType.DMA((NC,)),
            pltpu.SemaphoreType.DMA((3,)),
            pltpu.SemaphoreType.DMA((8,)),
            pltpu.SemaphoreType.DMA((3,)),
            pltpu.SemaphoreType.DMA(()),
            pltpu.SemaphoreType.DMA(()),
        ],
        compiler_params=pltpu.CompilerParams(
            dimension_semantics=("arbitrary",), vmem_limit_bytes=120 * 2**20),
    )(x, wr, wi, wr, wi, B_wqkv.astype(BF16), B_wo.astype(BF16),
      cst["small"], cst["f256"], cst["tw"], cst["d8"])
    return out.reshape(1, S, D)
```

```python
import functools

import jax
import jax.numpy as jnp
import numpy as np
from jax import lax
from jax.experimental import pallas as pl
from jax.experimental.pallas import tpu as pltpu

S, D = 2048, 1024
NT = D // 128
NC = 4
WIN = 8
HEAD_DIM = 32
EPS = 1e-5
F32, BF16, U32 = jnp.float32, jnp.bfloat16, jnp.uint32
PAIRS = ((0, 4), (1, 7), (2, 6), (3, 5))
RSQ2 = float(np.sqrt(0.5))
NB = S // 64

RING = 8
XGAP = 3
GLAG = 4
ALAG = 4
SGLAG = 3
S_LAG = 2
F0 = 120
KLEAD = 46
KPACE = 40
DGAP0 = 4.75
DGAP1 = 4.2
DPACE0 = 20
DPACE1 = 15.5
DSLOW = 0.6
SYNC = 3
ILAG = 3
FG = 10
TOFF = 3
WK0 = 24
ATT0 = 25
ATT1 = 95


def _residues(r):
    return (0, 8) if r == 0 else (r, 16 - r)


def _d_matrices():
    n = np.arange(64)[:, None]
    a = np.arange(32)
    fwd = np.zeros((8, 128, 128))
    inv = np.zeros((8, 128, 128))
    for r in range(8):
        kd = np.concatenate([16 * a + p for p in _residues(r)])
        weight = np.full(64, 2.0)
        if r == 0:
            kd[0], weight[0] = D // 2, 1.0
            ph = np.exp(-2j * np.pi * n * kd[None, :] / D)
            sgn = np.where(kd % 16 == 0, 1.0, -1.0)[None, :]
            m = np.concatenate([ph, ph * sgn], axis=0)
            re, im = m.real.copy(), m.imag.copy()
            ire, iim = re.copy(), im.copy()
            im[:, 0] = 1.0
            iim[:, 0] = 1.0
        else:
            p = 12 if r == 4 else r
            ph = np.exp(-2j * np.pi * n * kd[None, :] / D)
            si = np.where(kd % 16 == p, 1.0, -1.0)[None, :]
            m = np.concatenate([ph, 1j * si * ph], axis=0)
            re, im = m.real, m.imag
            ire, iim = re, im
        swapped = r in (4, 7, 6, 5)
        cols = [im, re] if swapped else [re, im]
        icols = [iim * weight, ire * weight] if swapped else [ire * weight, iim * weight]
        fwd[r] = np.concatenate(cols, axis=1)
        inv[r] = np.concatenate(icols, axis=1).T / D
    return fwd, inv


def _side_matrices():
    l = np.arange(256)
    f = np.exp(-2j * np.pi * ((l[:, None] * l[None, :]) % 256) / 256)
    f256 = np.concatenate([f.real, f.imag], axis=1)
    t = np.arange(8)
    tw = np.exp(-2j * np.pi * t[:, None] * l[None, :] / S)
    tw = np.concatenate([tw.real, tw.imag, np.zeros((8, 256))], axis=0)
    g = np.exp(-2j * np.pi * t[:, None] * t[None, :] / 8)
    d8 = np.zeros((2, 16, 128))
    d8[0, :, :16] = np.block([[g.real, -g.imag], [g.imag, g.real]])
    d8[1, :, :16] = d8[0, :, :16].T / S
    return f256, tw, d8


def _filter_rows():
    p = np.zeros((1, 128, 128))
    for k in range(32):
        for e in range(4):
            p[0, e * 32 + k, 4 * k + e] = 1.0
    return p


@functools.lru_cache(maxsize=None)
def _constants():
    dfw, div = _d_matrices()
    f256, tw, d8 = _side_matrices()
    small = np.concatenate([dfw, div, _filter_rows()], axis=0)
    b = lambda x: np.asarray(x, np.float32).astype(BF16)
    return dict(small=b(small), f256=b(f256),
                tw=np.asarray(tw, np.float32), d8=b(d8))


def _dot(a, b):
    return jnp.dot(a, b, preferred_element_type=F32)


def _dot_nt(a, b):
    return lax.dot_general(a, b, (((1,), (1,)), ((), ())), preferred_element_type=F32)


def _tree(op, xs):
    xs = list(xs)
    while len(xs) > 1:
        xs = [op(xs[i], xs[i + 1]) if i + 1 < len(xs) else xs[i] for i in range(0, len(xs), 2)]
    return xs[0]


def _chain(op, xs):
    return functools.reduce(op, xs)


def _lane(rows):
    return lax.broadcasted_iota(jnp.int32, (rows, 128), 1)


def _swap(x):
    return pltpu.roll(x, 64, 1)


def _unpack(w, i):
    return pltpu.unpack_elementwise(w, index=i, packed_dtype=BF16, unpacked_dtype=F32)


def _latency():
    for _ in range(XGAP):
        yield


def _add(a, b):
    return a + b


def _row_mean(xs):
    return jnp.sum(_tree(_add, xs), axis=1, keepdims=True) * (1.0 / D)


def _twiddle16(r, x, y):
    lo = _lane(x.shape[0]) < 64
    wr, wi = float(np.cos(np.pi * r / 8)), float(-np.sin(np.pi * r / 8))
    cross = jnp.where(lo, 0.0, wr)
    return x * jnp.where(lo, 1.0, wi) + y * cross, y * jnp.where(lo, 1.0, -wi) + x * cross


def _d_butterfly_fwd(a, emit, pin, wide):
    s = [a[j] + a[j + 4] for j in range(4)]
    e, o = s[0] + s[2], s[1] + s[3]
    total, t4 = e + o, e - o
    emit(4, t4)
    d0, nd2 = a[0] - a[4], a[6] - a[2]
    d1, d3 = a[1] - a[5], a[3] - a[7]
    p, q = (d1 - d3) * RSQ2, (d1 + d3) * -RSQ2
    ts = {1: (d0 + p, q + nd2), 2: (s[0] - s[2], s[3] - s[1]), 3: (d0 - p, q - nd2)}
    mean8 = jnp.sum(total, axis=1, keepdims=True) * (1.0 / 128)
    if wide:
        for r, (tr, ti) in ts.items():
            emit(r, tr)
            emit(8 - r, ti)
    else:
        ab = {r: _twiddle16(r, *t) for r, t in ts.items()}
        ab = {r: (a, _swap(b)) for r, (a, b) in ab.items()}
    dev = _tree(_add, [v * v for t in ts.values() for v in t]) * 2.0 + t4 * t4
    pin(dev)
    yield from _latency()
    t0 = total - mean8
    emit(0, t0)
    var = jnp.sum(dev + t0 * t0, axis=1, keepdims=True) * (1.0 / (NT * D))
    if not wide:
        for r, (x, y) in ab.items():
            emit(r, x + y)
            emit(8 - r, x - y)
    yield from _latency()
    return lax.rsqrt(var + EPS)


def _d_butterfly_inv(u, pin, gate):
    ab = {r: (u[r] + u[8 - r], _swap(u[r] - u[8 - r])) for r in (1, 2, 3)}
    e, o = u[0] + u[4], u[0] - u[4]
    yield from _latency()
    ts = {r: _twiddle16(r, x, gate(y)) for r, (x, y) in ab.items()}
    pin(*[t[0] for t in ts.values()])
    yield
    s = [e + ts[2][0], o - ts[2][1], e - ts[2][0], o + ts[2][1]]
    p = (ts[1][0] - ts[3][0]) * RSQ2
    q = (ts[1][1] + ts[3][1]) * RSQ2
    d0, d1, d2, nd3 = ts[1][0] + ts[3][0], p - q, ts[3][1] - ts[1][1], p + q
    return [s[0] + d0, s[1] + d1, s[2] + d2, s[3] - nd3,
            s[0] - d0, s[1] - d1, s[2] - d2, s[3] + nd3]


def _strassen_lhs(a11, a12, a21, a22):
    return [a11 + a22, a21 + a22, a11, a22, a11 + a12, a21 - a11, a12 - a22]


def _strassen_rhs(b11, b12, b21, b22):
    return [b11 + b22, b11, b22 - b12, b11 - b21, b22, b11 + b12, b21 + b22]


def _cadd(a, b):
    return a[0] + b[0], a[1] + b[1]


def _csub(a, b):
    return a[0] - b[0], a[1] - b[1]


def _dft4(z, inverse):
    a, b = _cadd(z[0], z[2]), _csub(z[0], z[2])
    c, d = _cadd(z[1], z[3]), _csub(z[1], z[3])
    minus = (b[0] + d[1], b[1] - d[0])
    plus = (b[0] - d[1], b[1] + d[0])
    return [_cadd(a, c), plus if inverse else minus, _csub(a, c), minus if inverse else plus]


def _dft8(z, inverse):
    ev = _dft4(z[0::2], inverse)
    od = _dft4(z[1::2], inverse)
    out = [None] * 8
    out[0], out[4] = _cadd(ev[0], od[0]), _csub(ev[0], od[0])
    (er, ei), (x, y) = ev[2], od[2]
    minus, plus = (er + y, ei - x), (er - y, ei + x)
    out[2], out[6] = (plus, minus) if inverse else (minus, plus)
    for k in (1, 3):
        (er, ei), (x, y) = ev[k], od[k]
        sm, df = (x + y) * RSQ2, (x - y) * RSQ2
        if not inverse:
            if k == 1:
                out[1], out[5] = (er + sm, ei - df), (er - sm, ei + df)
            else:
                out[3], out[7] = (er - df, ei - sm), (er + df, ei + sm)
        else:
            if k == 1:
                out[1], out[5] = (er + df, ei + sm), (er - df, ei - sm)
            else:
                out[3], out[7] = (er - sm, ei + df), (er + sm, ei - df)
    return out


class _Schedule:
    def __init__(self):
        self.pending = []

    def add(self, tick, gen):
        self.pending.append((int(tick), len(self.pending), gen))

    def run(self):
        pending = sorted(self.pending, key=lambda p: p[:2])
        active, tick, i = [], 0, 0
        while active or i < len(pending):
            while i < len(pending) and pending[i][0] <= tick:
                active.append(pending[i][2])
                i += 1
            for g in list(active):
                if next(g, 0) == 0:
                    active.remove(g)
            tick += 1
        self.pending = []


def _once(fn, *args):
    fn(*args)
    return
    yield


def _kernel(x_hbm, wr_hbm, wi_hbm, wr_edge, wi_edge, wqkv_hbm, wo_hbm,
            small_hbm, f256_hbm, tw_ref, d8_ref,
            out_hbm,
            io, small, sfw, siv, f256, wraw, wf, wqkv_raw, wtmp, wqkv, wo_raw, wo,
            xres, zin, zout, ubuf, uout, abuf, obuf, qbuf, kbuf, vbuf, side,
            wide, sem_x, sem_c, sem_w, sem_qkv, sem_wo, sem_out):

    def x_copies(c):
        return [pltpu.make_async_copy(x_hbm.at[:, c, :, pl.ds(j * 128, 128)], io.at[j, :, c],
                                      sem_x.at[c]) for j in range(NT)]

    def out_copies(c, lb):
        return [pltpu.make_async_copy(io.at[j, lb, c], out_hbm.at[lb, c, :, pl.ds(j * 128, 128)],
                                      sem_out) for j in range(NT)]

    perm_cp, dmat_cp, f256_cp = ([pltpu.make_async_copy(s, d, sem_c.at[i])] for i, (s, d) in enumerate((
        (small_hbm.at[pl.ds(16, 1)], small.at[pl.ds(16, 1)]),
        (small_hbm.at[pl.ds(0, 16)], small.at[pl.ds(0, 16)]), (f256_hbm, f256))))

    def w_tiles(g):
        return [(g // 2 % 2, 8 * (g % 2) + 2 * i + g // 4) for i in range(4)]

    def w_copies(g):
        return [pltpu.make_async_copy((wr_hbm, wi_hbm)[ri].at[pl.ds(0, 512), pl.ds(m * 128, 128)],
                                      wraw.at[ri, m], sem_w.at[g]) for ri, m in w_tiles(g)]

    def qkv_copies(g):
        return [pltpu.make_async_copy(wqkv_hbm.at[:, pl.ds(g * D + j * 128, 128)],
                                      wqkv_raw.at[g * NT + j], sem_qkv.at[g]) for j in range(NT)]

    wo_copies = [pltpu.make_async_copy(wo_hbm.at[:, pl.ds(j * 128, 128)], wo_raw.at[j], sem_wo)
                 for j in range(NT)]

    def start(cs):
        for cp in cs:
            cp.start()

    def wait(cs):
        for cp in cs:
            cp.wait()

    io32, wraw32, wo_raw32 = io.bitcast(U32), wraw.bitcast(U32), wo_raw.bitcast(U32)
    small32, sfw32, siv32, wide32 = (r.bitcast(U32) for r in (small, sfw, siv, wide))
    wqkv_raw32, wqkv32, wo32 = (r.bitcast(U32) for r in (wqkv_raw, wqkv, wo))
    ubuf32, abuf32, obuf32 = ubuf.bitcast(U32), abuf.bitcast(U32), obuf.bitcast(U32)

    never = tw_ref[16:24, 0:128] != 0.0
    never_wide = {n: jnp.concatenate([tw_ref[16:24, 0:128]] * n, axis=1) != 0.0 for n in (1, 2, 4)}
    token = {}

    def pin(*values):
        for v in values:
            key = v.shape[0], v.dtype == F32
            token[key] = (lax.max if key[1] else lax.bitwise_xor)(token[key], v) if key in token else v

    clock = []

    def gate(v, lag=GLAG):
        if len(clock) < lag:
            return v
        old = clock[-lag] if v.dtype == F32 else pltpu.bitcast(clock[-lag], v.dtype)
        if v.shape[0] == 8:
            return lax.select(never, old, v)
        return lax.concatenate([lax.select(never, old, v[0:8]), v[8:]], 0)

    def ticking(o):
        clock.append(o[0:8])
        del clock[:-16]
        return o

    def lhs(*tiles):
        if not token and len(tiles) == 4 and len(clock) >= SYNC:
            pin(clock[-SYNC])
        words = lax.concatenate(tiles, 1) if len(tiles) > 1 else tiles[0]
        if token:
            parts = [pltpu.bitcast(v, U32) if is_float else v for (_, is_float), v in token.items()]
            token.clear()
            w = _chain(lax.bitwise_xor, [v[i:i + 8] if v.shape[0] > 8 else v
                                         for v in parts for i in range(0, v.shape[0], 8)])
            w = lax.concatenate([w] * len(tiles), 1) if len(tiles) > 1 else w
            words = lax.concatenate([lax.select(never_wide[len(tiles)], w, words[0:8]), words[8:]], 0)
        return pltpu.bitcast(words, BF16)

    def bf(words):
        return pltpu.bitcast(words, BF16)

    def pack(a, b):
        return pltpu.bitcast(pltpu.pack_elementwise([a, b], packed_dtype=BF16), U32)

    def r16(i):
        return pl.ds(i * 16, 16)

    always = {}

    def put(ref, v):
        if v.shape not in always:
            always[v.shape] = jnp.ones(v.shape, jnp.bool_)
        pltpu.store(ref, v, mask=always[v.shape])

    def load_x(b, lb, from_input):
        if from_input:
            c, t = divmod(b, 8)
            return [_unpack(io32[j, lb, c, pl.ds(t // 2, 16, stride=4), :], t % 2) for j in range(NT)]
        return [xres[b, j, r16(lb), :] for j in range(NT)]

    def unit(p):
        angle = (((p + S // 2) & (S - 1)) - S // 2).astype(F32) * (2 * np.pi / S)
        return jnp.cos(angle), jnp.sin(angle)

    def times_row(a, b, i):
        br, bi = (jnp.broadcast_to(v[i:i + 1], (8, 128)) for v in b)
        return a[0] * br - a[1] * bi, a[0] * bi + a[1] * br

    def make_wide():
        row, lane = lax.broadcasted_iota(jnp.int32, (8, 128), 0), _lane(8)
        for ct, (ra, rb) in enumerate(PAIRS):
            res = _residues(ra) + _residues(rb)
            kd = (lane & 31) * 16 + _chain(
                _add, [jnp.where(lane >> 5 == g, p, 0) for g, p in enumerate(res)])
            if ct == 0:
                kd = jnp.where(lane == 0, D // 2, kd)
            fine, coarse = unit(-2 * row * kd), [unit(-16 * (row + 8 * h) * kd) for h in range(2)]
            for a in range(16):
                re, im = times_row(fine, coarse[a // 8], a % 8)
                if ct == 0:
                    even = kd & 7 == 0
                    top = jnp.where(even, re, 0.0), jnp.where(lane == 0, 1.0, jnp.where(even, im, 0.0))
                    bottom = jnp.where(even, 0.0, re), jnp.where(even, 0.0, im)
                else:
                    sign = jnp.where(kd & 7 == ra, 1.0, -1.0)
                    top, bottom = (re, im), (-sign * im, sign * re)
                for i in range(2):
                    wide[2 * ct + i, pl.ds(8 * a, 8), :] = top[i].astype(BF16)
                    wide[2 * ct + i, pl.ds(128 + 8 * a, 8), :] = bottom[i].astype(BF16)

    def make_s_fwd(t):
        row, lane = lax.broadcasted_iota(jnp.int32, (8, 128), 0), _lane(8)
        pos = 8 * (lane >> 1) + t
        fine = unit((lane & 1) * (S // 4) - 4 * row * pos)
        shift, coarse = unit(-row * pos), unit(-32 * row * pos)
        for e in range(4):
            base = times_row(fine, shift, e)
            for g in range(8):
                for i, v in enumerate(times_row(base, coarse, g)):
                    sfw[t * 4 + e, pl.ds(16 * g + 8 * i, 8), :] = v.astype(BF16)

    def make_s_inv(e):
        row, lane = lax.broadcasted_iota(jnp.int32, (8, 128), 0), _lane(8)
        freq = 4 * (lane >> 1) + e
        fine = [v * (1.0 / S) for v in unit((lane & 1) * (S // 4) + 8 * row * freq)]
        shift, coarse = unit(row * freq), unit(64 * row * freq)
        for t in range(8):
            base = times_row(fine, shift, t)
            for g in range(8):
                for i, v in enumerate(times_row(base, coarse, g)):
                    siv[t * 4 + e, pl.ds(64 * i + 8 * g, 8), :] = v.astype(BF16)

    def prep_filter(ri, m):
        sub = lax.broadcasted_iota(jnp.int32, (8, 128), 0)
        edge = (wr_edge, wi_edge)[ri]
        res = {}
        for i in range(8):
            words = wraw32[ri, m, pl.ds(i, 32, stride=8), :]
            res[2 * i], res[2 * i + 1] = _unpack(words, 0), _unpack(words, 1)
        first = res[0][0:8]
        dst = pl.ds((m % 2) * 16 + ri * 8, 8)
        prev = jnp.zeros((8, 128), F32) if m < 2 else side[1, dst, :]
        put(side.at[1, dst, :], jnp.where(sub == m // 2, jnp.broadcast_to(first[0:1], (8, 128)), prev))
        nyq = jnp.broadcast_to(edge[0:1, pl.ds(m * 128, 128)].astype(F32), (8, 128))
        res[0] = jnp.concatenate([jnp.where(sub == 0, nyq, first), res[0][8:]], axis=0)
        for ct, (ra, rb) in enumerate(PAIRS):
            blk = jnp.concatenate([res[p] for p in _residues(ra) + _residues(rb)], axis=0)
            o = _dot_nt(lhs(small32[16]), blk.astype(BF16))
            for e in range(4):
                put(wf.at[ri, ct, e, m // 2, pl.ds((m % 2) * 32, 32), :], o[e * 32:(e + 1) * 32])

    def prep_wqkv_cross(g, r):
        pos = (_lane(8) >> 2) & 7
        u = [wqkv_raw32[g * NT + (-j) % 8, pl.ds(r * 8, 8), :] for j in range(NT)]
        u[0], u[4] = gate(u[0]), gate(u[4])
        for bit in range(3):
            m = ((pos >> bit) & 1) == 1
            u = [lax.select(m, u[(j - (1 << bit)) % 8], u[j]) for j in range(NT)]
        for j in range(NT):
            if j < 4:
                pin(u[j])
            put(wtmp.at[j, pl.ds(r * 8, 8), :], u[j])

    def prep_wqkv_pair(g, p, part):
        lane = _lane(8)
        ws = {}
        for n in range(2):
            index = (lane & 3) * 32 + (((lane >> 2) + 2 * p + n) & 7) * 4 + (lane >> 5)
            for half in range(2):
                for r in range(part * 2, part * 2 + 2):
                    w = gate(wtmp[2 * p + n, pl.ds(half * 256 + r * 8, 8), :])
                    ws[r, half, n] = jnp.take_along_axis(w, index, axis=1)
        yield from _latency()
        for r in range(part * 2, part * 2 + 2):
            quad = [ws[r, half, n] for half in range(2) for n in range(2)]
            ops = [_strassen_rhs(*[_unpack(w, i) for w in quad]) for i in range(2)]
            for k in range(7):
                word = {1: quad[0], 4: quad[3]}.get(k)
                if word is None:
                    word = pack(ops[0][k], ops[1][k])
                if k in (2, 3):
                    pin(word)
                put(wqkv32.at[g * 4 + p, k, pl.ds(r * 8, 8), :], word)

    def add_prep_wqkv(sched, tick, g, ticks, pair_ticks):
        for r in range(64):
            sched.add(tick + r * ticks / 64, _once(prep_wqkv_cross, g, r))
        tick = int(tick + ticks) + 1
        done = []
        for p, n in enumerate(pair_ticks):
            for i in range(16):
                sched.add(tick + i * n / 16, prep_wqkv_pair(g, p, i))
            tick += n
            done.append(int(tick) + XGAP + 1)
        return done

    def prep_wo(p, part):
        v, pair = divmod(part, 2)
        upper = lax.broadcasted_iota(jnp.int32, (8, 128), 0) >= 4
        ws = [[wo_raw32[2 * p + n, pl.ds(128 * v + 2 * f + pair, 8, stride=16), :] for f in range(8)]
              for n in range(2)]
        for o in range(4):
            quad = [lax.select(upper, w[(2 * v + 1 + j) % 8], w[(2 * v + j) % 8])
                    for j in (o, o + 4) for w in ws]
            quad[0] = gate(quad[0])
            for i in range(2):
                for k, x in enumerate(_strassen_rhs(*[_unpack(w, i) for w in quad])):
                    if k in (2, 3):
                        pin(x)
                    wo[p, k, pl.ds(o * 128 + (2 * pair + i) * 32 + 8 * v, 8), :] = x.astype(BF16)
            if o < 3:
                yield

    def ln_stats(xs):
        lane_mean = _tree(_add, xs) * (1.0 / NT)
        lane_m2 = _tree(_add, [jnp.square(x - lane_mean) for x in xs])
        pin(lane_m2)
        mean = jnp.sum(lane_mean, axis=1, keepdims=True) * (1.0 / 128)
        yield from _latency()
        m2 = lane_m2 + jnp.square(gate(lane_mean) - mean) * float(NT)
        pin(m2)
        var = jnp.sum(m2, axis=1, keepdims=True) * (1.0 / D)
        yield from _latency()
        return mean, lax.rsqrt(gate(jnp.broadcast_to(var, (16, 128))) + EPS)

    def d_fwd_rows(b, lb, from_input=False):
        xs = load_x(b, lb, from_input)

        def emit(r, v):
            if r % 4 == 0 or (r < 4 and not from_input):
                pin(v)
            ubuf[b % RING, r, r16(lb), :] = v.astype(BF16)

        xs[:4] = [gate(x, ILAG if from_input else GLAG) for x in xs[:4]]
        inv = yield from _d_butterfly_fwd(xs, emit, pin, from_input)
        inv = jnp.broadcast_to(inv, (16, 128))
        pin(inv)
        put(uout.at[b % RING, 8, r16(lb), :], inv)

    def d_dots(b, base, per_tick):
        for r in range(8):
            o = _dot(lhs(ubuf32[b % RING, r]), bf(small32[base + r]))
            put(uout.at[b % RING, r], o)
            if r % per_tick == per_tick - 1 and r < 7:
                yield

    def d_dots_wide(b):
        for ct, (ra, rb) in enumerate(PAIRS):
            u = lhs(ubuf32[b % RING, ra], ubuf32[b % RING, rb])
            for i, r in enumerate((ra, rb)):
                o = _dot(u, bf(wide32[2 * ct + i]))
                put(uout.at[b % RING, r], ticking(o) if i else o)
            if ct < 3:
                yield

    def d_fwd_cols(b, ct, is_wide):
        c, t = divmod(b, 8)
        ra, rb = PAIRS[ct]
        lane = _lane(16)
        lo = lane < 64
        z, x0 = [], []
        for lb in range(4):
            a, bb, inv = (uout[b % RING, r, r16(lb), :] for r in (ra, rb, 8))
            inv = gate(inv, ILAG if is_wide else GLAG)
            a, bb = a * inv, bb * inv
            if is_wide:
                if ct == 0:
                    x0.append(pltpu.roll(bb, t, 1) if t else bb)
                    bb = jnp.where(lane == 0, 0.0, bb)
                z.append((a, bb))
                continue
            if ct == 0:
                x0.append(pltpu.roll(a, (t + 64) % 128, 1))
                a = jnp.where(lane == 64, 0.0, a)
            im = lax.select(lo, bb, a)
            z.append((lax.select(lo, a, bb), _swap(im)))
        if not is_wide:
            yield from _latency()
        for e, (re, im) in enumerate(_dft4(z, False)):
            words = pack(re, im)
            if e < 2:
                pin(words)
            put(zin.at[ct, t * 4 + e, r16(c), :], words)
        if is_wide and ct == 0:
            yield from _latency()
        for lb, v in enumerate(x0):
            ls = pl.ds(64 * lb + 16 * c, 16)
            prev = jnp.zeros((16, 128), F32) if t == 0 else side[0, ls, :]
            v = jnp.where(lane == t, v, prev)
            pin(v)
            put(side.at[0, ls, :], v)

    def add_d_fwd(sched, tick, b, gap, per_tick=4, from_input=False):
        for lb in range(4):
            sched.add(tick + lb * gap, d_fwd_rows(b, lb, from_input))
        tick = int(tick + 3 * gap) + XGAP + 1
        sched.add(tick, d_dots_wide(b) if from_input else d_dots(b, 0, per_tick))
        for ct in range(4):
            sched.add(tick + 8 // per_tick + 3 + ct * gap, d_fwd_cols(b, ct, from_input))
        return int(tick + 8 // per_tick + 3 + 3 * gap) + XGAP + 1

    def side_path():
        vt = side[0].T[0:8]
        yield
        zero8 = jnp.zeros((8, 256), F32)
        u = _dot(jnp.concatenate([vt, zero8], axis=0).astype(BF16), f256[...])[0:8]
        twr, twi = tw_ref[0:8, :], tw_ref[8:16, :]
        ur, ui = u[:, 0:256], u[:, 256:512]
        pad = jnp.zeros((112, 256), BF16)
        for _ in range(4):
            yield
        uu = jnp.concatenate([ur * twr - ui * twi, ur * twi + ui * twr], axis=0).astype(BF16)
        xk = _dot(d8_ref[0], jnp.concatenate([uu, pad], axis=0))
        for _ in range(4):
            yield
        wr = jnp.concatenate([side[1, 0:8, :], side[1, 16:24, :]], axis=1)
        wi = jnp.concatenate([side[1, 8:16, :], side[1, 24:32, :]], axis=1)
        xr, xi = xk[0:8], xk[8:16]
        yy = jnp.concatenate([xr * wr - xi * wi, xr * wi + xi * wr], axis=0).astype(BF16)
        p = _dot(d8_ref[1], jnp.concatenate([yy, pad], axis=0))
        for _ in range(4):
            yield
        twr, twi = tw_ref[0:8, :], tw_ref[8:16, :]
        pr, pi = p[0:8], p[8:16]
        g = jnp.concatenate([pr * twr + pi * twi, pi * twr - pr * twi], axis=1)
        g = jnp.concatenate([g, jnp.zeros((8, 512), F32)], axis=0).astype(BF16)
        y0 = _dot_nt(g, f256[...])
        for _ in range(4):
            yield
        put(side.at[2], jnp.concatenate([y0, jnp.zeros((112, 256), F32)], axis=0).T)

    def s_fwd(u, t):
        ct, e = divmod(u, 4)
        o = _dot(lhs(sfw32[t * 4 + e]), bf(zin[ct, t * 4 + e]))
        put(zout.at[ct, t * 4 + e], o if t % 2 else ticking(o))

    def s_filter(u, g):
        ct, e = divmod(u, 4)
        z = [tuple(zout[ct, t * 4 + e, pl.ds(g * 16 + i, 8), :] for i in (0, 8)) for t in range(8)]
        z[0], z[1] = [tuple(gate(v, SGLAG) for v in zz) for zz in z[0:2]]
        xk = _dft8(z, False)
        for k2 in range(8):
            wr = wf[0, ct, e, k2, pl.ds(g * 8, 8), :]
            wi = wf[1, ct, e, k2, pl.ds(g * 8, 8), :]
            re, im = xk[k2]
            xk[k2] = (re * wr - im * wi, re * wi + im * wr)
        for t, (re, im) in enumerate(_dft8(xk, True)):
            words = pack(re, im)
            if t < 4:
                pin(words)
            put(zin.at[ct, t * 4 + e, pl.ds(g * 8, 8), :], words)

    def s_inv(u, t):
        ct, e = divmod(u, 4)
        o = _dot(lhs(siv32[t * 4 + e]), bf(zin[ct, t * 4 + e]))
        put(zout.at[ct, t * 4 + e], o if t % 2 else ticking(o))

    def add_s_stage(sched, early, ready, t1, pause):
        ahead = 4 + S_LAG
        tick = early
        for t in sorted(range(8), key=lambda t: ready[t]):
            for i in range(t, 2 * ahead, 8):
                tick = max(tick + 0.5, ready[t])
                sched.add(tick, _once(s_fwd, i // 8, t))
        t1 = max(t1, int(tick) + 1)
        t2 = pause(t1 + 64 - ahead, t1 + 64)
        sched.add(max(max(ready), t2), side_path())
        for i in range(64):
            if i + ahead < 64:
                sched.add(t1 + i, _once(s_fwd, *divmod(2 * (i + ahead), 8)))
            sched.add(t1 + i, _once(s_filter, *divmod(i, 4)))
            if i + ahead < 64:
                sched.add(t1 + i, _once(s_fwd, *divmod(2 * (i + ahead) + 1, 8)))
        for i in range(69):
            if i >= 5:
                sched.add(t2 + min(i, 66), _once(s_inv, *divmod(2 * (i - 5), 8)))
            if i < 64:
                sched.add(t2 + i, _once(s_filter, i // 4, 4 + i % 4))
            if i >= 5:
                sched.add(t2 + min(i, 66), _once(s_inv, *divmod(2 * (i - 5) + 1, 8)))
        return [t2 + 16 * ct + 22 for ct in range(3)] + [t2 + 67]

    def d_inv_cols(b, ct):
        c, t = divmod(b, 8)
        ra, rb = PAIRS[ct]
        lane = _lane(16)
        lo = lane < 64
        u = [(zout[ct, t * 4 + e, r16(c), :], zout[ct, t * 4 + e, r16(4 + c), :]) for e in range(4)]
        u[0], u[1] = tuple(map(gate, u[0])), tuple(map(gate, u[1]))
        z = _dft4(u, True)
        z = [(re, _swap(im)) for re, im in z]
        if ct == 0:
            y0 = [pltpu.roll(side[2, pl.ds(64 * lb + 16 * c, 16), :], 64 - t, 1) for lb in range(4)]
        yield from _latency()
        for lb, (re, sw) in enumerate(z):
            sw = gate(sw)
            a, bb = lax.select(lo, re, sw), lax.select(lo, sw, re)
            if ct == 0:
                a = jnp.where(lane == 64, y0[lb], a)
            pin(a)
            ubuf[b % RING, ra, r16(lb), :] = a.astype(BF16)
            ubuf[b % RING, rb, r16(lb), :] = bb.astype(BF16)

    def d_inv_rows(b, lb, stats, first):
        u = [uout[b % RING, r, r16(lb), :] for r in range(8)]
        ys = yield from _d_butterfly_inv([gate(v) if r < 4 else v for r, v in enumerate(u)], pin, gate)
        xs = [x + y for x, y in zip(load_x(b, lb, first), ys)]
        for j in range(NT):
            put(xres.at[b, j, r16(lb), :], xs[j])
        stats[b, lb] = yield from ln_stats(xs)
        if b % 2:
            for j in range(4):
                a = [(xres[bb, j + o, r16(lb), :] - stats[bb, lb][0]) * stats[bb, lb][1]
                     for bb in (b - 1, b) for o in (0, 4)]
                a[0], a[3] = gate(a[0]), gate(a[3])
                for k, v in enumerate(_strassen_lhs(*a)):
                    if k in (1, 4):
                        pin(v)
                    abuf[b // 2, k, j, r16(lb), :] = v.astype(BF16)
                if j < 3:
                    yield

    def add_d_inv(sched, tick, b, gap, stats, first, cols=None):
        per_tick = 4
        cols = cols or [tick + ct * gap for ct in range(4)]
        for ct in range(4):
            sched.add(cols[ct], d_inv_cols(b, ct))
        tick = int(cols[3]) + XGAP + 1
        sched.add(tick, d_dots(b, 8, per_tick))
        tick += 8 // per_tick + 3
        for lb in range(4):
            sched.add(tick + lb * gap, d_inv_rows(b, lb, stats, first))
        return int(tick + 3 * gap) + 3 * XGAP + 1 + 4

    def gemm(lhs32, rhs32, jobs, sink):
        for slot, b, n in jobs:
            m = {}
            for k in (3, 1, 0, 6, 5, 4, 2):
                m[k] = ticking(_dot(lhs(*[lhs32[slot, k, j] for j in range(4)]), bf(rhs32[n // 2, k])))
                if k == 1:
                    sink(b + 1, n, m[1] - m[3])
                elif k == 0:
                    c11, c22 = m[3] - m[0], m[1] - m[0]
                elif k == 6:
                    c11 = m[6] - c11
                elif k == 5:
                    c22 = m[5] - c22
                elif k == 4:
                    sink(b, n, c11 - m[4])
                elif k == 2:
                    sink(b, n + 1, m[4] - m[2])
                    sink(b + 1, n + 1, c22 - m[2])
                yield

    def qkv_sink(b, n, o):
        c, t = divmod(b, 8)
        dst = (qbuf, kbuf, vbuf)[n // NT]
        for lb in range(4):
            put(dst.at[n % NT, t, pl.ds(8 + 64 * lb + 16 * c, 16), :], o[lb * 16:(lb + 1) * 16])
        if b == 0 and n >= NT:
            first = jnp.broadcast_to(o[0:1], (8, 128))
            for tt in range(8):
                dst[n % NT, tt, pl.ds(0, 8), :] = first

    def out_rows(r, i, last):
        c, t = divmod(r, 8)
        return (c * 8 + t % 2 * 4 + i, t // 2) if last and c == 0 else (r, i)

    def out_sink(last, r, n, o):
        for i in range(4):
            b, lb = out_rows(r, i, last)
            put(xres.at[b, n, r16(lb), :], xres[b, n, r16(lb), :] + o[i * 16:(i + 1) * 16])

    def attention(b, lb, h):
        c, t = divmod(b, 8)
        log2e = float(np.log2(np.e))
        scale = HEAD_DIM ** -0.5 * log2e
        r0 = 8 + 64 * lb + 16 * c + 8 * h
        src = [((t - 2 * w) % 8, -((t - 2 * w) // 8)) for w in range(WIN)]
        acc = [None] * WIN
        for j in range(NT):
            if j % 2 == 0:
                factor = gate(jnp.full((8, 128), scale, F32), ALAG)
            q = qbuf[j, t, pl.ds(r0, 8), :] * factor
            for w, (ts, sh) in enumerate(src):
                p = q * kbuf[j, ts, pl.ds(r0 - sh, 8), :]
                acc[w] = p if j == 0 else acc[w] + p
            if j % 2 and j < NT - 1:
                pin(*acc[j // 2 % 2::2])
                yield
        part = [(r, pltpu.roll(r, 64, 1)) for r in acc]
        yield from _latency()
        part = [r + rr for r, rr in part]
        part = [(r, pltpu.roll(r, 32, 1)) for r in part]
        yield from _latency()
        logits = [r + rr for r, rr in part]
        if r0 == 8:
            sub = lax.broadcasted_iota(jnp.int32, (8, 128), 0)
            logits = [jnp.where(sub >= sh, r, -1e9 * log2e) if sh else r
                      for r, (_, sh) in zip(logits, src)]
        logits[0] = gate(logits[0], ALAG)
        m = _tree(jnp.maximum, logits)
        ps = [jnp.exp2(r - m) for r in logits]
        total = _tree(_add, ps)
        pin(total)
        inv = pltpu.reciprocal(total, approx=True)
        inv = inv * (2.0 - total * inv)
        for j in range(NT):
            if j % 2 == 0:
                yield
                ps[0], ps[4] = gate(ps[0], ALAG), gate(ps[4], ALAG)
            o = _chain(_add, [ps[w] * vbuf[j, ts, pl.ds(r0 - sh, 8), :]
                              for w, (ts, sh) in enumerate(src)]) * inv
            if j % 2:
                pin(o)
            put(qbuf.at[j, t, pl.ds(r0, 8), :], o)

    def out_operands(r, i, last):
        for j in range(4):
            a = [qbuf[j + o, b % 8, pl.ds(8 + 64 * lb + 16 * (b // 8), 16), :]
                 for b, lb in (out_rows(r, i, last), out_rows(r + 1, i, last)) for o in (0, 4)]
            a[0], a[3] = gate(a[0]), gate(a[3])
            for k, v in enumerate(_strassen_lhs(*a)):
                if k in (1, 4):
                    pin(v)
                obuf[r // 2, k, j, r16(i), :] = v.astype(BF16)
            if j < 3:
                yield

    def store_rows(b, lb):
        c, t = divmod(b, 8)
        for j in range(NT):
            words = pack(xres[b, j, r16(lb), :], xres[b + 1, j, r16(lb), :])
            pin(words)
            io32[j, lb, c, pl.ds(t // 2, 16, stride=4), :] = words

    unit_ticks = NT + 2 * XGAP
    step = 2
    out_ticks = 28

    def add_proj(sched, tick, c, lo, hi):
        jobs = [(b // step, b, n) for b in range(8 * c, 8 * c + 8, step) for n in range(lo, hi, step)]
        sched.add(tick, gemm(abuf32, wqkv32, jobs, qkv_sink))
        return tick + len(jobs) * out_ticks * step // NT

    def add_attention(sched, tick, pace, rows, last):
        units = [(r, i, half, h) for r in rows[::2] for i in range(4) for half in range(2) for h in range(2)]
        for n, (r, i, half, h) in enumerate(units):
            sched.add(tick + n * pace, attention(*out_rows(r + half, i, last), h))
            if half and h:
                sched.add(int(tick + n * pace) + unit_ticks, out_operands(r, i, last))

    def add_out(sched, tick, rows, last):
        jobs = [(r // 2, r, n) for r in rows[::2] for n in range(0, NT, 2)]
        sched.add(tick, gemm(obuf32, wo32, jobs, functools.partial(out_sink, last)))

    def add_tail(sched, tick, rows, last):
        ready = {}
        for i, r in enumerate(rows):
            t0 = tick + (i // 2 + 1) * out_ticks
            fast = i >= len(rows) - (2 if last else 4)
            if not last:
                t0 += 0 if fast else TOFF + i % 2 * out_ticks // 2
                ready[r % 8] = add_d_fwd(sched, t0, r, i % 2 if fast else out_ticks / 8)
            elif r % 2:
                c, p = r // 8, r % 8 // 2
                gap = 0 if fast else 3
                for j in range(4):
                    sched.add(t0 + (j + 1) * gap, _once(store_rows, *((r - 1, j) if c else (2 * j, p))))
                for lb in ([p] if c == 0 else range(4) if p == 3 else []):
                    sched.add(t0 + 5 * gap + 1, _once(start, out_copies(c, lb)))
        return ready

    q_ticks = 8 * out_ticks // step
    att_ticks = unit_ticks + 1 + 2
    order = [(a + 8) % NB for a in range(NB)]

    def add_attention_block(sched, cols, last):
        stats = {}
        t0 = max([add_d_inv(sched, 0, b, 0, stats, not last, cols) for b in range(step)])
        if not last:
            sched.add(cols[3] - KLEAD, _once(wait, qkv_copies(1) + dmat_cp))
            done = add_prep_wqkv(sched, cols[3] - KLEAD, 1, KPACE, [7] * 4)
            t0 = max(t0, done[0])
            assert all(d <= t0 + p * out_ticks / 4 for p, d in enumerate(done))
            sched.add(t0 + out_ticks, _once(wait, qkv_copies(2)))
            sched.add(t0 + out_ticks, _once(start, qkv_copies(0)))
            done = add_prep_wqkv(sched, t0 + out_ticks, 2, 2 * out_ticks - 4, [out_ticks - 4] * 4)
            assert all(d <= t0 + q_ticks + p * out_ticks for p, d in enumerate(done))
            sched.add(t0 + 2 * q_ticks, _once(wait, qkv_copies(0)))
            sched.add(t0 + 2 * q_ticks, _once(start, wo_copies))
            done = add_prep_wqkv(sched, t0 + 2 * q_ticks, 0, q_ticks - 10, [q_ticks / 4] * 4)
            assert done[-1] <= t0 + 4 * q_ticks
            sched.add(t0 + 8 * q_ticks, _once(wait, wo_copies))
            for i in range(32):
                sched.add(t0 + 8 * q_ticks + i * q_ticks / 16, prep_wo(*divmod(i, 8)))
        tick, kv_start, q_start = t0, {}, {}
        for kind, c in ("k0", "k1", "q1", "k2", "q2", "k3", "q3", "q0"):
            if kind == "k":
                kv_start[int(c)] = tick
                if c == "0" and not last:
                    tick = add_proj(sched, tick, 0, NT, 2 * NT)
                    jobs = [(b // step, b, n) for n in range(2 * NT, 3 * NT, step) for b in range(0, 8, step)]
                    sched.add(tick, gemm(abuf32, wqkv32, jobs, qkv_sink))
                    tick += q_ticks
                    continue
                tick = add_proj(sched, tick, int(c), NT, 3 * NT)
            else:
                q_start[int(c)] = tick
                tick = add_proj(sched, tick, int(c), 0, NT)
        pace = 2 * out_ticks / step
        for b in range(step, NB):
            due = kv_start[b // 8] + (b % 8 // step) * (2 if last or b >= 8 else 1) * out_ticks
            gap = min(1 + (b - step) * 0.5, DGAP1 if last else DGAP0)
            pace = DPACE1 if last else DPACE0
            at = (b - step) * pace
            at = t0 + at + max(0, at - 4 * q_ticks - out_ticks) * DSLOW
            if not last and b < 8:
                at, gap = max(cols[3], t0 + (b // step - 1) * out_ticks - (step - b % step) * 8), 1
            end = add_d_inv(sched, at, b, gap, stats, not last)
            assert end <= due, (b, end, due)
        begin = [q_start[c] + out_ticks + 3 for c in (1, 2, 3)] + [tick + (ATT1 if last else ATT0)]
        begin.append(tick + (NB // step - 1) * out_ticks - att_ticks)
        for i, c in enumerate((1, 2, 3, 0)):
            pace = (begin[i + 1] - begin[i]) / 64
            assert begin[i] >= max(kv_start[c], kv_start[(c - 1) % 4]) + 2 * q_ticks
            for p in range(4):
                assert begin[i] + 16 * p * pace >= q_start[c] + (4 if last and c == 0 else p + 1) * out_ticks
                assert begin[i] + (16 * p + 15) * pace + att_ticks <= tick + (4 * i + p) * out_ticks + 1e-6
            add_attention(sched, begin[i], pace, range(8 * c, 8 * c + 8), last)
        add_out(sched, tick, order, last)
        return tick + (NB // step) * out_ticks, add_tail(sched, tick, order, last)

    def add_input(sched):
        ready = {}
        after = (x_copies(2), x_copies(3) + perm_cp + w_copies(0) + w_copies(1),
                 w_copies(2) + w_copies(3), w_copies(4))
        for c in range(NC):
            sched.add(c * 32, _once(wait, x_copies(c)))
            sched.add(c * 32, _once(start, after[c]))
            for t in range(8):
                ready[t] = add_d_fwd(sched, c * 32 + t * 4, c * 8 + t, 1, 2, True)
        return 128 + 9, ready

    def add_filter_prep(sched, upper, begin, end):
        after = (w_copies(5) + w_copies(6), w_copies(7) + f256_cp + dmat_cp, [], qkv_copies(2))
        for i in range(16):
            g, at = 4 * upper + i // 4, begin + i * (end - begin) / 16
            if i % 8 == 0:
                sched.add(at, _once(wait, w_copies(g) + w_copies(g + 1) + {0: perm_cp, 6: f256_cp}.get(g, [])))
                sched.add(at, _once(start, after[g // 2]))
            sched.add(at, _once(prep_filter, *w_tiles(g)[i % 4]))
        return end + 2

    def add_first_s_stage(sched):
        tick, ready = add_input(sched)
        sched.add(tick + WK0, _once(start, qkv_copies(1)))
        return add_s_stage(sched, tick, ready, add_filter_prep(sched, 0, F0, tick),
                           lambda begin, end: add_filter_prep(sched, 1, begin, end + FG))

    sched = _Schedule()

    start(x_copies(0))
    for ref in (abuf32, obuf32, ubuf32, wo32, sfw32, siv32, wide32):
        put(ref.at[(0,) * (len(ref.shape) - 2) + (pl.ds(0, 8),)], jnp.zeros((8, 128), U32))
    make_wide()
    start(x_copies(1))
    for t in range(8):
        make_s_fwd(t)
    for e in range(4):
        make_s_inv(e)
    cols = add_first_s_stage(sched)
    tick, ready = add_attention_block(sched, cols, False)
    cols = add_s_stage(sched, tick, ready, tick, lambda begin, end: end)
    add_attention_block(sched, cols, True)
    sched.run()
    for c in range(NC):
        for lb in range(4):
            wait(out_copies(c, lb))


@jax.jit
def pallas_interleave_layers__spectral_gfnet__sliding_local_dilated__prompt_kernel(
    A_x: jax.Array,
    A_w_r: jax.Array,
    A_w_i: jax.Array,
    B_x: jax.Array,
    B_wqkv: jax.Array,
    B_wo: jax.Array,
):
    del B_x
    assert A_x.shape == (1, S, D) and A_w_r.shape == (S, D // 2 + 1)
    cst = _constants()
    x = A_x.astype(BF16).reshape(4, NC, 128, D)
    wr, wi = A_w_r.astype(BF16).T, A_w_i.astype(BF16).T
    hbm = pl.BlockSpec(memory_space=pl.ANY)
    edge = pl.BlockSpec((16, S), lambda i: (D // 32, 0))
    vm = pltpu.VMEM
    out = pl.pallas_call(
        _kernel,
        grid=(1,),
        in_specs=[hbm, hbm, hbm, edge, edge, hbm, hbm, hbm, hbm,
                  pl.BlockSpec((24, 256), lambda i: (0, 0)),
                  pl.BlockSpec((2, 16, 128), lambda i: (0, 0, 0))],
        out_specs=hbm,
        out_shape=jax.ShapeDtypeStruct((4, NC, 128, D), BF16),
        scratch_shapes=[
            vm((NT, 4, NC, 128, 128), BF16),
            vm((17, 128, 128), BF16),
            vm((32, 128, 128), BF16),
            vm((32, 128, 128), BF16),
            vm((256, 512), BF16),
            vm((2, 16, 512, 128), BF16),
            vm((2, 4, 4, 8, 64, 128), F32),
            vm((3 * NT, D, 128), BF16),
            vm((NT, D // 2, 128), U32),
            vm((12, 7, 512, 128), BF16),
            vm((NT, D, 128), BF16),
            vm((4, 7, 512, 128), BF16),
            vm((NB, NT, 64, 128), F32),
            vm((4, 32, 64, 128), U32),
            vm((4, 32, 128, 128), F32),
            vm((RING, 8, 64, 128), BF16),
            vm((RING, 9, 64, 128), F32),
            vm((NB // 2, 7, 4, 64, 128), BF16),
            vm((NB // 2, 7, 4, 64, 128), BF16),
            vm((NT, 8, 264, 128), F32),
            vm((NT, 8, 264, 128), F32),
            vm((NT, 8, 264, 128), F32),
            vm((3, 256, 128), F32),
            vm((8, 256, 128), BF16),
            pltpu.SemaphoreType.DMA((NC,)),
            pltpu.SemaphoreType.DMA((3,)),
            pltpu.SemaphoreType.DMA((8,)),
            pltpu.SemaphoreType.DMA((3,)),
            pltpu.SemaphoreType.DMA(()),
            pltpu.SemaphoreType.DMA(()),
        ],
        compiler_params=pltpu.CompilerParams(
            dimension_semantics=("arbitrary",), vmem_limit_bytes=120 * 2**20),
    )(x, wr, wi, wr, wi, B_wqkv.astype(BF16), B_wo.astype(BF16),
      cst["small"], cst["f256"], cst["tw"], cst["d8"])
    return out.reshape(1, S, D)
```

```python
import functools

import jax
import jax.numpy as jnp
import numpy as np
from jax import lax
from jax.experimental import pallas as pl
from jax.experimental.pallas import tpu as pltpu

S, D = 2048, 1024
NT = D // 128
NC = 4
WIN = 8
HEAD_DIM = 32
EPS = 1e-5
F32, BF16, U32 = jnp.float32, jnp.bfloat16, jnp.uint32
PAIRS = ((0, 4), (1, 7), (2, 6), (3, 5))
RSQ2 = float(np.sqrt(0.5))
NB = S // 64

RING = 8
XGAP = 3
GLAG = 4
ALAG = 4
SGLAG = 3
S_LAG = 2
F0 = 120
KLEAD = 46
KPACE = 40
DGAP0 = 4.75
DGAP1 = 4.2
DPACE0 = 20
DPACE1 = 15.5
DSLOW = 0.6
SYNC = 3
ILAG = 3
FG = 10
TOFF = 4
WK0 = 24
ATT0 = 15
ATT1 = 95


def _residues(r):
    return (0, 8) if r == 0 else (r, 16 - r)


def _d_matrices():
    n = np.arange(64)[:, None]
    a = np.arange(32)
    fwd = np.zeros((8, 128, 128))
    inv = np.zeros((8, 128, 128))
    for r in range(8):
        kd = np.concatenate([16 * a + p for p in _residues(r)])
        weight = np.full(64, 2.0)
        if r == 0:
            kd[0], weight[0] = D // 2, 1.0
            ph = np.exp(-2j * np.pi * n * kd[None, :] / D)
            sgn = np.where(kd % 16 == 0, 1.0, -1.0)[None, :]
            m = np.concatenate([ph, ph * sgn], axis=0)
            re, im = m.real.copy(), m.imag.copy()
            ire, iim = re.copy(), im.copy()
            im[:, 0] = 1.0
            iim[:, 0] = 1.0
        else:
            p = 12 if r == 4 else r
            ph = np.exp(-2j * np.pi * n * kd[None, :] / D)
            si = np.where(kd % 16 == p, 1.0, -1.0)[None, :]
            m = np.concatenate([ph, 1j * si * ph], axis=0)
            re, im = m.real, m.imag
            ire, iim = re, im
        swapped = r in (4, 7, 6, 5)
        cols = [im, re] if swapped else [re, im]
        icols = [iim * weight, ire * weight] if swapped else [ire * weight, iim * weight]
        fwd[r] = np.concatenate(cols, axis=1)
        inv[r] = np.concatenate(icols, axis=1).T / D
    return fwd, inv


def _side_matrices():
    l = np.arange(256)
    f = np.exp(-2j * np.pi * ((l[:, None] * l[None, :]) % 256) / 256)
    f256 = np.concatenate([f.real, f.imag], axis=1)
    t = np.arange(8)
    tw = np.exp(-2j * np.pi * t[:, None] * l[None, :] / S)
    tw = np.concatenate([tw.real, tw.imag, np.zeros((8, 256))], axis=0)
    g = np.exp(-2j * np.pi * t[:, None] * t[None, :] / 8)
    d8 = np.zeros((2, 16, 128))
    d8[0, :, :16] = np.block([[g.real, -g.imag], [g.imag, g.real]])
    d8[1, :, :16] = d8[0, :, :16].T / S
    return f256, tw, d8


def _filter_rows():
    p = np.zeros((1, 128, 128))
    for k in range(32):
        for e in range(4):
            p[0, e * 32 + k, 4 * k + e] = 1.0
    return p


@functools.lru_cache(maxsize=None)
def _constants():
    dfw, div = _d_matrices()
    f256, tw, d8 = _side_matrices()
    small = np.concatenate([dfw, div, _filter_rows()], axis=0)
    b = lambda x: np.asarray(x, np.float32).astype(BF16)
    return dict(small=b(small), f256=b(f256),
                tw=np.asarray(tw, np.float32), d8=b(d8))


def _dot(a, b):
    return jnp.dot(a, b, preferred_element_type=F32)


def _dot_nt(a, b):
    return lax.dot_general(a, b, (((1,), (1,)), ((), ())), preferred_element_type=F32)


def _tree(op, xs):
    xs = list(xs)
    while len(xs) > 1:
        xs = [op(xs[i], xs[i + 1]) if i + 1 < len(xs) else xs[i] for i in range(0, len(xs), 2)]
    return xs[0]


def _chain(op, xs):
    return functools.reduce(op, xs)


def _lane(rows):
    return lax.broadcasted_iota(jnp.int32, (rows, 128), 1)


def _swap(x):
    return pltpu.roll(x, 64, 1)


def _unpack(w, i):
    return pltpu.unpack_elementwise(w, index=i, packed_dtype=BF16, unpacked_dtype=F32)


def _latency():
    for _ in range(XGAP):
        yield


def _add(a, b):
    return a + b


def _row_mean(xs):
    return jnp.sum(_tree(_add, xs), axis=1, keepdims=True) * (1.0 / D)


def _twiddle16(r, x, y):
    lo = _lane(x.shape[0]) < 64
    wr, wi = float(np.cos(np.pi * r / 8)), float(-np.sin(np.pi * r / 8))
    cross = jnp.where(lo, 0.0, wr)
    return x * jnp.where(lo, 1.0, wi) + y * cross, y * jnp.where(lo, 1.0, -wi) + x * cross


def _d_butterfly_fwd(a, emit, pin, wide):
    s = [a[j] + a[j + 4] for j in range(4)]
    e, o = s[0] + s[2], s[1] + s[3]
    total, t4 = e + o, e - o
    emit(4, t4)
    d0, nd2 = a[0] - a[4], a[6] - a[2]
    d1, d3 = a[1] - a[5], a[3] - a[7]
    p, q = (d1 - d3) * RSQ2, (d1 + d3) * -RSQ2
    ts = {1: (d0 + p, q + nd2), 2: (s[0] - s[2], s[3] - s[1]), 3: (d0 - p, q - nd2)}
    mean8 = jnp.sum(total, axis=1, keepdims=True) * (1.0 / 128)
    if wide:
        for r, (tr, ti) in ts.items():
            emit(r, tr)
            emit(8 - r, ti)
    else:
        ab = {r: _twiddle16(r, *t) for r, t in ts.items()}
        ab = {r: (a, _swap(b)) for r, (a, b) in ab.items()}
    dev = _tree(_add, [v * v for t in ts.values() for v in t]) * 2.0 + t4 * t4
    pin(dev)
    yield from _latency()
    t0 = total - mean8
    emit(0, t0)
    var = jnp.sum(dev + t0 * t0, axis=1, keepdims=True) * (1.0 / (NT * D))
    if not wide:
        for r, (x, y) in ab.items():
            emit(r, x + y)
            emit(8 - r, x - y)
    yield from _latency()
    return lax.rsqrt(var + EPS)


def _d_butterfly_inv(u, pin, gate):
    ab = {r: (u[r] + u[8 - r], _swap(u[r] - u[8 - r])) for r in (1, 2, 3)}
    e, o = u[0] + u[4], u[0] - u[4]
    yield from _latency()
    ts = {r: _twiddle16(r, x, gate(y)) for r, (x, y) in ab.items()}
    pin(*[t[0] for t in ts.values()])
    yield
    s = [e + ts[2][0], o - ts[2][1], e - ts[2][0], o + ts[2][1]]
    p = (ts[1][0] - ts[3][0]) * RSQ2
    q = (ts[1][1] + ts[3][1]) * RSQ2
    d0, d1, d2, nd3 = ts[1][0] + ts[3][0], p - q, ts[3][1] - ts[1][1], p + q
    return [s[0] + d0, s[1] + d1, s[2] + d2, s[3] - nd3,
            s[0] - d0, s[1] - d1, s[2] - d2, s[3] + nd3]


def _strassen_lhs(a11, a12, a21, a22):
    return [a11 + a22, a21 + a22, a11, a22, a11 + a12, a21 - a11, a12 - a22]


def _strassen_rhs(b11, b12, b21, b22):
    return [b11 + b22, b11, b22 - b12, b11 - b21, b22, b11 + b12, b21 + b22]


def _cadd(a, b):
    return a[0] + b[0], a[1] + b[1]


def _csub(a, b):
    return a[0] - b[0], a[1] - b[1]


def _dft4(z, inverse):
    a, b = _cadd(z[0], z[2]), _csub(z[0], z[2])
    c, d = _cadd(z[1], z[3]), _csub(z[1], z[3])
    minus = (b[0] + d[1], b[1] - d[0])
    plus = (b[0] - d[1], b[1] + d[0])
    return [_cadd(a, c), plus if inverse else minus, _csub(a, c), minus if inverse else plus]


def _dft8(z, inverse):
    ev = _dft4(z[0::2], inverse)
    od = _dft4(z[1::2], inverse)
    out = [None] * 8
    out[0], out[4] = _cadd(ev[0], od[0]), _csub(ev[0], od[0])
    (er, ei), (x, y) = ev[2], od[2]
    minus, plus = (er + y, ei - x), (er - y, ei + x)
    out[2], out[6] = (plus, minus) if inverse else (minus, plus)
    for k in (1, 3):
        (er, ei), (x, y) = ev[k], od[k]
        sm, df = (x + y) * RSQ2, (x - y) * RSQ2
        if not inverse:
            if k == 1:
                out[1], out[5] = (er + sm, ei - df), (er - sm, ei + df)
            else:
                out[3], out[7] = (er - df, ei - sm), (er + df, ei + sm)
        else:
            if k == 1:
                out[1], out[5] = (er + df, ei + sm), (er - df, ei - sm)
            else:
                out[3], out[7] = (er - sm, ei + df), (er + sm, ei - df)
    return out


class _Schedule:
    def __init__(self):
        self.pending = []

    def add(self, tick, gen):
        self.pending.append((int(tick), len(self.pending), gen))

    def run(self):
        pending = sorted(self.pending, key=lambda p: p[:2])
        active, tick, i = [], 0, 0
        while active or i < len(pending):
            while i < len(pending) and pending[i][0] <= tick:
                active.append(pending[i][2])
                i += 1
            for g in list(active):
                if next(g, 0) == 0:
                    active.remove(g)
            tick += 1
        self.pending = []


def _once(fn, *args):
    fn(*args)
    return
    yield


def _kernel(x_hbm, wr_hbm, wi_hbm, wr_edge, wi_edge, wqkv_hbm, wo_hbm,
            small_hbm, f256_hbm, tw_ref, d8_ref,
            out_hbm,
            io, small, sfw, siv, f256, wraw, wf, wqkv_raw, wtmp, wqkv, wo_raw, wo,
            xres, zin, zout, ubuf, uout, abuf, obuf, qbuf, kbuf, vbuf, side,
            wide, sem_x, sem_c, sem_w, sem_qkv, sem_wo, sem_out):

    def x_copies(c):
        return [pltpu.make_async_copy(x_hbm.at[:, c, :, pl.ds(j * 128, 128)], io.at[j, :, c],
                                      sem_x.at[c]) for j in range(NT)]

    def out_copies(c, lb, tiles):
        return [pltpu.make_async_copy(io.at[j, lb, c], out_hbm.at[lb, c, :, pl.ds(j * 128, 128)],
                                      sem_out) for j in tiles]

    perm_cp, dmat_cp, f256_cp = ([pltpu.make_async_copy(s, d, sem_c.at[i])] for i, (s, d) in enumerate((
        (small_hbm.at[pl.ds(16, 1)], small.at[pl.ds(16, 1)]),
        (small_hbm.at[pl.ds(0, 16)], small.at[pl.ds(0, 16)]), (f256_hbm, f256))))

    def w_tiles(g):
        return [(g // 2 % 2, 8 * (g % 2) + 2 * i + g // 4) for i in range(4)]

    def w_copies(g):
        return [pltpu.make_async_copy((wr_hbm, wi_hbm)[ri].at[pl.ds(0, 512), pl.ds(m * 128, 128)],
                                      wraw.at[ri, m], sem_w.at[g]) for ri, m in w_tiles(g)]

    def qkv_copies(g):
        return [pltpu.make_async_copy(wqkv_hbm.at[:, pl.ds(g * D + j * 128, 128)],
                                      wqkv_raw.at[g * NT + j], sem_qkv.at[g]) for j in range(NT)]

    wo_copies = [pltpu.make_async_copy(wo_hbm.at[:, pl.ds(j * 128, 128)], wo_raw.at[j], sem_wo)
                 for j in range(NT)]

    def start(cs):
        for cp in cs:
            cp.start()

    def wait(cs):
        for cp in cs:
            cp.wait()

    io32, wraw32, wo_raw32 = io.bitcast(U32), wraw.bitcast(U32), wo_raw.bitcast(U32)
    small32, sfw32, siv32, wide32 = (r.bitcast(U32) for r in (small, sfw, siv, wide))
    wqkv_raw32, wqkv32, wo32 = (r.bitcast(U32) for r in (wqkv_raw, wqkv, wo))
    ubuf32, abuf32, obuf32 = ubuf.bitcast(U32), abuf.bitcast(U32), obuf.bitcast(U32)

    never = tw_ref[16:24, 0:128] != 0.0
    never_wide = {n: jnp.concatenate([tw_ref[16:24, 0:128]] * n, axis=1) != 0.0 for n in (1, 2, 4)}
    token = {}

    def pin(*values):
        for v in values:
            key = v.shape[0], v.dtype == F32
            token[key] = (lax.max if key[1] else lax.bitwise_xor)(token[key], v) if key in token else v

    clock = []

    def gate(v, lag=GLAG):
        if len(clock) < lag:
            return v
        old = clock[-lag] if v.dtype == F32 else pltpu.bitcast(clock[-lag], v.dtype)
        if v.shape[0] == 8:
            return lax.select(never, old, v)
        return lax.concatenate([lax.select(never, old, v[0:8]), v[8:]], 0)

    def ticking(o):
        clock.append(o[0:8])
        del clock[:-16]
        return o

    def lhs(*tiles):
        if not token and len(tiles) == 4 and len(clock) >= SYNC:
            pin(clock[-SYNC])
        words = lax.concatenate(tiles, 1) if len(tiles) > 1 else tiles[0]
        if token:
            parts = [pltpu.bitcast(v, U32) if is_float else v for (_, is_float), v in token.items()]
            token.clear()
            w = _chain(lax.bitwise_xor, [v[i:i + 8] if v.shape[0] > 8 else v
                                         for v in parts for i in range(0, v.shape[0], 8)])
            w = lax.concatenate([w] * len(tiles), 1) if len(tiles) > 1 else w
            words = lax.concatenate([lax.select(never_wide[len(tiles)], w, words[0:8]), words[8:]], 0)
        return pltpu.bitcast(words, BF16)

    def bf(words):
        return pltpu.bitcast(words, BF16)

    def pack(a, b):
        return pltpu.bitcast(pltpu.pack_elementwise([a, b], packed_dtype=BF16), U32)

    def r16(i):
        return pl.ds(i * 16, 16)

    always = {}

    def put(ref, v):
        if v.shape not in always:
            always[v.shape] = jnp.ones(v.shape, jnp.bool_)
        pltpu.store(ref, v, mask=always[v.shape])

    def load_x(b, lb, from_input):
        if from_input:
            c, t = divmod(b, 8)
            return [_unpack(io32[j, lb, c, pl.ds(t // 2, 16, stride=4), :], t % 2) for j in range(NT)]
        return [xres[b, j, r16(lb), :] for j in range(NT)]

    def unit(p):
        angle = (((p + S // 2) & (S - 1)) - S // 2).astype(F32) * (2 * np.pi / S)
        return jnp.cos(angle), jnp.sin(angle)

    def times_row(a, b, i):
        br, bi = (jnp.broadcast_to(v[i:i + 1], (8, 128)) for v in b)
        return a[0] * br - a[1] * bi, a[0] * bi + a[1] * br

    def make_wide():
        row, lane = lax.broadcasted_iota(jnp.int32, (8, 128), 0), _lane(8)
        for ct, (ra, rb) in enumerate(PAIRS):
            res = _residues(ra) + _residues(rb)
            kd = (lane & 31) * 16 + _chain(
                _add, [jnp.where(lane >> 5 == g, p, 0) for g, p in enumerate(res)])
            if ct == 0:
                kd = jnp.where(lane == 0, D // 2, kd)
            fine, coarse = unit(-2 * row * kd), [unit(-16 * (row + 8 * h) * kd) for h in range(2)]
            for a in range(16):
                re, im = times_row(fine, coarse[a // 8], a % 8)
                if ct == 0:
                    even = kd & 7 == 0
                    top = jnp.where(even, re, 0.0), jnp.where(lane == 0, 1.0, jnp.where(even, im, 0.0))
                    bottom = jnp.where(even, 0.0, re), jnp.where(even, 0.0, im)
                else:
                    sign = jnp.where(kd & 7 == ra, 1.0, -1.0)
                    top, bottom = (re, im), (-sign * im, sign * re)
                for i in range(2):
                    wide[2 * ct + i, pl.ds(8 * a, 8), :] = top[i].astype(BF16)
                    wide[2 * ct + i, pl.ds(128 + 8 * a, 8), :] = bottom[i].astype(BF16)

    def make_s_fwd(t):
        row, lane = lax.broadcasted_iota(jnp.int32, (8, 128), 0), _lane(8)
        pos = 8 * (lane >> 1) + t
        fine = unit((lane & 1) * (S // 4) - 4 * row * pos)
        shift, coarse = unit(-row * pos), unit(-32 * row * pos)
        for e in range(4):
            base = times_row(fine, shift, e)
            for g in range(8):
                for i, v in enumerate(times_row(base, coarse, g)):
                    sfw[t * 4 + e, pl.ds(16 * g + 8 * i, 8), :] = v.astype(BF16)

    def make_s_inv(e):
        row, lane = lax.broadcasted_iota(jnp.int32, (8, 128), 0), _lane(8)
        freq = 4 * (lane >> 1) + e
        fine = [v * (1.0 / S) for v in unit((lane & 1) * (S // 4) + 8 * row * freq)]
        shift, coarse = unit(row * freq), unit(64 * row * freq)
        for t in range(8):
            base = times_row(fine, shift, t)
            for g in range(8):
                for i, v in enumerate(times_row(base, coarse, g)):
                    siv[t * 4 + e, pl.ds(64 * i + 8 * g, 8), :] = v.astype(BF16)

    def prep_filter(ri, m):
        sub = lax.broadcasted_iota(jnp.int32, (8, 128), 0)
        edge = (wr_edge, wi_edge)[ri]
        res = {}
        for i in range(8):
            words = wraw32[ri, m, pl.ds(i, 32, stride=8), :]
            res[2 * i], res[2 * i + 1] = _unpack(words, 0), _unpack(words, 1)
        first = res[0][0:8]
        dst = pl.ds((m % 2) * 16 + ri * 8, 8)
        prev = jnp.zeros((8, 128), F32) if m < 2 else side[1, dst, :]
        put(side.at[1, dst, :], jnp.where(sub == m // 2, jnp.broadcast_to(first[0:1], (8, 128)), prev))
        nyq = jnp.broadcast_to(edge[0:1, pl.ds(m * 128, 128)].astype(F32), (8, 128))
        res[0] = jnp.concatenate([jnp.where(sub == 0, nyq, first), res[0][8:]], axis=0)
        for ct, (ra, rb) in enumerate(PAIRS):
            blk = jnp.concatenate([res[p] for p in _residues(ra) + _residues(rb)], axis=0)
            o = _dot_nt(lhs(small32[16]), blk.astype(BF16))
            for e in range(4):
                put(wf.at[ri, ct, e, m // 2, pl.ds((m % 2) * 32, 32), :], o[e * 32:(e + 1) * 32])

    def prep_wqkv_cross(g, r):
        pos = (_lane(8) >> 2) & 7
        u = [wqkv_raw32[g * NT + (-j) % 8, pl.ds(r * 8, 8), :] for j in range(NT)]
        u[0], u[4] = gate(u[0]), gate(u[4])
        for bit in range(3):
            m = ((pos >> bit) & 1) == 1
            u = [lax.select(m, u[(j - (1 << bit)) % 8], u[j]) for j in range(NT)]
        for j in range(NT):
            if j < 4:
                pin(u[j])
            put(wtmp.at[j, pl.ds(r * 8, 8), :], u[j])

    def prep_wqkv_pair(g, p, part):
        lane = _lane(8)
        ws = {}
        for n in range(2):
            index = (lane & 3) * 32 + (((lane >> 2) + 2 * p + n) & 7) * 4 + (lane >> 5)
            for half in range(2):
                for r in range(part * 2, part * 2 + 2):
                    w = gate(wtmp[2 * p + n, pl.ds(half * 256 + r * 8, 8), :])
                    ws[r, half, n] = jnp.take_along_axis(w, index, axis=1)
        yield from _latency()
        for r in range(part * 2, part * 2 + 2):
            quad = [ws[r, half, n] for half in range(2) for n in range(2)]
            ops = [_strassen_rhs(*[_unpack(w, i) for w in quad]) for i in range(2)]
            for k in range(7):
                word = {1: quad[0], 4: quad[3]}.get(k)
                if word is None:
                    word = pack(ops[0][k], ops[1][k])
                if k in (2, 3):
                    pin(word)
                put(wqkv32.at[g * 4 + p, k, pl.ds(r * 8, 8), :], word)

    def add_prep_wqkv(sched, tick, g, ticks, pair_ticks):
        for r in range(64):
            sched.add(tick + r * ticks / 64, _once(prep_wqkv_cross, g, r))
        tick = int(tick + ticks) + 1
        done = []
        for p, n in enumerate(pair_ticks):
            for i in range(16):
                sched.add(tick + i * n / 16, prep_wqkv_pair(g, p, i))
            tick += n
            done.append(int(tick) + XGAP + 1)
        return done

    def prep_wo(p, part):
        v, pair = divmod(part, 2)
        upper = lax.broadcasted_iota(jnp.int32, (8, 128), 0) >= 4
        ws = [[wo_raw32[2 * p + n, pl.ds(128 * v + 2 * f + pair, 8, stride=16), :] for f in range(8)]
              for n in range(2)]
        for o in range(4):
            quad = [lax.select(upper, w[(2 * v + 1 + j) % 8], w[(2 * v + j) % 8])
                    for j in (o, o + 4) for w in ws]
            quad[0] = gate(quad[0])
            for i in range(2):
                for k, x in enumerate(_strassen_rhs(*[_unpack(w, i) for w in quad])):
                    if k in (2, 3):
                        pin(x)
                    wo[p, k, pl.ds(o * 128 + (2 * pair + i) * 32 + 8 * v, 8), :] = x.astype(BF16)
            if o < 3:
                yield

    def ln_stats(xs):
        lane_mean = _tree(_add, xs) * (1.0 / NT)
        lane_m2 = _tree(_add, [jnp.square(x - lane_mean) for x in xs])
        pin(lane_m2)
        mean = jnp.sum(lane_mean, axis=1, keepdims=True) * (1.0 / 128)
        yield from _latency()
        m2 = lane_m2 + jnp.square(gate(lane_mean) - mean) * float(NT)
        pin(m2)
        var = jnp.sum(m2, axis=1, keepdims=True) * (1.0 / D)
        yield from _latency()
        return mean, lax.rsqrt(gate(jnp.broadcast_to(var, (16, 128))) + EPS)

    def d_fwd_rows(b, lb, from_input=False):
        xs = load_x(b, lb, from_input)

        def emit(r, v):
            if r % 4 == 0 or (r < 4 and not from_input):
                pin(v)
            ubuf[b % RING, r, r16(lb), :] = v.astype(BF16)

        xs[:4] = [gate(x, ILAG if from_input else GLAG) for x in xs[:4]]
        inv = yield from _d_butterfly_fwd(xs, emit, pin, from_input)
        inv = jnp.broadcast_to(inv, (16, 128))
        pin(inv)
        put(uout.at[b % RING, 8, r16(lb), :], inv)

    def d_dots(b, base, per_tick):
        for r in range(8):
            o = _dot(lhs(ubuf32[b % RING, r]), bf(small32[base + r]))
            put(uout.at[b % RING, r], o)
            if r % per_tick == per_tick - 1 and r < 7:
                yield

    def d_dots_wide(b):
        for ct, (ra, rb) in enumerate(PAIRS):
            u = lhs(ubuf32[b % RING, ra], ubuf32[b % RING, rb])
            for i, r in enumerate((ra, rb)):
                o = _dot(u, bf(wide32[2 * ct + i]))
                put(uout.at[b % RING, r], ticking(o) if i else o)
            if ct < 3:
                yield

    def d_fwd_cols(b, ct, is_wide):
        c, t = divmod(b, 8)
        ra, rb = PAIRS[ct]
        lane = _lane(16)
        lo = lane < 64
        z, x0 = [], []
        for lb in range(4):
            a, bb, inv = (uout[b % RING, r, r16(lb), :] for r in (ra, rb, 8))
            inv = gate(inv, ILAG if is_wide else GLAG)
            a, bb = a * inv, bb * inv
            if is_wide:
                if ct == 0:
                    x0.append(pltpu.roll(bb, t, 1) if t else bb)
                    bb = jnp.where(lane == 0, 0.0, bb)
                z.append((a, bb))
                continue
            if ct == 0:
                x0.append(pltpu.roll(a, (t + 64) % 128, 1))
                a = jnp.where(lane == 64, 0.0, a)
            im = lax.select(lo, bb, a)
            z.append((lax.select(lo, a, bb), _swap(im)))
        if not is_wide:
            yield from _latency()
        for e, (re, im) in enumerate(_dft4(z, False)):
            words = pack(re, im)
            if e < 2:
                pin(words)
            put(zin.at[ct, t * 4 + e, r16(c), :], words)
        if is_wide and ct == 0:
            yield from _latency()
        for lb, v in enumerate(x0):
            ls = pl.ds(64 * lb + 16 * c, 16)
            prev = jnp.zeros((16, 128), F32) if t == 0 else side[0, ls, :]
            v = jnp.where(lane == t, v, prev)
            pin(v)
            put(side.at[0, ls, :], v)

    def add_d_fwd(sched, tick, b, gap, per_tick=4, from_input=False):
        for lb in range(4):
            sched.add(tick + lb * gap, d_fwd_rows(b, lb, from_input))
        tick = int(tick + 3 * gap) + XGAP + 1
        sched.add(tick, d_dots_wide(b) if from_input else d_dots(b, 0, per_tick))
        for ct in range(4):
            sched.add(tick + 8 // per_tick + 3 + ct * gap, d_fwd_cols(b, ct, from_input))
        return int(tick + 8 // per_tick + 3 + 3 * gap) + XGAP + 1

    def side_path():
        vt = side[0].T[0:8]
        yield
        zero8 = jnp.zeros((8, 256), F32)
        u = _dot(jnp.concatenate([vt, zero8], axis=0).astype(BF16), f256[...])[0:8]
        twr, twi = tw_ref[0:8, :], tw_ref[8:16, :]
        ur, ui = u[:, 0:256], u[:, 256:512]
        pad = jnp.zeros((112, 256), BF16)
        for _ in range(4):
            yield
        uu = jnp.concatenate([ur * twr - ui * twi, ur * twi + ui * twr], axis=0).astype(BF16)
        xk = _dot(d8_ref[0], jnp.concatenate([uu, pad], axis=0))
        for _ in range(4):
            yield
        wr = jnp.concatenate([side[1, 0:8, :], side[1, 16:24, :]], axis=1)
        wi = jnp.concatenate([side[1, 8:16, :], side[1, 24:32, :]], axis=1)
        xr, xi = xk[0:8], xk[8:16]
        yy = jnp.concatenate([xr * wr - xi * wi, xr * wi + xi * wr], axis=0).astype(BF16)
        p = _dot(d8_ref[1], jnp.concatenate([yy, pad], axis=0))
        for _ in range(4):
            yield
        twr, twi = tw_ref[0:8, :], tw_ref[8:16, :]
        pr, pi = p[0:8], p[8:16]
        g = jnp.concatenate([pr * twr + pi * twi, pi * twr - pr * twi], axis=1)
        g = jnp.concatenate([g, jnp.zeros((8, 512), F32)], axis=0).astype(BF16)
        y0 = _dot_nt(g, f256[...])
        for _ in range(4):
            yield
        put(side.at[2], jnp.concatenate([y0, jnp.zeros((112, 256), F32)], axis=0).T)

    def s_fwd(u, t):
        ct, e = divmod(u, 4)
        o = _dot(lhs(sfw32[t * 4 + e]), bf(zin[ct, t * 4 + e]))
        put(zout.at[ct, t * 4 + e], o if t % 2 else ticking(o))

    def s_filter(u, g):
        ct, e = divmod(u, 4)
        z = [tuple(zout[ct, t * 4 + e, pl.ds(g * 16 + i, 8), :] for i in (0, 8)) for t in range(8)]
        z[0], z[1] = [tuple(gate(v, SGLAG) for v in zz) for zz in z[0:2]]
        xk = _dft8(z, False)
        for k2 in range(8):
            wr = wf[0, ct, e, k2, pl.ds(g * 8, 8), :]
            wi = wf[1, ct, e, k2, pl.ds(g * 8, 8), :]
            re, im = xk[k2]
            xk[k2] = (re * wr - im * wi, re * wi + im * wr)
        for t, (re, im) in enumerate(_dft8(xk, True)):
            words = pack(re, im)
            if t < 4:
                pin(words)
            put(zin.at[ct, t * 4 + e, pl.ds(g * 8, 8), :], words)

    def s_inv(u, t):
        ct, e = divmod(u, 4)
        o = _dot(lhs(siv32[t * 4 + e]), bf(zin[ct, t * 4 + e]))
        put(zout.at[ct, t * 4 + e], o if t % 2 else ticking(o))

    def add_s_stage(sched, early, ready, t1, pause):
        ahead = 4 + S_LAG
        tick = early
        for t in sorted(range(8), key=lambda t: ready[t]):
            for i in range(t, 2 * ahead, 8):
                tick = max(tick + 0.5, ready[t])
                sched.add(tick, _once(s_fwd, i // 8, t))
        t1 = max(t1, int(tick) + 1)
        t2 = pause(t1 + 64 - ahead, t1 + 64)
        sched.add(max(max(ready), t2), side_path())
        for i in range(64):
            if i + ahead < 64:
                sched.add(t1 + i, _once(s_fwd, *divmod(2 * (i + ahead), 8)))
            sched.add(t1 + i, _once(s_filter, *divmod(i, 4)))
            if i + ahead < 64:
                sched.add(t1 + i, _once(s_fwd, *divmod(2 * (i + ahead) + 1, 8)))
        for i in range(69):
            if i >= 5:
                sched.add(t2 + min(i, 66), _once(s_inv, *divmod(2 * (i - 5), 8)))
            if i < 64:
                sched.add(t2 + i, _once(s_filter, i // 4, 4 + i % 4))
            if i >= 5:
                sched.add(t2 + min(i, 66), _once(s_inv, *divmod(2 * (i - 5) + 1, 8)))
        return [t2 + 16 * ct + 22 for ct in range(3)] + [t2 + 67]

    def d_inv_cols(b, ct):
        c, t = divmod(b, 8)
        ra, rb = PAIRS[ct]
        lane = _lane(16)
        lo = lane < 64
        u = [(zout[ct, t * 4 + e, r16(c), :], zout[ct, t * 4 + e, r16(4 + c), :]) for e in range(4)]
        u[0], u[1] = tuple(map(gate, u[0])), tuple(map(gate, u[1]))
        z = _dft4(u, True)
        z = [(re, _swap(im)) for re, im in z]
        if ct == 0:
            y0 = [pltpu.roll(side[2, pl.ds(64 * lb + 16 * c, 16), :], 64 - t, 1) for lb in range(4)]
        yield from _latency()
        for lb, (re, sw) in enumerate(z):
            sw = gate(sw)
            a, bb = lax.select(lo, re, sw), lax.select(lo, sw, re)
            if ct == 0:
                a = jnp.where(lane == 64, y0[lb], a)
            pin(a)
            ubuf[b % RING, ra, r16(lb), :] = a.astype(BF16)
            ubuf[b % RING, rb, r16(lb), :] = bb.astype(BF16)

    def d_inv_rows(b, lb, stats, first):
        u = [uout[b % RING, r, r16(lb), :] for r in range(8)]
        ys = yield from _d_butterfly_inv([gate(v) if r < 4 else v for r, v in enumerate(u)], pin, gate)
        xs = [x + y for x, y in zip(load_x(b, lb, first), ys)]
        for j in range(NT):
            put(xres.at[b, j, r16(lb), :], xs[j])
        stats[b, lb] = yield from ln_stats(xs)
        if b % 2:
            for j in range(4):
                a = [(xres[bb, j + o, r16(lb), :] - stats[bb, lb][0]) * stats[bb, lb][1]
                     for bb in (b - 1, b) for o in (0, 4)]
                a[0], a[3] = gate(a[0]), gate(a[3])
                for k, v in enumerate(_strassen_lhs(*a)):
                    if k in (1, 4):
                        pin(v)
                    abuf[b // 2, k, j, r16(lb), :] = v.astype(BF16)
                if j < 3:
                    yield

    def add_d_inv(sched, tick, b, gap, stats, first, cols=None):
        per_tick = 4
        cols = cols or [tick + ct * gap for ct in range(4)]
        for ct in range(4):
            sched.add(cols[ct], d_inv_cols(b, ct))
        tick = int(cols[3]) + XGAP + 1
        sched.add(tick, d_dots(b, 8, per_tick))
        tick += 8 // per_tick + 3
        for lb in range(4):
            sched.add(tick + lb * gap, d_inv_rows(b, lb, stats, first))
        return int(tick + 3 * gap) + 3 * XGAP + 1 + 4

    def gemm(lhs32, rhs32, jobs, sink):
        for slot, b, n in jobs:
            m = {}
            for k in (3, 1, 0, 6, 5, 4, 2):
                m[k] = ticking(_dot(lhs(*[lhs32[slot, k, j] for j in range(4)]), bf(rhs32[n // 2, k])))
                if k == 1:
                    sink(b + 1, n, m[1] - m[3])
                elif k == 0:
                    c11, c22 = m[3] - m[0], m[1] - m[0]
                elif k == 6:
                    c11 = m[6] - c11
                elif k == 5:
                    c22 = m[5] - c22
                elif k == 4:
                    sink(b, n, c11 - m[4])
                elif k == 2:
                    sink(b, n + 1, m[4] - m[2])
                    sink(b + 1, n + 1, c22 - m[2])
                yield

    def qkv_sink(b, n, o):
        c, t = divmod(b, 8)
        dst = (qbuf, kbuf, vbuf)[n // NT]
        for lb in range(4):
            put(dst.at[n % NT, t, pl.ds(8 + 64 * lb + 16 * c, 16), :], o[lb * 16:(lb + 1) * 16])
        if b == 0 and n >= NT:
            first = jnp.broadcast_to(o[0:1], (8, 128))
            for tt in range(8):
                dst[n % NT, tt, pl.ds(0, 8), :] = first

    def out_rows(r, i, last):
        c, t = divmod(r, 8)
        return (c * 8 + t % 2 * 4 + i, t // 2) if last and c == 0 else (r, i)

    def out_sink(last, r, n, o):
        for i in range(4):
            b, lb = out_rows(r, i, last)
            put(xres.at[b, n, r16(lb), :], xres[b, n, r16(lb), :] + o[i * 16:(i + 1) * 16])

    def attention(b, lb, h):
        c, t = divmod(b, 8)
        log2e = float(np.log2(np.e))
        scale = HEAD_DIM ** -0.5 * log2e
        r0 = 8 + 64 * lb + 16 * c + 8 * h
        src = [((t - 2 * w) % 8, -((t - 2 * w) // 8)) for w in range(WIN)]
        acc = [None] * WIN
        for j in range(NT):
            if j % 2 == 0:
                factor = gate(jnp.full((8, 128), scale, F32), ALAG)
            q = qbuf[j, t, pl.ds(r0, 8), :] * factor
            for w, (ts, sh) in enumerate(src):
                p = q * kbuf[j, ts, pl.ds(r0 - sh, 8), :]
                acc[w] = p if j == 0 else acc[w] + p
            if j % 2 and j < NT - 1:
                pin(*acc[j // 2 % 2::2])
                yield
        part = [(r, pltpu.roll(r, 64, 1)) for r in acc]
        yield from _latency()
        part = [r + rr for r, rr in part]
        part = [(r, pltpu.roll(r, 32, 1)) for r in part]
        yield from _latency()
        logits = [r + rr for r, rr in part]
        if r0 == 8:
            sub = lax.broadcasted_iota(jnp.int32, (8, 128), 0)
            logits = [jnp.where(sub >= sh, r, -1e9 * log2e) if sh else r
                      for r, (_, sh) in zip(logits, src)]
        logits[0] = gate(logits[0], ALAG)
        m = _tree(jnp.maximum, logits)
        ps = [jnp.exp2(r - m) for r in logits]
        total = _tree(_add, ps)
        pin(total)
        inv = pltpu.reciprocal(total, approx=True)
        inv = inv * (2.0 - total * inv)
        for j in range(NT):
            if j % 2 == 0:
                yield
                ps[0], ps[4] = gate(ps[0], ALAG), gate(ps[4], ALAG)
            o = _chain(_add, [ps[w] * vbuf[j, ts, pl.ds(r0 - sh, 8), :]
                              for w, (ts, sh) in enumerate(src)]) * inv
            if j % 2:
                pin(o)
            put(qbuf.at[j, t, pl.ds(r0, 8), :], o)

    def out_operands(r, i, last):
        for j in range(4):
            a = [qbuf[j + o, b % 8, pl.ds(8 + 64 * lb + 16 * (b // 8), 16), :]
                 for b, lb in (out_rows(r, i, last), out_rows(r + 1, i, last)) for o in (0, 4)]
            a[0], a[3] = gate(a[0]), gate(a[3])
            for k, v in enumerate(_strassen_lhs(*a)):
                if k in (1, 4):
                    pin(v)
                obuf[r // 2, k, j, r16(i), :] = v.astype(BF16)
            if j < 3:
                yield

    def store_rows(b, lb, tiles):
        c, t = divmod(b, 8)
        for j in tiles:
            words = pack(xres[b, j, r16(lb), :], xres[b + 1, j, r16(lb), :])
            pin(words)
            io32[j, lb, c, pl.ds(t // 2, 16, stride=4), :] = words

    unit_ticks = NT + 2 * XGAP
    step = 2
    out_ticks = 28

    def add_proj(sched, tick, c, lo, hi):
        jobs = [(b // step, b, n) for b in range(8 * c, 8 * c + 8, step) for n in range(lo, hi, step)]
        sched.add(tick, gemm(abuf32, wqkv32, jobs, qkv_sink))
        return tick + len(jobs) * out_ticks * step // NT

    def add_attention(sched, tick, pace, rows, last):
        units = [(r, i, half, h) for r in rows[::2] for i in range(4) for half in range(2) for h in range(2)]
        for n, (r, i, half, h) in enumerate(units):
            sched.add(tick + n * pace, attention(*out_rows(r + half, i, last), h))
            if half and h:
                sched.add(int(tick + n * pace) + unit_ticks, out_operands(r, i, last))

    def add_out(sched, tick, rows, last):
        jobs = [(r // 2, r, n) for r in rows[::2] for n in range(0, NT, 2)]
        sched.add(tick, gemm(obuf32, wo32, jobs, functools.partial(out_sink, last)))

    def add_tail(sched, tick, rows, last):
        ready = {}
        for i, r in enumerate(rows):
            t0 = tick + (i // 2 + 1) * out_ticks
            fast = i >= len(rows) - (2 if last else 4)
            if not last:
                t0 += 0 if fast else TOFF + i % 2 * out_ticks // 2
                ready[r % 8] = add_d_fwd(sched, t0, r, i % 2 if fast else out_ticks / 8)
            elif r % 2:
                c, p = r // 8, r % 8 // 2
                if fast:
                    for at, tiles in ((t0 - out_ticks // 4 + 3, range(6)), (t0, range(6, NT))):
                        for j in range(4):
                            sched.add(at, _once(store_rows, 2 * j, p, tiles))
                        sched.add(at + 1, _once(start, out_copies(c, p, tiles)))
                    continue
                for j in range(4):
                    sched.add(t0 + 3 * j + 3, _once(store_rows, *((r - 1, j) if c else (2 * j, p)), range(NT)))
                for lb in ([p] if c == 0 else range(4) if p == 3 else []):
                    sched.add(t0 + 16, _once(start, out_copies(c, lb, range(NT))))
        return ready

    q_ticks = 8 * out_ticks // step
    att_ticks = unit_ticks + 1 + 2
    order = [(a + 8) % NB for a in range(NB)]

    def add_attention_block(sched, cols, last):
        stats = {}
        t0 = max([add_d_inv(sched, 0, b, 0, stats, not last, cols) for b in range(step)])
        if not last:
            sched.add(cols[3] - KLEAD, _once(wait, qkv_copies(1) + dmat_cp))
            done = add_prep_wqkv(sched, cols[3] - KLEAD, 1, KPACE, [7] * 4)
            t0 = max(t0, done[0])
            assert all(d <= t0 + p * out_ticks / 4 for p, d in enumerate(done))
            sched.add(t0 + out_ticks, _once(wait, qkv_copies(2)))
            sched.add(t0 + out_ticks, _once(start, qkv_copies(0)))
            done = add_prep_wqkv(sched, t0 + out_ticks, 2, 2 * out_ticks - 4, [out_ticks - 4] * 4)
            assert all(d <= t0 + q_ticks + p * out_ticks for p, d in enumerate(done))
            sched.add(t0 + 2 * q_ticks, _once(wait, qkv_copies(0)))
            sched.add(t0 + 2 * q_ticks, _once(start, wo_copies))
            done = add_prep_wqkv(sched, t0 + 2 * q_ticks, 0, q_ticks - 10, [q_ticks / 4] * 4)
            assert done[-1] <= t0 + 4 * q_ticks
            sched.add(t0 + 8 * q_ticks, _once(wait, wo_copies))
            for i in range(32):
                sched.add(t0 + 8 * q_ticks + i * q_ticks / 16, prep_wo(*divmod(i, 8)))
        tick, kv_start, q_start = t0, {}, {}
        for kind, c in ("k0", "k1", "q1", "k2", "q2", "k3", "q3", "q0"):
            if kind == "k":
                kv_start[int(c)] = tick
                if c == "0" and not last:
                    tick = add_proj(sched, tick, 0, NT, 2 * NT)
                    jobs = [(b // step, b, n) for n in range(2 * NT, 3 * NT, step) for b in range(0, 8, step)]
                    sched.add(tick, gemm(abuf32, wqkv32, jobs, qkv_sink))
                    tick += q_ticks
                    continue
                tick = add_proj(sched, tick, int(c), NT, 3 * NT)
            else:
                q_start[int(c)] = tick
                tick = add_proj(sched, tick, int(c), 0, NT)
        pace = 2 * out_ticks / step
        for b in range(step, NB):
            due = kv_start[b // 8] + (b % 8 // step) * (2 if last or b >= 8 else 1) * out_ticks
            gap = min(1 + (b - step) * 0.5, DGAP1 if last else DGAP0)
            pace = DPACE1 if last else DPACE0
            at = (b - step) * pace
            at = t0 + at + max(0, at - 4 * q_ticks - out_ticks) * DSLOW
            if not last and b < 8:
                at, gap = max(cols[3], t0 + (b // step - 1) * out_ticks - (step - b % step) * 8), 1
            end = add_d_inv(sched, at, b, gap, stats, not last)
            assert end <= due, (b, end, due)
        begin = [q_start[c] + out_ticks + 3 for c in (1, 2, 3)] + [tick + (ATT1 if last else ATT0)]
        begin.append(tick + (NB // step - 1) * out_ticks - att_ticks)
        for i, c in enumerate((1, 2, 3, 0)):
            pace = (begin[i + 1] - begin[i]) / 64
            assert begin[i] >= max(kv_start[c], kv_start[(c - 1) % 4]) + 2 * q_ticks
            for p in range(4):
                assert begin[i] + 16 * p * pace >= q_start[c] + (4 if last and c == 0 else p + 1) * out_ticks
                assert begin[i] + (16 * p + 15) * pace + att_ticks <= tick + (4 * i + p) * out_ticks + 1e-6
            add_attention(sched, begin[i], pace, range(8 * c, 8 * c + 8), last)
        add_out(sched, tick, order, last)
        return tick + (NB // step) * out_ticks, add_tail(sched, tick, order, last)

    def add_input(sched):
        ready = {}
        after = (x_copies(2), x_copies(3) + perm_cp + w_copies(0) + w_copies(1),
                 w_copies(2) + w_copies(3), w_copies(4))
        for c in range(NC):
            sched.add(c * 32, _once(wait, x_copies(c)))
            sched.add(c * 32, _once(start, after[c]))
            for t in range(8):
                ready[t] = add_d_fwd(sched, c * 32 + t * 4, c * 8 + t, 1, 2, True)
        return 128 + 9, ready

    def add_filter_prep(sched, upper, begin, end):
        after = (w_copies(5) + w_copies(6), w_copies(7) + f256_cp + dmat_cp, [], qkv_copies(2))
        for i in range(16):
            g, at = 4 * upper + i // 4, begin + i * (end - begin) / 16
            if i % 8 == 0:
                sched.add(at, _once(wait, w_copies(g) + w_copies(g + 1) + {0: perm_cp, 6: f256_cp}.get(g, [])))
                sched.add(at, _once(start, after[g // 2]))
            sched.add(at, _once(prep_filter, *w_tiles(g)[i % 4]))
        return end + 2

    def add_first_s_stage(sched):
        tick, ready = add_input(sched)
        sched.add(tick + WK0, _once(start, qkv_copies(1)))
        return add_s_stage(sched, tick, ready, add_filter_prep(sched, 0, F0, tick),
                           lambda begin, end: add_filter_prep(sched, 1, begin, end + FG))

    sched = _Schedule()

    start(x_copies(0))
    for ref in (abuf32, obuf32, ubuf32, wo32, sfw32, siv32, wide32):
        put(ref.at[(0,) * (len(ref.shape) - 2) + (pl.ds(0, 8),)], jnp.zeros((8, 128), U32))
    make_wide()
    start(x_copies(1))
    for t in range(8):
        make_s_fwd(t)
    for e in range(4):
        make_s_inv(e)
    cols = add_first_s_stage(sched)
    tick, ready = add_attention_block(sched, cols, False)
    cols = add_s_stage(sched, tick, ready, tick, lambda begin, end: end)
    add_attention_block(sched, cols, True)
    sched.run()
    for c in range(NC):
        for lb in range(4):
            wait(out_copies(c, lb, range(NT)))


@jax.jit
def pallas_interleave_layers__spectral_gfnet__sliding_local_dilated__prompt_kernel(
    A_x: jax.Array,
    A_w_r: jax.Array,
    A_w_i: jax.Array,
    B_x: jax.Array,
    B_wqkv: jax.Array,
    B_wo: jax.Array,
):
    del B_x
    assert A_x.shape == (1, S, D) and A_w_r.shape == (S, D // 2 + 1)
    cst = _constants()
    x = A_x.astype(BF16).reshape(4, NC, 128, D)
    wr, wi = A_w_r.astype(BF16).T, A_w_i.astype(BF16).T
    hbm = pl.BlockSpec(memory_space=pl.ANY)
    edge = pl.BlockSpec((16, S), lambda i: (D // 32, 0))
    vm = pltpu.VMEM
    out = pl.pallas_call(
        _kernel,
        grid=(1,),
        in_specs=[hbm, hbm, hbm, edge, edge, hbm, hbm, hbm, hbm,
                  pl.BlockSpec((24, 256), lambda i: (0, 0)),
                  pl.BlockSpec((2, 16, 128), lambda i: (0, 0, 0))],
        out_specs=hbm,
        out_shape=jax.ShapeDtypeStruct((4, NC, 128, D), BF16),
        scratch_shapes=[
            vm((NT, 4, NC, 128, 128), BF16),
            vm((17, 128, 128), BF16),
            vm((32, 128, 128), BF16),
            vm((32, 128, 128), BF16),
            vm((256, 512), BF16),
            vm((2, 16, 512, 128), BF16),
            vm((2, 4, 4, 8, 64, 128), F32),
            vm((3 * NT, D, 128), BF16),
            vm((NT, D // 2, 128), U32),
            vm((12, 7, 512, 128), BF16),
            vm((NT, D, 128), BF16),
            vm((4, 7, 512, 128), BF16),
            vm((NB, NT, 64, 128), F32),
            vm((4, 32, 64, 128), U32),
            vm((4, 32, 128, 128), F32),
            vm((RING, 8, 64, 128), BF16),
            vm((RING, 9, 64, 128), F32),
            vm((NB // 2, 7, 4, 64, 128), BF16),
            vm((NB // 2, 7, 4, 64, 128), BF16),
            vm((NT, 8, 264, 128), F32),
            vm((NT, 8, 264, 128), F32),
            vm((NT, 8, 264, 128), F32),
            vm((3, 256, 128), F32),
            vm((8, 256, 128), BF16),
            pltpu.SemaphoreType.DMA((NC,)),
            pltpu.SemaphoreType.DMA((3,)),
            pltpu.SemaphoreType.DMA((8,)),
            pltpu.SemaphoreType.DMA((3,)),
            pltpu.SemaphoreType.DMA(()),
            pltpu.SemaphoreType.DMA(()),
        ],
        compiler_params=pltpu.CompilerParams(
            dimension_semantics=("arbitrary",), vmem_limit_bytes=120 * 2**20),
    )(x, wr, wi, wr, wi, B_wqkv.astype(BF16), B_wo.astype(BF16),
      cst["small"], cst["f256"], cst["tw"], cst["d8"])
    return out.reshape(1, S, D)
```

```python
import functools

import jax
import jax.numpy as jnp
import numpy as np
from jax import lax
from jax.experimental import pallas as pl
from jax.experimental.pallas import tpu as pltpu

S, D = 2048, 1024
NT = D // 128
NC = 4
WIN = 8
HEAD_DIM = 32
EPS = 1e-5
F32, BF16, U32 = jnp.float32, jnp.bfloat16, jnp.uint32
PAIRS = ((0, 4), (1, 7), (2, 6), (3, 5))
RSQ2 = float(np.sqrt(0.5))
NB = S // 64

RING = 8
XGAP = 3
GLAG = 4
ALAG = 4
SGLAG = 3
S_LAG = 2
F0 = 120
KLEAD = 46
KPACE = 40
DGAP0 = 4.75
DGAP1 = 4.2
DPACE0 = 20
DPACE1 = 15.5
DSLOW = 0.6
SYNC = 3
ILAG = 3
FG = 10
TOFF = 4
WK0 = 24
ATT0 = 15
ATT1 = 95


def _residues(r):
    return (0, 8) if r == 0 else (r, 16 - r)


def _d_matrices():
    n = np.arange(64)[:, None]
    a = np.arange(32)
    fwd = np.zeros((8, 128, 128))
    inv = np.zeros((8, 128, 128))
    for r in range(8):
        kd = np.concatenate([16 * a + p for p in _residues(r)])
        weight = np.full(64, 2.0)
        if r == 0:
            kd[0], weight[0] = D // 2, 1.0
            ph = np.exp(-2j * np.pi * n * kd[None, :] / D)
            sgn = np.where(kd % 16 == 0, 1.0, -1.0)[None, :]
            m = np.concatenate([ph, ph * sgn], axis=0)
            re, im = m.real.copy(), m.imag.copy()
            ire, iim = re.copy(), im.copy()
            im[:, 0] = 1.0
            iim[:, 0] = 1.0
        else:
            p = 12 if r == 4 else r
            ph = np.exp(-2j * np.pi * n * kd[None, :] / D)
            si = np.where(kd % 16 == p, 1.0, -1.0)[None, :]
            m = np.concatenate([ph, 1j * si * ph], axis=0)
            re, im = m.real, m.imag
            ire, iim = re, im
        swapped = r in (4, 7, 6, 5)
        cols = [im, re] if swapped else [re, im]
        icols = [iim * weight, ire * weight] if swapped else [ire * weight, iim * weight]
        fwd[r] = np.concatenate(cols, axis=1)
        inv[r] = np.concatenate(icols, axis=1).T / D
    return fwd, inv


def _side_matrices():
    l = np.arange(256)
    f = np.exp(-2j * np.pi * ((l[:, None] * l[None, :]) % 256) / 256)
    f256 = np.concatenate([f.real, f.imag], axis=1)
    t = np.arange(8)
    tw = np.exp(-2j * np.pi * t[:, None] * l[None, :] / S)
    tw = np.concatenate([tw.real, tw.imag, np.zeros((8, 256))], axis=0)
    g = np.exp(-2j * np.pi * t[:, None] * t[None, :] / 8)
    d8 = np.zeros((2, 16, 128))
    d8[0, :, :16] = np.block([[g.real, -g.imag], [g.imag, g.real]])
    d8[1, :, :16] = d8[0, :, :16].T / S
    return f256, tw, d8


def _filter_rows():
    p = np.zeros((1, 128, 128))
    for k in range(32):
        for e in range(4):
            p[0, e * 32 + k, 4 * k + e] = 1.0
    return p


@functools.lru_cache(maxsize=None)
def _constants():
    dfw, div = _d_matrices()
    f256, tw, d8 = _side_matrices()
    small = np.concatenate([dfw, div, _filter_rows()], axis=0)
    b = lambda x: np.asarray(x, np.float32).astype(BF16)
    return dict(small=b(small), f256=b(f256),
                tw=np.asarray(tw, np.float32), d8=b(d8))


def _dot(a, b):
    return jnp.dot(a, b, preferred_element_type=F32)


def _dot_nt(a, b):
    return lax.dot_general(a, b, (((1,), (1,)), ((), ())), preferred_element_type=F32)


def _tree(op, xs):
    xs = list(xs)
    while len(xs) > 1:
        xs = [op(xs[i], xs[i + 1]) if i + 1 < len(xs) else xs[i] for i in range(0, len(xs), 2)]
    return xs[0]


def _chain(op, xs):
    return functools.reduce(op, xs)


def _lane(rows):
    return lax.broadcasted_iota(jnp.int32, (rows, 128), 1)


def _swap(x):
    return pltpu.roll(x, 64, 1)


def _unpack(w, i):
    return pltpu.unpack_elementwise(w, index=i, packed_dtype=BF16, unpacked_dtype=F32)


def _latency():
    for _ in range(XGAP):
        yield


def _add(a, b):
    return a + b


def _row_mean(xs):
    return jnp.sum(_tree(_add, xs), axis=1, keepdims=True) * (1.0 / D)


def _twiddle16(r, x, y):
    lo = _lane(x.shape[0]) < 64
    wr, wi = float(np.cos(np.pi * r / 8)), float(-np.sin(np.pi * r / 8))
    cross = jnp.where(lo, 0.0, wr)
    return x * jnp.where(lo, 1.0, wi) + y * cross, y * jnp.where(lo, 1.0, -wi) + x * cross


def _d_butterfly_fwd(a, emit, pin, wide):
    s = [a[j] + a[j + 4] for j in range(4)]
    e, o = s[0] + s[2], s[1] + s[3]
    total, t4 = e + o, e - o
    emit(4, t4)
    d0, nd2 = a[0] - a[4], a[6] - a[2]
    d1, d3 = a[1] - a[5], a[3] - a[7]
    p, q = (d1 - d3) * RSQ2, (d1 + d3) * -RSQ2
    ts = {1: (d0 + p, q + nd2), 2: (s[0] - s[2], s[3] - s[1]), 3: (d0 - p, q - nd2)}
    mean8 = jnp.sum(total, axis=1, keepdims=True) * (1.0 / 128)
    if wide:
        for r, (tr, ti) in ts.items():
            emit(r, tr)
            emit(8 - r, ti)
    else:
        ab = {r: _twiddle16(r, *t) for r, t in ts.items()}
        ab = {r: (a, _swap(b)) for r, (a, b) in ab.items()}
    dev = _tree(_add, [v * v for t in ts.values() for v in t]) * 2.0 + t4 * t4
    pin(dev)
    yield from _latency()
    t0 = total - mean8
    emit(0, t0)
    var = jnp.sum(dev + t0 * t0, axis=1, keepdims=True) * (1.0 / (NT * D))
    if not wide:
        for r, (x, y) in ab.items():
            emit(r, x + y)
            emit(8 - r, x - y)
    yield from _latency()
    return lax.rsqrt(var + EPS)


def _d_butterfly_inv(u, pin, gate):
    ab = {r: (u[r] + u[8 - r], _swap(u[r] - u[8 - r])) for r in (1, 2, 3)}
    e, o = u[0] + u[4], u[0] - u[4]
    yield from _latency()
    ts = {r: _twiddle16(r, x, gate(y)) for r, (x, y) in ab.items()}
    pin(*[t[0] for t in ts.values()])
    yield
    s = [e + ts[2][0], o - ts[2][1], e - ts[2][0], o + ts[2][1]]
    p = (ts[1][0] - ts[3][0]) * RSQ2
    q = (ts[1][1] + ts[3][1]) * RSQ2
    d0, d1, d2, nd3 = ts[1][0] + ts[3][0], p - q, ts[3][1] - ts[1][1], p + q
    return [s[0] + d0, s[1] + d1, s[2] + d2, s[3] - nd3,
            s[0] - d0, s[1] - d1, s[2] - d2, s[3] + nd3]


def _strassen_lhs(a11, a12, a21, a22):
    return [a11 + a22, a21 + a22, a11, a22, a11 + a12, a21 - a11, a12 - a22]


def _strassen_rhs(b11, b12, b21, b22):
    return [b11 + b22, b11, b22 - b12, b11 - b21, b22, b11 + b12, b21 + b22]


def _cadd(a, b):
    return a[0] + b[0], a[1] + b[1]


def _csub(a, b):
    return a[0] - b[0], a[1] - b[1]


def _dft4(z, inverse):
    a, b = _cadd(z[0], z[2]), _csub(z[0], z[2])
    c, d = _cadd(z[1], z[3]), _csub(z[1], z[3])
    minus = (b[0] + d[1], b[1] - d[0])
    plus = (b[0] - d[1], b[1] + d[0])
    return [_cadd(a, c), plus if inverse else minus, _csub(a, c), minus if inverse else plus]


def _dft8(z, inverse):
    ev = _dft4(z[0::2], inverse)
    od = _dft4(z[1::2], inverse)
    out = [None] * 8
    out[0], out[4] = _cadd(ev[0], od[0]), _csub(ev[0], od[0])
    (er, ei), (x, y) = ev[2], od[2]
    minus, plus = (er + y, ei - x), (er - y, ei + x)
    out[2], out[6] = (plus, minus) if inverse else (minus, plus)
    for k in (1, 3):
        (er, ei), (x, y) = ev[k], od[k]
        sm, df = (x + y) * RSQ2, (x - y) * RSQ2
        if not inverse:
            if k == 1:
                out[1], out[5] = (er + sm, ei - df), (er - sm, ei + df)
            else:
                out[3], out[7] = (er - df, ei - sm), (er + df, ei + sm)
        else:
            if k == 1:
                out[1], out[5] = (er + df, ei + sm), (er - df, ei - sm)
            else:
                out[3], out[7] = (er - sm, ei + df), (er + sm, ei - df)
    return out


class _Schedule:
    def __init__(self):
        self.pending = []

    def add(self, tick, gen):
        self.pending.append((int(tick), len(self.pending), gen))

    def run(self):
        pending = sorted(self.pending, key=lambda p: p[:2])
        active, tick, i = [], 0, 0
        while active or i < len(pending):
            while i < len(pending) and pending[i][0] <= tick:
                active.append(pending[i][2])
                i += 1
            for g in list(active):
                if next(g, 0) == 0:
                    active.remove(g)
            tick += 1
        self.pending = []


def _once(fn, *args):
    fn(*args)
    return
    yield


def _kernel(x_hbm, wr_hbm, wi_hbm, wqkv_hbm, wo_hbm, small_hbm, f256_hbm, tw_hbm, d8_hbm,
            out_hbm,
            io, small, sfw, siv, f256, wraw, wf, wqkv_raw, wtmp, wqkv, wo_raw, wo,
            xres, zin, zout, ubuf, uout, abuf, obuf, qbuf, kbuf, vbuf, side,
            wide, tw_ref, d8_ref, wr_edge, wi_edge, sem_x, sem_c, sem_w, sem_qkv, sem_wo, sem_out):

    def x_copies(c):
        return [pltpu.make_async_copy(x_hbm.at[:, c, :, pl.ds(j * 128, 128)], io.at[j, :, c],
                                      sem_x.at[c]) for j in range(NT)]

    def out_copies(c, lb, tiles):
        return [pltpu.make_async_copy(io.at[j, lb, c], out_hbm.at[lb, c, :, pl.ds(j * 128, 128)],
                                      sem_out) for j in tiles]

    perm_cp, dmat_cp, f256_cp = ([pltpu.make_async_copy(s, d, sem_c.at[i])] for i, (s, d) in enumerate((
        (small_hbm.at[pl.ds(16, 1)], small.at[pl.ds(16, 1)]),
        (small_hbm.at[pl.ds(0, 16)], small.at[pl.ds(0, 16)]), (f256_hbm, f256))))

    tiny_cp = [pltpu.make_async_copy(s, d, sem_c.at[3]) for s, d in (
        (tw_hbm, tw_ref), (d8_hbm, d8_ref),
        (wr_hbm.at[pl.ds(D // 2, 1)], wr_edge), (wi_hbm.at[pl.ds(D // 2, 1)], wi_edge))]

    def w_tiles(g):
        return [(g // 2 % 2, 8 * (g % 2) + 2 * i + g // 4) for i in range(4)]

    def w_copies(g):
        return [pltpu.make_async_copy((wr_hbm, wi_hbm)[ri].at[pl.ds(0, 512), pl.ds(m * 128, 128)],
                                      wraw.at[ri, m], sem_w.at[g]) for ri, m in w_tiles(g)]

    def qkv_copies(g):
        return [pltpu.make_async_copy(wqkv_hbm.at[:, pl.ds(g * D + j * 128, 128)],
                                      wqkv_raw.at[g * NT + j], sem_qkv.at[g]) for j in range(NT)]

    wo_copies = [pltpu.make_async_copy(wo_hbm.at[:, pl.ds(j * 128, 128)], wo_raw.at[j], sem_wo)
                 for j in range(NT)]

    def start(cs):
        for cp in cs:
            cp.start()

    def wait(cs):
        for cp in cs:
            cp.wait()

    io32, wraw32, wo_raw32 = io.bitcast(U32), wraw.bitcast(U32), wo_raw.bitcast(U32)
    small32, sfw32, siv32, wide32 = (r.bitcast(U32) for r in (small, sfw, siv, wide))
    wqkv_raw32, wqkv32, wo32 = (r.bitcast(U32) for r in (wqkv_raw, wqkv, wo))
    ubuf32, abuf32, obuf32 = ubuf.bitcast(U32), abuf.bitcast(U32), obuf.bitcast(U32)

    never = {}
    token = {}

    def pin(*values):
        for v in values:
            key = v.shape[0], v.dtype == F32
            token[key] = (lax.max if key[1] else lax.bitwise_xor)(token[key], v) if key in token else v

    clock = []

    def gate(v, lag=GLAG):
        if len(clock) < lag:
            return v
        old = clock[-lag] if v.dtype == F32 else pltpu.bitcast(clock[-lag], v.dtype)
        if v.shape[0] == 8:
            return lax.select(never[1], old, v)
        return lax.concatenate([lax.select(never[1], old, v[0:8]), v[8:]], 0)

    def ticking(o):
        clock.append(o[0:8])
        del clock[:-16]
        return o

    def lhs(*tiles):
        if not token and len(tiles) == 4 and len(clock) >= SYNC:
            pin(clock[-SYNC])
        words = lax.concatenate(tiles, 1) if len(tiles) > 1 else tiles[0]
        if token:
            parts = [pltpu.bitcast(v, U32) if is_float else v for (_, is_float), v in token.items()]
            token.clear()
            w = _chain(lax.bitwise_xor, [v[i:i + 8] if v.shape[0] > 8 else v
                                         for v in parts for i in range(0, v.shape[0], 8)])
            w = lax.concatenate([w] * len(tiles), 1) if len(tiles) > 1 else w
            words = lax.concatenate([lax.select(never[len(tiles)], w, words[0:8]), words[8:]], 0)
        return pltpu.bitcast(words, BF16)

    def bf(words):
        return pltpu.bitcast(words, BF16)

    def pack(a, b):
        return pltpu.bitcast(pltpu.pack_elementwise([a, b], packed_dtype=BF16), U32)

    def r16(i):
        return pl.ds(i * 16, 16)

    always = {}

    def put(ref, v):
        if v.shape not in always:
            always[v.shape] = jnp.ones(v.shape, jnp.bool_)
        pltpu.store(ref, v, mask=always[v.shape])

    def load_x(b, lb, from_input):
        if from_input:
            c, t = divmod(b, 8)
            return [_unpack(io32[j, lb, c, pl.ds(t // 2, 16, stride=4), :], t % 2) for j in range(NT)]
        return [xres[b, j, r16(lb), :] for j in range(NT)]

    def unit(p):
        angle = (((p + S // 2) & (S - 1)) - S // 2).astype(F32) * (2 * np.pi / S)
        return jnp.cos(angle), jnp.sin(angle)

    def times_row(a, b, i):
        br, bi = (jnp.broadcast_to(v[i:i + 1], (8, 128)) for v in b)
        return a[0] * br - a[1] * bi, a[0] * bi + a[1] * br

    def make_wide():
        row, lane = lax.broadcasted_iota(jnp.int32, (8, 128), 0), _lane(8)
        for ct, (ra, rb) in enumerate(PAIRS):
            res = _residues(ra) + _residues(rb)
            kd = (lane & 31) * 16 + _chain(
                _add, [jnp.where(lane >> 5 == g, p, 0) for g, p in enumerate(res)])
            if ct == 0:
                kd = jnp.where(lane == 0, D // 2, kd)
            fine, coarse = unit(-2 * row * kd), [unit(-16 * (row + 8 * h) * kd) for h in range(2)]
            for a in range(16):
                re, im = times_row(fine, coarse[a // 8], a % 8)
                if ct == 0:
                    even = kd & 7 == 0
                    top = jnp.where(even, re, 0.0), jnp.where(lane == 0, 1.0, jnp.where(even, im, 0.0))
                    bottom = jnp.where(even, 0.0, re), jnp.where(even, 0.0, im)
                else:
                    sign = jnp.where(kd & 7 == ra, 1.0, -1.0)
                    top, bottom = (re, im), (-sign * im, sign * re)
                for i in range(2):
                    wide[2 * ct + i, pl.ds(8 * a, 8), :] = top[i].astype(BF16)
                    wide[2 * ct + i, pl.ds(128 + 8 * a, 8), :] = bottom[i].astype(BF16)

    def make_s_fwd(t):
        row, lane = lax.broadcasted_iota(jnp.int32, (8, 128), 0), _lane(8)
        pos = 8 * (lane >> 1) + t
        fine = unit((lane & 1) * (S // 4) - 4 * row * pos)
        shift, coarse = unit(-row * pos), unit(-32 * row * pos)
        for e in range(4):
            base = times_row(fine, shift, e)
            for g in range(8):
                for i, v in enumerate(times_row(base, coarse, g)):
                    sfw[t * 4 + e, pl.ds(16 * g + 8 * i, 8), :] = v.astype(BF16)

    def make_s_inv(e):
        row, lane = lax.broadcasted_iota(jnp.int32, (8, 128), 0), _lane(8)
        freq = 4 * (lane >> 1) + e
        fine = [v * (1.0 / S) for v in unit((lane & 1) * (S // 4) + 8 * row * freq)]
        shift, coarse = unit(row * freq), unit(64 * row * freq)
        for t in range(8):
            base = times_row(fine, shift, t)
            for g in range(8):
                for i, v in enumerate(times_row(base, coarse, g)):
                    siv[t * 4 + e, pl.ds(64 * i + 8 * g, 8), :] = v.astype(BF16)

    def prep_filter(ri, m):
        sub = lax.broadcasted_iota(jnp.int32, (8, 128), 0)
        edge = (wr_edge, wi_edge)[ri]
        res = {}
        for i in range(8):
            words = wraw32[ri, m, pl.ds(i, 32, stride=8), :]
            res[2 * i], res[2 * i + 1] = _unpack(words, 0), _unpack(words, 1)
        first = res[0][0:8]
        dst = pl.ds((m % 2) * 16 + ri * 8, 8)
        prev = jnp.zeros((8, 128), F32) if m < 2 else side[1, dst, :]
        put(side.at[1, dst, :], jnp.where(sub == m // 2, jnp.broadcast_to(first[0:1], (8, 128)), prev))
        nyq = jnp.broadcast_to(edge[0:1, pl.ds(m * 128, 128)].astype(F32), (8, 128))
        res[0] = jnp.concatenate([jnp.where(sub == 0, nyq, first), res[0][8:]], axis=0)
        for ct, (ra, rb) in enumerate(PAIRS):
            blk = jnp.concatenate([res[p] for p in _residues(ra) + _residues(rb)], axis=0)
            o = _dot_nt(lhs(small32[16]), blk.astype(BF16))
            for e in range(4):
                put(wf.at[ri, ct, e, m // 2, pl.ds((m % 2) * 32, 32), :], o[e * 32:(e + 1) * 32])

    def prep_wqkv_cross(g, r):
        pos = (_lane(8) >> 2) & 7
        u = [wqkv_raw32[g * NT + (-j) % 8, pl.ds(r * 8, 8), :] for j in range(NT)]
        u[0], u[4] = gate(u[0]), gate(u[4])
        for bit in range(3):
            m = ((pos >> bit) & 1) == 1
            u = [lax.select(m, u[(j - (1 << bit)) % 8], u[j]) for j in range(NT)]
        for j in range(NT):
            if j < 4:
                pin(u[j])
            put(wtmp.at[j, pl.ds(r * 8, 8), :], u[j])

    def prep_wqkv_pair(g, p, part):
        lane = _lane(8)
        ws = {}
        for n in range(2):
            index = (lane & 3) * 32 + (((lane >> 2) + 2 * p + n) & 7) * 4 + (lane >> 5)
            for half in range(2):
                for r in range(part * 2, part * 2 + 2):
                    w = gate(wtmp[2 * p + n, pl.ds(half * 256 + r * 8, 8), :])
                    ws[r, half, n] = jnp.take_along_axis(w, index, axis=1)
        yield from _latency()
        for r in range(part * 2, part * 2 + 2):
            quad = [ws[r, half, n] for half in range(2) for n in range(2)]
            ops = [_strassen_rhs(*[_unpack(w, i) for w in quad]) for i in range(2)]
            for k in range(7):
                word = {1: quad[0], 4: quad[3]}.get(k)
                if word is None:
                    word = pack(ops[0][k], ops[1][k])
                if k in (2, 3):
                    pin(word)
                put(wqkv32.at[g * 4 + p, k, pl.ds(r * 8, 8), :], word)

    def add_prep_wqkv(sched, tick, g, ticks, pair_ticks):
        for r in range(64):
            sched.add(tick + r * ticks / 64, _once(prep_wqkv_cross, g, r))
        tick = int(tick + ticks) + 1
        done = []
        for p, n in enumerate(pair_ticks):
            for i in range(16):
                sched.add(tick + i * n / 16, prep_wqkv_pair(g, p, i))
            tick += n
            done.append(int(tick) + XGAP + 1)
        return done

    def prep_wo(p, part):
        v, pair = divmod(part, 2)
        upper = lax.broadcasted_iota(jnp.int32, (8, 128), 0) >= 4
        ws = [[wo_raw32[2 * p + n, pl.ds(128 * v + 2 * f + pair, 8, stride=16), :] for f in range(8)]
              for n in range(2)]
        for o in range(4):
            quad = [lax.select(upper, w[(2 * v + 1 + j) % 8], w[(2 * v + j) % 8])
                    for j in (o, o + 4) for w in ws]
            quad[0] = gate(quad[0])
            for i in range(2):
                for k, x in enumerate(_strassen_rhs(*[_unpack(w, i) for w in quad])):
                    if k in (2, 3):
                        pin(x)
                    wo[p, k, pl.ds(o * 128 + (2 * pair + i) * 32 + 8 * v, 8), :] = x.astype(BF16)
            if o < 3:
                yield

    def ln_stats(xs):
        lane_mean = _tree(_add, xs) * (1.0 / NT)
        lane_m2 = _tree(_add, [jnp.square(x - lane_mean) for x in xs])
        pin(lane_m2)
        mean = jnp.sum(lane_mean, axis=1, keepdims=True) * (1.0 / 128)
        yield from _latency()
        m2 = lane_m2 + jnp.square(gate(lane_mean) - mean) * float(NT)
        pin(m2)
        var = jnp.sum(m2, axis=1, keepdims=True) * (1.0 / D)
        yield from _latency()
        return mean, lax.rsqrt(gate(jnp.broadcast_to(var, (16, 128))) + EPS)

    def d_fwd_rows(b, lb, from_input=False):
        xs = load_x(b, lb, from_input)

        def emit(r, v):
            if r % 4 == 0 or (r < 4 and not from_input):
                pin(v)
            ubuf[b % RING, r, r16(lb), :] = v.astype(BF16)

        xs[:4] = [gate(x, ILAG if from_input else GLAG) for x in xs[:4]]
        inv = yield from _d_butterfly_fwd(xs, emit, pin, from_input)
        inv = jnp.broadcast_to(inv, (16, 128))
        pin(inv)
        put(uout.at[b % RING, 8, r16(lb), :], inv)

    def d_dots(b, base, per_tick):
        for r in range(8):
            o = _dot(lhs(ubuf32[b % RING, r]), bf(small32[base + r]))
            put(uout.at[b % RING, r], o)
            if r % per_tick == per_tick - 1 and r < 7:
                yield

    def d_dots_wide(b):
        for ct, (ra, rb) in enumerate(PAIRS):
            u = lhs(ubuf32[b % RING, ra], ubuf32[b % RING, rb])
            for i, r in enumerate((ra, rb)):
                o = _dot(u, bf(wide32[2 * ct + i]))
                put(uout.at[b % RING, r], ticking(o) if i else o)
            if ct < 3:
                yield

    def d_fwd_cols(b, ct, is_wide):
        c, t = divmod(b, 8)
        ra, rb = PAIRS[ct]
        lane = _lane(16)
        lo = lane < 64
        z, x0 = [], []
        for lb in range(4):
            a, bb, inv = (uout[b % RING, r, r16(lb), :] for r in (ra, rb, 8))
            inv = gate(inv, ILAG if is_wide else GLAG)
            a, bb = a * inv, bb * inv
            if is_wide:
                if ct == 0:
                    x0.append(pltpu.roll(bb, t, 1) if t else bb)
                    bb = jnp.where(lane == 0, 0.0, bb)
                z.append((a, bb))
                continue
            if ct == 0:
                x0.append(pltpu.roll(a, (t + 64) % 128, 1))
                a = jnp.where(lane == 64, 0.0, a)
            im = lax.select(lo, bb, a)
            z.append((lax.select(lo, a, bb), _swap(im)))
        if not is_wide:
            yield from _latency()
        for e, (re, im) in enumerate(_dft4(z, False)):
            words = pack(re, im)
            if e < 2:
                pin(words)
            put(zin.at[ct, t * 4 + e, r16(c), :], words)
        if is_wide and ct == 0:
            yield from _latency()
        for lb, v in enumerate(x0):
            ls = pl.ds(64 * lb + 16 * c, 16)
            prev = jnp.zeros((16, 128), F32) if t == 0 else side[0, ls, :]
            v = jnp.where(lane == t, v, prev)
            pin(v)
            put(side.at[0, ls, :], v)

    def add_d_fwd(sched, tick, b, gap, per_tick=4, from_input=False):
        for lb in range(4):
            sched.add(tick + lb * gap, d_fwd_rows(b, lb, from_input))
        tick = int(tick + 3 * gap) + XGAP + 1
        sched.add(tick, d_dots_wide(b) if from_input else d_dots(b, 0, per_tick))
        for ct in range(4):
            sched.add(tick + 8 // per_tick + 3 + ct * gap, d_fwd_cols(b, ct, from_input))
        return int(tick + 8 // per_tick + 3 + 3 * gap) + XGAP + 1

    def side_path():
        vt = side[0].T[0:8]
        yield
        zero8 = jnp.zeros((8, 256), F32)
        u = _dot(jnp.concatenate([vt, zero8], axis=0).astype(BF16), f256[...])[0:8]
        twr, twi = tw_ref[0:8, :], tw_ref[8:16, :]
        ur, ui = u[:, 0:256], u[:, 256:512]
        pad = jnp.zeros((112, 256), BF16)
        for _ in range(4):
            yield
        uu = jnp.concatenate([ur * twr - ui * twi, ur * twi + ui * twr], axis=0).astype(BF16)
        xk = _dot(d8_ref[0], jnp.concatenate([uu, pad], axis=0))
        for _ in range(4):
            yield
        wr = jnp.concatenate([side[1, 0:8, :], side[1, 16:24, :]], axis=1)
        wi = jnp.concatenate([side[1, 8:16, :], side[1, 24:32, :]], axis=1)
        xr, xi = xk[0:8], xk[8:16]
        yy = jnp.concatenate([xr * wr - xi * wi, xr * wi + xi * wr], axis=0).astype(BF16)
        p = _dot(d8_ref[1], jnp.concatenate([yy, pad], axis=0))
        for _ in range(4):
            yield
        twr, twi = tw_ref[0:8, :], tw_ref[8:16, :]
        pr, pi = p[0:8], p[8:16]
        g = jnp.concatenate([pr * twr + pi * twi, pi * twr - pr * twi], axis=1)
        g = jnp.concatenate([g, jnp.zeros((8, 512), F32)], axis=0).astype(BF16)
        y0 = _dot_nt(g, f256[...])
        for _ in range(4):
            yield
        put(side.at[2], jnp.concatenate([y0, jnp.zeros((112, 256), F32)], axis=0).T)

    def s_fwd(u, t):
        ct, e = divmod(u, 4)
        o = _dot(lhs(sfw32[t * 4 + e]), bf(zin[ct, t * 4 + e]))
        put(zout.at[ct, t * 4 + e], o if t % 2 else ticking(o))

    def s_filter(u, g):
        ct, e = divmod(u, 4)
        z = [tuple(zout[ct, t * 4 + e, pl.ds(g * 16 + i, 8), :] for i in (0, 8)) for t in range(8)]
        z[0], z[1] = [tuple(gate(v, SGLAG) for v in zz) for zz in z[0:2]]
        xk = _dft8(z, False)
        for k2 in range(8):
            wr = wf[0, ct, e, k2, pl.ds(g * 8, 8), :]
            wi = wf[1, ct, e, k2, pl.ds(g * 8, 8), :]
            re, im = xk[k2]
            xk[k2] = (re * wr - im * wi, re * wi + im * wr)
        for t, (re, im) in enumerate(_dft8(xk, True)):
            words = pack(re, im)
            if t < 4:
                pin(words)
            put(zin.at[ct, t * 4 + e, pl.ds(g * 8, 8), :], words)

    def s_inv(u, t):
        ct, e = divmod(u, 4)
        o = _dot(lhs(siv32[t * 4 + e]), bf(zin[ct, t * 4 + e]))
        put(zout.at[ct, t * 4 + e], o if t % 2 else ticking(o))

    def add_s_stage(sched, early, ready, t1, pause):
        ahead = 4 + S_LAG
        tick = early
        for t in sorted(range(8), key=lambda t: ready[t]):
            for i in range(t, 2 * ahead, 8):
                tick = max(tick + 0.5, ready[t])
                sched.add(tick, _once(s_fwd, i // 8, t))
        t1 = max(t1, int(tick) + 1)
        t2 = pause(t1 + 64 - ahead, t1 + 64)
        sched.add(max(max(ready), t2), side_path())
        for i in range(64):
            if i + ahead < 64:
                sched.add(t1 + i, _once(s_fwd, *divmod(2 * (i + ahead), 8)))
            sched.add(t1 + i, _once(s_filter, *divmod(i, 4)))
            if i + ahead < 64:
                sched.add(t1 + i, _once(s_fwd, *divmod(2 * (i + ahead) + 1, 8)))
        for i in range(69):
            if i >= 5:
                sched.add(t2 + min(i, 66), _once(s_inv, *divmod(2 * (i - 5), 8)))
            if i < 64:
                sched.add(t2 + i, _once(s_filter, i // 4, 4 + i % 4))
            if i >= 5:
                sched.add(t2 + min(i, 66), _once(s_inv, *divmod(2 * (i - 5) + 1, 8)))
        return [t2 + 16 * ct + 22 for ct in range(3)] + [t2 + 67]

    def d_inv_cols(b, ct):
        c, t = divmod(b, 8)
        ra, rb = PAIRS[ct]
        lane = _lane(16)
        lo = lane < 64
        u = [(zout[ct, t * 4 + e, r16(c), :], zout[ct, t * 4 + e, r16(4 + c), :]) for e in range(4)]
        u[0], u[1] = tuple(map(gate, u[0])), tuple(map(gate, u[1]))
        z = _dft4(u, True)
        z = [(re, _swap(im)) for re, im in z]
        if ct == 0:
            y0 = [pltpu.roll(side[2, pl.ds(64 * lb + 16 * c, 16), :], 64 - t, 1) for lb in range(4)]
        yield from _latency()
        for lb, (re, sw) in enumerate(z):
            sw = gate(sw)
            a, bb = lax.select(lo, re, sw), lax.select(lo, sw, re)
            if ct == 0:
                a = jnp.where(lane == 64, y0[lb], a)
            pin(a)
            ubuf[b % RING, ra, r16(lb), :] = a.astype(BF16)
            ubuf[b % RING, rb, r16(lb), :] = bb.astype(BF16)

    def d_inv_rows(b, lb, stats, first):
        u = [uout[b % RING, r, r16(lb), :] for r in range(8)]
        ys = yield from _d_butterfly_inv([gate(v) if r < 4 else v for r, v in enumerate(u)], pin, gate)
        xs = [x + y for x, y in zip(load_x(b, lb, first), ys)]
        for j in range(NT):
            put(xres.at[b, j, r16(lb), :], xs[j])
        stats[b, lb] = yield from ln_stats(xs)
        if b % 2:
            for j in range(4):
                a = [(xres[bb, j + o, r16(lb), :] - stats[bb, lb][0]) * stats[bb, lb][1]
                     for bb in (b - 1, b) for o in (0, 4)]
                a[0], a[3] = gate(a[0]), gate(a[3])
                for k, v in enumerate(_strassen_lhs(*a)):
                    if k in (1, 4):
                        pin(v)
                    abuf[b // 2, k, j, r16(lb), :] = v.astype(BF16)
                if j < 3:
                    yield

    def add_d_inv(sched, tick, b, gap, stats, first, cols=None):
        per_tick = 4
        cols = cols or [tick + ct * gap for ct in range(4)]
        for ct in range(4):
            sched.add(cols[ct], d_inv_cols(b, ct))
        tick = int(cols[3]) + XGAP + 1
        sched.add(tick, d_dots(b, 8, per_tick))
        tick += 8 // per_tick + 3
        for lb in range(4):
            sched.add(tick + lb * gap, d_inv_rows(b, lb, stats, first))
        return int(tick + 3 * gap) + 3 * XGAP + 1 + 4

    def gemm(lhs32, rhs32, jobs, sink):
        for slot, b, n in jobs:
            m = {}
            for k in (3, 1, 0, 6, 5, 4, 2):
                m[k] = ticking(_dot(lhs(*[lhs32[slot, k, j] for j in range(4)]), bf(rhs32[n // 2, k])))
                if k == 1:
                    sink(b + 1, n, m[1] - m[3])
                elif k == 0:
                    c11, c22 = m[3] - m[0], m[1] - m[0]
                elif k == 6:
                    c11 = m[6] - c11
                elif k == 5:
                    c22 = m[5] - c22
                elif k == 4:
                    sink(b, n, c11 - m[4])
                elif k == 2:
                    sink(b, n + 1, m[4] - m[2])
                    sink(b + 1, n + 1, c22 - m[2])
                yield

    def qkv_sink(b, n, o):
        c, t = divmod(b, 8)
        dst = (qbuf, kbuf, vbuf)[n // NT]
        for lb in range(4):
            put(dst.at[n % NT, t, pl.ds(8 + 64 * lb + 16 * c, 16), :], o[lb * 16:(lb + 1) * 16])
        if b == 0 and n >= NT:
            first = jnp.broadcast_to(o[0:1], (8, 128))
            for tt in range(8):
                dst[n % NT, tt, pl.ds(0, 8), :] = first

    def out_rows(r, i, last):
        c, t = divmod(r, 8)
        return (c * 8 + t % 2 * 4 + i, t // 2) if last and c == 0 else (r, i)

    def out_sink(last, r, n, o):
        for i in range(4):
            b, lb = out_rows(r, i, last)
            put(xres.at[b, n, r16(lb), :], xres[b, n, r16(lb), :] + o[i * 16:(i + 1) * 16])

    def attention(b, lb, h):
        c, t = divmod(b, 8)
        log2e = float(np.log2(np.e))
        scale = HEAD_DIM ** -0.5 * log2e
        r0 = 8 + 64 * lb + 16 * c + 8 * h
        src = [((t - 2 * w) % 8, -((t - 2 * w) // 8)) for w in range(WIN)]
        acc = [None] * WIN
        for j in range(NT):
            if j % 2 == 0:
                factor = gate(jnp.full((8, 128), scale, F32), ALAG)
            q = qbuf[j, t, pl.ds(r0, 8), :] * factor
            for w, (ts, sh) in enumerate(src):
                p = q * kbuf[j, ts, pl.ds(r0 - sh, 8), :]
                acc[w] = p if j == 0 else acc[w] + p
            if j % 2 and j < NT - 1:
                pin(*acc[j // 2 % 2::2])
                yield
        part = [(r, pltpu.roll(r, 64, 1)) for r in acc]
        yield from _latency()
        part = [r + rr for r, rr in part]
        part = [(r, pltpu.roll(r, 32, 1)) for r in part]
        yield from _latency()
        logits = [r + rr for r, rr in part]
        if r0 == 8:
            sub = lax.broadcasted_iota(jnp.int32, (8, 128), 0)
            logits = [jnp.where(sub >= sh, r, -1e9 * log2e) if sh else r
                      for r, (_, sh) in zip(logits, src)]
        logits[0] = gate(logits[0], ALAG)
        m = _tree(jnp.maximum, logits)
        ps = [jnp.exp2(r - m) for r in logits]
        total = _tree(_add, ps)
        pin(total)
        inv = pltpu.reciprocal(total, approx=True)
        inv = inv * (2.0 - total * inv)
        for j in range(NT):
            if j % 2 == 0:
                yield
                ps[0], ps[4] = gate(ps[0], ALAG), gate(ps[4], ALAG)
            o = _chain(_add, [ps[w] * vbuf[j, ts, pl.ds(r0 - sh, 8), :]
                              for w, (ts, sh) in enumerate(src)]) * inv
            if j % 2:
                pin(o)
            put(qbuf.at[j, t, pl.ds(r0, 8), :], o)

    def out_operands(r, i, last):
        for j in range(4):
            a = [qbuf[j + o, b % 8, pl.ds(8 + 64 * lb + 16 * (b // 8), 16), :]
                 for b, lb in (out_rows(r, i, last), out_rows(r + 1, i, last)) for o in (0, 4)]
            a[0], a[3] = gate(a[0]), gate(a[3])
            for k, v in enumerate(_strassen_lhs(*a)):
                if k in (1, 4):
                    pin(v)
                obuf[r // 2, k, j, r16(i), :] = v.astype(BF16)
            if j < 3:
                yield

    def store_rows(b, lb, tiles):
        c, t = divmod(b, 8)
        for j in tiles:
            words = pack(xres[b, j, r16(lb), :], xres[b + 1, j, r16(lb), :])
            pin(words)
            io32[j, lb, c, pl.ds(t // 2, 16, stride=4), :] = words

    unit_ticks = NT + 2 * XGAP
    step = 2
    out_ticks = 28

    def add_proj(sched, tick, c, lo, hi):
        jobs = [(b // step, b, n) for b in range(8 * c, 8 * c + 8, step) for n in range(lo, hi, step)]
        sched.add(tick, gemm(abuf32, wqkv32, jobs, qkv_sink))
        return tick + len(jobs) * out_ticks * step // NT

    def add_attention(sched, tick, pace, rows, last):
        units = [(r, i, half, h) for r in rows[::2] for i in range(4) for half in range(2) for h in range(2)]
        for n, (r, i, half, h) in enumerate(units):
            sched.add(tick + n * pace, attention(*out_rows(r + half, i, last), h))
            if half and h:
                sched.add(int(tick + n * pace) + unit_ticks, out_operands(r, i, last))

    def add_out(sched, tick, rows, last):
        jobs = [(r // 2, r, n) for r in rows[::2] for n in range(0, NT, 2)]
        sched.add(tick, gemm(obuf32, wo32, jobs, functools.partial(out_sink, last)))

    def add_tail(sched, tick, rows, last):
        ready = {}
        for i, r in enumerate(rows):
            t0 = tick + (i // 2 + 1) * out_ticks
            fast = i >= len(rows) - (2 if last else 4)
            if not last:
                t0 += 0 if fast else TOFF + i % 2 * out_ticks // 2
                ready[r % 8] = add_d_fwd(sched, t0, r, i % 2 if fast else out_ticks / 8)
            elif r % 2:
                c, p = r // 8, r % 8 // 2
                if fast:
                    for at, tiles in ((t0 - out_ticks // 4 + 3, range(6)), (t0, range(6, NT))):
                        for j in range(4):
                            sched.add(at, _once(store_rows, 2 * j, p, tiles))
                        sched.add(at + 1, _once(start, out_copies(c, p, tiles)))
                    continue
                for j in range(4):
                    sched.add(t0 + 3 * j + 3, _once(store_rows, *((r - 1, j) if c else (2 * j, p)), range(NT)))
                for lb in ([p] if c == 0 else range(4) if p == 3 else []):
                    sched.add(t0 + 16, _once(start, out_copies(c, lb, range(NT))))
        return ready

    q_ticks = 8 * out_ticks // step
    att_ticks = unit_ticks + 1 + 2
    order = [(a + 8) % NB for a in range(NB)]

    def add_attention_block(sched, cols, last):
        stats = {}
        t0 = max([add_d_inv(sched, 0, b, 0, stats, not last, cols) for b in range(step)])
        if not last:
            sched.add(cols[3] - KLEAD, _once(wait, qkv_copies(1) + dmat_cp))
            done = add_prep_wqkv(sched, cols[3] - KLEAD, 1, KPACE, [7] * 4)
            t0 = max(t0, done[0])
            assert all(d <= t0 + p * out_ticks / 4 for p, d in enumerate(done))
            sched.add(t0 + out_ticks, _once(wait, qkv_copies(2)))
            sched.add(t0 + out_ticks, _once(start, qkv_copies(0)))
            done = add_prep_wqkv(sched, t0 + out_ticks, 2, 2 * out_ticks - 4, [out_ticks - 4] * 4)
            assert all(d <= t0 + q_ticks + p * out_ticks for p, d in enumerate(done))
            sched.add(t0 + 2 * q_ticks, _once(wait, qkv_copies(0)))
            sched.add(t0 + 2 * q_ticks, _once(start, wo_copies))
            done = add_prep_wqkv(sched, t0 + 2 * q_ticks, 0, q_ticks - 10, [q_ticks / 4] * 4)
            assert done[-1] <= t0 + 4 * q_ticks
            sched.add(t0 + 8 * q_ticks, _once(wait, wo_copies))
            for i in range(32):
                sched.add(t0 + 8 * q_ticks + i * q_ticks / 16, prep_wo(*divmod(i, 8)))
        tick, kv_start, q_start = t0, {}, {}
        for kind, c in ("k0", "k1", "q1", "k2", "q2", "k3", "q3", "q0"):
            if kind == "k":
                kv_start[int(c)] = tick
                if c == "0" and not last:
                    tick = add_proj(sched, tick, 0, NT, 2 * NT)
                    jobs = [(b // step, b, n) for n in range(2 * NT, 3 * NT, step) for b in range(0, 8, step)]
                    sched.add(tick, gemm(abuf32, wqkv32, jobs, qkv_sink))
                    tick += q_ticks
                    continue
                tick = add_proj(sched, tick, int(c), NT, 3 * NT)
            else:
                q_start[int(c)] = tick
                tick = add_proj(sched, tick, int(c), 0, NT)
        pace = 2 * out_ticks / step
        for b in range(step, NB):
            due = kv_start[b // 8] + (b % 8 // step) * (2 if last or b >= 8 else 1) * out_ticks
            gap = min(1 + (b - step) * 0.5, DGAP1 if last else DGAP0)
            pace = DPACE1 if last else DPACE0
            at = (b - step) * pace
            at = t0 + at + max(0, at - 4 * q_ticks - out_ticks) * DSLOW
            if not last and b < 8:
                at, gap = max(cols[3], t0 + (b // step - 1) * out_ticks - (step - b % step) * 8), 1
            end = add_d_inv(sched, at, b, gap, stats, not last)
            assert end <= due, (b, end, due)
        begin = [q_start[c] + out_ticks + 3 for c in (1, 2, 3)] + [tick + (ATT1 if last else ATT0)]
        begin.append(tick + (NB // step - 1) * out_ticks - att_ticks)
        for i, c in enumerate((1, 2, 3, 0)):
            pace = (begin[i + 1] - begin[i]) / 64
            assert begin[i] >= max(kv_start[c], kv_start[(c - 1) % 4]) + 2 * q_ticks
            for p in range(4):
                assert begin[i] + 16 * p * pace >= q_start[c] + (4 if last and c == 0 else p + 1) * out_ticks
                assert begin[i] + (16 * p + 15) * pace + att_ticks <= tick + (4 * i + p) * out_ticks + 1e-6
            add_attention(sched, begin[i], pace, range(8 * c, 8 * c + 8), last)
        add_out(sched, tick, order, last)
        return tick + (NB // step) * out_ticks, add_tail(sched, tick, order, last)

    def add_input(sched):
        ready = {}
        after = (x_copies(2), x_copies(3) + perm_cp + w_copies(0) + w_copies(1),
                 w_copies(2) + w_copies(3), w_copies(4))
        for c in range(NC):
            sched.add(c * 32, _once(wait, x_copies(c)))
            sched.add(c * 32, _once(start, after[c]))
            for t in range(8):
                ready[t] = add_d_fwd(sched, c * 32 + t * 4, c * 8 + t, 1, 2, True)
        return 128 + 9, ready

    def add_filter_prep(sched, upper, begin, end):
        after = (([], qkv_copies(2)) if upper else
                 (w_copies(5) + w_copies(6), w_copies(7) + f256_cp + dmat_cp))
        for i in range(16):
            g, at = 4 * upper + i // 4, begin + i * (end - begin) / 16
            if i % 8 == 0:
                sched.add(at, _once(wait, w_copies(g) + w_copies(g + 1) + {0: perm_cp, 6: f256_cp}.get(g, [])))
                sched.add(at, _once(start, after[i // 8]))
            sched.add(at, _once(prep_filter, *w_tiles(g)[i % 4]))
        return end + 2

    def add_first_s_stage(sched):
        tick, ready = add_input(sched)
        sched.add(tick + WK0, _once(start, qkv_copies(1)))
        return add_s_stage(sched, tick, ready, add_filter_prep(sched, 0, F0, tick),
                           lambda begin, end: add_filter_prep(sched, 1, begin, end + FG))

    sched = _Schedule()

    start(x_copies(0) + tiny_cp)
    for ref in (abuf32, obuf32, ubuf32, wo32, sfw32, siv32, wide32):
        put(ref.at[(0,) * (len(ref.shape) - 2) + (pl.ds(0, 8),)], jnp.zeros((8, 128), U32))
    make_wide()
    start(x_copies(1))
    for t in range(8):
        make_s_fwd(t)
    for e in range(4):
        make_s_inv(e)
    wait(tiny_cp)
    for n in (1, 2, 4):
        never[n] = jnp.concatenate([tw_ref[16:24, 0:128]] * n, axis=1) != 0.0
    cols = add_first_s_stage(sched)
    tick, ready = add_attention_block(sched, cols, False)
    cols = add_s_stage(sched, tick, ready, tick, lambda begin, end: end)
    add_attention_block(sched, cols, True)
    sched.run()
    for c in range(NC):
        for lb in range(4):
            wait(out_copies(c, lb, range(NT)))


@jax.jit
def pallas_interleave_layers__spectral_gfnet__sliding_local_dilated__prompt_kernel(
    A_x: jax.Array,
    A_w_r: jax.Array,
    A_w_i: jax.Array,
    B_x: jax.Array,
    B_wqkv: jax.Array,
    B_wo: jax.Array,
):
    del B_x
    assert A_x.shape == (1, S, D) and A_w_r.shape == (S, D // 2 + 1)
    cst = _constants()
    x = A_x.astype(BF16).reshape(4, NC, 128, D)
    wr, wi = A_w_r.astype(BF16).T, A_w_i.astype(BF16).T
    hbm = pl.BlockSpec(memory_space=pl.ANY)
    vm = pltpu.VMEM
    out = pl.pallas_call(
        _kernel,
        in_specs=[hbm] * 9,
        out_specs=hbm,
        out_shape=jax.ShapeDtypeStruct((4, NC, 128, D), BF16),
        scratch_shapes=[
            vm((NT, 4, NC, 128, 128), BF16),
            vm((17, 128, 128), BF16),
            vm((32, 128, 128), BF16),
            vm((32, 128, 128), BF16),
            vm((256, 512), BF16),
            vm((2, 16, 512, 128), BF16),
            vm((2, 4, 4, 8, 64, 128), F32),
            vm((3 * NT, D, 128), BF16),
            vm((NT, D // 2, 128), U32),
            vm((12, 7, 512, 128), BF16),
            vm((NT, D, 128), BF16),
            vm((4, 7, 512, 128), BF16),
            vm((NB, NT, 64, 128), F32),
            vm((4, 32, 64, 128), U32),
            vm((4, 32, 128, 128), F32),
            vm((RING, 8, 64, 128), BF16),
            vm((RING, 9, 64, 128), F32),
            vm((NB // 2, 7, 4, 64, 128), BF16),
            vm((NB // 2, 7, 4, 64, 128), BF16),
            vm((NT, 8, 264, 128), F32),
            vm((NT, 8, 264, 128), F32),
            vm((NT, 8, 264, 128), F32),
            vm((3, 256, 128), F32),
            vm((8, 256, 128), BF16),
            vm((24, 256), F32),
            vm((2, 16, 128), BF16),
            vm((1, S), BF16),
            vm((1, S), BF16),
            pltpu.SemaphoreType.DMA((NC,)),
            pltpu.SemaphoreType.DMA((4,)),
            pltpu.SemaphoreType.DMA((8,)),
            pltpu.SemaphoreType.DMA((3,)),
            pltpu.SemaphoreType.DMA(()),
            pltpu.SemaphoreType.DMA(()),
        ],
        compiler_params=pltpu.CompilerParams(
            vmem_limit_bytes=120 * 2**20),
    )(x, wr, wi, B_wqkv.astype(BF16), B_wo.astype(BF16),
      cst["small"], cst["f256"], cst["tw"], cst["d8"])
    return out.reshape(1, S, D)
```

```python
import functools

import jax
import jax.numpy as jnp
import numpy as np
from jax import lax
from jax.experimental import pallas as pl
from jax.experimental.pallas import tpu as pltpu

S, D = 2048, 1024
NT = D // 128
NC = 4
WIN = 8
HEAD_DIM = 32
EPS = 1e-5
F32, BF16, U32 = jnp.float32, jnp.bfloat16, jnp.uint32
PAIRS = ((0, 4), (1, 7), (2, 6), (3, 5))
RSQ2 = float(np.sqrt(0.5))
NB = S // 64

RING = 8
XGAP = 3
GLAG = 4
ALAG = 4
SGLAG = 3
S_LAG = 2
F0 = 120
KLEAD = 46
KPACE = 40
DGAP0 = 4.75
DGAP1 = 4.2
DPACE0 = 20
DPACE1 = 15.5
DSLOW = 0.6
SYNC = 3
ILAG = 3
FG = 10
TOFF = 2
WK0 = 24
ATT0 = 15
ATT1 = 95


def _residues(r):
    return (0, 8) if r == 0 else (r, 16 - r)


def _d_matrices():
    n = np.arange(64)[:, None]
    a = np.arange(32)
    fwd = np.zeros((8, 128, 128))
    inv = np.zeros((8, 128, 128))
    for r in range(8):
        kd = np.concatenate([16 * a + p for p in _residues(r)])
        weight = np.full(64, 2.0)
        if r == 0:
            kd[0], weight[0] = D // 2, 1.0
            ph = np.exp(-2j * np.pi * n * kd[None, :] / D)
            sgn = np.where(kd % 16 == 0, 1.0, -1.0)[None, :]
            m = np.concatenate([ph, ph * sgn], axis=0)
            re, im = m.real.copy(), m.imag.copy()
            ire, iim = re.copy(), im.copy()
            im[:, 0] = 1.0
            iim[:, 0] = 1.0
        else:
            p = 12 if r == 4 else r
            ph = np.exp(-2j * np.pi * n * kd[None, :] / D)
            si = np.where(kd % 16 == p, 1.0, -1.0)[None, :]
            m = np.concatenate([ph, 1j * si * ph], axis=0)
            re, im = m.real, m.imag
            ire, iim = re, im
        swapped = r in (4, 7, 6, 5)
        cols = [im, re] if swapped else [re, im]
        icols = [iim * weight, ire * weight] if swapped else [ire * weight, iim * weight]
        fwd[r] = np.concatenate(cols, axis=1)
        inv[r] = np.concatenate(icols, axis=1).T / D
    return fwd, inv


def _side_matrices():
    l = np.arange(256)
    f = np.exp(-2j * np.pi * ((l[:, None] * l[None, :]) % 256) / 256)
    f256 = np.concatenate([f.real, f.imag], axis=1)
    t = np.arange(8)
    tw = np.exp(-2j * np.pi * t[:, None] * l[None, :] / S)
    tw = np.concatenate([tw.real, tw.imag, np.zeros((8, 256))], axis=0)
    g = np.exp(-2j * np.pi * t[:, None] * t[None, :] / 8)
    d8 = np.zeros((2, 16, 128))
    d8[0, :, :16] = np.block([[g.real, -g.imag], [g.imag, g.real]])
    d8[1, :, :16] = d8[0, :, :16].T / S
    return f256, tw, d8


def _filter_rows():
    p = np.zeros((1, 128, 128))
    for k in range(32):
        for e in range(4):
            p[0, e * 32 + k, 4 * k + e] = 1.0
    return p


@functools.lru_cache(maxsize=None)
def _constants():
    dfw, div = _d_matrices()
    f256, tw, d8 = _side_matrices()
    small = np.concatenate([dfw, div, _filter_rows()], axis=0)
    b = lambda x: np.asarray(x, np.float32).astype(BF16)
    return dict(small=b(small), f256=b(f256),
                tw=np.asarray(tw, np.float32), d8=b(d8))


def _dot(a, b):
    return jnp.dot(a, b, preferred_element_type=F32)


def _dot_nt(a, b):
    return lax.dot_general(a, b, (((1,), (1,)), ((), ())), preferred_element_type=F32)


def _tree(op, xs):
    xs = list(xs)
    while len(xs) > 1:
        xs = [op(xs[i], xs[i + 1]) if i + 1 < len(xs) else xs[i] for i in range(0, len(xs), 2)]
    return xs[0]


def _chain(op, xs):
    return functools.reduce(op, xs)


def _lane(rows):
    return lax.broadcasted_iota(jnp.int32, (rows, 128), 1)


def _swap(x):
    return pltpu.roll(x, 64, 1)


def _unpack(w, i):
    return pltpu.unpack_elementwise(w, index=i, packed_dtype=BF16, unpacked_dtype=F32)


def _latency():
    for _ in range(XGAP):
        yield


def _add(a, b):
    return a + b


def _row_mean(xs):
    return jnp.sum(_tree(_add, xs), axis=1, keepdims=True) * (1.0 / D)


def _twiddle16(r, x, y):
    lo = _lane(x.shape[0]) < 64
    wr, wi = float(np.cos(np.pi * r / 8)), float(-np.sin(np.pi * r / 8))
    cross = jnp.where(lo, 0.0, wr)
    return x * jnp.where(lo, 1.0, wi) + y * cross, y * jnp.where(lo, 1.0, -wi) + x * cross


def _d_butterfly_fwd(a, emit, pin, wide):
    s = [a[j] + a[j + 4] for j in range(4)]
    e, o = s[0] + s[2], s[1] + s[3]
    total, t4 = e + o, e - o
    emit(4, t4)
    d0, nd2 = a[0] - a[4], a[6] - a[2]
    d1, d3 = a[1] - a[5], a[3] - a[7]
    p, q = (d1 - d3) * RSQ2, (d1 + d3) * -RSQ2
    ts = {1: (d0 + p, q + nd2), 2: (s[0] - s[2], s[3] - s[1]), 3: (d0 - p, q - nd2)}
    mean8 = jnp.sum(total, axis=1, keepdims=True) * (1.0 / 128)
    if wide:
        for r, (tr, ti) in ts.items():
            emit(r, tr)
            emit(8 - r, ti)
    else:
        ab = {r: _twiddle16(r, *t) for r, t in ts.items()}
        ab = {r: (a, _swap(b)) for r, (a, b) in ab.items()}
    dev = _tree(_add, [v * v for t in ts.values() for v in t]) * 2.0 + t4 * t4
    pin(dev)
    yield from _latency()
    t0 = total - mean8
    emit(0, t0)
    var = jnp.sum(dev + t0 * t0, axis=1, keepdims=True) * (1.0 / (NT * D))
    if not wide:
        for r, (x, y) in ab.items():
            emit(r, x + y)
            emit(8 - r, x - y)
    yield from _latency()
    return lax.rsqrt(var + EPS)


def _d_butterfly_inv(u, pin, gate):
    ab = {r: (u[r] + u[8 - r], _swap(u[r] - u[8 - r])) for r in (1, 2, 3)}
    e, o = u[0] + u[4], u[0] - u[4]
    yield from _latency()
    ts = {r: _twiddle16(r, x, gate(y)) for r, (x, y) in ab.items()}
    pin(*[t[0] for t in ts.values()])
    yield
    s = [e + ts[2][0], o - ts[2][1], e - ts[2][0], o + ts[2][1]]
    p = (ts[1][0] - ts[3][0]) * RSQ2
    q = (ts[1][1] + ts[3][1]) * RSQ2
    d0, d1, d2, nd3 = ts[1][0] + ts[3][0], p - q, ts[3][1] - ts[1][1], p + q
    return [s[0] + d0, s[1] + d1, s[2] + d2, s[3] - nd3,
            s[0] - d0, s[1] - d1, s[2] - d2, s[3] + nd3]


def _strassen_lhs(a11, a12, a21, a22):
    return [a11 + a22, a21 + a22, a11, a22, a11 + a12, a21 - a11, a12 - a22]


def _strassen_rhs(b11, b12, b21, b22):
    return [b11 + b22, b11, b22 - b12, b11 - b21, b22, b11 + b12, b21 + b22]


def _cadd(a, b):
    return a[0] + b[0], a[1] + b[1]


def _csub(a, b):
    return a[0] - b[0], a[1] - b[1]


def _dft4(z, inverse):
    a, b = _cadd(z[0], z[2]), _csub(z[0], z[2])
    c, d = _cadd(z[1], z[3]), _csub(z[1], z[3])
    minus = (b[0] + d[1], b[1] - d[0])
    plus = (b[0] - d[1], b[1] + d[0])
    return [_cadd(a, c), plus if inverse else minus, _csub(a, c), minus if inverse else plus]


def _dft8(z, inverse):
    ev = _dft4(z[0::2], inverse)
    od = _dft4(z[1::2], inverse)
    out = [None] * 8
    out[0], out[4] = _cadd(ev[0], od[0]), _csub(ev[0], od[0])
    (er, ei), (x, y) = ev[2], od[2]
    minus, plus = (er + y, ei - x), (er - y, ei + x)
    out[2], out[6] = (plus, minus) if inverse else (minus, plus)
    for k in (1, 3):
        (er, ei), (x, y) = ev[k], od[k]
        sm, df = (x + y) * RSQ2, (x - y) * RSQ2
        if not inverse:
            if k == 1:
                out[1], out[5] = (er + sm, ei - df), (er - sm, ei + df)
            else:
                out[3], out[7] = (er - df, ei - sm), (er + df, ei + sm)
        else:
            if k == 1:
                out[1], out[5] = (er + df, ei + sm), (er - df, ei - sm)
            else:
                out[3], out[7] = (er - sm, ei + df), (er + sm, ei - df)
    return out


class _Schedule:
    def __init__(self):
        self.pending = []

    def add(self, tick, gen):
        self.pending.append((int(tick), len(self.pending), gen))

    def run(self):
        pending = sorted(self.pending, key=lambda p: p[:2])
        active, tick, i = [], 0, 0
        while active or i < len(pending):
            while i < len(pending) and pending[i][0] <= tick:
                active.append(pending[i][2])
                i += 1
            for g in list(active):
                if next(g, 0) == 0:
                    active.remove(g)
            tick += 1
        self.pending = []


def _once(fn, *args):
    fn(*args)
    return
    yield


def _kernel(x_hbm, wr_hbm, wi_hbm, wqkv_hbm, wo_hbm, small_hbm, f256_hbm, tw_hbm, d8_hbm,
            out_hbm,
            io, small, sfw, siv, f256, wraw, wf, wqkv_raw, wtmp, wqkv, wo_raw, wo,
            xres, zin, zout, ubuf, uout, abuf, obuf, qbuf, kbuf, vbuf, side,
            wide, tw_ref, d8_ref, wr_edge, wi_edge, sem_x, sem_c, sem_w, sem_qkv, sem_wo, sem_out):

    def x_copies(c):
        return [pltpu.make_async_copy(x_hbm.at[:, c, :, pl.ds(j * 128, 128)], io.at[j, :, c],
                                      sem_x.at[c]) for j in range(NT)]

    def out_copies(c, lb, tiles):
        return [pltpu.make_async_copy(io.at[j, lb, c], out_hbm.at[lb, c, :, pl.ds(j * 128, 128)],
                                      sem_out) for j in tiles]

    perm_cp, dmat_cp, f256_cp = ([pltpu.make_async_copy(s, d, sem_c.at[i])] for i, (s, d) in enumerate((
        (small_hbm.at[pl.ds(16, 1)], small.at[pl.ds(16, 1)]),
        (small_hbm.at[pl.ds(0, 16)], small.at[pl.ds(0, 16)]), (f256_hbm, f256))))

    tiny_cp = [pltpu.make_async_copy(s, d, sem_c.at[3]) for s, d in (
        (tw_hbm, tw_ref), (d8_hbm, d8_ref),
        (wr_hbm.at[pl.ds(D // 2, 1)], wr_edge), (wi_hbm.at[pl.ds(D // 2, 1)], wi_edge))]

    def w_tiles(g):
        return [(g // 2 % 2, 8 * (g % 2) + 2 * i + g // 4) for i in range(4)]

    def w_copies(g):
        return [pltpu.make_async_copy((wr_hbm, wi_hbm)[ri].at[pl.ds(0, 512), pl.ds(m * 128, 128)],
                                      wraw.at[ri, m], sem_w.at[g]) for ri, m in w_tiles(g)]

    def qkv_copies(g):
        return [pltpu.make_async_copy(wqkv_hbm.at[:, pl.ds(g * D + j * 128, 128)],
                                      wqkv_raw.at[g * NT + j], sem_qkv.at[g]) for j in range(NT)]

    wo_copies = [pltpu.make_async_copy(wo_hbm.at[:, pl.ds(j * 128, 128)], wo_raw.at[j], sem_wo)
                 for j in range(NT)]

    def start(cs):
        for cp in cs:
            cp.start()

    def wait(cs):
        for cp in cs:
            cp.wait()

    io32, wraw32, wo_raw32 = io.bitcast(U32), wraw.bitcast(U32), wo_raw.bitcast(U32)
    small32, sfw32, siv32, wide32 = (r.bitcast(U32) for r in (small, sfw, siv, wide))
    wqkv_raw32, wqkv32, wo32 = (r.bitcast(U32) for r in (wqkv_raw, wqkv, wo))
    ubuf32, abuf32, obuf32 = ubuf.bitcast(U32), abuf.bitcast(U32), obuf.bitcast(U32)

    never = {}
    token = {}

    def pin(*values):
        for v in values:
            key = v.shape[0], v.dtype == F32
            token[key] = (lax.max if key[1] else lax.bitwise_xor)(token[key], v) if key in token else v

    clock = []

    def gate(v, lag=GLAG):
        if len(clock) < lag:
            return v
        old = clock[-lag] if v.dtype == F32 else pltpu.bitcast(clock[-lag], v.dtype)
        if v.shape[0] == 8:
            return lax.select(never[1], old, v)
        return lax.concatenate([lax.select(never[1], old, v[0:8]), v[8:]], 0)

    def ticking(o):
        clock.append(o[0:8])
        del clock[:-16]
        return o

    def lhs(*tiles):
        if not token and len(tiles) == 4 and len(clock) >= SYNC:
            pin(clock[-SYNC])
        words = lax.concatenate(tiles, 1) if len(tiles) > 1 else tiles[0]
        if token:
            parts = [pltpu.bitcast(v, U32) if is_float else v for (_, is_float), v in token.items()]
            token.clear()
            w = _chain(lax.bitwise_xor, [v[i:i + 8] if v.shape[0] > 8 else v
                                         for v in parts for i in range(0, v.shape[0], 8)])
            w = lax.concatenate([w] * len(tiles), 1) if len(tiles) > 1 else w
            words = lax.concatenate([lax.select(never[len(tiles)], w, words[0:8]), words[8:]], 0)
        return pltpu.bitcast(words, BF16)

    def bf(words):
        return pltpu.bitcast(words, BF16)

    def pack(a, b):
        return pltpu.bitcast(pltpu.pack_elementwise([a, b], packed_dtype=BF16), U32)

    def r16(i):
        return pl.ds(i * 16, 16)

    always = {}

    def put(ref, v):
        if v.shape not in always:
            always[v.shape] = jnp.ones(v.shape, jnp.bool_)
        pltpu.store(ref, v, mask=always[v.shape])

    def load_x(b, lb, from_input):
        if from_input:
            c, t = divmod(b, 8)
            return [_unpack(io32[j, lb, c, pl.ds(t // 2, 16, stride=4), :], t % 2) for j in range(NT)]
        return [xres[b, j, r16(lb), :] for j in range(NT)]

    def unit(p):
        angle = (((p + S // 2) & (S - 1)) - S // 2).astype(F32) * (2 * np.pi / S)
        return jnp.cos(angle), jnp.sin(angle)

    def times_row(a, b, i):
        br, bi = (jnp.broadcast_to(v[i:i + 1], (8, 128)) for v in b)
        return a[0] * br - a[1] * bi, a[0] * bi + a[1] * br

    def make_wide():
        row, lane = lax.broadcasted_iota(jnp.int32, (8, 128), 0), _lane(8)
        for ct, (ra, rb) in enumerate(PAIRS):
            res = _residues(ra) + _residues(rb)
            kd = (lane & 31) * 16 + _chain(
                _add, [jnp.where(lane >> 5 == g, p, 0) for g, p in enumerate(res)])
            if ct == 0:
                kd = jnp.where(lane == 0, D // 2, kd)
            fine, coarse = unit(-2 * row * kd), [unit(-16 * (row + 8 * h) * kd) for h in range(2)]
            for a in range(16):
                re, im = times_row(fine, coarse[a // 8], a % 8)
                if ct == 0:
                    even = kd & 7 == 0
                    top = jnp.where(even, re, 0.0), jnp.where(lane == 0, 1.0, jnp.where(even, im, 0.0))
                    bottom = jnp.where(even, 0.0, re), jnp.where(even, 0.0, im)
                else:
                    sign = jnp.where(kd & 7 == ra, 1.0, -1.0)
                    top, bottom = (re, im), (-sign * im, sign * re)
                for i in range(2):
                    wide[2 * ct + i, pl.ds(8 * a, 8), :] = top[i].astype(BF16)
                    wide[2 * ct + i, pl.ds(128 + 8 * a, 8), :] = bottom[i].astype(BF16)

    def make_s_fwd(t):
        row, lane = lax.broadcasted_iota(jnp.int32, (8, 128), 0), _lane(8)
        pos = 8 * (lane >> 1) + t
        fine = unit((lane & 1) * (S // 4) - 4 * row * pos)
        shift, coarse = unit(-row * pos), unit(-32 * row * pos)
        for e in range(4):
            base = times_row(fine, shift, e)
            for g in range(8):
                for i, v in enumerate(times_row(base, coarse, g)):
                    sfw[t * 4 + e, pl.ds(16 * g + 8 * i, 8), :] = v.astype(BF16)

    def make_s_inv(e):
        row, lane = lax.broadcasted_iota(jnp.int32, (8, 128), 0), _lane(8)
        freq = 4 * (lane >> 1) + e
        fine = [v * (1.0 / S) for v in unit((lane & 1) * (S // 4) + 8 * row * freq)]
        shift, coarse = unit(row * freq), unit(64 * row * freq)
        for t in range(8):
            base = times_row(fine, shift, t)
            for g in range(8):
                for i, v in enumerate(times_row(base, coarse, g)):
                    siv[t * 4 + e, pl.ds(64 * i + 8 * g, 8), :] = v.astype(BF16)

    def prep_filter(ri, m):
        sub = lax.broadcasted_iota(jnp.int32, (8, 128), 0)
        edge = (wr_edge, wi_edge)[ri]
        res = {}
        for i in range(8):
            words = wraw32[ri, m, pl.ds(i, 32, stride=8), :]
            res[2 * i], res[2 * i + 1] = _unpack(words, 0), _unpack(words, 1)
        first = res[0][0:8]
        dst = pl.ds((m % 2) * 16 + ri * 8, 8)
        prev = jnp.zeros((8, 128), F32) if m < 2 else side[1, dst, :]
        put(side.at[1, dst, :], jnp.where(sub == m // 2, jnp.broadcast_to(first[0:1], (8, 128)), prev))
        nyq = jnp.broadcast_to(edge[0:1, pl.ds(m * 128, 128)].astype(F32), (8, 128))
        res[0] = jnp.concatenate([jnp.where(sub == 0, nyq, first), res[0][8:]], axis=0)
        for ct, (ra, rb) in enumerate(PAIRS):
            blk = jnp.concatenate([res[p] for p in _residues(ra) + _residues(rb)], axis=0)
            o = _dot_nt(lhs(small32[16]), blk.astype(BF16))
            for e in range(4):
                put(wf.at[ri, ct, e, m // 2, pl.ds((m % 2) * 32, 32), :], o[e * 32:(e + 1) * 32])

    def prep_wqkv_cross(g, r):
        pos = (_lane(8) >> 2) & 7
        u = [wqkv_raw32[g * NT + (-j) % 8, pl.ds(r * 8, 8), :] for j in range(NT)]
        u[0], u[4] = gate(u[0]), gate(u[4])
        for bit in range(3):
            m = ((pos >> bit) & 1) == 1
            u = [lax.select(m, u[(j - (1 << bit)) % 8], u[j]) for j in range(NT)]
        for j in range(NT):
            if j < 4:
                pin(u[j])
            put(wtmp.at[j, pl.ds(r * 8, 8), :], u[j])

    def prep_wqkv_pair(g, p, part):
        lane = _lane(8)
        ws = {}
        for n in range(2):
            index = (lane & 3) * 32 + (((lane >> 2) + 2 * p + n) & 7) * 4 + (lane >> 5)
            for half in range(2):
                for r in range(part * 2, part * 2 + 2):
                    w = gate(wtmp[2 * p + n, pl.ds(half * 256 + r * 8, 8), :])
                    ws[r, half, n] = jnp.take_along_axis(w, index, axis=1)
        yield from _latency()
        for r in range(part * 2, part * 2 + 2):
            quad = [ws[r, half, n] for half in range(2) for n in range(2)]
            ops = [_strassen_rhs(*[_unpack(w, i) for w in quad]) for i in range(2)]
            for k in range(7):
                word = {1: quad[0], 4: quad[3]}.get(k)
                if word is None:
                    word = pack(ops[0][k], ops[1][k])
                if k in (2, 3):
                    pin(word)
                put(wqkv32.at[g * 4 + p, k, pl.ds(r * 8, 8), :], word)

    def add_prep_wqkv(sched, tick, g, ticks, pair_ticks):
        for r in range(64):
            sched.add(tick + r * ticks / 64, _once(prep_wqkv_cross, g, r))
        tick = int(tick + ticks) + 1
        done = []
        for p, n in enumerate(pair_ticks):
            for i in range(16):
                sched.add(tick + i * n / 16, prep_wqkv_pair(g, p, i))
            tick += n
            done.append(int(tick) + XGAP + 1)
        return done

    def prep_wo(p, part):
        v, pair = divmod(part, 2)
        upper = lax.broadcasted_iota(jnp.int32, (8, 128), 0) >= 4
        ws = [[wo_raw32[2 * p + n, pl.ds(128 * v + 2 * f + pair, 8, stride=16), :] for f in range(8)]
              for n in range(2)]
        for o in range(4):
            quad = [lax.select(upper, w[(2 * v + 1 + j) % 8], w[(2 * v + j) % 8])
                    for j in (o, o + 4) for w in ws]
            quad[0] = gate(quad[0])
            for i in range(2):
                for k, x in enumerate(_strassen_rhs(*[_unpack(w, i) for w in quad])):
                    if k in (2, 3):
                        pin(x)
                    wo[p, k, pl.ds(o * 128 + (2 * pair + i) * 32 + 8 * v, 8), :] = x.astype(BF16)
            if o < 3:
                yield

    def ln_stats(xs):
        lane_mean = _tree(_add, xs) * (1.0 / NT)
        lane_m2 = _tree(_add, [jnp.square(x - lane_mean) for x in xs])
        pin(lane_m2)
        mean = jnp.sum(lane_mean, axis=1, keepdims=True) * (1.0 / 128)
        yield from _latency()
        m2 = lane_m2 + jnp.square(gate(lane_mean) - mean) * float(NT)
        pin(m2)
        var = jnp.sum(m2, axis=1, keepdims=True) * (1.0 / D)
        yield from _latency()
        return mean, lax.rsqrt(gate(jnp.broadcast_to(var, (16, 128))) + EPS)

    def d_fwd_rows(b, lb, from_input=False):
        xs = load_x(b, lb, from_input)

        def emit(r, v):
            if r % 4 == 0 or (r < 4 and not from_input):
                pin(v)
            ubuf[b % RING, r, r16(lb), :] = v.astype(BF16)

        xs[:4] = [gate(x, ILAG if from_input else GLAG) for x in xs[:4]]
        inv = yield from _d_butterfly_fwd(xs, emit, pin, from_input)
        inv = jnp.broadcast_to(inv, (16, 128))
        pin(inv)
        put(uout.at[b % RING, 8, r16(lb), :], inv)

    def d_dots(b, base, per_tick):
        for r in range(8):
            o = _dot(lhs(ubuf32[b % RING, r]), bf(small32[base + r]))
            put(uout.at[b % RING, r], o)
            if r % per_tick == per_tick - 1 and r < 7:
                yield

    def d_dots_wide(b):
        for ct, (ra, rb) in enumerate(PAIRS):
            u = lhs(ubuf32[b % RING, ra], ubuf32[b % RING, rb])
            for i, r in enumerate((ra, rb)):
                o = _dot(u, bf(wide32[2 * ct + i]))
                put(uout.at[b % RING, r], ticking(o) if i else o)
            if ct < 3:
                yield

    def d_fwd_cols(b, ct, is_wide):
        c, t = divmod(b, 8)
        ra, rb = PAIRS[ct]
        lane = _lane(16)
        lo = lane < 64
        z, x0 = [], []
        for lb in range(4):
            a, bb, inv = (uout[b % RING, r, r16(lb), :] for r in (ra, rb, 8))
            inv = gate(inv, ILAG if is_wide else GLAG)
            a, bb = a * inv, bb * inv
            if is_wide:
                if ct == 0:
                    x0.append(pltpu.roll(bb, t, 1) if t else bb)
                    bb = jnp.where(lane == 0, 0.0, bb)
                z.append((a, bb))
                continue
            if ct == 0:
                x0.append(pltpu.roll(a, (t + 64) % 128, 1))
                a = jnp.where(lane == 64, 0.0, a)
            im = lax.select(lo, bb, a)
            z.append((lax.select(lo, a, bb), _swap(im)))
        if not is_wide:
            yield from _latency()
        for e, (re, im) in enumerate(_dft4(z, False)):
            words = pack(re, im)
            if e < 2:
                pin(words)
            put(zin.at[ct, t * 4 + e, r16(c), :], words)
        if is_wide and ct == 0:
            yield from _latency()
        for lb, v in enumerate(x0):
            ls = pl.ds(64 * lb + 16 * c, 16)
            prev = jnp.zeros((16, 128), F32) if t == 0 else side[0, ls, :]
            v = jnp.where(lane == t, v, prev)
            pin(v)
            put(side.at[0, ls, :], v)

    def add_d_fwd(sched, tick, b, gap, per_tick=4, from_input=False):
        for lb in range(4):
            sched.add(tick + lb * gap, d_fwd_rows(b, lb, from_input))
        tick = int(tick + 3 * gap) + XGAP + 1
        sched.add(tick, d_dots_wide(b) if from_input else d_dots(b, 0, per_tick))
        for ct in range(4):
            sched.add(tick + 8 // per_tick + 3 + ct * gap, d_fwd_cols(b, ct, from_input))
        return int(tick + 8 // per_tick + 3 + 3 * gap) + XGAP + 1

    def side_path():
        vt = side[0].T[0:8]
        yield
        zero8 = jnp.zeros((8, 256), F32)
        u = _dot(jnp.concatenate([vt, zero8], axis=0).astype(BF16), f256[...])[0:8]
        twr, twi = tw_ref[0:8, :], tw_ref[8:16, :]
        ur, ui = u[:, 0:256], u[:, 256:512]
        pad = jnp.zeros((112, 256), BF16)
        for _ in range(4):
            yield
        uu = jnp.concatenate([ur * twr - ui * twi, ur * twi + ui * twr], axis=0).astype(BF16)
        xk = _dot(d8_ref[0], jnp.concatenate([uu, pad], axis=0))
        for _ in range(4):
            yield
        wr = jnp.concatenate([side[1, 0:8, :], side[1, 16:24, :]], axis=1)
        wi = jnp.concatenate([side[1, 8:16, :], side[1, 24:32, :]], axis=1)
        xr, xi = xk[0:8], xk[8:16]
        yy = jnp.concatenate([xr * wr - xi * wi, xr * wi + xi * wr], axis=0).astype(BF16)
        p = _dot(d8_ref[1], jnp.concatenate([yy, pad], axis=0))
        for _ in range(4):
            yield
        twr, twi = tw_ref[0:8, :], tw_ref[8:16, :]
        pr, pi = p[0:8], p[8:16]
        g = jnp.concatenate([pr * twr + pi * twi, pi * twr - pr * twi], axis=1)
        g = jnp.concatenate([g, jnp.zeros((8, 512), F32)], axis=0).astype(BF16)
        y0 = _dot_nt(g, f256[...])
        for _ in range(4):
            yield
        put(side.at[2], jnp.concatenate([y0, jnp.zeros((112, 256), F32)], axis=0).T)

    def s_fwd(u, t, timed):
        ct, e = divmod(u, 4)
        o = _dot(lhs(sfw32[t * 4 + e]), bf(zin[ct, t * 4 + e]))
        put(zout.at[ct, t * 4 + e], ticking(o) if timed else o)

    def s_filter(u, g, lag=SGLAG):
        ct, e = divmod(u, 4)
        z = [tuple(zout[ct, t * 4 + e, pl.ds(g * 16 + i, 8), :] for i in (0, 8)) for t in range(8)]
        z[0], z[1] = [tuple(gate(v, lag) for v in zz) for zz in z[0:2]]
        xk = _dft8(z, False)
        for k2 in range(8):
            wr = wf[0, ct, e, k2, pl.ds(g * 8, 8), :]
            wi = wf[1, ct, e, k2, pl.ds(g * 8, 8), :]
            re, im = xk[k2]
            xk[k2] = (re * wr - im * wi, re * wi + im * wr)
        for t, (re, im) in enumerate(_dft8(xk, True)):
            words = pack(re, im)
            if t < 4:
                pin(words)
            put(zin.at[ct, t * 4 + e, pl.ds(g * 8, 8), :], words)

    def s_inv(u, t, timed):
        ct, e = divmod(u, 4)
        o = _dot(lhs(siv32[t * 4 + e]), bf(zin[ct, t * 4 + e]))
        put(zout.at[ct, t * 4 + e], ticking(o) if timed else o)

    def add_s_stage(sched, early, ready, t1, pause):
        ahead = 4 + S_LAG
        tick = early
        for t in sorted(range(8), key=lambda t: ready[t]):
            for i in range(t, 2 * ahead, 8):
                tick = max(tick + 0.5, ready[t])
                sched.add(tick, _once(s_fwd, i // 8, t, pause is None or t % 2 == 0))
        t1 = max(t1, int(tick) + 1)
        if pause is None:
            sched.add(max(max(ready), t1), side_path())
            for i in range(128):
                if i + 2 * ahead < 128:
                    sched.add(t1 + i, _once(s_fwd, *divmod(i + 2 * ahead, 8), True))
                sched.add(t1 + i, _once(s_filter, *divmod(i, 8), SGLAG if i < 119 else SGLAG + 2))
                sched.add(t1 + 9 + (i if i < 120 else 120 + (i - 120) // 4),
                          _once(s_inv, *divmod(i, 8), i >= 118 - 2 * ahead))
            return [t1 + 32 * ct + 40 for ct in range(3)] + [t1 + 131]
        t2 = pause(t1 + 64 - ahead, t1 + 64)
        sched.add(max(max(ready), t2), side_path())
        for i in range(64):
            if i + ahead < 64:
                sched.add(t1 + i, _once(s_fwd, *divmod(2 * (i + ahead), 8), True))
            sched.add(t1 + i, _once(s_filter, *divmod(i, 4)))
            if i + ahead < 64:
                sched.add(t1 + i, _once(s_fwd, *divmod(2 * (i + ahead) + 1, 8), False))
        for i in range(69):
            if i >= 5:
                sched.add(t2 + min(i, 66), _once(s_inv, *divmod(2 * (i - 5), 8), True))
            if i < 64:
                sched.add(t2 + i, _once(s_filter, i // 4, 4 + i % 4))
            if i >= 5:
                sched.add(t2 + min(i, 66), _once(s_inv, *divmod(2 * (i - 5) + 1, 8), False))
        return [t2 + 16 * ct + 22 for ct in range(3)] + [t2 + 67]

    def d_inv_cols(b, ct):
        c, t = divmod(b, 8)
        ra, rb = PAIRS[ct]
        lane = _lane(16)
        lo = lane < 64
        u = [(zout[ct, t * 4 + e, r16(c), :], zout[ct, t * 4 + e, r16(4 + c), :]) for e in range(4)]
        u[0], u[1] = tuple(map(gate, u[0])), tuple(map(gate, u[1]))
        z = _dft4(u, True)
        z = [(re, _swap(im)) for re, im in z]
        if ct == 0:
            y0 = [pltpu.roll(side[2, pl.ds(64 * lb + 16 * c, 16), :], 64 - t, 1) for lb in range(4)]
        yield from _latency()
        for lb, (re, sw) in enumerate(z):
            sw = gate(sw)
            a, bb = lax.select(lo, re, sw), lax.select(lo, sw, re)
            if ct == 0:
                a = jnp.where(lane == 64, y0[lb], a)
            pin(a)
            ubuf[b % RING, ra, r16(lb), :] = a.astype(BF16)
            ubuf[b % RING, rb, r16(lb), :] = bb.astype(BF16)

    def d_inv_rows(b, lb, stats, first):
        u = [uout[b % RING, r, r16(lb), :] for r in range(8)]
        ys = yield from _d_butterfly_inv([gate(v) if r < 4 else v for r, v in enumerate(u)], pin, gate)
        xs = [x + y for x, y in zip(load_x(b, lb, first), ys)]
        for j in range(NT):
            put(xres.at[b, j, r16(lb), :], xs[j])
        stats[b, lb] = yield from ln_stats(xs)
        if b % 2:
            for j in range(4):
                a = [(xres[bb, j + o, r16(lb), :] - stats[bb, lb][0]) * stats[bb, lb][1]
                     for bb in (b - 1, b) for o in (0, 4)]
                a[0], a[3] = gate(a[0]), gate(a[3])
                for k, v in enumerate(_strassen_lhs(*a)):
                    if k in (1, 4):
                        pin(v)
                    abuf[b // 2, k, j, r16(lb), :] = v.astype(BF16)
                if j < 3:
                    yield

    def add_d_inv(sched, tick, b, gap, stats, first, cols=None):
        per_tick = 4
        cols = cols or [tick + ct * gap for ct in range(4)]
        for ct in range(4):
            sched.add(cols[ct], d_inv_cols(b, ct))
        tick = int(cols[3]) + XGAP + 1
        sched.add(tick, d_dots(b, 8, per_tick))
        tick += 8 // per_tick + 3
        for lb in range(4):
            sched.add(tick + lb * gap, d_inv_rows(b, lb, stats, first))
        return int(tick + 3 * gap) + 3 * XGAP + 1 + 4

    def gemm(lhs32, rhs32, jobs, sink):
        for slot, b, n in jobs:
            m = {}
            for k in (3, 1, 0, 6, 5, 4, 2):
                m[k] = ticking(_dot(lhs(*[lhs32[slot, k, j] for j in range(4)]), bf(rhs32[n // 2, k])))
                if k == 1:
                    sink(b + 1, n, m[1] - m[3])
                elif k == 0:
                    c11, c22 = m[3] - m[0], m[1] - m[0]
                elif k == 6:
                    c11 = m[6] - c11
                elif k == 5:
                    c22 = m[5] - c22
                elif k == 4:
                    sink(b, n, c11 - m[4])
                elif k == 2:
                    sink(b, n + 1, m[4] - m[2])
                    sink(b + 1, n + 1, c22 - m[2])
                yield

    def qkv_sink(b, n, o):
        c, t = divmod(b, 8)
        dst = (qbuf, kbuf, vbuf)[n // NT]
        for lb in range(4):
            put(dst.at[n % NT, t, pl.ds(8 + 64 * lb + 16 * c, 16), :], o[lb * 16:(lb + 1) * 16])
        if b == 0 and n >= NT:
            first = jnp.broadcast_to(o[0:1], (8, 128))
            for tt in range(8):
                dst[n % NT, tt, pl.ds(0, 8), :] = first

    def out_rows(r, i, last):
        c, t = divmod(r, 8)
        return (c * 8 + t % 2 * 4 + i, t // 2) if last and c == 0 else (r, i)

    def out_sink(last, r, n, o):
        for i in range(4):
            b, lb = out_rows(r, i, last)
            put(xres.at[b, n, r16(lb), :], xres[b, n, r16(lb), :] + o[i * 16:(i + 1) * 16])

    def attention(b, lb, h):
        c, t = divmod(b, 8)
        log2e = float(np.log2(np.e))
        scale = HEAD_DIM ** -0.5 * log2e
        r0 = 8 + 64 * lb + 16 * c + 8 * h
        src = [((t - 2 * w) % 8, -((t - 2 * w) // 8)) for w in range(WIN)]
        acc = [None] * WIN
        for j in range(NT):
            if j % 2 == 0:
                factor = gate(jnp.full((8, 128), scale, F32), ALAG)
            q = qbuf[j, t, pl.ds(r0, 8), :] * factor
            for w, (ts, sh) in enumerate(src):
                p = q * kbuf[j, ts, pl.ds(r0 - sh, 8), :]
                acc[w] = p if j == 0 else acc[w] + p
            if j % 2 and j < NT - 1:
                pin(*acc[j // 2 % 2::2])
                yield
        part = [(r, pltpu.roll(r, 64, 1)) for r in acc]
        yield from _latency()
        part = [r + rr for r, rr in part]
        part = [(r, pltpu.roll(r, 32, 1)) for r in part]
        yield from _latency()
        logits = [r + rr for r, rr in part]
        if r0 == 8:
            sub = lax.broadcasted_iota(jnp.int32, (8, 128), 0)
            logits = [jnp.where(sub >= sh, r, -1e9 * log2e) if sh else r
                      for r, (_, sh) in zip(logits, src)]
        logits[0] = gate(logits[0], ALAG)
        m = _tree(jnp.maximum, logits)
        ps = [jnp.exp2(r - m) for r in logits]
        total = _tree(_add, ps)
        pin(total)
        inv = pltpu.reciprocal(total, approx=True)
        inv = inv * (2.0 - total * inv)
        for j in range(NT):
            if j % 2 == 0:
                yield
                ps[0], ps[4] = gate(ps[0], ALAG), gate(ps[4], ALAG)
            o = _chain(_add, [ps[w] * vbuf[j, ts, pl.ds(r0 - sh, 8), :]
                              for w, (ts, sh) in enumerate(src)]) * inv
            if j % 2:
                pin(o)
            put(qbuf.at[j, t, pl.ds(r0, 8), :], o)

    def out_operands(r, i, last):
        for j in range(4):
            a = [qbuf[j + o, b % 8, pl.ds(8 + 64 * lb + 16 * (b // 8), 16), :]
                 for b, lb in (out_rows(r, i, last), out_rows(r + 1, i, last)) for o in (0, 4)]
            a[0], a[3] = gate(a[0]), gate(a[3])
            for k, v in enumerate(_strassen_lhs(*a)):
                if k in (1, 4):
                    pin(v)
                obuf[r // 2, k, j, r16(i), :] = v.astype(BF16)
            if j < 3:
                yield

    def store_rows(b, lb, tiles):
        c, t = divmod(b, 8)
        for j in tiles:
            words = pack(xres[b, j, r16(lb), :], xres[b + 1, j, r16(lb), :])
            pin(words)
            io32[j, lb, c, pl.ds(t // 2, 16, stride=4), :] = words

    unit_ticks = NT + 2 * XGAP
    step = 2
    out_ticks = 28

    def add_proj(sched, tick, c, lo, hi):
        jobs = [(b // step, b, n) for b in range(8 * c, 8 * c + 8, step) for n in range(lo, hi, step)]
        sched.add(tick, gemm(abuf32, wqkv32, jobs, qkv_sink))
        return tick + len(jobs) * out_ticks * step // NT

    def add_attention(sched, tick, pace, rows, last):
        units = [(r, i, half, h) for r in rows[::2] for i in range(4) for half in range(2) for h in range(2)]
        for n, (r, i, half, h) in enumerate(units):
            sched.add(tick + n * pace, attention(*out_rows(r + half, i, last), h))
            if half and h:
                sched.add(int(tick + n * pace) + unit_ticks, out_operands(r, i, last))

    def add_out(sched, tick, rows, last):
        jobs = [(r // 2, r, n) for r in rows[::2] for n in range(0, NT, 2)]
        sched.add(tick, gemm(obuf32, wo32, jobs, functools.partial(out_sink, last)))

    def add_tail(sched, tick, rows, last):
        ready = {}
        for i, r in enumerate(rows):
            t0 = tick + (i // 2 + 1) * out_ticks
            fast = i >= len(rows) - 2
            if not last:
                t0 += 0 if fast else TOFF + i % 2 * out_ticks // 2
                ready[r % 8] = add_d_fwd(sched, t0, r, i % 2 if fast else out_ticks / 8)
            elif r % 2:
                c, p = r // 8, r % 8 // 2
                if fast:
                    for at, tiles in ((t0 - out_ticks // 4 + 3, range(6)), (t0, range(6, NT))):
                        for j in range(4):
                            sched.add(at, _once(store_rows, 2 * j, p, tiles))
                        sched.add(at + 1, _once(start, out_copies(c, p, tiles)))
                    continue
                for j in range(4):
                    sched.add(t0 + 3 * j + 3, _once(store_rows, *((r - 1, j) if c else (2 * j, p)), range(NT)))
                for lb in ([p] if c == 0 else range(4) if p == 3 else []):
                    sched.add(t0 + 16, _once(start, out_copies(c, lb, range(NT))))
        return ready

    q_ticks = 8 * out_ticks // step
    att_ticks = unit_ticks + 1 + 2
    order = [(a + 8) % NB for a in range(NB)]

    def add_attention_block(sched, cols, last):
        stats = {}
        t0 = max([add_d_inv(sched, 0, b, 0, stats, not last, cols) for b in range(step)])
        if not last:
            sched.add(cols[3] - KLEAD, _once(wait, qkv_copies(1) + dmat_cp))
            done = add_prep_wqkv(sched, cols[3] - KLEAD, 1, KPACE, [7] * 4)
            t0 = max(t0, done[0])
            assert all(d <= t0 + p * out_ticks / 4 for p, d in enumerate(done))
            sched.add(t0 + out_ticks, _once(wait, qkv_copies(2)))
            sched.add(t0 + out_ticks, _once(start, qkv_copies(0)))
            done = add_prep_wqkv(sched, t0 + out_ticks, 2, 2 * out_ticks - 4, [out_ticks - 4] * 4)
            assert all(d <= t0 + q_ticks + p * out_ticks for p, d in enumerate(done))
            sched.add(t0 + 2 * q_ticks, _once(wait, qkv_copies(0)))
            sched.add(t0 + 2 * q_ticks, _once(start, wo_copies))
            done = add_prep_wqkv(sched, t0 + 2 * q_ticks, 0, q_ticks - 10, [q_ticks / 4] * 4)
            assert done[-1] <= t0 + 4 * q_ticks
            sched.add(t0 + 8 * q_ticks, _once(wait, wo_copies))
            for i in range(32):
                sched.add(t0 + 8 * q_ticks + i * q_ticks / 16, prep_wo(*divmod(i, 8)))
        tick, kv_start, q_start = t0, {}, {}
        for kind, c in ("k0", "k1", "q1", "k2", "q2", "k3", "q3", "q0"):
            if kind == "k":
                kv_start[int(c)] = tick
                if c == "0" and not last:
                    tick = add_proj(sched, tick, 0, NT, 2 * NT)
                    jobs = [(b // step, b, n) for n in range(2 * NT, 3 * NT, step) for b in range(0, 8, step)]
                    sched.add(tick, gemm(abuf32, wqkv32, jobs, qkv_sink))
                    tick += q_ticks
                    continue
                tick = add_proj(sched, tick, int(c), NT, 3 * NT)
            else:
                q_start[int(c)] = tick
                tick = add_proj(sched, tick, int(c), 0, NT)
        pace = 2 * out_ticks / step
        for b in range(step, NB):
            due = kv_start[b // 8] + (b % 8 // step) * (2 if last or b >= 8 else 1) * out_ticks
            gap = min(1 + (b - step) * 0.5, DGAP1 if last else DGAP0)
            pace = DPACE1 if last else DPACE0
            at = (b - step) * pace
            at = t0 + at + max(0, at - 4 * q_ticks - out_ticks) * DSLOW
            if not last and b < 8:
                at, gap = max(cols[3], t0 + (b // step - 1) * out_ticks - (step - b % step) * 8), 1
            end = add_d_inv(sched, at, b, gap, stats, not last)
            assert end <= due, (b, end, due)
        begin = [q_start[c] + out_ticks + 3 for c in (1, 2, 3)] + [tick + (ATT1 if last else ATT0)]
        begin.append(tick + (NB // step - 1) * out_ticks - att_ticks)
        for i, c in enumerate((1, 2, 3, 0)):
            pace = (begin[i + 1] - begin[i]) / 64
            assert begin[i] >= max(kv_start[c], kv_start[(c - 1) % 4]) + 2 * q_ticks
            for p in range(4):
                assert begin[i] + 16 * p * pace >= q_start[c] + (4 if last and c == 0 else p + 1) * out_ticks
                assert begin[i] + (16 * p + 15) * pace + att_ticks <= tick + (4 * i + p) * out_ticks + 1e-6
            add_attention(sched, begin[i], pace, range(8 * c, 8 * c + 8), last)
        add_out(sched, tick, order, last)
        return tick + (NB // step) * out_ticks, add_tail(sched, tick, order, last)

    def add_input(sched):
        ready = {}
        after = (x_copies(2), x_copies(3) + perm_cp + w_copies(0) + w_copies(1),
                 w_copies(2) + w_copies(3), w_copies(4))
        for c in range(NC):
            sched.add(c * 32, _once(wait, x_copies(c)))
            sched.add(c * 32, _once(start, after[c]))
            for t in range(8):
                ready[t] = add_d_fwd(sched, c * 32 + t * 4, c * 8 + t, 1, 2, True)
        return 128 + 9, ready

    def add_filter_prep(sched, upper, begin, end):
        after = (([], qkv_copies(2)) if upper else
                 (w_copies(5) + w_copies(6), w_copies(7) + f256_cp + dmat_cp))
        for i in range(16):
            g, at = 4 * upper + i // 4, begin + i * (end - begin) / 16
            if i % 8 == 0:
                sched.add(at, _once(wait, w_copies(g) + w_copies(g + 1) + {0: perm_cp, 6: f256_cp}.get(g, [])))
                sched.add(at, _once(start, after[i // 8]))
            sched.add(at, _once(prep_filter, *w_tiles(g)[i % 4]))
        return end + 2

    def add_first_s_stage(sched):
        tick, ready = add_input(sched)
        sched.add(tick + WK0, _once(start, qkv_copies(1)))
        return add_s_stage(sched, tick, ready, add_filter_prep(sched, 0, F0, tick),
                           lambda begin, end: add_filter_prep(sched, 1, begin, end + FG))

    sched = _Schedule()

    start(x_copies(0) + tiny_cp)
    for ref in (abuf32, obuf32, ubuf32, wo32, sfw32, siv32, wide32):
        put(ref.at[(0,) * (len(ref.shape) - 2) + (pl.ds(0, 8),)], jnp.zeros((8, 128), U32))
    make_wide()
    start(x_copies(1))
    for t in range(8):
        make_s_fwd(t)
    for e in range(4):
        make_s_inv(e)
    wait(tiny_cp)
    for n in (1, 2, 4):
        never[n] = jnp.concatenate([tw_ref[16:24, 0:128]] * n, axis=1) != 0.0
    cols = add_first_s_stage(sched)
    tick, ready = add_attention_block(sched, cols, False)
    cols = add_s_stage(sched, tick, ready, tick, None)
    add_attention_block(sched, cols, True)
    sched.run()
    for c in range(NC):
        for lb in range(4):
            wait(out_copies(c, lb, range(NT)))


@jax.jit
def pallas_interleave_layers__spectral_gfnet__sliding_local_dilated__prompt_kernel(
    A_x: jax.Array,
    A_w_r: jax.Array,
    A_w_i: jax.Array,
    B_x: jax.Array,
    B_wqkv: jax.Array,
    B_wo: jax.Array,
):
    del B_x
    assert A_x.shape == (1, S, D) and A_w_r.shape == (S, D // 2 + 1)
    cst = _constants()
    x = A_x.astype(BF16).reshape(4, NC, 128, D)
    wr, wi = A_w_r.astype(BF16).T, A_w_i.astype(BF16).T
    hbm = pl.BlockSpec(memory_space=pl.ANY)
    vm = pltpu.VMEM
    out = pl.pallas_call(
        _kernel,
        in_specs=[hbm] * 9,
        out_specs=hbm,
        out_shape=jax.ShapeDtypeStruct((4, NC, 128, D), BF16),
        scratch_shapes=[
            vm((NT, 4, NC, 128, 128), BF16),
            vm((17, 128, 128), BF16),
            vm((32, 128, 128), BF16),
            vm((32, 128, 128), BF16),
            vm((256, 512), BF16),
            vm((2, 16, 512, 128), BF16),
            vm((2, 4, 4, 8, 64, 128), F32),
            vm((3 * NT, D, 128), BF16),
            vm((NT, D // 2, 128), U32),
            vm((12, 7, 512, 128), BF16),
            vm((NT, D, 128), BF16),
            vm((4, 7, 512, 128), BF16),
            vm((NB, NT, 64, 128), F32),
            vm((4, 32, 64, 128), U32),
            vm((4, 32, 128, 128), F32),
            vm((RING, 8, 64, 128), BF16),
            vm((RING, 9, 64, 128), F32),
            vm((NB // 2, 7, 4, 64, 128), BF16),
            vm((NB // 2, 7, 4, 64, 128), BF16),
            vm((NT, 8, 264, 128), F32),
            vm((NT, 8, 264, 128), F32),
            vm((NT, 8, 264, 128), F32),
            vm((3, 256, 128), F32),
            vm((8, 256, 128), BF16),
            vm((24, 256), F32),
            vm((2, 16, 128), BF16),
            vm((1, S), BF16),
            vm((1, S), BF16),
            pltpu.SemaphoreType.DMA((NC,)),
            pltpu.SemaphoreType.DMA((4,)),
            pltpu.SemaphoreType.DMA((8,)),
            pltpu.SemaphoreType.DMA((3,)),
            pltpu.SemaphoreType.DMA(()),
            pltpu.SemaphoreType.DMA(()),
        ],
        compiler_params=pltpu.CompilerParams(
            vmem_limit_bytes=120 * 2**20),
    )(x, wr, wi, B_wqkv.astype(BF16), B_wo.astype(BF16),
      cst["small"], cst["f256"], cst["tw"], cst["d8"])
    return out.reshape(1, S, D)
```

```python
import functools

import jax
import jax.numpy as jnp
import numpy as np
from jax import lax
from jax.experimental import pallas as pl
from jax.experimental.pallas import tpu as pltpu

S, D = 2048, 1024
NT = D // 128
NC = 4
WIN = 8
HEAD_DIM = 32
EPS = 1e-5
F32, BF16, U32 = jnp.float32, jnp.bfloat16, jnp.uint32
PAIRS = ((0, 4), (1, 7), (2, 6), (3, 5))
RSQ2 = float(np.sqrt(0.5))
NB = S // 64

RING = 8
XGAP = 3
GLAG = 4
ALAG = 4
SGLAG = 3
S_LAG = 2
F0 = 120
KLEAD = 46
KPACE = 40
DGAP0 = 4.75
DGAP1 = 4.2
DPACE0 = 20
DPACE1 = 15.5
DSLOW = 0.6
SYNC = 3
ILAG = 3
FG = 10
TOFF = 2
WK0 = 24
ATT0 = 15
ATT1 = 95


def _residues(r):
    return (0, 8) if r == 0 else (r, 16 - r)


def _d_matrices():
    n = np.arange(64)[:, None]
    a = np.arange(32)
    fwd = np.zeros((8, 128, 128))
    inv = np.zeros((8, 128, 128))
    for r in range(8):
        kd = np.concatenate([16 * a + p for p in _residues(r)])
        weight = np.full(64, 2.0)
        if r == 0:
            kd[0], weight[0] = D // 2, 1.0
            ph = np.exp(-2j * np.pi * n * kd[None, :] / D)
            sgn = np.where(kd % 16 == 0, 1.0, -1.0)[None, :]
            m = np.concatenate([ph, ph * sgn], axis=0)
            re, im = m.real.copy(), m.imag.copy()
            ire, iim = re.copy(), im.copy()
            im[:, 0] = 1.0
            iim[:, 0] = 1.0
        else:
            p = 12 if r == 4 else r
            ph = np.exp(-2j * np.pi * n * kd[None, :] / D)
            si = np.where(kd % 16 == p, 1.0, -1.0)[None, :]
            m = np.concatenate([ph, 1j * si * ph], axis=0)
            re, im = m.real, m.imag
            ire, iim = re, im
        swapped = r in (4, 7, 6, 5)
        cols = [im, re] if swapped else [re, im]
        icols = [iim * weight, ire * weight] if swapped else [ire * weight, iim * weight]
        fwd[r] = np.concatenate(cols, axis=1)
        inv[r] = np.concatenate(icols, axis=1).T / D
    return fwd, inv


def _side_matrices():
    l = np.arange(256)
    f = np.exp(-2j * np.pi * ((l[:, None] * l[None, :]) % 256) / 256)
    f256 = np.concatenate([f.real, f.imag], axis=1)
    t = np.arange(8)
    tw = np.exp(-2j * np.pi * t[:, None] * l[None, :] / S)
    tw = np.concatenate([tw.real, tw.imag, np.zeros((8, 256))], axis=0)
    g = np.exp(-2j * np.pi * t[:, None] * t[None, :] / 8)
    d8 = np.zeros((2, 16, 128))
    d8[0, :, :16] = np.block([[g.real, -g.imag], [g.imag, g.real]])
    d8[1, :, :16] = d8[0, :, :16].T / S
    return f256, tw, d8


def _filter_rows():
    p = np.zeros((1, 128, 128))
    for k in range(32):
        for e in range(4):
            p[0, e * 32 + k, 4 * k + e] = 1.0
    return p


@functools.lru_cache(maxsize=None)
def _constants():
    dfw, div = _d_matrices()
    f256, tw, d8 = _side_matrices()
    small = np.concatenate([dfw, div, _filter_rows()], axis=0)
    b = lambda x: np.asarray(x, np.float32).astype(BF16)
    return dict(small=b(small), f256=b(f256),
                tw=np.asarray(tw, np.float32), d8=b(d8))


def _dot(a, b):
    return jnp.dot(a, b, preferred_element_type=F32)


def _dot_nt(a, b):
    return lax.dot_general(a, b, (((1,), (1,)), ((), ())), preferred_element_type=F32)


def _tree(op, xs):
    xs = list(xs)
    while len(xs) > 1:
        xs = [op(xs[i], xs[i + 1]) if i + 1 < len(xs) else xs[i] for i in range(0, len(xs), 2)]
    return xs[0]


def _chain(op, xs):
    return functools.reduce(op, xs)


def _lane(rows):
    return lax.broadcasted_iota(jnp.int32, (rows, 128), 1)


def _swap(x):
    return pltpu.roll(x, 64, 1)


def _unpack(w, i):
    return pltpu.unpack_elementwise(w, index=i, packed_dtype=BF16, unpacked_dtype=F32)


def _latency():
    for _ in range(XGAP):
        yield


def _add(a, b):
    return a + b


def _row_mean(xs):
    return jnp.sum(_tree(_add, xs), axis=1, keepdims=True) * (1.0 / D)


def _twiddle16(r, x, y):
    lo = _lane(x.shape[0]) < 64
    wr, wi = float(np.cos(np.pi * r / 8)), float(-np.sin(np.pi * r / 8))
    cross = jnp.where(lo, 0.0, wr)
    return x * jnp.where(lo, 1.0, wi) + y * cross, y * jnp.where(lo, 1.0, -wi) + x * cross


def _d_butterfly_fwd(a, emit, pin, wide):
    s = [a[j] + a[j + 4] for j in range(4)]
    e, o = s[0] + s[2], s[1] + s[3]
    total, t4 = e + o, e - o
    emit(4, t4)
    d0, nd2 = a[0] - a[4], a[6] - a[2]
    d1, d3 = a[1] - a[5], a[3] - a[7]
    p, q = (d1 - d3) * RSQ2, (d1 + d3) * -RSQ2
    ts = {1: (d0 + p, q + nd2), 2: (s[0] - s[2], s[3] - s[1]), 3: (d0 - p, q - nd2)}
    mean8 = jnp.sum(total, axis=1, keepdims=True) * (1.0 / 128)
    if wide:
        for r, (tr, ti) in ts.items():
            emit(r, tr)
            emit(8 - r, ti)
    else:
        ab = {r: _twiddle16(r, *t) for r, t in ts.items()}
        ab = {r: (a, _swap(b)) for r, (a, b) in ab.items()}
    dev = _tree(_add, [v * v for t in ts.values() for v in t]) * 2.0 + t4 * t4
    pin(dev)
    yield from _latency()
    t0 = total - mean8
    emit(0, t0)
    var = jnp.sum(dev + t0 * t0, axis=1, keepdims=True) * (1.0 / (NT * D))
    if not wide:
        for r, (x, y) in ab.items():
            emit(r, x + y)
            emit(8 - r, x - y)
    yield from _latency()
    return lax.rsqrt(var + EPS)


def _d_butterfly_inv(u, pin, gate):
    ab = {r: (u[r] + u[8 - r], _swap(u[r] - u[8 - r])) for r in (1, 2, 3)}
    e, o = u[0] + u[4], u[0] - u[4]
    yield from _latency()
    ts = {r: _twiddle16(r, x, gate(y)) for r, (x, y) in ab.items()}
    pin(*[t[0] for t in ts.values()])
    yield
    s = [e + ts[2][0], o - ts[2][1], e - ts[2][0], o + ts[2][1]]
    p = (ts[1][0] - ts[3][0]) * RSQ2
    q = (ts[1][1] + ts[3][1]) * RSQ2
    d0, d1, d2, nd3 = ts[1][0] + ts[3][0], p - q, ts[3][1] - ts[1][1], p + q
    return [s[0] + d0, s[1] + d1, s[2] + d2, s[3] - nd3,
            s[0] - d0, s[1] - d1, s[2] - d2, s[3] + nd3]


def _strassen_lhs(a11, a12, a21, a22):
    return [a11 + a22, a21 + a22, a11, a22, a11 + a12, a21 - a11, a12 - a22]


def _strassen_rhs(b11, b12, b21, b22):
    return [b11 + b22, b11, b22 - b12, b11 - b21, b22, b11 + b12, b21 + b22]


def _cadd(a, b):
    return a[0] + b[0], a[1] + b[1]


def _csub(a, b):
    return a[0] - b[0], a[1] - b[1]


def _dft4(z, inverse):
    a, b = _cadd(z[0], z[2]), _csub(z[0], z[2])
    c, d = _cadd(z[1], z[3]), _csub(z[1], z[3])
    minus = (b[0] + d[1], b[1] - d[0])
    plus = (b[0] - d[1], b[1] + d[0])
    return [_cadd(a, c), plus if inverse else minus, _csub(a, c), minus if inverse else plus]


def _dft8(z, inverse):
    ev = _dft4(z[0::2], inverse)
    od = _dft4(z[1::2], inverse)
    out = [None] * 8
    out[0], out[4] = _cadd(ev[0], od[0]), _csub(ev[0], od[0])
    (er, ei), (x, y) = ev[2], od[2]
    minus, plus = (er + y, ei - x), (er - y, ei + x)
    out[2], out[6] = (plus, minus) if inverse else (minus, plus)
    for k in (1, 3):
        (er, ei), (x, y) = ev[k], od[k]
        sm, df = (x + y) * RSQ2, (x - y) * RSQ2
        if not inverse:
            if k == 1:
                out[1], out[5] = (er + sm, ei - df), (er - sm, ei + df)
            else:
                out[3], out[7] = (er - df, ei - sm), (er + df, ei + sm)
        else:
            if k == 1:
                out[1], out[5] = (er + df, ei + sm), (er - df, ei - sm)
            else:
                out[3], out[7] = (er - sm, ei + df), (er + sm, ei - df)
    return out


class _Schedule:
    def __init__(self):
        self.pending = []

    def add(self, tick, gen):
        self.pending.append((int(tick), len(self.pending), gen))

    def run(self):
        pending = sorted(self.pending, key=lambda p: p[:2])
        active, tick, i = [], 0, 0
        while active or i < len(pending):
            while i < len(pending) and pending[i][0] <= tick:
                active.append(pending[i][2])
                i += 1
            for g in list(active):
                if next(g, 0) == 0:
                    active.remove(g)
            tick += 1
        self.pending = []


def _once(fn, *args):
    fn(*args)
    return
    yield


def _kernel(x_hbm, wr_hbm, wi_hbm, wqkv_hbm, wo_hbm, small_hbm, f256_hbm, tw_hbm, d8_hbm,
            out_hbm,
            io, small, sfw, siv, f256, wraw, wf, wqkv_raw, wtmp, wqkv, wo_raw, wo,
            xres, zin, zout, ubuf, uout, abuf, obuf, qbuf, kbuf, vbuf, side,
            wide, tw_ref, d8_ref, wr_edge, wi_edge, sem_x, sem_c, sem_w, sem_qkv, sem_wo, sem_out):

    def x_copies(c):
        return [pltpu.make_async_copy(x_hbm.at[:, c, :, pl.ds(j * 128, 128)], io.at[j, :, c],
                                      sem_x.at[c]) for j in range(NT)]

    def out_copies(c, lb, tiles):
        return [pltpu.make_async_copy(io.at[j, lb, c], out_hbm.at[lb, c, :, pl.ds(j * 128, 128)],
                                      sem_out) for j in tiles]

    perm_cp, dmat_cp, f256_cp = ([pltpu.make_async_copy(s, d, sem_c.at[i])] for i, (s, d) in enumerate((
        (small_hbm.at[pl.ds(16, 1)], small.at[pl.ds(16, 1)]),
        (small_hbm.at[pl.ds(0, 16)], small.at[pl.ds(0, 16)]), (f256_hbm, f256))))

    tiny_cp = [pltpu.make_async_copy(s, d, sem_c.at[3]) for s, d in (
        (tw_hbm, tw_ref), (d8_hbm, d8_ref),
        (wr_hbm.at[pl.ds(D // 2, 1)], wr_edge), (wi_hbm.at[pl.ds(D // 2, 1)], wi_edge))]

    def w_tiles(g):
        return [(g // 2 % 2, 8 * (g % 2) + 2 * i + g // 4) for i in range(4)]

    def w_copies(g):
        return [pltpu.make_async_copy((wr_hbm, wi_hbm)[ri].at[pl.ds(0, 512), pl.ds(m * 128, 128)],
                                      wraw.at[ri, m], sem_w.at[g]) for ri, m in w_tiles(g)]

    def qkv_copies(g):
        return [pltpu.make_async_copy(wqkv_hbm.at[:, pl.ds(g * D + j * 128, 128)],
                                      wqkv_raw.at[g * NT + j], sem_qkv.at[g]) for j in range(NT)]

    wo_copies = [pltpu.make_async_copy(wo_hbm.at[:, pl.ds(j * 128, 128)], wo_raw.at[j], sem_wo)
                 for j in range(NT)]

    def start(cs):
        for cp in cs:
            cp.start()

    def wait(cs):
        for cp in cs:
            cp.wait()

    io32, wraw32, wo_raw32 = io.bitcast(U32), wraw.bitcast(U32), wo_raw.bitcast(U32)
    small32, sfw32, siv32, wide32 = (r.bitcast(U32) for r in (small, sfw, siv, wide))
    wqkv_raw32, wqkv32, wo32 = (r.bitcast(U32) for r in (wqkv_raw, wqkv, wo))
    ubuf32, abuf32, obuf32 = ubuf.bitcast(U32), abuf.bitcast(U32), obuf.bitcast(U32)

    never = {}
    token = {}

    def pin(*values):
        for v in values:
            key = v.shape[0], v.dtype == F32
            token[key] = (lax.max if key[1] else lax.bitwise_xor)(token[key], v) if key in token else v

    clock = []

    def gate(v, lag=GLAG):
        if len(clock) < lag:
            return v
        old = clock[-lag] if v.dtype == F32 else pltpu.bitcast(clock[-lag], v.dtype)
        if v.shape[0] == 8:
            return lax.select(never[1], old, v)
        return lax.concatenate([lax.select(never[1], old, v[0:8]), v[8:]], 0)

    def ticking(o):
        clock.append(o[0:8])
        del clock[:-16]
        return o

    def lhs(*tiles):
        if not token and len(tiles) == 4 and len(clock) >= SYNC:
            pin(clock[-SYNC])
        words = lax.concatenate(tiles, 1) if len(tiles) > 1 else tiles[0]
        if token:
            parts = [pltpu.bitcast(v, U32) if is_float else v for (_, is_float), v in token.items()]
            token.clear()
            w = _chain(lax.bitwise_xor, [v[i:i + 8] if v.shape[0] > 8 else v
                                         for v in parts for i in range(0, v.shape[0], 8)])
            w = lax.concatenate([w] * len(tiles), 1) if len(tiles) > 1 else w
            words = lax.concatenate([lax.select(never[len(tiles)], w, words[0:8]), words[8:]], 0)
        return pltpu.bitcast(words, BF16)

    def bf(words):
        return pltpu.bitcast(words, BF16)

    def pack(a, b):
        return pltpu.bitcast(pltpu.pack_elementwise([a, b], packed_dtype=BF16), U32)

    def r16(i):
        return pl.ds(i * 16, 16)

    always = {}

    def put(ref, v):
        if v.shape not in always:
            always[v.shape] = jnp.ones(v.shape, jnp.bool_)
        pltpu.store(ref, v, mask=always[v.shape])

    def load_x(b, lb, from_input):
        if from_input:
            c, t = divmod(b, 8)
            return [_unpack(io32[j, lb, c, pl.ds(t // 2, 16, stride=4), :], t % 2) for j in range(NT)]
        return [xres[b, j, r16(lb), :] for j in range(NT)]

    def unit(p):
        angle = (((p + S // 2) & (S - 1)) - S // 2).astype(F32) * (2 * np.pi / S)
        return jnp.cos(angle), jnp.sin(angle)

    def times(a, b):
        return a[0] * b[0] - a[1] * b[1], a[0] * b[1] + a[1] * b[0]

    def times_row(a, b, i):
        return times(a, [jnp.broadcast_to(v[i:i + 1], (8, 128)) for v in b])

    def make_wide():
        row, lane = lax.broadcasted_iota(jnp.int32, (8, 128), 0), _lane(8)
        for ct, (ra, rb) in enumerate(PAIRS):
            res = _residues(ra) + _residues(rb)
            kd = (lane & 31) * 16 + _chain(
                _add, [jnp.where(lane >> 5 == g, p, 0) for g, p in enumerate(res)])
            if ct == 0:
                kd = jnp.where(lane == 0, D // 2, kd)
            fine, coarse = unit(-2 * row * kd), [unit(-16 * (row + 8 * h) * kd) for h in range(2)]
            for a in range(16):
                re, im = times_row(fine, coarse[a // 8], a % 8)
                if ct == 0:
                    even = kd & 7 == 0
                    top = jnp.where(even, re, 0.0), jnp.where(lane == 0, 1.0, jnp.where(even, im, 0.0))
                    bottom = jnp.where(even, 0.0, re), jnp.where(even, 0.0, im)
                else:
                    sign = jnp.where(kd & 7 == ra, 1.0, -1.0)
                    top, bottom = (re, im), (-sign * im, sign * re)
                for i in range(2):
                    wide[2 * ct + i, pl.ds(8 * a, 8), :] = top[i].astype(BF16)
                    wide[2 * ct + i, pl.ds(128 + 8 * a, 8), :] = bottom[i].astype(BF16)

    def make_s_fwd():
        row, lane = lax.broadcasted_iota(jnp.int32, (8, 128), 0), _lane(8)
        pos = 8 * (lane >> 1)
        parts = [unit((lane & 1) * (S // 4) - 4 * row * pos), unit(-row * pos), unit(-32 * row * pos)]
        steps = [unit(-4 * row), unit(-row), unit(-32 * row)]
        for t in range(8):
            fine, shift, coarse = parts
            for e in range(4):
                base = times_row(fine, shift, e)
                for g in range(8):
                    for i, v in enumerate(times_row(base, coarse, g)):
                        sfw[t * 4 + e, pl.ds(16 * g + 8 * i, 8), :] = v.astype(BF16)
            parts = [times(a, b) for a, b in zip(parts, steps)]

    def make_s_inv():
        row, lane = lax.broadcasted_iota(jnp.int32, (8, 128), 0), _lane(8)
        freq = 4 * (lane >> 1)
        parts = [[v * (1.0 / S) for v in unit((lane & 1) * (S // 4) + 8 * row * freq)],
                 unit(row * freq), unit(64 * row * freq)]
        steps = [unit(8 * row), unit(row), unit(64 * row)]
        for e in range(4):
            fine, shift, coarse = parts
            for t in range(8):
                base = times_row(fine, shift, t)
                for g in range(8):
                    for i, v in enumerate(times_row(base, coarse, g)):
                        siv[t * 4 + e, pl.ds(64 * i + 8 * g, 8), :] = v.astype(BF16)
            parts = [times(a, b) for a, b in zip(parts, steps)]

    def prep_filter(ri, m):
        sub = lax.broadcasted_iota(jnp.int32, (8, 128), 0)
        edge = (wr_edge, wi_edge)[ri]
        res = {}
        for i in range(8):
            words = wraw32[ri, m, pl.ds(i, 32, stride=8), :]
            res[2 * i], res[2 * i + 1] = _unpack(words, 0), _unpack(words, 1)
        first = res[0][0:8]
        dst = pl.ds((m % 2) * 16 + ri * 8, 8)
        prev = jnp.zeros((8, 128), F32) if m < 2 else side[1, dst, :]
        put(side.at[1, dst, :], jnp.where(sub == m // 2, jnp.broadcast_to(first[0:1], (8, 128)), prev))
        nyq = jnp.broadcast_to(edge[0:1, pl.ds(m * 128, 128)].astype(F32), (8, 128))
        res[0] = jnp.concatenate([jnp.where(sub == 0, nyq, first), res[0][8:]], axis=0)
        for ct, (ra, rb) in enumerate(PAIRS):
            blk = jnp.concatenate([res[p] for p in _residues(ra) + _residues(rb)], axis=0)
            o = _dot_nt(lhs(small32[16]), blk.astype(BF16))
            for e in range(4):
                put(wf.at[ri, ct, e, m // 2, pl.ds((m % 2) * 32, 32), :], o[e * 32:(e + 1) * 32])

    def prep_wqkv_cross(g, r):
        pos = (_lane(8) >> 2) & 7
        u = [wqkv_raw32[g * NT + (-j) % 8, pl.ds(r * 8, 8), :] for j in range(NT)]
        u[0], u[4] = gate(u[0]), gate(u[4])
        for bit in range(3):
            m = ((pos >> bit) & 1) == 1
            u = [lax.select(m, u[(j - (1 << bit)) % 8], u[j]) for j in range(NT)]
        for j in range(NT):
            if j < 4:
                pin(u[j])
            put(wtmp.at[j, pl.ds(r * 8, 8), :], u[j])

    def prep_wqkv_pair(g, p, part):
        lane = _lane(8)
        ws = {}
        for n in range(2):
            index = (lane & 3) * 32 + (((lane >> 2) + 2 * p + n) & 7) * 4 + (lane >> 5)
            for half in range(2):
                for r in range(part * 2, part * 2 + 2):
                    w = gate(wtmp[2 * p + n, pl.ds(half * 256 + r * 8, 8), :])
                    ws[r, half, n] = jnp.take_along_axis(w, index, axis=1)
        yield from _latency()
        for r in range(part * 2, part * 2 + 2):
            quad = [ws[r, half, n] for half in range(2) for n in range(2)]
            ops = [_strassen_rhs(*[_unpack(w, i) for w in quad]) for i in range(2)]
            for k in range(7):
                word = {1: quad[0], 4: quad[3]}.get(k)
                if word is None:
                    word = pack(ops[0][k], ops[1][k])
                if k in (2, 3):
                    pin(word)
                put(wqkv32.at[g * 4 + p, k, pl.ds(r * 8, 8), :], word)

    def add_prep_wqkv(sched, tick, g, ticks, pair_ticks):
        for r in range(64):
            sched.add(tick + r * ticks / 64, _once(prep_wqkv_cross, g, r))
        tick = int(tick + ticks) + 1
        done = []
        for p, n in enumerate(pair_ticks):
            for i in range(16):
                sched.add(tick + i * n / 16, prep_wqkv_pair(g, p, i))
            tick += n
            done.append(int(tick) + XGAP + 1)
        return done

    def prep_wo(p, part):
        v, pair = divmod(part, 2)
        upper = lax.broadcasted_iota(jnp.int32, (8, 128), 0) >= 4
        ws = [[wo_raw32[2 * p + n, pl.ds(128 * v + 2 * f + pair, 8, stride=16), :] for f in range(8)]
              for n in range(2)]
        for o in range(4):
            quad = [lax.select(upper, w[(2 * v + 1 + j) % 8], w[(2 * v + j) % 8])
                    for j in (o, o + 4) for w in ws]
            quad[0] = gate(quad[0])
            for i in range(2):
                for k, x in enumerate(_strassen_rhs(*[_unpack(w, i) for w in quad])):
                    if k in (2, 3):
                        pin(x)
                    wo[p, k, pl.ds(o * 128 + (2 * pair + i) * 32 + 8 * v, 8), :] = x.astype(BF16)
            if o < 3:
                yield

    def ln_stats(xs):
        lane_mean = _tree(_add, xs) * (1.0 / NT)
        lane_m2 = _tree(_add, [jnp.square(x - lane_mean) for x in xs])
        pin(lane_m2)
        mean = jnp.sum(lane_mean, axis=1, keepdims=True) * (1.0 / 128)
        yield from _latency()
        m2 = lane_m2 + jnp.square(gate(lane_mean) - mean) * float(NT)
        pin(m2)
        var = jnp.sum(m2, axis=1, keepdims=True) * (1.0 / D)
        yield from _latency()
        return mean, lax.rsqrt(gate(jnp.broadcast_to(var, (16, 128))) + EPS)

    def d_fwd_rows(b, lb, from_input=False):
        xs = load_x(b, lb, from_input)

        def emit(r, v):
            if r % 4 == 0 or (r < 4 and not from_input):
                pin(v)
            ubuf[b % RING, r, r16(lb), :] = v.astype(BF16)

        xs[:4] = [gate(x, ILAG if from_input else GLAG) for x in xs[:4]]
        inv = yield from _d_butterfly_fwd(xs, emit, pin, from_input)
        inv = jnp.broadcast_to(inv, (16, 128))
        pin(inv)
        put(uout.at[b % RING, 8, r16(lb), :], inv)

    def d_dots(b, base, per_tick):
        for r in range(8):
            o = _dot(lhs(ubuf32[b % RING, r]), bf(small32[base + r]))
            put(uout.at[b % RING, r], o)
            if r % per_tick == per_tick - 1 and r < 7:
                yield

    def d_dots_wide(b):
        for ct, (ra, rb) in enumerate(PAIRS):
            u = lhs(ubuf32[b % RING, ra], ubuf32[b % RING, rb])
            for i, r in enumerate((ra, rb)):
                o = _dot(u, bf(wide32[2 * ct + i]))
                put(uout.at[b % RING, r], ticking(o) if i else o)
            if ct < 3:
                yield

    def d_fwd_cols(b, ct, is_wide):
        c, t = divmod(b, 8)
        ra, rb = PAIRS[ct]
        lane = _lane(16)
        lo = lane < 64
        z, x0 = [], []
        for lb in range(4):
            a, bb, inv = (uout[b % RING, r, r16(lb), :] for r in (ra, rb, 8))
            inv = gate(inv, ILAG if is_wide else GLAG)
            a, bb = a * inv, bb * inv
            if is_wide:
                if ct == 0:
                    x0.append(pltpu.roll(bb, t, 1) if t else bb)
                    bb = jnp.where(lane == 0, 0.0, bb)
                z.append((a, bb))
                continue
            if ct == 0:
                x0.append(pltpu.roll(a, (t + 64) % 128, 1))
                a = jnp.where(lane == 64, 0.0, a)
            im = lax.select(lo, bb, a)
            z.append((lax.select(lo, a, bb), _swap(im)))
        if not is_wide:
            yield from _latency()
        for e, (re, im) in enumerate(_dft4(z, False)):
            words = pack(re, im)
            if e < 2:
                pin(words)
            put(zin.at[ct, t * 4 + e, r16(c), :], words)
        if is_wide and ct == 0:
            yield from _latency()
        for lb, v in enumerate(x0):
            ls = pl.ds(64 * lb + 16 * c, 16)
            prev = jnp.zeros((16, 128), F32) if t == 0 else side[0, ls, :]
            v = jnp.where(lane == t, v, prev)
            pin(v)
            put(side.at[0, ls, :], v)

    def add_d_fwd(sched, tick, b, gap, per_tick=4, from_input=False):
        for lb in range(4):
            sched.add(tick + lb * gap, d_fwd_rows(b, lb, from_input))
        tick = int(tick + 3 * gap) + XGAP + 1
        sched.add(tick, d_dots_wide(b) if from_input else d_dots(b, 0, per_tick))
        for ct in range(4):
            sched.add(tick + 8 // per_tick + 3 + ct * gap, d_fwd_cols(b, ct, from_input))
        return int(tick + 8 // per_tick + 3 + 3 * gap) + XGAP + 1

    def side_path():
        vt = side[0].T[0:8]
        yield
        zero8 = jnp.zeros((8, 256), F32)
        u = _dot(jnp.concatenate([vt, zero8], axis=0).astype(BF16), f256[...])[0:8]
        twr, twi = tw_ref[0:8, :], tw_ref[8:16, :]
        ur, ui = u[:, 0:256], u[:, 256:512]
        pad = jnp.zeros((112, 256), BF16)
        for _ in range(4):
            yield
        uu = jnp.concatenate([ur * twr - ui * twi, ur * twi + ui * twr], axis=0).astype(BF16)
        xk = _dot(d8_ref[0], jnp.concatenate([uu, pad], axis=0))
        for _ in range(4):
            yield
        wr = jnp.concatenate([side[1, 0:8, :], side[1, 16:24, :]], axis=1)
        wi = jnp.concatenate([side[1, 8:16, :], side[1, 24:32, :]], axis=1)
        xr, xi = xk[0:8], xk[8:16]
        yy = jnp.concatenate([xr * wr - xi * wi, xr * wi + xi * wr], axis=0).astype(BF16)
        p = _dot(d8_ref[1], jnp.concatenate([yy, pad], axis=0))
        for _ in range(4):
            yield
        twr, twi = tw_ref[0:8, :], tw_ref[8:16, :]
        pr, pi = p[0:8], p[8:16]
        g = jnp.concatenate([pr * twr + pi * twi, pi * twr - pr * twi], axis=1)
        g = jnp.concatenate([g, jnp.zeros((8, 512), F32)], axis=0).astype(BF16)
        y0 = _dot_nt(g, f256[...])
        for _ in range(4):
            yield
        put(side.at[2], jnp.concatenate([y0, jnp.zeros((112, 256), F32)], axis=0).T)

    def s_fwd(u, t, timed):
        ct, e = divmod(u, 4)
        o = _dot(lhs(sfw32[t * 4 + e]), bf(zin[ct, t * 4 + e]))
        put(zout.at[ct, t * 4 + e], ticking(o) if timed else o)

    def s_filter(u, g, lag=SGLAG):
        ct, e = divmod(u, 4)
        z = [tuple(zout[ct, t * 4 + e, pl.ds(g * 16 + i, 8), :] for i in (0, 8)) for t in range(8)]
        z[0], z[1] = [tuple(gate(v, lag) for v in zz) for zz in z[0:2]]
        xk = _dft8(z, False)
        for k2 in range(8):
            wr = wf[0, ct, e, k2, pl.ds(g * 8, 8), :]
            wi = wf[1, ct, e, k2, pl.ds(g * 8, 8), :]
            re, im = xk[k2]
            xk[k2] = (re * wr - im * wi, re * wi + im * wr)
        for t, (re, im) in enumerate(_dft8(xk, True)):
            words = pack(re, im)
            if t < 4:
                pin(words)
            put(zin.at[ct, t * 4 + e, pl.ds(g * 8, 8), :], words)

    def s_inv(u, t, timed):
        ct, e = divmod(u, 4)
        o = _dot(lhs(siv32[t * 4 + e]), bf(zin[ct, t * 4 + e]))
        put(zout.at[ct, t * 4 + e], ticking(o) if timed else o)

    def add_s_stage(sched, early, ready, t1, pause):
        ahead = 4 + S_LAG
        tick = early
        for t in sorted(range(8), key=lambda t: ready[t]):
            for i in range(t, 2 * ahead, 8):
                tick = max(tick + 0.5, ready[t])
                sched.add(tick, _once(s_fwd, i // 8, t, pause is None or t % 2 == 0))
        t1 = max(t1, int(tick) + 1)
        if pause is None:
            sched.add(max(max(ready), t1), side_path())
            for i in range(128):
                if i + 2 * ahead < 128:
                    sched.add(t1 + i, _once(s_fwd, *divmod(i + 2 * ahead, 8), True))
                sched.add(t1 + i, _once(s_filter, *divmod(i, 8), SGLAG if i < 119 else SGLAG + 2))
                sched.add(t1 + 9 + (i if i < 120 else 120 + (i - 120) // 4),
                          _once(s_inv, *divmod(i, 8), i >= 118 - 2 * ahead))
            return [t1 + 32 * ct + 40 for ct in range(3)] + [t1 + 131]
        t2 = pause(t1 + 64 - ahead, t1 + 64)
        sched.add(max(max(ready), t2), side_path())
        for i in range(64):
            if i + ahead < 64:
                sched.add(t1 + i, _once(s_fwd, *divmod(2 * (i + ahead), 8), True))
            sched.add(t1 + i, _once(s_filter, *divmod(i, 4)))
            if i + ahead < 64:
                sched.add(t1 + i, _once(s_fwd, *divmod(2 * (i + ahead) + 1, 8), False))
        for i in range(69):
            if i >= 5:
                sched.add(t2 + min(i, 66), _once(s_inv, *divmod(2 * (i - 5), 8), True))
            if i < 64:
                sched.add(t2 + i, _once(s_filter, i // 4, 4 + i % 4))
            if i >= 5:
                sched.add(t2 + min(i, 66), _once(s_inv, *divmod(2 * (i - 5) + 1, 8), False))
        return [t2 + 16 * ct + 22 for ct in range(3)] + [t2 + 67]

    def d_inv_cols(b, ct):
        c, t = divmod(b, 8)
        ra, rb = PAIRS[ct]
        lane = _lane(16)
        lo = lane < 64
        u = [(zout[ct, t * 4 + e, r16(c), :], zout[ct, t * 4 + e, r16(4 + c), :]) for e in range(4)]
        u[0], u[1] = tuple(map(gate, u[0])), tuple(map(gate, u[1]))
        z = _dft4(u, True)
        z = [(re, _swap(im)) for re, im in z]
        if ct == 0:
            y0 = [pltpu.roll(side[2, pl.ds(64 * lb + 16 * c, 16), :], 64 - t, 1) for lb in range(4)]
        yield from _latency()
        for lb, (re, sw) in enumerate(z):
            sw = gate(sw)
            a, bb = lax.select(lo, re, sw), lax.select(lo, sw, re)
            if ct == 0:
                a = jnp.where(lane == 64, y0[lb], a)
            pin(a)
            ubuf[b % RING, ra, r16(lb), :] = a.astype(BF16)
            ubuf[b % RING, rb, r16(lb), :] = bb.astype(BF16)

    def d_inv_rows(b, lb, stats, first):
        u = [uout[b % RING, r, r16(lb), :] for r in range(8)]
        ys = yield from _d_butterfly_inv([gate(v) if r < 4 else v for r, v in enumerate(u)], pin, gate)
        xs = [x + y for x, y in zip(load_x(b, lb, first), ys)]
        for j in range(NT):
            put(xres.at[b, j, r16(lb), :], xs[j])
        stats[b, lb] = yield from ln_stats(xs)
        if b % 2:
            for j in range(4):
                a = [(xres[bb, j + o, r16(lb), :] - stats[bb, lb][0]) * stats[bb, lb][1]
                     for bb in (b - 1, b) for o in (0, 4)]
                a[0], a[3] = gate(a[0]), gate(a[3])
                for k, v in enumerate(_strassen_lhs(*a)):
                    if k in (1, 4):
                        pin(v)
                    abuf[b // 2, k, j, r16(lb), :] = v.astype(BF16)
                if j < 3:
                    yield

    def add_d_inv(sched, tick, b, gap, stats, first, cols=None):
        per_tick = 4
        cols = cols or [tick + ct * gap for ct in range(4)]
        for ct in range(4):
            sched.add(cols[ct], d_inv_cols(b, ct))
        tick = int(cols[3]) + XGAP + 1
        sched.add(tick, d_dots(b, 8, per_tick))
        tick += 8 // per_tick + 3
        for lb in range(4):
            sched.add(tick + lb * gap, d_inv_rows(b, lb, stats, first))
        return int(tick + 3 * gap) + 3 * XGAP + 1 + 4

    def gemm(lhs32, rhs32, jobs, sink):
        for slot, b, n in jobs:
            m = {}
            for k in (3, 1, 0, 6, 5, 4, 2):
                m[k] = ticking(_dot(lhs(*[lhs32[slot, k, j] for j in range(4)]), bf(rhs32[n // 2, k])))
                if k == 1:
                    sink(b + 1, n, m[1] - m[3])
                elif k == 0:
                    c11, c22 = m[3] - m[0], m[1] - m[0]
                elif k == 6:
                    c11 = m[6] - c11
                elif k == 5:
                    c22 = m[5] - c22
                elif k == 4:
                    sink(b, n, c11 - m[4])
                elif k == 2:
                    sink(b, n + 1, m[4] - m[2])
                    sink(b + 1, n + 1, c22 - m[2])
                yield

    def qkv_sink(b, n, o):
        c, t = divmod(b, 8)
        dst = (qbuf, kbuf, vbuf)[n // NT]
        for lb in range(4):
            put(dst.at[n % NT, t, pl.ds(8 + 64 * lb + 16 * c, 16), :], o[lb * 16:(lb + 1) * 16])
        if b == 0 and n >= NT:
            first = jnp.broadcast_to(o[0:1], (8, 128))
            for tt in range(8):
                dst[n % NT, tt, pl.ds(0, 8), :] = first

    def out_rows(r, i, last):
        c, t = divmod(r, 8)
        return (c * 8 + t % 2 * 4 + i, t // 2) if last and c == 0 else (r, i)

    def out_sink(last, r, n, o):
        for i in range(4):
            b, lb = out_rows(r, i, last)
            put(xres.at[b, n, r16(lb), :], xres[b, n, r16(lb), :] + o[i * 16:(i + 1) * 16])

    def attention(b, lb, h):
        c, t = divmod(b, 8)
        log2e = float(np.log2(np.e))
        scale = HEAD_DIM ** -0.5 * log2e
        r0 = 8 + 64 * lb + 16 * c + 8 * h
        src = [((t - 2 * w) % 8, -((t - 2 * w) // 8)) for w in range(WIN)]
        acc = [None] * WIN
        for j in range(NT):
            if j % 2 == 0:
                factor = gate(jnp.full((8, 128), scale, F32), ALAG)
            q = qbuf[j, t, pl.ds(r0, 8), :] * factor
            for w, (ts, sh) in enumerate(src):
                p = q * kbuf[j, ts, pl.ds(r0 - sh, 8), :]
                acc[w] = p if j == 0 else acc[w] + p
            if j % 2 and j < NT - 1:
                pin(*acc[j // 2 % 2::2])
                yield
        part = [(r, pltpu.roll(r, 64, 1)) for r in acc]
        yield from _latency()
        part = [r + rr for r, rr in part]
        part = [(r, pltpu.roll(r, 32, 1)) for r in part]
        yield from _latency()
        logits = [r + rr for r, rr in part]
        if r0 == 8:
            sub = lax.broadcasted_iota(jnp.int32, (8, 128), 0)
            logits = [jnp.where(sub >= sh, r, -1e9 * log2e) if sh else r
                      for r, (_, sh) in zip(logits, src)]
        logits[0] = gate(logits[0], ALAG)
        m = _tree(jnp.maximum, logits)
        ps = [jnp.exp2(r - m) for r in logits]
        total = _tree(_add, ps)
        pin(total)
        inv = pltpu.reciprocal(total, approx=True)
        inv = inv * (2.0 - total * inv)
        for j in range(NT):
            if j % 2 == 0:
                yield
                ps[0], ps[4] = gate(ps[0], ALAG), gate(ps[4], ALAG)
            o = _chain(_add, [ps[w] * vbuf[j, ts, pl.ds(r0 - sh, 8), :]
                              for w, (ts, sh) in enumerate(src)]) * inv
            if j % 2:
                pin(o)
            put(qbuf.at[j, t, pl.ds(r0, 8), :], o)

    def out_operands(r, i, last):
        for j in range(4):
            a = [qbuf[j + o, b % 8, pl.ds(8 + 64 * lb + 16 * (b // 8), 16), :]
                 for b, lb in (out_rows(r, i, last), out_rows(r + 1, i, last)) for o in (0, 4)]
            a[0], a[3] = gate(a[0]), gate(a[3])
            for k, v in enumerate(_strassen_lhs(*a)):
                if k in (1, 4):
                    pin(v)
                obuf[r // 2, k, j, r16(i), :] = v.astype(BF16)
            if j < 3:
                yield

    def store_rows(b, lb, tiles):
        c, t = divmod(b, 8)
        for j in tiles:
            words = pack(xres[b, j, r16(lb), :], xres[b + 1, j, r16(lb), :])
            pin(words)
            io32[j, lb, c, pl.ds(t // 2, 16, stride=4), :] = words

    unit_ticks = NT + 2 * XGAP
    step = 2
    out_ticks = 28

    def add_proj(sched, tick, c, lo, hi):
        jobs = [(b // step, b, n) for b in range(8 * c, 8 * c + 8, step) for n in range(lo, hi, step)]
        sched.add(tick, gemm(abuf32, wqkv32, jobs, qkv_sink))
        return tick + len(jobs) * out_ticks * step // NT

    def add_attention(sched, tick, pace, rows, last):
        units = [(r, i, half, h) for r in rows[::2] for i in range(4) for half in range(2) for h in range(2)]
        for n, (r, i, half, h) in enumerate(units):
            sched.add(tick + n * pace, attention(*out_rows(r + half, i, last), h))
            if half and h:
                sched.add(int(tick + n * pace) + unit_ticks, out_operands(r, i, last))

    def add_out(sched, tick, rows, last):
        jobs = [(r // 2, r, n) for r in rows[::2] for n in range(0, NT, 2)]
        sched.add(tick, gemm(obuf32, wo32, jobs, functools.partial(out_sink, last)))

    def add_tail(sched, tick, rows, last):
        ready = {}
        for i, r in enumerate(rows):
            t0 = tick + (i // 2 + 1) * out_ticks
            fast = i >= len(rows) - 2
            if not last:
                t0 += 0 if fast else TOFF + i % 2 * out_ticks // 2
                ready[r % 8] = add_d_fwd(sched, t0, r, i % 2 if fast else out_ticks / 8)
            elif r % 2:
                c, p = r // 8, r % 8 // 2
                if fast:
                    for at, tiles in ((t0 - out_ticks // 4 + 3, range(6)), (t0, range(6, NT))):
                        for j in range(4):
                            sched.add(at, _once(store_rows, 2 * j, p, tiles))
                        sched.add(at + 1, _once(start, out_copies(c, p, tiles)))
                    continue
                for j in range(4):
                    sched.add(t0 + 3 * j + 3, _once(store_rows, *((r - 1, j) if c else (2 * j, p)), range(NT)))
                for lb in ([p] if c == 0 else range(4) if p == 3 else []):
                    sched.add(t0 + 16, _once(start, out_copies(c, lb, range(NT))))
        return ready

    q_ticks = 8 * out_ticks // step
    att_ticks = unit_ticks + 1 + 2
    order = [(a + 8) % NB for a in range(NB)]

    def add_attention_block(sched, cols, last):
        stats = {}
        t0 = max([add_d_inv(sched, 0, b, 0, stats, not last, cols) for b in range(step)])
        if not last:
            sched.add(cols[3] - KLEAD, _once(wait, qkv_copies(1) + dmat_cp))
            done = add_prep_wqkv(sched, cols[3] - KLEAD, 1, KPACE, [7] * 4)
            t0 = max(t0, done[0])
            assert all(d <= t0 + p * out_ticks / 4 for p, d in enumerate(done))
            sched.add(t0 + out_ticks, _once(wait, qkv_copies(2)))
            sched.add(t0 + out_ticks, _once(start, qkv_copies(0)))
            done = add_prep_wqkv(sched, t0 + out_ticks, 2, 2 * out_ticks - 4, [out_ticks - 4] * 4)
            assert all(d <= t0 + q_ticks + p * out_ticks for p, d in enumerate(done))
            sched.add(t0 + 2 * q_ticks, _once(wait, qkv_copies(0)))
            sched.add(t0 + 2 * q_ticks, _once(start, wo_copies))
            done = add_prep_wqkv(sched, t0 + 2 * q_ticks, 0, q_ticks - 10, [q_ticks / 4] * 4)
            assert done[-1] <= t0 + 4 * q_ticks
            sched.add(t0 + 8 * q_ticks, _once(wait, wo_copies))
            for i in range(32):
                sched.add(t0 + 8 * q_ticks + i * q_ticks / 16, prep_wo(*divmod(i, 8)))
        tick, kv_start, q_start = t0, {}, {}
        for kind, c in ("k0", "k1", "q1", "k2", "q2", "k3", "q3", "q0"):
            if kind == "k":
                kv_start[int(c)] = tick
                if c == "0" and not last:
                    tick = add_proj(sched, tick, 0, NT, 2 * NT)
                    jobs = [(b // step, b, n) for n in range(2 * NT, 3 * NT, step) for b in range(0, 8, step)]
                    sched.add(tick, gemm(abuf32, wqkv32, jobs, qkv_sink))
                    tick += q_ticks
                    continue
                tick = add_proj(sched, tick, int(c), NT, 3 * NT)
            else:
                q_start[int(c)] = tick
                tick = add_proj(sched, tick, int(c), 0, NT)
        pace = 2 * out_ticks / step
        for b in range(step, NB):
            due = kv_start[b // 8] + (b % 8 // step) * (2 if last or b >= 8 else 1) * out_ticks
            gap = min(1 + (b - step) * 0.5, DGAP1 if last else DGAP0)
            pace = DPACE1 if last else DPACE0
            at = (b - step) * pace
            at = t0 + at + max(0, at - 4 * q_ticks - out_ticks) * DSLOW
            if not last and b < 8:
                at, gap = max(cols[3], t0 + (b // step - 1) * out_ticks - (step - b % step) * 8), 1
            end = add_d_inv(sched, at, b, gap, stats, not last)
            assert end <= due, (b, end, due)
        begin = [q_start[c] + out_ticks + 3 for c in (1, 2, 3)] + [tick + (ATT1 if last else ATT0)]
        begin.append(tick + (NB // step - 1) * out_ticks - att_ticks)
        for i, c in enumerate((1, 2, 3, 0)):
            pace = (begin[i + 1] - begin[i]) / 64
            assert begin[i] >= max(kv_start[c], kv_start[(c - 1) % 4]) + 2 * q_ticks
            for p in range(4):
                assert begin[i] + 16 * p * pace >= q_start[c] + (4 if last and c == 0 else p + 1) * out_ticks
                assert begin[i] + (16 * p + 15) * pace + att_ticks <= tick + (4 * i + p) * out_ticks + 1e-6
            add_attention(sched, begin[i], pace, range(8 * c, 8 * c + 8), last)
        add_out(sched, tick, order, last)
        return tick + (NB // step) * out_ticks, add_tail(sched, tick, order, last)

    def add_input(sched):
        ready = {}
        after = (x_copies(3), perm_cp + w_copies(0) + w_copies(1), w_copies(2) + w_copies(3), w_copies(4))
        for c in range(NC):
            sched.add(c * 32, _once(wait, x_copies(c)))
            sched.add(c * 32, _once(start, after[c]))
            for t in range(8):
                ready[t] = add_d_fwd(sched, c * 32 + t * 4, c * 8 + t, 1, 2, True)
        return 128 + 9, ready

    def add_filter_prep(sched, upper, begin, end):
        after = (([], qkv_copies(2)) if upper else
                 (w_copies(5) + w_copies(6), w_copies(7) + f256_cp + dmat_cp))
        for i in range(16):
            g, at = 4 * upper + i // 4, begin + i * (end - begin) / 16
            if i % 8 == 0:
                sched.add(at, _once(wait, w_copies(g) + w_copies(g + 1) + {0: perm_cp, 6: f256_cp}.get(g, [])))
                sched.add(at, _once(start, after[i // 8]))
            sched.add(at, _once(prep_filter, *w_tiles(g)[i % 4]))
        return end + 2

    def add_first_s_stage(sched):
        tick, ready = add_input(sched)
        sched.add(tick + WK0, _once(start, qkv_copies(1)))
        return add_s_stage(sched, tick, ready, add_filter_prep(sched, 0, F0, tick),
                           lambda begin, end: add_filter_prep(sched, 1, begin, end + FG))

    sched = _Schedule()

    start(x_copies(0) + tiny_cp)
    for ref in (abuf32, obuf32, ubuf32, wo32, sfw32, siv32, wide32):
        put(ref.at[(0,) * (len(ref.shape) - 2) + (pl.ds(0, 8),)], jnp.zeros((8, 128), U32))
    make_wide()
    start(x_copies(1))
    make_s_fwd()
    start(x_copies(2))
    make_s_inv()
    wait(tiny_cp)
    for n in (1, 2, 4):
        never[n] = jnp.concatenate([tw_ref[16:24, 0:128]] * n, axis=1) != 0.0
    cols = add_first_s_stage(sched)
    tick, ready = add_attention_block(sched, cols, False)
    cols = add_s_stage(sched, tick, ready, tick, None)
    add_attention_block(sched, cols, True)
    sched.run()
    for c in range(NC):
        for lb in range(4):
            wait(out_copies(c, lb, range(NT)))


@jax.jit
def pallas_interleave_layers__spectral_gfnet__sliding_local_dilated__prompt_kernel(
    A_x: jax.Array,
    A_w_r: jax.Array,
    A_w_i: jax.Array,
    B_x: jax.Array,
    B_wqkv: jax.Array,
    B_wo: jax.Array,
):
    del B_x
    assert A_x.shape == (1, S, D) and A_w_r.shape == (S, D // 2 + 1)
    cst = _constants()
    x = A_x.astype(BF16).reshape(4, NC, 128, D)
    wr, wi = A_w_r.astype(BF16).T, A_w_i.astype(BF16).T
    hbm = pl.BlockSpec(memory_space=pl.ANY)
    vm = pltpu.VMEM
    out = pl.pallas_call(
        _kernel,
        in_specs=[hbm] * 9,
        out_specs=hbm,
        out_shape=jax.ShapeDtypeStruct((4, NC, 128, D), BF16),
        scratch_shapes=[
            vm((NT, 4, NC, 128, 128), BF16),
            vm((17, 128, 128), BF16),
            vm((32, 128, 128), BF16),
            vm((32, 128, 128), BF16),
            vm((256, 512), BF16),
            vm((2, 16, 512, 128), BF16),
            vm((2, 4, 4, 8, 64, 128), F32),
            vm((3 * NT, D, 128), BF16),
            vm((NT, D // 2, 128), U32),
            vm((12, 7, 512, 128), BF16),
            vm((NT, D, 128), BF16),
            vm((4, 7, 512, 128), BF16),
            vm((NB, NT, 64, 128), F32),
            vm((4, 32, 64, 128), U32),
            vm((4, 32, 128, 128), F32),
            vm((RING, 8, 64, 128), BF16),
            vm((RING, 9, 64, 128), F32),
            vm((NB // 2, 7, 4, 64, 128), BF16),
            vm((NB // 2, 7, 4, 64, 128), BF16),
            vm((NT, 8, 264, 128), F32),
            vm((NT, 8, 264, 128), F32),
            vm((NT, 8, 264, 128), F32),
            vm((3, 256, 128), F32),
            vm((8, 256, 128), BF16),
            vm((24, 256), F32),
            vm((2, 16, 128), BF16),
            vm((1, S), BF16),
            vm((1, S), BF16),
            pltpu.SemaphoreType.DMA((NC,)),
            pltpu.SemaphoreType.DMA((4,)),
            pltpu.SemaphoreType.DMA((8,)),
            pltpu.SemaphoreType.DMA((3,)),
            pltpu.SemaphoreType.DMA(()),
            pltpu.SemaphoreType.DMA(()),
        ],
        compiler_params=pltpu.CompilerParams(
            vmem_limit_bytes=120 * 2**20),
    )(x, wr, wi, B_wqkv.astype(BF16), B_wo.astype(BF16),
      cst["small"], cst["f256"], cst["tw"], cst["d8"])
    return out.reshape(1, S, D)
```
